```python
import jax
import jax.numpy as jnp

def _softmax(x, axis=-1):
    return jax.nn.softmax(x, axis=axis)
def _gelu(x):
    return jax.nn.gelu(x, approximate=True)
def _silu(x):
    return jax.nn.silu(x)
def _sigmoid(x):
    return jax.nn.sigmoid(x)
def _layernorm(x, axis=-1, eps=1e-5):
    m = jnp.mean(x, axis=axis, keepdims=True)
    v = jnp.var(x, axis=axis, keepdims=True)
    return (x - m) / jnp.sqrt(v + eps)
def _scatter_add(tgt, idx, src, axis=0):
    return tgt.at[idx].add(src)
def _segment_sum(src, seg, n):
    return jax.ops.segment_sum(src, seg, n)
class _Rng:
    def __init__(self, key):
        self._k = key
    def _next(self):
        self._k, sub = jax.random.split(self._k)
        return sub
    def normal(self, shape):
        return jax.random.normal(self._next(), shape, dtype=jnp.bfloat16)
    def randint(self, lo, hi, shape):
        return jax.random.randint(self._next(), shape, lo, hi, dtype=jnp.int32)
    def uniform(self, shape, lo=0.0, hi=1.0):
        return jax.random.uniform(self._next(), shape, jnp.bfloat16, lo, hi)
    def permutation(self, n):
        return jax.random.permutation(self._next(), n)


kernel_name = 'sequential_preLN__ssm_conv_s4__moe_arch_mod__prompt'

def setup_inputs():
    _rng = _Rng(jax.random.key(int.from_bytes(__import__("os").urandom(4), "little")))
    _w = (lambda a: (lambda t: t.astype(jnp.bfloat16) if jnp.issubdtype(t.dtype, jnp.floating) else t)(jnp.asarray(a)))
    def _A_setup():
        B, L, D, N = 1, 2048, 576, 128
        A_re = -jnp.exp((lambda *s: _rng.normal(s) * 0.05)(D, N))
        A_im = jnp.pi * (lambda *s: _rng.normal(s) * 0.05)(D, N)
        B_re = (lambda *s: _rng.normal(s) * 0.05)(D, N)
        B_im = (lambda *s: _rng.normal(s) * 0.05)(D, N)
        C_re = (lambda *s: _rng.normal(s) * 0.05)(D, N)
        C_im = (lambda *s: _rng.normal(s) * 0.05)(D, N)
        log_dt = (lambda *s: _rng.normal(s) * 0.05)(D) * 0.5 - 4.0
        Dskip = (lambda *s: _rng.normal(s) * 0.05)(D)
        return {
            "u": _w((lambda *s: _rng.normal(s) * 0.05)(B, L, D)),
            "A_re": _w(A_re),
            "A_im": _w(A_im),
            "B_re": _w(B_re),
            "B_im": _w(B_im),
            "C_re": _w(C_re),
            "C_im": _w(C_im),
            "log_dt": _w(log_dt),
            "Dskip": _w(Dskip),
        }
    _A_in = _A_setup()

    def _B_setup():
        B, S, D, F, C = 1, 2048, 576, 4608, 8
        return {
            "x": _w((lambda *s: _rng.normal(s) * 0.05)(B, S, D)),
            "w_r": _w((lambda *s: _rng.normal(s) * 0.05)(D)),
            "w_gate": _w((lambda *s: _rng.normal(s) * 0.05)(D, F)),
            "w_up": _w((lambda *s: _rng.normal(s) * 0.05)(D, F)),
            "w_down": _w((lambda *s: _rng.normal(s) * 0.05)(F, D)),
        }
    _B_in = _B_setup()

    return {
        "A_u": _A_in["u"],
        "A_A_re": _A_in["A_re"],
        "A_A_im": _A_in["A_im"],
        "A_B_re": _A_in["B_re"],
        "A_B_im": _A_in["B_im"],
        "A_C_re": _A_in["C_re"],
        "A_C_im": _A_in["C_im"],
        "A_log_dt": _A_in["log_dt"],
        "A_Dskip": _A_in["Dskip"],
        "B_x": _B_in["x"],
        "B_w_r": _B_in["w_r"],
        "B_w_gate": _B_in["w_gate"],
        "B_w_up": _B_in["w_up"],
        "B_w_down": _B_in["w_down"],
    }

def reference(A_u, A_A_re, A_A_im, A_B_re, A_B_im, A_C_re, A_C_im, A_log_dt, A_Dskip, B_x, B_w_r, B_w_gate, B_w_up, B_w_down):
    def _A_ref(u, A_re, A_im, B_re, B_im, C_re, C_im, log_dt, Dskip):
        Bsz, L, D = u.shape
        dt = jnp.exp(log_dt)[:, None]
        A = A_re + 1j * A_im
        Bc = B_re + 1j * B_im
        Cc = C_re + 1j * C_im
        logdA = dt * A
        dB = dt * Bc
        l = (lambda x, dt: x.astype(dt))(jnp.arange(L), A_re.dtype)
        P = jnp.exp(logdA[:, :, None] * l[None, None, :])
        K = jnp.einsum("dn,dnl,dn->dl", Cc, P, dB).real
        L2 = 2 * L
        Kp = jnp.pad(K, ((0, 0), (0, L)))
        up = (lambda x, *d: x.transpose(*d))(u, 0, 2, 1)
        up = jnp.pad(up, ((0, 0), (0, 0), (0, L)))
        Kf = (lambda x, axes=(-2,-1): jnp.fft.rfft2(x.astype(jnp.float32), axes=axes))(Kp[:, None, :], axes=(-2, -1))
        Uf = (lambda x, axes=(-2,-1): jnp.fft.rfft2(x.astype(jnp.float32), axes=axes))(up[:, :, None, :], axes=(-2, -1))
        Yf = Uf * Kf[None, :, :, :]
        y = (lambda x, s, axes=(-2,-1): jnp.fft.irfft2(x, s=s, axes=axes).astype(jnp.bfloat16))(Yf, (1, L2), axes=(-2, -1))[:, :, 0, :L]
        y = (lambda x, *d: x.transpose(*d))(y, 0, 2, 1) + u * Dskip[None, None, :]
        return y

    def _B_ref(x, w_r, w_gate, w_up, w_down):
        B, S, D = x.shape
        C = 8
        r = x @ w_r
        idx = jnp.argsort(-r, axis=-1)[:, :C]
        idx_e = jnp.repeat(idx.reshape(B, C, 1), D, axis=2)
        x_sel = jnp.take_along_axis(x, idx_e, axis=1)
        g = _silu(x_sel @ w_gate)
        u = x_sel @ w_up
        y = (g * u) @ w_down
        r_sel = _sigmoid(jnp.take_along_axis(r, idx, axis=1))
        y = y * r_sel.reshape(B, C, 1)
        b_off = (jnp.arange(B) * S).reshape(B, 1)
        flat_idx = (idx + b_off).reshape(B * C)
        zero = (x * 0.0).reshape(B * S, D)
        upd = _scatter_add(zero, flat_idx, y.reshape(B * C, D), axis=0)
        return x + upd.reshape(B, S, D)

    x = A_u
    h = x + _A_ref(_layernorm(x, axis=-1), A_A_re, A_A_im, A_B_re, A_B_im, A_C_re, A_C_im, A_log_dt, A_Dskip)
    h2 = h + _B_ref(_layernorm(h, axis=-1), B_w_r, B_w_gate, B_w_up, B_w_down)
    return h2
```

```python
import functools

import numpy as np
import jax
import jax.numpy as jnp
import jax.experimental.pallas as pl
import jax.experimental.pallas.tpu as pltpu

F32 = jnp.float32
BF16 = jnp.bfloat16
I32 = jnp.int32

L = 2048
D = 576
N = 128
FF = 4608
CAP = 8
NT = L // 128
EPS = 1e-5
MB = 64
NT_DIMS = (((1,), (1,)), ((), ()))


def _round_res(step):
    return [int(np.round(r / step)) * step for r in range(16)]


RES1, RES2, RES3 = _round_res(2), _round_res(4), _round_res(8)


def _iota(shape, dim):
    return jax.lax.broadcasted_iota(I32, shape, dim)


def _rbf(x):
    return x.astype(BF16).astype(F32)


def _cmul(a, b):
    return (a[0] * b[0] - a[1] * b[1], a[0] * b[1] + a[1] * b[0])


def _csq(a):
    t = a[0] * a[1]
    return ((a[0] + a[1]) * (a[0] - a[1]), t + t)


def _cadd(a, b):
    return (a[0] + b[0], a[1] + b[1])


def _csub(a, b):
    return (a[0] - b[0], a[1] - b[1])


def _bfly4(a0, a1, a2, a3, inverse=False):
    s02, d02 = _cadd(a0, a2), _csub(a0, a2)
    s13, d13 = _cadd(a1, a3), _csub(a1, a3)
    p = (d02[0] - d13[1], d02[1] + d13[0])
    m = (d02[0] + d13[1], d02[1] - d13[0])
    if inverse:
        p, m = m, p
    return _cadd(s02, s13), p, _csub(s02, s13), m


def _prod_mod_1(a, b):
    fa, fb = _bfly4(*a), _bfly4(*b)
    return _bfly4(*[_cmul(x, y) for x, y in zip(fa, fb)], inverse=True)


def _prod2(a0, a1, b0, b1, sgn):
    p00, p11 = _cmul(a0, b0), _cmul(a1, b1)
    c1 = _cadd(_cmul(a0, b1), _cmul(a1, b0))
    if sgn > 0:
        return (p00[0] - p11[1], p00[1] + p11[0]), c1
    return (p00[0] + p11[1], p00[1] - p11[0]), c1


def _prod_mod_m1(a, b):
    def split(x):
        p = [(x[k][0] - x[k + 2][1], x[k][1] + x[k + 2][0]) for k in range(2)]
        m = [(x[k][0] + x[k + 2][1], x[k][1] - x[k + 2][0]) for k in range(2)]
        return p, m
    ap, am = split(a)
    bp, bm = split(b)
    cp = _prod2(*ap, *bp, 1)
    cm = _prod2(*am, *bm, -1)
    lo = [_cadd(cp[k], cm[k]) for k in range(2)]
    hi = [(cp[k][1] - cm[k][1], cm[k][0] - cp[k][0]) for k in range(2)]
    return lo + hi


def _prod_mod_i(a, b, sgn):
    sm = [x[0] + x[1] for x in b]
    df = [x[1] - x[0] for x in b]
    asum = [x[0] + x[1] for x in a]
    out = []
    for k in range(4):
        acc = [None, None, None]
        for j in range(4):
            m = (k - j) % 4
            if j <= k:
                t = ((b[m][0], 1), (df[m], 1), (sm[m], 1))
            elif sgn > 0:
                t = ((b[m][1], -1), (sm[m], 1), (df[m], -1))
            else:
                t = ((b[m][1], 1), (sm[m], -1), (df[m], 1))
            for q, (v, (w, s)) in enumerate(zip((asum[j], a[j][0], a[j][1]), t)):
                p = v * w
                if acc[q] is None:
                    acc[q] = p
                else:
                    acc[q] = acc[q] + p if s > 0 else acc[q] - p
        out.append((acc[0] - acc[2], acc[0] + acc[1]))
    return out


def _cyclic16(a, b):
    fa = [_bfly4(*a[k::4]) for k in range(4)]
    fb = [_bfly4(*b[k::4]) for k in range(4)]

    def br(f, q, scale=None):
        v = [f[k][q] for k in range(4)]
        return v if scale is None else [(x[0] * scale, x[1] * scale) for x in v]

    c = [_prod_mod_1(br(fa, 0), br(fb, 0)),
         _prod_mod_i(br(fa, 1), br(fb, 1, 4.0), 1),
         _prod_mod_m1(br(fa, 2), br(fb, 2, 2.0)),
         _prod_mod_i(br(fa, 3), br(fb, 3, 4.0), -1)]
    out = [None] * 16
    for k in range(4):
        e = _bfly4(*[c[q][k] for q in range(4)], inverse=True)
        for j in range(4):
            out[k + 4 * j] = e[j]
    return out


def _barrel(v, lane, sign):
    for bit in range(4):
        m = ((lane >> bit) & 1) == 1
        v = [jnp.where(m, v[(i + (1 << bit)) % 16], v[i]) for i in range(16)]
    return [v[(sign * s) % 16] for s in range(16)]


def _lane_t1(lane):
    return 32 * (lane & 3) + (lane >> 2)


def _to_residues(tiles):
    lane = _iota((8, 128), 1)
    v = [t if j == 0 else pltpu.roll(t, j, 1) for j, t in enumerate(tiles)]
    v = _barrel(v, lane, -1)
    t1 = _lane_t1(lane)
    src = 16 * (t1 & 7) + (t1 >> 3)
    return [jnp.take_along_axis(v[s], (src + s) & 127, axis=1) for s in range(16)]


def _to_time(res):
    lane = _iota((8, 128), 1)
    v = []
    for s in range(16):
        mu = (lane - s) & 127
        t1 = 8 * (mu & 15) + (mu >> 4)
        v.append(jnp.take_along_axis(res[s], 4 * (t1 & 31) + (t1 >> 5), axis=1))
    v = _barrel(v, lane, -1)
    return [t if j == 0 else pltpu.roll(t, 128 - j, 1) for j, t in enumerate(v)]


def _k_residues(z, c):
    sub = _iota((8, 128), 0)
    lane = _iota((8, 128), 1)
    lo = sub < 4
    zr = tuple(pltpu.roll(x, 4, 0) for x in z)
    cr = tuple(pltpu.roll(x, 4, 0) for x in c)
    prods, tail = [], []
    for g in range(2):
        def mix(nat, rot):
            a, b = (nat, rot) if g == 0 else (rot, nat)
            return tuple(jnp.where(lo, p, q) for p, q in zip(a, b))
        pw = {1: mix(z, zr)}
        for e in range(1, 10):
            pw[1 << e] = _csq(pw[1 << (e - 1)])
        first = lo if g == 0 else jnp.logical_not(lo)
        fa = {0: _cmul(mix(c, cr), (jnp.where(first, 1.0, pw[8][0]),
                                    jnp.where(first, 0.0, pw[8][1])))}
        for r in range(1, 8):
            h = 1 << (r.bit_length() - 1)
            fa[r] = _cmul(fa[r - h], pw[h])
        fa[512] = _cmul(fa[0], pw[512])
        fa[516] = _cmul(fa[4], pw[512])
        fa[1024] = _cmul(fa[512], pw[512])
        fa[1536] = _cmul(fa[1024], pw[512])
        tail.append(fa[1536][0] * pw[512][0] - fa[1536][1] * pw[512][1])
        cj = {k: (pw[k][0], -pw[k][1]) for k in (32, 64, 128, 256)}
        fb = [(jnp.where(lo, 1.0, pw[16][0]), jnp.where(lo, 0.0, -pw[16][1]))]
        for m in range(1, 16):
            h = 1 << (m.bit_length() - 1)
            fb.append(_cmul(fb[m - h], cj[32 * h]))
        keys = list(fa)
        lhs = jnp.concatenate(
            [jnp.concatenate([fa[k][p] for k in keys], axis=0).astype(BF16) for p in range(2)],
            axis=1)
        rhs = jnp.concatenate(
            [jnp.concatenate([x[p] for x in fb], axis=0).astype(BF16) for p in range(2)],
            axis=1)
        res = jax.lax.dot_general(lhs, rhs, NT_DIMS, preferred_element_type=F32)
        prods.append({k: res[8 * i:8 * i + 8] for i, k in enumerate(keys)})
    idx = (lane & ~3) | (sub & 3)
    kv = {}
    for k in prods[0]:
        kv[k] = jnp.take_along_axis(jnp.where(lo, prods[0][k], prods[1][k]), idx, axis=1)
        odd = pltpu.roll(jnp.where(lo, prods[1][k], prods[0][k]), 4, 0)
        kv[k + 8] = jnp.take_along_axis(odd, idx, axis=1)
    k_last = jnp.sum(jnp.where(lo, tail[0], tail[1]), axis=1, keepdims=True)
    q = lane & 3
    s3 = {r: jnp.where(q == 2, kv[1024 + r], kv[1536 + r]) for r in (0, 8)}
    v0 = jnp.where(q == 0, kv[0], jnp.where(q == 1, kv[512], s3[0]))
    nxt = jnp.where(lane < 124, lane + 4, (lane - 123) & 127)
    v16 = jnp.where(lane == 127, k_last, jnp.take_along_axis(v0, nxt, axis=1))
    s3[16] = v16
    s23, s123, out = {}, {}, [v0]
    for r in range(1, 16):
        k23 = (RES2[r], RES3[r])
        if k23 not in s23:
            s23[k23] = v16 if k23 == (16, 16) else jnp.where(q == 1, kv[512 + k23[0]], s3[k23[1]])
        k123 = (RES1[r],) + k23
        if k123 not in s123:
            s123[k123] = v16 if k123[0] == 16 else jnp.where(q == 0, kv[k123[0]], s23[k23])
        if RES1[r] == r:
            out.append(s123[k123])
        else:
            out.append(jnp.where((q == 0) & (lane < 64), kv[r], s123[k123]))
    return out


def _ln_scalars(s1, s2):
    mean = s1 * (1.0 / D)
    var = jnp.maximum(s2 * (1.0 / D) - mean * mean, 0.0)
    eps = float(np.asarray(EPS, dtype=BF16))
    sd = _rbf(jnp.sqrt(_rbf(_rbf(var) + eps)))
    return _rbf(mean), 1.0 / sd


def _column(vec):
    row = vec.astype(F32).reshape(1, D)
    parts = []
    for lo in range(0, D, 128):
        start = min(lo, D - 128)
        t = jnp.broadcast_to(row[:, start:start + 128], (128, 128)).T
        parts.append(t[lo - start:])
    return jnp.concatenate(parts, axis=0)


def _kernel(x_hbm, are_ref, aim_ref, bre_ref, bim_ref, cre_ref, cim_ref,
            ldt_ref, dsk_ref, wr_ref, wg_hbm, wu_hbm, wd_hbm, out_hbm,
            x_v, wg_v, wu_v, wd_v, w_v, wt_v, col_v, uk_v, u_v, ab_v, e_v, y_v, h_v,
            st_v, acc_v, out_v, sem):
    cp_x = pltpu.make_async_copy(x_hbm, x_v, sem.at[0])
    cp_g = pltpu.make_async_copy(wg_hbm, wg_v, sem.at[1])
    cp_u = pltpu.make_async_copy(wu_hbm, wu_v, sem.at[2])
    cp_d = pltpu.make_async_copy(wd_hbm, wd_v, sem.at[3])
    cp_x.start()
    cp_g.start()
    cp_u.start()
    cp_d.start()

    k4 = 4 * _iota((128, 128), 1) + 1
    ph = ((k4 * _lane_t1(_iota((128, 128), 0))) & 511).astype(F32) * (2 * np.pi / 512)
    w = (jnp.cos(ph), jnp.sin(ph))
    ph1 = (4 * _iota((8, 128), 1) + 1).astype(F32) * (2 * np.pi / (4 * L))
    tw = (jnp.tile(jnp.cos(ph1), (16, 1)), jnp.tile(jnp.sin(ph1), (16, 1)))
    for s in range(16):
        wr, wi = w[0].astype(BF16), w[1].astype(BF16)
        w_v[s, :, 0:128] = wr
        w_v[s, :, 128:256] = wi
        wt_v[s, 0:128, :] = wr.T
        wt_v[s, 128:256, :] = wi.T
        if s < 15:
            w = _cmul(w, tw)

    col_v[0] = _rbf(jnp.exp(_column(ldt_ref[...])))
    col_v[1] = _column(dsk_ref[...])
    col_v[2] = _column(wr_ref[...])

    def k_step(i, carry):
        blk = i // (MB // 16)
        r0 = pl.multiple_of((i % (MB // 16)) * 16, 16)
        rows = pl.ds(pl.multiple_of(i * 16, 16), 16)
        dt = col_v[0, rows, :]
        mag = jnp.exp(dt * are_ref[rows, :].astype(F32))
        ang = dt * aim_ref[rows, :].astype(F32)
        z = (mag * jnp.cos(ang), mag * jnp.sin(ang))
        sc = dt * (1.0 / L)
        c = _cmul((cre_ref[rows, :].astype(F32), cim_ref[rows, :].astype(F32)),
                  (sc * bre_ref[rows, :].astype(F32), sc * bim_ref[rows, :].astype(F32)))
        halves = [_k_residues(tuple(p[8 * h:8 * h + 8] for p in z),
                              tuple(p[8 * h:8 * h + 8] for p in c)) for h in range(2)]
        for s in range(16):
            uk_v[blk, s, pl.ds(MB + r0, 16), :] = jnp.concatenate(
                [halves[0][s], halves[1][s]], axis=0).astype(BF16)
        return carry

    jax.lax.fori_loop(0, D // 16, k_step, 0)

    cp_x.wait()
    for j in range(NT):
        xs = x_v[:, 128 * j:128 * j + 128].astype(F32)
        m, inv = _ln_scalars(jnp.sum(xs, axis=0, keepdims=True),
                             jnp.sum(xs * xs, axis=0, keepdims=True))
        st_v[0, j] = jnp.broadcast_to(m, (8, 128))
        st_v[1, j] = jnp.broadcast_to(inv, (8, 128))
    acc_v[...] = jnp.zeros(acc_v.shape, F32)

    def conv_step(b, carry):
        base = pl.multiple_of(b * MB, MB)
        for r in range(MB // 16):
            rows = pl.ds(pl.multiple_of(base + 16 * r, 16), 16)
            tiles = []
            for j in range(NT):
                xs = x_v[rows, 128 * j:128 * j + 128].astype(F32)
                m, inv = st_v[0, j], st_v[1, j]
                u = jnp.concatenate([(xs[0:8] - m) * inv, (xs[8:16] - m) * inv],
                                    axis=0).astype(BF16)
                u_v[j, 16 * r:16 * r + 16, :] = u
                tiles.append(pltpu.bitcast(u, I32))
            for s, t in enumerate(_to_residues(tiles)):
                uk_v[b, s, 16 * r:16 * r + 16, :] = pltpu.bitcast(t, BF16)
        for s in range(16):
            ab_v[s] = jnp.dot(uk_v[b, s], w_v[s], preferred_element_type=F32)
        for r in range(MB // 16):
            halves = []
            for h in range(2):
                ra = pl.ds(16 * r + 8 * h, 8)
                rb = pl.ds(MB + 16 * r + 8 * h, 8)
                a = [(ab_v[s, ra, 0:128], ab_v[s, ra, 128:256]) for s in range(16)]
                k = [(ab_v[s, rb, 0:128], ab_v[s, rb, 128:256]) for s in range(16)]
                halves.append(_cyclic16(a, k))
            for s in range(16):
                for p in range(2):
                    e_v[s, 16 * r:16 * r + 16, 128 * p:128 * p + 128] = jnp.concatenate(
                        [halves[0][s][p], halves[1][s][p]], axis=0).astype(BF16)
        for s in range(16):
            y_v[s] = jnp.dot(e_v[s], wt_v[s], preferred_element_type=F32).astype(BF16)
        for r in range(MB // 16):
            rows = pl.ds(pl.multiple_of(base + 16 * r, 16), 16)
            dsk = col_v[1, rows, :]
            wr = col_v[2, rows, :]
            ys = _to_time([pltpu.bitcast(y_v[s, 16 * r:16 * r + 16, :], I32) for s in range(16)])
            for j in range(NT):
                y = pltpu.bitcast(ys[j], BF16).astype(F32)
                u = u_v[j, 16 * r:16 * r + 16, :].astype(F32)
                xs = x_v[rows, 128 * j:128 * j + 128].astype(F32)
                h = xs + (y + u * dsk)
                h_v[j, rows, :] = h
                hh, hw = h * h, h * wr
                acc_v[0, j] += h[0:8] + h[8:16]
                acc_v[1, j] += hh[0:8] + hh[8:16]
                acc_v[2, j] += hw[0:8] + hw[8:16]
        return carry

    jax.lax.fori_loop(0, D // MB, conv_step, 0)

    def rows_of(q):
        return jnp.concatenate(
            [jnp.sum(acc_v[q, j], axis=0, keepdims=True) for j in range(NT)], axis=0)

    m2, inv2 = _ln_scalars(rows_of(0), rows_of(1))
    wsum = jnp.sum(col_v[2], axis=0, keepdims=True)
    score = _rbf((rows_of(2) - m2 * wsum) * inv2 + 0.0)
    bits = pltpu.bitcast(score, I32) >> 16
    order = jnp.where(bits < 0, -1 - bits, bits + 32768)
    pos = 128 * _iota((NT, 128), 0) + _iota((NT, 128), 1)
    key = pltpu.bitcast((order << 11) + (L - 1 - pos) + (1 << 29), F32)

    lane = _iota((D, 128), 1)
    sel = jnp.zeros((D, 128), F32)
    aux = jnp.zeros((8, 128), F32)
    lane8, sub8 = _iota((8, 128), 1), _iota((8, 128), 0)
    picks = []
    for c in range(CAP):
        top = jnp.max(key, axis=(0, 1), keepdims=True)
        hit = key == top
        key = jnp.where(hit, 0.0, key)
        t = jnp.max(jnp.where(hit, pos, 0))
        j, i = jnp.clip(t >> 7, 0, NT - 1), t & 127
        picks.append((j, i))
        sel = jnp.where(lane == c, pltpu.roll(h_v[j], (128 + c - i) & 127, 1), sel)
        for q, v in enumerate((m2, inv2, score)):
            val = jnp.sum(jnp.where(hit, v, 0.0), axis=(0, 1), keepdims=True)
            aux = jnp.where((sub8 == c) & (lane8 == q), val, aux)
    h_sel = sel.T[0:CAP]
    x_sel = _rbf((h_sel - aux[:, 0:1]) * aux[:, 1:2])
    gate = _rbf(jax.nn.sigmoid(aux[:, 2:3]))

    for j in range(NT):
        h = h_v[j]
        out_v[:, 128 * j:128 * j + 128] = (
            h + (h - m2[j:j + 1]) * inv2[j:j + 1]).astype(BF16)

    xb = x_sel.astype(BF16)
    cp_g.wait()
    g = _rbf(jnp.dot(xb, wg_v[...], preferred_element_type=F32))
    cp_u.wait()
    up = _rbf(jnp.dot(xb, wu_v[...], preferred_element_type=F32))
    act = (_rbf(g * jax.nn.sigmoid(g)) * up).astype(BF16)
    cp_d.wait()
    y = _rbf(jax.lax.dot_general(act, wd_v[...], NT_DIMS, preferred_element_type=F32))
    new = h_sel + _rbf(x_sel + _rbf(y * gate))
    new = jnp.concatenate([new, jnp.zeros((128 - CAP, D), F32)], axis=0).T.astype(BF16)
    new = pltpu.bitcast(new, I32)
    lane_p = _iota((D // 2, 128), 1)
    for c, (j, i) in enumerate(picks):
        cols = pl.ds(pl.multiple_of(j * 128, 128), 128)
        old = pltpu.bitcast(out_v[:, cols], I32)
        upd = jnp.where(lane_p == i, pltpu.roll(new, (128 + i - c) & 127, 1), old)
        out_v[:, cols] = pltpu.bitcast(upd, BF16)
    cp_o = pltpu.make_async_copy(out_v, out_hbm, sem.at[4])
    cp_o.start()
    cp_o.wait()


@jax.jit
def pallas_sequential_preLN__ssm_conv_s4__moe_arch_mod__prompt_kernel(
    A_u: jax.Array,
    A_A_re: jax.Array,
    A_A_im: jax.Array,
    A_B_re: jax.Array,
    A_B_im: jax.Array,
    A_C_re: jax.Array,
    A_C_im: jax.Array,
    A_log_dt: jax.Array,
    A_Dskip: jax.Array,
    B_x: jax.Array,
    B_w_r: jax.Array,
    B_w_gate: jax.Array,
    B_w_up: jax.Array,
    B_w_down: jax.Array,
):
    del B_x
    hbm = pl.BlockSpec(memory_space=pl.ANY)
    vmem = pl.BlockSpec(memory_space=pltpu.VMEM)
    out = pl.pallas_call(
        _kernel,
        out_shape=jax.ShapeDtypeStruct((D, L), BF16),
        in_specs=[hbm] + [vmem] * 9 + [hbm] * 3,
        out_specs=hbm,
        scratch_shapes=[
            pltpu.VMEM((D, L), BF16),
            pltpu.VMEM((D, FF), BF16),
            pltpu.VMEM((D, FF), BF16),
            pltpu.VMEM((D, FF), BF16),
            pltpu.VMEM((16, 128, 256), BF16),
            pltpu.VMEM((16, 256, 128), BF16),
            pltpu.VMEM((3, D, 128), F32),
            pltpu.VMEM((D // MB, 16, 2 * MB, 128), BF16),
            pltpu.VMEM((NT, MB, 128), BF16),
            pltpu.VMEM((16, 2 * MB, 256), F32),
            pltpu.VMEM((16, MB, 256), BF16),
            pltpu.VMEM((16, MB, 128), BF16),
            pltpu.VMEM((NT, D, 128), F32),
            pltpu.VMEM((2, NT, 8, 128), F32),
            pltpu.VMEM((3, NT, 8, 128), F32),
            pltpu.VMEM((D, L), BF16),
            pltpu.SemaphoreType.DMA((5,)),
        ],
        compiler_params=pltpu.CompilerParams(vmem_limit_bytes=100 * 1024 * 1024),
    )(A_u.reshape(L, D).T, A_A_re, A_A_im, A_B_re, A_B_im, A_C_re, A_C_im,
      A_log_dt, A_Dskip, B_w_r, B_w_gate, B_w_up, B_w_down.T)
    return out.T.reshape(1, L, D)
```

```python
import functools

import numpy as np
import jax
import jax.numpy as jnp
import jax.experimental.pallas as pl
import jax.experimental.pallas.tpu as pltpu

F32 = jnp.float32
BF16 = jnp.bfloat16
I32 = jnp.int32

L = 2048
D = 576
N = 128
FF = 4608
CAP = 8
NT = L // 128
EPS = 1e-5
MB = 64
NT_DIMS = (((1,), (1,)), ((), ()))


def _round_res(step):
    return [int(np.round(r / step)) * step for r in range(16)]


RES1, RES2, RES3 = _round_res(2), _round_res(4), _round_res(8)


def _iota(shape, dim):
    return jax.lax.broadcasted_iota(I32, shape, dim)


def _rbf(x):
    return x.astype(BF16).astype(F32)


def _cmul(a, b):
    return (a[0] * b[0] - a[1] * b[1], a[0] * b[1] + a[1] * b[0])


def _csq(a):
    t = a[0] * a[1]
    return ((a[0] + a[1]) * (a[0] - a[1]), t + t)


def _cadd(a, b):
    return (a[0] + b[0], a[1] + b[1])


def _csub(a, b):
    return (a[0] - b[0], a[1] - b[1])


def _bfly4(a0, a1, a2, a3, inverse=False):
    s02, d02 = _cadd(a0, a2), _csub(a0, a2)
    s13, d13 = _cadd(a1, a3), _csub(a1, a3)
    p = (d02[0] - d13[1], d02[1] + d13[0])
    m = (d02[0] + d13[1], d02[1] - d13[0])
    if inverse:
        p, m = m, p
    return _cadd(s02, s13), p, _csub(s02, s13), m


def _prod_mod_1(a, b):
    fa, fb = _bfly4(*a), _bfly4(*b)
    return _bfly4(*[_cmul(x, y) for x, y in zip(fa, fb)], inverse=True)


def _prod2(a0, a1, b0, b1, sgn):
    p00, p11 = _cmul(a0, b0), _cmul(a1, b1)
    c1 = _cadd(_cmul(a0, b1), _cmul(a1, b0))
    if sgn > 0:
        return (p00[0] - p11[1], p00[1] + p11[0]), c1
    return (p00[0] + p11[1], p00[1] - p11[0]), c1


def _prod_mod_m1(a, b):
    def split(x):
        p = [(x[k][0] - x[k + 2][1], x[k][1] + x[k + 2][0]) for k in range(2)]
        m = [(x[k][0] + x[k + 2][1], x[k][1] - x[k + 2][0]) for k in range(2)]
        return p, m
    ap, am = split(a)
    bp, bm = split(b)
    cp = _prod2(*ap, *bp, 1)
    cm = _prod2(*am, *bm, -1)
    lo = [_cadd(cp[k], cm[k]) for k in range(2)]
    hi = [(cp[k][1] - cm[k][1], cm[k][0] - cp[k][0]) for k in range(2)]
    return lo + hi


def _prod_mod_i(a, b, sgn):
    sm = [x[0] + x[1] for x in b]
    df = [x[1] - x[0] for x in b]
    asum = [x[0] + x[1] for x in a]
    out = []
    for k in range(4):
        acc = [None, None, None]
        for j in range(4):
            m = (k - j) % 4
            if j <= k:
                t = ((b[m][0], 1), (df[m], 1), (sm[m], 1))
            elif sgn > 0:
                t = ((b[m][1], -1), (sm[m], 1), (df[m], -1))
            else:
                t = ((b[m][1], 1), (sm[m], -1), (df[m], 1))
            for q, (v, (w, s)) in enumerate(zip((asum[j], a[j][0], a[j][1]), t)):
                p = v * w
                if acc[q] is None:
                    acc[q] = p
                else:
                    acc[q] = acc[q] + p if s > 0 else acc[q] - p
        out.append((acc[0] - acc[2], acc[0] + acc[1]))
    return out


def _middle(a, b):
    scale = lambda v, f: [(x[0] * f, x[1] * f) for x in v]
    c0 = _prod_mod_1([_cadd(x[0], x[2]) for x in a], [_cadd(x[0], x[2]) for x in b])
    c2 = _prod_mod_m1([_csub(x[0], x[2]) for x in a],
                      scale([_csub(x[0], x[2]) for x in b], 2.0))
    even = [(_cadd(p, q), _csub(p, q)) for p, q in zip(c0, c2)]
    c1 = _prod_mod_i([x[1] for x in a], scale([x[1] for x in b], 4.0), 1)
    c3 = _prod_mod_i([x[3] for x in a], scale([x[3] for x in b], 4.0), -1)
    return [e + (_cadd(p, q), _csub(p, q)) for e, p, q in zip(even, c1, c3)]


def _barrel(v, lane, sign):
    for bit in range(4):
        m = ((lane >> bit) & 1) == 1
        v = [jnp.where(m, v[(i + (1 << bit)) % 16], v[i]) for i in range(16)]
    return [v[(sign * s) % 16] for s in range(16)]


def _lane_t1(lane):
    return 32 * (lane & 3) + (lane >> 2)


def _to_residues(tiles):
    lane = _iota((8, 128), 1)
    v = [t if j == 0 else pltpu.roll(t, j, 1) for j, t in enumerate(tiles)]
    v = _barrel(v, lane, -1)
    t1 = _lane_t1(lane)
    src = 16 * (t1 & 7) + (t1 >> 3)
    return [jnp.take_along_axis(v[s], (src + s) & 127, axis=1) for s in range(16)]


def _to_time(res):
    lane = _iota((8, 128), 1)
    v = []
    for s in range(16):
        mu = (lane - s) & 127
        t1 = 8 * (mu & 15) + (mu >> 4)
        v.append(jnp.take_along_axis(res[s], 4 * (t1 & 31) + (t1 >> 5), axis=1))
    v = _barrel(v, lane, -1)
    return [t if j == 0 else pltpu.roll(t, 128 - j, 1) for j, t in enumerate(v)]


def _pack(a, b):
    return pltpu.pack_elementwise([a, b], packed_dtype=BF16)


def _unpack(w):
    return [pltpu.unpack_elementwise(w, index=i, packed_dtype=BF16, unpacked_dtype=F32)
            for i in range(2)]


FINE = (0, 1, 2, 3, 4, 5, 6, 7, 512, 516, 1024, 1536)


def _k_seeds(z, c):
    lo = _iota((8, 128), 0) < 4
    pw = {1: z}
    for e in range(1, 10):
        pw[1 << e] = _csq(pw[1 << (e - 1)])
    rot = lambda v: tuple(pltpu.roll(x, 4, 0) for x in v)
    sel = lambda a, b: tuple(jnp.where(lo, p, q) for p, q in zip(a, b))
    z16 = (pw[16][0], 0.0 - pw[16][1])
    pairs = [(z, rot(z)), (pw[32], rot(pw[32])), (pw[512], rot(pw[512])),
             (c, rot(_cmul(c, pw[8])))]
    return [[sel(a, b) for a, b in pairs] + [sel((1.0, 0.0), rot(z16))],
            [sel(b, a) for a, b in pairs] + [sel((1.0, 0.0), z16)]]


def _mxu(words):
    return pltpu.bitcast(words, BF16)


def _k_tables(seeds, ta_ref, tb_ref):
    m1, m32, m512, a0, b0 = seeds
    fa = [a0]
    for r in range(1, 8):
        fa.append(_cmul(fa[-1], m1))
    for src in (0, 4, 8, 10):
        fa.append(_cmul(fa[src], m512))
    tail = fa[11][0] * m512[0] - fa[11][1] * m512[1]
    fb = [b0]
    for m in range(1, 16):
        p = fb[-1]
        fb.append((p[0] * m32[0] + p[1] * m32[1], p[1] * m32[0] - p[0] * m32[1]))
    for ref, tab in ((ta_ref, fa), (tb_ref, fb)):
        for i in range(0, len(tab), 2):
            for p in range(2):
                ref[p, 8 * i:8 * i + 16, :] = jnp.concatenate(
                    [tab[i][p], tab[i + 1][p]], axis=0).astype(BF16)
    return tail


def _k_residues(groups, k_last, dskip):
    sub = _iota((8, 128), 0)
    lane = _iota((8, 128), 1)
    lo = sub < 4
    idx = (lane & ~3) | (sub & 3)
    kv = {}
    for i, k in enumerate(FINE):
        v = [g[8 * i:8 * i + 8] for g in groups]
        if k == 0:
            v = [x + jnp.where((lane < 4) & (lo if n % 2 == 0 else ~lo),
                               dskip[n // 2], 0.0)
                 for n, x in enumerate(v)]
        p = [_pack(v[g], v[2 + g]) for g in range(2)]
        kv[k] = jnp.take_along_axis(jnp.where(lo, p[0], p[1]), idx, axis=1)
        kv[k + 8] = jnp.take_along_axis(pltpu.roll(jnp.where(lo, p[1], p[0]), 4, 0), idx, axis=1)
    q = lane & 3
    s3 = {r: jnp.where(q == 2, kv[1024 + r], kv[1536 + r]) for r in (0, 8)}
    v0 = jnp.where(q == 0, kv[0], jnp.where(q == 1, kv[512], s3[0]))
    nxt = jnp.where(lane < 124, lane + 4, (lane - 123) & 127)
    v16 = jnp.where(lane == 127, k_last, jnp.take_along_axis(v0, nxt, axis=1))
    s3[16] = v16
    s23, s123, out = {}, {}, [v0]
    for r in range(1, 16):
        k23 = (RES2[r], RES3[r])
        if k23 not in s23:
            s23[k23] = v16 if k23 == (16, 16) else jnp.where(q == 1, kv[512 + k23[0]], s3[k23[1]])
        k123 = (RES1[r],) + k23
        if k123 not in s123:
            s123[k123] = v16 if k123[0] == 16 else jnp.where(q == 0, kv[k123[0]], s23[k23])
        if RES1[r] == r:
            out.append(s123[k123])
        else:
            out.append(jnp.where((q == 0) & (lane < 64), kv[r], s123[k123]))
    return out


def _ln_scalars(s1, s2):
    mean = s1 * (1.0 / D)
    var = jnp.maximum(s2 * (1.0 / D) - mean * mean, 0.0)
    eps = float(np.asarray(EPS, dtype=BF16))
    sd = _rbf(jnp.sqrt(_rbf(_rbf(var) + eps)))
    return _rbf(mean), 1.0 / sd


def _column(vec):
    row = vec.astype(F32).reshape(1, D)
    parts = []
    for lo in range(0, D, 128):
        start = min(lo, D - 128)
        t = jnp.broadcast_to(row[:, start:start + 128], (128, 128)).T
        parts.append(t[lo - start:])
    return jnp.concatenate(parts, axis=0)


def _kernel(x_hbm, are_ref, aim_ref, bre_ref, bim_ref, cre_ref, cim_ref,
            ldt_ref, dsk_ref, wr_ref, wg_hbm, wu_hbm, wd_hbm, out_hbm,
            x_v, wg_v, wu_v, wd_v, w_v, wt_v, col_v, seed_v, h_v, st_v, acc_v, out_v,
            ta0, ta1, tb0, tb1, kl0, kl1, uk0, uk1, ab0, ab1, c0, c1, y0, y1, sem):
    cp_x = [pltpu.make_async_copy(x_hbm.at[:, 128 * j:128 * j + 128], x_v.at[j], sem.at[5 + j])
            for j in range(NT)]
    cp_g = pltpu.make_async_copy(wg_hbm, wg_v, sem.at[1])
    cp_u = pltpu.make_async_copy(wu_hbm, wu_v, sem.at[2])
    cp_d = pltpu.make_async_copy(wd_hbm, wd_v, sem.at[3])
    for cp in cp_x:
        cp.start()
    cp_g.start()
    cp_u.start()
    cp_d.start()

    k4 = 4 * _iota((128, 128), 1) + 1
    ph = ((k4 * _lane_t1(_iota((128, 128), 0))) & 511).astype(F32) * (2 * np.pi / 512)
    w = (jnp.cos(ph), jnp.sin(ph))
    ph1 = (4 * _iota((8, 128), 1) + 1).astype(F32) * (2 * np.pi / (4 * L))
    tw = (jnp.tile(jnp.cos(ph1), (16, 1)), jnp.tile(jnp.sin(ph1), (16, 1)))
    for s in range(16):
        wr, wi = w[0].astype(BF16), w[1].astype(BF16)
        w_v[s, 0] = wr
        w_v[s, 1] = wi
        wt_v[s, 0] = w_v[s, 0].T
        wt_v[s, 1] = w_v[s, 1].T
        if s < 15:
            w = _cmul(w, tw)

    col_v[0] = _rbf(jnp.exp(_column(ldt_ref[...])))
    col_v[1] = _column(dsk_ref[...]) * (1.0 / L)
    col_v[2] = _column(wr_ref[...])

    def seed_step(i, carry):
        for r in range(2):
            rows = pl.ds(pl.multiple_of(i * 16 + 8 * r, 8), 8)
            par = [_unpack(ref.bitcast(I32)[rows, :])
                   for ref in (are_ref, aim_ref, bre_ref, bim_ref, cre_ref, cim_ref)]
            for h in range(2):
                a_re, a_im, b_re, b_im, c_re, c_im = [v[h] for v in par]
                dt = col_v[0, pl.ds(i * 32 + 16 * r + h, 8, stride=2), :]
                mag, ang = jnp.exp(dt * a_re), dt * a_im
                sc = dt * (1.0 / L)
                seeds = _k_seeds((mag * jnp.cos(ang), mag * jnp.sin(ang)),
                                 _cmul((c_re, c_im), (sc * b_re, sc * b_im)))
                for g in range(2):
                    for n, v in enumerate(seeds[g]):
                        for p in range(2):
                            seed_v[2 * i + r, 2 * h + g, 2 * n + p] = v[p]
        return carry

    with jax.named_scope("S_seed"):
        jax.lax.fori_loop(0, D // 32, seed_step, 0)

    ta, tb, kl = (ta0, ta1), (tb0, tb1), (kl0, kl1)
    uk, ab, cc, yy = (uk0, uk1), (ab0, ab1), (c0, c1), (y0, y1)
    w_w, wt_w = w_v.bitcast(I32), wt_v.bitcast(I32)

    def chan(b, r):
        return pl.ds(pl.multiple_of(b * MB + 16 * r, 16), 16)

    def table_stage(b, r):
        tail = [_k_tables([(seed_v[4 * b + r, g, 2 * n], seed_v[4 * b + r, g, 2 * n + 1])
                           for n in range(5)], ta[b % 2].at[r, g], tb[b % 2].at[r, g])
                for g in range(4)]
        lo = _iota((8, 128), 0) < 4
        kl[b % 2][r] = _pack(*[jnp.broadcast_to(
            jnp.sum(jnp.where(lo, tail[2 * h], tail[2 * h + 1]), axis=1, keepdims=True),
            (8, 128)) for h in range(2)])

    def kernel_stage(b, r):
        ta_w, tb_w = ta[b % 2].bitcast(I32), tb[b % 2].bitcast(I32)
        groups = []
        for g in range(4):
            res = [jax.lax.dot_general(_mxu(ta_w[r, g, p]), _mxu(tb_w[r, g, p]), NT_DIMS,
                                       preferred_element_type=F32) for p in range(2)]
            groups.append(res[0] + res[1])
        dskip = [col_v[1, pl.ds(b * MB + 16 * r + h, 8, stride=2), :] for h in range(2)]
        dst = pl.ds(pl.multiple_of(MB // 2 + 8 * r, 8), 8)
        for s, t in enumerate(_k_residues(groups, kl[b % 2][r], dskip)):
            uk[b % 2][s, dst, :] = t

    def norm_stage(b, r):
        tiles = []
        rows = pl.ds(pl.multiple_of(b * MB // 2 + 8 * r, 8), 8)
        for j in range(NT):
            m, inv = st_v[0, j], st_v[1, j]
            tiles.append(_pack(*[(v - m) * inv for v in _unpack(x_v.bitcast(I32)[j, rows, :])]))
        dst = pl.ds(pl.multiple_of(8 * r, 8), 8)
        for s, t in enumerate(_to_residues(tiles)):
            uk[b % 2][s, dst, :] = t

    def forward_stage(b, k):
        lhs = [_mxu(uk[b % 2][k + 4 * n]) for n in range(4)]
        dst = ab[b % 2]
        for p in range(2):
            v = [jnp.dot(lhs[n], _mxu(w_w[k + 4 * n, p ^ (n & 1)]), preferred_element_type=F32)
                 for n in range(4)]
            d02, d13 = v[0] - v[2], v[1] - v[3]
            dst[k, 0, p] = v[0] + v[2]
            dst[k, 2, 1 - p] = v[1] + v[3]
            dst[k, 1, p] = d02 - d13 if p == 0 else d02 + d13
            dst[k, 3, p] = d02 + d13 if p == 0 else d02 - d13

    def middle_stage(b, r):
        src = ab[b % 2]
        for h in range(2):
            ra = pl.ds(pl.multiple_of(16 * r + 8 * h, 8), 8)
            rb = pl.ds(pl.multiple_of(MB + 16 * r + 8 * h, 8), 8)
            u, kk = ([[(src[k, q, 0, rr, :], src[k, q, 1, rr, :]) for q in range(4)]
                      for k in range(4)] for rr in (ra, rb))
            for k, v in enumerate(_middle(u, kk)):
                for q in range(4):
                    for p in range(2):
                        cc[b % 2][k, q, p, ra, :] = v[q][p]

    def inverse_stage(b, k):
        src = cc[b % 2]

        def lhs(v):
            return _mxu(jnp.concatenate(
                [_pack(v[i:i + 8], v[i + 8:i + 16]) for i in range(0, MB, 16)], axis=0))

        s02, d02, s13, d13 = [(src[k, q, 0], src[k, q, 1]) for q in range(4)]
        e = {0: _cadd(s02, s13), 2: _csub(s02, s13),
             1: (d02[0] + d13[1], d02[1] - d13[0]), 3: (d02[0] - d13[1], d02[1] + d13[0])}
        for n in e:
            y = [jnp.dot(lhs(e[n][p]), _mxu(wt_w[k + 4 * n, p]), preferred_element_type=F32)
                 for p in range(2)]
            yy[b % 2][k + 4 * n] = (y[0] + y[1]).astype(BF16)

    def residual_stage(b, r):
        rows = chan(b, r)
        wr = col_v[2, rows, :]
        src = yy[b % 2].bitcast(I32)
        ys = _to_time([src[s, pl.ds(pl.multiple_of(8 * r, 8), 8), :] for s in range(16)])
        for j in range(NT):
            h = x_v[j, rows, :].astype(F32) + jnp.concatenate(
                _unpack(ys[j]), axis=0)
            h_v[j, rows, :] = h
            hh, hw = h * h, h * wr
            acc_v[0, j] += h[0:8] + h[8:16]
            acc_v[1, j] += hh[0:8] + hh[8:16]
            acc_v[2, j] += hw[0:8] + hw[8:16]

    nb = D // MB

    def run(step, stages):
        live = [(f, step - lag) for f, lag in stages if 0 <= step - lag < nb]

        def body(r, carry):
            for f, b in live:
                f(b, r)
            return carry

        with jax.named_scope("S_p%d" % step):
            jax.lax.fori_loop(0, 4, body, 0)

    stages = [(kernel_stage, 1), (forward_stage, 2), (inverse_stage, 4), (norm_stage, 1),
              (residual_stage, 5), (middle_stage, 3), (table_stage, 0)]
    run(0, stages)

    with jax.named_scope("S_xwait"):
        for cp in cp_x:
            cp.wait()
    for j in range(NT):
        xs = x_v[j].astype(F32)
        m, inv = _ln_scalars(jnp.sum(xs, axis=0, keepdims=True),
                             jnp.sum(xs * xs, axis=0, keepdims=True))
        st_v[0, j] = jnp.broadcast_to(m, (8, 128))
        st_v[1, j] = jnp.broadcast_to(inv, (8, 128))
    acc_v[...] = jnp.zeros(acc_v.shape, F32)

    for step in range(1, nb + 5):
        run(step, stages)

    def rows_of(q):
        return jnp.concatenate(
            [jnp.sum(acc_v[q, j], axis=0, keepdims=True) for j in range(NT)], axis=0)

    m2, inv2 = _ln_scalars(rows_of(0), rows_of(1))
    wsum = jnp.sum(col_v[2], axis=0, keepdims=True)
    score = _rbf((rows_of(2) - m2 * wsum) * inv2 + 0.0)
    bits = pltpu.bitcast(score, I32) >> 16
    order = jnp.where(bits < 0, -1 - bits, bits + 32768)
    pos = 128 * _iota((NT, 128), 0) + _iota((NT, 128), 1)
    key = pltpu.bitcast((order << 11) + (L - 1 - pos) + (1 << 29), F32)

    lane = _iota((D, 128), 1)
    sel = jnp.zeros((D, 128), F32)
    aux = jnp.zeros((8, 128), F32)
    lane8, sub8 = _iota((8, 128), 1), _iota((8, 128), 0)
    picks = []
    for c in range(CAP):
        top = jnp.max(key, axis=(0, 1), keepdims=True)
        hit = key == top
        key = jnp.where(hit, 0.0, key)
        t = jnp.max(jnp.where(hit, pos, 0))
        j, i = jnp.clip(t >> 7, 0, NT - 1), t & 127
        picks.append((j, i))
        sel = jnp.where(lane == c, pltpu.roll(h_v[j], (128 + c - i) & 127, 1), sel)
        for q, v in enumerate((m2, inv2, score)):
            val = jnp.sum(jnp.where(hit, v, 0.0), axis=(0, 1), keepdims=True)
            aux = jnp.where((sub8 == c) & (lane8 == q), val, aux)
    h_sel = sel.T[0:CAP]
    x_sel = _rbf((h_sel - aux[:, 0:1]) * aux[:, 1:2])
    gate = _rbf(jax.nn.sigmoid(aux[:, 2:3]))

    for j in range(NT):
        h = h_v[j]
        out_v[:, 128 * j:128 * j + 128] = (
            h + (h - m2[j:j + 1]) * inv2[j:j + 1]).astype(BF16)

    xb = x_sel.astype(BF16)
    with jax.named_scope("S_gwait"):
        cp_g.wait()
    g = _rbf(jnp.dot(xb, wg_v[...], preferred_element_type=F32))
    with jax.named_scope("S_uwait"):
        cp_u.wait()
    up = _rbf(jnp.dot(xb, wu_v[...], preferred_element_type=F32))
    act = (_rbf(g * jax.nn.sigmoid(g)) * up).astype(BF16)
    with jax.named_scope("S_dwait"):
        cp_d.wait()
    y = _rbf(jax.lax.dot_general(act, wd_v[...], NT_DIMS, preferred_element_type=F32))
    new = h_sel + _rbf(x_sel + _rbf(y * gate))
    new = jnp.concatenate([new, jnp.zeros((128 - CAP, D), F32)], axis=0).T.astype(BF16)
    new = pltpu.bitcast(new, I32)
    lane_p = _iota((D // 2, 128), 1)
    for c, (j, i) in enumerate(picks):
        cols = pl.ds(pl.multiple_of(j * 128, 128), 128)
        old = pltpu.bitcast(out_v[:, cols], I32)
        upd = jnp.where(lane_p == i, pltpu.roll(new, (128 + i - c) & 127, 1), old)
        out_v[:, cols] = pltpu.bitcast(upd, BF16)
    cp_o = pltpu.make_async_copy(out_v, out_hbm, sem.at[4])
    cp_o.start()
    with jax.named_scope("S_owait"):
        cp_o.wait()


@jax.jit
def pallas_sequential_preLN__ssm_conv_s4__moe_arch_mod__prompt_kernel(
    A_u: jax.Array,
    A_A_re: jax.Array,
    A_A_im: jax.Array,
    A_B_re: jax.Array,
    A_B_im: jax.Array,
    A_C_re: jax.Array,
    A_C_im: jax.Array,
    A_log_dt: jax.Array,
    A_Dskip: jax.Array,
    B_x: jax.Array,
    B_w_r: jax.Array,
    B_w_gate: jax.Array,
    B_w_up: jax.Array,
    B_w_down: jax.Array,
):
    del B_x
    hbm = pl.BlockSpec(memory_space=pl.ANY)
    vmem = pl.BlockSpec(memory_space=pltpu.VMEM)
    out = pl.pallas_call(
        _kernel,
        out_shape=jax.ShapeDtypeStruct((D, L), BF16),
        in_specs=[hbm] + [vmem] * 9 + [hbm] * 3,
        out_specs=hbm,
        scratch_shapes=[
            pltpu.VMEM((NT, D, 128), BF16),
            pltpu.VMEM((D, FF), BF16),
            pltpu.VMEM((D, FF), BF16),
            pltpu.VMEM((D, FF), BF16),
            pltpu.VMEM((16, 2, 128, 128), BF16),
            pltpu.VMEM((16, 2, 128, 128), BF16),
            pltpu.VMEM((3, D, 128), F32),
            pltpu.VMEM((D // 16, 4, 10, 8, 128), F32),
            pltpu.VMEM((NT, D, 128), F32),
            pltpu.VMEM((2, NT, 8, 128), F32),
            pltpu.VMEM((3, NT, 8, 128), F32),
            pltpu.VMEM((D, L), BF16),
            *[pltpu.VMEM((4, 4, 2, 96, 128), BF16)] * 2,
            *[pltpu.VMEM((4, 4, 2, 128, 128), BF16)] * 2,
            *[pltpu.VMEM((4, 8, 128), I32)] * 2,
            *[pltpu.VMEM((16, MB, 128), I32)] * 2,
            *[pltpu.VMEM((4, 4, 2, 2 * MB, 128), F32)] * 2,
            *[pltpu.VMEM((4, 4, 2, MB, 128), F32)] * 2,
            *[pltpu.VMEM((16, MB, 128), BF16)] * 2,
            pltpu.SemaphoreType.DMA((5 + NT,)),
        ],
        compiler_params=pltpu.CompilerParams(vmem_limit_bytes=100 * 1024 * 1024),
    )(A_u.reshape(L, D).T, A_A_re, A_A_im, A_B_re, A_B_im, A_C_re, A_C_im,
      A_log_dt, A_Dskip, B_w_r, B_w_gate, B_w_up, B_w_down.T)
    return out.T.reshape(1, L, D)
```

```python
import functools

import numpy as np
import jax
import jax.numpy as jnp
import jax.experimental.pallas as pl
import jax.experimental.pallas.tpu as pltpu

F32 = jnp.float32
BF16 = jnp.bfloat16
I32 = jnp.int32

L = 2048
D = 576
N = 128
FF = 4608
CAP = 8
NT = L // 128
EPS = 1e-5
MB = 64
import os
STEPS = eval(os.environ["ONE"]) if os.environ.get("ONE") else range(3, D // MB + 6)
PLAN = [(x[0],) + tuple(int(v) for v in (x[1:].split(":") if len(x) > 1 else (-1, -1)))
        for x in os.environ.get("PLAN", "s-1:20,s-1:-1,t-1:4,m-1:7,m-1:10,f,m2:15,f,m6:17,k,t8:21,r11:27,k,m16:28,m19:33,k-1:-1,i,n23:-1,f,t24:-1,i,t28:-1,f,r34:-1").split(",")]
ROW_CHUNKS = ((0, 384), (384, D))
NT_DIMS = (((1,), (1,)), ((), ()))


def _round_res(step):
    return [int(np.round(r / step)) * step for r in range(16)]


RES1, RES2, RES3 = _round_res(2), _round_res(4), _round_res(8)


def _ds(start, size):
    return pl.ds(start if isinstance(start, int) else pl.multiple_of(start, size), size)


def _iota(shape, dim):
    return jax.lax.broadcasted_iota(I32, shape, dim)


def _rbf(x):
    return x.astype(BF16).astype(F32)


def _cmul(a, b):
    return (a[0] * b[0] - a[1] * b[1], a[0] * b[1] + a[1] * b[0])


def _csq(a):
    t = a[0] * a[1]
    return ((a[0] + a[1]) * (a[0] - a[1]), t + t)


def _cadd(a, b):
    return (a[0] + b[0], a[1] + b[1])


def _csub(a, b):
    return (a[0] - b[0], a[1] - b[1])


def _bfly4(a0, a1, a2, a3, inverse=False):
    s02, d02 = _cadd(a0, a2), _csub(a0, a2)
    s13, d13 = _cadd(a1, a3), _csub(a1, a3)
    p = (d02[0] - d13[1], d02[1] + d13[0])
    m = (d02[0] + d13[1], d02[1] - d13[0])
    if inverse:
        p, m = m, p
    return _cadd(s02, s13), p, _csub(s02, s13), m


def _prod_mod_1(a, b):
    fa, fb = _bfly4(*a), _bfly4(*b)
    return _bfly4(*[_cmul(x, y) for x, y in zip(fa, fb)], inverse=True)


def _prod2(a0, a1, b0, b1, sgn):
    p00, p11 = _cmul(a0, b0), _cmul(a1, b1)
    c1 = _cadd(_cmul(a0, b1), _cmul(a1, b0))
    if sgn > 0:
        return (p00[0] - p11[1], p00[1] + p11[0]), c1
    return (p00[0] + p11[1], p00[1] - p11[0]), c1


def _prod_mod_m1(a, b):
    def split(x):
        p = [(x[k][0] - x[k + 2][1], x[k][1] + x[k + 2][0]) for k in range(2)]
        m = [(x[k][0] + x[k + 2][1], x[k][1] - x[k + 2][0]) for k in range(2)]
        return p, m
    ap, am = split(a)
    bp, bm = split(b)
    cp = _prod2(*ap, *bp, 1)
    cm = _prod2(*am, *bm, -1)
    lo = [_cadd(cp[k], cm[k]) for k in range(2)]
    hi = [(cp[k][1] - cm[k][1], cm[k][0] - cp[k][0]) for k in range(2)]
    return lo + hi


def _prod_mod_i(a, b, sgn):
    sm = [x[0] + x[1] for x in b]
    df = [x[1] - x[0] for x in b]
    asum = [x[0] + x[1] for x in a]
    out = []
    for k in range(4):
        acc = [None, None, None]
        for j in range(4):
            m = (k - j) % 4
            if j <= k:
                t = ((b[m][0], 1), (df[m], 1), (sm[m], 1))
            elif sgn > 0:
                t = ((b[m][1], -1), (sm[m], 1), (df[m], -1))
            else:
                t = ((b[m][1], 1), (sm[m], -1), (df[m], 1))
            for q, (v, (w, s)) in enumerate(zip((asum[j], a[j][0], a[j][1]), t)):
                p = v * w
                if acc[q] is None:
                    acc[q] = p
                else:
                    acc[q] = acc[q] + p if s > 0 else acc[q] - p
        out.append((acc[0] - acc[2], acc[0] + acc[1]))
    return out


def _barrel(v):
    lane = _iota((8, 128), 1)
    for bit in range(4):
        m = ((lane >> bit) & 1) == 1
        v = [jnp.where(m, v[(i + (1 << bit)) % 16], v[i]) for i in range(16)]
    return [v[-s % 16] for s in range(16)]


def _to_residues(tiles):
    return _barrel([t if j == 0 else pltpu.roll(t, j, 1) for j, t in enumerate(tiles)])


def _to_time(res):
    return [t if j == 0 else pltpu.roll(t, 128 - j, 1) for j, t in enumerate(_barrel(res))]


def _gather(x, idx):
    return jnp.take_along_axis(x, idx, axis=1, mode="promise_in_bounds")


def _init_dft(wu_ref, wk_ref, wt_ref, tmp_ref):
    sub, k4 = _iota((8, 128), 0), 4 * _iota((8, 128), 1) + 1

    def cis(t):
        ph = ((k4 * t) & (4 * L - 1)).astype(F32) * (2 * np.pi / (4 * L))
        return jnp.cos(ph), jnp.sin(ph)

    w1, w16 = cis(1), cis(16)
    w32 = _csq(w16)
    fk = [cis(16 * (32 * (sub & 3) + (sub >> 2)))]
    fu = [cis(128 * sub), cis(128 * (sub + 8))]
    for v in range(1, 16):
        fk.append(_cmul(fk[-1], w32))
        if v >= 2:
            fu.append(_cmul(fu[-2], w16))
    for p in range(2):
        for v in range(32):
            tmp_ref[p, 8 * v:8 * v + 8, :] = fu[v % 16][p]
    tw = None
    for s in range(16):
        for v in range(0, 16, 2):
            rows = [slice(128 - s + 8 * i, 136 - s + 8 * i) for i in (v, v + 1)]
            for ref, f in ((wk_ref, fk[v:v + 2]),
                           (wu_ref, [(tmp_ref[0, r, :], tmp_ref[1, r, :]) for r in rows])):
                if s:
                    f = [_cmul(x, tw) for x in f]
                for p in range(2):
                    ref[s, p, 8 * v:8 * v + 16, :] = jnp.concatenate(
                        [f[0][p], f[1][p]], axis=0).astype(BF16)
        for p in range(2):
            wt_ref[s, p] = pltpu.bitcast(_mxu(wu_ref.bitcast(I32)[s, p]).T, I32)
        tw = _cmul(tw, w1) if s else w1


def _pack(a, b):
    return pltpu.pack_elementwise([a, b], packed_dtype=BF16)


def _unpack(w):
    return [pltpu.unpack_elementwise(w, index=i, packed_dtype=BF16, unpacked_dtype=F32)
            for i in range(2)]


FINE = (0, 1, 2, 3, 4, 5, 6, 7, 512, 516, 1024, 1536)


def _k_seeds(z, c):
    lo = _iota((8, 128), 0) < 4
    pw = {1: z}
    for e in range(1, 10):
        pw[1 << e] = _csq(pw[1 << (e - 1)])
    rot = lambda v: tuple(pltpu.roll(x, 4, 0) for x in v)
    sel = lambda a, b: tuple(jnp.where(lo, p, q) for p, q in zip(a, b))
    z16 = (pw[16][0], 0.0 - pw[16][1])
    pairs = [(z, rot(z)), (pw[32], rot(pw[32])), (pw[512], rot(pw[512])),
             (c, rot(_cmul(c, pw[8])))]
    return [[sel(a, b) for a, b in pairs] + [sel((1.0, 0.0), rot(z16))],
            [sel(b, a) for a, b in pairs] + [sel((1.0, 0.0), z16)]]


def _mxu(words):
    return pltpu.bitcast(words, BF16)


def _store_table(ref, tab):
    for i in range(0, len(tab), 2):
        for p in range(2):
            ref[p, 8 * i:8 * i + 16, :] = jnp.concatenate(
                [tab[i][p], tab[i + 1][p]], axis=0).astype(BF16)


def _k_residues(groups, k_last, dskip):
    sub = _iota((8, 128), 0)
    lane = _iota((8, 128), 1)
    lo = sub < 4
    idx = (lane & ~3) | (sub & 3)
    nxt = ((idx + 4) & 127)
    kv, up = {}, {}
    for i, k in enumerate(FINE):
        v = [g[8 * i:8 * i + 8] for g in groups]
        if k == 0:
            v = [x + jnp.where((lane < 4) & (lo if n % 2 == 0 else ~lo),
                               dskip[n // 2], 0.0)
                 for n, x in enumerate(v)]
        p = [_pack(v[g], v[2 + g]) for g in range(2)]
        even = jnp.where(lo, p[0], p[1])
        kv[k] = _gather(even, idx)
        kv[k + 8] = _gather(pltpu.roll(jnp.where(lo, p[1], p[0]), 4, 0), idx)
        if k % 512 == 0:
            up[k] = _gather(even, nxt)
    q = lane & 3
    s3 = {r: jnp.where(q == 2, kv[1024 + r], kv[1536 + r]) for r in (0, 8)}
    v0 = jnp.where(q == 0, kv[0], jnp.where(q == 1, kv[512], s3[0]))
    q16 = q + jnp.where(lane >= 124, 1, 0)
    v16 = jnp.where(q16 < 2, jnp.where(q16 == 0, up[0], up[512]),
                    jnp.where(q16 == 2, up[1024], jnp.where(q16 == 3, up[1536], k_last)))
    s3[16] = v16
    s23, s123, out = {}, {}, [v0]
    for r in range(1, 16):
        k23 = (RES2[r], RES3[r])
        if k23 not in s23:
            s23[k23] = v16 if k23 == (16, 16) else jnp.where(q == 1, kv[512 + k23[0]], s3[k23[1]])
        k123 = (RES1[r],) + k23
        if k123 not in s123:
            s123[k123] = v16 if k123[0] == 16 else jnp.where(q == 0, kv[k123[0]], s23[k23])
        if RES1[r] == r:
            out.append(s123[k123])
        else:
            out.append(jnp.where((q == 0) & (lane < 64), kv[r], s123[k123]))
    return out


def _ln_scalars(s1, s2):
    mean = s1 * (1.0 / D)
    var = jnp.maximum(s2 * (1.0 / D) - mean * mean, 0.0)
    eps = float(np.asarray(EPS, dtype=BF16))
    sd = _rbf(jnp.sqrt(_rbf(_rbf(var) + eps)))
    return _rbf(mean), 1.0 / sd


def _column(vec):
    row = vec.astype(F32).reshape(1, D)
    parts = []
    for lo in range(0, D, 128):
        start = min(lo, D - 128)
        t = jnp.broadcast_to(row[:, start:start + 128], (128, 128)).T
        parts.append(t[lo - start:])
    return jnp.concatenate(parts, axis=0)


class _Schedule:
    def __init__(self, r):
        self.true = _iota((8, 128), 0) + r >= 0
        self.done, self.pending, self.wait = [], {}, -1

    def tie(self, x, token):
        return jnp.where(self.true, x, token if token.dtype == x.dtype
                         else pltpu.bitcast(token, x.dtype))

    def start(self, x):
        return self.tie(x, self.done[self.wait]) if 0 <= self.wait < len(self.done) else x

    def lhs(self, words, first):
        tiles = [words[i:i + 8] for i in range(0, words.shape[0], 8)]
        for i in range(len(tiles) if first else 0):
            for token in self.pending.pop(len(self.done) + i, ()):
                tiles[i] = self.tie(tiles[i], token)
        return _mxu(jnp.concatenate(tiles, axis=0))

    def results(self, v):
        self.done += [v[i + 8:i + 16] for i in range(0, v.shape[0], 16)]

    def run(self, stage, wait, before):
        self.wait = wait
        self.pending.setdefault(before, []).extend(next(stage))


def _kernel(x_hbm, are_hbm, aim_hbm, bre_hbm, bim_hbm, cre_hbm, cim_hbm,
            ldt_hbm, dsk_hbm, wr_hbm, wg_hbm, wu_hbm, wd_hbm, out_hbm,
            x_v, wg_v, wu_v, wd_v, par_v, ldt_v, dsk_v, wr_v, w_v, wk_v, wt_v, col_v,
            tmp_v, h_v, st_v, acc_v, out_v, sd0, sd1, ta0, ta1, tb0, tb1, kl0, kl1,
            u0, u1, k0, k1, ab0, ab1, c0, c1, y0, y1, pick_s, sem_p, sem_x, sem_w, sem_o):
    cp_vec = [pltpu.make_async_copy(s, d, sem_p.at[n]) for n, (s, d) in enumerate(
        ((ldt_hbm, ldt_v), (dsk_hbm, dsk_v), (wr_hbm, wr_v)))]
    cp_par = [[pltpu.make_async_copy(s.at[lo:hi], par_v.at[n, lo:hi], sem_p.at[3 + 6 * m + n])
               for n, s in enumerate((are_hbm, aim_hbm, bre_hbm, bim_hbm, cre_hbm, cim_hbm))]
              for m, (lo, hi) in enumerate(((0, 3 * MB), (3 * MB, D)))]
    cp_x = [pltpu.make_async_copy(x_hbm.at[:, 128 * j:128 * j + 128], x_v.at[j], sem_x.at[j])
            for j in range(NT)]
    cp_w = [pltpu.make_async_copy(s, d, sem_w.at[n]) for n, (s, d) in enumerate(
        ((wg_hbm, wg_v), (wu_hbm, wu_v), (wd_hbm, wd_v)))]
    for cp in cp_vec + cp_par[0] + cp_x + cp_par[1] + cp_w:
        cp.start()

    with jax.named_scope("S_dft"):
        _init_dft(w_v, wk_v, wt_v, tmp_v)
    for cp in cp_vec:
        cp.wait()
    col_v[0] = _rbf(jnp.exp(_column(ldt_v[...])))
    col_v[1] = _column(dsk_v[...]) * (1.0 / L)
    col_v[2] = _column(wr_v[...])
    with jax.named_scope("S_pwait"):
        for cp in cp_par[0]:
            cp.wait()

    sd, ta, tb, kl = (sd0, sd1), (ta0, ta1), (tb0, tb1), (kl0, kl1)
    uk, ab, cc, yy = ((u0, u1), (k0, k1)), (ab0, ab1), (c0, c1), (y0, y1)
    ww, wt_w = (w_v.bitcast(I32), wk_v.bitcast(I32)), wt_v

    def chan(b, r):
        return pl.ds(pl.multiple_of(b * MB + 16 * r, 16), 16)

    def seed_stage(b, r, sch):
        rows = _ds(b * MB // 2 + 8 * r, 8)
        par = [_unpack(par_v.bitcast(I32)[n, rows, :]) for n in range(6)]
        for h in range(2):
            a_re, a_im, b_re, b_im, c_re, c_im = [v[h] for v in par]
            dt = sch.start(col_v[0, pl.ds(b * MB + 16 * r + h, 8, stride=2), :])
            mag, ang = jnp.exp(dt * a_re), dt * a_im
            sc = dt * (1.0 / L)
            seeds = _k_seeds((mag * jnp.cos(ang), mag * jnp.sin(ang)),
                             _cmul((c_re, c_im), (sc * b_re, sc * b_im)))
            for g in range(2):
                for n, v in enumerate(seeds[g]):
                    for p in range(2):
                        sd[b % 2][r, 2 * h + g, 2 * n + p] = v[p]
            yield [seeds[1][2][0]]

    def table_stage(b, r, sch):
        tail = []
        for g in range(4):
            m1, m32, m512, a0, b0 = [
                (sd[b % 2][r, g, 2 * n], sd[b % 2][r, g, 2 * n + 1]) for n in range(5)]
            m1, m32 = (sch.start(m1[0]), m1[1]), (sch.start(m32[0]), m32[1])
            fa = [a0]
            for _ in range(7):
                fa.append(_cmul(fa[-1], m1))
            for src in (0, 4, 8, 10):
                fa.append(_cmul(fa[src], m512))
            tail.append(fa[11][0] * m512[0] - fa[11][1] * m512[1])
            _store_table(ta[b % 2].at[r, g], fa)
            fb = [b0]
            for _ in range(15):
                p = fb[-1]
                fb.append((p[0] * m32[0] + p[1] * m32[1], p[1] * m32[0] - p[0] * m32[1]))
            _store_table(tb[b % 2].at[r, g], fb)
            yield [tail[-1], fb[-1][0]]
        lo = _iota((8, 128), 0) < 4
        kl[b % 2][r] = _pack(*[jnp.broadcast_to(
            jnp.sum(jnp.where(lo, tail[2 * h], tail[2 * h + 1]), axis=1, keepdims=True),
            (8, 128)) for h in range(2)])

    def kernel_stage(b, r, sch):
        ta_w, tb_w = ta[b % 2].bitcast(I32), tb[b % 2].bitcast(I32)
        groups = [None] * 4
        for g0 in range(2):
            res = [jax.lax.dot_general(sch.lhs(ta_w[r, g, p], g == g0 and p == 0),
                                       _mxu(tb_w[r, g, p]), NT_DIMS, preferred_element_type=F32)
                   for g in (g0, g0 + 2) for p in range(2)]
            groups[g0], groups[g0 + 2] = res[0] + res[1], res[2] + res[3]
            sch.results(groups[g0 + 2])
            yield []
        dskip = [col_v[1, pl.ds(b * MB + 16 * r + h, 8, stride=2), :] for h in range(2)]
        dst = _ds(8 * r, 8)
        res = _k_residues(groups, kl[b % 2][r], dskip)
        for s, t in enumerate(res):
            uk[1][b % 2][s, dst, :] = t
        yield [res[15]]

    def norm_stage(b, r, sch):
        tiles = []
        rows = _ds(b * MB // 2 + 8 * r, 8)
        for j in range(NT):
            m, inv = sch.start(st_v[0, j]), st_v[1, j]
            tiles.append(_pack(*[(v - m) * inv for v in _unpack(x_v.bitcast(I32)[j, rows, :])]))
        dst = _ds(8 * r, 8)
        res = _to_residues(tiles)
        for s, t in enumerate(res):
            uk[0][b % 2][s, dst, :] = t
        yield [res[0]]

    def forward_stage(b, k, sch):
        dst = ab[b % 2]
        for w in range(2):
            rows = slice(w * MB, w * MB + MB)
            for p in range(2):
                v = [jnp.dot(sch.lhs(uk[w][b % 2][k + 4 * n], n == 0),
                             _mxu(ww[w][k + 4 * n, p ^ (n & 1)]),
                             preferred_element_type=F32) for n in range(4)]
                d02, d13 = v[0] - v[2], v[1] - v[3]
                x1 = d02 - d13 if p == 0 else d02 + d13
                dst[k, 0, p, rows] = v[0] + v[2]
                dst[k, 2, 1 - p, rows] = v[1] + v[3]
                dst[k, 1, p, rows] = x1
                dst[k, 3, p, rows] = d02 + d13 if p == 0 else d02 - d13
                sch.results(x1)
                yield []

    def middle_stage(b, r, sch):
        src = ab[b % 2]
        scale = lambda v, f: [(x[0] * f, x[1] * f) for x in v]
        for h in range(2):
            ra = pl.ds(pl.multiple_of(16 * r + 8 * h, 8), 8)
            rb = pl.ds(pl.multiple_of(MB + 16 * r + 8 * h, 8), 8)
            ld = lambda q, rr: [(src[k, q, 0, rr, :], src[k, q, 1, rr, :]) for k in range(4)]

            def put(q, x, y):
                for k in range(4):
                    for p in range(2):
                        cc[b % 2][k, q, p, ra, :] = x[k][p] + y[k][p]
                        cc[b % 2][k, q + 1, p, ra, :] = x[k][p] - y[k][p]

            gate = sch.start
            a0, a2, b0, b2 = ld(0, ra), ld(2, ra), ld(0, rb), ld(2, rb)
            a0[0], b0[0] = (gate(a0[0][0]), gate(a0[0][1])), (gate(b0[0][0]), gate(b0[0][1]))
            e0 = _prod_mod_1(list(map(_cadd, a0, a2)), list(map(_cadd, b0, b2)))
            e2 = _prod_mod_m1(list(map(_csub, a0, a2)), scale(map(_csub, b0, b2), 2.0))
            put(0, e0, e2)
            yield [e0[3][1], e2[3][1]]
            four = sch.start(jnp.full((8, 128), 4.0, F32))
            e1 = _prod_mod_i(ld(1, ra), scale(ld(1, rb), four), 1)
            yield [e1[3][1]]
            four = sch.start(jnp.full((8, 128), 4.0, F32))
            e3 = _prod_mod_i(ld(3, ra), scale(ld(3, rb), four), -1)
            put(2, e1, e3)
            yield [e3[3][1]]

    def inverse_stage(b, k, sch):
        src = cc[b % 2]

        def lhs(v, first):
            return sch.lhs(jnp.concatenate(
                [_pack(v[i:i + 8], v[i + 8:i + 16]) for i in range(0, MB, 16)], axis=0), first)

        for o in range(2):
            p0, p1 = [(src[k, q, 0], src[k, q, 1]) for q in (o, o + 2)]
            if o == 0:
                e = {0: _cadd(p0, p1), 2: _csub(p0, p1)}
            else:
                e = {1: (p0[0] + p1[1], p0[1] - p1[0]), 3: (p0[0] - p1[1], p0[1] + p1[0])}
            ys = []
            for n in e:
                y = [jnp.dot(lhs(e[n][p], n == o and p == 0), _mxu(wt_w[k + 4 * n, p]),
                             preferred_element_type=F32)
                     for p in range(2)]
                ys.append(y[0] + y[1])
                yy[b % 2][k + 4 * n] = ys[-1].astype(BF16)
            sch.results(ys[-1])
            yield []

    def residual_stage(b, r, sch):
        rows = chan(b, r)
        wr = col_v[2, rows, :]
        src = yy[b % 2].bitcast(I32)
        ys = _to_time([src[s, _ds(8 * r, 8), :] for s in range(16)])
        for j in range(NT):
            h = x_v[j, rows, :].astype(F32) + jnp.concatenate(_unpack(sch.start(ys[j])), axis=0)
            h_v[j, rows, :] = h.astype(BF16)
            hh, hw = h * h, h * wr
            acc_v[0, j] += h[0:8] + h[8:16]
            acc_v[1, j] += hh[0:8] + hh[8:16]
            acc_v[2, j] += hw[0:8] + hw[8:16]
            if j % 8 == 7:
                yield [hw[8:16]]

    nb = D // MB
    stages = dict(s=(seed_stage, 0), t=(table_stage, 1), k=(kernel_stage, 2),
                  n=(norm_stage, 2), f=(forward_stage, 3), m=(middle_stage, 4),
                  i=(inverse_stage, 5), r=(residual_stage, 6))

    def run(step, skip=""):
        def body(r, carry):
            sch = _Schedule(r)
            live = {n: f(step - lag, r, sch) for n, (f, lag) in stages.items()
                    if 0 <= step - lag < nb and n not in skip}
            for n, wait, before in PLAN:
                if n in live:
                    sch.run(live[n], wait, before)
            for g in live.values():
                for _ in g:
                    pass
            return carry

        with jax.named_scope("S_p%d" % step):
            jax.lax.fori_loop(0, 4, body, 0)

    run(0)
    run(1)
    run(2, "n")

    with jax.named_scope("S_xwait"):
        for cp in cp_x + cp_par[1]:
            cp.wait()
    for j in range(NT):
        xs = x_v[j].astype(F32)
        m, inv = _ln_scalars(jnp.sum(xs, axis=0, keepdims=True),
                             jnp.sum(xs * xs, axis=0, keepdims=True))
        st_v[0, j] = jnp.broadcast_to(m, (8, 128))
        st_v[1, j] = jnp.broadcast_to(inv, (8, 128))
    acc_v[...] = jnp.zeros(acc_v.shape, F32)
    for r in range(4):
        next(norm_stage(0, r, _Schedule(r)))

    for step in STEPS:
        run(step)

    def rows_of(q):
        return jnp.concatenate(
            [jnp.sum(acc_v[q, j], axis=0, keepdims=True) for j in range(NT)], axis=0)

    m2, inv2 = _ln_scalars(rows_of(0), rows_of(1))
    wsum = jnp.sum(col_v[2], axis=0, keepdims=True)
    score = _rbf((rows_of(2) - m2 * wsum) * inv2 + 0.0)
    bits = pltpu.bitcast(score, I32) >> 16
    order = jnp.where(bits < 0, -1 - bits, bits + 32768)
    pos = 128 * _iota((NT, 128), 0) + _iota((NT, 128), 1)
    key = pltpu.bitcast((order << 11) + (L - 1 - pos) + (1 << 29), F32)

    for j in range(NT):
        st_v[0, j] = jnp.broadcast_to(m2[j:j + 1], (8, 128))
        st_v[1, j] = jnp.broadcast_to(inv2[j:j + 1], (8, 128))

    sub8 = _iota((CAP, 128), 0)

    def pick(c, carry):
        key, aux = carry
        top = jnp.max(key, axis=(0, 1), keepdims=True)
        hit = key == top
        pick_s[c] = pltpu.bitcast(jnp.broadcast_to(top, (8, 128)), I32)[0, 0]
        vals = [jnp.sum(jnp.where(hit, v, 0.0), axis=0, keepdims=True) for v in (m2, inv2, score)]
        for j in (2 * c, 2 * c + 1):
            m, inv = jnp.tile(st_v[0, j], (2, 1)), jnp.tile(st_v[1, j], (2, 1))
            for i in range(0, D, 16):
                h = h_v[j, i:i + 16, :].astype(F32)
                out_v[j, i:i + 16, :] = (h + (h - m) * inv).astype(BF16)
        return (jnp.where(hit, 0.0, key),
                [jnp.where(sub8 == c, v, a) for v, a in zip(vals, aux)])

    with jax.named_scope("S_top"):
        _, aux = jax.lax.fori_loop(0, CAP, pick, (key, [jnp.zeros((CAP, 128), F32)] * 3))
    picks = [L - 1 - (pick_s[c] & (L - 1)) for c in range(CAP)]
    picks = [(t >> 7, t & 127) for t in picks]

    def out_copy(j, lo, hi, n):
        cols = pl.ds(j * 128 if isinstance(j, int) else pl.multiple_of(j * 128, 128), 128)
        return pltpu.make_async_copy(out_v.at[j, lo:hi], out_hbm.at[lo:hi, cols], sem_o.at[n])

    routed = functools.reduce(jnp.bitwise_or, [1 << j for j, _ in picks])
    first, seen = [], 0
    for j, _ in picks:
        first.append(((seen >> j) & 1) == 0)
        seen = seen | (1 << j)
    for j in range(NT):
        pl.when(((routed >> j) & 1) == 0)(out_copy(j, 0, D, j).start)

    lane16, sub16 = _iota((16, 128), 1), _iota((16, 128), 0)
    h_sel = sum(jax.lax.dot_general(
        jnp.where((sub16 == c) & (lane16 == i), 1.0, 0.0).astype(BF16),
        _mxu(h_v.bitcast(I32)[j]), NT_DIMS, preferred_element_type=F32)[0:CAP]
        for c, (j, i) in enumerate(picks))
    m_sel, inv_sel, score_sel = [jnp.sum(a, axis=1, keepdims=True) for a in aux]
    x_sel = _rbf((h_sel - m_sel) * inv_sel)
    gate = _rbf(jax.nn.sigmoid(score_sel))
    xb = x_sel.astype(BF16)
    with jax.named_scope("S_gwait"):
        cp_w[0].wait()
        cp_w[1].wait()
    g = _rbf(jnp.dot(xb, wg_v[...], preferred_element_type=F32))
    up = _rbf(jnp.dot(xb, wu_v[...], preferred_element_type=F32))
    act = (_rbf(g * jax.nn.sigmoid(g)) * up).astype(BF16)
    with jax.named_scope("S_dwait"):
        cp_w[2].wait()
    out_w = out_v.bitcast(I32)
    for n, (lo, hi) in enumerate(ROW_CHUNKS):
        y = _rbf(jax.lax.dot_general(act, wd_v[lo:hi, :], NT_DIMS, preferred_element_type=F32))
        new = h_sel[:, lo:hi] + _rbf(x_sel[:, lo:hi] + _rbf(y * gate))
        new = jnp.concatenate([new, jnp.zeros((128 - CAP, hi - lo), F32)], axis=0).T
        new = pltpu.bitcast(new.astype(BF16), I32)
        lane = _iota(new.shape, 1)
        for c, (j, i) in enumerate(picks):
            out_w[j, lo // 2:hi // 2, :] = jnp.where(
                lane == i, pltpu.roll(new, (128 + i - c) & 127, 1), out_w[j, lo // 2:hi // 2, :])
        for c, (j, _) in enumerate(picks):
            pl.when(first[c])(out_copy(j, lo, hi, NT + CAP * n + c).start)
    with jax.named_scope("S_owait"):
        for j in range(NT):
            pl.when(((routed >> j) & 1) == 0)(out_copy(j, 0, D, j).wait)
        for n, (lo, hi) in enumerate(ROW_CHUNKS):
            for c, (j, _) in enumerate(picks):
                pl.when(first[c])(out_copy(j, lo, hi, NT + CAP * n + c).wait)


@jax.jit
def pallas_sequential_preLN__ssm_conv_s4__moe_arch_mod__prompt_kernel(
    A_u: jax.Array,
    A_A_re: jax.Array,
    A_A_im: jax.Array,
    A_B_re: jax.Array,
    A_B_im: jax.Array,
    A_C_re: jax.Array,
    A_C_im: jax.Array,
    A_log_dt: jax.Array,
    A_Dskip: jax.Array,
    B_x: jax.Array,
    B_w_r: jax.Array,
    B_w_gate: jax.Array,
    B_w_up: jax.Array,
    B_w_down: jax.Array,
):
    del B_x
    hbm = pl.BlockSpec(memory_space=pl.ANY)
    out = pl.pallas_call(
        _kernel,
        out_shape=jax.ShapeDtypeStruct((D, L), BF16),
        in_specs=[hbm] * 13,
        out_specs=hbm,
        scratch_shapes=[
            pltpu.VMEM((NT, D, 128), BF16),
            pltpu.VMEM((D, FF), BF16),
            pltpu.VMEM((D, FF), BF16),
            pltpu.VMEM((D, FF), BF16),
            pltpu.VMEM((6, D, N), BF16),
            *[pltpu.VMEM((D,), BF16)] * 3,
            *[pltpu.VMEM((16, 2, 128, 128), BF16)] * 2,
            pltpu.VMEM((16, 2, 64, 128), I32),
            pltpu.VMEM((3, D, 128), F32),
            pltpu.VMEM((2, 256, 128), F32),
            pltpu.VMEM((NT, D, 128), BF16),
            pltpu.VMEM((2, NT, 8, 128), F32),
            pltpu.VMEM((3, NT, 8, 128), F32),
            pltpu.VMEM((NT, D, 128), BF16),
            *[pltpu.VMEM((4, 4, 10, 8, 128), F32)] * 2,
            *[pltpu.VMEM((4, 4, 2, 96, 128), BF16)] * 2,
            *[pltpu.VMEM((4, 4, 2, 128, 128), BF16)] * 2,
            *[pltpu.VMEM((4, 8, 128), I32)] * 2,
            *[pltpu.VMEM((16, MB // 2, 128), I32)] * 4,
            *[pltpu.VMEM((4, 4, 2, 2 * MB, 128), F32)] * 2,
            *[pltpu.VMEM((4, 4, 2, MB, 128), F32)] * 2,
            *[pltpu.VMEM((16, MB, 128), BF16)] * 2,
            pltpu.SMEM((CAP,), I32),
            pltpu.SemaphoreType.DMA((15,)),
            pltpu.SemaphoreType.DMA((NT,)),
            pltpu.SemaphoreType.DMA((3,)),
            pltpu.SemaphoreType.DMA((NT + CAP * len(ROW_CHUNKS),)),
        ],
        compiler_params=pltpu.CompilerParams(vmem_limit_bytes=100 * 1024 * 1024),
    )(A_u.reshape(L, D).T, A_A_re, A_A_im, A_B_re, A_B_im, A_C_re, A_C_im,
      A_log_dt, A_Dskip, B_w_r, B_w_gate, B_w_up, B_w_down.T)
    return out.T.reshape(1, L, D)
```

```python
import functools

import numpy as np
import jax
import jax.numpy as jnp
import jax.experimental.pallas as pl
import jax.experimental.pallas.tpu as pltpu

F32 = jnp.float32
BF16 = jnp.bfloat16
I32 = jnp.int32

L = 2048
D = 576
N = 128
FF = 4608
CAP = 8
NT = L // 128
EPS = 1e-5
MB = 64
import os
STEPS = eval(os.environ["ONE"]) if os.environ.get("ONE") else range(3, D // MB + 6)
PLANS = dict(
    default="",
    stknfmir="t-1:3,t-1:3,m-1:6,n-1:9,s-1:28,f,s1:35,k,m4:16,r9:20,k,m13:25,k-1:30,f,t16:30,t14:33,f,f,r25:-1,i,i,m32:-1",
    tknfmir="t-1:3,t-1:3,m-1:6,n-1:8,f,k,m4:16,r9:20,k,m13:25,k-1:30,f,t16:30,t16:33,f,f,r25:-1,i,i,m32:-1",
    knfmir="m-1:7,f,n0:10,m2:20,f,k,m10:22,k,r15:27,m15:35,k-1:-1,f,f,i,r29:-1,i",
    fmir="m-1:6,m-1:9,f,f,m4:18,m5:23,f,f,i,r16:-1,r17:-1,i",
    mir="m-1:1,m-1:3,r-1:-1,r-1:-1,i,m0:-1,m2:-1,i",
    stknfmi="t-1:3,t-1:3,m-1:6,n-1:9,s-1:32,f,s0:31,k,m6:17,k,m13:25,k-1:30,f,t16:30,t14:33,f,f,i,i,m32:-1",
    stknfm="m-1:3,t-1:7,t-1:13,t-1:9,s-1:-1,s-1:-1,f,m1:16,f,m6:18,k,t9:22,k,m14:-1,n17:-1,k-1:-1,f,f",
    stknf="n-1:10,t-1:6,s-1:17,s-1:27,f,t3:19,k,k,t13:-1,k-1:-1,f,f,t21:-1,f",
    stk="t-1:2,t-1:7,t-1:8,k,s0:-1,t2:-1,s-1:-1,k,k-1:-1",
)
if os.environ.get("PLAN"):
    PLANS = dict(default=os.environ["PLAN"])
ROW_CHUNKS = ((0, 128), (128, 256), (256, 384), (384, 512), (512, D))
NT_DIMS = (((1,), (1,)), ((), ()))


def _round_res(step):
    return [int(np.round(r / step)) * step for r in range(16)]


RES1, RES2, RES3 = _round_res(2), _round_res(4), _round_res(8)


def _ds(start, size):
    return pl.ds(start if isinstance(start, int) else pl.multiple_of(start, size), size)


def _iota(shape, dim):
    return jax.lax.broadcasted_iota(I32, shape, dim)


def _rbf(x):
    return x.astype(BF16).astype(F32)


def _cmul(a, b):
    return (a[0] * b[0] - a[1] * b[1], a[0] * b[1] + a[1] * b[0])


def _csq(a):
    t = a[0] * a[1]
    return ((a[0] + a[1]) * (a[0] - a[1]), t + t)


def _cadd(a, b):
    return (a[0] + b[0], a[1] + b[1])


def _csub(a, b):
    return (a[0] - b[0], a[1] - b[1])


def _bfly4(a0, a1, a2, a3, inverse=False):
    s02, d02 = _cadd(a0, a2), _csub(a0, a2)
    s13, d13 = _cadd(a1, a3), _csub(a1, a3)
    p = (d02[0] - d13[1], d02[1] + d13[0])
    m = (d02[0] + d13[1], d02[1] - d13[0])
    if inverse:
        p, m = m, p
    return _cadd(s02, s13), p, _csub(s02, s13), m


def _prod_mod_1(a, b):
    fa, fb = _bfly4(*a), _bfly4(*b)
    return _bfly4(*[_cmul(x, y) for x, y in zip(fa, fb)], inverse=True)


def _prod2(a0, a1, b0, b1, sgn):
    p00, p11 = _cmul(a0, b0), _cmul(a1, b1)
    c1 = _cadd(_cmul(a0, b1), _cmul(a1, b0))
    if sgn > 0:
        return (p00[0] - p11[1], p00[1] + p11[0]), c1
    return (p00[0] + p11[1], p00[1] - p11[0]), c1


def _prod_mod_m1(a, b):
    def split(x):
        p = [(x[k][0] - x[k + 2][1], x[k][1] + x[k + 2][0]) for k in range(2)]
        m = [(x[k][0] + x[k + 2][1], x[k][1] - x[k + 2][0]) for k in range(2)]
        return p, m
    ap, am = split(a)
    bp, bm = split(b)
    cp = _prod2(*ap, *bp, 1)
    cm = _prod2(*am, *bm, -1)
    lo = [_cadd(cp[k], cm[k]) for k in range(2)]
    hi = [(cp[k][1] - cm[k][1], cm[k][0] - cp[k][0]) for k in range(2)]
    return lo + hi


def _prod_mod_i(a, b, sgn):
    sm = [x[0] + x[1] for x in b]
    df = [x[1] - x[0] for x in b]
    asum = [x[0] + x[1] for x in a]
    out = []
    for k in range(4):
        acc = [None, None, None]
        for j in range(4):
            m = (k - j) % 4
            if j <= k:
                t = ((b[m][0], 1), (df[m], 1), (sm[m], 1))
            elif sgn > 0:
                t = ((b[m][1], -1), (sm[m], 1), (df[m], -1))
            else:
                t = ((b[m][1], 1), (sm[m], -1), (df[m], 1))
            for q, (v, (w, s)) in enumerate(zip((asum[j], a[j][0], a[j][1]), t)):
                p = v * w
                if acc[q] is None:
                    acc[q] = p
                else:
                    acc[q] = acc[q] + p if s > 0 else acc[q] - p
        out.append((acc[0] - acc[2], acc[0] + acc[1]))
    return out


def _barrel(v):
    lane = _iota((8, 128), 1)
    for bit in range(4):
        m = ((lane >> bit) & 1) == 1
        v = [jnp.where(m, v[(i + (1 << bit)) % 16], v[i]) for i in range(16)]
    return [v[-s % 16] for s in range(16)]


def _to_residues(tiles):
    return _barrel([t if j == 0 else pltpu.roll(t, j, 1) for j, t in enumerate(tiles)])


def _to_time(res):
    return [t if j == 0 else pltpu.roll(t, 128 - j, 1) for j, t in enumerate(_barrel(res))]


def _gather(x, idx):
    return jnp.take_along_axis(x, idx, axis=1, mode="promise_in_bounds")


def _init_dft(wu_ref, wk_ref, wt_ref, tmp_ref):
    sub, k4 = _iota((8, 128), 0), 4 * _iota((8, 128), 1) + 1

    def cis(t):
        ph = ((k4 * t) & (4 * L - 1)).astype(F32) * (2 * np.pi / (4 * L))
        return jnp.cos(ph), jnp.sin(ph)

    w1, w16 = cis(1), cis(16)
    w32 = _csq(w16)
    fk = [cis(16 * (32 * (sub & 3) + (sub >> 2)))]
    fu = [cis(128 * sub), cis(128 * (sub + 8))]
    for v in range(1, 16):
        fk.append(_cmul(fk[-1], w32))
        if v >= 2:
            fu.append(_cmul(fu[-2], w16))
    for p in range(2):
        for v in range(32):
            tmp_ref[p, 8 * v:8 * v + 8, :] = fu[v % 16][p]
    tw = None
    for s in range(16):
        for v in range(0, 16, 2):
            rows = [slice(128 - s + 8 * i, 136 - s + 8 * i) for i in (v, v + 1)]
            for ref, f in ((wk_ref, fk[v:v + 2]),
                           (wu_ref, [(tmp_ref[0, r, :], tmp_ref[1, r, :]) for r in rows])):
                if s:
                    f = [_cmul(x, tw) for x in f]
                for p in range(2):
                    ref[s, p, 8 * v:8 * v + 16, :] = jnp.concatenate(
                        [f[0][p], f[1][p]], axis=0).astype(BF16)
        for p in range(2):
            wt_ref[s, p] = pltpu.bitcast(_mxu(wu_ref.bitcast(I32)[s, p]).T, I32)
        tw = _cmul(tw, w1) if s else w1


def _pack(a, b):
    return pltpu.pack_elementwise([a, b], packed_dtype=BF16)


def _unpack(w):
    return [pltpu.unpack_elementwise(w, index=i, packed_dtype=BF16, unpacked_dtype=F32)
            for i in range(2)]


FINE = (0, 1, 2, 3, 4, 5, 6, 7, 512, 516, 1024, 1536)


def _k_seeds(z, c):
    lo = _iota((8, 128), 0) < 4
    pw = {1: z}
    for e in range(1, 10):
        pw[1 << e] = _csq(pw[1 << (e - 1)])
    rot = lambda v: tuple(pltpu.roll(x, 4, 0) for x in v)
    sel = lambda a, b: tuple(jnp.where(lo, p, q) for p, q in zip(a, b))
    z16 = (pw[16][0], 0.0 - pw[16][1])
    pairs = [(z, rot(z)), (pw[32], rot(pw[32])), (pw[512], rot(pw[512])),
             (c, rot(_cmul(c, pw[8])))]
    return [[sel(a, b) for a, b in pairs] + [sel((1.0, 0.0), rot(z16))],
            [sel(b, a) for a, b in pairs] + [sel((1.0, 0.0), z16)]]


def _mxu(words):
    return pltpu.bitcast(words, BF16)


def _store_table(ref, tab):
    for i in range(0, len(tab), 2):
        for p in range(2):
            ref[p, 8 * i:8 * i + 16, :] = jnp.concatenate(
                [tab[i][p], tab[i + 1][p]], axis=0).astype(BF16)


def _k_residues(groups, k_last, dskip):
    sub = _iota((8, 128), 0)
    lane = _iota((8, 128), 1)
    lo = sub < 4
    idx = (lane & ~3) | (sub & 3)
    nxt = ((idx + 4) & 127)
    kv, up = {}, {}
    for i, k in enumerate(FINE):
        v = [g[8 * i:8 * i + 8] for g in groups]
        if k == 0:
            v = [x + jnp.where((lane < 4) & (lo if n % 2 == 0 else ~lo),
                               dskip[n // 2], 0.0)
                 for n, x in enumerate(v)]
        p = [_pack(v[g], v[2 + g]) for g in range(2)]
        even = jnp.where(lo, p[0], p[1])
        kv[k] = _gather(even, idx)
        kv[k + 8] = _gather(pltpu.roll(jnp.where(lo, p[1], p[0]), 4, 0), idx)
        if k % 512 == 0:
            up[k] = _gather(even, nxt)
    q = lane & 3
    s3 = {r: jnp.where(q == 2, kv[1024 + r], kv[1536 + r]) for r in (0, 8)}
    v0 = jnp.where(q == 0, kv[0], jnp.where(q == 1, kv[512], s3[0]))
    q16 = q + jnp.where(lane >= 124, 1, 0)
    v16 = jnp.where(q16 < 2, jnp.where(q16 == 0, up[0], up[512]),
                    jnp.where(q16 == 2, up[1024], jnp.where(q16 == 3, up[1536], k_last)))
    s3[16] = v16
    s23, s123, out = {}, {}, [v0]
    for r in range(1, 16):
        k23 = (RES2[r], RES3[r])
        if k23 not in s23:
            s23[k23] = v16 if k23 == (16, 16) else jnp.where(q == 1, kv[512 + k23[0]], s3[k23[1]])
        k123 = (RES1[r],) + k23
        if k123 not in s123:
            s123[k123] = v16 if k123[0] == 16 else jnp.where(q == 0, kv[k123[0]], s23[k23])
        if RES1[r] == r:
            out.append(s123[k123])
        else:
            out.append(jnp.where((q == 0) & (lane < 64), kv[r], s123[k123]))
    return out


def _ln_scalars(s1, s2):
    mean = s1 * (1.0 / D)
    var = jnp.maximum(s2 * (1.0 / D) - mean * mean, 0.0)
    eps = float(np.asarray(EPS, dtype=BF16))
    sd = _rbf(jnp.sqrt(_rbf(_rbf(var) + eps)))
    return _rbf(mean), 1.0 / sd


def _top8(x):
    def swap(v, pairs):
        for i, j in pairs:
            v[i], v[j] = jnp.maximum(v[i], v[j]), jnp.minimum(v[i], v[j])
        return v

    def merge(a, b):
        v = [jnp.maximum(a[i], b[7 - i]) for i in range(8)]
        return swap(v, [(i, i + d) for d in (4, 2, 1) for i in range(8) if not i & d])

    sort8 = ((0, 2), (1, 3), (4, 6), (5, 7), (0, 4), (1, 5), (2, 6), (3, 7), (0, 1), (2, 3),
             (4, 5), (6, 7), (2, 4), (3, 5), (1, 4), (3, 6), (1, 2), (3, 4), (5, 6))
    v = merge(*[swap([x[64 * h + 8 * i:64 * h + 8 * i + 8] for i in range(8)], sort8)
                for h in range(2)])
    for d in (4, 2, 1):
        v = merge(v, [pltpu.roll(t, d, 0) for t in v])
    return v


def _column(vec):
    row = vec.astype(F32).reshape(1, D)
    parts = []
    for lo in range(0, D, 128):
        start = min(lo, D - 128)
        t = jnp.broadcast_to(row[:, start:start + 128], (128, 128)).T
        parts.append(t[lo - start:])
    return jnp.concatenate(parts, axis=0)


class _Schedule:
    def __init__(self, r):
        self.true = _iota((8, 128), 0) + r >= 0
        self.done, self.pending, self.wait = [], {}, -1
        self.r = (r | 64) & 63

    def tie(self, x, token):
        return jnp.where(self.true, x, token if token.dtype == x.dtype
                         else pltpu.bitcast(token, x.dtype))

    def start(self, x):
        return self.tie(x, self.done[self.wait]) if 0 <= self.wait < len(self.done) else x

    def lhs(self, words, first):
        tiles = [words[i:i + 8] for i in range(0, words.shape[0], 8)]
        for i in range(len(tiles) if first else 0):
            for token in self.pending.pop(len(self.done) + i, ()):
                tiles[i] = self.tie(tiles[i], token)
        return _mxu(jnp.concatenate(tiles, axis=0))

    def results(self, v):
        self.done += [v[i + 8:i + 16] for i in range(0, v.shape[0], 16)]

    def run(self, stage, wait, before):
        self.wait = wait
        self.pending.setdefault(before, []).extend(next(stage))


def _kernel(x_hbm, are_hbm, aim_hbm, bre_hbm, bim_hbm, cre_hbm, cim_hbm,
            ldt_hbm, dsk_hbm, wr_hbm, wg_hbm, wu_hbm, wd_hbm, out_hbm,
            x_v, wg_v, wu_v, wd_v, par_v, ldt_v, dsk_v, wr_v, w_v, wk_v, wt_v, col_v,
            tmp_v, xf_v, h_v, st_v, acc_v, out_v, sd0, sd1, ta0, ta1, tb0, tb1, kl0, kl1,
            u0, u1, k0, k1, ab0, ab1, c0, c1, y0, y1, new_v, order_s, sem_p, sem_x, sem_w, sem_o):
    cp_vec = [pltpu.make_async_copy(s, d, sem_p.at[n]) for n, (s, d) in enumerate(
        ((ldt_hbm, ldt_v), (dsk_hbm, dsk_v), (wr_hbm, wr_v)))]
    cp_par = [[pltpu.make_async_copy(s.at[lo:hi], par_v.at[n, lo:hi], sem_p.at[3 + 6 * m + n])
               for n, s in enumerate((are_hbm, aim_hbm, bre_hbm, bim_hbm, cre_hbm, cim_hbm))]
              for m, (lo, hi) in enumerate(((0, 3 * MB), (3 * MB, D)))]
    cp_x = [pltpu.make_async_copy(x_hbm.at[:, 128 * j:128 * j + 128], x_v.at[j], sem_x.at[j])
            for j in range(NT)]
    cp_w = [pltpu.make_async_copy(s, d, sem_w.at[n]) for n, (s, d) in enumerate(
        ((wg_hbm, wg_v), (wu_hbm, wu_v), (wd_hbm, wd_v)))]
    for cp in cp_vec + cp_par[0]:
        cp.start()
    for cp in cp_x:
        cp.start(priority=1)

    with jax.named_scope("S_dft"):
        _init_dft(w_v, wk_v, wt_v, tmp_v)
    for cp in cp_vec:
        cp.wait()
    col_v[0] = _rbf(jnp.exp(_column(ldt_v[...])))
    col_v[1] = _column(dsk_v[...]) * (1.0 / L)
    col_v[2] = _column(wr_v[...])
    with jax.named_scope("S_pwait"):
        for cp in cp_par[0]:
            cp.wait()

    sd, ta, tb, kl = (sd0, sd1), (ta0, ta1), (tb0, tb1), (kl0, kl1)
    uk, ab, cc, yy = ((u0, u1), (k0, k1)), (ab0, ab1), (c0, c1), (y0, y1)
    ww, wt_w = (w_v.bitcast(I32), wk_v.bitcast(I32)), wt_v

    def chan(b, r):
        return pl.ds(pl.multiple_of(b * MB + 16 * r, 16), 16)

    def seed_stage(b, r, sch):
        rows = _ds(b * MB // 2 + 8 * r, 8)
        par = [_unpack(par_v.bitcast(I32)[n, rows, :]) for n in range(6)]
        for h in range(2):
            a_re, a_im, b_re, b_im, c_re, c_im = [v[h] for v in par]
            dt = sch.start(col_v[0, pl.ds(b * MB + 16 * r + h, 8, stride=2), :])
            mag, ang = jnp.exp(dt * a_re), dt * a_im
            sc = dt * (1.0 / L)
            seeds = _k_seeds((mag * jnp.cos(ang), mag * jnp.sin(ang)),
                             _cmul((c_re, c_im), (sc * b_re, sc * b_im)))
            for g in range(2):
                for n, v in enumerate(seeds[g]):
                    for p in range(2):
                        sd[b % 2][r, 2 * h + g, 2 * n + p] = v[p]
            yield [sd[b % 2][sch.r, 2 * h, 0]]

    def table_stage(b, r, sch):
        tail = []
        for g in range(4):
            m1, m32, m512, a0, b0 = [
                (sd[b % 2][r, g, 2 * n], sd[b % 2][r, g, 2 * n + 1]) for n in range(5)]
            m32 = (sch.start(m32[0]), m32[1])
            fa = [a0]
            for _ in range(7):
                fa.append(_cmul(fa[-1], m1))
            for src in (0, 4, 8, 10):
                fa.append(_cmul(fa[src], m512))
            tail.append(fa[11][0] * m512[0] - fa[11][1] * m512[1])
            _store_table(ta[b % 2].at[r, g], fa)
            fb = [b0]
            for _ in range(15):
                p = fb[-1]
                fb.append((p[0] * m32[0] + p[1] * m32[1], p[1] * m32[0] - p[0] * m32[1]))
            _store_table(tb[b % 2].at[r, g], fb)
            yield [ta[b % 2].bitcast(I32)[sch.r, g, 0, 0:8, :],
                   tb[b % 2].bitcast(I32)[sch.r, g, 0, 0:8, :]]
        lo = _iota((8, 128), 0) < 4
        kl[b % 2][r] = _pack(*[jnp.broadcast_to(
            jnp.sum(jnp.where(lo, tail[2 * h], tail[2 * h + 1]), axis=1, keepdims=True),
            (8, 128)) for h in range(2)])

    def kernel_stage(b, r, sch):
        ta_w, tb_w = ta[b % 2].bitcast(I32), tb[b % 2].bitcast(I32)
        groups = [None] * 4
        for g0 in range(2):
            res = [jax.lax.dot_general(sch.lhs(ta_w[r, g, p], g == g0 and p == 0),
                                       _mxu(tb_w[r, g, p]), NT_DIMS, preferred_element_type=F32)
                   for g in (g0, g0 + 2) for p in range(2)]
            groups[g0], groups[g0 + 2] = res[0] + res[1], res[2] + res[3]
            sch.results(groups[g0 + 2])
            yield []
        dskip = [col_v[1, pl.ds(b * MB + 16 * r + h, 8, stride=2), :] for h in range(2)]
        dst = _ds(8 * r, 8)
        res = _k_residues(groups, kl[b % 2][r], dskip)
        for s, t in enumerate(res):
            uk[1][b % 2][s, dst, :] = t
        yield [uk[1][b % 2][0, _ds(8 * sch.r, 8), :]]

    def norm_stage(b, r, sch):
        tiles = []
        for j in range(NT):
            m, inv = st_v[0, j] if j else sch.start(st_v[0, j]), st_v[1, j]
            tiles.append(_pack(*[
                (xf_v[j, pl.ds(b * MB + 16 * r + h, 8, stride=2), :] - m) * inv for h in range(2)]))
        dst = _ds(8 * r, 8)
        res = _to_residues(tiles)
        for s, t in enumerate(res):
            uk[0][b % 2][s, dst, :] = t
        yield [uk[0][b % 2][0, _ds(8 * sch.r, 8), :]]

    def forward_stage(b, k, sch):
        dst = ab[b % 2]
        for w in range(2):
            rows = slice(w * MB, w * MB + MB)
            for p in range(2):
                v = [jnp.dot(sch.lhs(uk[w][b % 2][k + 4 * n], n == 0),
                             _mxu(ww[w][k + 4 * n, p ^ (n & 1)]),
                             preferred_element_type=F32) for n in range(4)]
                d02, d13 = v[0] - v[2], v[1] - v[3]
                x1 = d02 - d13 if p == 0 else d02 + d13
                dst[k, 0, p, rows] = v[0] + v[2]
                dst[k, 2, 1 - p, rows] = v[1] + v[3]
                dst[k, 1, p, rows] = x1
                dst[k, 3, p, rows] = d02 + d13 if p == 0 else d02 - d13
                sch.results(x1)
                yield []

    def middle_stage(b, r, sch):
        src = ab[b % 2]
        scale = lambda v, f: [(x[0] * f, x[1] * f) for x in v]
        for h in range(2):
            ra = pl.ds(pl.multiple_of(16 * r + 8 * h, 8), 8)
            rb = pl.ds(pl.multiple_of(MB + 16 * r + 8 * h, 8), 8)
            ld = lambda q, rr: [(src[k, q, 0, rr, :], src[k, q, 1, rr, :]) for k in range(4)]

            def put(q, x, y):
                for k in range(4):
                    for p in range(2):
                        cc[b % 2][k, q, p, ra, :] = x[k][p] + y[k][p]
                        cc[b % 2][k, q + 1, p, ra, :] = x[k][p] - y[k][p]

            gate = sch.start
            a0, a2, b0, b2 = ld(0, ra), ld(2, ra), ld(0, rb), ld(2, rb)
            a0[0] = (gate(a0[0][0]), a0[0][1])
            e0 = _prod_mod_1(list(map(_cadd, a0, a2)), list(map(_cadd, b0, b2)))
            e2 = _prod_mod_m1(list(map(_csub, a0, a2)), scale(map(_csub, b0, b2), 2.0))
            put(0, e0, e2)
            again = _ds(16 * sch.r + 8 * h, 8)
            yield [cc[b % 2][0, 0, 0, again, :]]
            four = sch.start(jnp.full((8, 128), 4.0, F32))
            e1 = _prod_mod_i(ld(1, ra), scale(ld(1, rb), four), 1)
            e3 = _prod_mod_i(ld(3, ra), scale(ld(3, rb), four), -1)
            put(2, e1, e3)
            yield [cc[b % 2][0, 2, 0, again, :]]

    def inverse_stage(b, k, sch):
        src = cc[b % 2]

        def lhs(v, first):
            return sch.lhs(jnp.concatenate(
                [_pack(v[i:i + 8], v[i + 8:i + 16]) for i in range(0, MB, 16)], axis=0), first)

        for o in range(2):
            p0, p1 = [(src[k, q, 0], src[k, q, 1]) for q in (o, o + 2)]
            if o == 0:
                e = {0: _cadd(p0, p1), 2: _csub(p0, p1)}
            else:
                e = {1: (p0[0] + p1[1], p0[1] - p1[0]), 3: (p0[0] - p1[1], p0[1] + p1[0])}
            ys = []
            for n in e:
                y = [jnp.dot(lhs(e[n][p], n == o and p == 0), _mxu(wt_w[k + 4 * n, p]),
                             preferred_element_type=F32)
                     for p in range(2)]
                ys.append(y[0] + y[1])
                yy[b % 2][k + 4 * n] = ys[-1].astype(BF16)
            sch.results(ys[-1])
            yield []

    def residual_stage(b, r, sch):
        rows = chan(b, r)
        wr = col_v[2, rows, :]
        src = yy[b % 2].bitcast(I32)
        ys = _to_time([src[s, _ds(8 * r, 8), :] for s in range(16)])
        for j in range(NT):
            h = xf_v[j, rows, :] + jnp.concatenate(
                _unpack(ys[j] if j % 8 else sch.start(ys[j])), axis=0)
            h_v[j, rows, :] = h.astype(BF16)
            hh, hw = h * h, h * wr
            acc_v[0, j] += h[0:8] + h[8:16]
            acc_v[1, j] += hh[0:8] + hh[8:16]
            acc_v[2, j] += hw[0:8] + hw[8:16]
            if j % 8 == 7:
                yield [acc_v[0, sch.r]]

    nb = D // MB
    stages = dict(s=(seed_stage, 0), t=(table_stage, 1), k=(kernel_stage, 2),
                  n=(norm_stage, 2), f=(forward_stage, 3), m=(middle_stage, 4),
                  i=(inverse_stage, 5), r=(residual_stage, 6))

    def run(step, skip=""):
        def body(r, carry):
            sch = _Schedule(r)
            live = {n: f(step - lag, r, sch) for n, (f, lag) in stages.items()
                    if 0 <= step - lag < nb and n not in skip}
            for item in PLANS.get("".join(live), PLANS["default"]).split(","):
                if item and item[0] in live:
                    sch.run(live[item[0]], *map(int, (item[1:] or "-1:-1").split(":")))
            for g in live.values():
                for _ in g:
                    pass
            return carry

        with jax.named_scope("S_p%d" % step):
            jax.lax.fori_loop(0, 4, body, 0)

    run(0)
    run(1)
    for cp in cp_par[1]:
        cp.start()
    for cp in cp_w:
        cp.start(priority=1)
    run(2, "n")

    with jax.named_scope("S_xwait"):
        for cp in cp_x + cp_par[1]:
            cp.wait()
    for j in range(NT):
        xs = x_v[j].astype(F32)
        xf_v[j] = xs
        m, inv = _ln_scalars(jnp.sum(xs, axis=0, keepdims=True),
                             jnp.sum(xs * xs, axis=0, keepdims=True))
        st_v[0, j] = jnp.broadcast_to(m, (8, 128))
        st_v[1, j] = jnp.broadcast_to(inv, (8, 128))
    acc_v[...] = jnp.zeros(acc_v.shape, F32)
    for r in range(4):
        next(norm_stage(0, r, _Schedule(r)))

    for step in STEPS:
        run(step)

    def rows_of(q):
        return jnp.concatenate(
            [jnp.sum(acc_v[q, j], axis=0, keepdims=True) for j in range(NT)], axis=0)

    m2, inv2 = _ln_scalars(rows_of(0), rows_of(1))
    wsum = jnp.sum(col_v[2], axis=0, keepdims=True)
    score = _rbf((rows_of(2) - m2 * wsum) * inv2 + 0.0)
    bits = pltpu.bitcast(score, I32) >> 16
    order = jnp.where(bits < 0, -1 - bits, bits + 32768)
    pos = 128 * _iota((NT, 128), 0) + _iota((NT, 128), 1)
    key = pltpu.bitcast((order << 11) + (L - 1 - pos) + (1 << 29), F32)

    lane8, sub8 = _iota((CAP, 128), 1), _iota((CAP, 128), 0)
    best = _top8(jnp.tile(key, (8, 1)).T)
    cand = best[0]
    for c in range(1, CAP):
        cand = jnp.where((lane8 >> 4) == c, best[c], cand)
    best = [pltpu.bitcast(v, I32)[0, 0] for v in _top8(cand.T)]
    aux = [jnp.zeros((CAP, 128), F32)] * 3
    for c in range(CAP):
        hit = pltpu.bitcast(key, I32) == best[c]
        aux = [jnp.where(sub8 == c, jnp.sum(jnp.where(hit, v, 0.0), axis=0, keepdims=True), a)
               for a, v in zip(aux, (m2, inv2, score))]
    m_sel, inv_sel, score_sel = [jnp.sum(a, axis=1, keepdims=True) for a in aux]
    picks = [L - 1 - (v & (L - 1)) for v in best]
    tile, col = [t >> 7 for t in picks], [t & 127 for t in picks]
    rnd = [sum([(col[e] == col[c]).astype(I32) for e in range(c)], 0) for c in range(CAP)]
    rounds = functools.reduce(jnp.maximum, rnd) + 1
    lane_in = lambda n, c: lane8 == jnp.where(rnd[c] == n, col[c], -1)

    def out_copy(q, lo, hi, n):
        j = order_s[q]
        return pltpu.make_async_copy(
            out_v.at[j, lo:hi], out_hbm.at[lo:hi, _ds(j * 128, 128)], sem_o.at[n])

    h_w, out_w = h_v.bitcast(I32), out_v.bitcast(I32)

    def gather(n, acc):
        masks = [lane_in(n, c) for c in range(CAP)]
        tiles = []
        for i in range(0, D // 2, 8):
            v = jnp.zeros((8, 128), I32)
            for c in range(CAP):
                v = jnp.where(masks[c], h_w[tile[c], i:i + 8, :], v)
            tiles.append(v)
        lhs = jnp.zeros((CAP, 128), F32)
        for c in range(CAP):
            lhs = jnp.where(masks[c] & (sub8 == c), 1.0, lhs)
        return acc + jax.lax.dot_general(lhs.astype(BF16), _mxu(jnp.concatenate(tiles, axis=0)),
                                         NT_DIMS, preferred_element_type=F32)

    with jax.named_scope("S_gather"):
        h_sel = jax.lax.fori_loop(0, rounds, gather, jnp.zeros((CAP, D), F32))
    x_sel = _rbf((h_sel - m_sel) * inv_sel)
    gate = _rbf(jax.nn.sigmoid(score_sel))

    true = lane8 + picks[0] >= 0
    tie = lambda x, token: jnp.where(true, x, token)

    def unrouted(j0):
        token = lane8
        for j in range(j0, j0 + NT // 2):
            inv = jnp.broadcast_to(inv2[j:j + 1], (8, 128))
            mul, sub = 1.0 + inv, m2[j:j + 1] * inv
            for i in range(0, D // 2, 8):
                res = _pack(*[h * mul - sub for h in _unpack(h_w[j, i:i + 8, :])])
                out_w[j, i:i + 8, :] = res
                token = token ^ res
                yield pltpu.bitcast(token, F32)

    def project(w_ref, j0):
        parts, side = [], unrouted(j0)
        for n in range(0, FF, 128):
            token = [next(side) for _ in range(8)][-1]
            xs = jnp.concatenate([tie(x_sel[:, :128], token), x_sel[:, 128:]], axis=1)
            parts.append(jnp.dot(xs.astype(BF16), w_ref[:, n:n + 128],
                                 preferred_element_type=F32))
        return _rbf(jnp.concatenate(parts, axis=1))

    with jax.named_scope("S_gwait"):
        cp_w[0].wait()
        cp_w[1].wait()
    g = project(wg_v, 0)
    act = _rbf(g * jax.nn.sigmoid(g)) * project(wu_v, NT // 2)
    routed = functools.reduce(jnp.bitwise_or, [1 << j for j in tile])
    spare = CAP - sum((routed >> j) & 1 for j in range(NT))
    n_late = 0
    for j in range(NT):
        hit = (routed >> j) & 1
        fill = (1 - hit) & (spare > 0).astype(I32)
        spare = spare - fill
        order_s[jnp.clip(jnp.where(hit + fill == 1, CAP + n_late, j - n_late), 0, NT - 1)] = j
        n_late = n_late + hit + fill

    for q in range(CAP):
        out_copy(q, 0, D, q).start()
    with jax.named_scope("S_dwait"):
        cp_w[2].wait()

    def placed(r, words):
        idx = jnp.zeros((CAP, 128), I32)
        for c in range(1, CAP):
            idx = jnp.where(lane_in(r, c), c, idx)
        return [_gather(w, idx) for w in words]

    def late_copies(n, lo, hi):
        return [out_copy(CAP + q, lo, hi, CAP * (n + 1) + q) for q in range(CAP)]

    new_w = new_v.bitcast(I32)
    tokens = []
    for n, (lo, hi) in enumerate(ROW_CHUNKS):
        a = act
        if n >= 2:
            cut = 128 * 12
            a = jnp.concatenate(
                [a[:, :cut], tie(a[:, cut:cut + 128], tokens[n - 2]), a[:, cut + 128:]], axis=1)
        y = _rbf(jax.lax.dot_general(a.astype(BF16), wd_v[lo:hi, :], NT_DIMS,
                                     preferred_element_type=F32))
        new = h_sel[:, lo:hi] + _rbf(x_sel[:, lo:hi] + _rbf(y * gate))
        new_v[lo:hi, :] = jnp.concatenate(
            [new, jnp.zeros((128 - CAP, hi - lo), F32)], axis=0).T.astype(BF16)
        rows = range(lo // 2, hi // 2, 8)
        words = [new_w[i:i + 8, :] for i in rows]
        both = list(zip(rows, placed(0, words), placed(1, words)))
        for c in range(CAP):
            for i, v0, v1 in both:
                pltpu.store(out_w.at[tile[c], pl.ds(i, 8), :],
                            jnp.where(rnd[c] == 0, v0, v1), mask=lane8 == col[c])
        tokens.append(pltpu.bitcast(both[-1][2], F32))
        for cp in late_copies(n, lo, hi):
            cp.start()
    with jax.named_scope("S_owait"):
        for q in range(CAP):
            out_copy(q, 0, D, q).wait()
        for n, (lo, hi) in enumerate(ROW_CHUNKS):
            for cp in late_copies(n, lo, hi):
                cp.wait()

    @pl.when(rounds > 2)
    def _():
        def fix(r, carry):
            rows = range(0, D // 2, 8)
            vals = placed(r, [new_w[i:i + 8, :] for i in rows])
            for c in range(CAP):
                for i, v in zip(rows, vals):
                    pltpu.store(out_w.at[tile[c], pl.ds(i, 8), :], v, mask=lane_in(r, c))
            return carry

        jax.lax.fori_loop(2, rounds, fix, 0)
        for cp in late_copies(0, 0, D):
            cp.start()
        for cp in late_copies(0, 0, D):
            cp.wait()


@jax.jit
def pallas_sequential_preLN__ssm_conv_s4__moe_arch_mod__prompt_kernel(
    A_u: jax.Array,
    A_A_re: jax.Array,
    A_A_im: jax.Array,
    A_B_re: jax.Array,
    A_B_im: jax.Array,
    A_C_re: jax.Array,
    A_C_im: jax.Array,
    A_log_dt: jax.Array,
    A_Dskip: jax.Array,
    B_x: jax.Array,
    B_w_r: jax.Array,
    B_w_gate: jax.Array,
    B_w_up: jax.Array,
    B_w_down: jax.Array,
):
    del B_x
    hbm = pl.BlockSpec(memory_space=pl.ANY)
    out = pl.pallas_call(
        _kernel,
        out_shape=jax.ShapeDtypeStruct((D, L), BF16),
        in_specs=[hbm] * 13,
        out_specs=hbm,
        scratch_shapes=[
            pltpu.VMEM((NT, D, 128), BF16),
            pltpu.VMEM((D, FF), BF16),
            pltpu.VMEM((D, FF), BF16),
            pltpu.VMEM((D, FF), BF16),
            pltpu.VMEM((6, D, N), BF16),
            *[pltpu.VMEM((D,), BF16)] * 3,
            *[pltpu.VMEM((16, 2, 128, 128), BF16)] * 2,
            pltpu.VMEM((16, 2, 64, 128), I32),
            pltpu.VMEM((3, D, 128), F32),
            pltpu.VMEM((2, 256, 128), F32),
            pltpu.VMEM((NT, D, 128), F32),
            pltpu.VMEM((NT, D, 128), BF16),
            pltpu.VMEM((2, NT, 8, 128), F32),
            pltpu.VMEM((3, NT, 8, 128), F32),
            pltpu.VMEM((NT, D, 128), BF16),
            *[pltpu.VMEM((4, 4, 10, 8, 128), F32)] * 2,
            *[pltpu.VMEM((4, 4, 2, 96, 128), BF16)] * 2,
            *[pltpu.VMEM((4, 4, 2, 128, 128), BF16)] * 2,
            *[pltpu.VMEM((4, 8, 128), I32)] * 2,
            *[pltpu.VMEM((16, MB // 2, 128), I32)] * 4,
            *[pltpu.VMEM((4, 4, 2, 2 * MB, 128), F32)] * 2,
            *[pltpu.VMEM((4, 4, 2, MB, 128), F32)] * 2,
            *[pltpu.VMEM((16, MB, 128), BF16)] * 2,
            pltpu.VMEM((D, 128), BF16),
            pltpu.SMEM((NT,), I32),
            pltpu.SemaphoreType.DMA((15,)),
            pltpu.SemaphoreType.DMA((NT,)),
            pltpu.SemaphoreType.DMA((3,)),
            pltpu.SemaphoreType.DMA((CAP * (1 + len(ROW_CHUNKS)),)),
        ],
        compiler_params=pltpu.CompilerParams(vmem_limit_bytes=100 * 1024 * 1024,
                                             disable_bounds_checks=True,
                                             disable_semaphore_checks=True),
    )(A_u.reshape(L, D).T, A_A_re, A_A_im, A_B_re, A_B_im, A_C_re, A_C_im,
      A_log_dt, A_Dskip, B_w_r, B_w_gate, B_w_up, B_w_down.T)
    return out.T.reshape(1, L, D)
```

```python
import functools

import numpy as np
import jax
import jax.numpy as jnp
import jax.experimental.pallas as pl
import jax.experimental.pallas.tpu as pltpu

F32 = jnp.float32
BF16 = jnp.bfloat16
I32 = jnp.int32

L = 2048
D = 576
N = 128
FF = 4608
CAP = 8
NT = L // 128
EPS = 1e-5
MB = 64
import os
STEPS = eval(os.environ["ONE"]) if os.environ.get("ONE") else range(1, D // MB + 6)
PLANS = dict(
    Ffmir=(1, "0:m:-1:6 0:m:-1:9 0:f 0:f 0:m:4:18 0:m:5:23 0:F 0:F 0:i 0:r:16:-1 0:r:17:-1 0:i "),
    ir=(4, "0:i 0:r:-1:6 0:r:12:27 0:i 3:r:-1:11 3:r:31:-1 1:i 1:i 1:r:1:16 2:r:8:19 1:r:16:31 "
           "2:r:22:-1 2:i 2:i 3:i 3:i "),
    kFnfmir=(1, "0:m:-1:7 0:f 0:n:0:10 0:m:2:20 0:f 0:k 0:m:10:22 0:k 0:r:15:27 0:m:15:35 0:k "
                "0:F 0:F 0:i 0:r:29:-1 0:i "),
    mir=(2, "0:m:-1:0 0:m:-1:3 0:m:-1:4 0:m:-1:9 0:i 0:i 1:r:-1:9 0:r:0:10 0:r:1:12 1:r:7:-1 "
            "1:i 1:i 1:m:7:-1 1:m:7:-1 1:m:9:-1 1:m:12:-1 "),
    stk=(2, "0:t:-1:2 1:t:-1:4 0:t:-1:6 0:t:-1:8 1:t:-1:10 0:t:-1:12 1:t:5:23 1:t:14:22 0:k "
            "0:k 1:k 0:s:-1:20 0:s:-1:22 1:k 1:s:13:-1 0:k 1:s 1:k "),
    stkFnf=(1, "0:n:-1:10 0:t:-1:6 0:s:-1:17 0:s:-1:27 0:f 0:t:3:19 0:k 0:k 0:t:13:-1 0:k 0:f "
               "0:F 0:t:21:-1 0:F "),
    stkFnfm=(1, "0:m:-1:3 0:t:-1:7 0:t:-1:13 0:t:-1:9 0:s 0:s 0:f 0:m:1:16 0:f 0:m:6:18 0:k "
                "0:t:9:22 0:k 0:m:14:-1 0:n:17:-1 0:k 0:F 0:F "),
    stkFnfmi=(1, "0:t:-1:3 0:t:-1:3 0:m:-1:6 0:n:-1:9 0:s:-1:32 0:f 0:s:0:31 0:k 0:m:6:17 0:k "
                 "0:m:13:25 0:k:-1:30 0:f 0:t:16:30 0:t:14:33 0:F 0:F 0:i 0:i 0:m:32:-1 "),
    stkFnfmir=(1, "0:t:-1:3 0:t:-1:3 0:m:-1:6 0:n:-1:9 0:s:-1:28 0:f 0:s:1:35 0:k 0:m:4:16 "
                  "0:r:9:20 0:k 0:m:13:25 0:k:-1:30 0:f 0:t:16:30 0:t:14:33 0:F 0:F 0:r:25:-1 "
                  "0:i 0:i 0:m:32:-1 "),
    tkFnfmir=(1, "0:t:-1:3 0:t:-1:3 0:m:-1:6 0:n:-1:8 0:f 0:k 0:m:4:16 0:r:9:20 0:k 0:m:13:25 "
                 "0:k:-1:30 0:f 0:t:16:30 0:t:16:33 0:F 0:F 0:r:25:-1 0:i 0:i 0:m:32:-1 "),
    n=(4, ""),
    r=(4, ""),
    default=(1, ""),
)
if os.environ.get("PLAN"):
    PLANS = dict(default=eval(os.environ["PLAN"]), s=(1, ""))
ROW_CHUNKS = ((0, 128), (128, 256), (256, 384), (384, 512), (512, D))
NT_DIMS = (((1,), (1,)), ((), ()))


def _round_res(step):
    return [int(np.round(r / step)) * step for r in range(16)]


RES1, RES2, RES3 = _round_res(2), _round_res(4), _round_res(8)


def _ds(start, size):
    return pl.ds(start if isinstance(start, int) else pl.multiple_of(start, size), size)


def _iota(shape, dim):
    return jax.lax.broadcasted_iota(I32, shape, dim)


def _rbf(x):
    return x.astype(BF16).astype(F32)


def _cmul(a, b):
    return (a[0] * b[0] - a[1] * b[1], a[0] * b[1] + a[1] * b[0])


def _csq(a):
    t = a[0] * a[1]
    return ((a[0] + a[1]) * (a[0] - a[1]), t + t)


def _cadd(a, b):
    return (a[0] + b[0], a[1] + b[1])


def _csub(a, b):
    return (a[0] - b[0], a[1] - b[1])


def _bfly4(a0, a1, a2, a3, inverse=False):
    s02, d02 = _cadd(a0, a2), _csub(a0, a2)
    s13, d13 = _cadd(a1, a3), _csub(a1, a3)
    p = (d02[0] - d13[1], d02[1] + d13[0])
    m = (d02[0] + d13[1], d02[1] - d13[0])
    if inverse:
        p, m = m, p
    return _cadd(s02, s13), p, _csub(s02, s13), m


def _prod_mod_1(a, b):
    fa, fb = _bfly4(*a), _bfly4(*b)
    return _bfly4(*[_cmul(x, y) for x, y in zip(fa, fb)], inverse=True)


def _prod2(a0, a1, b0, b1, sgn):
    p00, p11 = _cmul(a0, b0), _cmul(a1, b1)
    c1 = _cadd(_cmul(a0, b1), _cmul(a1, b0))
    if sgn > 0:
        return (p00[0] - p11[1], p00[1] + p11[0]), c1
    return (p00[0] + p11[1], p00[1] - p11[0]), c1


def _prod_mod_m1(a, b):
    def split(x):
        p = [(x[k][0] - x[k + 2][1], x[k][1] + x[k + 2][0]) for k in range(2)]
        m = [(x[k][0] + x[k + 2][1], x[k][1] - x[k + 2][0]) for k in range(2)]
        return p, m
    ap, am = split(a)
    bp, bm = split(b)
    cp = _prod2(*ap, *bp, 1)
    cm = _prod2(*am, *bm, -1)
    lo = [_cadd(cp[k], cm[k]) for k in range(2)]
    hi = [(cp[k][1] - cm[k][1], cm[k][0] - cp[k][0]) for k in range(2)]
    return lo + hi


def _prod_mod_i(a, b, sgn):
    sm = [x[0] + x[1] for x in b]
    df = [x[1] - x[0] for x in b]
    asum = [x[0] + x[1] for x in a]
    out = []
    for k in range(4):
        acc = [None, None, None]
        for j in range(4):
            m = (k - j) % 4
            if j <= k:
                t = ((b[m][0], 1), (df[m], 1), (sm[m], 1))
            elif sgn > 0:
                t = ((b[m][1], -1), (sm[m], 1), (df[m], -1))
            else:
                t = ((b[m][1], 1), (sm[m], -1), (df[m], 1))
            for q, (v, (w, s)) in enumerate(zip((asum[j], a[j][0], a[j][1]), t)):
                p = v * w
                if acc[q] is None:
                    acc[q] = p
                else:
                    acc[q] = acc[q] + p if s > 0 else acc[q] - p
        out.append((acc[0] - acc[2], acc[0] + acc[1]))
    return out


def _barrel(v):
    lane = _iota((8, 128), 1)
    for bit in range(4):
        m = ((lane >> bit) & 1) == 1
        v = [jnp.where(m, v[(i + (1 << bit)) % 16], v[i]) for i in range(16)]
    return [v[-s % 16] for s in range(16)]


def _to_residues(tiles):
    return _barrel([t if j == 0 else pltpu.roll(t, j, 1) for j, t in enumerate(tiles)])


def _to_time(res):
    return [t if j == 0 else pltpu.roll(t, 128 - j, 1) for j, t in enumerate(_barrel(res))]


def _gather(x, idx):
    return jnp.take_along_axis(x, idx, axis=1, mode="promise_in_bounds")


def _init_dft(wu_ref, wk_ref, wt_ref, tmp_ref):
    sub, k4 = _iota((8, 128), 0), 4 * _iota((8, 128), 1) + 1

    def cis(t):
        ph = ((k4 * t) & (4 * L - 1)).astype(F32) * (2 * np.pi / (4 * L))
        return jnp.cos(ph), jnp.sin(ph)

    w1, w16 = cis(1), cis(16)
    w32 = _csq(w16)
    fk = [cis(16 * (32 * (sub & 3) + (sub >> 2)))]
    fu = [cis(128 * sub), cis(128 * (sub + 8))]
    for v in range(1, 16):
        fk.append(_cmul(fk[-1], w32))
        if v >= 2:
            fu.append(_cmul(fu[-2], w16))
    for p in range(2):
        for v in range(32):
            tmp_ref[p, 8 * v:8 * v + 8, :] = fu[v % 16][p]
    tw = None
    for s in range(16):
        for v in range(0, 16, 2):
            rows = [slice(128 - s + 8 * i, 136 - s + 8 * i) for i in (v, v + 1)]
            for ref, f in ((wk_ref, fk[v:v + 2]),
                           (wu_ref, [(tmp_ref[0, r, :], tmp_ref[1, r, :]) for r in rows])):
                if s:
                    f = [_cmul(x, tw) for x in f]
                for p in range(2):
                    ref[s, p, 8 * v:8 * v + 16, :] = jnp.concatenate(
                        [f[0][p], f[1][p]], axis=0).astype(BF16)
        for p in range(2):
            wt_ref[s, p] = pltpu.bitcast(_mxu(wu_ref.bitcast(I32)[s, p]).T, I32)
        tw = _cmul(tw, w1) if s else w1


def _pack(a, b):
    return pltpu.pack_elementwise([a, b], packed_dtype=BF16)


def _unpack(w):
    return [pltpu.unpack_elementwise(w, index=i, packed_dtype=BF16, unpacked_dtype=F32)
            for i in range(2)]


FINE = (0, 1, 2, 3, 4, 5, 6, 7, 512, 516, 1024, 1536)


def _k_seeds(z, c):
    lo = _iota((8, 128), 0) < 4
    pw = {1: z}
    for e in range(1, 10):
        pw[1 << e] = _csq(pw[1 << (e - 1)])
    rot = lambda v: tuple(pltpu.roll(x, 4, 0) for x in v)
    sel = lambda a, b: tuple(jnp.where(lo, p, q) for p, q in zip(a, b))
    z16 = (pw[16][0], 0.0 - pw[16][1])
    pairs = [(z, rot(z)), (pw[32], rot(pw[32])), (pw[512], rot(pw[512])),
             (c, rot(_cmul(c, pw[8])))]
    return [[sel(a, b) for a, b in pairs] + [sel((1.0, 0.0), rot(z16))],
            [sel(b, a) for a, b in pairs] + [sel((1.0, 0.0), z16)]]


def _mxu(words):
    return pltpu.bitcast(words, BF16)


def _store_table(ref, tab):
    for i in range(0, len(tab), 2):
        for p in range(2):
            ref[p, 8 * i:8 * i + 16, :] = jnp.concatenate(
                [tab[i][p], tab[i + 1][p]], axis=0).astype(BF16)


def _k_residues(groups, k_last, dskip):
    sub = _iota((8, 128), 0)
    lane = _iota((8, 128), 1)
    lo = sub < 4
    idx = (lane & ~3) | (sub & 3)
    nxt = ((idx + 4) & 127)
    kv, up = {}, {}
    for i, k in enumerate(FINE):
        v = [g[8 * i:8 * i + 8] for g in groups]
        if k == 0:
            v = [x + jnp.where((lane < 4) & (lo if n % 2 == 0 else ~lo),
                               dskip[n // 2], 0.0)
                 for n, x in enumerate(v)]
        p = [_pack(v[g], v[2 + g]) for g in range(2)]
        even = jnp.where(lo, p[0], p[1])
        kv[k] = _gather(even, idx)
        kv[k + 8] = _gather(pltpu.roll(jnp.where(lo, p[1], p[0]), 4, 0), idx)
        if k % 512 == 0:
            up[k] = _gather(even, nxt)
    q = lane & 3
    s3 = {r: jnp.where(q == 2, kv[1024 + r], kv[1536 + r]) for r in (0, 8)}
    v0 = jnp.where(q == 0, kv[0], jnp.where(q == 1, kv[512], s3[0]))
    q16 = q + jnp.where(lane >= 124, 1, 0)
    v16 = jnp.where(q16 < 2, jnp.where(q16 == 0, up[0], up[512]),
                    jnp.where(q16 == 2, up[1024], jnp.where(q16 == 3, up[1536], k_last)))
    s3[16] = v16
    s23, s123, out = {}, {}, [v0]
    for r in range(1, 16):
        k23 = (RES2[r], RES3[r])
        if k23 not in s23:
            s23[k23] = v16 if k23 == (16, 16) else jnp.where(q == 1, kv[512 + k23[0]], s3[k23[1]])
        k123 = (RES1[r],) + k23
        if k123 not in s123:
            s123[k123] = v16 if k123[0] == 16 else jnp.where(q == 0, kv[k123[0]], s23[k23])
        if RES1[r] == r:
            out.append(s123[k123])
        else:
            out.append(jnp.where((q == 0) & (lane < 64), kv[r], s123[k123]))
    return out


def _ln_scalars(s1, s2):
    mean = s1 * (1.0 / D)
    var = jnp.maximum(s2 * (1.0 / D) - mean * mean, 0.0)
    eps = float(np.asarray(EPS, dtype=BF16))
    sd = _rbf(jnp.sqrt(_rbf(_rbf(var) + eps)))
    return _rbf(mean), 1.0 / sd


def _top8(x):
    def swap(v, pairs):
        for i, j in pairs:
            v[i], v[j] = jnp.maximum(v[i], v[j]), jnp.minimum(v[i], v[j])
        return v

    def merge(a, b):
        v = [jnp.maximum(a[i], b[7 - i]) for i in range(8)]
        return swap(v, [(i, i + d) for d in (4, 2, 1) for i in range(8) if not i & d])

    sort8 = ((0, 2), (1, 3), (4, 6), (5, 7), (0, 4), (1, 5), (2, 6), (3, 7), (0, 1), (2, 3),
             (4, 5), (6, 7), (2, 4), (3, 5), (1, 4), (3, 6), (1, 2), (3, 4), (5, 6))
    v = merge(*[swap([x[64 * h + 8 * i:64 * h + 8 * i + 8] for i in range(8)], sort8)
                for h in range(2)])
    for d in (4, 2, 1):
        v = merge(v, [pltpu.roll(t, d, 0) for t in v])
    return v


def _column(vec, split):
    row = vec.astype(F32).reshape(1, D)
    starts = [min(lo, D - 128) for lo in range(0, D, 128)]
    rows = jnp.concatenate([row[:, i:i + 128] for i in starts + starts[:3]], axis=0)
    if split:
        lane = _iota((8, 128), 1)
        rows = _gather(rows, (lane & ~15) + 2 * (lane & 7) + ((lane >> 3) & 1))
    parts = [jnp.broadcast_to(rows[n:n + 1], (128, 128)).T[128 * n - i:]
             for n, i in enumerate(starts)]
    return jnp.concatenate(parts, axis=0)


class _Schedule:
    def __init__(self, zero):
        self.zero = zero
        self.true = _iota((8, 128), 0) + zero >= 0
        self.done, self.pending, self.wait = [], {}, -1

    def tie(self, x, token):
        return jnp.where(self.true, x, token if token.dtype == x.dtype
                         else pltpu.bitcast(token, x.dtype))

    def start(self, x):
        return self.tie(x, self.done[self.wait]) if 0 <= self.wait < len(self.done) else x

    def lhs(self, words, first):
        tiles = [words[i:i + 8] for i in range(0, words.shape[0], 8)]
        for i in range(len(tiles) if first else 0):
            for token in self.pending.pop(len(self.done) + i, ()):
                tiles[i] = self.tie(tiles[i], token)
        return _mxu(jnp.concatenate(tiles, axis=0))

    def results(self, v):
        self.done += [v[i + 8:i + 16] for i in range(0, v.shape[0], 16)]

    def run(self, stage, wait, before):
        self.wait = wait
        self.pending.setdefault(before, []).extend(next(stage))


def _kernel(x_hbm, are_hbm, aim_hbm, bre_hbm, bim_hbm, cre_hbm, cim_hbm,
            ldt_hbm, dsk_hbm, wr_hbm, wg_hbm, wu_hbm, wd_hbm, out_hbm,
            x_v, wg_v, wu_v, wd_v, par_v, ldt_v, dsk_v, wr_v, w_v, wk_v, wt_v, col_v,
            tmp_v, h_v, st_v, acc_v, out_v, sd0, sd1, ta0, ta1, tb0, tb1, kl0, kl1,
            u0, u1, k0, k1, a0_v, a1_v, c0, c1, y0, y1, new_v, order_s,
            sem_p, sem_x, sem_w, sem_o, *kf_v):
    cp_vec = [pltpu.make_async_copy(s, d, sem_p.at[n]) for n, (s, d) in enumerate(
        ((ldt_hbm, ldt_v), (dsk_hbm, dsk_v), (wr_hbm, wr_v)))]
    cp_par = [[pltpu.make_async_copy(s.at[lo:hi], par_v.at[n, lo:hi], sem_p.at[3 + 6 * m + n])
               for n, s in enumerate((are_hbm, aim_hbm, bre_hbm, bim_hbm, cre_hbm, cim_hbm))]
              for m, (lo, hi) in enumerate(((0, 3 * MB), (3 * MB, D)))]
    cp_x = [pltpu.make_async_copy(x_hbm.at[:, 128 * j:128 * j + 128], x_v.at[j], sem_x.at[j])
            for j in range(NT)]
    cp_w = [pltpu.make_async_copy(s, d, sem_w.at[n]) for n, (s, d) in enumerate(
        ((wg_hbm, wg_v), (wu_hbm, wu_v), (wd_hbm, wd_v)))]
    for cp in cp_vec + cp_par[0]:
        cp.start()
    for cp in cp_x:
        cp.start(priority=1)

    with jax.named_scope("S_dft"):
        _init_dft(w_v, wk_v, wt_v, tmp_v)
    for cp in cp_vec:
        cp.wait()
    col_v[0] = _rbf(jnp.exp(_column(ldt_v[...], True)))
    col_v[1] = _column(dsk_v[...], True) * (1.0 / L)
    col_v[2] = _column(wr_v[...], False)
    with jax.named_scope("S_pwait"):
        for cp in cp_par[0]:
            cp.wait()

    sd, ta, tb, kl = (sd0, sd1), (ta0, ta1), (tb0, tb1), (kl0, kl1)
    uk, ab, cc, yy = ((u0, u1), (k0, k1)), ((a0_v, a1_v), kf_v), (c0, c1), (y0, y1)
    ww, wt_w = (w_v.bitcast(I32), wk_v.bitcast(I32)), wt_v

    def chan(b, r):
        return _ds(b * MB + 16 * r, 16)

    def seed_stage(b, r, sch):
        rows = _ds(b * MB // 2 + 8 * r, 8)
        par = [_unpack(par_v.bitcast(I32)[n, rows, :]) for n in range(6)]
        for h in range(2):
            a_re, a_im, b_re, b_im, c_re, c_im = [v[h] for v in par]
            dt = sch.start(col_v[0, _ds(b * MB + 16 * r + 8 * h, 8), :])
            mag, ang = jnp.exp(dt * a_re), dt * a_im
            sc = dt * (1.0 / L)
            seeds = _k_seeds((mag * jnp.cos(ang), mag * jnp.sin(ang)),
                             _cmul((c_re, c_im), (sc * b_re, sc * b_im)))
            for g in range(2):
                for n, v in enumerate(seeds[g]):
                    for p in range(2):
                        sd[b % 2][r, 2 * h + g, 2 * n + p] = v[p]
            yield [sd[b % 2][(r + sch.zero), 2 * h, 0]]

    def table_stage(b, r, sch):
        tail = []
        for g in range(4):
            m1, m32, m512, a0, b0 = [
                (sd[b % 2][r, g, 2 * n], sd[b % 2][r, g, 2 * n + 1]) for n in range(5)]
            m32 = (sch.start(m32[0]), m32[1])
            fa = [a0]
            for _ in range(7):
                fa.append(_cmul(fa[-1], m1))
            for src in (0, 4, 8, 10):
                fa.append(_cmul(fa[src], m512))
            tail.append(fa[11][0] * m512[0] - fa[11][1] * m512[1])
            _store_table(ta[b % 2].at[r, g], fa)
            fb = [b0]
            for _ in range(15):
                p = fb[-1]
                fb.append((p[0] * m32[0] + p[1] * m32[1], p[1] * m32[0] - p[0] * m32[1]))
            _store_table(tb[b % 2].at[r, g], fb)
            yield [ta[b % 2].bitcast(I32)[(r + sch.zero), g, 0, 0:8, :],
                   tb[b % 2].bitcast(I32)[(r + sch.zero), g, 0, 0:8, :]]
        lo = _iota((8, 128), 0) < 4
        kl[b % 2][r] = _pack(*[jnp.broadcast_to(
            jnp.sum(jnp.where(lo, tail[2 * h], tail[2 * h + 1]), axis=1, keepdims=True),
            (8, 128)) for h in range(2)])

    def kernel_stage(b, r, sch):
        ta_w, tb_w = ta[b % 2].bitcast(I32), tb[b % 2].bitcast(I32)
        groups = [None] * 4
        for g0 in range(2):
            res = [jax.lax.dot_general(sch.lhs(ta_w[r, g, p], g == g0 and p == 0),
                                       _mxu(tb_w[r, g, p]), NT_DIMS, preferred_element_type=F32)
                   for g in (g0, g0 + 2) for p in range(2)]
            groups[g0], groups[g0 + 2] = res[0] + res[1], res[2] + res[3]
            sch.results(groups[g0 + 2])
            yield []
        dskip = [col_v[1, _ds(b * MB + 16 * r + 8 * h, 8), :] for h in range(2)]
        dst = _ds(8 * r, 8)
        res = _k_residues(groups, kl[b % 2][r], dskip)
        for s, t in enumerate(res):
            uk[1][b % 2][s, dst, :] = t
        yield [uk[1][b % 2][0, _ds(8 * (r + sch.zero), 8), :]]

    def norm_stage(b, r, sch):
        tiles = []
        rows = _ds(b * MB // 2 + 8 * r, 8)
        for j in range(NT):
            m, inv = st_v[0, j] if j else sch.start(st_v[0, j]), st_v[1, j]
            tiles.append(_pack(*[(v - m) * inv for v in _unpack(x_v.bitcast(I32)[j, rows, :])]))
        dst = _ds(8 * r, 8)
        res = _to_residues(tiles)
        for s, t in enumerate(res):
            uk[0][b % 2][s, dst, :] = t
        yield [uk[0][b % 2][0, _ds(8 * (r + sch.zero), 8), :]]

    def forward_stage(w, b, k, sch):
        dst = ab[w][b % len(ab[w])]
        for p in range(2):
            v = [jnp.dot(sch.lhs(uk[w][b % 2][k + 4 * n], n == 0),
                         _mxu(ww[w][k + 4 * n, p ^ (n & 1)]),
                         preferred_element_type=F32) for n in range(4)]
            d02, d13 = v[0] - v[2], v[1] - v[3]
            x1 = d02 - d13 if p == 0 else d02 + d13
            dst[k, 0, p] = v[0] + v[2]
            dst[k, 2, 1 - p] = v[1] + v[3]
            dst[k, 1, p] = x1
            dst[k, 3, p] = d02 + d13 if p == 0 else d02 - d13
            sch.results(x1)
            yield []

    def stats_stage(b, r, sch):
        for n in range(4):
            j = 4 * r + n
            s1 = sch.start(jnp.zeros((8, 128), F32))
            s2 = s1
            for i in range(0, D // 2, 8):
                v0, v1 = _unpack(x_v.bitcast(I32)[j, i:i + 8, :])
                s1, s2 = s1 + (v0 + v1), s2 + (v0 * v0 + v1 * v1)
            for d in (4, 2, 1):
                s1, s2 = s1 + pltpu.roll(s1, d, 0), s2 + pltpu.roll(s2, d, 0)
            st_v[0, j], st_v[1, j] = m, inv = _ln_scalars(s1, s2)
            yield [inv]

    def middle_stage(b, r, sch):
        src = [v[b % len(v)] for v in ab]
        scale = lambda v, f: [(x[0] * f, x[1] * f) for x in v]
        for h in range(2):
            ra = _ds(16 * r + 8 * h, 8)
            ld = lambda q, w: [(src[w][k, q, 0, ra, :], src[w][k, q, 1, ra, :]) for k in range(4)]

            def put(q, x, y):
                for k in range(4):
                    for p in range(2):
                        cc[b % 2][k, q, p, ra, :] = x[k][p] + y[k][p]
                        cc[b % 2][k, q + 1, p, ra, :] = x[k][p] - y[k][p]

            gate = sch.start
            a0, a2, b0, b2 = ld(0, 0), ld(2, 0), ld(0, 1), ld(2, 1)
            a0[0] = (gate(a0[0][0]), a0[0][1])
            e0 = _prod_mod_1(list(map(_cadd, a0, a2)), list(map(_cadd, b0, b2)))
            e2 = _prod_mod_m1(list(map(_csub, a0, a2)), scale(map(_csub, b0, b2), 2.0))
            put(0, e0, e2)
            again = _ds(16 * (r + sch.zero) + 8 * h, 8)
            yield [cc[b % 2][0, 0, 0, again, :]]
            four = sch.start(jnp.full((8, 128), 4.0, F32))
            e1 = _prod_mod_i(ld(1, 0), scale(ld(1, 1), four), 1)
            e3 = _prod_mod_i(ld(3, 0), scale(ld(3, 1), four), -1)
            put(2, e1, e3)
            yield [cc[b % 2][0, 2, 0, again, :]]

    def inverse_stage(b, k, sch):
        src = cc[b % 2]

        def lhs(v, first):
            return sch.lhs(jnp.concatenate(
                [_pack(v[i:i + 8], v[i + 8:i + 16]) for i in range(0, MB, 16)], axis=0), first)

        for o in range(2):
            p0, p1 = [(src[k, q, 0], src[k, q, 1]) for q in (o, o + 2)]
            if o == 0:
                e = {0: _cadd(p0, p1), 2: _csub(p0, p1)}
            else:
                e = {1: (p0[0] + p1[1], p0[1] - p1[0]), 3: (p0[0] - p1[1], p0[1] + p1[0])}
            ys = []
            for n in e:
                y = [jnp.dot(lhs(e[n][p], n == o and p == 0), _mxu(wt_w[k + 4 * n, p]),
                             preferred_element_type=F32)
                     for p in range(2)]
                ys.append(y[0] + y[1])
                yy[b % 2][k + 4 * n] = ys[-1].astype(BF16)
            sch.results(ys[-1])
            yield []

    def residual_stage(b, r, sch):
        rows = chan(b, r)
        wr = col_v[2, rows, :]
        src = yy[b % 2].bitcast(I32)
        ys = _to_time([src[s, _ds(8 * r, 8), :] for s in range(16)])
        for j in range(NT):
            h = x_v[j, rows, :].astype(F32) + jnp.concatenate(
                _unpack(ys[j] if j % 8 else sch.start(ys[j])), axis=0)
            h_v[j, rows, :] = h.astype(BF16)
            hh, hw = h * h, h * wr
            acc_v[0, j] += h[0:8] + h[8:16]
            acc_v[1, j] += hh[0:8] + hh[8:16]
            acc_v[2, j] += hw[0:8] + hw[8:16]
            if j % 8 == 7:
                yield [acc_v[0, (r + sch.zero)]]

    nb = D // MB
    stages = dict(
        s=(seed_stage, 0), t=(table_stage, 1), k=(kernel_stage, 2),
        F=(functools.partial(forward_stage, 1), 3), n=(norm_stage, 2),
        f=(functools.partial(forward_stage, 0), 3), m=(middle_stage, 4),
        i=(inverse_stage, 5), r=(residual_stage, 6))

    def run(step, zero, live=None):
        live = live or {n: (f, step - lag) for n, (f, lag) in stages.items()
                        if 0 <= step - lag < nb and (n, step) != ("n", 2)}
        unroll, plan = PLANS.get("".join(live), PLANS["default"])

        def body(it, carry):
            sch = _Schedule(zero)
            gens = [{n: f(b, it * unroll + u, sch) for n, (f, b) in live.items()}
                    for u in range(unroll)]
            for item in plan.split():
                u, n, *ties = item.split(":")
                if n in live:
                    sch.run(gens[int(u)][n], *map(int, ties or (-1, -1)))
            for g in gens:
                for v in g.values():
                    for _ in v:
                        pass
            return carry + it

        with jax.named_scope("S_p%d" % step):
            if unroll == 4:
                return body(0, 0)
            return jax.lax.fori_loop(0, 4 // unroll, body, 0)

    acc_v[...] = jnp.zeros(acc_v.shape, F32)
    zero = run(0, 0) - 6
    for step in STEPS:
        if step == 1:
            for cp in cp_par[1]:
                cp.start()
        if step == 2:
            for cp in cp_w:
                cp.start(priority=1)
        if step == 3:
            for cp in cp_par[1]:
                cp.wait()
            with jax.named_scope("S_xwait"):
                for cp in cp_x:
                    cp.wait()
            run(100, zero, dict(l=(stats_stage, 0)))
            run(101, zero, dict(n=(norm_stage, 0)))
        run(step, zero)

    def rows_of(q):
        return jnp.concatenate(
            [jnp.sum(acc_v[q, j], axis=0, keepdims=True) for j in range(NT)], axis=0)

    m2, inv2 = _ln_scalars(rows_of(0), rows_of(1))
    wsum = jnp.sum(col_v[2], axis=0, keepdims=True)
    score = _rbf((rows_of(2) - m2 * wsum) * inv2 + 0.0)
    bits = pltpu.bitcast(score, I32) >> 16
    order = jnp.where(bits < 0, -1 - bits, bits + 32768)
    pos = 128 * _iota((NT, 128), 0) + _iota((NT, 128), 1)
    key = pltpu.bitcast((order << 11) + (L - 1 - pos) + (1 << 29), F32)

    lane8, sub8 = _iota((CAP, 128), 1), _iota((CAP, 128), 0)
    best = _top8(jnp.tile(key, (8, 1)).T)
    cand = best[0]
    for c in range(1, CAP):
        cand = jnp.where((lane8 >> 4) == c, best[c], cand)
    best = [pltpu.bitcast(v, I32)[0, 0] for v in _top8(cand.T)]
    aux = [jnp.zeros((CAP, 128), F32)] * 3
    for c in range(CAP):
        hit = pltpu.bitcast(key, I32) == best[c]
        aux = [jnp.where(sub8 == c, jnp.sum(jnp.where(hit, v, 0.0), axis=0, keepdims=True), a)
               for a, v in zip(aux, (m2, inv2, score))]
    m_sel, inv_sel, score_sel = [jnp.sum(a, axis=1, keepdims=True) for a in aux]
    picks = [L - 1 - (v & (L - 1)) for v in best]
    tile, col = [t >> 7 for t in picks], [t & 127 for t in picks]
    rnd = [sum([(col[e] == col[c]).astype(I32) for e in range(c)], 0) for c in range(CAP)]
    rounds = functools.reduce(jnp.maximum, rnd) + 1
    lane_in = lambda n, c: lane8 == jnp.where(rnd[c] == n, col[c], -1)

    def out_copy(q, lo, hi, n):
        j = order_s[q]
        return pltpu.make_async_copy(
            out_v.at[j, lo:hi], out_hbm.at[lo:hi, _ds(j * 128, 128)], sem_o.at[n])

    h_w, out_w = h_v.bitcast(I32), out_v.bitcast(I32)

    def gather(n, acc):
        masks = [lane_in(n, c) for c in range(CAP)]
        tiles = []
        for i in range(0, D // 2, 8):
            v = jnp.zeros((8, 128), I32)
            for c in range(CAP):
                v = jnp.where(masks[c], h_w[tile[c], i:i + 8, :], v)
            tiles.append(v)
        lhs = jnp.zeros((CAP, 128), F32)
        for c in range(CAP):
            lhs = jnp.where(masks[c] & (sub8 == c), 1.0, lhs)
        return acc + jax.lax.dot_general(lhs.astype(BF16), _mxu(jnp.concatenate(tiles, axis=0)),
                                         NT_DIMS, preferred_element_type=F32)

    with jax.named_scope("S_gather"):
        h_sel = jax.lax.fori_loop(0, rounds, gather, jnp.zeros((CAP, D), F32))
    x_sel = _rbf((h_sel - m_sel) * inv_sel)
    gate = _rbf(jax.nn.sigmoid(score_sel))

    true = lane8 + picks[0] >= 0
    tie = lambda x, token: jnp.where(true, x, token)

    def unrouted(j0):
        token = lane8
        for j in range(j0, j0 + NT // 2):
            inv = jnp.broadcast_to(inv2[j:j + 1], (8, 128))
            mul, sub = 1.0 + inv, m2[j:j + 1] * inv
            for i in range(0, D // 2, 8):
                res = _pack(*[h * mul - sub for h in _unpack(h_w[j, i:i + 8, :])])
                out_w[j, i:i + 8, :] = res
                token = token ^ res
                yield pltpu.bitcast(token, F32)

    def project(w_ref, j0):
        parts, side = [], unrouted(j0)
        for n in range(0, FF, 128):
            token = [next(side) for _ in range(8)][-1]
            xs = jnp.concatenate([tie(x_sel[:, :128], token), x_sel[:, 128:]], axis=1)
            parts.append(jnp.dot(xs.astype(BF16), w_ref[:, n:n + 128],
                                 preferred_element_type=F32))
        return _rbf(jnp.concatenate(parts, axis=1))

    with jax.named_scope("S_gwait"):
        cp_w[0].wait()
        cp_w[1].wait()
    g = project(wg_v, 0)
    act = _rbf(g * jax.nn.sigmoid(g)) * project(wu_v, NT // 2)
    routed = functools.reduce(jnp.bitwise_or, [1 << j for j in tile])
    spare = CAP - sum((routed >> j) & 1 for j in range(NT))
    n_late = 0
    for j in range(NT):
        hit = (routed >> j) & 1
        fill = (1 - hit) & (spare > 0).astype(I32)
        spare = spare - fill
        order_s[jnp.clip(jnp.where(hit + fill == 1, CAP + n_late, j - n_late), 0, NT - 1)] = j
        n_late = n_late + hit + fill

    for q in range(CAP):
        out_copy(q, 0, D, q).start()
    with jax.named_scope("S_dwait"):
        cp_w[2].wait()

    def placed(r, words):
        idx = jnp.zeros((CAP, 128), I32)
        for c in range(1, CAP):
            idx = jnp.where(lane_in(r, c), c, idx)
        return [_gather(w, idx) for w in words]

    def late_copies(n, lo, hi):
        return [out_copy(CAP + q, lo, hi, CAP * (n + 1) + q) for q in range(CAP)]

    new_w = new_v.bitcast(I32)
    tokens = []
    for n, (lo, hi) in enumerate(ROW_CHUNKS):
        a = act
        if n >= 2:
            cut = 128 * 12
            a = jnp.concatenate(
                [a[:, :cut], tie(a[:, cut:cut + 128], tokens[n - 2]), a[:, cut + 128:]], axis=1)
        y = _rbf(jax.lax.dot_general(a.astype(BF16), wd_v[lo:hi, :], NT_DIMS,
                                     preferred_element_type=F32))
        new = h_sel[:, lo:hi] + _rbf(x_sel[:, lo:hi] + _rbf(y * gate))
        new_v[lo:hi, :] = jnp.concatenate(
            [new, jnp.zeros((128 - CAP, hi - lo), F32)], axis=0).T.astype(BF16)
        rows = range(lo // 2, hi // 2, 8)
        words = [new_w[i:i + 8, :] for i in rows]
        both = list(zip(rows, placed(0, words), placed(1, words)))
        for c in range(CAP):
            for i, v0, v1 in both:
                pltpu.store(out_w.at[tile[c], pl.ds(i, 8), :],
                            jnp.where(rnd[c] == 0, v0, v1), mask=lane8 == col[c])
        tokens.append(pltpu.bitcast(both[-1][2], F32))
        for cp in late_copies(n, lo, hi):
            cp.start()
    with jax.named_scope("S_owait"):
        for q in range(CAP):
            out_copy(q, 0, D, q).wait()
        for n, (lo, hi) in enumerate(ROW_CHUNKS):
            for cp in late_copies(n, lo, hi):
                cp.wait()

    @pl.when(rounds > 2)
    def _():
        def fix(r, carry):
            rows = range(0, D // 2, 8)
            vals = placed(r, [new_w[i:i + 8, :] for i in rows])
            for c in range(CAP):
                for i, v in zip(rows, vals):
                    pltpu.store(out_w.at[tile[c], pl.ds(i, 8), :], v, mask=lane_in(r, c))
            return carry

        jax.lax.fori_loop(2, rounds, fix, 0)
        for cp in late_copies(0, 0, D):
            cp.start()
        for cp in late_copies(0, 0, D):
            cp.wait()


@jax.jit
def pallas_sequential_preLN__ssm_conv_s4__moe_arch_mod__prompt_kernel(
    A_u: jax.Array,
    A_A_re: jax.Array,
    A_A_im: jax.Array,
    A_B_re: jax.Array,
    A_B_im: jax.Array,
    A_C_re: jax.Array,
    A_C_im: jax.Array,
    A_log_dt: jax.Array,
    A_Dskip: jax.Array,
    B_x: jax.Array,
    B_w_r: jax.Array,
    B_w_gate: jax.Array,
    B_w_up: jax.Array,
    B_w_down: jax.Array,
):
    del B_x
    hbm = pl.BlockSpec(memory_space=pl.ANY)
    out = pl.pallas_call(
        _kernel,
        out_shape=jax.ShapeDtypeStruct((D, L), BF16),
        in_specs=[hbm] * 13,
        out_specs=hbm,
        scratch_shapes=[
            pltpu.VMEM((NT, D, 128), BF16),
            pltpu.VMEM((D, FF), BF16),
            pltpu.VMEM((D, FF), BF16),
            pltpu.VMEM((D, FF), BF16),
            pltpu.VMEM((6, D, N), BF16),
            *[pltpu.VMEM((D,), BF16)] * 3,
            *[pltpu.VMEM((16, 2, 128, 128), BF16)] * 2,
            pltpu.VMEM((16, 2, 64, 128), I32),
            pltpu.VMEM((3, D, 128), F32),
            pltpu.VMEM((2, 256, 128), F32),
            pltpu.VMEM((NT, D, 128), BF16),
            pltpu.VMEM((2, NT, 8, 128), F32),
            pltpu.VMEM((3, NT, 8, 128), F32),
            pltpu.VMEM((NT, D, 128), BF16),
            *[pltpu.VMEM((4, 4, 10, 8, 128), F32)] * 2,
            *[pltpu.VMEM((4, 4, 2, 96, 128), BF16)] * 2,
            *[pltpu.VMEM((4, 4, 2, 128, 128), BF16)] * 2,
            *[pltpu.VMEM((4, 8, 128), I32)] * 2,
            *[pltpu.VMEM((16, MB // 2, 128), I32)] * 4,
            *[pltpu.VMEM((4, 4, 2, MB, 128), F32)] * 2,
            *[pltpu.VMEM((4, 4, 2, MB, 128), F32)] * 2,
            *[pltpu.VMEM((16, MB, 128), BF16)] * 2,
            pltpu.VMEM((D, 128), BF16),
            pltpu.SMEM((NT,), I32),
            pltpu.SemaphoreType.DMA((15,)),
            pltpu.SemaphoreType.DMA((NT,)),
            pltpu.SemaphoreType.DMA((3,)),
            pltpu.SemaphoreType.DMA((CAP * (1 + len(ROW_CHUNKS)),)),
            *[pltpu.VMEM((4, 4, 2, MB, 128), F32)] * 2,
        ],
        compiler_params=pltpu.CompilerParams(vmem_limit_bytes=100 * 1024 * 1024,
                                             disable_bounds_checks=True,
                                             disable_semaphore_checks=True),
    )(A_u.reshape(L, D).T, A_A_re, A_A_im, A_B_re, A_B_im, A_C_re, A_C_im,
      A_log_dt, A_Dskip, B_w_r, B_w_gate, B_w_up, B_w_down.T)
    return out.T.reshape(1, L, D)
```

```python
import functools

import numpy as np
import jax
import jax.numpy as jnp
import jax.experimental.pallas as pl
import jax.experimental.pallas.tpu as pltpu

F32 = jnp.float32
BF16 = jnp.bfloat16
I32 = jnp.int32

L = 2048
D = 576
N = 128
FF = 4608
CAP = 8
NT = L // 128
EPS = 1e-5
MB = 64
import os
STEPS = eval(os.environ["ONE"]) if os.environ.get("ONE") else range(1, D // MB + 6)
PLANS = dict(
    Ffmir=(1, "0:m:-1:6 0:m:-1:9 0:f 0:f 0:m:4:18 0:m:5:23 0:F 0:F 0:i 0:r:16:-1 0:r:17:-1 0:i "),
    ir=(4, "0:i 0:r:-1:6 0:r:12:27 0:i 3:r:-1:11 3:r:31:-1 1:i 1:i 1:r:1:16 2:r:8:19 1:r:16:31 "
           "2:r:22:-1 2:i 2:i 3:i 3:i "),
    kFnfmir=(1, "0:m:-1:7 0:f 0:n:0:10 0:m:2:20 0:f 0:k 0:m:10:22 0:k 0:r:15:27 0:m:15:35 0:k "
                "0:F 0:F 0:i 0:r:29:-1 0:i "),
    mir=(2, "0:m:-1:0 0:m:-1:3 0:m:-1:4 0:m:-1:9 0:i 0:i 1:r:-1:9 0:r:0:10 0:r:1:12 1:r:7:-1 "
            "1:i 1:i 1:m:7:-1 1:m:7:-1 1:m:9:-1 1:m:12:-1 "),
    stk=(2, "0:t:-1:2 1:t:-1:4 0:t:-1:6 0:t:-1:8 1:t:-1:10 0:t:-1:12 1:t:5:23 1:t:14:22 0:k "
            "0:k 1:k 0:s:-1:20 0:s:-1:22 1:k 1:s:13:-1 0:k 1:s 1:k "),
    stkFnf=(1, "0:n:-1:10 0:t:-1:6 0:s:-1:17 0:s:-1:27 0:f 0:t:3:19 0:k 0:k 0:t:13:-1 0:k 0:f "
               "0:F 0:t:21:-1 0:F "),
    stkFnfm=(1, "0:m:-1:3 0:t:-1:7 0:t:-1:13 0:t:-1:9 0:s 0:s 0:f 0:m:1:16 0:f 0:m:6:18 0:k "
                "0:t:9:22 0:k 0:m:14:-1 0:n:17:-1 0:k 0:F 0:F "),
    stkFnfmi=(1, "0:t:-1:3 0:t:-1:3 0:m:-1:6 0:n:-1:9 0:s:-1:32 0:f 0:s:0:31 0:k 0:m:6:17 0:k "
                 "0:m:13:25 0:k:-1:30 0:f 0:t:16:30 0:t:14:33 0:F 0:F 0:i 0:i 0:m:32:-1 "),
    stkFnfmir=(1, "0:t:-1:3 0:t:-1:3 0:m:-1:6 0:n:-1:9 0:s:-1:28 0:f 0:s:1:35 0:k 0:m:4:16 "
                  "0:r:9:20 0:k 0:m:13:25 0:k:-1:30 0:f 0:t:16:30 0:t:14:33 0:F 0:F 0:r:25:-1 "
                  "0:i 0:i 0:m:32:-1 "),
    tkFnfmir=(1, "0:t:-1:3 0:t:-1:3 0:m:-1:6 0:n:-1:8 0:f 0:k 0:m:4:16 0:r:9:20 0:k 0:m:13:25 "
                 "0:k:-1:30 0:f 0:t:16:30 0:t:16:33 0:F 0:F 0:r:25:-1 0:i 0:i 0:m:32:-1 "),
    l=(2, ""),
    n=(4, ""),
    r=(4, ""),
    default=(1, ""),
)
if os.environ.get("PLAN"):
    PLANS = dict(default=eval(os.environ["PLAN"]), s=(1, ""))
ROW_CHUNKS = ((0, 128), (128, 256), (256, 384), (384, 512), (512, D))
NT_DIMS = (((1,), (1,)), ((), ()))


def _round_res(step):
    return [int(np.round(r / step)) * step for r in range(16)]


RES1, RES2, RES3 = _round_res(2), _round_res(4), _round_res(8)


def _ds(start, size):
    return pl.ds(start if isinstance(start, int) else pl.multiple_of(start, size), size)


def _iota(shape, dim):
    return jax.lax.broadcasted_iota(I32, shape, dim)


def _rbf(x):
    return x.astype(BF16).astype(F32)


def _cmul(a, b):
    return (a[0] * b[0] - a[1] * b[1], a[0] * b[1] + a[1] * b[0])


def _csq(a):
    t = a[0] * a[1]
    return ((a[0] + a[1]) * (a[0] - a[1]), t + t)


def _cadd(a, b):
    return (a[0] + b[0], a[1] + b[1])


def _csub(a, b):
    return (a[0] - b[0], a[1] - b[1])


def _bfly4(a0, a1, a2, a3, inverse=False):
    s02, d02 = _cadd(a0, a2), _csub(a0, a2)
    s13, d13 = _cadd(a1, a3), _csub(a1, a3)
    p = (d02[0] - d13[1], d02[1] + d13[0])
    m = (d02[0] + d13[1], d02[1] - d13[0])
    if inverse:
        p, m = m, p
    return _cadd(s02, s13), p, _csub(s02, s13), m


def _prod_mod_1(a, b):
    fa, fb = _bfly4(*a), _bfly4(*b)
    return _bfly4(*[_cmul(x, y) for x, y in zip(fa, fb)], inverse=True)


def _prod2(a0, a1, b0, b1, sgn):
    p00, p11 = _cmul(a0, b0), _cmul(a1, b1)
    c1 = _cadd(_cmul(a0, b1), _cmul(a1, b0))
    if sgn > 0:
        return (p00[0] - p11[1], p00[1] + p11[0]), c1
    return (p00[0] + p11[1], p00[1] - p11[0]), c1


def _prod_mod_m1(a, b):
    def split(x):
        p = [(x[k][0] - x[k + 2][1], x[k][1] + x[k + 2][0]) for k in range(2)]
        m = [(x[k][0] + x[k + 2][1], x[k][1] - x[k + 2][0]) for k in range(2)]
        return p, m
    ap, am = split(a)
    bp, bm = split(b)
    cp = _prod2(*ap, *bp, 1)
    cm = _prod2(*am, *bm, -1)
    lo = [_cadd(cp[k], cm[k]) for k in range(2)]
    hi = [(cp[k][1] - cm[k][1], cm[k][0] - cp[k][0]) for k in range(2)]
    return lo + hi


def _prod_mod_i(a, b, sgn):
    sm = [x[0] + x[1] for x in b]
    df = [x[1] - x[0] for x in b]
    asum = [x[0] + x[1] for x in a]
    out = []
    for k in range(4):
        acc = [None, None, None]
        for j in range(4):
            m = (k - j) % 4
            if j <= k:
                t = ((b[m][0], 1), (df[m], 1), (sm[m], 1))
            elif sgn > 0:
                t = ((b[m][1], -1), (sm[m], 1), (df[m], -1))
            else:
                t = ((b[m][1], 1), (sm[m], -1), (df[m], 1))
            for q, (v, (w, s)) in enumerate(zip((asum[j], a[j][0], a[j][1]), t)):
                p = v * w
                if acc[q] is None:
                    acc[q] = p
                else:
                    acc[q] = acc[q] + p if s > 0 else acc[q] - p
        out.append((acc[0] - acc[2], acc[0] + acc[1]))
    return out


def _barrel(v, lane):
    for bit in range(4):
        m = ((lane >> bit) & 1) == 1
        v = [jnp.where(m, v[(i + (1 << bit)) % 16], v[i]) for i in range(16)]
    return [v[-s % 16] for s in range(16)]


def _to_residues(tiles, lane):
    return _barrel([t if j == 0 else pltpu.roll(t, j, 1) for j, t in enumerate(tiles)], lane)


def _to_time(res, lane):
    return [t if j == 0 else pltpu.roll(t, 128 - j, 1)
            for j, t in enumerate(_barrel(res, lane))]


def _gather(x, idx):
    return jnp.take_along_axis(x, idx, axis=1, mode="promise_in_bounds")


def _init_dft(wu_ref, wk_ref, wt_ref, tmp_ref, halfway):
    sub, k4 = _iota((8, 128), 0), 4 * _iota((8, 128), 1) + 1

    def cis(t):
        ph = ((k4 * t) & (4 * L - 1)).astype(F32) * (2 * np.pi / (4 * L))
        return jnp.cos(ph), jnp.sin(ph)

    w1, w16 = cis(1), cis(16)
    w32 = _csq(w16)
    fk = [cis(16 * (32 * (sub & 3) + (sub >> 2)))]
    fu = [cis(128 * sub), cis(128 * (sub + 8))]
    for v in range(1, 16):
        fk.append(_cmul(fk[-1], w32))
        if v >= 2:
            fu.append(_cmul(fu[-2], w16))
    for p in range(2):
        for v in range(32):
            tmp_ref[p, 8 * v:8 * v + 8, :] = fu[v % 16][p]
    tw = None
    for s in range(16):
        for v in range(0, 16, 2):
            rows = [slice(128 - s + 8 * i, 136 - s + 8 * i) for i in (v, v + 1)]
            for ref, f in ((wk_ref, fk[v:v + 2]),
                           (wu_ref, [(tmp_ref[0, r, :], tmp_ref[1, r, :]) for r in rows])):
                if s:
                    f = [_cmul(x, tw) for x in f]
                for p in range(2):
                    ref[s, p, 8 * v:8 * v + 16, :] = jnp.concatenate(
                        [f[0][p], f[1][p]], axis=0).astype(BF16)
        for p in range(2):
            wt_ref[s, p, 0:64] = pltpu.bitcast(_mxu(wu_ref.bitcast(I32)[s, p, 0:64]).T, I32)
        tw = _cmul(tw, w1) if s else w1
        if s == 7:
            halfway()


def _pack(a, b):
    return pltpu.pack_elementwise([a, b], packed_dtype=BF16)


def _unpack(w):
    return [pltpu.unpack_elementwise(w, index=i, packed_dtype=BF16, unpacked_dtype=F32)
            for i in range(2)]


FINE = (0, 1, 2, 3, 4, 5, 6, 7, 512, 516, 1024, 1536)


def _k_seeds(z, c, lo):
    pw = {1: z}
    for e in range(1, 10):
        pw[1 << e] = _csq(pw[1 << (e - 1)])
    rot = lambda v: tuple(pltpu.roll(x, 4, 0) for x in v)
    sel = lambda a, b: tuple(jnp.where(lo, p, q) for p, q in zip(a, b))
    z16 = (pw[16][0], 0.0 - pw[16][1])
    pairs = [(z, rot(z)), (pw[32], rot(pw[32])), (pw[512], rot(pw[512])),
             (c, rot(_cmul(c, pw[8])))]
    return [[sel(a, b) for a, b in pairs] + [sel((1.0, 0.0), rot(z16))],
            [sel(b, a) for a, b in pairs] + [sel((1.0, 0.0), z16)]]


def _mxu(words):
    return pltpu.bitcast(words, BF16)


def _store_table(ref, tab):
    for i in range(0, len(tab), 2):
        for p in range(2):
            ref[p, 8 * i:8 * i + 16, :] = jnp.concatenate(
                [tab[i][p], tab[i + 1][p]], axis=0).astype(BF16)


def _k_residues(groups, k_last, dskip, sub, lane):
    lo = sub < 4
    idx = (lane & ~3) | (sub & 3)
    nxt = ((idx + 4) & 127)
    kv, up = {}, {}
    for i, k in enumerate(FINE):
        v = [g[8 * i:8 * i + 8] for g in groups]
        if k == 0:
            v = [x + jnp.where((lane < 4) & (lo if n % 2 == 0 else ~lo),
                               dskip[n // 2], 0.0)
                 for n, x in enumerate(v)]
        p = [_pack(v[g], v[2 + g]) for g in range(2)]
        even = jnp.where(lo, p[0], p[1])
        kv[k] = _gather(even, idx)
        kv[k + 8] = _gather(pltpu.roll(jnp.where(lo, p[1], p[0]), 4, 0), idx)
        if k % 512 == 0:
            up[k] = _gather(even, nxt)
    q = lane & 3
    s3 = {r: jnp.where(q == 2, kv[1024 + r], kv[1536 + r]) for r in (0, 8)}
    v0 = jnp.where(q == 0, kv[0], jnp.where(q == 1, kv[512], s3[0]))
    q16 = q + jnp.where(lane >= 124, 1, 0)
    v16 = jnp.where(q16 < 2, jnp.where(q16 == 0, up[0], up[512]),
                    jnp.where(q16 == 2, up[1024], jnp.where(q16 == 3, up[1536], k_last)))
    s3[16] = v16
    s23, s123, out = {}, {}, [v0]
    for r in range(1, 16):
        k23 = (RES2[r], RES3[r])
        if k23 not in s23:
            s23[k23] = v16 if k23 == (16, 16) else jnp.where(q == 1, kv[512 + k23[0]], s3[k23[1]])
        k123 = (RES1[r],) + k23
        if k123 not in s123:
            s123[k123] = v16 if k123[0] == 16 else jnp.where(q == 0, kv[k123[0]], s23[k23])
        if RES1[r] == r:
            out.append(s123[k123])
        else:
            out.append(jnp.where((q == 0) & (lane < 64), kv[r], s123[k123]))
    return out


def _ln_scalars(s1, s2):
    mean = s1 * (1.0 / D)
    var = jnp.maximum(s2 * (1.0 / D) - mean * mean, 0.0)
    eps = float(np.asarray(EPS, dtype=BF16))
    sd = _rbf(jnp.sqrt(_rbf(_rbf(var) + eps)))
    return _rbf(mean), 1.0 / sd


def _top8(x):
    def swap(v, pairs):
        for i, j in pairs:
            v[i], v[j] = jnp.maximum(v[i], v[j]), jnp.minimum(v[i], v[j])
        return v

    def merge(a, b):
        v = [jnp.maximum(a[i], b[7 - i]) for i in range(8)]
        return swap(v, [(i, i + d) for d in (4, 2, 1) for i in range(8) if not i & d])

    sort8 = ((0, 2), (1, 3), (4, 6), (5, 7), (0, 4), (1, 5), (2, 6), (3, 7), (0, 1), (2, 3),
             (4, 5), (6, 7), (2, 4), (3, 5), (1, 4), (3, 6), (1, 2), (3, 4), (5, 6))
    v = merge(*[swap([x[64 * h + 8 * i:64 * h + 8 * i + 8] for i in range(8)], sort8)
                for h in range(2)])
    for d in (4, 2, 1):
        v = merge(v, [pltpu.roll(t, d, 0) for t in v])
    return v


def _init_columns(col_ref, ldt_ref, dsk_ref, wr_ref):
    row, lane = _iota((128, 128), 0), _iota((128, 128), 1)
    split = (row & ~15) + 2 * (row & 7) + ((row >> 3) & 1)
    ldt, dsk, wr = (ref[...].astype(F32).reshape(1, D) for ref in (ldt_ref, dsk_ref, wr_ref))
    for n, (vec, src) in enumerate(((jnp.exp(ldt), split), (dsk * (1.0 / L), split), (wr, row))):
        for lo in range(0, D, 128):
            i = min(lo, D - 128)
            diag = jnp.where(src == lane, vec[:, i:i + 128], 0.0)[lo - i:].astype(BF16)
            col_ref[n, lo:i + 128, :] = jnp.dot(diag, jnp.ones((128, 128), BF16),
                                                preferred_element_type=F32)


class _Schedule:
    def __init__(self, zero):
        self.zero = zero
        self.sub, self.lane = _iota((8, 128), 0) + zero, _iota((8, 128), 1) + zero
        self.true = self.sub >= 0
        self.done, self.pending, self.wait = [], {}, -1

    def tie(self, x, token):
        return jnp.where(self.true, x, token if token.dtype == x.dtype
                         else pltpu.bitcast(token, x.dtype))

    def start(self, x):
        return self.tie(x, self.done[self.wait]) if 0 <= self.wait < len(self.done) else x

    def lhs(self, words, first):
        tiles = [words[i:i + 8] for i in range(0, words.shape[0], 8)]
        for i in range(len(tiles) if first else 0):
            for token in self.pending.pop(len(self.done) + i, ()):
                tiles[i] = self.tie(tiles[i], token)
        return _mxu(jnp.concatenate(tiles, axis=0))

    def results(self, v):
        self.done += [v[i + 8:i + 16] for i in range(0, v.shape[0], 16)]

    def run(self, stage, wait, before):
        self.wait = wait
        self.pending.setdefault(before, []).extend(next(stage))


def _kernel(x_hbm, are_hbm, aim_hbm, bre_hbm, bim_hbm, cre_hbm, cim_hbm,
            ldt_hbm, dsk_hbm, wr_hbm, wg_hbm, wu_hbm, wd_hbm, out_hbm,
            x_v, wg_v, wu_v, wd_v, par_v, ldt_v, dsk_v, wr_v, w_v, wk_v, wt_v, col_v,
            tmp_v, h_v, st_v, acc_v, out_v, sd0, sd1, ta0, ta1, tb0, tb1, kl0, kl1,
            u0, u1, k0, k1, a0_v, a1_v, c0, c1, y0, y1, order_s,
            sem_p, sem_x, sem_w, sem_o, f0_v, f1_v, *new_v):
    cp_vec = [pltpu.make_async_copy(s, d, sem_p.at[n]) for n, (s, d) in enumerate(
        ((ldt_hbm, ldt_v), (dsk_hbm, dsk_v), (wr_hbm, wr_v)))]
    cp_par = [[pltpu.make_async_copy(s.at[lo:hi], par_v.at[n, lo:hi], sem_p.at[3 + 6 * m + n])
               for n, s in enumerate((are_hbm, aim_hbm, bre_hbm, bim_hbm, cre_hbm, cim_hbm))]
              for m, (lo, hi) in enumerate(((0, 3 * MB), (3 * MB, D)))]
    cp_x = [pltpu.make_async_copy(x_hbm.at[:, 128 * j:128 * j + 128], x_v.at[j], sem_x.at[j])
            for j in range(NT)]
    cp_w = [pltpu.make_async_copy(s, d, sem_w.at[n]) for n, (s, d) in enumerate(
        ((wg_hbm, wg_v), (wu_hbm, wu_v), (wd_hbm, wd_v)))]
    for cp in cp_vec + cp_par[0]:
        cp.start()
    for cp in cp_x[:NT // 2]:
        cp.start(priority=1)

    def columns():
        for cp in cp_vec:
            cp.wait()
        for cp in cp_x[NT // 2:]:
            cp.start(priority=1)
        _init_columns(col_v, ldt_v, dsk_v, wr_v)

    _init_dft(w_v, wk_v, wt_v, tmp_v, columns)
    with jax.named_scope("S_pwait"):
        for cp in cp_par[0]:
            cp.wait()

    sd, ta, tb, kl = (sd0, sd1), (ta0, ta1), (tb0, tb1), (kl0, kl1)
    uk, ab, cc, yy = ((u0, u1), (k0, k1)), ((a0_v, a1_v), (f0_v, f1_v)), (c0, c1), (y0, y1)
    ww, wt_w = (w_v.bitcast(I32), wk_v.bitcast(I32)), wt_v

    def chan(b, r):
        return _ds(b * MB + 16 * r, 16)

    def seed_stage(b, r, sch):
        rows = _ds(b * MB // 2 + 8 * r, 8)
        par = [_unpack(par_v.bitcast(I32)[n, rows, :]) for n in range(6)]
        for h in range(2):
            a_re, a_im, b_re, b_im, c_re, c_im = [v[h] for v in par]
            dt = sch.start(col_v[0, _ds(b * MB + 16 * r + 8 * h, 8), :])
            mag, ang = jnp.exp(dt * a_re), dt * a_im
            sc = dt * (1.0 / L)
            seeds = _k_seeds((mag * jnp.cos(ang), mag * jnp.sin(ang)),
                             _cmul((c_re, c_im), (sc * b_re, sc * b_im)), sch.sub < 4)
            for g in range(2):
                for n, v in enumerate(seeds[g]):
                    for p in range(2):
                        sd[b % 2][r, 2 * h + g, 2 * n + p] = v[p]
            yield [sd[b % 2][(r + sch.zero), 2 * h, 0]]

    def table_stage(b, r, sch):
        tail = []
        for g in range(4):
            m1, m32, m512, a0, b0 = [
                (sd[b % 2][r, g, 2 * n], sd[b % 2][r, g, 2 * n + 1]) for n in range(5)]
            m32 = (sch.start(m32[0]), m32[1])
            fa = [a0]
            for _ in range(7):
                fa.append(_cmul(fa[-1], m1))
            for src in (0, 4, 8, 10):
                fa.append(_cmul(fa[src], m512))
            tail.append(fa[11][0] * m512[0] - fa[11][1] * m512[1])
            _store_table(ta[b % 2].at[r, g], fa)
            fb = [b0]
            for _ in range(15):
                p = fb[-1]
                fb.append((p[0] * m32[0] + p[1] * m32[1], p[1] * m32[0] - p[0] * m32[1]))
            _store_table(tb[b % 2].at[r, g], fb)
            yield [ta[b % 2].bitcast(I32)[(r + sch.zero), g, 0, 0:8, :],
                   tb[b % 2].bitcast(I32)[(r + sch.zero), g, 0, 0:8, :]]
        lo = sch.sub < 4
        kl[b % 2][r] = _pack(*[jnp.broadcast_to(
            jnp.sum(jnp.where(lo, tail[2 * h], tail[2 * h + 1]), axis=1, keepdims=True),
            (8, 128)) for h in range(2)])

    def kernel_stage(b, r, sch):
        ta_w, tb_w = ta[b % 2].bitcast(I32), tb[b % 2].bitcast(I32)
        groups = [None] * 4
        for g0 in range(2):
            res = [jax.lax.dot_general(sch.lhs(ta_w[r, g, p, 0:48], g == g0 and p == 0),
                                       _mxu(tb_w[r, g, p, 0:64]), NT_DIMS, preferred_element_type=F32)
                   for g in (g0, g0 + 2) for p in range(2)]
            groups[g0], groups[g0 + 2] = res[0] + res[1], res[2] + res[3]
            sch.results(groups[g0 + 2])
            yield []
        dskip = [col_v[1, _ds(b * MB + 16 * r + 8 * h, 8), :] for h in range(2)]
        dst = _ds(8 * r, 8)
        res = _k_residues(groups, kl[b % 2][r], dskip, sch.sub, sch.lane)
        for s, t in enumerate(res):
            uk[1][b % 2][s, dst, :] = t
        yield [uk[1][b % 2][0, _ds(8 * (r + sch.zero), 8), :]]

    def norm_stage(b, r, sch):
        tiles = []
        rows = _ds(b * MB // 2 + 8 * r, 8)
        for j in range(NT):
            m, inv = st_v[0, j] if j else sch.start(st_v[0, j]), st_v[1, j]
            tiles.append(_pack(*[(v - m) * inv for v in _unpack(x_v.bitcast(I32)[j, rows, :])]))
        dst = _ds(8 * r, 8)
        res = _to_residues(tiles, sch.lane)
        for s, t in enumerate(res):
            uk[0][b % 2][s, dst, :] = t
        yield [uk[0][b % 2][0, _ds(8 * (r + sch.zero), 8), :]]

    def forward_stage(w, b, k, sch):
        dst = ab[w][b % len(ab[w])]
        for p in range(2):
            v = [jnp.dot(sch.lhs(uk[w][b % 2][k + 4 * n, 0:MB // 2], n == 0),
                         _mxu(ww[w][k + 4 * n, p ^ (n & 1), 0:64]),
                         preferred_element_type=F32) for n in range(4)]
            d02, d13 = v[0] - v[2], v[1] - v[3]
            x1 = d02 - d13 if p == 0 else d02 + d13
            dst[k, 0, p, 0:MB] = v[0] + v[2]
            dst[k, 2, 1 - p, 0:MB] = v[1] + v[3]
            dst[k, 1, p, 0:MB] = x1
            dst[k, 3, p, 0:MB] = d02 + d13 if p == 0 else d02 - d13
            sch.results(x1)
            yield []

    def stats_stage(b, r, sch):
        for n in range(2):
            j = 8 * b + 2 * r + n
            acc = None
            for i in range(0, D // 2, 8):
                v = _unpack(x_v.bitcast(I32)[j, i:i + 8, :])
                v += [t * t for t in v]
                acc = v if acc is None else [p + q for p, q in zip(acc, v)]
            s1, s2 = acc[0] + acc[1], acc[2] + acc[3]
            for d in (4, 2, 1):
                s1, s2 = s1 + pltpu.roll(s1, d, 0), s2 + pltpu.roll(s2, d, 0)
            st_v[0, j], st_v[1, j] = m, inv = _ln_scalars(s1, s2)
            yield [inv]

    def middle_stage(b, r, sch):
        src = [v[b % len(v)] for v in ab]
        scale = lambda v, f: [(x[0] * f, x[1] * f) for x in v]
        for h in range(2):
            ra = _ds(16 * r + 8 * h, 8)
            ld = lambda q, w: [(src[w][k, q, 0, ra, :], src[w][k, q, 1, ra, :]) for k in range(4)]

            def put(q, x, y):
                for k in range(4):
                    for p in range(2):
                        cc[b % 2][k, q, p, ra, :] = x[k][p] + y[k][p]
                        cc[b % 2][k, q + 1, p, ra, :] = x[k][p] - y[k][p]

            gate = sch.start
            a0, a2, b0, b2 = ld(0, 0), ld(2, 0), ld(0, 1), ld(2, 1)
            a0[0] = (gate(a0[0][0]), a0[0][1])
            e0 = _prod_mod_1(list(map(_cadd, a0, a2)), list(map(_cadd, b0, b2)))
            e2 = _prod_mod_m1(list(map(_csub, a0, a2)), scale(map(_csub, b0, b2), 2.0))
            put(0, e0, e2)
            again = _ds(16 * (r + sch.zero) + 8 * h, 8)
            yield [cc[b % 2][0, 0, 0, again, :]]
            four = sch.start(jnp.full((8, 128), 4.0, F32))
            e1 = _prod_mod_i(ld(1, 0), scale(ld(1, 1), four), 1)
            e3 = _prod_mod_i(ld(3, 0), scale(ld(3, 1), four), -1)
            put(2, e1, e3)
            yield [cc[b % 2][0, 2, 0, again, :]]

    def inverse_stage(b, k, sch):
        src = cc[b % 2]

        def lhs(v, first):
            return sch.lhs(jnp.concatenate(
                [_pack(v[i:i + 8], v[i + 8:i + 16]) for i in range(0, MB, 16)], axis=0), first)

        for o in range(2):
            p0, p1 = [(src[k, q, 0, 0:MB], src[k, q, 1, 0:MB]) for q in (o, o + 2)]
            if o == 0:
                e = {0: _cadd(p0, p1), 2: _csub(p0, p1)}
            else:
                e = {1: (p0[0] + p1[1], p0[1] - p1[0]), 3: (p0[0] - p1[1], p0[1] + p1[0])}
            ys = []
            for n in e:
                y = [jnp.dot(lhs(e[n][p], n == o and p == 0), _mxu(wt_w[k + 4 * n, p, 0:64]),
                             preferred_element_type=F32)
                     for p in range(2)]
                ys.append(y[0] + y[1])
                yy[b % 2][k + 4 * n, 0:MB] = ys[-1].astype(BF16)
            sch.results(ys[-1])
            yield []

    def residual_stage(b, r, sch):
        rows = chan(b, r)
        wr = col_v[2, rows, :]
        src = yy[b % 2].bitcast(I32)
        ys = _to_time([src[s, _ds(8 * r, 8), :] for s in range(16)], sch.lane)
        for j in range(NT):
            h = x_v[j, rows, :].astype(F32) + jnp.concatenate(
                _unpack(ys[j] if j % 8 else sch.start(ys[j])), axis=0)
            h_v[j, rows, :] = h.astype(BF16)
            hh, hw = h * h, h * wr
            acc_v[0, j] += h[0:8] + h[8:16]
            acc_v[1, j] += hh[0:8] + hh[8:16]
            acc_v[2, j] += hw[0:8] + hw[8:16]
            if j % 8 == 7:
                yield [acc_v[0, (r + sch.zero)]]

    nb = D // MB
    stages = dict(
        s=(seed_stage, 0), t=(table_stage, 1), k=(kernel_stage, 2),
        F=(functools.partial(forward_stage, 1), 3), n=(norm_stage, 2),
        f=(functools.partial(forward_stage, 0), 3), m=(middle_stage, 4),
        i=(inverse_stage, 5), r=(residual_stage, 6))

    def run(step, zero, live=None):
        live = live or {n: (f, step - lag) for n, (f, lag) in stages.items()
                        if 0 <= step - lag < nb and (n, step) != ("n", 2)}
        unroll, plan = PLANS.get("".join(live), PLANS["default"])

        def body(it, carry):
            sch = _Schedule(zero >> (step % 32) if unroll == 4 else zero & it)
            gens = [{n: f(b, it * unroll + u, sch) for n, (f, b) in live.items()}
                    for u in range(unroll)]
            for item in plan.split():
                u, n, *ties = item.split(":")
                if n in live:
                    sch.run(gens[int(u)][n], *map(int, ties or (-1, -1)))
            for g in gens:
                for v in g.values():
                    for _ in v:
                        pass
            return carry + it

        with jax.named_scope("S_p%d" % step):
            if unroll == 4:
                return body(0, 0)
            return jax.lax.fori_loop(0, 4 // unroll, body, 0)

    acc_v[...] = jnp.zeros(acc_v.shape, F32)
    zero = run(0, 0) - 6
    for step in STEPS:
        if step == 1:
            for cp in cp_par[1]:
                cp.start()
        if step == 2:
            for cp in cp_w:
                cp.start(priority=1)
        if step == 3:
            for cp in cp_par[1]:
                cp.wait()
            for half in range(2):
                with jax.named_scope("S_xwait"):
                    for cp in cp_x[NT // 2 * half:NT // 2 * (half + 1)]:
                        cp.wait()
                run(100, zero, dict(l=(stats_stage, half)))
            run(101, zero, dict(n=(norm_stage, 0)))
        run(step, zero)

    def rows_of(q):
        return jnp.concatenate(
            [jnp.sum(acc_v[q, j], axis=0, keepdims=True) for j in range(NT)], axis=0)

    m2, inv2 = _ln_scalars(rows_of(0), rows_of(1))
    wsum = jnp.sum(col_v[2], axis=0, keepdims=True)
    score = _rbf((rows_of(2) - m2 * wsum) * inv2 + 0.0)
    bits = pltpu.bitcast(score, I32) >> 16
    order = jnp.where(bits < 0, -1 - bits, bits + 32768)
    pos = 128 * _iota((NT, 128), 0) + _iota((NT, 128), 1)
    key = pltpu.bitcast((order << 11) + (L - 1 - pos) + (1 << 29), F32)

    lane8, sub8 = _iota((CAP, 128), 1), _iota((CAP, 128), 0)
    best = _top8(jnp.tile(key, (8, 1)).T)
    cand = best[0]
    for c in range(1, CAP):
        cand = jnp.where((lane8 >> 4) == c, best[c], cand)
    best = [pltpu.bitcast(v, I32)[0, 0] for v in _top8(cand.T)]
    aux = [jnp.zeros((CAP, 128), F32)] * 3
    for c in range(CAP):
        hit = pltpu.bitcast(key, I32) == best[c]
        aux = [jnp.where(sub8 == c, jnp.sum(jnp.where(hit, v, 0.0), axis=0, keepdims=True), a)
               for a, v in zip(aux, (m2, inv2, score))]
    m_sel, inv_sel, score_sel = [jnp.sum(a, axis=1, keepdims=True) for a in aux]
    picks = [L - 1 - (v & (L - 1)) for v in best]
    tile, col = [t >> 7 for t in picks], [t & 127 for t in picks]
    rnd = [sum([(col[e] == col[c]).astype(I32) for e in range(c)], 0) for c in range(CAP)]
    rounds = functools.reduce(jnp.maximum, rnd) + 1
    lane_in = lambda n, c: lane8 == jnp.where(rnd[c] == n, col[c], -1)

    def out_copy(q, lo, hi, n):
        j = order[q]
        return pltpu.make_async_copy(
            out_v.at[j, lo:hi], out_hbm.at[lo:hi, _ds(j * 128, 128)], sem_o.at[n])

    h_w, out_w = h_v.bitcast(I32), out_v.bitcast(I32)

    def gather(n, acc):
        masks = [lane_in(n, c) for c in range(CAP)]
        tiles = []
        for i in range(0, D // 2, 8):
            v = jnp.zeros((8, 128), I32)
            for c in range(CAP):
                v = jnp.where(masks[c], h_w[tile[c], i:i + 8, :], v)
            tiles.append(v)
        lhs = jnp.zeros((CAP, 128), F32)
        for c in range(CAP):
            lhs = jnp.where(masks[c] & (sub8 == c), 1.0, lhs)
        return acc + jax.lax.dot_general(lhs.astype(BF16), _mxu(jnp.concatenate(tiles, axis=0)),
                                         NT_DIMS, preferred_element_type=F32)

    with jax.named_scope("S_gather"):
        h_sel = jax.lax.fori_loop(0, rounds, gather, jnp.zeros((CAP, D), F32))
    x_sel = _rbf((h_sel - m_sel) * inv_sel)
    gate = _rbf(jax.nn.sigmoid(score_sel))

    true = lane8 + picks[0] >= 0
    tie = lambda x, token: jnp.where(true, x, token)

    def unrouted(j0):
        token = lane8
        for j in range(j0, j0 + NT // 2):
            inv = jnp.broadcast_to(inv2[j:j + 1], (8, 128))
            mul, sub = 1.0 + inv, m2[j:j + 1] * inv
            for i in range(0, D // 2, 8):
                res = _pack(*[h * mul - sub for h in _unpack(h_w[j, i:i + 8, :])])
                out_w[j, i:i + 8, :] = res
                token = token ^ res
                yield pltpu.bitcast(token, F32)

    def project(w_ref, j0):
        parts, side = [], unrouted(j0)
        for n in range(0, FF, 128):
            token = [next(side) for _ in range(8)][-1]
            xs = jnp.concatenate([tie(x_sel[:, :128], token), x_sel[:, 128:]], axis=1)
            parts.append(jnp.dot(xs.astype(BF16), w_ref[:, n:n + 128],
                                 preferred_element_type=F32))
        return _rbf(jnp.concatenate(parts, axis=1))

    with jax.named_scope("S_gwait"):
        cp_w[0].wait()
        cp_w[1].wait()
    g = project(wg_v, 0)
    act = _rbf(g * jax.nn.sigmoid(g)) * project(wu_v, NT // 2)
    routed = functools.reduce(jnp.bitwise_or, [1 << j for j in tile])
    spare = CAP - sum((routed >> j) & 1 for j in range(NT))
    n_late = 0
    for j in range(NT):
        hit = (routed >> j) & 1
        fill = (1 - hit) & (spare > 0).astype(I32)
        spare = spare - fill
        order_s[jnp.clip(jnp.where(hit + fill == 1, CAP + n_late, j - n_late), 0, NT - 1)] = j
        n_late = n_late + hit + fill

    order = [order_s[q] for q in range(NT)]
    for q in range(CAP):
        out_copy(q, 0, D, q).start()
    with jax.named_scope("S_dwait"):
        cp_w[2].wait()

    def placed(r, words):
        idx = jnp.zeros((CAP, 128), I32)
        for c in range(1, CAP):
            idx = jnp.where(lane_in(r, c), c, idx)
        return [_gather(w, idx) for w in words]

    def late_copies(n, lo, hi):
        return [out_copy(CAP + q, lo, hi, CAP * (n + 1) + q) for q in range(CAP)]

    def words_of(n):
        return [new_v[n].bitcast(I32)[i:i + 8, :] for i in range(0, new_v[n].shape[0] // 2, 8)]

    tokens = []
    for n, (lo, hi) in enumerate(ROW_CHUNKS):
        a = [act[:, i:i + 128] for i in range(0, FF, 128)]
        if n >= 2:
            cut = 12 * 128 // (hi - lo)
            a[cut] = tie(a[cut], tokens[n - 2])
        a = jnp.concatenate(a, axis=1)
        y = _rbf(jax.lax.dot_general(a.astype(BF16), wd_v[lo:hi, :], NT_DIMS,
                                     preferred_element_type=F32))
        new = h_sel[:, lo:hi] + _rbf(x_sel[:, lo:hi] + _rbf(y * gate))
        new_v[n][...] = jnp.concatenate(
            [new.T, jnp.zeros((hi - lo, 128 - CAP), F32)], axis=1).astype(BF16)
        rows = range(lo // 2, hi // 2, 8)
        words = words_of(n)
        both = list(zip(rows, placed(0, words), placed(1, words)))
        for c in range(CAP):
            for i, v0, v1 in both:
                pltpu.store(out_w.at[tile[c], pl.ds(i, 8), :],
                            jnp.where(rnd[c] == 0, v0, v1), mask=lane8 == col[c])
        for cp in late_copies(n, lo, hi):
            cp.start()
        out_w[tile[0], D // 2:, :] = lane8
        tokens.append(pltpu.bitcast(out_w[tile[0] | zero, D // 2:, :], F32))
    with jax.named_scope("S_owait"):
        for q in range(CAP):
            out_copy(q, 0, D, q).wait()
        for n, (lo, hi) in enumerate(ROW_CHUNKS):
            for cp in late_copies(n, lo, hi):
                cp.wait()

    @pl.when(rounds > 2)
    def _():
        def fix(r, carry):
            rows = range(0, D // 2, 8)
            vals = placed(r, sum(map(words_of, range(len(new_v))), []))
            for c in range(CAP):
                for i, v in zip(rows, vals):
                    pltpu.store(out_w.at[tile[c], pl.ds(i, 8), :], v, mask=lane_in(r, c))
            return carry

        jax.lax.fori_loop(2, rounds, fix, 0)
        for cp in late_copies(0, 0, D):
            cp.start()
        for cp in late_copies(0, 0, D):
            cp.wait()


@jax.jit
def pallas_sequential_preLN__ssm_conv_s4__moe_arch_mod__prompt_kernel(
    A_u: jax.Array,
    A_A_re: jax.Array,
    A_A_im: jax.Array,
    A_B_re: jax.Array,
    A_B_im: jax.Array,
    A_C_re: jax.Array,
    A_C_im: jax.Array,
    A_log_dt: jax.Array,
    A_Dskip: jax.Array,
    B_x: jax.Array,
    B_w_r: jax.Array,
    B_w_gate: jax.Array,
    B_w_up: jax.Array,
    B_w_down: jax.Array,
):
    del B_x
    hbm = pl.BlockSpec(memory_space=pl.ANY)
    out = pl.pallas_call(
        _kernel,
        out_shape=jax.ShapeDtypeStruct((D, L), BF16),
        in_specs=[hbm] * 13,
        out_specs=hbm,
        scratch_shapes=[
            pltpu.VMEM((NT, D, 128), BF16),
            pltpu.VMEM((D, FF), BF16),
            pltpu.VMEM((D, FF), BF16),
            pltpu.VMEM((D, FF), BF16),
            pltpu.VMEM((6, D, N), BF16),
            *[pltpu.VMEM((D,), BF16)] * 3,
            *[pltpu.VMEM((16, 2, 144, 128), BF16)] * 2,
            pltpu.VMEM((16, 2, 72, 128), I32),
            pltpu.VMEM((3, D, 128), F32),
            pltpu.VMEM((2, 256, 128), F32),
            pltpu.VMEM((NT, D, 128), BF16),
            pltpu.VMEM((2, NT, 8, 128), F32),
            pltpu.VMEM((3, NT, 8, 128), F32),
            pltpu.VMEM((NT, D + 16, 128), BF16),
            *[pltpu.VMEM((4, 4, 10, 8, 128), F32)] * 2,
            *[pltpu.VMEM((4, 4, 2, 112, 128), BF16)] * 2,
            *[pltpu.VMEM((4, 4, 2, 144, 128), BF16)] * 2,
            *[pltpu.VMEM((4, 8, 128), I32)] * 2,
            *[pltpu.VMEM((16, MB // 2 + 8, 128), I32)] * 4,
            *[pltpu.VMEM((4, 4, 2, MB + 8, 128), F32)] * 2,
            *[pltpu.VMEM((4, 4, 2, MB + 8, 128), F32)] * 2,
            *[pltpu.VMEM((16, MB + 16, 128), BF16)] * 2,
            pltpu.SMEM((NT,), I32),
            pltpu.SemaphoreType.DMA((15,)),
            pltpu.SemaphoreType.DMA((NT,)),
            pltpu.SemaphoreType.DMA((3,)),
            pltpu.SemaphoreType.DMA((CAP * (1 + len(ROW_CHUNKS)),)),
            *[pltpu.VMEM((4, 4, 2, MB + 8, 128), F32)] * 2,
            *[pltpu.VMEM((hi - lo, 128), BF16) for lo, hi in ROW_CHUNKS],
        ],
        compiler_params=pltpu.CompilerParams(vmem_limit_bytes=100 * 1024 * 1024,
                                             disable_bounds_checks=True,
                                             disable_semaphore_checks=True),
    )(A_u.reshape(L, D).T, A_A_re, A_A_im, A_B_re, A_B_im, A_C_re, A_C_im,
      A_log_dt, A_Dskip, B_w_r, B_w_gate, B_w_up, B_w_down.T)
    return out.T.reshape(1, L, D)
```

```python
import functools

import numpy as np
import jax
import jax.numpy as jnp
import jax.experimental.pallas as pl
import jax.experimental.pallas.tpu as pltpu

F32 = jnp.float32
BF16 = jnp.bfloat16
I32 = jnp.int32

L = 2048
D = 576
N = 128
FF = 4608
CAP = 8
NT = L // 128
EPS = 1e-5
MB = 64
PLANS = dict(
    stk=(2, "0:t:-1:3 1:t:-1:4 0:t:-1:6 0:t:-1:8 1:t:-1:10 0:t:-1:12 1:t:3:17 1:t:11:-1 0:k "
            "0:k 1:k 0:s:-1:20 0:s:11:-1 0:k:-1:22 1:k 1:s:23:-1 1:s 1:k "),
    stkFnf=(1, "0:n:-1:10 0:t:-1:6 0:s:-1:16 0:s 0:f 0:t:3:19 0:k 0:k 0:t:13:-1 0:k 0:f 0:F "
               "0:t:21:-1 0:F "),
    stkFnfm=(1, "0:m:-1:3 0:t:-1:7 0:t:-1:16 0:t:-1:9 0:s:-1:25 0:s 0:f 0:m:1:13 0:f 0:m:6:18 "
                "0:k 0:t:9:22 0:n:10:27 0:k 0:m:14:26 0:k 0:F 0:F "),
    stkFnfmi=(1, "0:t:-1:6 0:t:-1:3 0:m:-1:6 0:n:-1:9 0:s:-1:32 0:f 0:s:0:31 0:k 0:m:8:22 0:k "
                 "0:m:13:25 0:k:-1:30 0:f 0:t:16:30 0:t:14:-1 0:F 0:F 0:i 0:i 0:m:32:-1 "),
    stkFnfmiar=(1, "0:t:-1:3 0:t:-1:3 0:n:-1:9 0:m:-1:6 0:s 0:f 0:m:0:16 0:k 0:s:4:35 0:k "
                   "0:r:11:22 0:m:14:25 0:k:-1:33 0:f 0:t:16:33 0:t:17:33 0:F 0:r:22:-1 0:F "
                   "0:i 0:i 0:m:33:-1 0:a "),
    tkFnfmiar=(1, "0:t:-1:6 0:t:-1:3 0:n:-1:6 0:m:-1:6 0:f 0:m:2:19 0:k 0:r:9:21 0:k 0:m:14:28 "
                  "0:k:-1:33 0:f 0:t:16:33 0:t:19:-1 0:F 0:r:23:-1 0:F 0:i 0:i 0:m:32:-1 0:a "),
    kFnfmiar=(2, "1:m:-1:5 0:F 0:n:0:13 0:k 0:m:4:15 0:m:8:19 0:F 0:m:12:22 0:k 0:m:19:31 "
                 "0:k:-1:39 0:f 0:i 0:f 0:i 0:r:32:43 1:n:35:51 0:a 1:F 1:m:40:52 1:k "
                 "1:r:44:56 1:F 1:m:49:58 1:k 0:r:54:64 1:k:-1:72 1:f 1:i 1:f 1:r:65:-1 "
                 "1:m:67:-1 1:i 1:a "),
    Ffmiar=(2, "1:m:-1:6 1:m:-1:11 0:F 0:F 0:m:4:16 0:f 0:m:8:21 0:i 0:m:13:28 0:f 0:m:18:31 "
               "0:i 0:r:23:34 0:a 1:F 0:r:27:39 1:F 1:f 1:r:34:45 1:r:35:-1 1:i 1:f 1:m:41:-1 "
               "1:i 1:m:45:-1 1:a "),
    miar=(2, "1:m:-1:2 0:m:-1:6 0:i 0:m:0:8 0:m:1:11 0:r:3:14 0:i 1:r:5:15 0:r:5:14 0:a "
             "1:m:8:17 1:i 1:r:10:-1 1:m:12:-1 1:i 0:m:15:-1 1:a 1:m:17:-1 "),
    iar=(4, "2:r:-1:14 0:i 0:i 0:r:7:19 0:a 1:i 0:r:10:23 1:i 1:r:13:27 2:r:15:29 1:a 2:i 2:i "
            "3:r:22:-1 1:r:24:35 2:a 3:i 3:i 3:r:34:-1 3:a "),
    ar=(4, "0:a 1:a 2:a 3:a "),
    l=(2, ""),
    n=(4, ""),
    default=(1, ""),
)
ROW_CHUNKS = ((0, 128), (128, 256), (256, 384), (384, 512), (512, D))
NT_DIMS = (((1,), (1,)), ((), ()))


def _round_res(step):
    return [int(np.round(r / step)) * step for r in range(16)]


RES1, RES2, RES3 = _round_res(2), _round_res(4), _round_res(8)


def _ds(start, size):
    return pl.ds(start if isinstance(start, int) else pl.multiple_of(start, size), size)


def _iota(shape, dim):
    return jax.lax.broadcasted_iota(I32, shape, dim)


def _rbf(x):
    return x.astype(BF16).astype(F32)


def _cmul(a, b):
    return (a[0] * b[0] - a[1] * b[1], a[0] * b[1] + a[1] * b[0])


def _csq(a):
    t = a[0] * a[1]
    return ((a[0] + a[1]) * (a[0] - a[1]), t + t)


def _cadd(a, b):
    return (a[0] + b[0], a[1] + b[1])


def _csub(a, b):
    return (a[0] - b[0], a[1] - b[1])


def _bfly4(a0, a1, a2, a3, inverse=False):
    s02, d02 = _cadd(a0, a2), _csub(a0, a2)
    s13, d13 = _cadd(a1, a3), _csub(a1, a3)
    p = (d02[0] - d13[1], d02[1] + d13[0])
    m = (d02[0] + d13[1], d02[1] - d13[0])
    if inverse:
        p, m = m, p
    return _cadd(s02, s13), p, _csub(s02, s13), m


def _prod_mod_1(a, b):
    fa, fb = _bfly4(*a), _bfly4(*b)
    return _bfly4(*[_cmul(x, y) for x, y in zip(fa, fb)], inverse=True)


def _prod2(a0, a1, b0, b1, sgn):
    p00, p11 = _cmul(a0, b0), _cmul(a1, b1)
    c1 = _cadd(_cmul(a0, b1), _cmul(a1, b0))
    if sgn > 0:
        return (p00[0] - p11[1], p00[1] + p11[0]), c1
    return (p00[0] + p11[1], p00[1] - p11[0]), c1


def _prod_mod_m1(a, b):
    def split(x):
        p = [(x[k][0] - x[k + 2][1], x[k][1] + x[k + 2][0]) for k in range(2)]
        m = [(x[k][0] + x[k + 2][1], x[k][1] - x[k + 2][0]) for k in range(2)]
        return p, m
    ap, am = split(a)
    bp, bm = split(b)
    cp = _prod2(*ap, *bp, 1)
    cm = _prod2(*am, *bm, -1)
    lo = [_cadd(cp[k], cm[k]) for k in range(2)]
    hi = [(cp[k][1] - cm[k][1], cm[k][0] - cp[k][0]) for k in range(2)]
    return lo + hi


def _prod_mod_i(a, b, sgn):
    sm = [x[0] + x[1] for x in b]
    df = [x[1] - x[0] for x in b]
    asum = [x[0] + x[1] for x in a]
    out = []
    for k in range(4):
        acc = [None, None, None]
        for j in range(4):
            m = (k - j) % 4
            if j <= k:
                t = ((b[m][0], 1), (df[m], 1), (sm[m], 1))
            elif sgn > 0:
                t = ((b[m][1], -1), (sm[m], 1), (df[m], -1))
            else:
                t = ((b[m][1], 1), (sm[m], -1), (df[m], 1))
            for q, (v, (w, s)) in enumerate(zip((asum[j], a[j][0], a[j][1]), t)):
                p = v * w
                if acc[q] is None:
                    acc[q] = p
                else:
                    acc[q] = acc[q] + p if s > 0 else acc[q] - p
        out.append((acc[0] - acc[2], acc[0] + acc[1]))
    return out


def _barrel(v, lane):
    for bit in range(4):
        m = ((lane >> bit) & 1) == 1
        v = [jnp.where(m, v[(i + (1 << bit)) % 16], v[i]) for i in range(16)]
    return [v[-s % 16] for s in range(16)]


def _to_residues(tiles, lane):
    return _barrel([t if j == 0 else pltpu.roll(t, j, 1) for j, t in enumerate(tiles)], lane)


def _to_time(res, lane):
    return [t if j == 0 else pltpu.roll(t, 128 - j, 1)
            for j, t in enumerate(_barrel(res, lane))]


def _gather(x, idx, axis=1):
    return jnp.take_along_axis(x, idx, axis=axis, mode="promise_in_bounds")


def _init_dft(wu_ref, wk_ref, wt_ref, tmp_ref, halfway):
    sub, k4 = _iota((8, 128), 0), 4 * _iota((8, 128), 1) + 1

    def cis(t):
        ph = ((k4 * t) & (4 * L - 1)).astype(F32) * (2 * np.pi / (4 * L))
        return jnp.cos(ph), jnp.sin(ph)

    w1, w16 = cis(1), cis(16)
    w32 = _csq(w16)
    fk = [cis(16 * (32 * (sub & 3) + (sub >> 2)))]
    fu = [cis(128 * sub), cis(128 * (sub + 8))]
    for v in range(1, 16):
        fk.append(_cmul(fk[-1], w32))
        if v >= 2:
            fu.append(_cmul(fu[-2], w16))
    for p in range(2):
        for v in range(32):
            tmp_ref[p, 8 * v:8 * v + 8, :] = fu[v % 16][p]
    tw = None
    for s in range(16):
        for v in range(0, 16, 2):
            rows = [slice(128 - s + 8 * i, 136 - s + 8 * i) for i in (v, v + 1)]
            for ref, f in ((wk_ref, fk[v:v + 2]),
                           (wu_ref, [(tmp_ref[0, r, :], tmp_ref[1, r, :]) for r in rows])):
                if s:
                    f = [_cmul(x, tw) for x in f]
                for p in range(2):
                    ref[s, p, 8 * v:8 * v + 16, :] = jnp.concatenate(
                        [f[0][p], f[1][p]], axis=0).astype(BF16)
        for p in range(2):
            wt_ref[s, p, 0:64] = pltpu.bitcast(_mxu(wu_ref.bitcast(I32)[s, p, 0:64]).T, I32)
        tw = _cmul(tw, w1) if s else w1
        if s == 7:
            halfway()


def _pack(ref, n, a, b):
    ref[n] = jnp.concatenate([a, b], axis=0).astype(BF16)
    return ref.bitcast(I32)[n]


def _split(w):
    return [pltpu.bitcast(w << 16, F32), pltpu.bitcast(w & -65536, F32)]


FINE = (0, 1, 2, 3, 4, 5, 6, 7, 512, 516, 1024, 1536)


def _k_seeds(z, c, sub):
    pw = {1: z}
    for e in range(1, 10):
        pw[1 << e] = _csq(pw[1 << (e - 1)])
    c8, z16 = _cmul(c, pw[8]), (pw[16][0], 0.0 - pw[16][1])
    pair = lambda a, b: tuple(jnp.where((sub & 1) == 0, p, q) for p, q in zip(a, b))
    seeds = []
    for g in range(2):
        twice = lambda v: tuple(_gather(x, 4 * g + (sub >> 1), 0) for x in v)
        seeds.append([twice(z), twice(pw[32]), twice(pw[512]),
                      pair(twice(c), twice(c8)), pair((1.0, 0.0), twice(z16))])
    return seeds


def _mxu(words):
    return pltpu.bitcast(words, BF16)


def _store_table(ref, tab):
    for i in range(0, len(tab), 2):
        for p in range(2):
            ref[p, 8 * i:8 * i + 16, :] = jnp.concatenate(
                [tab[i][p], tab[i + 1][p]], axis=0).astype(BF16)


def _k_residues(groups, k_last, dskip, tmp_ref, sub, lane):
    src = lambda b: 8 * ((b >> 1) & 15) + 2 * (sub & 3) + (b & 1)
    idx, nxt = src(lane >> 2), src((lane >> 2) + 1)
    low = lambda x, y: (x & 65535) | (y << 16)
    high = lambda x, y: jax.lax.shift_right_logical(x, 16) | (y & -65536)
    kv, up = {}, {}
    for i, k in enumerate(FINE):
        v = [g[8 * i:8 * i + 8] for g in groups]
        if k == 0:
            v = [x + jnp.where((lane == sub) & ((sub & 1) == 0),
                               _gather(dskip[n // 2], 4 * (n % 2) + (sub >> 1), 0), 0.0)
                 for n, x in enumerate(v)]
        p = [_pack(tmp_ref, 2 * i + h, v[2 * h], v[2 * h + 1]) for h in range(2)]
        both = [_gather(x, idx) for x in p]
        kv[k], kv[k + 8] = low(*both), high(*both)
        if k % 512 == 0:
            up[k] = low(*[_gather(x, nxt) for x in p])
    k_last = _gather(k_last, 2 * (sub & 3) + (sub >> 2), 0)
    q = lane & 3
    s3 = {r: jnp.where(q == 2, kv[1024 + r], kv[1536 + r]) for r in (0, 8)}
    v0 = jnp.where(q == 0, kv[0], jnp.where(q == 1, kv[512], s3[0]))
    q16 = q + jnp.where(lane >= 124, 1, 0)
    v16 = jnp.where(q16 < 2, jnp.where(q16 == 0, up[0], up[512]),
                    jnp.where(q16 == 2, up[1024], jnp.where(q16 == 3, up[1536], k_last)))
    s3[16] = v16
    s23, s123, out = {}, {}, [v0]
    for r in range(1, 16):
        k23 = (RES2[r], RES3[r])
        if k23 not in s23:
            s23[k23] = v16 if k23 == (16, 16) else jnp.where(q == 1, kv[512 + k23[0]], s3[k23[1]])
        k123 = (RES1[r],) + k23
        if k123 not in s123:
            s123[k123] = v16 if k123[0] == 16 else jnp.where(q == 0, kv[k123[0]], s23[k23])
        if RES1[r] == r:
            out.append(s123[k123])
        else:
            out.append(jnp.where((q == 0) & (lane < 64), kv[r], s123[k123]))
    return out


def _ln_scalars(s1, s2):
    mean = s1 * (1.0 / D)
    var = jnp.maximum(s2 * (1.0 / D) - mean * mean, 0.0)
    eps = float(np.asarray(EPS, dtype=BF16))
    sd = _rbf(jnp.sqrt(_rbf(_rbf(var) + eps)))
    return _rbf(mean), 1.0 / sd


def _top8(x):
    def swap(v, pairs):
        for i, j in pairs:
            v[i], v[j] = jnp.maximum(v[i], v[j]), jnp.minimum(v[i], v[j])
        return v

    def merge(a, b):
        v = [jnp.maximum(a[i], b[7 - i]) for i in range(8)]
        return swap(v, [(i, i + d) for d in (4, 2, 1) for i in range(8) if not i & d])

    sort8 = ((0, 2), (1, 3), (4, 6), (5, 7), (0, 4), (1, 5), (2, 6), (3, 7), (0, 1), (2, 3),
             (4, 5), (6, 7), (2, 4), (3, 5), (1, 4), (3, 6), (1, 2), (3, 4), (5, 6))
    v = merge(*[swap([x[64 * h + 8 * i:64 * h + 8 * i + 8] for i in range(8)], sort8)
                for h in range(2)])
    for d in (4, 2, 1):
        v = merge(v, [pltpu.roll(t, d, 0) for t in v])
    return v


def _init_columns(col_ref, wx_ref, wy_ref, ldt_ref, dsk_ref, wr_ref):
    row, lane = _iota((128, 128), 0), _iota((128, 128), 1)
    split = (row & ~15) + 2 * (row & 7) + ((row >> 3) & 1)
    ldt, dsk, wr = (ref[...].astype(F32).reshape(1, D) for ref in (ldt_ref, dsk_ref, wr_ref))
    for n, vec in enumerate((jnp.exp(ldt), dsk * (1.0 / L))):
        for lo in range(0, D, 128):
            i = min(lo, D - 128)
            diag = jnp.where(split == lane, vec[:, i:i + 128], 0.0)[lo - i:].astype(BF16)
            col_ref[n, lo:i + 128, :] = jnp.dot(diag, jnp.ones((128, 128), BF16),
                                                preferred_element_type=F32)
    sub = _iota((16, D), 0)
    ones_w = jnp.where(sub == 0, 1.0, jnp.where(sub == 1, wr, 0.0))
    wx_ref[...] = ones_w.astype(BF16)
    for lo in range(0, D, MB):
        wy_ref[lo // MB, :, 0:MB] = ones_w[:, lo:lo + MB].astype(BF16)
        wy_ref[lo // MB, :, MB:] = jnp.zeros((16, 128 - MB), BF16)


class _Schedule:
    def __init__(self, zero):
        self.zero = zero
        self.sub, self.lane = _iota((8, 128), 0) + zero, _iota((8, 128), 1) + zero
        self.true = self.sub >= 0
        self.done, self.pending, self.wait = [], {}, -1

    def tie(self, x, token):
        return jnp.where(self.true, x, token if token.dtype == x.dtype
                         else pltpu.bitcast(token, x.dtype))

    def start(self, x):
        return self.tie(x, self.done[self.wait]) if 0 <= self.wait < len(self.done) else x

    def lhs(self, words, first):
        tiles = [words[i:i + 8] for i in range(0, words.shape[0], 8)]
        for i in range(len(tiles) if first else 0):
            for token in self.pending.pop(len(self.done) + i, ()):
                tiles[i] = self.tie(tiles[i], token)
        return _mxu(jnp.concatenate(tiles, axis=0))

    def results(self, v):
        self.done += [v[i + 8:i + 16] for i in range(0, v.shape[0], 16)]

    def run(self, stage, wait, before):
        self.wait = wait
        self.pending.setdefault(before, []).extend(next(stage))


def _kernel(x_hbm, are_hbm, aim_hbm, bre_hbm, bim_hbm, cre_hbm, cim_hbm,
            ldt_hbm, dsk_hbm, wr_hbm, wg_hbm, wu_hbm, wd_hbm, out_hbm,
            x_v, wg_v, wu_v, wd_v, par_v, ldt_v, dsk_v, wr_v, w_v, wk_v, wt_v, col_v, wx_v, wy_v,
            tmp_v, pk_v, h_v, st_v, acc_v, out_v, sd0, sd1, ta0, ta1, tb0, tb1, kl0, kl1,
            u0, u1, k0, k1, a0_v, a1_v, c0, c1, y0, y1, order_s,
            sem_p, sem_x, sem_w, sem_o, f0_v, f1_v, *new_v):
    cp_vec = [pltpu.make_async_copy(s, d, sem_p.at[n]) for n, (s, d) in enumerate(
        ((ldt_hbm, ldt_v), (dsk_hbm, dsk_v), (wr_hbm, wr_v)))]
    cp_par = [[pltpu.make_async_copy(s.at[lo:hi], par_v.at[n, lo:hi], sem_p.at[3 + 6 * m + n])
               for n, s in enumerate((are_hbm, aim_hbm, bre_hbm, bim_hbm, cre_hbm, cim_hbm))]
              for m, (lo, hi) in enumerate(((0, 3 * MB), (3 * MB, D)))]
    cp_x = [pltpu.make_async_copy(x_hbm.at[:, 128 * j:128 * j + 128], x_v.at[j], sem_x.at[j])
            for j in range(NT)]
    cp_w = [pltpu.make_async_copy(s, d, sem_w.at[n]) for n, (s, d) in enumerate(
        ((wg_hbm, wg_v), (wu_hbm, wu_v), (wd_hbm, wd_v)))]
    for cp in cp_vec + cp_par[0]:
        cp.start()
    for cp in cp_x[:NT // 2]:
        cp.start(priority=1)

    def columns():
        for cp in cp_vec:
            cp.wait()
        for cp in cp_x[NT // 2:]:
            cp.start(priority=1)
        _init_columns(col_v, wx_v, wy_v, ldt_v, dsk_v, wr_v)

    _init_dft(w_v, wk_v, wt_v, tmp_v, columns)
    for cp in cp_par[0]:
        cp.wait()

    sd, ta, tb, kl = (sd0, sd1), (ta0, ta1), (tb0, tb1), (kl0, kl1)
    uk, ab, cc, yy = ((u0, u1), (k0, k1)), ((a0_v, a1_v), (f0_v, f1_v)), (c0, c1), (y0, y1)
    ww, wt_w = (w_v.bitcast(I32), wk_v.bitcast(I32)), wt_v

    def chan(b, r):
        return _ds(b * MB + 16 * r, 16)

    def seed_stage(b, r, sch):
        rows = _ds(b * MB // 2 + 8 * r, 8)
        par = [_split(par_v.bitcast(I32)[n, rows, :]) for n in range(6)]
        for h in range(2):
            a_re, a_im, b_re, b_im, c_re, c_im = [v[h] for v in par]
            dt = sch.start(col_v[0, _ds(b * MB + 16 * r + 8 * h, 8), :])
            mag, ang = jnp.exp(dt * a_re), dt * a_im
            sc = dt * (1.0 / L)
            seeds = _k_seeds((mag * jnp.cos(ang), mag * jnp.sin(ang)),
                             _cmul((c_re, c_im), (sc * b_re, sc * b_im)), sch.sub)
            for g in range(2):
                for n, v in enumerate(seeds[g]):
                    for p in range(2):
                        sd[b % 2][r, 2 * h + g, 2 * n + p] = v[p]
            yield [sd[b % 2][(r + sch.zero), 2 * h, 0]]

    def table_stage(b, r, sch):
        tail = []
        for g in range(4):
            m1, m32, m512, a0, b0 = [
                (sd[b % 2][r, g, 2 * n], sd[b % 2][r, g, 2 * n + 1]) for n in range(5)]
            m32 = (sch.start(m32[0]), m32[1])
            fa = [a0]
            for _ in range(7):
                fa.append(_cmul(fa[-1], m1))
            for src in (0, 4, 8, 10):
                fa.append(_cmul(fa[src], m512))
            tail.append(fa[11][0] * m512[0] - fa[11][1] * m512[1])
            _store_table(ta[b % 2].at[r, g], fa)
            fb = [b0]
            for _ in range(15):
                p = fb[-1]
                fb.append((p[0] * m32[0] + p[1] * m32[1], p[1] * m32[0] - p[0] * m32[1]))
            _store_table(tb[b % 2].at[r, g], fb)
            yield [ta[b % 2].bitcast(I32)[(r + sch.zero), g, 0, 0:8, :],
                   tb[b % 2].bitcast(I32)[(r + sch.zero), g, 0, 0:8, :]]
        last = [jnp.where((sch.sub & 1) == 0, tail[h], pltpu.roll(tail[h + 1], 1, 0))
                for h in (0, 2)]
        last = [pltpu.bitcast(_rbf(jnp.broadcast_to(jnp.sum(v, axis=1, keepdims=True),
                                                    (8, 128))), I32) for v in last]
        kl[b % 2][r] = jax.lax.shift_right_logical(last[0], 16) | last[1]

    def kernel_stage(b, r, sch):
        ta_w, tb_w = ta[b % 2].bitcast(I32), tb[b % 2].bitcast(I32)
        groups = [None] * 4
        for g0 in (0, 2):
            res = [jax.lax.dot_general(sch.lhs(ta_w[r, g, p, 0:48], g == g0 and p == 0),
                                       _mxu(tb_w[r, g, p, 0:64]), NT_DIMS, preferred_element_type=F32)
                   for g in (g0, g0 + 1) for p in range(2)]
            groups[g0], groups[g0 + 1] = res[0] + res[1], res[2] + res[3]
            sch.results(groups[g0 + 1])
            yield []
        dskip = [col_v[1, _ds(b * MB + 16 * r + 8 * h, 8), :] for h in range(2)]
        dst = _ds(8 * r, 8)
        res = _k_residues(groups, kl[b % 2][r], dskip, pk_v.at[sch.slot, 0], sch.sub, sch.lane)
        for s, t in enumerate(res):
            uk[1][b % 2][s, dst, :] = t
        yield [uk[1][b % 2][0, _ds(8 * (r + sch.zero), 8), :]]

    def norm_stage(b, r, sch):
        tiles = []
        for j in range(NT):
            m, inv = st_v[0, j] if j else sch.start(st_v[0, j]), st_v[1, j]
            xs = x_v[j, chan(b, r), :].astype(F32)
            tiles.append(_pack(pk_v.at[sch.slot, 1], j, (xs[0:8] - m) * inv, (xs[8:16] - m) * inv))
        dst = _ds(8 * r, 8)
        res = _to_residues(tiles, sch.lane)
        for s, t in enumerate(res):
            uk[0][b % 2][s, dst, :] = t
        yield [uk[0][b % 2][0, _ds(8 * (r + sch.zero), 8), :]]

    def forward_stage(w, b, k, sch):
        dst = ab[w][b % len(ab[w])]
        for p in range(2):
            v = [jnp.dot(sch.lhs(uk[w][b % 2][k + 4 * n, 0:MB // 2], n == 0),
                         _mxu(ww[w][k + 4 * n, p ^ (n & 1), 0:64]),
                         preferred_element_type=F32) for n in range(4)]
            d02, d13 = v[0] - v[2], v[1] - v[3]
            x1 = d02 - d13 if p == 0 else d02 + d13
            dst[k, 0, p, 0:MB] = v[0] + v[2]
            dst[k, 2, 1 - p, 0:MB] = v[1] + v[3]
            dst[k, 1, p, 0:MB] = x1
            dst[k, 3, p, 0:MB] = d02 + d13 if p == 0 else d02 - d13
            sch.results(x1)
            yield []

    def stats_stage(b, r, sch):
        for n in range(2):
            j = 8 * b + 2 * r + n
            sums = jnp.dot(sch.lhs(pltpu.bitcast(wx_v[...], I32), True),
                           _mxu(x_v.bitcast(I32)[j]), preferred_element_type=F32)
            sch.results(sums)
            acc_v[1, j] = sums[0:8]
            acc = None
            for i in range(0, D // 2, 8):
                v = [t * t for t in _split(x_v.bitcast(I32)[j, i:i + 8, :])]
                acc = v if acc is None else [p + q for p, q in zip(acc, v)]
            s1, s2 = jnp.broadcast_to(sums[0:1], (8, 128)), acc[0] + acc[1]
            for d in (4, 2, 1):
                s2 = s2 + pltpu.roll(s2, d, 0)
            st_v[0, j], st_v[1, j] = m, inv = _ln_scalars(s1, s2)
            yield [s2]

    def middle_stage(b, r, sch):
        src = [v[b % len(v)] for v in ab]
        scale = lambda v, f: [(x[0] * f, x[1] * f) for x in v]
        for h in range(2):
            ra = _ds(16 * r + 8 * h, 8)
            ld = lambda q, w: [(src[w][k, q, 0, ra, :], src[w][k, q, 1, ra, :]) for k in range(4)]

            def put(q, x, y):
                for k in range(4):
                    for p in range(2):
                        cc[b % 2][k, q, p, ra, :] = x[k][p] + y[k][p]
                        cc[b % 2][k, q + 1, p, ra, :] = x[k][p] - y[k][p]

            gate = sch.start
            a0, a2, b0, b2 = ld(0, 0), ld(2, 0), ld(0, 1), ld(2, 1)
            a0[0] = (gate(a0[0][0]), a0[0][1])
            e0 = _prod_mod_1(list(map(_cadd, a0, a2)), list(map(_cadd, b0, b2)))
            e2 = _prod_mod_m1(list(map(_csub, a0, a2)), scale(map(_csub, b0, b2), 2.0))
            put(0, e0, e2)
            again = _ds(16 * (r + sch.zero) + 8 * h, 8)
            yield [cc[b % 2][0, 0, 0, again, :]]
            four = sch.start(jnp.full((8, 128), 4.0, F32))
            e1 = _prod_mod_i(ld(1, 0), scale(ld(1, 1), four), 1)
            e3 = _prod_mod_i(ld(3, 0), scale(ld(3, 1), four), -1)
            put(2, e1, e3)
            yield [cc[b % 2][0, 2, 0, again, :]]

    def inverse_stage(b, k, sch):
        src = cc[b % 2]

        def lhs(v, n, first):
            return sch.lhs(jnp.concatenate(
                [_pack(pk_v.at[sch.slot, 2], 4 * n + i // 16, v[i:i + 8], v[i + 8:i + 16])
                 for i in range(0, MB, 16)], axis=0), first)

        for o in range(2):
            p0, p1 = [(src[k, q, 0, 0:MB], src[k, q, 1, 0:MB]) for q in (o, o + 2)]
            if o == 0:
                e = {0: _cadd(p0, p1), 2: _csub(p0, p1)}
            else:
                e = {1: (p0[0] + p1[1], p0[1] - p1[0]), 3: (p0[0] - p1[1], p0[1] + p1[0])}
            ys = []
            for n in e:
                y = [jnp.dot(lhs(e[n][p], 2 * n + p, n == o and p == 0),
                             _mxu(wt_w[k + 4 * n, p, 0:64]),
                             preferred_element_type=F32)
                     for p in range(2)]
                ys.append(y[0] + y[1])
                yy[b % 2][k + 4 * n, 0:MB] = ys[-1].astype(BF16)
            sch.results(ys[-1])
            yield []

    def residual_stage(b, r, sch):
        rows = chan(b, r)
        src = yy[b % 2].bitcast(I32)
        ys = _to_time([src[s, _ds(8 * r, 8), :] for s in range(16)], sch.lane)
        for j in range(NT):
            h = x_v[j, rows, :].astype(F32) + _mxu(
                ys[j] if j % 8 else sch.start(ys[j])).astype(F32)
            h_v[j, rows, :] = h.astype(BF16)
            hh = h * h
            acc_v[0, j] += hh[0:8] + hh[8:16]
            if j % 8 == 7:
                yield [acc_v[0, (r + sch.zero)]]

    def sum_stage(b, r, sch):
        for n in range(4):
            sums = jnp.dot(sch.lhs(wy_v.bitcast(I32)[b], n == 0)[:, :MB],
                           _mxu(yy[b % 2].bitcast(I32)[4 * r + n, 0:MB // 2]),
                           preferred_element_type=F32)
            acc_v[2, 4 * r + n] += sums[0:8]
        sch.results(sums)
        yield []

    nb = D // MB
    stages = dict(
        s=(seed_stage, 0), t=(table_stage, 1), k=(kernel_stage, 2),
        F=(functools.partial(forward_stage, 1), 3), n=(norm_stage, 2),
        f=(functools.partial(forward_stage, 0), 3), m=(middle_stage, 4),
        i=(inverse_stage, 5), a=(sum_stage, 6), r=(residual_stage, 6))

    def run(step, zero, live=None):
        live = live or {n: (f, step - lag) for n, (f, lag) in stages.items()
                        if 0 <= step - lag < nb and (n, step) != ("n", 2)}
        unroll, plan = PLANS.get("".join(live)) or PLANS.get("".join(live).replace("a", ""), PLANS["default"])

        def body(it, carry):
            sch = _Schedule(zero >> (step % 32) if unroll == 4 else zero & it)
            gens = [{n: f(b, it * unroll + u, sch) for n, (f, b) in live.items()}
                    for u in range(unroll)]
            for item in plan.split():
                u, n, *ties = item.split(":")
                if n in live:
                    sch.slot = int(u)
                    sch.run(gens[int(u)][n], *map(int, ties or (-1, -1)))
            for sch.slot, g in enumerate(gens):
                for v in g.values():
                    for _ in v:
                        pass
            return carry + it

        if unroll == 4:
            return body(0, 0)
        return jax.lax.fori_loop(0, 4 // unroll, body, 0)

    acc_v[...] = jnp.zeros(acc_v.shape, F32)
    zero = run(0, 0) - 6
    for step in range(1, nb + 6):
        if step == 1:
            for cp in cp_par[1]:
                cp.start()
        if step == 2:
            for cp in cp_w:
                cp.start(priority=1)
        if step == 3:
            for cp in cp_par[1]:
                cp.wait()
            for half in range(2):
                for cp in cp_x[NT // 2 * half:NT // 2 * (half + 1)]:
                    cp.wait()
                run(100, zero, dict(l=(stats_stage, half)))
            run(101, zero, dict(n=(norm_stage, 0)))
        run(step, zero)

    sums = [acc_v[1, j] + v
            for j, v in enumerate(_to_time([acc_v[2, s] for s in range(16)], _iota((8, 128), 1)))]
    m2, inv2 = _ln_scalars(
        jnp.concatenate([v[0:1] for v in sums], axis=0),
        jnp.concatenate([jnp.sum(acc_v[0, j], axis=0, keepdims=True) for j in range(NT)], axis=0))
    wsum = jnp.sum(wr_v[...].astype(F32).reshape(1, D), axis=1, keepdims=True)
    score = _rbf((jnp.concatenate([v[1:2] for v in sums], axis=0) - m2 * wsum) * inv2 + 0.0)
    bits = pltpu.bitcast(score, I32) >> 16
    order = jnp.where(bits < 0, -1 - bits, bits + 32768)
    pos = 128 * _iota((NT, 128), 0) + _iota((NT, 128), 1)
    key = pltpu.bitcast((order << 11) + (L - 1 - pos) + (1 << 29), F32)

    lane8, sub8 = _iota((CAP, 128), 1), _iota((CAP, 128), 0)
    best = _top8(jnp.tile(key, (8, 1)).T)
    cand = best[0]
    for c in range(1, CAP):
        cand = jnp.where((lane8 >> 4) == c, best[c], cand)
    best = [pltpu.bitcast(v, I32)[0, 0] for v in _top8(cand.T)]
    aux = [jnp.zeros((CAP, 128), F32)] * 3
    for c in range(CAP):
        hit = pltpu.bitcast(key, I32) == best[c]
        aux = [jnp.where(sub8 == c, jnp.sum(jnp.where(hit, v, 0.0), axis=0, keepdims=True), a)
               for a, v in zip(aux, (m2, inv2, score))]
    m_sel, inv_sel, score_sel = [jnp.sum(a, axis=1, keepdims=True) for a in aux]
    picks = [L - 1 - (v & (L - 1)) for v in best]
    tile, col = [t >> 7 for t in picks], [t & 127 for t in picks]
    rnd = [sum([(col[e] == col[c]).astype(I32) for e in range(c)], 0) for c in range(CAP)]
    rounds = functools.reduce(jnp.maximum, rnd) + 1
    lane_in = lambda n, c: lane8 == jnp.where(rnd[c] == n, col[c], -1)

    def out_copy(q, lo, hi, n):
        j = order[q]
        return pltpu.make_async_copy(
            out_v.at[j, lo:hi], out_hbm.at[lo:hi, _ds(j * 128, 128)], sem_o.at[n])

    h_w, out_w = h_v.bitcast(I32), out_v.bitcast(I32)

    def gather(n, acc):
        masks = [lane_in(n, c) for c in range(CAP)]
        tiles = []
        for i in range(0, D // 2, 8):
            v = jnp.zeros((8, 128), I32)
            for c in range(CAP):
                v = jnp.where(masks[c], h_w[tile[c], i:i + 8, :], v)
            tiles.append(v)
        lhs = jnp.zeros((CAP, 128), F32)
        for c in range(CAP):
            lhs = jnp.where(masks[c] & (sub8 == c), 1.0, lhs)
        return acc + jax.lax.dot_general(lhs.astype(BF16), _mxu(jnp.concatenate(tiles, axis=0)),
                                         NT_DIMS, preferred_element_type=F32)

    h_sel = jax.lax.fori_loop(0, rounds, gather, jnp.zeros((CAP, D), F32))
    x_sel = _rbf((h_sel - m_sel) * inv_sel)
    gate = _rbf(jax.nn.sigmoid(score_sel))

    true = lane8 + picks[0] >= 0
    tie = lambda x, token: jnp.where(true, x, token)

    def unrouted(j0):
        token = lane8
        for j in range(j0, j0 + NT // 2):
            inv = jnp.broadcast_to(inv2[j:j + 1], (16, 128))
            mul, sub = 1.0 + inv, m2[j:j + 1] * inv
            for i in range(0, D, 16):
                out_v[j, i:i + 16, :] = (h_v[j, i:i + 16, :].astype(F32) * mul - sub).astype(BF16)
                token = token ^ out_w[j, i // 2:i // 2 + 8, :]
                yield pltpu.bitcast(token, F32)

    def project(w_ref, j0):
        parts, side = [], unrouted(j0)
        for n in range(0, FF, 128):
            token = [next(side) for _ in range(8)][-1]
            xs = jnp.concatenate([tie(x_sel[:, :128], token), x_sel[:, 128:]], axis=1)
            parts.append(jnp.dot(xs.astype(BF16), w_ref[:, n:n + 128],
                                 preferred_element_type=F32))
        return _rbf(jnp.concatenate(parts, axis=1))

    cp_w[0].wait()
    cp_w[1].wait()
    g = project(wg_v, 0)
    act = _rbf(g * jax.nn.sigmoid(g)) * project(wu_v, NT // 2)
    routed = functools.reduce(jnp.bitwise_or, [1 << j for j in tile])
    spare = CAP - sum((routed >> j) & 1 for j in range(NT))
    n_late = 0
    for j in range(NT):
        hit = (routed >> j) & 1
        fill = (1 - hit) & (spare > 0).astype(I32)
        spare = spare - fill
        order_s[jnp.clip(jnp.where(hit + fill == 1, CAP + n_late, j - n_late), 0, NT - 1)] = j
        n_late = n_late + hit + fill

    order = [order_s[q] for q in range(NT)]
    for q in range(CAP):
        out_copy(q, 0, D, q).start()
    cp_w[2].wait()

    def placed(r, words):
        idx = jnp.zeros((CAP, 128), I32)
        for c in range(1, CAP):
            idx = jnp.where(lane_in(r, c), c, idx)
        return [_gather(w, idx) for w in words]

    def late_copies(n, lo, hi):
        return [out_copy(CAP + q, lo, hi, CAP * (n + 1) + q) for q in range(CAP)]

    def words_of(n):
        return [new_v[n].bitcast(I32)[i:i + 8, :] for i in range(0, new_v[n].shape[0] // 2, 8)]

    tokens = []
    for n, (lo, hi) in enumerate(ROW_CHUNKS):
        a = [act[:, i:i + 128] for i in range(0, FF, 128)]
        if n >= 2:
            cut = 12 * 128 // (hi - lo)
            a[cut] = tie(a[cut], tokens[n - 2])
        a = jnp.concatenate(a, axis=1)
        y = _rbf(jax.lax.dot_general(a.astype(BF16), wd_v[lo:hi, :], NT_DIMS,
                                     preferred_element_type=F32))
        new = h_sel[:, lo:hi] + _rbf(x_sel[:, lo:hi] + _rbf(y * gate))
        new_v[n][...] = jnp.concatenate(
            [new.T, jnp.zeros((hi - lo, 128 - CAP), F32)], axis=1).astype(BF16)
        rows = range(lo // 2, hi // 2, 8)
        words = words_of(n)
        both = list(zip(rows, placed(0, words), placed(1, words)))
        for c in range(CAP):
            for i, v0, v1 in both:
                pltpu.store(out_w.at[tile[c], pl.ds(i, 8), :],
                            jnp.where(rnd[c] == 0, v0, v1), mask=lane8 == col[c])
        for cp in late_copies(n, lo, hi):
            cp.start()
        out_w[tile[0], D // 2:, :] = lane8
        tokens.append(pltpu.bitcast(out_w[tile[0] | zero, D // 2:, :], F32))
    for q in range(CAP):
        out_copy(q, 0, D, q).wait()
    for n, (lo, hi) in enumerate(ROW_CHUNKS):
        for cp in late_copies(n, lo, hi):
            cp.wait()

    @pl.when(rounds > 2)
    def _():
        def fix(r, carry):
            rows = range(0, D // 2, 8)
            vals = placed(r, sum(map(words_of, range(len(new_v))), []))
            for c in range(CAP):
                for i, v in zip(rows, vals):
                    pltpu.store(out_w.at[tile[c], pl.ds(i, 8), :], v, mask=lane_in(r, c))
            return carry

        jax.lax.fori_loop(2, rounds, fix, 0)
        for cp in late_copies(0, 0, D):
            cp.start()
        for cp in late_copies(0, 0, D):
            cp.wait()


@jax.jit
def pallas_sequential_preLN__ssm_conv_s4__moe_arch_mod__prompt_kernel(
    A_u: jax.Array,
    A_A_re: jax.Array,
    A_A_im: jax.Array,
    A_B_re: jax.Array,
    A_B_im: jax.Array,
    A_C_re: jax.Array,
    A_C_im: jax.Array,
    A_log_dt: jax.Array,
    A_Dskip: jax.Array,
    B_x: jax.Array,
    B_w_r: jax.Array,
    B_w_gate: jax.Array,
    B_w_up: jax.Array,
    B_w_down: jax.Array,
):
    del B_x
    hbm = pl.BlockSpec(memory_space=pl.ANY)
    out = pl.pallas_call(
        _kernel,
        out_shape=jax.ShapeDtypeStruct((D, L), BF16),
        in_specs=[hbm] * 13,
        out_specs=hbm,
        scratch_shapes=[
            pltpu.VMEM((NT, D, 128), BF16),
            pltpu.VMEM((D, FF), BF16),
            pltpu.VMEM((D, FF), BF16),
            pltpu.VMEM((D, FF), BF16),
            pltpu.VMEM((6, D, N), BF16),
            *[pltpu.VMEM((D,), BF16)] * 3,
            *[pltpu.VMEM((16, 2, 144, 128), BF16)] * 2,
            pltpu.VMEM((16, 2, 72, 128), I32),
            pltpu.VMEM((2, D, 128), F32),
            pltpu.VMEM((16, D), BF16),
            pltpu.VMEM((D // MB, 16, 128), BF16),
            pltpu.VMEM((2, 256, 128), F32),
            pltpu.VMEM((4, 3, 32, 16, 128), BF16),
            pltpu.VMEM((NT, D, 128), BF16),
            pltpu.VMEM((2, NT, 8, 128), F32),
            pltpu.VMEM((3, NT, 8, 128), F32),
            pltpu.VMEM((NT, D + 16, 128), BF16),
            *[pltpu.VMEM((4, 4, 10, 8, 128), F32)] * 2,
            *[pltpu.VMEM((4, 4, 2, 112, 128), BF16)] * 2,
            *[pltpu.VMEM((4, 4, 2, 144, 128), BF16)] * 2,
            *[pltpu.VMEM((4, 8, 128), I32)] * 2,
            *[pltpu.VMEM((16, MB // 2 + 8, 128), I32)] * 4,
            *[pltpu.VMEM((4, 4, 2, MB + 8, 128), F32)] * 2,
            *[pltpu.VMEM((4, 4, 2, MB + 8, 128), F32)] * 2,
            *[pltpu.VMEM((16, MB + 16, 128), BF16)] * 2,
            pltpu.SMEM((NT,), I32),
            pltpu.SemaphoreType.DMA((15,)),
            pltpu.SemaphoreType.DMA((NT,)),
            pltpu.SemaphoreType.DMA((3,)),
            pltpu.SemaphoreType.DMA((CAP * (1 + len(ROW_CHUNKS)),)),
            *[pltpu.VMEM((4, 4, 2, MB + 8, 128), F32)] * 2,
            *[pltpu.VMEM((hi - lo, 128), BF16) for lo, hi in ROW_CHUNKS],
        ],
        compiler_params=pltpu.CompilerParams(vmem_limit_bytes=100 * 1024 * 1024,
                                             disable_bounds_checks=True,
                                             disable_semaphore_checks=True),
    )(A_u.reshape(L, D).T, A_A_re, A_A_im, A_B_re, A_B_im, A_C_re, A_C_im,
      A_log_dt, A_Dskip, B_w_r, B_w_gate, B_w_up, B_w_down.T)
    return out.T.reshape(1, L, D)
```

```python
import functools

import numpy as np
import jax
import jax.numpy as jnp
import jax.experimental.pallas as pl
import jax.experimental.pallas.tpu as pltpu

F32 = jnp.float32
BF16 = jnp.bfloat16
I32 = jnp.int32

L = 2048
D = 576
N = 128
FF = 4608
CAP = 8
NT = L // 128
EPS = 1e-5
MB = 64
PLANS = dict(
    st=(2, ""),
    stk=(2, "0:t:-1:3 1:t:-1:4 0:t:-1:5 0:t:-1:7 1:t:-1:10 0:t:-1:12 1:t:1:15 1:t:11:-1 0:k "
            "0:k 1:k 0:s:-1:20 0:s:11:23 0:k:-1:22 1:k 1:s:23:-1 1:s 1:k "),
    stkFnf=(2, "1:t:-1:7 0:s:-1:16 0:n:-1:16 0:s:-1:31 1:s:-1:36 1:s:-1:53 0:f 0:t:0:17 0:F "
               "0:t:4:25 0:k 0:k 0:k:-1:35 0:F 0:t:20:38 0:f 1:t:27:45 1:f 1:F 1:n:35:47 1:k "
               "1:t:39:55 1:t:41:-1 1:k 1:k 0:t:46:55 1:F 1:f "),
    stkFnfm=(1, "0:m:-1:2 0:m:-1:3 0:t:-1:6 0:t:-1:16 0:t:-1:9 0:f 0:m:1:12 0:m:-1:14 0:f "
                "0:m:6:18 0:m:7:20 0:k 0:t:9:22 0:n:9:26 0:k 0:s:16:-1 0:m:15:25 0:m:11:24 0:k "
                "0:F 0:s:20:-1 0:F "),
    stkFnfmi=(1, "0:t:-1:3 0:t:-1:3 0:n:-1:8 0:m:-1:10 0:m:-1:6 0:m:-1:16 0:s 0:f 0:m:0:17 0:k "
                 "0:s:4:33 0:k 0:m:13:24 0:m:-1:25 0:k:-1:33 0:f 0:t:16:33 0:t:17:33 0:F 0:F "
                 "0:i 0:i 0:m:32:-1 0:m:34:-1 0:a "),
    stkFnfmiar=(1, "0:t:-1:3 0:t:-1:3 0:n:-1:9 0:m:-1:5 0:m:-1:6 0:m:-1:18 0:s 0:f 0:m:0:17 "
                   "0:k 0:s:4:36 0:f 0:r:10:21 0:k 0:m:14:26 0:m:-1:25 0:k:-1:33 0:t:16:33 "
                   "0:t:17:33 0:F 0:r:22:-1 0:F 0:i 0:i 0:m:32:-1 0:m 0:a "),
    tkFnfmiar=(1, "0:t:-1:6 0:t:-1:4 0:n:-1:8 0:m:-1:8 0:m:-1:6 0:f 0:k 0:m:4:18 0:m:0:17 0:k "
                  "0:r:11:21 0:m:14:24 0:m:-1:25 0:k:-1:33 0:f 0:t:16:33 0:t:17:33 0:F 0:F "
                  "0:r:26:-1 0:i 0:i 0:m:32:-1 0:m:34:-1 0:a "),
    kFnfmiar=(2, "1:m:-1:4 1:m:-1:5 0:F 0:n:0:11 0:k 0:m:4:14 0:m:-1:15 0:m:7:21 0:m:6:19 0:F "
                 "0:m:12:23 0:m:-1:22 0:k 0:m:16:28 0:m:-1:31 0:k:-1:39 0:i 0:f 0:f 0:i "
                 "0:r:32:41 1:n:34:50 0:a 1:F 1:k 1:m:41:55 1:m:38:58 1:r:44:56 1:F 1:k "
                 "1:m:51:59 1:m:53:63 0:r:54:64 1:k:-1:72 1:i 1:f 1:r:63:72 1:f 1:m:67:-1 1:i "
                 "1:a 1:m:73:-1 "),
    Ffmiar=(2, "1:m:-1:7 0:m:-1:6 0:m:-1:9 0:F 0:m:0:14 1:m:3:15 0:F 0:m:6:18 0:f 0:r:10:21 "
               "0:m:10:21 0:f 0:i 1:m:16:28 0:m:18:29 0:i 1:r:21:35 0:a 1:F 0:m:26:37 "
               "1:m:27:40 1:F 0:m:29:42 1:f 1:m:34:47 0:r:36:48 1:f 1:m:38:-1 1:i 1:m:42:-1 "
               "1:i 1:m:45:-1 1:r:45:-1 1:a "),
    miar=(2, "1:m:-1:1 1:m:-1:2 0:m:-1:2 0:m:-1:6 0:i 0:m:0:8 0:m:-1:8 0:m:1:10 0:m:-1:11 "
             "0:r:3:14 0:a 0:i 1:r:5:15 0:r:5:14 1:m:8:16 1:m:-1:17 1:i 1:r:10:-1 1:m:12:-1 "
             "1:m 1:m 1:a 1:i 0:m:15:-1 0:m 1:m:17:-1 "),
    iar=(4, "2:r:-1:14 0:i 0:i 0:r:6:20 0:a 1:i 0:r:10:23 1:i 1:r:13:27 2:r:15:29 1:a 2:i 2:i "
            "3:r:22:-1 1:r:24:35 2:a 3:i 3:i 3:r:34:-1 3:a "),
    ar=(4, "0:a 1:a 2:a 3:a "),
    s=(2, ""),
    n=(4, ""),
    default=(1, ""),
)
ROW_CHUNKS = ((0, 128), (128, 256), (256, 384), (384, 512), (512, D))
NT_DIMS = (((1,), (1,)), ((), ()))


def _round_res(step):
    return [int(np.round(r / step)) * step for r in range(16)]


RES1, RES2, RES3 = _round_res(2), _round_res(4), _round_res(8)


def _ds(start, size):
    return pl.ds(start if isinstance(start, int) else pl.multiple_of(start, size), size)


def _iota(shape, dim):
    return jax.lax.broadcasted_iota(I32, shape, dim)


def _rbf(x):
    return x.astype(BF16).astype(F32)


def _cmul(a, b):
    return (a[0] * b[0] - a[1] * b[1], a[0] * b[1] + a[1] * b[0])


def _csq(a):
    t = a[0] * a[1]
    return ((a[0] + a[1]) * (a[0] - a[1]), t + t)


def _cadd(a, b):
    return (a[0] + b[0], a[1] + b[1])


def _csub(a, b):
    return (a[0] - b[0], a[1] - b[1])


def _bfly4(a0, a1, a2, a3, inverse=False):
    s02, d02 = _cadd(a0, a2), _csub(a0, a2)
    s13, d13 = _cadd(a1, a3), _csub(a1, a3)
    p = (d02[0] - d13[1], d02[1] + d13[0])
    m = (d02[0] + d13[1], d02[1] - d13[0])
    if inverse:
        p, m = m, p
    return _cadd(s02, s13), p, _csub(s02, s13), m


def _prod_mod_1(a, b):
    fa, fb = _bfly4(*a), _bfly4(*b)
    return _bfly4(*[_cmul(x, y) for x, y in zip(fa, fb)], inverse=True)


def _prod2(a0, a1, b0, b1, sgn):
    p00, p11 = _cmul(a0, b0), _cmul(a1, b1)
    c1 = _cadd(_cmul(a0, b1), _cmul(a1, b0))
    if sgn > 0:
        return (p00[0] - p11[1], p00[1] + p11[0]), c1
    return (p00[0] + p11[1], p00[1] - p11[0]), c1


def _prod_mod_m1(a, b):
    def split(x):
        p = [(x[k][0] - x[k + 2][1], x[k][1] + x[k + 2][0]) for k in range(2)]
        m = [(x[k][0] + x[k + 2][1], x[k][1] - x[k + 2][0]) for k in range(2)]
        return p, m
    ap, am = split(a)
    bp, bm = split(b)
    cp = _prod2(*ap, *bp, 1)
    cm = _prod2(*am, *bm, -1)
    lo = [_cadd(cp[k], cm[k]) for k in range(2)]
    hi = [(cp[k][1] - cm[k][1], cm[k][0] - cp[k][0]) for k in range(2)]
    return lo + hi


def _prod_mod_i(a, b, sgn):
    sm = [x[0] + x[1] for x in b]
    df = [x[1] - x[0] for x in b]
    asum = [x[0] + x[1] for x in a]
    out = []
    for k in range(4):
        acc = [None, None, None]
        for j in range(4):
            m = (k - j) % 4
            if j <= k:
                t = ((b[m][0], 1), (df[m], 1), (sm[m], 1))
            elif sgn > 0:
                t = ((b[m][1], -1), (sm[m], 1), (df[m], -1))
            else:
                t = ((b[m][1], 1), (sm[m], -1), (df[m], 1))
            for q, (v, (w, s)) in enumerate(zip((asum[j], a[j][0], a[j][1]), t)):
                p = v * w
                if acc[q] is None:
                    acc[q] = p
                else:
                    acc[q] = acc[q] + p if s > 0 else acc[q] - p
        out.append((acc[0] - acc[2], acc[0] + acc[1]))
    return out


def _barrel(v, sch):
    for bit in range(4):
        m = sch.mask("bit%d" % bit)
        v = [jnp.where(m, v[(i + (1 << bit)) % 16], v[i]) for i in range(16)]
    return [v[-s % 16] for s in range(16)]


def _to_residues(tiles, sch):
    return _barrel([t if j == 0 else pltpu.roll(t, j, 1) for j, t in enumerate(tiles)], sch)


def _to_time(res, sch):
    return [t if j == 0 else pltpu.roll(t, 128 - j, 1)
            for j, t in enumerate(_barrel(res, sch))]


def _gather(x, idx, axis=1):
    return jnp.take_along_axis(x, idx, axis=axis, mode="promise_in_bounds")


def _init_dft(wu_ref, wk_ref, wt_ref, tmp_ref, halfway):
    sub, k4 = _iota((8, 128), 0), 4 * _iota((8, 128), 1) + 1

    def cis(t):
        ph = ((k4 * t) & (4 * L - 1)).astype(F32) * (2 * np.pi / (4 * L))
        return jnp.cos(ph), jnp.sin(ph)

    w1, w16 = cis(1), cis(16)
    w32 = _csq(w16)
    fk = [cis(16 * (32 * (sub & 3) + (sub >> 2)))]
    fu = [cis(128 * sub), cis(128 * (sub + 8))]
    for v in range(1, 16):
        fk.append(_cmul(fk[-1], w32))
        if v >= 2:
            fu.append(_cmul(fu[-2], w16))
    for p in range(2):
        for v in range(32):
            tmp_ref[p, 8 * v:8 * v + 8, :] = fu[v % 16][p]
    tw = None
    for s in range(16):
        for v in range(0, 16, 2):
            rows = [slice(128 - s + 8 * i, 136 - s + 8 * i) for i in (v, v + 1)]
            for ref, f in ((wk_ref, fk[v:v + 2]),
                           (wu_ref, [(tmp_ref[0, r, :], tmp_ref[1, r, :]) for r in rows])):
                if s:
                    f = [_cmul(x, tw) for x in f]
                for p in range(2):
                    ref[p, 4 * (s % 4) + s // 4, 8 * v:8 * v + 16, :] = jnp.concatenate(
                        [f[0][p], f[1][p]], axis=0).astype(BF16)
        for p in range(2):
            wt_ref[4 * (s % 4) + (0, 2, 1, 3)[s // 4], p, 0:64] = pltpu.bitcast(
                _mxu(wu_ref.bitcast(I32)[p, 4 * (s % 4) + s // 4, 0:64]).T, I32)
        tw = _cmul(tw, w1) if s else w1
        if s == 7:
            halfway()


def _pack(ref, n, a, b):
    ref[n] = jnp.concatenate([a, b], axis=0).astype(BF16)
    return ref.bitcast(I32)[n]


def _split(w):
    return [pltpu.bitcast(w << 16, F32), pltpu.bitcast(w & -65536, F32)]


FINE = (0, 1, 2, 3, 4, 5, 6, 7, 512, 516, 1024, 1536)


def _k_seeds(z, c, sch):
    pw = {1: z}
    for e in range(1, 10):
        pw[1 << e] = _csq(pw[1 << (e - 1)])
    c8, z16 = _cmul(c, pw[8]), (pw[16][0], 0.0 - pw[16][1])
    pair = lambda a, b: tuple(jnp.where(sch.mask("odd"), q, p) for p, q in zip(a, b))
    seeds = []
    for g in range(2):
        twice = lambda v: tuple(_gather(x, sch.idx("dup%d" % g), 0) for x in v)
        seeds.append([twice(z), twice(pw[32]), twice(pw[512]),
                      pair(twice(c), twice(c8)), pair((1.0, 0.0), twice(z16))])
    return seeds


def _mxu(words):
    return pltpu.bitcast(words, BF16)


def _store_table(ref, tab):
    for i in range(0, len(tab), 2):
        for p in range(2):
            ref[p, 8 * i:8 * i + 16, :] = jnp.concatenate(
                [tab[i][p], tab[i + 1][p]], axis=0).astype(BF16)


def _k_residues(groups, k_last, dskip, tmp_ref, sch):
    idx, nxt = sch.idx("src"), sch.idx("nxt")
    low = lambda x, y: (x & 65535) | (y << 16)
    high = lambda x, y: jax.lax.shift_right_logical(x, 16) | (y & -65536)
    kv, up = {}, {}
    for i, k in enumerate(FINE):
        v = [g[8 * i:8 * i + 8] for g in groups]
        if k == 0:
            v = [x + jnp.where(sch.mask("diag"),
                               _gather(dskip[n // 2], sch.idx("dup%d" % (n % 2)), 0), 0.0)
                 for n, x in enumerate(v)]
        p = [_pack(tmp_ref, 2 * i + h, v[2 * h], v[2 * h + 1]) for h in range(2)]
        both = [_gather(x, idx) for x in p]
        kv[k], kv[k + 8] = low(*both), high(*both)
        if k % 512 == 0:
            up[k] = low(*[_gather(x, nxt) for x in p])
    k_last = _gather(k_last, sch.idx("rows"), 0)
    q0, q1, q2, up0, up01, up2, up3, fine = map(sch.mask, INDEX[-8:])
    s3 = {r: jnp.where(q2, kv[1024 + r], kv[1536 + r]) for r in (0, 8)}
    v0 = jnp.where(q0, kv[0], jnp.where(q1, kv[512], s3[0]))
    v16 = jnp.where(up01, jnp.where(up0, up[0], up[512]),
                    jnp.where(up2, up[1024], jnp.where(up3, up[1536], k_last)))
    s3[16] = v16
    s23, s123, out = {}, {}, [v0]
    for r in range(1, 16):
        k23 = (RES2[r], RES3[r])
        if k23 not in s23:
            s23[k23] = v16 if k23 == (16, 16) else jnp.where(q1, kv[512 + k23[0]], s3[k23[1]])
        k123 = (RES1[r],) + k23
        if k123 not in s123:
            s123[k123] = v16 if k123[0] == 16 else jnp.where(q0, kv[k123[0]], s23[k23])
        if RES1[r] == r:
            out.append(s123[k123])
        else:
            out.append(jnp.where(fine, kv[r], s123[k123]))
    return out


def _ln_scalars(s1, s2):
    mean = s1 * (1.0 / D)
    var = jnp.maximum(s2 * (1.0 / D) - mean * mean, 0.0)
    eps = float(np.asarray(EPS, dtype=BF16))
    sd = _rbf(jnp.sqrt(_rbf(_rbf(var) + eps)))
    return _rbf(mean), 1.0 / sd


def _top8(x):
    def swap(v, pairs):
        for i, j in pairs:
            v[i], v[j] = jnp.maximum(v[i], v[j]), jnp.minimum(v[i], v[j])
        return v

    def merge(a, b):
        v = [jnp.maximum(a[i], b[7 - i]) for i in range(8)]
        return swap(v, [(i, i + d) for d in (4, 2, 1) for i in range(8) if not i & d])

    sort8 = ((0, 2), (1, 3), (4, 6), (5, 7), (0, 4), (1, 5), (2, 6), (3, 7), (0, 1), (2, 3),
             (4, 5), (6, 7), (2, 4), (3, 5), (1, 4), (3, 6), (1, 2), (3, 4), (5, 6))
    v = merge(*[swap(x[i:i + 8], sort8) for i in (0, 8)])
    for d in (4, 2, 1):
        v = merge(v, [pltpu.roll(t, d, 0) for t in v])
    return v


def _init_columns(col_ref, wx_ref, wy_ref, ldt_ref, dsk_ref, wr_ref):
    row, lane = _iota((128, 128), 0), _iota((128, 128), 1)
    split = (row & ~15) + 2 * (row & 7) + ((row >> 3) & 1)
    ldt, dsk, wr = (ref[...].astype(F32).reshape(1, D) for ref in (ldt_ref, dsk_ref, wr_ref))
    for n, vec in enumerate((jnp.exp(ldt), dsk * (1.0 / L))):
        for lo in range(0, D, 128):
            i = min(lo, D - 128)
            diag = jnp.where(split == lane, vec[:, i:i + 128], 0.0)[lo - i:].astype(BF16)
            col_ref[n, lo:i + 128, :] = jnp.dot(diag, jnp.ones((128, 128), BF16),
                                                preferred_element_type=F32)
    sub = _iota((16, D), 0)
    ones_w = jnp.where(sub == 0, 1.0, jnp.where(sub == 1, wr, 0.0))
    wx_ref[...] = ones_w.astype(BF16)
    for lo in range(0, D, MB):
        wy_ref[lo // MB, :, 0:MB] = ones_w[:, lo:lo + MB].astype(BF16)
        wy_ref[lo // MB, :, MB:] = jnp.zeros((16, 128 - MB), BF16)


INDEX = ("true", "bit0", "bit1", "bit2", "bit3", "odd", "dup0", "dup1", "rows", "src", "nxt",
         "diag", "q0", "q1", "q2", "up0", "up01", "up2", "up3", "fine")


def _init_index(idx_ref):
    sub, lane = _iota((8, 128), 0), _iota((8, 128), 1)
    src = lambda b: 8 * ((b >> 1) & 15) + 2 * (sub & 3) + (b & 1)
    is_ = lambda m: jnp.where(m, 1, 0)
    q = lane & 3
    q16 = q + is_(lane >= 124)
    tiles = dict(true=sub + 1, odd=sub & 1, dup0=sub >> 1, dup1=4 + (sub >> 1),
                 rows=2 * (sub & 3) + (sub >> 2), src=src(lane >> 2), nxt=src((lane >> 2) + 1),
                 diag=is_((lane == sub) & ((sub & 1) == 0)), up01=is_(q16 < 2),
                 fine=is_((q == 0) & (lane < 64)),
                 **{"bit%d" % n: (lane >> n) & 1 for n in range(4)},
                 **{"q%d" % n: is_(q == n) for n in range(3)},
                 **{"up%d" % n: is_(q16 == n) for n in (0, 2, 3)})
    for n, name in enumerate(INDEX):
        idx_ref[n] = tiles[name]


class _Schedule:
    def __init__(self, zero, idx_ref):
        self.zero = zero
        self.idx = lambda name: idx_ref[INDEX.index(name) + zero]
        self.mask = lambda name: self.idx(name) != 0
        self.true = self.mask("true")
        self.done, self.pending, self.wait = [], {}, -1

    def tie(self, x, token):
        return jnp.where(self.true, x, token if token.dtype == x.dtype
                         else pltpu.bitcast(token, x.dtype))

    def start(self, x):
        return self.tie(x, self.done[self.wait]) if 0 <= self.wait < len(self.done) else x

    def lhs(self, words, first):
        tiles = [words[i:i + 8] for i in range(0, words.shape[0], 8)]
        for i in range(len(tiles) if first else 0):
            for token in self.pending.pop(len(self.done) + i, ()):
                tiles[i] = self.tie(tiles[i], token)
        return _mxu(jnp.concatenate(tiles, axis=0))

    def results(self, v):
        self.done += [v[i + 8:i + 16] for i in range(0, v.shape[0], 16)]

    def run(self, stage, wait, before):
        self.wait = wait
        self.pending.setdefault(before, []).extend(next(stage))


def _kernel(x_hbm, are_hbm, aim_hbm, bre_hbm, bim_hbm, cre_hbm, cim_hbm,
            ldt_hbm, dsk_hbm, wr_hbm, wg_hbm, wu_hbm, wd_hbm, out_hbm,
            x_v, wg_v, wu_v, wd_v, par_v, ldt_v, dsk_v, wr_v, w_v, wk_v, wt_v, col_v, wx_v, wy_v,
            tmp_v, idx_v, pk_v, h_v, st_v, acc_v, out_v, sd0, sd1, ta0, ta1, tb0, tb1, kl0, kl1,
            u0, u1, k0, k1, a0_v, a1_v, c0, c1, y0, y1, order_s,
            sem_p, sem_x, sem_w, sem_o, f0_v, f1_v, *new_v):
    cp_vec = [pltpu.make_async_copy(s, d, sem_p.at[n]) for n, (s, d) in enumerate(
        ((ldt_hbm, ldt_v), (dsk_hbm, dsk_v), (wr_hbm, wr_v)))]
    cp_par = [[pltpu.make_async_copy(s.at[lo:hi], par_v.at[n, lo:hi], sem_p.at[3 + 6 * m + n])
               for n, s in enumerate((are_hbm, aim_hbm, bre_hbm, bim_hbm, cre_hbm, cim_hbm))]
              for m, (lo, hi) in enumerate(((0, 4 * MB), (4 * MB, D)))]
    cp_x = [pltpu.make_async_copy(x_hbm.at[:, 128 * j:128 * j + 128], x_v.at[j, 0:D],
                                  sem_x.at[j])
            for j in range(NT)]
    cp_w = [pltpu.make_async_copy(s, d, sem_w.at[n]) for n, (s, d) in enumerate(
        ((wg_hbm, wg_v), (wu_hbm, wu_v), (wd_hbm, wd_v)))]
    for cp in cp_vec + cp_par[0]:
        cp.start()
    for cp in cp_x[:NT // 2]:
        cp.start(priority=1)

    def columns():
        for cp in cp_vec:
            cp.wait()
        for cp in cp_x[NT // 2:]:
            cp.start(priority=1)
        _init_columns(col_v, wx_v, wy_v, ldt_v, dsk_v, wr_v)

    _init_dft(w_v, wk_v, wt_v, tmp_v, columns)
    for cp in cp_par[0]:
        cp.wait()

    sd, ta, tb, kl = (sd0, sd1), (ta0, ta1), (tb0, tb1), (kl0, kl1)
    uk, ab, cc, yy = ((u0, u1), (k0, k1)), ((a0_v, a1_v), (f0_v, f1_v)), (c0, c1), (y0, y1)
    ww, wt_w = (w_v.bitcast(I32), wk_v.bitcast(I32)), wt_v

    def chan(b, r):
        return _ds(b * MB + 16 * r, 16)

    def seed_stage(b, r, sch):
        rows = _ds(b * MB // 2 + 8 * r, 8)
        par = [_split(par_v.bitcast(I32)[n, rows, :]) for n in range(6)]
        for h in range(2):
            a_re, a_im, b_re, b_im, c_re, c_im = [v[h] for v in par]
            dt = sch.start(col_v[0, _ds(b * MB + 16 * r + 8 * h, 8), :])
            mag, ang = jnp.exp(dt * a_re), dt * a_im
            sc = dt * (1.0 / L)
            seeds = _k_seeds((mag * jnp.cos(ang), mag * jnp.sin(ang)),
                             _cmul((c_re, c_im), (sc * b_re, sc * b_im)), sch)
            for g in range(2):
                for n, v in enumerate(seeds[g]):
                    for p in range(2):
                        sd[b % 2][r, 2 * h + g, 2 * n + p] = v[p]
            yield [sd[b % 2][(r + sch.zero), 2 * h, 0]]

    def table_stage(b, r, sch):
        tail = []
        for g in range(4):
            m1, m32, m512, a0, b0 = [
                (sd[b % 2][r, g, 2 * n], sd[b % 2][r, g, 2 * n + 1]) for n in range(5)]
            m32 = (sch.start(m32[0]), m32[1])
            fa = [a0]
            for _ in range(7):
                fa.append(_cmul(fa[-1], m1))
            for src in (0, 4, 8, 10):
                fa.append(_cmul(fa[src], m512))
            tail.append(fa[11][0] * m512[0] - fa[11][1] * m512[1])
            _store_table(ta[b % 2].at[r, g], fa)
            fb = [b0]
            for _ in range(15):
                p = fb[-1]
                fb.append((p[0] * m32[0] + p[1] * m32[1], p[1] * m32[0] - p[0] * m32[1]))
            _store_table(tb[b % 2].at[r, g], fb)
            yield [ta[b % 2].bitcast(I32)[(r + sch.zero), g, 0, 0:8, :],
                   tb[b % 2].bitcast(I32)[(r + sch.zero), g, 0, 0:8, :]]
        last = [jnp.where(sch.mask("odd"), pltpu.roll(tail[h + 1], 1, 0), tail[h])
                for h in (0, 2)]
        last = [pltpu.bitcast(_rbf(jnp.broadcast_to(jnp.sum(v, axis=1, keepdims=True),
                                                    (8, 128))), I32) for v in last]
        kl[b % 2][r] = jax.lax.shift_right_logical(last[0], 16) | last[1]

    def kernel_stage(b, r, sch):
        ta_w, tb_w = ta[b % 2].bitcast(I32), tb[b % 2].bitcast(I32)
        groups = [None] * 4
        for g0 in (0, 2):
            res = [jax.lax.dot_general(sch.lhs(ta_w[r, g, p, 0:48], g == g0 and p == 0),
                                       _mxu(tb_w[r, g, p, 0:64]), NT_DIMS, preferred_element_type=F32)
                   for g in (g0, g0 + 1) for p in range(2)]
            groups[g0], groups[g0 + 1] = res[0] + res[1], res[2] + res[3]
            sch.results(groups[g0 + 1])
            yield []
        dskip = [col_v[1, _ds(b * MB + 16 * r + 8 * h, 8), :] for h in range(2)]
        dst = _ds(8 * r, 8)
        res = _k_residues(groups, kl[b % 2][r], dskip, pk_v.at[sch.slot, 0], sch)
        for s, t in enumerate(res):
            uk[1][b % 2][4 * (s % 4) + s // 4, dst, :] = t
        yield [uk[1][b % 2][0, _ds(8 * (r + sch.zero), 8), :]]

    def norm_stage(b, r, sch):
        tiles = []
        for j in range(NT):
            m, inv = st_v[j, 0] if j else sch.start(st_v[j, 0]), st_v[j, 1]
            xs = x_v[j, chan(b, r), :].astype(F32)
            tiles.append(_pack(pk_v.at[sch.slot, 1], j, (xs[0:8] - m) * inv, (xs[8:16] - m) * inv))
        dst = _ds(8 * r, 8)
        res = _to_residues(tiles, sch)
        for s, t in enumerate(res):
            uk[0][b % 2][4 * (s % 4) + s // 4, dst, :] = t
        yield [uk[0][b % 2][0, _ds(8 * (r + sch.zero), 8), :]]

    def forward_stage(w, b, k, sch):
        dst = ab[w][b % len(ab[w])]
        for p in range(2):
            v = [jnp.dot(sch.lhs(uk[w][b % 2][4 * k + n, 0:MB // 2], n == 0),
                         _mxu(ww[w][p ^ (n & 1), 4 * k + n, 0:64]),
                         preferred_element_type=F32) for n in range(4)]
            d02, d13 = v[0] - v[2], v[1] - v[3]
            x1 = d02 - d13 if p == 0 else d02 + d13
            dst[0, k, p, 0:MB] = v[0] + v[2]
            dst[2, k, 1 - p, 0:MB] = v[1] + v[3]
            dst[1, k, p, 0:MB] = x1
            dst[3, k, p, 0:MB] = d02 + d13 if p == 0 else d02 - d13
            sch.results(x1)
            yield []

    def stats(tiles, sch):
        ones_w = wx_v.bitcast(I32)[...]
        for j in tiles:
            acc = None
            for i in range(0, D // 2, 8):
                v = [t * t for t in _split(x_v.bitcast(I32)[j, i:i + 8, :])]
                acc = v if acc is None else [p + q for p, q in zip(acc, v)]
            sums = jnp.dot(_mxu(jnp.concatenate(
                [ones_w[:, :128] if j % 2 == 0 else sch.tie(ones_w[:, :128], prev),
                 ones_w[:, 128:]], axis=1)),
                           _mxu(x_v.bitcast(I32)[j, 0:D // 2]), preferred_element_type=F32)
            acc_v[1, j] = sums[0:8]
            s2 = prev = acc[0] + acc[1]
            for d in (4, 2, 1):
                s2 = s2 + pltpu.roll(s2, d, 0)
            st_v[j, 0], st_v[j, 1] = _ln_scalars(jnp.broadcast_to(sums[0:1], (8, 128)), s2)

    def middle_stage(b, r, sch):
        src = [v[b % len(v)] for v in ab]
        scale = lambda v, f: [(x[0] * f, x[1] * f) for x in v]
        for h in range(2):
            ra = _ds(16 * r + 8 * h, 8)
            ld = lambda q, w: [(src[w][q, k, 0, ra, :], src[w][q, k, 1, ra, :]) for k in range(4)]

            def put(q, x, y):
                for k in range(4):
                    for p in range(2):
                        cc[b % 2][k, q, p, ra, :] = x[k][p] + y[k][p]
                        cc[b % 2][k, q + 2, p, ra, :] = x[k][p] - y[k][p]

            def park(x):
                for k in range(4):
                    for p in range(2):
                        cc[b % 2][k, 0, p, MB:, :] = x[k][p]
                return [cc[b % 2][sch.zero, 0, 0, MB:, :]]

            gate = sch.start
            a0, a2, b0, b2 = ld(0, 0), ld(2, 0), ld(0, 1), ld(2, 1)
            a0[0] = (gate(a0[0][0]), a0[0][1])
            e0 = _prod_mod_1(list(map(_cadd, a0, a2)), list(map(_cadd, b0, b2)))
            again = _ds(16 * (r + sch.zero) + 8 * h, 8)
            yield park(e0)
            a2[0] = (gate(a2[0][0]), a2[0][1])
            e2 = _prod_mod_m1(list(map(_csub, a0, a2)), scale(map(_csub, b0, b2), 2.0))
            put(0, e0, e2)
            yield [cc[b % 2][0, 0, 0, again, :]]
            four = sch.start(jnp.full((8, 128), 4.0, F32))
            e1 = _prod_mod_i(ld(1, 0), scale(ld(1, 1), four), 1)
            yield park(e1)
            four = sch.start(jnp.full((8, 128), 4.0, F32))
            e3 = _prod_mod_i(ld(3, 0), scale(ld(3, 1), four), -1)
            put(1, e1, e3)
            yield [cc[b % 2][0, 1, 0, again, :]]

    def inverse_stage(b, k, sch):
        src = cc[b % 2]

        def lhs(v, n, first):
            return sch.lhs(jnp.concatenate(
                [_pack(pk_v.at[sch.slot, 2], 4 * n + i // 16, v[i:i + 8], v[i + 8:i + 16])
                 for i in range(0, MB, 16)], axis=0), first)

        for o in range(2):
            p0, p1 = [(src[k, q, 0, 0:MB], src[k, q, 1, 0:MB]) for q in (2 * o, 2 * o + 1)]
            if o == 0:
                e = {0: _cadd(p0, p1), 2: _csub(p0, p1)}
            else:
                e = {1: (p0[0] + p1[1], p0[1] - p1[0]), 3: (p0[0] - p1[1], p0[1] + p1[0])}
            ys = []
            for n in e:
                y = [jnp.dot(lhs(e[n][p], 2 * n + p, n == o and p == 0),
                             _mxu(wt_w[4 * k + (0, 2, 1, 3)[n], p, 0:64]),
                             preferred_element_type=F32)
                     for p in range(2)]
                ys.append(y[0] + y[1])
                yy[b % 2][k + 4 * n, 0:MB] = ys[-1].astype(BF16)
            sch.results(ys[-1])
            yield []

    def residual_stage(b, r, sch):
        rows = chan(b, r)
        src = yy[b % 2].bitcast(I32)
        ys = _to_time([src[s, _ds(8 * r, 8), :] for s in range(16)], sch)
        for j in range(NT):
            h = x_v[j, rows, :].astype(F32) + _mxu(
                ys[j] if j % 8 else sch.start(ys[j])).astype(F32)
            h_v[j, rows, :] = h.astype(BF16)
            hh = h * h
            acc_v[0, j] += hh[0:8] + hh[8:16]
            if j % 8 == 7:
                yield [acc_v[0, (r + sch.zero)]]

    def sum_stage(b, r, sch):
        for n in range(4):
            sums = jnp.dot(sch.lhs(wy_v.bitcast(I32)[b], n == 0)[:, :MB],
                           _mxu(yy[b % 2].bitcast(I32)[4 * r + n, 0:MB // 2]),
                           preferred_element_type=F32)
            acc_v[2, 4 * r + n] += sums[0:8]
        sch.results(sums)
        yield []

    nb = D // MB
    stages = dict(
        s=(seed_stage, 0), t=(table_stage, 1), k=(kernel_stage, 2),
        F=(functools.partial(forward_stage, 1), 3), n=(norm_stage, 2),
        f=(functools.partial(forward_stage, 0), 3), m=(middle_stage, 4),
        i=(inverse_stage, 5), a=(sum_stage, 6), r=(residual_stage, 6))

    def run(step, zero, live=None):
        live = live or {n: (f, step - lag) for n, (f, lag) in stages.items()
                        if 0 <= step - lag < nb and (n, step) != ("n", 2)}
        unroll, plan = PLANS.get("".join(live)) or PLANS.get("".join(live).replace("a", ""), PLANS["default"])

        def body(it, carry):
            sch = _Schedule(zero >> (step % 32) if unroll == 4 else zero & it, idx_v)
            gens = [{n: f(b, it * unroll + u, sch) for n, (f, b) in live.items()}
                    for u in range(unroll)]
            for item in plan.split():
                u, n, *ties = item.split(":")
                if n in live:
                    sch.slot = int(u)
                    sch.run(gens[int(u)][n], *map(int, ties or (-1, -1)))
            for sch.slot, g in enumerate(gens):
                for v in g.values():
                    for _ in v:
                        pass
            return carry + it

        if unroll == 4:
            return body(0, 0)
        return jax.lax.fori_loop(0, 4 // unroll, body, 0)

    _init_index(idx_v)
    acc_v[...] = jnp.zeros(acc_v.shape, F32)
    zero = run(0, 0) - 1
    for step in range(1, nb + 6):
        if step == 4:
            for cp in cp_par[1]:
                cp.wait()
        if step == 3:
            for half in range(2):
                tiles = range(NT // 2 * half, NT // 2 * (half + 1))
                for j in tiles:
                    cp_x[j].wait()
                if half:
                    for cp in cp_par[1]:
                        cp.start()
                    for cp in cp_w:
                        cp.start(priority=1)
                stats(tiles, _Schedule(zero, idx_v))
            run(101, zero, dict(n=(norm_stage, 0)))
        run(step, zero)

    sums = [acc_v[1, j] + v
            for j, v in enumerate(_to_time([acc_v[2, s] for s in range(16)],
                                          _Schedule(0, idx_v)))]
    m2, inv2 = _ln_scalars(
        jnp.concatenate([v[0:1] for v in sums], axis=0),
        jnp.concatenate([jnp.sum(acc_v[0, j], axis=0, keepdims=True) for j in range(NT)], axis=0))
    wsum = jnp.sum(wr_v[...].astype(F32).reshape(1, D), axis=1, keepdims=True)
    score = _rbf((jnp.concatenate([v[1:2] for v in sums], axis=0) - m2 * wsum) * inv2 + 0.0)
    bits = pltpu.bitcast(score, I32) >> 16
    order = jnp.where(bits < 0, -1 - bits, bits + 32768)
    pos = 128 * _iota((NT, 128), 0) + _iota((NT, 128), 1)
    key = pltpu.bitcast((order << 11) + (L - 1 - pos) + (1 << 29), F32)

    lane8, sub8 = _iota((CAP, 128), 1), _iota((CAP, 128), 0)
    best = _top8([pltpu.roll(key[i:i + 8], n, 1) if n else key[i:i + 8]
                  for i in (0, 8) for n in range(8)])
    cand = best[0]
    for c in range(1, CAP):
        cand = jnp.where(sub8 == c, best[c], cand)
    best = [pltpu.bitcast(v, I32)[0, 0]
            for v in _top8([pltpu.roll(cand, n, 1) if n else cand for n in range(0, 128, 8)])]
    picks = [L - 1 - (v & (L - 1)) for v in best]
    tile, col = [t >> 7 for t in picks], [t & 127 for t in picks]
    rnd = [sum([(col[e] == col[c]).astype(I32) for e in range(c)], 0) for c in range(CAP)]
    rounds = functools.reduce(jnp.maximum, rnd) + 1
    lane_in = lambda n, c: lane8 == jnp.where(rnd[c] == n, col[c], -1)

    def out_copy(q, lo, hi, n):
        j = order[q]
        return pltpu.make_async_copy(
            out_v.at[j, lo:hi], out_hbm.at[lo:hi, _ds(j * 128, 128)], sem_o.at[n])

    h_w, out_w = h_v.bitcast(I32), out_v.bitcast(I32)

    def gather(n, acc):
        masks = [lane_in(n, c) for c in range(CAP)]
        tiles = []
        for i in range(0, D // 2, 8):
            v = jnp.zeros((8, 128), I32)
            for c in range(CAP):
                v = jnp.where(masks[c], h_w[tile[c], i:i + 8, :], v)
            tiles.append(v)
        lhs = jnp.zeros((CAP, 128), F32)
        for c in range(CAP):
            lhs = jnp.where(masks[c] & (sub8 == c), 1.0, lhs)
        aux = [jnp.zeros((CAP, 128), F32)] * 3
        for c in range(CAP):
            hit = pltpu.bitcast(key, I32) == best[c]
            aux = [jnp.where(sub8 == c, jnp.sum(jnp.where(hit, v, 0.0), axis=0, keepdims=True), a)
                   for a, v in zip(aux, (m2, inv2, score))]
        return (acc[0] + jax.lax.dot_general(lhs.astype(BF16), _mxu(jnp.concatenate(tiles, axis=0)),
                                             NT_DIMS, preferred_element_type=F32),
                *[jnp.sum(a, axis=1, keepdims=True) for a in aux])

    h_sel, m_sel, inv_sel, score_sel = jax.lax.fori_loop(
        0, rounds, gather, (jnp.zeros((CAP, D), F32), *[jnp.zeros((CAP, 1), F32)] * 3))
    x_sel = _rbf((h_sel - m_sel) * inv_sel)
    gate = _rbf(jax.nn.sigmoid(score_sel))

    true = lane8 + picks[0] >= 0
    tie = lambda x, token: jnp.where(true, x, token)

    def unrouted(j0):
        token = lane8
        for j in range(j0, j0 + NT // 2):
            inv = jnp.broadcast_to(inv2[j:j + 1], (16, 128))
            mul, sub = 1.0 + inv, m2[j:j + 1] * inv
            for i in range(0, D, 16):
                out_v[j, i:i + 16, :] = (h_v[j, i:i + 16, :].astype(F32) * mul - sub).astype(BF16)
                token = token ^ out_w[j, i // 2:i // 2 + 8, :]
                yield pltpu.bitcast(token, F32)

    def project(w_ref, j0):
        parts, side = [], unrouted(j0)
        for n in range(0, FF, 128):
            token = [next(side) for _ in range(8)][-1]
            xs = jnp.concatenate([tie(x_sel[:, :128], token), x_sel[:, 128:]], axis=1)
            parts.append(jnp.dot(xs.astype(BF16), w_ref[:, n:n + 128],
                                 preferred_element_type=F32))
        return _rbf(jnp.concatenate(parts, axis=1))

    cp_w[0].wait()
    cp_w[1].wait()
    g = project(wg_v, 0)
    act = _rbf(g * jax.nn.sigmoid(g)) * project(wu_v, NT // 2)
    routed = functools.reduce(jnp.bitwise_or, [1 << j for j in tile])
    spare = CAP - sum((routed >> j) & 1 for j in range(NT))
    n_late = 0
    for j in range(NT):
        hit = (routed >> j) & 1
        fill = (1 - hit) & (spare > 0).astype(I32)
        spare = spare - fill
        order_s[jnp.clip(jnp.where(hit + fill == 1, CAP + n_late, j - n_late), 0, NT - 1)] = j
        n_late = n_late + hit + fill

    order = [order_s[q] for q in range(NT)]
    for q in range(CAP):
        out_copy(q, 0, D, q).start()
    cp_w[2].wait()

    def placed(r, words):
        idx = jnp.zeros((CAP, 128), I32)
        for c in range(1, CAP):
            idx = jnp.where(lane_in(r, c), c, idx)
        return [_gather(w, idx) for w in words]

    def late_copies(n, lo, hi):
        return [out_copy(CAP + q, lo, hi, CAP * (n + 1) + q) for q in range(CAP)]

    def words_of(n):
        return [new_v[n].bitcast(I32)[i:i + 8, :] for i in range(0, new_v[n].shape[0] // 2, 8)]

    tokens = []
    for n, (lo, hi) in enumerate(ROW_CHUNKS):
        a = [act[:, i:i + 128] for i in range(0, FF, 128)]
        if n >= 2:
            cut = 12 * 128 // (hi - lo)
            a[cut] = tie(a[cut], tokens[n - 2])
        a = jnp.concatenate(a, axis=1)
        y = _rbf(jax.lax.dot_general(a.astype(BF16), wd_v[lo:hi, :], NT_DIMS,
                                     preferred_element_type=F32))
        new = h_sel[:, lo:hi] + _rbf(x_sel[:, lo:hi] + _rbf(y * gate))
        new_v[n][...] = jnp.concatenate(
            [new.T, jnp.zeros((hi - lo, 128 - CAP), F32)], axis=1).astype(BF16)
        rows = range(lo // 2, hi // 2, 8)
        words = words_of(n)
        both = list(zip(rows, placed(0, words), placed(1, words)))
        for c in range(CAP):
            for i, v0, v1 in both:
                pltpu.store(out_w.at[tile[c], pl.ds(i, 8), :],
                            jnp.where(rnd[c] == 0, v0, v1), mask=lane8 == col[c])
        for cp in late_copies(n, lo, hi):
            cp.start()
        out_w[tile[0], D // 2:, :] = lane8
        tokens.append(pltpu.bitcast(out_w[tile[0] | zero, D // 2:, :], F32))
    for q in range(CAP):
        out_copy(q, 0, D, q).wait()
    for n, (lo, hi) in enumerate(ROW_CHUNKS):
        for cp in late_copies(n, lo, hi):
            cp.wait()

    @pl.when(rounds > 2)
    def _():
        def fix(r, carry):
            rows = range(0, D // 2, 8)
            vals = placed(r, sum(map(words_of, range(len(new_v))), []))
            for c in range(CAP):
                for i, v in zip(rows, vals):
                    pltpu.store(out_w.at[tile[c], pl.ds(i, 8), :], v, mask=lane_in(r, c))
            return carry

        jax.lax.fori_loop(2, rounds, fix, 0)
        for cp in late_copies(0, 0, D):
            cp.start()
        for cp in late_copies(0, 0, D):
            cp.wait()


@jax.jit
def pallas_sequential_preLN__ssm_conv_s4__moe_arch_mod__prompt_kernel(
    A_u: jax.Array,
    A_A_re: jax.Array,
    A_A_im: jax.Array,
    A_B_re: jax.Array,
    A_B_im: jax.Array,
    A_C_re: jax.Array,
    A_C_im: jax.Array,
    A_log_dt: jax.Array,
    A_Dskip: jax.Array,
    B_x: jax.Array,
    B_w_r: jax.Array,
    B_w_gate: jax.Array,
    B_w_up: jax.Array,
    B_w_down: jax.Array,
):
    del B_x
    hbm = pl.BlockSpec(memory_space=pl.ANY)
    out = pl.pallas_call(
        _kernel,
        out_shape=jax.ShapeDtypeStruct((D, L), BF16),
        in_specs=[hbm] * 13,
        out_specs=hbm,
        scratch_shapes=[
            pltpu.VMEM((NT, D + 16, 128), BF16),
            pltpu.VMEM((D, FF), BF16),
            pltpu.VMEM((D, FF), BF16),
            pltpu.VMEM((D, FF), BF16),
            pltpu.VMEM((6, D, N), BF16),
            *[pltpu.VMEM((D,), BF16)] * 3,
            *[pltpu.VMEM((2, 16, 144, 128), BF16)] * 2,
            pltpu.VMEM((16, 2, 72, 128), I32),
            pltpu.VMEM((2, D, 128), F32),
            pltpu.VMEM((16, D), BF16),
            pltpu.VMEM((D // MB, 16, 128), BF16),
            pltpu.VMEM((2, 256, 128), F32),
            pltpu.VMEM((len(INDEX), 8, 128), I32),
            pltpu.VMEM((4, 3, 32, 16, 128), BF16),
            pltpu.VMEM((NT, D + 16, 128), BF16),
            pltpu.VMEM((NT, 2, 8, 128), F32),
            pltpu.VMEM((3, NT, 8, 128), F32),
            pltpu.VMEM((NT, D + 16, 128), BF16),
            *[pltpu.VMEM((4, 4, 10, 8, 128), F32)] * 2,
            *[pltpu.VMEM((4, 4, 2, 112, 128), BF16)] * 2,
            *[pltpu.VMEM((4, 4, 2, 144, 128), BF16)] * 2,
            *[pltpu.VMEM((4, 8, 128), I32)] * 2,
            *[pltpu.VMEM((16, MB // 2 + 8, 128), I32)] * 4,
            *[pltpu.VMEM((4, 4, 2, MB + 8, 128), F32)] * 2,
            *[pltpu.VMEM((4, 4, 2, MB + 8, 128), F32)] * 2,
            *[pltpu.VMEM((16, MB + 16, 128), BF16)] * 2,
            pltpu.SMEM((NT,), I32),
            pltpu.SemaphoreType.DMA((15,)),
            pltpu.SemaphoreType.DMA((NT,)),
            pltpu.SemaphoreType.DMA((3,)),
            pltpu.SemaphoreType.DMA((CAP * (1 + len(ROW_CHUNKS)),)),
            *[pltpu.VMEM((4, 4, 2, MB + 8, 128), F32)] * 2,
            *[pltpu.VMEM((hi - lo, 128), BF16) for lo, hi in ROW_CHUNKS],
        ],
        compiler_params=pltpu.CompilerParams(vmem_limit_bytes=100 * 1024 * 1024,
                                             disable_bounds_checks=True,
                                             disable_semaphore_checks=True),
    )(A_u.reshape(L, D).T, A_A_re, A_A_im, A_B_re, A_B_im, A_C_re, A_C_im,
      A_log_dt, A_Dskip, B_w_r, B_w_gate, B_w_up, B_w_down.T)
    return out.T.reshape(1, L, D)
```

```python
import functools

import numpy as np
import jax
import jax.numpy as jnp
import jax.experimental.pallas as pl
import jax.experimental.pallas.tpu as pltpu

F32 = jnp.float32
BF16 = jnp.bfloat16
I32 = jnp.int32

L = 2048
D = 576
N = 128
FF = 4608
CAP = 8
NT = L // 128
EPS = 1e-5
MB = 64
PLANS = dict(
    s=(2, ""),
    st=(2, ""),
    n=(4, ""),
    stk=(2, "0:t:-1:4 1:t:-1:3 0:t:-1:4 0:t:-1:8 0:t:-1:12 1:t:-1:10 1:t:-1:16 1:t:11:21 0:k "
            "0:k 1:k 0:s:-1:20 0:s:11:23 0:k:-1:23 1:k 1:s:20:-1 1:s 1:k "),
    stkFnf=(2, "1:t:-1:10 0:s:-1:16 0:s:-1:31 1:s:-1:36 1:s:-1:54 0:f 0:n:1:16 0:t:0:18 0:F "
               "0:t:4:25 0:k 0:k 0:k:-1:35 0:F 0:t:20:38 0:f 1:t:27:44 1:f 1:F 1:n:35:47 1:k "
               "1:t:39:55 1:k 1:t:42:55 1:k 0:t:44:53 1:F 1:f "),
    stkFnfm=(1, "0:m:-1:2 0:m:-1:5 0:t:-1:7 0:t:-1:16 0:t:-1:9 0:f 0:m:1:14 0:m:-1:15 0:f "
                "0:m:7:19 0:k 0:m:8:20 0:t:9:22 0:n:9:27 0:k 0:s:16:-1 0:m:15:-1 0:m:13:25 0:k "
                "0:s:19:-1 0:F 0:F "),
    stkFnfmi=(1, "0:t:-1:3 0:n:-1:9 0:t:-1:3 0:m:-1:10 0:m:-1:5 0:m:-1:16 0:s 0:f 0:m:0:10 0:k "
                 "0:s:4:33 0:k 0:m:13:24 0:k:-1:33 0:m:14:25 0:f 0:t:16:33 0:t:18:33 0:F 0:F "
                 "0:i 0:i 0:m:32:-1 0:m:34:-1 "),
    stkFnfmiar=(1, "0:t:-1:5 0:t:-1:3 0:n:-1:8 0:m:-1:5 0:m:-1:7 0:m:-1:18 0:s 0:f 0:m:0:17 "
                   "0:k 0:s:4:36 0:k 0:m:14:26 0:r:10:24 0:m:-1:28 0:t:13:30 0:k:-1:33 0:f "
                   "0:t:17:33 0:F 0:F 0:r:24:34 0:i 0:i 0:m:32:-1 0:a 0:m:36:-1 "),
    tkFnfmiar=(1, "0:t:-1:6 0:t:-1:4 0:n:-1:8 0:m:-1:6 0:m:-1:8 0:f 0:k 0:m:6:17 0:m:0:20 0:k "
                  "0:r:10:20 0:m:14:27 0:m:-1:26 0:k:-1:33 0:f 0:t:16:33 0:F 0:t:20:-1 0:F "
                  "0:r:25:-1 0:i 0:i 0:m:33:-1 0:m:31:-1 0:a "),
    kFnfmiar=(2, "1:m:-1:4 1:m:-1:5 0:F 0:n:0:11 0:k 0:m:4:14 0:m:-1:16 0:m:6:18 0:m:6:19 0:F "
                 "0:m:12:23 0:k 0:m:14:24 0:m:17:28 0:m:-1:31 0:k:-1:39 0:i 0:f 0:f 0:r:31:43 "
                 "0:i 0:a 1:F 1:n:37:53 1:k 1:m:41:56 1:m:39:59 1:r:44:59 1:F 1:k 1:m:51:59 "
                 "1:m:53:62 1:k 1:i 0:r:57:65 1:f 1:f 1:r:67:-1 1:i 1:m:70:-1 1:m:72:-1 1:a "),
    Ffmiar=(2, "1:m:-1:7 0:m:-1:4 0:m:-1:11 0:F 0:m:0:14 1:m:3:15 0:F 0:r:7:21 0:m:4:17 0:f "
               "0:m:11:21 0:f 0:i 1:m:16:30 0:m:18:29 0:i 1:r:21:36 0:a 1:m:24:40 1:F "
               "0:m:26:37 1:F 0:m:29:42 1:f 1:m:34:47 0:r:36:46 1:f 1:m:40:-1 1:i 1:m:41:-1 "
               "1:r:42:-1 1:i 1:m:45:-1 1:a "),
    miar=(2, "1:m:-1:2 0:m:-1:3 0:m:-1:6 0:m:-1:6 0:m:-1:7 1:r:-1:7 1:m:-1:9 0:i 0:m:1:9 "
             "0:r:2:14 0:r:3:14 0:a 1:m:4:15 0:i 1:m:6:-1 1:i 0:m:9:-1 0:m:9:-1 1:m:10:-1 "
             "1:r:11:-1 1:a 1:m:13:-1 1:i 1:m:14:-1 0:m:15:-1 1:m:17:-1 "),
    iar=(4, "2:r:-1:14 0:i 0:i 0:r:6:20 0:a 1:i 0:r:10:23 1:i 1:r:13:27 2:r:15:29 1:a 2:i 2:i 3:r:22:-1 1:r:24:35 2:a 3:i 3:i 3:r:34:-1 3:a"),
    ar=(4, "0:a 1:a 2:a 3:a"),
)
ROW_CHUNKS = ((0, 128), (128, 256), (256, 384), (384, 512), (512, D))
NT_DIMS = (((1,), (1,)), ((), ()))


def _round_res(step):
    return [int(np.round(r / step)) * step for r in range(16)]


RES1, RES2, RES3 = _round_res(2), _round_res(4), _round_res(8)


def _ds(start, size):
    return pl.ds(start if isinstance(start, int) else pl.multiple_of(start, size), size)


def _iota(shape, dim):
    return jax.lax.broadcasted_iota(I32, shape, dim)


def _rbf(x):
    return x.astype(BF16).astype(F32)


def _cmul(a, b):
    return (a[0] * b[0] - a[1] * b[1], a[0] * b[1] + a[1] * b[0])


def _csq(a):
    t = a[0] * a[1]
    return ((a[0] + a[1]) * (a[0] - a[1]), t + t)


def _cadd(a, b):
    return (a[0] + b[0], a[1] + b[1])


def _csub(a, b):
    return (a[0] - b[0], a[1] - b[1])


def _bfly4(a0, a1, a2, a3, inverse=False):
    s02, d02 = _cadd(a0, a2), _csub(a0, a2)
    s13, d13 = _cadd(a1, a3), _csub(a1, a3)
    p = (d02[0] - d13[1], d02[1] + d13[0])
    m = (d02[0] + d13[1], d02[1] - d13[0])
    if inverse:
        p, m = m, p
    return _cadd(s02, s13), p, _csub(s02, s13), m


def _prod_mod_1(a, b):
    fa, fb = _bfly4(*a), _bfly4(*b)
    return _bfly4(*[_cmul(x, y) for x, y in zip(fa, fb)], inverse=True)


def _prod2(a0, a1, b0, b1, sgn):
    p00, p11 = _cmul(a0, b0), _cmul(a1, b1)
    c1 = _cadd(_cmul(a0, b1), _cmul(a1, b0))
    if sgn > 0:
        return (p00[0] - p11[1], p00[1] + p11[0]), c1
    return (p00[0] + p11[1], p00[1] - p11[0]), c1


def _prod_mod_m1(a, b):
    def split(x):
        p = [(x[k][0] - x[k + 2][1], x[k][1] + x[k + 2][0]) for k in range(2)]
        m = [(x[k][0] + x[k + 2][1], x[k][1] - x[k + 2][0]) for k in range(2)]
        return p, m
    ap, am = split(a)
    bp, bm = split(b)
    cp = _prod2(*ap, *bp, 1)
    cm = _prod2(*am, *bm, -1)
    lo = [_cadd(cp[k], cm[k]) for k in range(2)]
    hi = [(cp[k][1] - cm[k][1], cm[k][0] - cp[k][0]) for k in range(2)]
    return lo + hi


def _prod_mod_i(a, b, sgn):
    sm = [x[0] + x[1] for x in b]
    df = [x[1] - x[0] for x in b]
    asum = [x[0] + x[1] for x in a]
    out = []
    for k in range(4):
        acc = [None, None, None]
        for j in range(4):
            m = (k - j) % 4
            if j <= k:
                t = ((b[m][0], 1), (df[m], 1), (sm[m], 1))
            elif sgn > 0:
                t = ((b[m][1], -1), (sm[m], 1), (df[m], -1))
            else:
                t = ((b[m][1], 1), (sm[m], -1), (df[m], 1))
            for q, (v, (w, s)) in enumerate(zip((asum[j], a[j][0], a[j][1]), t)):
                p = v * w
                if acc[q] is None:
                    acc[q] = p
                else:
                    acc[q] = acc[q] + p if s > 0 else acc[q] - p
        out.append((acc[0] - acc[2], acc[0] + acc[1]))
    return out


def _barrel(v, sch):
    for bit in range(4):
        m = sch.mask("bit%d" % bit)
        v = [jnp.where(m, v[(i + (1 << bit)) % 16], v[i]) for i in range(16)]
    return [v[-s % 16] for s in range(16)]


def _to_residues(tiles, sch):
    return _barrel([t if j == 0 else pltpu.roll(t, j, 1) for j, t in enumerate(tiles)], sch)


def _to_time(res, sch):
    return [t if j == 0 else pltpu.roll(t, 128 - j, 1)
            for j, t in enumerate(_barrel(res, sch))]


def _gather(x, idx, axis=1):
    return jnp.take_along_axis(x, idx, axis=axis, mode="promise_in_bounds")


def _transpose_dft(wt_ref, wu_ref, residues):
    for s in residues:
        for p in range(2):
            wt_ref[4 * (s % 4) + (0, 2, 1, 3)[s // 4], p, 0:64] = pltpu.bitcast(
                _mxu(wu_ref.bitcast(I32)[p, 4 * (s % 4) + s // 4, 0:64]).T, I32)


def _init_dft(wu_ref, wk_ref, tmp_ref, halfway):
    sub, k4 = _iota((8, 128), 0), 4 * _iota((8, 128), 1) + 1

    def cis(t):
        ph = ((k4 * t) & (4 * L - 1)).astype(F32) * (2 * np.pi / (4 * L))
        return jnp.cos(ph), jnp.sin(ph)

    w1, w16 = cis(1), cis(16)
    w32 = _csq(w16)
    fk = [cis(16 * (32 * (sub & 3) + (sub >> 2)))]
    fu = [cis(128 * sub), cis(128 * (sub + 8))]
    for v in range(1, 16):
        fk.append(_cmul(fk[-1], w32))
        if v >= 2:
            fu.append(_cmul(fu[-2], w16))
    for p in range(2):
        for v in range(32):
            tmp_ref[p, 8 * v:8 * v + 8, :] = fu[v % 16][p]
    tw = None
    for s in range(16):
        for v in range(0, 16, 2):
            rows = [slice(128 - s + 8 * i, 136 - s + 8 * i) for i in (v, v + 1)]
            for ref, f in ((wk_ref, fk[v:v + 2]),
                           (wu_ref, [(tmp_ref[0, r, :], tmp_ref[1, r, :]) for r in rows])):
                if s:
                    f = [_cmul(x, tw) for x in f]
                for p in range(2):
                    ref[p, 4 * (s % 4) + s // 4, 8 * v:8 * v + 16, :] = jnp.concatenate(
                        [f[0][p], f[1][p]], axis=0).astype(BF16)
        tw = _cmul(tw, w1) if s else w1
        if s == 7:
            halfway()


def _pack(ref, n, a, b):
    ref[n] = jnp.concatenate([a, b], axis=0).astype(BF16)
    return ref.bitcast(I32)[n]


def _split(w):
    return [pltpu.bitcast(w << 16, F32), pltpu.bitcast(w & -65536, F32)]


FINE = (0, 1, 2, 3, 4, 5, 6, 7, 512, 516, 1024, 1536)


def _k_seeds(z, c, sch):
    pw = {1: z}
    for e in range(1, 10):
        pw[1 << e] = _csq(pw[1 << (e - 1)])
    c8, z16 = _cmul(c, pw[8]), (pw[16][0], 0.0 - pw[16][1])
    pair = lambda a, b: tuple(jnp.where(sch.mask("odd"), q, p) for p, q in zip(a, b))
    seeds = []
    for g in range(2):
        twice = lambda v: tuple(_gather(x, sch.idx("dup%d" % g), 0) for x in v)
        seeds.append([twice(z), twice(pw[32]), twice(pw[512]),
                      pair(twice(c), twice(c8)), pair((1.0, 0.0), twice(z16))])
    return seeds


def _mxu(words):
    return pltpu.bitcast(words, BF16)


def _store_table(ref, tab):
    for i in range(0, len(tab), 2):
        for p in range(2):
            ref[p, 8 * i:8 * i + 16, :] = jnp.concatenate(
                [tab[i][p], tab[i + 1][p]], axis=0).astype(BF16)


def _k_residues(groups, k_last, dskip, tmp_ref, sch):
    idx, nxt = sch.idx("src"), sch.idx("nxt")
    low = lambda x, y: (x & 65535) | (y << 16)
    high = lambda x, y: jax.lax.shift_right_logical(x, 16) | (y & -65536)
    kv, up = {}, {}
    for i, k in enumerate(FINE):
        v = [g[8 * i:8 * i + 8] for g in groups]
        if k == 0:
            v = [x + jnp.where(sch.mask("diag"),
                               _gather(dskip[n // 2], sch.idx("dup%d" % (n % 2)), 0), 0.0)
                 for n, x in enumerate(v)]
        p = [_pack(tmp_ref, 2 * i + h, v[2 * h], v[2 * h + 1]) for h in range(2)]
        both = [_gather(x, idx) for x in p]
        kv[k], kv[k + 8] = low(*both), high(*both)
        if k % 512 == 0:
            up[k] = low(*[_gather(x, nxt) for x in p])
    k_last = _gather(k_last, sch.idx("rows"), 0)
    q0, q1, q2, up0, up01, up2, up3, fine = map(sch.mask, INDEX[-8:])
    s3 = {r: jnp.where(q2, kv[1024 + r], kv[1536 + r]) for r in (0, 8)}
    v0 = jnp.where(q0, kv[0], jnp.where(q1, kv[512], s3[0]))
    v16 = jnp.where(up01, jnp.where(up0, up[0], up[512]),
                    jnp.where(up2, up[1024], jnp.where(up3, up[1536], k_last)))
    s3[16] = v16
    s23, s123, out = {}, {}, [v0]
    for r in range(1, 16):
        k23 = (RES2[r], RES3[r])
        if k23 not in s23:
            s23[k23] = v16 if k23 == (16, 16) else jnp.where(q1, kv[512 + k23[0]], s3[k23[1]])
        k123 = (RES1[r],) + k23
        if k123 not in s123:
            s123[k123] = v16 if k123[0] == 16 else jnp.where(q0, kv[k123[0]], s23[k23])
        if RES1[r] == r:
            out.append(s123[k123])
        else:
            out.append(jnp.where(fine, kv[r], s123[k123]))
    return out


def _ln_scalars(s1, s2):
    mean = s1 * (1.0 / D)
    var = jnp.maximum(s2 * (1.0 / D) - mean * mean, 0.0)
    eps = float(np.asarray(EPS, dtype=BF16))
    sd = _rbf(jnp.sqrt(_rbf(_rbf(var) + eps)))
    return _rbf(mean), 1.0 / sd


def _top8(x):
    def swap(v, pairs):
        for i, j in pairs:
            v[i], v[j] = jnp.maximum(v[i], v[j]), jnp.minimum(v[i], v[j])
        return v

    def merge(a, b):
        v = [jnp.maximum(a[i], b[7 - i]) for i in range(8)]
        return swap(v, [(i, i + d) for d in (4, 2, 1) for i in range(8) if not i & d])

    sort8 = ((0, 2), (1, 3), (4, 6), (5, 7), (0, 4), (1, 5), (2, 6), (3, 7), (0, 1), (2, 3),
             (4, 5), (6, 7), (2, 4), (3, 5), (1, 4), (3, 6), (1, 2), (3, 4), (5, 6))
    v = merge(*[swap(x[i:i + 8], sort8) for i in (0, 8)])
    for d in (4, 2, 1):
        v = merge(v, [pltpu.roll(t, d, 0) for t in v])
    return v


def _init_columns(col_ref, wx_ref, wy_ref, ldt_ref, dsk_ref, wr_ref):
    row, lane = _iota((128, 128), 0), _iota((128, 128), 1)
    split = (row & ~15) + 2 * (row & 7) + ((row >> 3) & 1)
    ldt, dsk, wr = (ref[...].astype(F32).reshape(1, D) for ref in (ldt_ref, dsk_ref, wr_ref))
    for n, vec in enumerate((jnp.exp(ldt), dsk * (1.0 / L))):
        for lo in range(0, D, 128):
            i = min(lo, D - 128)
            diag = jnp.where(split == lane, vec[:, i:i + 128], 0.0)[lo - i:].astype(BF16)
            col_ref[n, lo:i + 128, :] = jnp.dot(diag, jnp.ones((128, 128), BF16),
                                                preferred_element_type=F32)
    sub = _iota((16, D), 0)
    ones_w = jnp.where(sub == 0, 1.0, jnp.where(sub == 1, wr, 0.0))
    wx_ref[...] = ones_w.astype(BF16)
    for lo in range(0, D, MB):
        wy_ref[lo // MB, :, 0:MB] = ones_w[:, lo:lo + MB].astype(BF16)
        wy_ref[lo // MB, :, MB:] = jnp.zeros((16, 128 - MB), BF16)


INDEX = ("true", "bit0", "bit1", "bit2", "bit3", "odd", "dup0", "dup1", "rows", "src", "nxt",
         "diag", "q0", "q1", "q2", "up0", "up01", "up2", "up3", "fine")


def _init_index(idx_ref):
    sub, lane = _iota((8, 128), 0), _iota((8, 128), 1)
    src = lambda b: 8 * ((b >> 1) & 15) + 2 * (sub & 3) + (b & 1)
    is_ = lambda m: jnp.where(m, 1, 0)
    q = lane & 3
    q16 = q + is_(lane >= 124)
    tiles = dict(true=sub + 1, odd=sub & 1, dup0=sub >> 1, dup1=4 + (sub >> 1),
                 rows=2 * (sub & 3) + (sub >> 2), src=src(lane >> 2), nxt=src((lane >> 2) + 1),
                 diag=is_((lane == sub) & ((sub & 1) == 0)), up01=is_(q16 < 2),
                 fine=is_((q == 0) & (lane < 64)),
                 **{"bit%d" % n: (lane >> n) & 1 for n in range(4)},
                 **{"q%d" % n: is_(q == n) for n in range(3)},
                 **{"up%d" % n: is_(q16 == n) for n in (0, 2, 3)})
    for n, name in enumerate(INDEX):
        idx_ref[n] = tiles[name]


class _Schedule:
    def __init__(self, zero, idx_ref):
        self.zero = zero
        self.idx = lambda name: idx_ref[INDEX.index(name) + zero]
        self.mask = lambda name: self.idx(name) != 0
        self.true = self.mask("true")
        self.done, self.pending, self.wait = [], {}, -1

    def tie(self, x, token):
        return jnp.where(self.true, x, token if token.dtype == x.dtype
                         else pltpu.bitcast(token, x.dtype))

    def start(self, x):
        return self.tie(x, self.done[self.wait]) if 0 <= self.wait < len(self.done) else x

    def lhs(self, words, first):
        tiles = [words[i:i + 8] for i in range(0, words.shape[0], 8)]
        for i in range(len(tiles) if first else 0):
            for token in self.pending.pop(len(self.done) + i, ()):
                tiles[i] = self.tie(tiles[i], token)
        return _mxu(jnp.concatenate(tiles, axis=0))

    def results(self, v):
        self.done += [v[i + 8:i + 16] for i in range(0, v.shape[0], 16)]

    def run(self, stage, wait, before):
        self.wait = wait
        self.pending.setdefault(before, []).extend(next(stage))


def _kernel(x_hbm, are_hbm, aim_hbm, bre_hbm, bim_hbm, cre_hbm, cim_hbm,
            ldt_hbm, dsk_hbm, wr_hbm, wg_hbm, wu_hbm, wd_hbm, out_hbm,
            x_v, wg_v, wu_v, wd_v, par_v, ldt_v, dsk_v, wr_v, w_v, wk_v, wt_v, col_v, wx_v, wy_v,
            tmp_v, idx_v, pk_v, h_v, st_v, acc_v, out_v, sd0, sd1, ta0, ta1, tb0, tb1, kl0, kl1,
            u0, u1, k0, k1, a0_v, a1_v, c0, c1, y0, y1, order_s,
            sem_p, sem_x, sem_w, sem_o, f0_v, f1_v, *rest):
    half_v, new_v = rest[:4], rest[4:]
    cp_vec = [pltpu.make_async_copy(s, d, sem_p.at[n]) for n, (s, d) in enumerate(
        ((ldt_hbm, ldt_v), (dsk_hbm, dsk_v), (wr_hbm, wr_v)))]
    cp_par = [[pltpu.make_async_copy(s.at[lo:hi], par_v.at[n, lo:hi], sem_p.at[3 + 6 * m + n])
               for n, s in enumerate((are_hbm, aim_hbm, bre_hbm, bim_hbm, cre_hbm, cim_hbm))]
              for m, (lo, hi) in enumerate(((0, 4 * MB), (4 * MB, D)))]
    cp_x = [pltpu.make_async_copy(x_hbm.at[:, 128 * j:128 * j + 128], x_v.at[j, 0:D],
                                  sem_x.at[j])
            for j in range(NT)]
    cp_w = [pltpu.make_async_copy(s, d, sem_w.at[n]) for n, (s, d) in enumerate(
        ((wg_hbm, wg_v), (wu_hbm, wu_v), (wd_hbm, wd_v)))]
    for cp in cp_vec + cp_par[0]:
        cp.start()
    for cp in cp_x[:NT // 2]:
        cp.start(priority=1)

    def columns():
        for cp in cp_vec:
            cp.wait()
        for cp in cp_x[NT // 2:]:
            cp.start(priority=1)
        _transpose_dft(wt_v, w_v, range(4))
        _init_columns(col_v, wx_v, wy_v, ldt_v, dsk_v, wr_v)

    _init_dft(w_v, wk_v, tmp_v, columns)
    for cp in cp_par[0]:
        cp.wait()

    sd, ta, tb, kl = (sd0, sd1), (ta0, ta1), (tb0, tb1), (kl0, kl1)
    uk, ab, cc, yy = ((u0, u1), (k0, k1)), ((a0_v, a1_v), (f0_v, f1_v)), (c0, c1), (y0, y1)
    ww, wt_w = (w_v.bitcast(I32), wk_v.bitcast(I32)), wt_v

    def chan(b, r):
        return _ds(b * MB + 16 * r, 16)

    def seed_stage(b, r, sch):
        rows = _ds(b * MB // 2 + 8 * r, 8)
        par = [_split(par_v.bitcast(I32)[n, rows, :]) for n in range(6)]
        for h in range(2):
            a_re, a_im, b_re, b_im, c_re, c_im = [v[h] for v in par]
            dt = sch.start(col_v[0, _ds(b * MB + 16 * r + 8 * h, 8), :])
            mag, ang = jnp.exp(dt * a_re), dt * a_im
            sc = dt * (1.0 / L)
            seeds = _k_seeds((mag * jnp.cos(ang), mag * jnp.sin(ang)),
                             _cmul((c_re, c_im), (sc * b_re, sc * b_im)), sch)
            for g in range(2):
                for n, v in enumerate(seeds[g]):
                    for p in range(2):
                        sd[b % 2][r, 2 * h + g, 2 * n + p] = v[p]
            yield [sd[b % 2][(r + sch.zero), 2 * h, 0]]

    def table_stage(b, r, sch):
        tail = []
        for g in range(4):
            m1, m32, m512, a0, b0 = [
                (sd[b % 2][r, g, 2 * n], sd[b % 2][r, g, 2 * n + 1]) for n in range(5)]
            m32 = (sch.start(m32[0]), m32[1])
            fa = [a0]
            for _ in range(7):
                fa.append(_cmul(fa[-1], m1))
            for src in (0, 4, 8, 10):
                fa.append(_cmul(fa[src], m512))
            tail.append(fa[11][0] * m512[0] - fa[11][1] * m512[1])
            _store_table(ta[b % 2].at[r, g], fa)
            fb = [b0]
            for _ in range(15):
                p = fb[-1]
                fb.append((p[0] * m32[0] + p[1] * m32[1], p[1] * m32[0] - p[0] * m32[1]))
            _store_table(tb[b % 2].at[r, g], fb)
            yield [ta[b % 2].bitcast(I32)[(r + sch.zero), g, 0, 0:8, :],
                   tb[b % 2].bitcast(I32)[(r + sch.zero), g, 0, 0:8, :]]
        last = [jnp.where(sch.mask("odd"), pltpu.roll(tail[h + 1], 1, 0), tail[h])
                for h in (0, 2)]
        last = [pltpu.bitcast(_rbf(jnp.broadcast_to(jnp.sum(v, axis=1, keepdims=True),
                                                    (8, 128))), I32) for v in last]
        kl[b % 2][r] = jax.lax.shift_right_logical(last[0], 16) | last[1]

    def kernel_stage(b, r, sch):
        ta_w, tb_w = ta[b % 2].bitcast(I32), tb[b % 2].bitcast(I32)
        groups = [None] * 4
        for g0 in (0, 2):
            res = [jax.lax.dot_general(sch.lhs(ta_w[r, g, p, 0:48], g == g0 and p == 0),
                                       _mxu(tb_w[r, g, p, 0:64]), NT_DIMS, preferred_element_type=F32)
                   for g in (g0, g0 + 1) for p in range(2)]
            groups[g0], groups[g0 + 1] = res[0] + res[1], res[2] + res[3]
            sch.results(groups[g0 + 1])
            yield []
        dskip = [col_v[1, _ds(b * MB + 16 * r + 8 * h, 8), :] for h in range(2)]
        dst = _ds(8 * r, 8)
        res = _k_residues(groups, kl[b % 2][r], dskip, pk_v.at[sch.slot, 0], sch)
        for s, t in enumerate(res):
            uk[1][b % 2][4 * (s % 4) + s // 4, dst, :] = t
        yield [uk[1][b % 2][0, _ds(8 * (r + sch.zero), 8), :]]

    def norm_stage(b, r, sch):
        tiles = []
        for j in range(NT):
            m, inv = st_v[j, 0] if j else sch.start(st_v[j, 0]), st_v[j, 1]
            xs = x_v[j, chan(b, r), :].astype(F32)
            tiles.append(_pack(pk_v.at[sch.slot, 1], j, (xs[0:8] - m) * inv, (xs[8:16] - m) * inv))
        dst = _ds(8 * r, 8)
        res = _to_residues(tiles, sch)
        for s, t in enumerate(res):
            uk[0][b % 2][4 * (s % 4) + s // 4, dst, :] = t
        yield [uk[0][b % 2][0, _ds(8 * (r + sch.zero), 8), :]]

    def forward_stage(w, b, k, sch):
        dst = ab[w][b % len(ab[w])]
        for p in range(2):
            v = [jnp.dot(sch.lhs(uk[w][b % 2][4 * k + n, 0:MB // 2], n == 0),
                         _mxu(ww[w][p ^ (n & 1), 4 * k + n, 0:64]),
                         preferred_element_type=F32) for n in range(4)]
            d02, d13 = v[0] - v[2], v[1] - v[3]
            x1 = d02 - d13 if p == 0 else d02 + d13
            dst[0, k, p, 0:MB] = v[0] + v[2]
            dst[2, k, 1 - p, 0:MB] = v[1] + v[3]
            dst[1, k, p, 0:MB] = x1
            dst[3, k, p, 0:MB] = d02 + d13 if p == 0 else d02 - d13
            sch.results(x1)
            yield []

    def stats(tiles, sch):
        ones_w = wx_v.bitcast(I32)[...]
        for j in tiles:
            acc = None
            for i in range(0, D // 2, 8):
                v = [t * t for t in _split(x_v.bitcast(I32)[j, i:i + 8, :])]
                acc = v if acc is None else [p + q for p, q in zip(acc, v)]
            sums = jnp.dot(_mxu(jnp.concatenate(
                [ones_w[:, :128] if j % 2 == 0 else sch.tie(ones_w[:, :128], prev),
                 ones_w[:, 128:]], axis=1)),
                           _mxu(x_v.bitcast(I32)[j, 0:D // 2]), preferred_element_type=F32)
            acc_v[1, j] = sums[0:8]
            s2 = prev = acc[0] + acc[1]
            for d in (4, 2, 1):
                s2 = s2 + pltpu.roll(s2, d, 0)
            st_v[j, 0], st_v[j, 1] = _ln_scalars(jnp.broadcast_to(sums[0:1], (8, 128)), s2)

    def middle_stage(b, r, sch):
        src = [v[b % len(v)] for v in ab]
        scale = lambda v, f: [(x[0] * f, x[1] * f) for x in v]
        for h in range(2):
            ra = _ds(16 * r + 8 * h, 8)
            ld = lambda q, w, ra=ra: [(src[w][q, k, 0, ra, :], src[w][q, k, 1, ra, :]) for k in range(4)]

            park_v = half_v[2 * (sch.slot % 2) + h]

            def put(q, y):
                x = [park_v[n + sch.zero] for n in range(8)]
                for k in range(4):
                    for p in range(2):
                        cc[b % 2][k, q, p, ra, :] = x[2 * k + p] + y[k][p]
                        cc[b % 2][k, q + 2, p, ra, :] = x[2 * k + p] - y[k][p]

            def park(x):
                for k in range(4):
                    for p in range(2):
                        park_v[2 * k + p] = x[k][p]
                return [park_v[sch.zero]]

            gate = sch.start
            a0, a2, b0, b2 = ld(0, 0), ld(2, 0), ld(0, 1), ld(2, 1)
            a0[0] = (gate(a0[0][0]), a0[0][1])
            e0 = _prod_mod_1(list(map(_cadd, a0, a2)), list(map(_cadd, b0, b2)))
            again = _ds(16 * (r + sch.zero) + 8 * h, 8)
            yield park(e0)
            a0, a2, b0, b2 = (ld(q, w, again) for w in range(2) for q in (0, 2))
            a2[0] = (gate(a2[0][0]), a2[0][1])
            e2 = _prod_mod_m1(list(map(_csub, a0, a2)), scale(map(_csub, b0, b2), 2.0))
            put(0, e2)
            yield [cc[b % 2][0, 0, 0, again, :]]
            four = sch.start(jnp.full((8, 128), 4.0, F32))
            e1 = _prod_mod_i(ld(1, 0), scale(ld(1, 1), four), 1)
            yield park(e1)
            four = sch.start(jnp.full((8, 128), 4.0, F32))
            e3 = _prod_mod_i(ld(3, 0), scale(ld(3, 1), four), -1)
            put(1, e3)
            yield [cc[b % 2][0, 1, 0, again, :]]

    def inverse_stage(b, k, sch):
        src = cc[b % 2]

        def lhs(v, n, first):
            return sch.lhs(jnp.concatenate(
                [_pack(pk_v.at[sch.slot, 2], 4 * n + i // 16, v[i:i + 8], v[i + 8:i + 16])
                 for i in range(0, MB, 16)], axis=0), first)

        for o in range(2):
            p0, p1 = [(src[k, q, 0, 0:MB], src[k, q, 1, 0:MB]) for q in (2 * o, 2 * o + 1)]
            if o == 0:
                e = {0: _cadd(p0, p1), 2: _csub(p0, p1)}
            else:
                e = {1: (p0[0] + p1[1], p0[1] - p1[0]), 3: (p0[0] - p1[1], p0[1] + p1[0])}
            ys = []
            for n in e:
                y = [jnp.dot(lhs(e[n][p], 2 * n + p, n == o and p == 0),
                             _mxu(wt_w[4 * k + (0, 2, 1, 3)[n], p, 0:64]),
                             preferred_element_type=F32)
                     for p in range(2)]
                ys.append(y[0] + y[1])
                yy[b % 2][k + 4 * n, 0:MB] = ys[-1].astype(BF16)
            sch.results(ys[-1])
            yield []

    def residual_stage(b, r, sch):
        rows = chan(b, r)
        src = yy[b % 2].bitcast(I32)
        ys = _to_time([src[s, _ds(8 * r, 8), :] for s in range(16)], sch)
        for j in range(NT):
            h = x_v[j, rows, :].astype(F32) + _mxu(
                ys[j] if j % 8 else sch.start(ys[j])).astype(F32)
            h_v[j, rows, :] = h.astype(BF16)
            hh = h * h
            acc_v[0, j] += hh[0:8] + hh[8:16]
            if j % 8 == 7:
                yield [acc_v[0, (r + sch.zero)]]

    def sum_stage(b, r, sch):
        for n in range(4):
            sums = jnp.dot(sch.lhs(wy_v.bitcast(I32)[b], n == 0)[:, :MB],
                           _mxu(yy[b % 2].bitcast(I32)[4 * r + n, 0:MB // 2]),
                           preferred_element_type=F32)
            acc_v[2, 4 * r + n] += sums[0:8]
        sch.results(sums)
        yield []

    nb = D // MB
    stages = dict(
        s=(seed_stage, 0), t=(table_stage, 1), k=(kernel_stage, 2),
        F=(functools.partial(forward_stage, 1), 3), n=(norm_stage, 2),
        f=(functools.partial(forward_stage, 0), 3), m=(middle_stage, 4),
        i=(inverse_stage, 5), a=(sum_stage, 6), r=(residual_stage, 6))

    def run(step, zero, live=None):
        live = live or {n: (f, step - lag) for n, (f, lag) in stages.items()
                        if 0 <= step - lag < nb and (n, step) != ("n", 2)}
        unroll, plan = PLANS["".join(live)]

        def body(it, carry):
            sch = _Schedule(zero >> (step % 32) if unroll == 4 else zero & it, idx_v)
            gens = [{n: f(b, it * unroll + u, sch) for n, (f, b) in live.items()}
                    for u in range(unroll)]
            for item in plan.split():
                u, n, *ties = item.split(":")
                if n in live:
                    sch.slot = int(u)
                    sch.run(gens[int(u)][n], *map(int, ties or (-1, -1)))
            for sch.slot, g in enumerate(gens):
                for v in g.values():
                    for _ in v:
                        pass
            return carry + it

        if unroll == 4:
            return body(0, 0)
        return jax.lax.fori_loop(0, 4 // unroll, body, 0)

    _init_index(idx_v)
    acc_v[...] = jnp.zeros(acc_v.shape, F32)
    zero = run(0, 0) - 1
    for step in range(1, nb + 6):
        if step == 4:
            for cp in cp_par[1]:
                cp.wait()
        if step == 3:
            for half in range(2):
                tiles = range(NT // 2 * half, NT // 2 * (half + 1))
                for j in tiles:
                    cp_x[j].wait()
                if half:
                    for cp in cp_par[1]:
                        cp.start()
                    for cp in cp_w:
                        cp.start(priority=1)
                _transpose_dft(wt_v, w_v, range(4 + 6 * half, 10 + 6 * half))
                stats(tiles, _Schedule(zero, idx_v))
            run(101, zero, dict(n=(norm_stage, 0)))
        run(step, zero)

    sums = [acc_v[1, j] + v
            for j, v in enumerate(_to_time([acc_v[2, s] for s in range(16)],
                                          _Schedule(0, idx_v)))]
    m2, inv2 = _ln_scalars(
        jnp.concatenate([v[0:1] for v in sums], axis=0),
        jnp.concatenate([jnp.sum(acc_v[0, j], axis=0, keepdims=True) for j in range(NT)], axis=0))
    wsum = jnp.sum(wr_v[...].astype(F32).reshape(1, D), axis=1, keepdims=True)
    score = _rbf((jnp.concatenate([v[1:2] for v in sums], axis=0) - m2 * wsum) * inv2 + 0.0)
    bits = pltpu.bitcast(score, I32) >> 16
    order = jnp.where(bits < 0, -1 - bits, bits + 32768)
    pos = 128 * _iota((NT, 128), 0) + _iota((NT, 128), 1)
    key = pltpu.bitcast((order << 11) + (L - 1 - pos) + (1 << 29), F32)

    lane8, sub8 = _iota((CAP, 128), 1), _iota((CAP, 128), 0)
    best = _top8([pltpu.roll(key[i:i + 8], n, 1) if n else key[i:i + 8]
                  for i in (0, 8) for n in range(8)])
    cand = best[0]
    for c in range(1, CAP):
        cand = jnp.where(sub8 == c, best[c], cand)
    best = [pltpu.bitcast(v, I32)[0, 0]
            for v in _top8([pltpu.roll(cand, n, 1) if n else cand for n in range(0, 128, 8)])]
    picks = [L - 1 - (v & (L - 1)) for v in best]
    tile, col = [t >> 7 for t in picks], [t & 127 for t in picks]
    rnd = [sum([(col[e] == col[c]).astype(I32) for e in range(c)], 0) for c in range(CAP)]
    rounds = functools.reduce(jnp.maximum, rnd) + 1
    lane_in = lambda n, c: lane8 == jnp.where(rnd[c] == n, col[c], -1)

    def out_copy(q, lo, hi, n):
        j = order[q]
        return pltpu.make_async_copy(
            out_v.at[j, lo:hi], out_hbm.at[lo:hi, _ds(j * 128, 128)], sem_o.at[n])

    h_w, out_w = h_v.bitcast(I32), out_v.bitcast(I32)

    def gather(n, acc):
        masks = [lane_in(n, c) for c in range(CAP)]
        tiles = []
        for i in range(0, D // 2, 8):
            v = jnp.zeros((8, 128), I32)
            for c in range(CAP):
                v = jnp.where(masks[c], h_w[tile[c], i:i + 8, :], v)
            tiles.append(v)
        lhs = jnp.zeros((CAP, 128), F32)
        for c in range(CAP):
            lhs = jnp.where(masks[c] & (sub8 == c), 1.0, lhs)
        aux = [jnp.zeros((CAP, 128), F32)] * 3
        for c in range(CAP):
            hit = pltpu.bitcast(key, I32) == best[c]
            aux = [jnp.where(sub8 == c, jnp.sum(jnp.where(hit, v, 0.0), axis=0, keepdims=True), a)
                   for a, v in zip(aux, (m2, inv2, score))]
        return (acc[0] + jax.lax.dot_general(lhs.astype(BF16), _mxu(jnp.concatenate(tiles, axis=0)),
                                             NT_DIMS, preferred_element_type=F32),
                *[jnp.sum(a, axis=1, keepdims=True) for a in aux])

    h_sel, m_sel, inv_sel, score_sel = jax.lax.fori_loop(
        0, rounds, gather, (jnp.zeros((CAP, D), F32), *[jnp.zeros((CAP, 1), F32)] * 3))
    x_sel = _rbf((h_sel - m_sel) * inv_sel)
    gate = _rbf(jax.nn.sigmoid(score_sel))

    true = lane8 + picks[0] >= 0
    tie = lambda x, token: jnp.where(true, x, token)

    def unrouted(j0):
        token = lane8
        for j in range(j0, j0 + NT // 2):
            inv = jnp.broadcast_to(inv2[j:j + 1], (16, 128))
            mul, sub = 1.0 + inv, m2[j:j + 1] * inv
            for i in range(0, D, 16):
                out_v[j, i:i + 16, :] = (h_v[j, i:i + 16, :].astype(F32) * mul - sub).astype(BF16)
                token = token ^ out_w[j, i // 2:i // 2 + 8, :]
                yield pltpu.bitcast(token, F32)

    def project(w_ref, j0):
        parts, side = [], unrouted(j0)
        for n in range(0, FF, 128):
            token = [next(side) for _ in range(8)][-1]
            xs = jnp.concatenate([tie(x_sel[:, :128], token), x_sel[:, 128:]], axis=1)
            parts.append(jnp.dot(xs.astype(BF16), w_ref[:, n:n + 128],
                                 preferred_element_type=F32))
        return _rbf(jnp.concatenate(parts, axis=1))

    cp_w[0].wait()
    cp_w[1].wait()
    g = project(wg_v, 0)
    act = _rbf(g * jax.nn.sigmoid(g)) * project(wu_v, NT // 2)
    routed = functools.reduce(jnp.bitwise_or, [1 << j for j in tile])
    spare = CAP - sum((routed >> j) & 1 for j in range(NT))
    n_late = 0
    for j in range(NT):
        hit = (routed >> j) & 1
        fill = (1 - hit) & (spare > 0).astype(I32)
        spare = spare - fill
        order_s[jnp.clip(jnp.where(hit + fill == 1, CAP + n_late, j - n_late), 0, NT - 1)] = j
        n_late = n_late + hit + fill

    order = [order_s[q] for q in range(NT)]
    for q in range(CAP):
        out_copy(q, 0, D, q).start()
    cp_w[2].wait()

    def placed(r, words):
        idx = jnp.zeros((CAP, 128), I32)
        for c in range(1, CAP):
            idx = jnp.where(lane_in(r, c), c, idx)
        return [_gather(w, idx) for w in words]

    def late_copies(n, lo, hi):
        return [out_copy(CAP + q, lo, hi, CAP * (n + 1) + q) for q in range(CAP)]

    def words_of(n):
        return [new_v[n].bitcast(I32)[i:i + 8, :] for i in range(0, new_v[n].shape[0] // 2, 8)]

    tokens = []
    for n, (lo, hi) in enumerate(ROW_CHUNKS):
        a = [act[:, i:i + 128] for i in range(0, FF, 128)]
        if n >= 2:
            cut = 12 * 128 // (hi - lo)
            a[cut] = tie(a[cut], tokens[n - 2])
        a = jnp.concatenate(a, axis=1)
        y = _rbf(jax.lax.dot_general(a.astype(BF16), wd_v[lo:hi, :], NT_DIMS,
                                     preferred_element_type=F32))
        new = h_sel[:, lo:hi] + _rbf(x_sel[:, lo:hi] + _rbf(y * gate))
        new_v[n][...] = jnp.concatenate(
            [new.T, jnp.zeros((hi - lo, 128 - CAP), F32)], axis=1).astype(BF16)
        rows = range(lo // 2, hi // 2, 8)
        words = words_of(n)
        both = list(zip(rows, placed(0, words), placed(1, words)))
        for c in range(CAP):
            for i, v0, v1 in both:
                pltpu.store(out_w.at[tile[c], pl.ds(i, 8), :],
                            jnp.where(rnd[c] == 0, v0, v1), mask=lane8 == col[c])
        for cp in late_copies(n, lo, hi):
            cp.start()
        out_w[tile[0], D // 2:, :] = lane8
        tokens.append(pltpu.bitcast(out_w[tile[0] | zero, D // 2:, :], F32))
    for q in range(CAP):
        out_copy(q, 0, D, q).wait()
    for n, (lo, hi) in enumerate(ROW_CHUNKS):
        for cp in late_copies(n, lo, hi):
            cp.wait()

    @pl.when(rounds > 2)
    def _():
        def fix(r, carry):
            rows = range(0, D // 2, 8)
            vals = placed(r, sum(map(words_of, range(len(new_v))), []))
            for c in range(CAP):
                for i, v in zip(rows, vals):
                    pltpu.store(out_w.at[tile[c], pl.ds(i, 8), :], v, mask=lane_in(r, c))
            return carry

        jax.lax.fori_loop(2, rounds, fix, 0)
        for cp in late_copies(0, 0, D):
            cp.start()
        for cp in late_copies(0, 0, D):
            cp.wait()


@jax.jit
def pallas_sequential_preLN__ssm_conv_s4__moe_arch_mod__prompt_kernel(
    A_u: jax.Array,
    A_A_re: jax.Array,
    A_A_im: jax.Array,
    A_B_re: jax.Array,
    A_B_im: jax.Array,
    A_C_re: jax.Array,
    A_C_im: jax.Array,
    A_log_dt: jax.Array,
    A_Dskip: jax.Array,
    B_x: jax.Array,
    B_w_r: jax.Array,
    B_w_gate: jax.Array,
    B_w_up: jax.Array,
    B_w_down: jax.Array,
):
    del B_x
    hbm = pl.BlockSpec(memory_space=pl.ANY)
    out = pl.pallas_call(
        _kernel,
        out_shape=jax.ShapeDtypeStruct((D, L), BF16),
        in_specs=[hbm] * 13,
        out_specs=hbm,
        scratch_shapes=[
            pltpu.VMEM((NT, D + 16, 128), BF16),
            pltpu.VMEM((D, FF), BF16),
            pltpu.VMEM((D, FF), BF16),
            pltpu.VMEM((D, FF), BF16),
            pltpu.VMEM((6, D, N), BF16),
            *[pltpu.VMEM((D,), BF16)] * 3,
            *[pltpu.VMEM((2, 16, 144, 128), BF16)] * 2,
            pltpu.VMEM((16, 2, 72, 128), I32),
            pltpu.VMEM((2, D, 128), F32),
            pltpu.VMEM((16, D), BF16),
            pltpu.VMEM((D // MB, 16, 128), BF16),
            pltpu.VMEM((2, 256, 128), F32),
            pltpu.VMEM((len(INDEX), 8, 128), I32),
            pltpu.VMEM((4, 3, 32, 16, 128), BF16),
            pltpu.VMEM((NT, D + 16, 128), BF16),
            pltpu.VMEM((NT, 2, 8, 128), F32),
            pltpu.VMEM((3, NT, 8, 128), F32),
            pltpu.VMEM((NT, D + 16, 128), BF16),
            *[pltpu.VMEM((4, 4, 10, 8, 128), F32)] * 2,
            *[pltpu.VMEM((4, 4, 2, 112, 128), BF16)] * 2,
            *[pltpu.VMEM((4, 4, 2, 144, 128), BF16)] * 2,
            *[pltpu.VMEM((4, 8, 128), I32)] * 2,
            *[pltpu.VMEM((16, MB // 2 + 8, 128), I32)] * 4,
            *[pltpu.VMEM((4, 4, 2, MB + 8, 128), F32)] * 2,
            *[pltpu.VMEM((4, 4, 2, MB + 8, 128), F32)] * 2,
            *[pltpu.VMEM((16, MB + 16, 128), BF16)] * 2,
            pltpu.SMEM((NT,), I32),
            pltpu.SemaphoreType.DMA((15,)),
            pltpu.SemaphoreType.DMA((NT,)),
            pltpu.SemaphoreType.DMA((3,)),
            pltpu.SemaphoreType.DMA((CAP * (1 + len(ROW_CHUNKS)),)),
            *[pltpu.VMEM((4, 4, 2, MB + 8, 128), F32)] * 2,
            *[pltpu.VMEM((8, 8, 128), F32)] * 4,
            *[pltpu.VMEM((hi - lo, 128), BF16) for lo, hi in ROW_CHUNKS],
        ],
        compiler_params=pltpu.CompilerParams(vmem_limit_bytes=100 * 1024 * 1024,
                                             disable_bounds_checks=True,
                                             disable_semaphore_checks=True),
    )(A_u.reshape(L, D).T, A_A_re, A_A_im, A_B_re, A_B_im, A_C_re, A_C_im,
      A_log_dt, A_Dskip, B_w_r, B_w_gate, B_w_up, B_w_down.T)
    return out.T.reshape(1, L, D)
```

```python
import functools

import numpy as np
import jax
import jax.numpy as jnp
import jax.experimental.pallas as pl
import jax.experimental.pallas.tpu as pltpu

F32 = jnp.float32
BF16 = jnp.bfloat16
I32 = jnp.int32

L = 2048
D = 576
N = 128
FF = 4608
CAP = 8
NT = L // 128
EPS = 1e-5
MB = 64
PLANS = dict(
    s=(2, ""),
    st=(2, ""),
    n=(4, ""),
    stk=(2, "0:t:-1:4 1:t:-1:3 0:t:-1:4 0:t:-1:7 0:t:-1:15 1:t:-1:10 1:t:6:16 1:t:11:21 0:k "
            "0:k 1:k 0:s:-1:20 0:s:11:23 0:k:-1:23 1:k 1:s:20:-1 1:s 1:k "),
    stkFnf=(2, "1:t:-1:4 0:s:-1:16 0:s:-1:34 1:s:-1:36 1:s:-1:54 0:f 0:n:1:16 0:F 0:t:4:25 "
               "0:t:0:21 0:k 0:k 0:k:-1:35 0:t:17:36 0:F 0:f 1:f 1:t:29:43 1:F 1:n:33:47 1:k "
               "1:t:39:55 1:k 1:t:42:53 1:k 0:t:44:53 1:F 1:f "),
    stkFnfm=(1, "0:m:-1:2 0:m:-1:5 0:t:-1:7 0:t:-1:14 0:t:-1:9 0:f 0:m:1:14 0:m:-1:18 0:f "
                "0:m:7:21 0:m:6:20 0:k 0:t:9:22 0:n:9:27 0:k 0:s:16:-1 0:m:15:-1 0:m:13:25 0:k "
                "0:s:19:-1 0:F 0:F "),
    stkFnfmi=(2, "0:t:-1:3 0:n:-1:8 0:t:-1:3 0:m:-1:7 0:m:-1:7 0:m:-1:19 0:s:-1:40 1:s 0:f "
                 "0:m:0:11 0:k 0:s:4:33 0:k 0:m:13:23 0:k:-1:33 0:m:14:25 0:t:14:33 0:f "
                 "0:t:18:33 0:F 1:t:23:41 0:F 1:t:24:38 1:m:27:44 0:i 1:n:29:47 1:m:29:47 0:i "
                 "0:m:32:40 0:m:31:42 1:f 1:m:39:57 1:m:36:49 1:k 1:s:40:71 1:k 1:m:49:61 "
                 "1:k:-1:71 1:m:51:63 1:f 1:t:55:-1 1:t:51:68 1:F 1:F 1:i 1:i 1:m:68:-1 "
                 "1:m:67:-1 "),
    stkFnfmia=(1, "0:t:-1:6 0:t:-1:4 0:n:-1:9 0:m:-1:6 0:m:-1:8 0:m:-1:19 0:s 0:a 0:f 0:m:1:18 "
                  "0:k 0:s:5:-1 0:k 0:m:15:27 0:m:-1:29 0:k 0:t:16:30 0:f 0:t:18:34 0:F 0:F "
                  "0:i 0:m:32:-1 0:i 0:m:34:-1 "),
    tkFnfmia=(1, "0:t:-1:10 0:t:-1:5 0:n:-1:9 0:m:-1:6 0:m:-1:9 0:a 0:f 0:k 0:m:7:18 0:m:1:23 "
                 "0:k 0:m:15:28 0:m:-1:27 0:k:-1:36 0:f 0:t:17:34 0:t:20:-1 0:F 0:F 0:i "
                 "0:m:31:-1 0:i 0:m:34:-1 "),
    kFnfmia=(2, "1:m:-1:5 1:m:-1:3 0:n:-1:12 0:F 0:m:2:14 0:m:-1:15 0:a 0:F 0:m:7:21 0:k "
                "0:m:9:27 0:m:13:23 0:k 0:m:15:25 0:m:18:31 0:m:-1:32 0:k:-1:45 0:i 0:i 0:f "
                "0:f 1:n:36:50 1:F 1:a 1:F 1:m:42:57 1:m:37:59 1:k 1:m:47:67 1:k 1:m:53:66 1:k "
                "1:i 1:i 1:f 1:m:68:-1 1:f 1:m:71:-1 "),
    Ffmia=(2, "1:m:-1:8 0:m:-1:5 0:m:-1:10 0:m:-1:12 0:a 0:F 1:m:4:15 0:i 0:m:6:18 0:i "
              "0:m:9:22 0:F 1:m:15:30 0:f 0:m:20:30 0:f 0:m:22:33 1:a 1:m:25:43 1:F 0:m:29:43 "
              "1:i 1:i 1:m:35:48 1:F 1:m:40:-1 1:f 1:m:42:-1 1:m:45:-1 1:f "),
    mia=(4, "1:m:-1:3 0:m:-1:8 0:m:-1:6 0:m:-1:7 0:m:-1:8 0:i 1:m:0:13 0:m:2:10 0:a 0:i "
            "1:m:5:16 1:i 1:m:9:22 0:m:10:23 0:m:8:20 1:m:8:20 3:m:11:25 2:m:11:25 1:a "
            "2:m:13:27 1:i 1:m:14:22 1:m:17:25 0:m:14:22 1:m:17:25 2:m:14:28 2:m:13:27 2:i "
            "3:m:18:32 2:m:20:32 2:a 2:i 3:m:23:-1 3:m:25:-1 3:m:25:-1 3:i 2:m:28:-1 2:m:27:-1 "
            "3:a 3:i 3:m:32:-1 3:m:35:-1 2:m:33:-1 3:m:35:-1 "),
    ia=(4, "0:a 0:i 0:i 1:a 1:i 1:i 2:a 2:i 2:i 3:a 3:i 3:i"),
    a=(4, "0:a 1:a 2:a 3:a"),
)
ROW_CHUNKS = ((0, 128), (128, 256), (256, 384), (384, 512), (512, D))
LAG = 16
MID, SPAN, EARLY = 384, 50, 8
NT_DIMS = (((1,), (1,)), ((), ()))


def _round_res(step):
    return [int(np.round(r / step)) * step for r in range(16)]


RES1, RES2, RES3 = _round_res(2), _round_res(4), _round_res(8)


def _ds(start, size):
    return pl.ds(start if isinstance(start, int) else pl.multiple_of(start, size), size)


def _iota(shape, dim):
    return jax.lax.broadcasted_iota(I32, shape, dim)


def _rbf(x):
    return x.astype(BF16).astype(F32)


def _cmul(a, b):
    return (a[0] * b[0] - a[1] * b[1], a[0] * b[1] + a[1] * b[0])


def _csq(a):
    t = a[0] * a[1]
    return ((a[0] + a[1]) * (a[0] - a[1]), t + t)


def _cadd(a, b):
    return (a[0] + b[0], a[1] + b[1])


def _csub(a, b):
    return (a[0] - b[0], a[1] - b[1])


def _bfly4(a0, a1, a2, a3, inverse=False):
    s02, d02 = _cadd(a0, a2), _csub(a0, a2)
    s13, d13 = _cadd(a1, a3), _csub(a1, a3)
    p = (d02[0] - d13[1], d02[1] + d13[0])
    m = (d02[0] + d13[1], d02[1] - d13[0])
    if inverse:
        p, m = m, p
    return _cadd(s02, s13), p, _csub(s02, s13), m


def _prod_mod_1(a, b):
    fa, fb = _bfly4(*a), _bfly4(*b)
    return _bfly4(*[_cmul(x, y) for x, y in zip(fa, fb)], inverse=True)


def _prod2(a0, a1, b0, b1, sgn):
    p00, p11 = _cmul(a0, b0), _cmul(a1, b1)
    c1 = _cadd(_cmul(a0, b1), _cmul(a1, b0))
    if sgn > 0:
        return (p00[0] - p11[1], p00[1] + p11[0]), c1
    return (p00[0] + p11[1], p00[1] - p11[0]), c1


def _prod_mod_m1(a, b):
    def split(x):
        p = [(x[k][0] - x[k + 2][1], x[k][1] + x[k + 2][0]) for k in range(2)]
        m = [(x[k][0] + x[k + 2][1], x[k][1] - x[k + 2][0]) for k in range(2)]
        return p, m
    ap, am = split(a)
    bp, bm = split(b)
    cp = _prod2(*ap, *bp, 1)
    cm = _prod2(*am, *bm, -1)
    lo = [_cadd(cp[k], cm[k]) for k in range(2)]
    hi = [(cp[k][1] - cm[k][1], cm[k][0] - cp[k][0]) for k in range(2)]
    return lo + hi


def _prod_mod_i(a, b, sgn):
    sm = [x[0] + x[1] for x in b]
    df = [x[1] - x[0] for x in b]
    asum = [x[0] + x[1] for x in a]
    out = []
    for k in range(4):
        acc = [None, None, None]
        for j in range(4):
            m = (k - j) % 4
            if j <= k:
                t = ((b[m][0], 1), (df[m], 1), (sm[m], 1))
            elif sgn > 0:
                t = ((b[m][1], -1), (sm[m], 1), (df[m], -1))
            else:
                t = ((b[m][1], 1), (sm[m], -1), (df[m], 1))
            for q, (v, (w, s)) in enumerate(zip((asum[j], a[j][0], a[j][1]), t)):
                p = v * w
                if acc[q] is None:
                    acc[q] = p
                else:
                    acc[q] = acc[q] + p if s > 0 else acc[q] - p
        out.append((acc[0] - acc[2], acc[0] + acc[1]))
    return out


def _barrel(v, sch):
    for bit in range(4):
        m = sch.mask("bit%d" % bit)
        v = [jnp.where(m, v[(i + (1 << bit)) % 16], v[i]) for i in range(16)]
    return [v[-s % 16] for s in range(16)]


def _to_residues(tiles, sch):
    return _barrel([t if j == 0 else pltpu.roll(t, j, 1) for j, t in enumerate(tiles)], sch)


def _to_time(res, sch):
    return [t if j == 0 else pltpu.roll(t, 128 - j, 1)
            for j, t in enumerate(_barrel(res, sch))]


def _gather(x, idx, axis=1):
    return jnp.take_along_axis(x, idx, axis=axis, mode="promise_in_bounds")


def _transpose_dft(wt_ref, wu_ref, residues):
    for s in residues:
        for p in range(2):
            wt_ref[4 * (s % 4) + (0, 2, 1, 3)[s // 4], p, 0:64] = pltpu.bitcast(
                _mxu(wu_ref.bitcast(I32)[p, 4 * (s % 4) + s // 4, 0:64]).T, I32)


def _init_dft(wu_ref, wk_ref, tmp_ref, halfway):
    sub, k4 = _iota((8, 128), 0), 4 * _iota((8, 128), 1) + 1

    def cis(t):
        ph = ((k4 * t) & (4 * L - 1)).astype(F32) * (2 * np.pi / (4 * L))
        return jnp.cos(ph), jnp.sin(ph)

    w1, w16 = cis(1), cis(16)
    w32 = _csq(w16)
    fk = [cis(16 * (32 * (sub & 3) + (sub >> 2)))]
    fu = [cis(128 * sub), cis(128 * (sub + 8))]
    for v in range(1, 16):
        fk.append(_cmul(fk[-1], w32))
        if v >= 2:
            fu.append(_cmul(fu[-2], w16))
    for p in range(2):
        for v in range(32):
            tmp_ref[p, 8 * v:8 * v + 8, :] = fu[v % 16][p]
    tw = None
    for s in range(16):
        for v in range(0, 16, 2):
            rows = [slice(128 - s + 8 * i, 136 - s + 8 * i) for i in (v, v + 1)]
            for ref, f in ((wk_ref, fk[v:v + 2]),
                           (wu_ref, [(tmp_ref[0, r, :], tmp_ref[1, r, :]) for r in rows])):
                if s:
                    f = [_cmul(x, tw) for x in f]
                for p in range(2):
                    ref[p, 4 * (s % 4) + s // 4, 8 * v:8 * v + 16, :] = jnp.concatenate(
                        [f[0][p], f[1][p]], axis=0).astype(BF16)
        tw = _cmul(tw, w1) if s else w1
        if s == 7:
            halfway()


def _pack(ref, n, a, b):
    ref[n] = jnp.concatenate([a, b], axis=0).astype(BF16)
    return ref.bitcast(I32)[n]


def _split(w):
    return [pltpu.bitcast(w << 16, F32), pltpu.bitcast(w & -65536, F32)]


FINE = (0, 1, 2, 3, 4, 5, 6, 7, 512, 516, 1024, 1536)


def _k_seeds(z, c, sch):
    pw = {1: z}
    for e in range(1, 10):
        pw[1 << e] = _csq(pw[1 << (e - 1)])
    c8, z16 = _cmul(c, pw[8]), (pw[16][0], 0.0 - pw[16][1])
    pair = lambda a, b: tuple(jnp.where(sch.mask("odd"), q, p) for p, q in zip(a, b))
    seeds = []
    for g in range(2):
        twice = lambda v: tuple(_gather(x, sch.idx("dup%d" % g), 0) for x in v)
        seeds.append([twice(z), twice(pw[32]), twice(pw[512]),
                      pair(twice(c), twice(c8)), pair((1.0, 0.0), twice(z16))])
    return seeds


def _mxu(words):
    return pltpu.bitcast(words, BF16)


def _store_table(ref, tab):
    for i in range(0, len(tab), 2):
        for p in range(2):
            ref[p, 8 * i:8 * i + 16, :] = jnp.concatenate(
                [tab[i][p], tab[i + 1][p]], axis=0).astype(BF16)


def _k_residues(groups, k_last, dskip, tmp_ref, sch):
    idx, nxt = sch.idx("src"), sch.idx("nxt")
    low = lambda x, y: (x & 65535) | (y << 16)
    high = lambda x, y: jax.lax.shift_right_logical(x, 16) | (y & -65536)
    kv, up = {}, {}
    for i, k in enumerate(FINE):
        v = [g[8 * i:8 * i + 8] for g in groups]
        if k == 0:
            v = [x + jnp.where(sch.mask("diag"),
                               _gather(dskip[n // 2], sch.idx("dup%d" % (n % 2)), 0), 0.0)
                 for n, x in enumerate(v)]
        p = [_pack(tmp_ref, 2 * i + h, v[2 * h], v[2 * h + 1]) for h in range(2)]
        both = [_gather(x, idx) for x in p]
        kv[k], kv[k + 8] = low(*both), high(*both)
        if k % 512 == 0:
            up[k] = low(*[_gather(x, nxt) for x in p])
    k_last = _gather(k_last, sch.idx("rows"), 0)
    q0, q1, q2, up0, up01, up2, up3, fine = map(sch.mask, INDEX[-8:])
    s3 = {r: jnp.where(q2, kv[1024 + r], kv[1536 + r]) for r in (0, 8)}
    v0 = jnp.where(q0, kv[0], jnp.where(q1, kv[512], s3[0]))
    v16 = jnp.where(up01, jnp.where(up0, up[0], up[512]),
                    jnp.where(up2, up[1024], jnp.where(up3, up[1536], k_last)))
    s3[16] = v16
    s23, s123, out = {}, {}, [v0]
    for r in range(1, 16):
        k23 = (RES2[r], RES3[r])
        if k23 not in s23:
            s23[k23] = v16 if k23 == (16, 16) else jnp.where(q1, kv[512 + k23[0]], s3[k23[1]])
        k123 = (RES1[r],) + k23
        if k123 not in s123:
            s123[k123] = v16 if k123[0] == 16 else jnp.where(q0, kv[k123[0]], s23[k23])
        if RES1[r] == r:
            out.append(s123[k123])
        else:
            out.append(jnp.where(fine, kv[r], s123[k123]))
    return out


def _ln_scalars(s1, s2):
    mean = s1 * (1.0 / D)
    var = jnp.maximum(s2 * (1.0 / D) - mean * mean, 0.0)
    eps = float(np.asarray(EPS, dtype=BF16))
    sd = _rbf(jnp.sqrt(_rbf(_rbf(var) + eps)))
    return _rbf(mean), 1.0 / sd


def _top8(x):
    def swap(v, pairs):
        for i, j in pairs:
            v[i], v[j] = jnp.maximum(v[i], v[j]), jnp.minimum(v[i], v[j])
        return v

    def merge(a, b):
        v = [jnp.maximum(a[i], b[7 - i]) for i in range(8)]
        return swap(v, [(i, i + d) for d in (4, 2, 1) for i in range(8) if not i & d])

    sort8 = ((0, 2), (1, 3), (4, 6), (5, 7), (0, 4), (1, 5), (2, 6), (3, 7), (0, 1), (2, 3),
             (4, 5), (6, 7), (2, 4), (3, 5), (1, 4), (3, 6), (1, 2), (3, 4), (5, 6))
    v = merge(*[swap(x[i:i + 8], sort8) for i in (0, 8)])
    for d in (4, 2, 1):
        v = merge(v, [pltpu.roll(t, d, 0) for t in v])
    return v


def _init_columns(col_ref, wx_ref, wy_ref, ldt_ref, dsk_ref, wr_ref):
    row, lane = _iota((128, 128), 0), _iota((128, 128), 1)
    split = (row & ~15) + 2 * (row & 7) + ((row >> 3) & 1)
    ldt, dsk, wr = (ref[...].astype(F32).reshape(1, D) for ref in (ldt_ref, dsk_ref, wr_ref))
    for n, vec in enumerate((jnp.exp(ldt), dsk * (1.0 / L))):
        for lo in range(0, D, 128):
            i = min(lo, D - 128)
            diag = jnp.where(split == lane, vec[:, i:i + 128], 0.0)[lo - i:].astype(BF16)
            col_ref[n, lo:i + 128, :] = jnp.dot(diag, jnp.ones((128, 128), BF16),
                                                preferred_element_type=F32)
    sub = _iota((16, D), 0)
    ones_w = jnp.where(sub == 0, 1.0, jnp.where(sub == 1, wr, 0.0))
    wx_ref[...] = ones_w.astype(BF16)
    for lo in range(0, D, MB):
        wy_ref[lo // MB, :, 0:MB] = ones_w[:, lo:lo + MB].astype(BF16)
        wy_ref[lo // MB, :, MB:] = jnp.zeros((16, 128 - MB), BF16)


INDEX = ("true", "bit0", "bit1", "bit2", "bit3", "odd", "dup0", "dup1", "rows", "src", "nxt",
         "diag", "q0", "q1", "q2", "up0", "up01", "up2", "up3", "fine")


def _init_index(idx_ref):
    sub, lane = _iota((8, 128), 0), _iota((8, 128), 1)
    src = lambda b: 8 * ((b >> 1) & 15) + 2 * (sub & 3) + (b & 1)
    is_ = lambda m: jnp.where(m, 1, 0)
    q = lane & 3
    q16 = q + is_(lane >= 124)
    tiles = dict(true=sub + 1, odd=sub & 1, dup0=sub >> 1, dup1=4 + (sub >> 1),
                 rows=2 * (sub & 3) + (sub >> 2), src=src(lane >> 2), nxt=src((lane >> 2) + 1),
                 diag=is_((lane == sub) & ((sub & 1) == 0)), up01=is_(q16 < 2),
                 fine=is_((q == 0) & (lane < 64)),
                 **{"bit%d" % n: (lane >> n) & 1 for n in range(4)},
                 **{"q%d" % n: is_(q == n) for n in range(3)},
                 **{"up%d" % n: is_(q16 == n) for n in (0, 2, 3)})
    for n, name in enumerate(INDEX):
        idx_ref[n] = tiles[name]


class _Schedule:
    def __init__(self, zero, idx_ref):
        self.zero = zero
        self.idx = lambda name: idx_ref[INDEX.index(name) + zero]
        self.mask = lambda name: self.idx(name) != 0
        self.true = self.mask("true")
        self.done, self.pending, self.wait = [], {}, -1

    def tie(self, x, token):
        return jnp.where(self.true, x, token if token.dtype == x.dtype
                         else pltpu.bitcast(token, x.dtype))

    def start(self, x):
        return self.tie(x, self.done[self.wait]) if 0 <= self.wait < len(self.done) else x

    def lhs(self, words, first):
        tiles = [words[i:i + 8] for i in range(0, words.shape[0], 8)]
        for i in range(len(tiles) if first else 0):
            for token in self.pending.pop(len(self.done) + i, ()):
                tiles[i] = self.tie(tiles[i], token)
        return _mxu(jnp.concatenate(tiles, axis=0))

    def results(self, v):
        self.done += [v[i + 8:i + 16] for i in range(0, v.shape[0], 16)]

    def run(self, stage, wait, before):
        self.wait = wait
        self.pending.setdefault(before, []).extend(next(stage))


def _kernel(x_hbm, are_hbm, aim_hbm, bre_hbm, bim_hbm, cre_hbm, cim_hbm,
            ldt_hbm, dsk_hbm, wr_hbm, wg_hbm, wu_hbm, wd_hbm, out_hbm,
            x_v, wg_v, wu_v, wd_v, par_v, ldt_v, dsk_v, wr_v, w_v, wk_v, wt_v, col_v, wx_v, wy_v,
            tmp_v, idx_v, pk_v, h_v, st_v, acc_v, out_v, sd0, sd1, ta0, ta1, tb0, tb1, kl0, kl1,
            u0, u1, k0, k1, a0_v, a1_v, c0, c1, r0, r1, r2, r3, order_s,
            sem_p, sem_x, sem_w, sem_o, f0_v, f1_v, *rest):
    half_v, new_v = rest[:4], rest[4:]
    cp_vec = [pltpu.make_async_copy(s, d, sem_p.at[n]) for n, (s, d) in enumerate(
        ((ldt_hbm, ldt_v), (dsk_hbm, dsk_v), (wr_hbm, wr_v)))]
    cp_par = [[pltpu.make_async_copy(s.at[lo:hi], par_v.at[n, lo:hi], sem_p.at[3 + 6 * m + n])
               for n, s in enumerate((are_hbm, aim_hbm, bre_hbm, bim_hbm, cre_hbm, cim_hbm))]
              for m, (lo, hi) in enumerate(((0, 4 * MB), (4 * MB, D)))]
    cp_x = [pltpu.make_async_copy(x_hbm.at[:, 128 * j:128 * j + 128], x_v.at[j, 0:D],
                                  sem_x.at[j])
            for j in range(NT)]
    cp_d = pltpu.make_async_copy(wd_hbm, wd_v, sem_w.at[2])

    def cp_w(i):
        return [pltpu.make_async_copy(s.at[:, _ds(128 * i, 128)], d.at[i, 0:D], sem_w.at[n])
                for n, (s, d) in enumerate(((wg_hbm, wg_v), (wu_hbm, wu_v)))]

    for cp in cp_vec + cp_par[0]:
        cp.start()
    for cp in cp_x[:NT // 2]:
        cp.start(priority=1)

    def columns():
        for cp in cp_vec:
            cp.wait()
        for cp in cp_x[NT // 2:]:
            cp.start(priority=1)
        _transpose_dft(wt_v, w_v, range(4))
        _init_columns(col_v, wx_v, wy_v, ldt_v, dsk_v, wr_v)

    _init_dft(w_v, wk_v, tmp_v, columns)
    for cp in cp_par[0]:
        cp.wait()

    sd, ta, tb, kl = (sd0, sd1), (ta0, ta1), (tb0, tb1), (kl0, kl1)
    uk, ab, cc, xr = ((u0, u1), (k0, k1)), ((a0_v, a1_v), (f0_v, f1_v)), (c0, c1), (r0, r1, r2, r3)
    ww, wt_w = (w_v.bitcast(I32), wk_v.bitcast(I32)), wt_v

    def chan(b, r):
        return _ds(b * MB + 16 * r, 16)

    def seed_stage(b, r, sch):
        rows = _ds(b * MB // 2 + 8 * r, 8)
        par = [_split(par_v.bitcast(I32)[n, rows, :]) for n in range(6)]
        for h in range(2):
            a_re, a_im, b_re, b_im, c_re, c_im = [v[h] for v in par]
            dt = sch.start(col_v[0, _ds(b * MB + 16 * r + 8 * h, 8), :])
            mag, ang = jnp.exp(dt * a_re), dt * a_im
            sc = dt * (1.0 / L)
            seeds = _k_seeds((mag * jnp.cos(ang), mag * jnp.sin(ang)),
                             _cmul((c_re, c_im), (sc * b_re, sc * b_im)), sch)
            for g in range(2):
                for n, v in enumerate(seeds[g]):
                    for p in range(2):
                        sd[b % 2][r, 2 * h + g, 2 * n + p] = v[p]
            yield [sd[b % 2][(r + sch.zero), 2 * h, 0]]

    def table_stage(b, r, sch):
        tail = []
        for g in range(4):
            m1, m32, m512, a0, b0 = [
                (sd[b % 2][r, g, 2 * n], sd[b % 2][r, g, 2 * n + 1]) for n in range(5)]
            m32 = (sch.start(m32[0]), m32[1])
            fa = [a0]
            for _ in range(7):
                fa.append(_cmul(fa[-1], m1))
            for src in (0, 4, 8, 10):
                fa.append(_cmul(fa[src], m512))
            tail.append(fa[11][0] * m512[0] - fa[11][1] * m512[1])
            _store_table(ta[b % 2].at[r, g], fa)
            fb = [b0]
            for _ in range(15):
                p = fb[-1]
                fb.append((p[0] * m32[0] + p[1] * m32[1], p[1] * m32[0] - p[0] * m32[1]))
            _store_table(tb[b % 2].at[r, g], fb)
            yield [ta[b % 2].bitcast(I32)[(r + sch.zero), g, 0, 0:8, :],
                   tb[b % 2].bitcast(I32)[(r + sch.zero), g, 0, 0:8, :]]
        last = [jnp.where(sch.mask("odd"), pltpu.roll(tail[h + 1], 1, 0), tail[h])
                for h in (0, 2)]
        last = [pltpu.bitcast(_rbf(jnp.broadcast_to(jnp.sum(v, axis=1, keepdims=True),
                                                    (8, 128))), I32) for v in last]
        kl[b % 2][r] = jax.lax.shift_right_logical(last[0], 16) | last[1]

    def kernel_stage(b, r, sch):
        ta_w, tb_w = ta[b % 2].bitcast(I32), tb[b % 2].bitcast(I32)
        groups = [None] * 4
        for g0 in (0, 2):
            res = [jax.lax.dot_general(sch.lhs(ta_w[r, g, p, 0:48], g == g0 and p == 0),
                                       _mxu(tb_w[r, g, p, 0:64]), NT_DIMS, preferred_element_type=F32)
                   for g in (g0, g0 + 1) for p in range(2)]
            groups[g0], groups[g0 + 1] = res[0] + res[1], res[2] + res[3]
            sch.results(groups[g0 + 1])
            yield []
        dskip = [col_v[1, _ds(b * MB + 16 * r + 8 * h, 8), :] for h in range(2)]
        dst = _ds(8 * r, 8)
        res = _k_residues(groups, kl[b % 2][r], dskip, pk_v.at[sch.slot, 0], sch)
        for s, t in enumerate(res):
            uk[1][b % 2][4 * (s % 4) + s // 4, dst, :] = t
        yield [uk[1][b % 2][0, _ds(8 * (r + sch.zero), 8), :]]

    def norm_stage(b, r, sch):
        rows, dst = _ds(b * MB // 2 + 8 * r, 8), _ds(8 * r, 8)
        tiles = [x_v.bitcast(I32)[j, rows, :] for j in range(NT)]
        for s, t in enumerate(_to_residues([sch.start(tiles[0])] + tiles[1:], sch)):
            xr[b % 4][4 * (s % 4) + s // 4, dst, :] = t
            xs, m, inv = _mxu(t).astype(F32), st_v[s, 0], st_v[s, 1]
            uk[0][b % 2][4 * (s % 4) + s // 4, _ds(16 * r, 16), :] = jnp.concatenate(
                [(xs[0:8] - m) * inv, (xs[8:16] - m) * inv], axis=0).astype(BF16)
        yield [uk[0][b % 2].bitcast(I32)[0, _ds(8 * (r + sch.zero), 8), :]]

    def forward_stage(w, b, k, sch):
        dst = ab[w][b % len(ab[w])]
        for p in range(2):
            v = [jnp.dot(sch.lhs((uk[w][b % 2] if w else uk[w][b % 2].bitcast(I32))[
                4 * k + n, 0:MB // 2], n == 0),
                         _mxu(ww[w][p ^ (n & 1), 4 * k + n, 0:64]),
                         preferred_element_type=F32) for n in range(4)]
            d02, d13 = v[0] - v[2], v[1] - v[3]
            x1 = d02 - d13 if p == 0 else d02 + d13
            dst[0, k, p, 0:MB] = v[0] + v[2]
            dst[2, k, 1 - p, 0:MB] = v[1] + v[3]
            dst[1, k, p, 0:MB] = x1
            dst[3, k, p, 0:MB] = d02 + d13 if p == 0 else d02 - d13
            sch.results(x1)
            yield []

    def stats(tiles, sch):
        ones_w = wx_v.bitcast(I32)[...]
        for j in tiles:
            acc = None
            for i in range(0, D // 2, 8):
                v = [t * t for t in _split(x_v.bitcast(I32)[j, i:i + 8, :])]
                acc = v if acc is None else [p + q for p, q in zip(acc, v)]
            sums = jnp.dot(_mxu(jnp.concatenate(
                [ones_w[:, :128] if j % 2 == 0 else sch.tie(ones_w[:, :128], prev),
                 ones_w[:, 128:]], axis=1)),
                           _mxu(x_v.bitcast(I32)[j, 0:D // 2]), preferred_element_type=F32)
            s2 = prev = acc[0] + acc[1]
            for d in (4, 2, 1):
                s2 = s2 + pltpu.roll(s2, d, 0)
            st_v[j, 0], st_v[j, 1] = _ln_scalars(jnp.broadcast_to(sums[0:1], (8, 128)), s2)

    def middle_stage(b, r, sch):
        src = [v[b % len(v)] for v in ab]
        scale = lambda v, f: [(x[0] * f, x[1] * f) for x in v]
        for h in range(2):
            ra = _ds(16 * r + 8 * h, 8)
            ld = lambda q, w, ra=ra: [(src[w][q, k, 0, ra, :], src[w][q, k, 1, ra, :]) for k in range(4)]

            park_v = half_v[2 * (sch.slot % 2) + h]

            def put(q, y):
                x = [park_v[n + sch.zero] for n in range(8)]
                for k in range(4):
                    for p in range(2):
                        cc[b % 2][k, q, p, ra, :] = x[2 * k + p] + y[k][p]
                        cc[b % 2][k, q + 2, p, ra, :] = x[2 * k + p] - y[k][p]

            def park(x):
                for k in range(4):
                    for p in range(2):
                        park_v[2 * k + p] = x[k][p]
                return [park_v[sch.zero]]

            gate = sch.start
            a0, a2, b0, b2 = ld(0, 0), ld(2, 0), ld(0, 1), ld(2, 1)
            a0[0] = (gate(a0[0][0]), a0[0][1])
            e0 = _prod_mod_1(list(map(_cadd, a0, a2)), list(map(_cadd, b0, b2)))
            again = _ds(16 * (r + sch.zero) + 8 * h, 8)
            yield park(e0)
            a0, a2, b0, b2 = (ld(q, w, again) for w in range(2) for q in (0, 2))
            a2[0] = (gate(a2[0][0]), a2[0][1])
            e2 = _prod_mod_m1(list(map(_csub, a0, a2)), scale(map(_csub, b0, b2), 2.0))
            put(0, e2)
            yield [cc[b % 2][0, 0, 0, again, :]]
            four = sch.start(jnp.full((8, 128), 4.0, F32))
            e1 = _prod_mod_i(ld(1, 0), scale(ld(1, 1), four), 1)
            yield park(e1)
            four = sch.start(jnp.full((8, 128), 4.0, F32))
            e3 = _prod_mod_i(ld(3, 0), scale(ld(3, 1), four), -1)
            put(1, e3)
            yield [cc[b % 2][0, 1, 0, again, :]]

    def inverse_stage(b, k, sch):
        src = cc[b % 2]

        def lhs(v, n, first):
            return sch.lhs(jnp.concatenate(
                [_pack(pk_v.at[sch.slot, 2], 4 * n + i // 16, v[i:i + 8], v[i + 8:i + 16])
                 for i in range(0, MB, 16)], axis=0), first)

        for o in range(2):
            p0, p1 = [(src[k, q, 0, 0:MB], src[k, q, 1, 0:MB]) for q in (2 * o, 2 * o + 1)]
            if o == 0:
                e = {0: _cadd(p0, p1), 2: _csub(p0, p1)}
            else:
                e = {1: (p0[0] + p1[1], p0[1] - p1[0]), 3: (p0[0] - p1[1], p0[1] + p1[0])}
            ys = []
            for n in e:
                y = [jnp.dot(lhs(e[n][p], 2 * n + p, n == o and p == 0),
                             _mxu(wt_w[4 * k + (0, 2, 1, 3)[n], p, 0:64]),
                             preferred_element_type=F32)
                     for p in range(2)]
                h = y[0] + y[1] + _mxu(xr[b % 4][4 * k + n, 0:MB // 2]).astype(F32)
                h_v[k + 4 * n, b * MB:b * MB + MB, :] = h.astype(BF16)
                hh = h * h
                acc_v[0, k + 4 * n] += sum((hh[i:i + 8] for i in range(8, MB, 8)), hh[0:8])
                ys.append(h)
            sch.results(ys[-1])
            yield []

    def sum_stage(b, r, sch):
        for n in range(4):
            sums = jnp.dot(sch.lhs(wy_v.bitcast(I32)[b], n == 0)[:, :MB],
                           _mxu(h_v.bitcast(I32)[4 * r + n, b * MB // 2:(b + 1) * MB // 2]),
                           preferred_element_type=F32)
            acc_v[1, 4 * r + n] += sums[0:8]
        sch.results(sums)
        yield []

    nb = D // MB
    stages = dict(
        s=(seed_stage, 0), t=(table_stage, 1), k=(kernel_stage, 2),
        F=(functools.partial(forward_stage, 1), 3), n=(norm_stage, 2),
        f=(functools.partial(forward_stage, 0), 3), m=(middle_stage, 4),
        i=(inverse_stage, 5), a=(sum_stage, 6))

    def run(step, zero, live=None):
        live = live or {n: (f, step - lag) for n, (f, lag) in stages.items()
                        if 0 <= step - lag < nb and (n, step) != ("n", 2)}
        unroll, plan = PLANS["".join(live)]

        def body(it, carry):
            sch = _Schedule(zero >> (step % 32) if unroll == 4 else zero & it, idx_v)
            gens = [{n: f(b, it * unroll + u, sch) for n, (f, b) in live.items()}
                    for u in range(unroll)]
            if step == 3:
                for i in range(9 * unroll):
                    for cp in cp_w(9 * unroll * it + i):
                        cp.start()
            for item in plan.split():
                u, n, *ties = item.split(":")
                if n in live:
                    sch.slot = int(u)
                    sch.run(gens[int(u)][n], *map(int, ties or (-1, -1)))
            for sch.slot, g in enumerate(gens):
                for v in g.values():
                    for _ in v:
                        pass
            return carry + it

        if unroll == 4:
            return body(0, 0)
        return jax.lax.fori_loop(0, 4 // unroll, body, 0)

    _init_index(idx_v)
    acc_v[...] = jnp.zeros(acc_v.shape, F32)
    zero = run(0, 0) - 1
    for step in range(1, nb + 6):
        if step == 7:
            cp_d.start()
        if step == 4:
            for cp in cp_par[1]:
                cp.wait()
        if step == 3:
            for half in range(2):
                tiles = range(NT // 2 * half, NT // 2 * (half + 1))
                for j in tiles:
                    cp_x[j].wait()
                if not half:
                    for cp in cp_par[1]:
                        cp.start()
                _transpose_dft(wt_v, w_v, range(4 + 6 * half, 10 + 6 * half))
                stats(tiles, _Schedule(zero, idx_v))
            for q in range(2):
                for s, v in enumerate(_to_residues([st_v[j, q] for j in range(NT)],
                                                   _Schedule(zero, idx_v))):
                    st_v[s, q] = v
            run(101, zero, dict(n=(norm_stage, 0)))
        run(step, zero)

    sums = [acc_v[1, s] for s in range(16)]
    m2, inv2 = _ln_scalars(
        jnp.concatenate([v[0:1] for v in sums], axis=0),
        jnp.concatenate([jnp.sum(acc_v[0, j], axis=0, keepdims=True) for j in range(NT)], axis=0))
    wsum = jnp.sum(wr_v[...].astype(F32).reshape(1, D), axis=1, keepdims=True)
    score = _rbf((jnp.concatenate([v[1:2] for v in sums], axis=0) - m2 * wsum) * inv2 + 0.0)
    bits = pltpu.bitcast(score, I32) >> 16
    order = jnp.where(bits < 0, -1 - bits, bits + 32768)
    mu = (_iota((NT, 128), 1) - _iota((NT, 128), 0)) & 127
    pos = 128 * (mu & 15) + 16 * (mu >> 4) + _iota((NT, 128), 0)
    key = pltpu.bitcast((order << 11) + (L - 1 - pos) + (1 << 29), F32)

    h_w, out_w = h_v.bitcast(I32), out_v.bitcast(I32)
    sch, done = _Schedule(zero, idx_v), []
    tie = sch.tie

    def unrouted():
        for q, v in enumerate((1.0 + inv2, m2 * inv2)):
            for j, t in enumerate(_to_time(
                    [jnp.broadcast_to(v[s:s + 1], (8, 128)) for s in range(16)], sch)):
                st_v[j, q] = t
        for i in range(0, D, 16):
            scal = st_v.at[pl.ds(zero * (i + 1), NT)]
            tiles = [h_w[s, i // 2:i // 2 + 8, :] for s in range(16)]
            if len(done) > LAG:
                tiles[0] = tie(tiles[0], done[-LAG])
            for j, v in enumerate(_to_time(tiles, sch)):
                h, mul, sub = _mxu(v).astype(F32), scal[j, 0], scal[j, 1]
                out_v[j, i:i + 16, :] = jnp.concatenate(
                    [h[0:8] * mul - sub, h[8:16] * mul - sub], axis=0).astype(BF16)
                if j % 8 == 7:
                    yield pltpu.bitcast(out_w[j + zero, i // 2:i // 2 + 8, :], F32)

    side = unrouted()

    lane8, sub8 = _iota((CAP, 128), 1), _iota((CAP, 128), 0)
    best = _top8([pltpu.roll(key[i:i + 8], n, 1) if n else key[i:i + 8]
                  for i in (0, 8) for n in range(8)])
    cand = best[0]
    for c in range(1, CAP):
        cand = jnp.where(sub8 == c, best[c], cand)
    best = _top8([pltpu.roll(cand, n, 1) if n else cand for n in range(0, 128, 8)])
    for _ in range(2 * EARLY):
        best[-1] = tie(best[-1], next(side))
    best = [pltpu.bitcast(v, I32)[0, 0] for v in best]
    picks = [L - 1 - (v & (L - 1)) for v in best]

    def schedule(col):
        rnd = [sum([(col[e] == col[c]).astype(I32) for e in range(c)], 0) for c in range(CAP)]
        return (rnd, functools.reduce(jnp.maximum, rnd) + 1,
                lambda n: [lane8 == jnp.where(rnd[c] == n, col[c], -1) for c in range(CAP)])

    _, rounds, lanes = schedule([((t >> 7) + (t & 127)) & 127 for t in picks])

    def out_copy(q, lo, hi, n):
        j = order[q]
        return pltpu.make_async_copy(
            out_v.at[j, lo:hi], out_hbm.at[lo:hi, _ds(j * 128, 128)], sem_o.at[n])

    def gather(n, acc):
        masks = lanes(n)
        tiles = []
        for i in range(0, D // 2, 8):
            v = jnp.zeros((8, 128), I32)
            for c in range(CAP):
                v = jnp.where(masks[c], h_w[picks[c] & 15, i:i + 8, :], v)
            tiles.append(v)
        lhs = jnp.zeros((CAP, 128), F32)
        for c in range(CAP):
            lhs = jnp.where(masks[c] & (sub8 == c), 1.0, lhs)
        aux = [jnp.zeros((CAP, 128), F32)] * 3
        for c in range(CAP):
            hit = pltpu.bitcast(key, I32) == best[c]
            aux = [jnp.where(sub8 == c, jnp.sum(jnp.where(hit, v, 0.0), axis=0, keepdims=True), a)
                   for a, v in zip(aux, (m2, inv2, score))]
        return (acc[0] + jax.lax.dot_general(lhs.astype(BF16), _mxu(jnp.concatenate(tiles, axis=0)),
                                             NT_DIMS, preferred_element_type=F32),
                *[jnp.sum(a, axis=1, keepdims=True) for a in aux])

    h_sel, m_sel, inv_sel, score_sel = jax.lax.fori_loop(
        0, rounds, gather, (jnp.zeros((CAP, D), F32), *[jnp.zeros((CAP, 1), F32)] * 3))
    x_sel = _rbf((h_sel - m_sel) * inv_sel)
    gate = _rbf(jax.nn.sigmoid(score_sel))

    rate, sent = MID // 8 - 2 * EARLY, [0]

    def project(w_ref):
        parts = []
        for n in range(0, FF // 128, 4):
            for lo in range(0, D, 128):
                hi = min(lo + 128, D)
                xs = x_sel[:, lo:hi]
                if hi - lo == 128 and min(rate, (len(done) - 4) * rate // 70) > sent[0]:
                    sent[0] += 1
                    xs = tie(xs, next(side))
                w = [w_ref.bitcast(I32)[i, lo // 2:hi // 2, :] for i in range(n, n + 4)]
                v = jnp.dot(xs.astype(BF16), _mxu(jnp.concatenate(w, axis=1)),
                            preferred_element_type=F32)
                done.append(v[:, 0:128])
                acc = acc + v if lo else v
            parts.append(acc)
        return _rbf(jnp.concatenate(parts, axis=1))

    for n, ref in enumerate((wg_v, wu_v)):
        pltpu.make_async_copy(ref.at[:, 0:D], ref.at[:, 0:D], sem_w.at[n]).wait()
    g = project(wg_v)
    act = _rbf(g * jax.nn.sigmoid(g)) * project(wu_v)
    for _ in range(rate - sent[0]):
        next(side)
    done.clear()

    tile, col = [t >> 7 for t in picks], [t & 127 for t in picks]
    rnd, rounds, lanes = schedule(col)
    routed = functools.reduce(jnp.bitwise_or, [1 << j for j in tile])
    spare = CAP - sum((routed >> j) & 1 for j in range(NT))
    n_late = 0
    for j in range(NT):
        hit = (routed >> j) & 1
        fill = (1 - hit) & (spare > 0).astype(I32)
        spare = spare - fill
        order_s[jnp.clip(jnp.where(hit + fill == 1, CAP + n_late, j - n_late), 0, NT - 1)] = j
        n_late = n_late + hit + fill

    order = [order_s[q] for q in range(NT)]
    cp_d.wait()

    for q in range(CAP):
        out_copy(q, 0, MID, q).start()
    rest_side = list(side)

    def placed(r, words):
        idx = jnp.zeros((CAP, 128), I32)
        for c, m in enumerate(lanes(r)):
            idx = jnp.where(m, c, idx)
        return [_gather(w, idx) for w in words]

    def late_copies(n, lo, hi):
        return [out_copy(CAP + q, lo, hi, CAP * (n + 1) + q) for q in range(CAP)]

    def words_of(n):
        return [new_v[n].bitcast(I32)[i:i + 8, :] for i in range(0, new_v[n].shape[0] // 2, 8)]

    tokens = []
    for n, (lo, hi) in enumerate(ROW_CHUNKS):
        a = [act[:, i:i + 128] for i in range(0, FF, 128)]
        for i, token in enumerate(rest_side):
            at = 8 + i * SPAN // len(rest_side) - n * len(a)
            if 0 <= at < len(a):
                a[at] = tie(a[at], token)
        if n == 1:
            for q in range(CAP):
                out_copy(q, MID, D, NT * 3 + q).start()
        if n >= 2:
            cut = 12 * 128 // (hi - lo)
            a[cut] = tie(a[cut], tokens[n - 2])
        a = jnp.concatenate(a, axis=1)
        y = _rbf(jax.lax.dot_general(a.astype(BF16), wd_v[lo:hi, :], NT_DIMS,
                                     preferred_element_type=F32))
        new = h_sel[:, lo:hi] + _rbf(x_sel[:, lo:hi] + _rbf(y * gate))
        new_v[n][...] = jnp.concatenate(
            [new.T, jnp.zeros((hi - lo, 128 - CAP), F32)], axis=1).astype(BF16)
        rows = range(lo // 2, hi // 2, 8)
        words = words_of(n)
        both = list(zip(rows, placed(0, words), placed(1, words)))
        for c in range(CAP):
            for i, v0, v1 in both:
                pltpu.store(out_w.at[tile[c], pl.ds(i, 8), :],
                            jnp.where(rnd[c] == 0, v0, v1), mask=lane8 == col[c])
        for cp in late_copies(n, lo, hi):
            cp.start()
        out_w[tile[0], D // 2:, :] = lane8
        tokens.append(pltpu.bitcast(out_w[tile[0] | zero, D // 2:, :], F32))
    for q in range(CAP):
        out_copy(q, 0, MID, q).wait()
        out_copy(q, MID, D, NT * 3 + q).wait()
    for n, (lo, hi) in enumerate(ROW_CHUNKS):
        for cp in late_copies(n, lo, hi):
            cp.wait()

    @pl.when(rounds > 2)
    def _():
        def fix(r, carry):
            rows = range(0, D // 2, 8)
            vals = placed(r, sum(map(words_of, range(len(new_v))), []))
            for c, m in enumerate(lanes(r)):
                for i, v in zip(rows, vals):
                    pltpu.store(out_w.at[tile[c], pl.ds(i, 8), :], v, mask=m)
            return carry

        jax.lax.fori_loop(2, rounds, fix, 0)
        for cp in late_copies(0, 0, D):
            cp.start()
        for cp in late_copies(0, 0, D):
            cp.wait()


@jax.jit
def pallas_sequential_preLN__ssm_conv_s4__moe_arch_mod__prompt_kernel(
    A_u: jax.Array,
    A_A_re: jax.Array,
    A_A_im: jax.Array,
    A_B_re: jax.Array,
    A_B_im: jax.Array,
    A_C_re: jax.Array,
    A_C_im: jax.Array,
    A_log_dt: jax.Array,
    A_Dskip: jax.Array,
    B_x: jax.Array,
    B_w_r: jax.Array,
    B_w_gate: jax.Array,
    B_w_up: jax.Array,
    B_w_down: jax.Array,
):
    del B_x
    hbm = pl.BlockSpec(memory_space=pl.ANY)
    out = pl.pallas_call(
        _kernel,
        out_shape=jax.ShapeDtypeStruct((D, L), BF16),
        in_specs=[hbm] * 13,
        out_specs=hbm,
        scratch_shapes=[
            pltpu.VMEM((NT, D + 16, 128), BF16),
            *[pltpu.VMEM((FF // 128, D + 16, 128), BF16)] * 2,
            pltpu.VMEM((D, FF), BF16),
            pltpu.VMEM((6, D, N), BF16),
            *[pltpu.VMEM((D,), BF16)] * 3,
            *[pltpu.VMEM((2, 16, 144, 128), BF16)] * 2,
            pltpu.VMEM((16, 2, 72, 128), I32),
            pltpu.VMEM((2, D, 128), F32),
            pltpu.VMEM((16, D), BF16),
            pltpu.VMEM((D // MB, 16, 128), BF16),
            pltpu.VMEM((2, 256, 128), F32),
            pltpu.VMEM((len(INDEX), 8, 128), I32),
            pltpu.VMEM((4, 3, 32, 16, 128), BF16),
            pltpu.VMEM((NT, D + 16, 128), BF16),
            pltpu.VMEM((NT, 2, 8, 128), F32),
            pltpu.VMEM((2, NT, 8, 128), F32),
            pltpu.VMEM((NT, D + 16, 128), BF16),
            *[pltpu.VMEM((4, 4, 10, 8, 128), F32)] * 2,
            *[pltpu.VMEM((4, 4, 2, 112, 128), BF16)] * 2,
            *[pltpu.VMEM((4, 4, 2, 144, 128), BF16)] * 2,
            *[pltpu.VMEM((4, 8, 128), I32)] * 2,
            *[pltpu.VMEM((16, MB + 16, 128), BF16)] * 2,
            *[pltpu.VMEM((16, MB // 2 + 8, 128), I32)] * 2,
            *[pltpu.VMEM((4, 4, 2, MB + 8, 128), F32)] * 2,
            *[pltpu.VMEM((4, 4, 2, MB + 8, 128), F32)] * 2,
            *[pltpu.VMEM((16, MB // 2 + 8, 128), I32)] * 4,
            pltpu.SMEM((NT,), I32),
            pltpu.SemaphoreType.DMA((15,)),
            pltpu.SemaphoreType.DMA((NT,)),
            pltpu.SemaphoreType.DMA((3,)),
            pltpu.SemaphoreType.DMA((CAP * (2 + len(ROW_CHUNKS)),)),
            *[pltpu.VMEM((4, 4, 2, MB + 8, 128), F32)] * 2,
            *[pltpu.VMEM((8, 8, 128), F32)] * 4,
            *[pltpu.VMEM((hi - lo, 128), BF16) for lo, hi in ROW_CHUNKS],
        ],
        compiler_params=pltpu.CompilerParams(vmem_limit_bytes=100 * 1024 * 1024,
                                             disable_bounds_checks=True,
                                             disable_semaphore_checks=True),
    )(A_u.reshape(L, D).T, A_A_re, A_A_im, A_B_re, A_B_im, A_C_re, A_C_im,
      A_log_dt, A_Dskip, B_w_r, B_w_gate, B_w_up, B_w_down.T)
    return out.T.reshape(1, L, D)
```

```python
import functools

import numpy as np
import jax
import jax.numpy as jnp
import jax.experimental.pallas as pl
import jax.experimental.pallas.tpu as pltpu

F32 = jnp.float32
BF16 = jnp.bfloat16
I32 = jnp.int32

L = 2048
D = 576
N = 128
FF = 4608
CAP = 8
NT = L // 128
EPS = 1e-5
MB = 64
PLANS = dict(
    s=(2, ""),
    st=(2, ""),
    n=(4, ""),
    stk=(2, "0:t:-1:4 1:t:-1:3 0:t:-1:4 0:t:-1:7 0:t:-1:15 1:t:-1:10 1:t:6:16 1:t:11:21 0:k "
            "0:k 1:k 0:s:-1:20 0:s:11:23 0:k:-1:23 1:k 1:s:20:-1 1:s 1:k "),
    stkFnf=(2, "1:t:-1:4 0:s:-1:16 0:s:-1:34 1:s:-1:36 1:s:-1:54 0:f 0:n:1:16 0:F 0:t:4:25 "
               "0:t:0:21 0:k 0:k 0:k:-1:35 0:t:17:36 0:F 0:f 1:f 1:t:29:43 1:F 1:n:33:47 1:k "
               "1:t:39:55 1:k 1:t:42:53 1:k 0:t:44:53 1:F 1:f "),
    stkFnfm=(1, "0:m:-1:2 0:m:-1:5 0:t:-1:7 0:t:-1:14 0:t:-1:9 0:f 0:m:1:14 0:m:-1:18 0:f "
                "0:m:7:21 0:m:6:20 0:k 0:t:9:22 0:n:9:27 0:k 0:s:16:-1 0:m:15:-1 0:m:13:25 0:k "
                "0:s:19:-1 0:F 0:F "),
    stkFnfmi=(4, "0:t:-1:3 0:n:-1:8 0:t:-1:3 0:m:-1:7 0:m:-1:6 0:m:-1:19 0:s:-1:40 1:s:-1:76 "
                 "2:s:-1:112 3:s 0:f 0:m:0:11 0:k 0:s:4:33 0:k 0:m:13:23 0:k:-1:33 0:m:14:25 "
                 "0:t:14:32 0:f 0:t:18:33 0:F 1:t:23:41 0:F 1:t:24:38 1:m:27:44 0:i 1:n:29:47 "
                 "1:m:29:47 0:i 0:m:32:40 0:m:31:42 1:f 1:m:39:57 1:m:36:49 1:k 1:s:40:71 1:k "
                 "1:m:49:61 1:k:-1:71 1:m:51:63 1:f 1:t:55:76 1:t:51:68 1:F 2:t:59:75 1:F "
                 "2:t:62:78 2:m:63:79 2:m:63:79 1:i 2:n:64:80 1:i 1:m:68:76 1:m:67:76 2:f "
                 "2:m:75:91 2:m:72:83 2:k 2:s:76:105 2:k 2:m:85:95 2:k:-1:105 2:m:86:97 "
                 "2:t:86:105 2:f 2:t:90:105 2:F 3:t:95:113 2:F 3:t:96:110 3:m:99:116 2:i "
                 "3:n:101:119 3:m:101:119 2:i 2:m:104:112 2:m:106:117 3:f 3:m:111:129 "
                 "3:m:108:121 3:k 3:s:112:143 3:k 3:m:121:133 3:k:-1:142 3:m:123:135 3:f "
                 "3:t:127:-1 3:t:123:140 3:F 3:F 3:i 3:i 3:m:140:-1 3:m:139:-1 "),
    stkFnfmia=(4, "0:t:-1:6 0:t:-1:2 0:n:-1:9 0:m:-1:6 0:m:-1:8 0:m:-1:19 0:s:-1:40 1:s:-1:77 "
                  "2:s:-1:114 3:s 0:a 0:f 0:m:1:18 0:k 0:s:5:40 0:k 0:m:15:27 0:m:-1:29 "
                  "0:k:-1:40 0:t:16:30 0:f 0:t:18:34 0:F 0:F 1:t:25:43 1:t:23:41 1:n:28:46 "
                  "1:m:25:43 1:m:27:45 0:i 0:m:32:40 0:i 0:m:34:42 1:a 1:f 1:m:38:56 1:m:36:55 "
                  "1:k 1:s:42:77 1:k 1:m:52:64 1:m:48:66 1:k:-1:77 1:t:53:67 1:f 1:t:55:71 1:F "
                  "1:F 2:t:64:80 2:t:60:78 2:n:65:83 2:m:62:80 2:m:64:82 1:i 1:m:69:77 1:i "
                  "1:m:71:81 2:m:73:93 2:a 2:f 2:m:75:92 2:k 2:s:79:114 2:k 2:m:89:101 "
                  "2:m:85:103 2:k:-1:114 2:t:90:104 2:f 2:t:92:108 2:F 2:F 3:t:99:117 "
                  "3:t:97:115 3:n:102:120 3:m:99:117 3:m:101:119 2:i 2:m:106:114 2:i "
                  "2:m:108:116 3:a 3:f 3:m:112:130 3:m:112:129 3:k 3:s:116:-1 3:k 3:m:126:138 "
                  "3:m:122:140 3:k 3:t:127:141 3:f 3:t:129:-1 3:F 3:F 3:i 3:m:143:-1 3:i "
                  "3:m:145:-1 "),
    tkFnfmia=(4, "0:t:-1:10 0:t:-1:5 0:n:-1:9 0:m:-1:6 0:m:-1:9 0:a 0:f 0:k 0:m:7:18 0:m:1:23 "
                 "0:k 0:m:15:28 0:m:-1:27 0:k:-1:36 0:f 0:t:17:34 0:t:20:38 0:F 0:F 1:m:27:43 "
                 "0:i 0:m:31:39 1:t:31:47 1:t:26:42 1:n:30:46 1:m:30:46 0:i 0:m:34:42 1:a 1:f "
                 "1:k 1:m:44:55 1:m:38:58 1:k 1:m:52:65 1:m:48:64 1:k:-1:73 1:f 1:t:54:71 "
                 "1:t:57:75 1:F 1:F 2:m:64:80 1:i 1:m:68:76 2:t:68:84 2:t:64:80 2:n:67:83 "
                 "2:m:67:83 1:i 1:m:71:79 2:a 2:f 2:k 2:m:81:92 2:m:75:97 2:k 2:m:89:102 "
                 "2:m:85:101 2:t:90:108 2:k:-1:110 2:f 2:t:94:112 2:F 2:F 3:m:101:117 2:i "
                 "2:m:106:114 3:t:105:121 3:t:100:116 3:n:104:120 3:m:104:120 2:i 2:m:108:116 "
                 "3:a 3:f 3:k 3:m:118:129 3:m:109:131 3:k 3:m:126:139 3:m:122:138 3:k:-1:147 "
                 "3:f 3:t:128:145 3:t:131:-1 3:F 3:F 3:i 3:m:143:-1 3:i 3:m:145:-1 "),
    kFnfmia=(4, "1:m:-1:5 1:m:-1:3 0:n:-1:12 0:F 0:m:2:14 0:m:-1:15 0:a 0:F 0:m:7:21 0:k "
                "0:m:9:27 0:m:13:23 0:k 0:m:15:25 0:m:18:31 0:m:20:32 0:k:-1:45 0:i 0:i 0:f "
                "0:f 1:n:36:50 1:F 1:a 1:F 1:m:42:57 1:m:34:56 1:k 1:m:47:64 1:k 1:m:53:66 "
                "1:k:-1:75 1:i 1:i 3:m:63:79 3:m:61:77 1:f 1:m:68:76 1:f 1:m:73:81 2:n:70:86 "
                "2:F 2:m:76:88 2:m:73:89 2:a 2:F 2:m:79:93 2:k 2:m:83:101 2:m:87:97 2:k "
                "2:m:89:101 2:m:92:105 2:m:90:106 2:k:-1:119 2:i 2:i 2:f 2:f 3:n:110:124 3:F "
                "3:a 3:F 3:m:116:130 3:m:111:134 3:k 3:m:121:141 3:m:124:141 3:k 3:k 3:i 3:i "
                "3:f 3:m:142:-1 3:f 3:m:145:-1 "),
    Ffmia=(4, "1:m:-1:9 0:m:-1:5 0:m:-1:10 0:m:-1:12 0:a 0:F 1:m:4:15 0:i 0:m:6:18 0:i "
              "0:m:9:22 0:F 1:m:16:31 0:f 0:m:20:33 0:f 0:m:22:33 1:a 1:m:25:43 1:F 0:m:29:41 "
              "1:i 1:i 1:m:35:48 1:F 1:m:40:54 1:f 1:m:42:57 1:m:45:56 3:m:45:59 2:m:42:58 1:f "
              "2:a 2:F 2:m:53:63 2:m:49:65 3:m:54:68 2:i 2:m:56:67 2:i 2:m:59:75 2:F 3:m:66:83 "
              "2:f 2:m:70:83 2:f 2:m:72:84 3:a 3:m:75:93 3:F 2:m:79:96 3:i 3:i 3:m:85:-1 3:F "
              "3:m:90:-1 3:f 3:m:92:-1 3:m:95:-1 3:f "),
    mia=(4, "1:m:-1:3 0:m:-1:8 0:m:-1:6 0:m:-1:7 0:m:-1:8 0:i 1:m:0:13 0:m:2:10 0:a 0:i "
            "1:m:5:16 2:m:8:25 1:i 1:m:9:22 0:m:10:23 0:m:8:20 1:m:8:20 3:m:11:25 1:a "
            "2:m:13:27 1:i 1:m:14:22 1:m:17:25 0:m:14:22 1:m:17:25 2:m:14:28 2:m:13:27 2:i "
            "3:m:18:32 2:m:20:32 2:a 2:i 3:m:23:-1 3:m:25:-1 3:m:25:-1 3:i 2:m:28:-1 2:m:27:-1 "
            "3:a 3:i 3:m:32:-1 3:m:35:-1 2:m:33:-1 3:m:35:-1 "),
    ia=(4, "0:a 0:i 0:i 1:a 1:i 1:i 2:a 2:i 2:i 3:a 3:i 3:i"),
    a=(4, "0:a 1:a 2:a 3:a"),
)
ROW_CHUNKS = ((0, 128), (128, 256), (256, 384), (384, 512), (512, D))
LAG = 16
MID, SPAN, EARLY = 384, 50, 8
NT_DIMS = (((1,), (1,)), ((), ()))


def _round_res(step):
    return [int(np.round(r / step)) * step for r in range(16)]


RES1, RES2, RES3 = _round_res(2), _round_res(4), _round_res(8)


def _ds(start, size):
    return pl.ds(start if isinstance(start, int) else pl.multiple_of(start, size), size)


def _iota(shape, dim):
    return jax.lax.broadcasted_iota(I32, shape, dim)


def _rbf(x):
    return x.astype(BF16).astype(F32)


def _cmul(a, b):
    return (a[0] * b[0] - a[1] * b[1], a[0] * b[1] + a[1] * b[0])


def _csq(a):
    t = a[0] * a[1]
    return ((a[0] + a[1]) * (a[0] - a[1]), t + t)


def _cadd(a, b):
    return (a[0] + b[0], a[1] + b[1])


def _csub(a, b):
    return (a[0] - b[0], a[1] - b[1])


def _bfly4(a0, a1, a2, a3, inverse=False):
    s02, d02 = _cadd(a0, a2), _csub(a0, a2)
    s13, d13 = _cadd(a1, a3), _csub(a1, a3)
    p = (d02[0] - d13[1], d02[1] + d13[0])
    m = (d02[0] + d13[1], d02[1] - d13[0])
    if inverse:
        p, m = m, p
    return _cadd(s02, s13), p, _csub(s02, s13), m


def _prod_mod_1(a, b):
    fa, fb = _bfly4(*a), _bfly4(*b)
    return _bfly4(*[_cmul(x, y) for x, y in zip(fa, fb)], inverse=True)


def _prod2(a0, a1, b0, b1, sgn):
    p00, p11 = _cmul(a0, b0), _cmul(a1, b1)
    c1 = _cadd(_cmul(a0, b1), _cmul(a1, b0))
    if sgn > 0:
        return (p00[0] - p11[1], p00[1] + p11[0]), c1
    return (p00[0] + p11[1], p00[1] - p11[0]), c1


def _prod_mod_m1(a, b):
    def split(x):
        p = [(x[k][0] - x[k + 2][1], x[k][1] + x[k + 2][0]) for k in range(2)]
        m = [(x[k][0] + x[k + 2][1], x[k][1] - x[k + 2][0]) for k in range(2)]
        return p, m
    ap, am = split(a)
    bp, bm = split(b)
    cp = _prod2(*ap, *bp, 1)
    cm = _prod2(*am, *bm, -1)
    lo = [_cadd(cp[k], cm[k]) for k in range(2)]
    hi = [(cp[k][1] - cm[k][1], cm[k][0] - cp[k][0]) for k in range(2)]
    return lo + hi


def _prod_mod_i(a, b, sgn):
    sm = [x[0] + x[1] for x in b]
    df = [x[1] - x[0] for x in b]
    asum = [x[0] + x[1] for x in a]
    out = []
    for k in range(4):
        acc = [None, None, None]
        for j in range(4):
            m = (k - j) % 4
            if j <= k:
                t = ((b[m][0], 1), (df[m], 1), (sm[m], 1))
            elif sgn > 0:
                t = ((b[m][1], -1), (sm[m], 1), (df[m], -1))
            else:
                t = ((b[m][1], 1), (sm[m], -1), (df[m], 1))
            for q, (v, (w, s)) in enumerate(zip((asum[j], a[j][0], a[j][1]), t)):
                p = v * w
                if acc[q] is None:
                    acc[q] = p
                else:
                    acc[q] = acc[q] + p if s > 0 else acc[q] - p
        out.append((acc[0] - acc[2], acc[0] + acc[1]))
    return out


def _barrel(v, sch):
    for bit in range(4):
        m = sch.mask("bit%d" % bit)
        v = [jnp.where(m, v[(i + (1 << bit)) % 16], v[i]) for i in range(16)]
    return [v[-s % 16] for s in range(16)]


def _to_residues(tiles, sch):
    return _barrel([t if j == 0 else pltpu.roll(t, j, 1) for j, t in enumerate(tiles)], sch)


def _to_time(res, sch):
    return [t if j == 0 else pltpu.roll(t, 128 - j, 1)
            for j, t in enumerate(_barrel(res, sch))]


def _gather(x, idx, axis=1):
    return jnp.take_along_axis(x, idx, axis=axis, mode="promise_in_bounds")


def _transpose_dft(wt_ref, wu_ref, residues):
    for s in residues:
        for p in range(2):
            wt_ref[4 * (s % 4) + (0, 2, 1, 3)[s // 4], p, 0:64] = pltpu.bitcast(
                _mxu(wu_ref.bitcast(I32)[p, 4 * (s % 4) + s // 4, 0:64]).T, I32)


def _init_dft(wu_ref, wk_ref, tmp_ref, halfway):
    sub, k4 = _iota((8, 128), 0), 4 * _iota((8, 128), 1) + 1

    def cis(t):
        ph = ((k4 * t) & (4 * L - 1)).astype(F32) * (2 * np.pi / (4 * L))
        return jnp.cos(ph), jnp.sin(ph)

    w1, w16 = cis(1), cis(16)
    w32 = _csq(w16)
    fk = [cis(16 * (32 * (sub & 3) + (sub >> 2)))]
    fu = [cis(128 * sub), cis(128 * (sub + 8))]
    for v in range(1, 16):
        fk.append(_cmul(fk[-1], w32))
        if v >= 2:
            fu.append(_cmul(fu[-2], w16))
    for p in range(2):
        for v in range(32):
            tmp_ref[p, 8 * v:8 * v + 8, :] = fu[v % 16][p]
    tw = None
    for s in range(16):
        for v in range(0, 16, 2):
            rows = [slice(128 - s + 8 * i, 136 - s + 8 * i) for i in (v, v + 1)]
            for ref, f in ((wk_ref, fk[v:v + 2]),
                           (wu_ref, [(tmp_ref[0, r, :], tmp_ref[1, r, :]) for r in rows])):
                if s:
                    f = [_cmul(x, tw) for x in f]
                for p in range(2):
                    ref[p, 4 * (s % 4) + s // 4, 8 * v:8 * v + 16, :] = jnp.concatenate(
                        [f[0][p], f[1][p]], axis=0).astype(BF16)
        tw = _cmul(tw, w1) if s else w1
        if s == 7:
            halfway()


def _pack(ref, n, a, b):
    ref[n] = jnp.concatenate([a, b], axis=0).astype(BF16)
    return ref.bitcast(I32)[n]


def _split(w):
    return [pltpu.bitcast(w << 16, F32), pltpu.bitcast(w & -65536, F32)]


FINE = (0, 1, 2, 3, 4, 5, 6, 7, 512, 516, 1024, 1536)


def _k_seeds(z, c, sch):
    pw = {1: z}
    for e in range(1, 10):
        pw[1 << e] = _csq(pw[1 << (e - 1)])
    c8, z16 = _cmul(c, pw[8]), (pw[16][0], 0.0 - pw[16][1])
    pair = lambda a, b: tuple(jnp.where(sch.mask("odd"), q, p) for p, q in zip(a, b))
    seeds = []
    for g in range(2):
        twice = lambda v: tuple(_gather(x, sch.idx("dup%d" % g), 0) for x in v)
        seeds.append([twice(z), twice(pw[32]), twice(pw[512]),
                      pair(twice(c), twice(c8)), pair((1.0, 0.0), twice(z16))])
    return seeds


def _mxu(words):
    return pltpu.bitcast(words, BF16)


def _store_table(ref, tab):
    for i in range(0, len(tab), 2):
        for p in range(2):
            ref[p, 8 * i:8 * i + 16, :] = jnp.concatenate(
                [tab[i][p], tab[i + 1][p]], axis=0).astype(BF16)


def _k_residues(groups, k_last, dskip, tmp_ref, sch):
    idx, nxt = sch.idx("src"), sch.idx("nxt")
    low = lambda x, y: (x & 65535) | (y << 16)
    high = lambda x, y: jax.lax.shift_right_logical(x, 16) | (y & -65536)
    kv, up = {}, {}
    for i, k in enumerate(FINE):
        v = [g[8 * i:8 * i + 8] for g in groups]
        if k == 0:
            v = [x + jnp.where(sch.mask("diag"),
                               _gather(dskip[n // 2], sch.idx("dup%d" % (n % 2)), 0), 0.0)
                 for n, x in enumerate(v)]
        p = [_pack(tmp_ref, 2 * i + h, v[2 * h], v[2 * h + 1]) for h in range(2)]
        both = [_gather(x, idx) for x in p]
        kv[k], kv[k + 8] = low(*both), high(*both)
        if k % 512 == 0:
            up[k] = low(*[_gather(x, nxt) for x in p])
    k_last = _gather(k_last, sch.idx("rows"), 0)
    q0, q1, q2, up0, up01, up2, up3, fine = map(sch.mask, INDEX[-8:])
    s3 = {r: jnp.where(q2, kv[1024 + r], kv[1536 + r]) for r in (0, 8)}
    v0 = jnp.where(q0, kv[0], jnp.where(q1, kv[512], s3[0]))
    v16 = jnp.where(up01, jnp.where(up0, up[0], up[512]),
                    jnp.where(up2, up[1024], jnp.where(up3, up[1536], k_last)))
    s3[16] = v16
    s23, s123, out = {}, {}, [v0]
    for r in range(1, 16):
        k23 = (RES2[r], RES3[r])
        if k23 not in s23:
            s23[k23] = v16 if k23 == (16, 16) else jnp.where(q1, kv[512 + k23[0]], s3[k23[1]])
        k123 = (RES1[r],) + k23
        if k123 not in s123:
            s123[k123] = v16 if k123[0] == 16 else jnp.where(q0, kv[k123[0]], s23[k23])
        if RES1[r] == r:
            out.append(s123[k123])
        else:
            out.append(jnp.where(fine, kv[r], s123[k123]))
    return out


def _ln_scalars(s1, s2):
    mean = s1 * (1.0 / D)
    var = jnp.maximum(s2 * (1.0 / D) - mean * mean, 0.0)
    eps = float(np.asarray(EPS, dtype=BF16))
    sd = _rbf(jnp.sqrt(_rbf(_rbf(var) + eps)))
    return _rbf(mean), 1.0 / sd


def _top8(x):
    def swap(v, pairs):
        for i, j in pairs:
            v[i], v[j] = jnp.maximum(v[i], v[j]), jnp.minimum(v[i], v[j])
        return v

    def merge(a, b):
        v = [jnp.maximum(a[i], b[7 - i]) for i in range(8)]
        return swap(v, [(i, i + d) for d in (4, 2, 1) for i in range(8) if not i & d])

    sort8 = ((0, 2), (1, 3), (4, 6), (5, 7), (0, 4), (1, 5), (2, 6), (3, 7), (0, 1), (2, 3),
             (4, 5), (6, 7), (2, 4), (3, 5), (1, 4), (3, 6), (1, 2), (3, 4), (5, 6))
    v = merge(*[swap(x[i:i + 8], sort8) for i in (0, 8)])
    for d in (4, 2, 1):
        v = merge(v, [pltpu.roll(t, d, 0) for t in v])
    return v


def _init_columns(col_ref, wx_ref, wy_ref, ldt_ref, dsk_ref, wr_ref):
    row, lane = _iota((128, 128), 0), _iota((128, 128), 1)
    split = (row & ~15) + 2 * (row & 7) + ((row >> 3) & 1)
    ldt, dsk, wr = (ref[...].astype(F32).reshape(1, D) for ref in (ldt_ref, dsk_ref, wr_ref))
    for n, vec in enumerate((jnp.exp(ldt), dsk * (1.0 / L))):
        for lo in range(0, D, 128):
            i = min(lo, D - 128)
            diag = jnp.where(split == lane, vec[:, i:i + 128], 0.0)[lo - i:].astype(BF16)
            col_ref[n, lo:i + 128, :] = jnp.dot(diag, jnp.ones((128, 128), BF16),
                                                preferred_element_type=F32)
    sub = _iota((16, D), 0)
    ones_w = jnp.where(sub == 0, 1.0, jnp.where(sub == 1, wr, 0.0))
    wx_ref[...] = ones_w.astype(BF16)
    for lo in range(0, D, MB):
        wy_ref[lo // MB, :, 0:MB] = ones_w[:, lo:lo + MB].astype(BF16)
        wy_ref[lo // MB, :, MB:] = jnp.zeros((16, 128 - MB), BF16)


INDEX = ("true", "bit0", "bit1", "bit2", "bit3", "odd", "dup0", "dup1", "rows", "src", "nxt",
         "diag", "q0", "q1", "q2", "up0", "up01", "up2", "up3", "fine")


def _init_index(idx_ref):
    sub, lane = _iota((8, 128), 0), _iota((8, 128), 1)
    src = lambda b: 8 * ((b >> 1) & 15) + 2 * (sub & 3) + (b & 1)
    is_ = lambda m: jnp.where(m, 1, 0)
    q = lane & 3
    q16 = q + is_(lane >= 124)
    tiles = dict(true=sub + 1, odd=sub & 1, dup0=sub >> 1, dup1=4 + (sub >> 1),
                 rows=2 * (sub & 3) + (sub >> 2), src=src(lane >> 2), nxt=src((lane >> 2) + 1),
                 diag=is_((lane == sub) & ((sub & 1) == 0)), up01=is_(q16 < 2),
                 fine=is_((q == 0) & (lane < 64)),
                 **{"bit%d" % n: (lane >> n) & 1 for n in range(4)},
                 **{"q%d" % n: is_(q == n) for n in range(3)},
                 **{"up%d" % n: is_(q16 == n) for n in (0, 2, 3)})
    for n, name in enumerate(INDEX):
        idx_ref[n] = tiles[name]


class _Schedule:
    def __init__(self, zero, idx_ref):
        self.zero = zero
        self.idx = lambda name: idx_ref[INDEX.index(name) + zero]
        self.mask = lambda name: self.idx(name) != 0
        self.true = self.mask("true")
        self.done, self.pending, self.wait = [], {}, -1

    def tie(self, x, token):
        return jnp.where(self.true, x, token if token.dtype == x.dtype
                         else pltpu.bitcast(token, x.dtype))

    def start(self, x):
        return self.tie(x, self.done[self.wait]) if 0 <= self.wait < len(self.done) else x

    def lhs(self, words, first):
        tiles = [words[i:i + 8] for i in range(0, words.shape[0], 8)]
        for i in range(len(tiles) if first else 0):
            for token in self.pending.pop(len(self.done) + i, ()):
                tiles[i] = self.tie(tiles[i], token)
        return _mxu(jnp.concatenate(tiles, axis=0))

    def results(self, v):
        self.done += [v[i + 8:i + 16] for i in range(0, v.shape[0], 16)]

    def run(self, stage, wait, before):
        self.wait = wait
        self.pending.setdefault(before, []).extend(next(stage))


def _kernel(x_hbm, are_hbm, aim_hbm, bre_hbm, bim_hbm, cre_hbm, cim_hbm,
            ldt_hbm, dsk_hbm, wr_hbm, wg_hbm, wu_hbm, wd_hbm, out_hbm,
            x_v, wg_v, wu_v, wd_v, par_v, ldt_v, dsk_v, wr_v, w_v, wk_v, wt_v, col_v, wx_v, wy_v,
            tmp_v, idx_v, pk_v, h_v, st_v, acc_v, sq_v, out_v, sd0, sd1, ta0, ta1, tb0, tb1, kl0, kl1,
            u0, u1, k0, k1, a0_v, a1_v, c0, c1, r0, r1, r2, r3, order_s,
            sem_p, sem_x, sem_w, sem_o, f0_v, f1_v, *rest):
    half_v, new_v = rest[:4], rest[4:]
    cp_vec = [pltpu.make_async_copy(s, d, sem_p.at[n]) for n, (s, d) in enumerate(
        ((ldt_hbm, ldt_v), (dsk_hbm, dsk_v), (wr_hbm, wr_v)))]
    cp_par = [[pltpu.make_async_copy(s.at[lo:hi], par_v.at[n, lo:hi], sem_p.at[3 + 6 * m + n])
               for n, s in enumerate((are_hbm, aim_hbm, bre_hbm, bim_hbm, cre_hbm, cim_hbm))]
              for m, (lo, hi) in enumerate(((0, 4 * MB), (4 * MB, D)))]
    cp_x = [pltpu.make_async_copy(x_hbm.at[:, 128 * j:128 * j + 128], x_v.at[j, 0:D],
                                  sem_x.at[j])
            for j in range(NT)]
    cp_d = pltpu.make_async_copy(wd_hbm, wd_v, sem_w.at[2])

    def cp_w(i):
        return [pltpu.make_async_copy(s.at[:, _ds(128 * i, 128)], d.at[i, 0:D], sem_w.at[n])
                for n, (s, d) in enumerate(((wg_hbm, wg_v), (wu_hbm, wu_v)))]

    for cp in cp_vec + cp_par[0]:
        cp.start()
    for cp in cp_x[:NT // 2]:
        cp.start(priority=1)

    def columns():
        for cp in cp_vec:
            cp.wait()
        for cp in cp_x[NT // 2:]:
            cp.start(priority=1)
        _transpose_dft(wt_v, w_v, range(4))
        _init_columns(col_v, wx_v, wy_v, ldt_v, dsk_v, wr_v)

    _init_dft(w_v, wk_v, tmp_v, columns)
    for cp in cp_par[0]:
        cp.wait()

    sd, ta, tb, kl = (sd0, sd1), (ta0, ta1), (tb0, tb1), (kl0, kl1)
    uk, ab, cc, xr = ((u0, u1), (k0, k1)), ((a0_v, a1_v), (f0_v, f1_v)), (c0, c1), (r0, r1, r2, r3)
    ww, wt_w = (w_v.bitcast(I32), wk_v.bitcast(I32)), wt_v

    def chan(b, r):
        return _ds(b * MB + 16 * r, 16)

    def seed_stage(b, r, sch):
        rows = _ds(b * MB // 2 + 8 * r, 8)
        par = [_split(par_v.bitcast(I32)[n, rows, :]) for n in range(6)]
        for h in range(2):
            a_re, a_im, b_re, b_im, c_re, c_im = [v[h] for v in par]
            dt = sch.start(col_v[0, _ds(b * MB + 16 * r + 8 * h, 8), :])
            mag, ang = jnp.exp(dt * a_re), dt * a_im
            sc = dt * (1.0 / L)
            seeds = _k_seeds((mag * jnp.cos(ang), mag * jnp.sin(ang)),
                             _cmul((c_re, c_im), (sc * b_re, sc * b_im)), sch)
            for g in range(2):
                for n, v in enumerate(seeds[g]):
                    for p in range(2):
                        sd[b % 2][r, 2 * h + g, 2 * n + p] = v[p]
            yield [sd[b % 2][(r + sch.zero), 2 * h, 0]]

    def table_stage(b, r, sch):
        tail = []
        for g in range(4):
            m1, m32, m512, a0, b0 = [
                (sd[b % 2][r, g, 2 * n], sd[b % 2][r, g, 2 * n + 1]) for n in range(5)]
            m32 = (sch.start(m32[0]), m32[1])
            fa = [a0]
            for _ in range(7):
                fa.append(_cmul(fa[-1], m1))
            for src in (0, 4, 8, 10):
                fa.append(_cmul(fa[src], m512))
            tail.append(fa[11][0] * m512[0] - fa[11][1] * m512[1])
            _store_table(ta[b % 2].at[r, g], fa)
            fb = [b0]
            for _ in range(15):
                p = fb[-1]
                fb.append((p[0] * m32[0] + p[1] * m32[1], p[1] * m32[0] - p[0] * m32[1]))
            _store_table(tb[b % 2].at[r, g], fb)
            yield [ta[b % 2].bitcast(I32)[(r + sch.zero), g, 0, 0:8, :],
                   tb[b % 2].bitcast(I32)[(r + sch.zero), g, 0, 0:8, :]]
        last = [jnp.where(sch.mask("odd"), pltpu.roll(tail[h + 1], 1, 0), tail[h])
                for h in (0, 2)]
        last = [pltpu.bitcast(_rbf(jnp.broadcast_to(jnp.sum(v, axis=1, keepdims=True),
                                                    (8, 128))), I32) for v in last]
        kl[b % 2][r] = jax.lax.shift_right_logical(last[0], 16) | last[1]

    def kernel_stage(b, r, sch):
        ta_w, tb_w = ta[b % 2].bitcast(I32), tb[b % 2].bitcast(I32)
        groups = [None] * 4
        for g0 in (0, 2):
            res = [jax.lax.dot_general(sch.lhs(ta_w[r, g, p, 0:48], g == g0 and p == 0),
                                       _mxu(tb_w[r, g, p, 0:64]), NT_DIMS, preferred_element_type=F32)
                   for g in (g0, g0 + 1) for p in range(2)]
            groups[g0], groups[g0 + 1] = res[0] + res[1], res[2] + res[3]
            sch.results(groups[g0 + 1])
            yield []
        dskip = [col_v[1, _ds(b * MB + 16 * r + 8 * h, 8), :] for h in range(2)]
        dst = _ds(8 * r, 8)
        res = _k_residues(groups, kl[b % 2][r], dskip, pk_v.at[sch.slot, 0], sch)
        for s, t in enumerate(res):
            uk[1][b % 2][4 * (s % 4) + s // 4, dst, :] = t
        yield [uk[1][b % 2][0, _ds(8 * (r + sch.zero), 8), :]]

    def norm_stage(b, r, sch):
        rows, dst = _ds(b * MB // 2 + 8 * r, 8), _ds(8 * r, 8)
        tiles = [x_v.bitcast(I32)[j, rows, :] for j in range(NT)]
        for s, t in enumerate(_to_residues([sch.start(tiles[0])] + tiles[1:], sch)):
            xr[b % 4][4 * (s % 4) + s // 4, dst, :] = t
            xs, m, inv = _mxu(t).astype(F32), st_v[s, 0], st_v[s, 1]
            uk[0][b % 2][4 * (s % 4) + s // 4, _ds(16 * r, 16), :] = jnp.concatenate(
                [(xs[0:8] - m) * inv, (xs[8:16] - m) * inv], axis=0).astype(BF16)
        yield [uk[0][b % 2].bitcast(I32)[0, _ds(8 * (r + sch.zero), 8), :]]

    def forward_stage(w, b, k, sch):
        dst = ab[w][b % len(ab[w])]
        for p in range(2):
            v = [jnp.dot(sch.lhs((uk[w][b % 2] if w else uk[w][b % 2].bitcast(I32))[
                4 * k + n, 0:MB // 2], n == 0),
                         _mxu(ww[w][p ^ (n & 1), 4 * k + n, 0:64]),
                         preferred_element_type=F32) for n in range(4)]
            d02, d13 = v[0] - v[2], v[1] - v[3]
            x1 = d02 - d13 if p == 0 else d02 + d13
            dst[0, k, p, 0:MB] = v[0] + v[2]
            dst[2, k, 1 - p, 0:MB] = v[1] + v[3]
            dst[1, k, p, 0:MB] = x1
            dst[3, k, p, 0:MB] = d02 + d13 if p == 0 else d02 - d13
            sch.results(x1)
            yield []

    def stats(tiles, sch):
        ones_w = wx_v.bitcast(I32)[...]
        for j in tiles:
            acc = None
            for i in range(0, D // 2, 8):
                v = [t * t for t in _split(x_v.bitcast(I32)[j, i:i + 8, :])]
                acc = v if acc is None else [p + q for p, q in zip(acc, v)]
            sums = jnp.dot(_mxu(jnp.concatenate(
                [ones_w[:, :128] if j % 2 == 0 else sch.tie(ones_w[:, :128], prev),
                 ones_w[:, 128:]], axis=1)),
                           _mxu(x_v.bitcast(I32)[j, 0:D // 2]), preferred_element_type=F32)
            s2 = prev = acc[0] + acc[1]
            for d in (4, 2, 1):
                s2 = s2 + pltpu.roll(s2, d, 0)
            st_v[j, 0], st_v[j, 1] = _ln_scalars(jnp.broadcast_to(sums[0:1], (8, 128)), s2)

    def middle_stage(b, r, sch):
        src = [v[b % len(v)] for v in ab]
        scale = lambda v, f: [(x[0] * f, x[1] * f) for x in v]
        for h in range(2):
            ra = _ds(16 * r + 8 * h, 8)
            ld = lambda q, w, ra=ra: [(src[w][q, k, 0, ra, :], src[w][q, k, 1, ra, :]) for k in range(4)]

            park_v = half_v[2 * (sch.slot % 2) + h]

            def put(q, y):
                x = [park_v[n + sch.zero] for n in range(8)]
                for k in range(4):
                    for p in range(2):
                        cc[b % 2][k, q, p, ra, :] = x[2 * k + p] + y[k][p]
                        cc[b % 2][k, q + 2, p, ra, :] = x[2 * k + p] - y[k][p]

            def park(x):
                for k in range(4):
                    for p in range(2):
                        park_v[2 * k + p] = x[k][p]
                return [park_v[sch.zero]]

            gate = sch.start
            a0, a2, b0, b2 = ld(0, 0), ld(2, 0), ld(0, 1), ld(2, 1)
            a0[0] = (gate(a0[0][0]), a0[0][1])
            e0 = _prod_mod_1(list(map(_cadd, a0, a2)), list(map(_cadd, b0, b2)))
            again = _ds(16 * (r + sch.zero) + 8 * h, 8)
            yield park(e0)
            a0, a2, b0, b2 = (ld(q, w, again) for w in range(2) for q in (0, 2))
            a2[0] = (gate(a2[0][0]), a2[0][1])
            e2 = _prod_mod_m1(list(map(_csub, a0, a2)), scale(map(_csub, b0, b2), 2.0))
            put(0, e2)
            yield [cc[b % 2][0, 0, 0, again, :]]
            four = sch.start(jnp.full((8, 128), 4.0, F32))
            e1 = _prod_mod_i(ld(1, 0), scale(ld(1, 1), four), 1)
            yield park(e1)
            four = sch.start(jnp.full((8, 128), 4.0, F32))
            e3 = _prod_mod_i(ld(3, 0), scale(ld(3, 1), four), -1)
            put(1, e3)
            yield [cc[b % 2][0, 1, 0, again, :]]

    def inverse_stage(b, k, sch):
        src = cc[b % 2]

        def lhs(v, n, first):
            return sch.lhs(jnp.concatenate(
                [_pack(pk_v.at[sch.slot, 2], 4 * n + i // 16, v[i:i + 8], v[i + 8:i + 16])
                 for i in range(0, MB, 16)], axis=0), first)

        for o in range(2):
            p0, p1 = [(src[k, q, 0, 0:MB], src[k, q, 1, 0:MB]) for q in (2 * o, 2 * o + 1)]
            if o == 0:
                e = {0: _cadd(p0, p1), 2: _csub(p0, p1)}
            else:
                e = {1: (p0[0] + p1[1], p0[1] - p1[0]), 3: (p0[0] - p1[1], p0[1] + p1[0])}
            ys = []
            for n in e:
                y = [jnp.dot(lhs(e[n][p], 2 * n + p, n == o and p == 0),
                             _mxu(wt_w[4 * k + (0, 2, 1, 3)[n], p, 0:64]),
                             preferred_element_type=F32)
                     for p in range(2)]
                h = y[0] + y[1] + _mxu(xr[b % 4][4 * k + n, 0:MB // 2]).astype(F32)
                h_v[k + 4 * n, b * MB:b * MB + MB, :] = h.astype(BF16)
                hh = h * h
                sq_v[k + 4 * n] += sum((hh[i:i + 8] for i in range(8, MB, 8)), hh[0:8])
                ys.append(h)
            sch.results(ys[-1])
            yield []

    def sum_stage(b, r, sch):
        for n in range(4):
            sums = jnp.dot(sch.lhs(wy_v.bitcast(I32)[b], n == 0)[:, :MB],
                           _mxu(h_v.bitcast(I32)[4 * r + n, b * MB // 2:(b + 1) * MB // 2]),
                           preferred_element_type=F32)
            acc_v[4 * r + n] += sums[0:8]
        sch.results(sums)
        yield []

    nb = D // MB
    stages = dict(
        s=(seed_stage, 0), t=(table_stage, 1), k=(kernel_stage, 2),
        F=(functools.partial(forward_stage, 1), 3), n=(norm_stage, 2),
        f=(functools.partial(forward_stage, 0), 3), m=(middle_stage, 4),
        i=(inverse_stage, 5), a=(sum_stage, 6))

    def run(step, zero, live=None):
        live = live or {n: (f, step - lag) for n, (f, lag) in stages.items()
                        if 0 <= step - lag < nb and (n, step) != ("n", 2)}
        unroll, plan = PLANS["".join(live)]

        def body(it, carry):
            sch = _Schedule(zero >> (step % 32) if unroll == 4 else zero & it, idx_v)
            gens = [{n: f(b, it * unroll + u, sch) for n, (f, b) in live.items()}
                    for u in range(unroll)]
            if step == 3:
                for i in range(9 * unroll):
                    for cp in cp_w(9 * unroll * it + i):
                        cp.start()
            for item in plan.split():
                u, n, *ties = item.split(":")
                if n in live:
                    sch.slot = int(u)
                    sch.run(gens[int(u)][n], *map(int, ties or (-1, -1)))
            for sch.slot, g in enumerate(gens):
                for v in g.values():
                    for _ in v:
                        pass
            return carry + it

        if unroll == 4:
            if step == 101 or step > nb + 3:
                return body(0, 0)
            return jax.lax.fori_loop(zero, 1, lambda _, c: body(0, c), 0)
        return jax.lax.fori_loop(0, 4 // unroll, body, 0)

    _init_index(idx_v)
    acc_v[...] = sq_v[...] = jnp.zeros(acc_v.shape, F32)
    zero = run(0, 0) - 1
    for step in range(1, nb + 6):
        if step == 7:
            cp_d.start()
        if step == 4:
            for cp in cp_par[1]:
                cp.wait()
        if step == 3:
            for half in range(2):
                tiles = range(NT // 2 * half, NT // 2 * (half + 1))
                for j in tiles:
                    cp_x[j].wait()
                if not half:
                    for cp in cp_par[1]:
                        cp.start()
                _transpose_dft(wt_v, w_v, range(4 + 6 * half, 10 + 6 * half))
                stats(tiles, _Schedule(zero, idx_v))
            for q in range(2):
                for s, v in enumerate(_to_residues([st_v[j, q] for j in range(NT)],
                                                   _Schedule(zero, idx_v))):
                    st_v[s, q] = v
            run(101, zero, dict(n=(norm_stage, 0)))
        run(step, zero)

    sums = [acc_v[s] for s in range(16)]
    m2, inv2 = _ln_scalars(
        jnp.concatenate([v[0:1] for v in sums], axis=0),
        jnp.concatenate([jnp.sum(sq_v[j], axis=0, keepdims=True) for j in range(NT)], axis=0))
    wsum = jnp.sum(wr_v[...].astype(F32).reshape(1, D), axis=1, keepdims=True)
    score = _rbf((jnp.concatenate([v[1:2] for v in sums], axis=0) - m2 * wsum) * inv2 + 0.0)
    bits = pltpu.bitcast(score, I32) >> 16
    order = jnp.where(bits < 0, -1 - bits, bits + 32768)
    mu = (_iota((NT, 128), 1) - _iota((NT, 128), 0)) & 127
    pos = 128 * (mu & 15) + 16 * (mu >> 4) + _iota((NT, 128), 0)
    key = pltpu.bitcast((order << 11) + (L - 1 - pos) + (1 << 29), F32)

    h_w, out_w = h_v.bitcast(I32), out_v.bitcast(I32)
    sch, done = _Schedule(zero, idx_v), []
    tie = sch.tie

    def unrouted():
        for q, v in enumerate((1.0 + inv2, m2 * inv2)):
            for j, t in enumerate(_to_time(
                    [jnp.broadcast_to(v[s:s + 1], (8, 128)) for s in range(16)], sch)):
                st_v[j, q] = t
        for i in range(0, D, 16):
            scal = st_v.at[pl.ds(zero * (i + 1), NT)]
            tiles = [h_w[s, i // 2:i // 2 + 8, :] for s in range(16)]
            if len(done) > LAG:
                tiles[0] = tie(tiles[0], done[-LAG])
            for j, v in enumerate(_to_time(tiles, sch)):
                h, mul, sub = _mxu(v).astype(F32), scal[j, 0], scal[j, 1]
                out_v[j, i:i + 16, :] = jnp.concatenate(
                    [h[0:8] * mul - sub, h[8:16] * mul - sub], axis=0).astype(BF16)
                if j % 8 == 7:
                    yield pltpu.bitcast(out_w[j + zero, i // 2:i // 2 + 8, :], F32)

    side = unrouted()

    lane8, sub8 = _iota((CAP, 128), 1), _iota((CAP, 128), 0)
    best = _top8([pltpu.roll(key[i:i + 8], n, 1) if n else key[i:i + 8]
                  for i in (0, 8) for n in range(8)])
    cand = best[0]
    for c in range(1, CAP):
        cand = jnp.where(sub8 == c, best[c], cand)
    best = _top8([pltpu.roll(cand, n, 1) if n else cand for n in range(0, 128, 8)])
    for _ in range(2 * EARLY):
        best[-1] = tie(best[-1], next(side))
    best = [pltpu.bitcast(v, I32)[0, 0] for v in best]
    picks = [L - 1 - (v & (L - 1)) for v in best]

    def schedule(col):
        rnd = [sum([(col[e] == col[c]).astype(I32) for e in range(c)], 0) for c in range(CAP)]
        return (rnd, functools.reduce(jnp.maximum, rnd) + 1,
                lambda n: [lane8 == jnp.where(rnd[c] == n, col[c], -1) for c in range(CAP)])

    _, rounds, lanes = schedule([((t >> 7) + (t & 127)) & 127 for t in picks])

    def out_copy(q, lo, hi):
        j = order[q]
        return pltpu.make_async_copy(
            out_v.at[j, lo:hi], out_hbm.at[lo:hi, _ds(j * 128, 128)], sem_o)

    for n, ref in enumerate((wg_v, wu_v)):
        pltpu.make_async_copy(ref.at[:, 0:D], ref.at[:, 0:D], sem_w.at[n]).wait()

    def gather(n, acc):
        masks = lanes(n)
        tiles = []
        for i in range(0, D // 2, 8):
            v = jnp.zeros((8, 128), I32)
            for c in range(CAP):
                v = jnp.where(masks[c], h_w[picks[c] & 15, i:i + 8, :], v)
            tiles.append(v)
        lhs = jnp.zeros((CAP, 128), F32)
        for c in range(CAP):
            lhs = jnp.where(masks[c] & (sub8 == c), 1.0, lhs)
        aux = [jnp.zeros((CAP, 128), F32)] * 3
        for c in range(CAP):
            hit = pltpu.bitcast(key, I32) == best[c]
            aux = [jnp.where(sub8 == c, jnp.sum(jnp.where(hit, v, 0.0), axis=0, keepdims=True), a)
                   for a, v in zip(aux, (m2, inv2, score))]
        return (acc[0] + jax.lax.dot_general(lhs.astype(BF16), _mxu(jnp.concatenate(tiles, axis=0)),
                                             NT_DIMS, preferred_element_type=F32),
                *[jnp.sum(a, axis=1, keepdims=True) for a in aux])

    h_sel, m_sel, inv_sel, score_sel = jax.lax.fori_loop(
        0, rounds, gather, (jnp.zeros((CAP, D), F32), *[jnp.zeros((CAP, 1), F32)] * 3))
    x_sel = _rbf((h_sel - m_sel) * inv_sel)
    gate = _rbf(jax.nn.sigmoid(score_sel))

    tile, col = [t >> 7 for t in picks], [t & 127 for t in picks]
    rnd, rounds, lanes = schedule(col)
    routed = functools.reduce(jnp.bitwise_or, [1 << j for j in tile])
    spare = CAP - sum((routed >> j) & 1 for j in range(NT))
    n_late = 0
    for j in range(NT):
        hit = (routed >> j) & 1
        fill = (1 - hit) & (spare > 0).astype(I32)
        spare = spare - fill
        order_s[jnp.clip(jnp.where(hit + fill == 1, CAP + n_late, j - n_late), 0, NT - 1)] = j
        n_late = n_late + hit + fill

    order = [order_s[q] for q in range(NT)]

    def early_copies(n):
        lo, hi = (0, 16 * EARLY, MID, D)[n:n + 2]
        return [out_copy(q, lo, hi) for q in range(CAP)]

    def start(copies):
        for cp in copies:
            cp.start()

    start(early_copies(0))
    rate, sent = MID // 8 - 2 * EARLY, [0]

    def project(w_ref):
        parts = []
        for n in range(0, FF // 128, 4):
            for lo in range(0, D, 128):
                hi = min(lo + 128, D)
                xs = x_sel[:, lo:hi]
                if hi - lo == 128 and min(rate, (len(done) - 4) * rate // 70) > sent[0]:
                    sent[0] += 1
                    xs = tie(xs, next(side))
                w = [w_ref.bitcast(I32)[i, lo // 2:hi // 2, :] for i in range(n, n + 4)]
                v = jnp.dot(xs.astype(BF16), _mxu(jnp.concatenate(w, axis=1)),
                            preferred_element_type=F32)
                done.append(v[:, 0:128])
                acc = acc + v if lo else v
            parts.append(acc)
        return _rbf(jnp.concatenate(parts, axis=1))

    g = project(wg_v)
    act = _rbf(g * jax.nn.sigmoid(g)) * project(wu_v)
    for _ in range(rate - sent[0]):
        next(side)
    done.clear()

    cp_d.wait()

    start(early_copies(1))
    rest_side = list(side)

    def placed(r, words):
        idx = jnp.zeros((CAP, 128), I32)
        for c, m in enumerate(lanes(r)):
            idx = jnp.where(m, c, idx)
        return [_gather(w, idx) for w in words]

    def late_copies(lo, hi):
        return [out_copy(CAP + q, lo, hi) for q in range(CAP)]

    def words_of(n):
        return [new_v[n].bitcast(I32)[i:i + 8, :] for i in range(0, new_v[n].shape[0] // 2, 8)]

    tokens = []
    for n, (lo, hi) in enumerate(ROW_CHUNKS):
        a = [act[:, i:i + 128] for i in range(0, FF, 128)]
        for i, token in enumerate(rest_side):
            at = 8 + i * SPAN // len(rest_side) - n * len(a)
            if 0 <= at < len(a):
                a[at] = tie(a[at], token)
        if n == 1:
            start(early_copies(2))
        if n >= 2:
            cut = 12 * 128 // (hi - lo)
            a[cut] = tie(a[cut], tokens[n - 2])
        a = jnp.concatenate(a, axis=1)
        y = _rbf(jax.lax.dot_general(a.astype(BF16), wd_v[lo:hi, :], NT_DIMS,
                                     preferred_element_type=F32))
        new = h_sel[:, lo:hi] + _rbf(x_sel[:, lo:hi] + _rbf(y * gate))
        new_v[n][...] = jnp.concatenate(
            [new.T, jnp.zeros((hi - lo, 128 - CAP), F32)], axis=1).astype(BF16)
        rows = range(lo // 2, hi // 2, 8)
        words = words_of(n)
        both = list(zip(rows, placed(0, words), placed(1, words)))
        for c in range(CAP):
            for i, v0, v1 in both:
                pltpu.store(out_w.at[tile[c], pl.ds(i, 8), :],
                            jnp.where(rnd[c] == 0, v0, v1), mask=lane8 == col[c])
        for cp in late_copies(lo, hi):
            cp.start()
        out_w[tile[0], D // 2:, :] = lane8
        tokens.append(pltpu.bitcast(out_w[tile[0] | zero, D // 2:, :], F32))
    pltpu.make_async_copy(out_v.at[:, 0:D], out_v.at[:, 0:D], sem_o).wait()

    @pl.when(rounds > 2)
    def _():
        def fix(r, carry):
            rows = range(0, D // 2, 8)
            vals = placed(r, sum(map(words_of, range(len(new_v))), []))
            for c, m in enumerate(lanes(r)):
                for i, v in zip(rows, vals):
                    pltpu.store(out_w.at[tile[c], pl.ds(i, 8), :], v, mask=m)
            return carry

        jax.lax.fori_loop(2, rounds, fix, 0)
        for cp in late_copies(0, D):
            cp.start()
        for cp in late_copies(0, D):
            cp.wait()


@jax.jit
def pallas_sequential_preLN__ssm_conv_s4__moe_arch_mod__prompt_kernel(
    A_u: jax.Array,
    A_A_re: jax.Array,
    A_A_im: jax.Array,
    A_B_re: jax.Array,
    A_B_im: jax.Array,
    A_C_re: jax.Array,
    A_C_im: jax.Array,
    A_log_dt: jax.Array,
    A_Dskip: jax.Array,
    B_x: jax.Array,
    B_w_r: jax.Array,
    B_w_gate: jax.Array,
    B_w_up: jax.Array,
    B_w_down: jax.Array,
):
    del B_x
    hbm = pl.BlockSpec(memory_space=pl.ANY)
    out = pl.pallas_call(
        _kernel,
        out_shape=jax.ShapeDtypeStruct((D, L), BF16),
        in_specs=[hbm] * 13,
        out_specs=hbm,
        scratch_shapes=[
            pltpu.VMEM((NT, D + 16, 128), BF16),
            *[pltpu.VMEM((FF // 128, D + 16, 128), BF16)] * 2,
            pltpu.VMEM((D, FF), BF16),
            pltpu.VMEM((6, D, N), BF16),
            *[pltpu.VMEM((D,), BF16)] * 3,
            *[pltpu.VMEM((2, 16, 144, 128), BF16)] * 2,
            pltpu.VMEM((16, 2, 72, 128), I32),
            pltpu.VMEM((2, D, 128), F32),
            pltpu.VMEM((16, D), BF16),
            pltpu.VMEM((D // MB, 16, 128), BF16),
            pltpu.VMEM((2, 256, 128), F32),
            pltpu.VMEM((len(INDEX), 8, 128), I32),
            pltpu.VMEM((4, 3, 32, 16, 128), BF16),
            pltpu.VMEM((NT, D + 16, 128), BF16),
            pltpu.VMEM((NT, 2, 8, 128), F32),
            *[pltpu.VMEM((NT, 8, 128), F32)] * 2,
            pltpu.VMEM((NT, D + 16, 128), BF16),
            *[pltpu.VMEM((4, 4, 10, 8, 128), F32)] * 2,
            *[pltpu.VMEM((4, 4, 2, 112, 128), BF16)] * 2,
            *[pltpu.VMEM((4, 4, 2, 144, 128), BF16)] * 2,
            *[pltpu.VMEM((4, 8, 128), I32)] * 2,
            *[pltpu.VMEM((16, MB + 16, 128), BF16)] * 2,
            *[pltpu.VMEM((16, MB // 2 + 8, 128), I32)] * 2,
            *[pltpu.VMEM((4, 4, 2, MB + 8, 128), F32)] * 2,
            *[pltpu.VMEM((4, 4, 2, MB + 8, 128), F32)] * 2,
            *[pltpu.VMEM((16, MB // 2 + 8, 128), I32)] * 4,
            pltpu.SMEM((NT,), I32),
            pltpu.SemaphoreType.DMA((15,)),
            pltpu.SemaphoreType.DMA((NT,)),
            pltpu.SemaphoreType.DMA((3,)),
            pltpu.SemaphoreType.DMA,
            *[pltpu.VMEM((4, 4, 2, MB + 8, 128), F32)] * 2,
            *[pltpu.VMEM((8, 8, 128), F32)] * 4,
            *[pltpu.VMEM((hi - lo, 128), BF16) for lo, hi in ROW_CHUNKS],
        ],
        compiler_params=pltpu.CompilerParams(vmem_limit_bytes=100 * 1024 * 1024,
                                             disable_bounds_checks=True,
                                             disable_semaphore_checks=True),
    )(A_u.reshape(L, D).T, A_A_re, A_A_im, A_B_re, A_B_im, A_C_re, A_C_im,
      A_log_dt, A_Dskip, B_w_r, B_w_gate, B_w_up, B_w_down.T)
    return out.T.reshape(1, L, D)
```

```python
import functools

import numpy as np
import jax
import jax.numpy as jnp
import jax.experimental.pallas as pl
import jax.experimental.pallas.tpu as pltpu

F32 = jnp.float32
BF16 = jnp.bfloat16
I32 = jnp.int32

L = 2048
D = 576
N = 128
FF = 4608
CAP = 8
NT = L // 128
EPS = 1e-5
MB = 64
PLANS = dict(
    s=(2, ""),
    st=(2, ""),
    n=(4, ""),
    stk=(2, "0:t:-1:4 1:t:-1:3 0:t:-1:4 0:t:-1:7 0:t:-1:15 1:t:-1:10 1:t:6:16 1:t:11:21 0:k "
            "0:k 1:k 0:s:-1:20 0:s:11:23 0:k:-1:23 1:k 1:s:20:-1 1:s 1:k "),
    stkFnf=(2, "1:t:-1:4 0:s:-1:16 0:s:-1:34 1:s:-1:36 1:s:-1:54 0:f 0:n:1:16 0:F 0:t:4:25 "
               "0:t:0:21 0:k 0:k 0:k:-1:35 0:t:17:36 0:F 0:f 1:f 1:t:29:43 1:F 1:n:33:47 1:k "
               "1:t:39:55 1:k 1:t:42:53 1:k 0:t:44:53 1:F 1:f "),
    stkFnfm=(1, "0:m:-1:2 0:m:-1:5 0:t:-1:7 0:t:-1:14 0:t:-1:9 0:f 0:m:1:14 0:m:-1:18 0:f "
                "0:m:7:21 0:m:6:20 0:k 0:t:9:22 0:n:9:27 0:k 0:s:16:-1 0:m:15:-1 0:m:13:25 0:k "
                "0:s:19:-1 0:F 0:F "),
    stkFnfmi=(4, "0:t:-1:2 0:n:-1:8 0:t:-1:3 0:m:-1:4 0:m:-1:7 0:m:-1:19 0:s:-1:40 1:s:-1:76 "
                 "2:s:-1:112 3:s 0:f 0:m:0:13 0:k 0:s:4:33 0:k 0:m:13:23 0:k:-1:33 0:m:14:25 "
                 "0:t:14:32 0:f 0:t:18:33 0:F 1:t:23:40 0:F 1:n:26:47 1:t:24:38 1:m:27:41 0:i "
                 "1:m:29:47 0:i 0:m:32:40 0:m:31:44 1:m:33:54 1:f 1:m:36:51 1:k 1:s:40:71 1:k "
                 "1:m:49:61 1:k:-1:71 1:m:51:63 1:f 1:t:55:76 1:t:51:68 1:F 2:t:59:74 "
                 "2:t:59:75 1:F 2:m:63:76 2:m:63:79 1:i 2:n:64:80 1:i 1:m:68:76 1:m:67:78 2:f "
                 "2:m:72:91 2:m:71:84 2:k 2:s:76:105 2:k 2:m:83:95 2:k:-1:105 2:m:86:97 "
                 "2:t:86:105 2:f 2:t:90:105 2:F 3:t:94:112 2:F 3:t:96:110 3:m:99:113 2:i "
                 "3:n:101:119 3:m:101:119 2:i 2:m:104:112 2:m:103:116 3:f 3:m:108:126 "
                 "3:m:110:123 3:k 3:s:112:143 3:k 3:m:121:133 3:k:-1:142 3:m:123:135 3:f "
                 "3:t:127:-1 3:t:123:140 3:F 3:F 3:i 3:m:139:-1 3:m:139:-1 3:i "),
    stkFnfmia=(4, "0:t:-1:6 0:t:-1:2 0:n:-1:10 0:m:-1:6 0:m:-1:6 0:m:-1:19 0:s:-1:40 1:s:-1:77 "
                  "2:s:-1:114 3:s 0:a 0:f 0:m:1:18 0:k 0:s:5:40 0:k 0:m:15:27 0:m:-1:26 "
                  "0:k:-1:40 0:t:16:30 0:f 0:t:18:34 0:F 0:F 1:t:25:43 1:t:23:41 1:n:28:47 "
                  "1:m:25:43 1:m:27:44 0:i 0:m:32:40 0:i 0:m:34:42 1:a 1:f 1:m:38:56 1:m:36:55 "
                  "1:k 1:s:42:77 1:k 1:m:52:64 1:m:48:66 1:k:-1:77 1:t:53:67 1:f 1:t:55:71 1:F "
                  "1:F 2:t:64:80 2:t:60:78 2:n:65:84 2:m:62:80 2:m:64:81 1:i 1:m:69:77 1:i "
                  "1:m:71:81 2:m:73:93 2:a 2:f 2:m:75:92 2:k 2:s:79:114 2:k 2:m:89:101 "
                  "2:m:85:103 2:k:-1:114 2:t:90:104 2:f 2:t:92:108 2:F 2:F 3:t:99:117 "
                  "3:t:97:115 3:m:99:117 3:m:101:118 2:i 2:m:106:114 3:n:103:121 2:i "
                  "2:m:108:116 3:a 3:f 3:m:112:130 3:m:112:129 3:k 3:s:116:-1 3:k 3:m:126:138 "
                  "3:m:122:140 3:k:-1:147 3:t:127:141 3:f 3:t:129:-1 3:F 3:F 3:i 3:m:143:-1 "
                  "3:i 3:m:145:-1 "),
    tkFnfmia=(4, "0:t:-1:10 0:t:-1:5 0:n:-1:9 0:m:-1:6 0:m:-1:6 0:f 0:a 0:k 0:m:7:18 0:m:1:23 "
                 "0:k 0:m:15:28 0:m:-1:27 0:k:-1:36 0:f 0:t:17:33 0:t:20:38 0:F 0:F 1:n:28:46 "
                 "1:m:27:43 0:i 0:m:31:39 1:t:31:47 1:t:23:42 1:m:30:43 0:i 0:m:34:44 1:f 1:a "
                 "1:k 1:m:44:55 1:m:38:58 1:k 1:m:52:65 1:m:50:64 1:k:-1:73 1:f 1:t:54:70 "
                 "1:t:57:75 1:F 1:F 2:n:65:83 2:m:64:80 1:i 1:m:68:76 2:t:68:84 2:t:61:80 "
                 "2:m:69:80 1:i 1:m:71:79 2:f 2:a 2:k 2:m:81:92 2:m:75:97 2:k 2:m:89:102 "
                 "2:m:87:101 2:t:90:107 2:k:-1:108 2:f 2:t:94:112 2:F 2:F 3:m:101:117 "
                 "3:n:102:120 2:i 2:m:106:114 3:t:105:121 3:t:97:116 3:m:104:118 2:i "
                 "2:m:108:116 3:f 3:a 3:k 3:m:118:129 3:m:109:131 3:k 3:m:126:139 3:m:124:138 "
                 "3:k:-1:147 3:f 3:t:128:144 3:t:131:-1 3:F 3:F 3:i 3:m:143:-1 3:i 3:m:145:-1 "),
    kFnfmia=(4, "1:m:-1:5 1:m:-1:3 0:n:-1:12 0:F 0:m:2:14 0:m:-1:15 0:a 0:F 0:m:7:21 0:k "
                "0:m:9:27 0:m:13:23 0:k 0:m:15:25 0:m:18:31 0:m:20:32 0:k:-1:45 0:i 0:i 0:f "
                "0:f 1:n:36:50 1:F 1:a 1:F 1:m:42:57 1:m:34:56 1:k 1:m:47:64 1:k 1:m:53:66 "
                "1:k:-1:75 1:i 1:i 3:m:63:79 3:m:61:77 1:f 1:m:68:76 1:f 1:m:73:81 2:n:70:86 "
                "2:F 2:m:76:88 2:m:73:89 2:a 2:F 2:m:79:93 2:k 2:m:83:101 2:m:87:97 2:k "
                "2:m:89:101 2:m:92:105 2:m:90:106 2:k:-1:119 2:i 2:i 2:f 2:f 3:n:110:124 3:F "
                "3:a 3:F 3:m:116:130 3:m:111:134 3:k 3:m:121:141 3:m:124:141 3:k 3:k 3:i 3:i "
                "3:f 3:m:142:-1 3:f 3:m:145:-1 "),
    Ffmia=(4, "1:m:-1:9 0:m:-1:5 0:m:-1:10 0:m:-1:12 0:a 0:F 1:m:4:15 0:i 0:m:6:18 0:i "
              "0:m:9:22 0:F 1:m:16:31 0:f 0:m:20:33 0:f 0:m:22:33 1:a 1:m:25:43 1:F 0:m:29:41 "
              "1:i 1:i 1:m:35:48 1:F 1:m:40:54 1:f 1:m:42:57 1:m:45:56 3:m:45:59 2:m:42:58 1:f "
              "2:a 2:F 2:m:53:63 2:m:49:65 3:m:54:68 2:i 2:m:56:67 2:i 2:m:59:75 2:F 3:m:66:83 "
              "2:f 2:m:70:83 2:f 2:m:72:84 3:a 3:m:75:93 3:F 2:m:79:96 3:i 3:i 3:m:85:-1 3:F "
              "3:m:90:-1 3:f 3:m:92:-1 3:m:95:-1 3:f "),
    mia=(4, "1:m:-1:3 0:m:-1:8 0:m:-1:6 0:m:-1:7 0:m:-1:8 0:i 1:m:0:13 0:m:2:10 0:a 0:i "
            "1:m:5:16 2:m:8:25 1:i 1:m:9:22 0:m:10:23 0:m:8:20 1:m:8:20 3:m:11:25 1:a "
            "2:m:13:27 1:i 1:m:14:22 1:m:17:25 0:m:14:22 1:m:17:25 2:m:14:28 2:m:13:27 2:i "
            "3:m:18:32 2:m:20:32 2:a 2:i 3:m:23:-1 3:m:25:-1 3:m:25:-1 3:i 2:m:28:-1 2:m:27:-1 "
            "3:a 3:i 3:m:32:-1 3:m:35:-1 2:m:33:-1 3:m:35:-1 "),
    iaz=(4, "0:i 0:i 1:i 1:i 0:z 2:i 2:i 1:z 3:i 3:i 2:z 0:a 1:a 2:a 3:a 3:z"),
)
ROW_CHUNKS = ((0, 128), (128, 256), (256, 384), (384, 512), (512, D))
LAG = 16
MID, SPAN, EARLY = 384, 50, 8
NT_DIMS = (((1,), (1,)), ((), ()))


def _round_res(step):
    return [int(np.round(r / step)) * step for r in range(16)]


RES1, RES2, RES3 = _round_res(2), _round_res(4), _round_res(8)


def _ds(start, size):
    return pl.ds(start if isinstance(start, int) else pl.multiple_of(start, size), size)


def _iota(shape, dim):
    return jax.lax.broadcasted_iota(I32, shape, dim)


def _rbf(x):
    return x.astype(BF16).astype(F32)


def _cmul(a, b):
    return (a[0] * b[0] - a[1] * b[1], a[0] * b[1] + a[1] * b[0])


def _csq(a):
    t = a[0] * a[1]
    return ((a[0] + a[1]) * (a[0] - a[1]), t + t)


def _cadd(a, b):
    return (a[0] + b[0], a[1] + b[1])


def _csub(a, b):
    return (a[0] - b[0], a[1] - b[1])


def _bfly4(a0, a1, a2, a3, inverse=False):
    s02, d02 = _cadd(a0, a2), _csub(a0, a2)
    s13, d13 = _cadd(a1, a3), _csub(a1, a3)
    p = (d02[0] - d13[1], d02[1] + d13[0])
    m = (d02[0] + d13[1], d02[1] - d13[0])
    if inverse:
        p, m = m, p
    return _cadd(s02, s13), p, _csub(s02, s13), m


def _prod_mod_1(a, b):
    fa, fb = _bfly4(*a), _bfly4(*b)
    return _bfly4(*[_cmul(x, y) for x, y in zip(fa, fb)], inverse=True)


def _prod2(a0, a1, b0, b1, sgn):
    p00, p11 = _cmul(a0, b0), _cmul(a1, b1)
    c1 = _cadd(_cmul(a0, b1), _cmul(a1, b0))
    if sgn > 0:
        return (p00[0] - p11[1], p00[1] + p11[0]), c1
    return (p00[0] + p11[1], p00[1] - p11[0]), c1


def _prod_mod_m1(a, b):
    def split(x):
        p = [(x[k][0] - x[k + 2][1], x[k][1] + x[k + 2][0]) for k in range(2)]
        m = [(x[k][0] + x[k + 2][1], x[k][1] - x[k + 2][0]) for k in range(2)]
        return p, m
    ap, am = split(a)
    bp, bm = split(b)
    cp = _prod2(*ap, *bp, 1)
    cm = _prod2(*am, *bm, -1)
    lo = [_cadd(cp[k], cm[k]) for k in range(2)]
    hi = [(cp[k][1] - cm[k][1], cm[k][0] - cp[k][0]) for k in range(2)]
    return lo + hi


def _prod_mod_i(a, b, sgn):
    sm = [x[0] + x[1] for x in b]
    df = [x[1] - x[0] for x in b]
    asum = [x[0] + x[1] for x in a]
    out = []
    for k in range(4):
        acc = [None, None, None]
        for j in range(4):
            m = (k - j) % 4
            if j <= k:
                t = ((b[m][0], 1), (df[m], 1), (sm[m], 1))
            elif sgn > 0:
                t = ((b[m][1], -1), (sm[m], 1), (df[m], -1))
            else:
                t = ((b[m][1], 1), (sm[m], -1), (df[m], 1))
            for q, (v, (w, s)) in enumerate(zip((asum[j], a[j][0], a[j][1]), t)):
                p = v * w
                if acc[q] is None:
                    acc[q] = p
                else:
                    acc[q] = acc[q] + p if s > 0 else acc[q] - p
        out.append((acc[0] - acc[2], acc[0] + acc[1]))
    return out


def _barrel(v, sch):
    for bit in range(4):
        m = sch.mask("bit%d" % bit)
        v = [jnp.where(m, v[(i + (1 << bit)) % 16], v[i]) for i in range(16)]
    return [v[-s % 16] for s in range(16)]


def _to_residues(tiles, sch):
    return _barrel([t if j == 0 else pltpu.roll(t, j, 1) for j, t in enumerate(tiles)], sch)


def _to_time(res, sch):
    return [t if j == 0 else pltpu.roll(t, 128 - j, 1)
            for j, t in enumerate(_barrel(res, sch))]


def _gather(x, idx, axis=1):
    return jnp.take_along_axis(x, idx, axis=axis, mode="promise_in_bounds")


def _transpose_dft(wt_ref, wu_ref, residues):
    for s in residues:
        for p in range(2):
            wt_ref[4 * (s % 4) + (0, 2, 1, 3)[s // 4], p, 0:64] = pltpu.bitcast(
                _mxu(wu_ref.bitcast(I32)[p, 4 * (s % 4) + s // 4, 0:64]).T, I32)


def _init_dft(wu_ref, wk_ref, tmp_ref, halfway):
    sub, k4 = _iota((8, 128), 0), 4 * _iota((8, 128), 1) + 1

    def cis(t):
        ph = ((k4 * t) & (4 * L - 1)).astype(F32) * (2 * np.pi / (4 * L))
        return jnp.cos(ph), jnp.sin(ph)

    w1, w16 = cis(1), cis(16)
    w32 = _csq(w16)
    fk = [cis(16 * (32 * (sub & 3) + (sub >> 2)))]
    fu = [cis(128 * sub), cis(128 * (sub + 8))]
    for v in range(1, 16):
        fk.append(_cmul(fk[-1], w32))
        if v >= 2:
            fu.append(_cmul(fu[-2], w16))
    for p in range(2):
        for v in range(32):
            tmp_ref[p, 8 * v:8 * v + 8, :] = fu[v % 16][p]
    tw = None
    for s in range(16):
        for v in range(0, 16, 2):
            rows = [slice(128 - s + 8 * i, 136 - s + 8 * i) for i in (v, v + 1)]
            for ref, f in ((wk_ref, fk[v:v + 2]),
                           (wu_ref, [(tmp_ref[0, r, :], tmp_ref[1, r, :]) for r in rows])):
                if s:
                    f = [_cmul(x, tw) for x in f]
                for p in range(2):
                    ref[p, 4 * (s % 4) + s // 4, 8 * v:8 * v + 16, :] = jnp.concatenate(
                        [f[0][p], f[1][p]], axis=0).astype(BF16)
        tw = _cmul(tw, w1) if s else w1
        if s == 7:
            halfway()


def _pack(ref, n, a, b):
    ref[n] = jnp.concatenate([a, b], axis=0).astype(BF16)
    return ref.bitcast(I32)[n]


def _split(w):
    return [pltpu.bitcast(w << 16, F32), pltpu.bitcast(w & -65536, F32)]


FINE = (0, 1, 2, 3, 4, 5, 6, 7, 512, 516, 1024, 1536)


def _k_seeds(z, c, sch):
    pw = {1: z}
    for e in range(1, 10):
        pw[1 << e] = _csq(pw[1 << (e - 1)])
    c8, z16 = _cmul(c, pw[8]), (pw[16][0], 0.0 - pw[16][1])
    pair = lambda a, b: tuple(jnp.where(sch.mask("odd"), q, p) for p, q in zip(a, b))
    seeds = []
    for g in range(2):
        twice = lambda v: tuple(_gather(x, sch.idx("dup%d" % g), 0) for x in v)
        seeds.append([twice(z), twice(pw[32]), twice(pw[512]),
                      pair(twice(c), twice(c8)), pair((1.0, 0.0), twice(z16))])
    return seeds


def _mxu(words):
    return pltpu.bitcast(words, BF16)


def _store_table(ref, tab):
    for i in range(0, len(tab), 2):
        for p in range(2):
            ref[p, 8 * i:8 * i + 16, :] = jnp.concatenate(
                [tab[i][p], tab[i + 1][p]], axis=0).astype(BF16)


def _k_residues(groups, k_last, dskip, tmp_ref, sch):
    idx, nxt = sch.idx("src"), sch.idx("nxt")
    low = lambda x, y: (x & 65535) | (y << 16)
    high = lambda x, y: jax.lax.shift_right_logical(x, 16) | (y & -65536)
    kv, up = {}, {}
    for i, k in enumerate(FINE):
        v = [g[8 * i:8 * i + 8] for g in groups]
        if k == 0:
            v = [x + jnp.where(sch.mask("diag"),
                               _gather(dskip[n // 2], sch.idx("dup%d" % (n % 2)), 0), 0.0)
                 for n, x in enumerate(v)]
        p = [_pack(tmp_ref, 2 * i + h, v[2 * h], v[2 * h + 1]) for h in range(2)]
        both = [_gather(x, idx) for x in p]
        kv[k], kv[k + 8] = low(*both), high(*both)
        if k % 512 == 0:
            up[k] = low(*[_gather(x, nxt) for x in p])
    k_last = _gather(k_last, sch.idx("rows"), 0)
    q0, q1, q2, up0, up01, up2, up3, fine = map(sch.mask, INDEX[-8:])
    s3 = {r: jnp.where(q2, kv[1024 + r], kv[1536 + r]) for r in (0, 8)}
    v0 = jnp.where(q0, kv[0], jnp.where(q1, kv[512], s3[0]))
    v16 = jnp.where(up01, jnp.where(up0, up[0], up[512]),
                    jnp.where(up2, up[1024], jnp.where(up3, up[1536], k_last)))
    s3[16] = v16
    s23, s123, out = {}, {}, [v0]
    for r in range(1, 16):
        k23 = (RES2[r], RES3[r])
        if k23 not in s23:
            s23[k23] = v16 if k23 == (16, 16) else jnp.where(q1, kv[512 + k23[0]], s3[k23[1]])
        k123 = (RES1[r],) + k23
        if k123 not in s123:
            s123[k123] = v16 if k123[0] == 16 else jnp.where(q0, kv[k123[0]], s23[k23])
        if RES1[r] == r:
            out.append(s123[k123])
        else:
            out.append(jnp.where(fine, kv[r], s123[k123]))
    return out


def _ln_scalars(s1, s2):
    mean = s1 * (1.0 / D)
    var = jnp.maximum(s2 * (1.0 / D) - mean * mean, 0.0)
    eps = float(np.asarray(EPS, dtype=BF16))
    sd = _rbf(jnp.sqrt(_rbf(_rbf(var) + eps)))
    return _rbf(mean), 1.0 / sd


def _top8(x):
    def swap(v, pairs):
        for i, j in pairs:
            v[i], v[j] = jnp.maximum(v[i], v[j]), jnp.minimum(v[i], v[j])
        return v

    def merge(a, b):
        v = [jnp.maximum(a[i], b[7 - i]) for i in range(8)]
        return swap(v, [(i, i + d) for d in (4, 2, 1) for i in range(8) if not i & d])

    sort8 = ((0, 2), (1, 3), (4, 6), (5, 7), (0, 4), (1, 5), (2, 6), (3, 7), (0, 1), (2, 3),
             (4, 5), (6, 7), (2, 4), (3, 5), (1, 4), (3, 6), (1, 2), (3, 4), (5, 6))
    v = merge(*[swap(x[i:i + 8], sort8) for i in (0, 8)])
    for d in (4, 2, 1):
        v = merge(v, [pltpu.roll(t, d, 0) for t in v])
    return v


def _init_columns(col_ref, wx_ref, wy_ref, ldt_ref, dsk_ref, wr_ref):
    row, lane = _iota((128, 128), 0), _iota((128, 128), 1)
    split = (row & ~15) + 2 * (row & 7) + ((row >> 3) & 1)
    ldt, dsk, wr = (ref[...].astype(F32).reshape(1, D) for ref in (ldt_ref, dsk_ref, wr_ref))
    for n, vec in enumerate((jnp.exp(ldt), dsk * (1.0 / L))):
        for lo in range(0, D, 128):
            i = min(lo, D - 128)
            diag = jnp.where(split == lane, vec[:, i:i + 128], 0.0)[lo - i:].astype(BF16)
            col_ref[n, lo:i + 128, :] = jnp.dot(diag, jnp.ones((128, 128), BF16),
                                                preferred_element_type=F32)
    sub = _iota((16, D), 0)
    ones_w = jnp.where(sub == 0, 1.0, jnp.where(sub == 1, wr, 0.0))
    wx_ref[...] = ones_w.astype(BF16)
    for lo in range(0, D, MB):
        wy_ref[lo // MB, :, 0:MB] = ones_w[:, lo:lo + MB].astype(BF16)
        wy_ref[lo // MB, :, MB:] = jnp.zeros((16, 128 - MB), BF16)


INDEX = ("true", "bit0", "bit1", "bit2", "bit3", "odd", "dup0", "dup1", "rows", "src", "nxt",
         "diag", "q0", "q1", "q2", "up0", "up01", "up2", "up3", "fine")


def _init_index(idx_ref):
    sub, lane = _iota((8, 128), 0), _iota((8, 128), 1)
    src = lambda b: 8 * ((b >> 1) & 15) + 2 * (sub & 3) + (b & 1)
    is_ = lambda m: jnp.where(m, 1, 0)
    q = lane & 3
    q16 = q + is_(lane >= 124)
    tiles = dict(true=sub + 1, odd=sub & 1, dup0=sub >> 1, dup1=4 + (sub >> 1),
                 rows=2 * (sub & 3) + (sub >> 2), src=src(lane >> 2), nxt=src((lane >> 2) + 1),
                 diag=is_((lane == sub) & ((sub & 1) == 0)), up01=is_(q16 < 2),
                 fine=is_((q == 0) & (lane < 64)),
                 **{"bit%d" % n: (lane >> n) & 1 for n in range(4)},
                 **{"q%d" % n: is_(q == n) for n in range(3)},
                 **{"up%d" % n: is_(q16 == n) for n in (0, 2, 3)})
    for n, name in enumerate(INDEX):
        idx_ref[n] = tiles[name]


class _Schedule:
    def __init__(self, zero, idx_ref):
        self.zero = zero
        self.idx = lambda name: idx_ref[INDEX.index(name) + zero]
        self.mask = lambda name: self.idx(name) != 0
        self.true = self.mask("true")
        self.done, self.pending, self.wait = [], {}, -1

    def tie(self, x, token):
        return jnp.where(self.true, x, token if token.dtype == x.dtype
                         else pltpu.bitcast(token, x.dtype))

    def start(self, x):
        return self.tie(x, self.done[self.wait]) if 0 <= self.wait < len(self.done) else x

    def lhs(self, words, first):
        tiles = [words[i:i + 8] for i in range(0, words.shape[0], 8)]
        for i in range(len(tiles) if first else 0):
            for token in self.pending.pop(len(self.done) + i, ()):
                tiles[i] = self.tie(tiles[i], token)
        return _mxu(jnp.concatenate(tiles, axis=0))

    def results(self, v):
        self.done += [v[i + 8:i + 16] for i in range(0, v.shape[0], 16)]

    def run(self, stage, wait, before):
        self.wait = wait
        self.pending.setdefault(before, []).extend(next(stage))


def _kernel(x_hbm, are_hbm, aim_hbm, bre_hbm, bim_hbm, cre_hbm, cim_hbm,
            ldt_hbm, dsk_hbm, wr_hbm, wg_hbm, wu_hbm, wd_hbm, out_hbm,
            x_v, wg_v, wu_v, wd_v, par_v, ldt_v, dsk_v, wr_v, w_v, wk_v, wt_v, col_v, wx_v, wy_v,
            tmp_v, idx_v, pk_v, h_v, st_v, acc_v, sq_v, out_v, sd0, sd1, ta0, ta1, tb0, tb1, kl0, kl1,
            u0, u1, k0, k1, a0_v, a1_v, c0, c1, r0, r1, r2, r3, order_s,
            sem_p, sem_x, sem_w, sem_o, f0_v, f1_v, *rest):
    half_v, new_v = rest[:4], rest[4:]
    cp_vec = [pltpu.make_async_copy(s, d, sem_p.at[n]) for n, (s, d) in enumerate(
        ((ldt_hbm, ldt_v), (dsk_hbm, dsk_v), (wr_hbm, wr_v)))]
    cp_par = [[pltpu.make_async_copy(s.at[lo:hi], par_v.at[n, lo:hi], sem_p.at[3 + 6 * m + n])
               for n, s in enumerate((are_hbm, aim_hbm, bre_hbm, bim_hbm, cre_hbm, cim_hbm))]
              for m, (lo, hi) in enumerate(((0, 4 * MB), (4 * MB, D)))]
    cp_x = [pltpu.make_async_copy(x_hbm.at[:, 128 * j:128 * j + 128], x_v.at[j, 0:D],
                                  sem_x.at[j])
            for j in range(NT)]
    cp_d = pltpu.make_async_copy(wd_hbm, wd_v, sem_w.at[2])

    def cp_w(i):
        return [pltpu.make_async_copy(s.at[:, _ds(128 * i, 128)], d.at[i, 0:D], sem_w.at[n])
                for n, (s, d) in enumerate(((wg_hbm, wg_v), (wu_hbm, wu_v)))]

    for cp in cp_vec + cp_par[0]:
        cp.start()
    for cp in cp_x[:NT // 2]:
        cp.start(priority=1)

    def columns():
        for cp in cp_vec:
            cp.wait()
        for cp in cp_x[NT // 2:]:
            cp.start(priority=1)
        _transpose_dft(wt_v, w_v, range(4))
        _init_columns(col_v, wx_v, wy_v, ldt_v, dsk_v, wr_v)

    _init_dft(w_v, wk_v, tmp_v, columns)
    for cp in cp_par[0]:
        cp.wait()

    sd, ta, tb, kl = (sd0, sd1), (ta0, ta1), (tb0, tb1), (kl0, kl1)
    uk, ab, cc, xr = ((u0, u1), (k0, k1)), ((a0_v, a1_v), (f0_v, f1_v)), (c0, c1), (r0, r1, r2, r3)
    ww, wt_w = (w_v.bitcast(I32), wk_v.bitcast(I32)), wt_v

    def chan(b, r):
        return _ds(b * MB + 16 * r, 16)

    def seed_stage(b, r, sch):
        rows = _ds(b * MB // 2 + 8 * r, 8)
        par = [_split(par_v.bitcast(I32)[n, rows, :]) for n in range(6)]
        for h in range(2):
            a_re, a_im, b_re, b_im, c_re, c_im = [v[h] for v in par]
            dt = sch.start(col_v[0, _ds(b * MB + 16 * r + 8 * h, 8), :])
            mag, ang = jnp.exp(dt * a_re), dt * a_im
            sc = dt * (1.0 / L)
            seeds = _k_seeds((mag * jnp.cos(ang), mag * jnp.sin(ang)),
                             _cmul((c_re, c_im), (sc * b_re, sc * b_im)), sch)
            for g in range(2):
                for n, v in enumerate(seeds[g]):
                    for p in range(2):
                        sd[b % 2][r, 2 * h + g, 2 * n + p] = v[p]
            yield [sd[b % 2][(r + sch.zero), 2 * h, 0]]

    def table_stage(b, r, sch):
        tail = []
        for g in range(4):
            m1, m32, m512, a0, b0 = [
                (sd[b % 2][r, g, 2 * n], sd[b % 2][r, g, 2 * n + 1]) for n in range(5)]
            m32 = (sch.start(m32[0]), m32[1])
            fa = [a0]
            for _ in range(7):
                fa.append(_cmul(fa[-1], m1))
            for src in (0, 4, 8, 10):
                fa.append(_cmul(fa[src], m512))
            tail.append(fa[11][0] * m512[0] - fa[11][1] * m512[1])
            _store_table(ta[b % 2].at[r, g], fa)
            fb = [b0]
            for _ in range(15):
                p = fb[-1]
                fb.append((p[0] * m32[0] + p[1] * m32[1], p[1] * m32[0] - p[0] * m32[1]))
            _store_table(tb[b % 2].at[r, g], fb)
            yield [ta[b % 2].bitcast(I32)[(r + sch.zero), g, 0, 0:8, :],
                   tb[b % 2].bitcast(I32)[(r + sch.zero), g, 0, 0:8, :]]
        last = [jnp.where(sch.mask("odd"), pltpu.roll(tail[h + 1], 1, 0), tail[h])
                for h in (0, 2)]
        last = [pltpu.bitcast(_rbf(jnp.broadcast_to(jnp.sum(v, axis=1, keepdims=True),
                                                    (8, 128))), I32) for v in last]
        kl[b % 2][r] = jax.lax.shift_right_logical(last[0], 16) | last[1]

    def kernel_stage(b, r, sch):
        ta_w, tb_w = ta[b % 2].bitcast(I32), tb[b % 2].bitcast(I32)
        groups = [None] * 4
        for g0 in (0, 2):
            res = [jax.lax.dot_general(sch.lhs(ta_w[r, g, p, 0:48], g == g0 and p == 0),
                                       _mxu(tb_w[r, g, p, 0:64]), NT_DIMS, preferred_element_type=F32)
                   for g in (g0, g0 + 1) for p in range(2)]
            groups[g0], groups[g0 + 1] = res[0] + res[1], res[2] + res[3]
            sch.results(groups[g0 + 1])
            yield []
        dskip = [col_v[1, _ds(b * MB + 16 * r + 8 * h, 8), :] for h in range(2)]
        dst = _ds(8 * r, 8)
        res = _k_residues(groups, kl[b % 2][r], dskip, pk_v.at[sch.slot, 0], sch)
        for s, t in enumerate(res):
            uk[1][b % 2][4 * (s % 4) + s // 4, dst, :] = t
        yield [uk[1][b % 2][0, _ds(8 * (r + sch.zero), 8), :]]

    def norm_stage(b, r, sch):
        rows, dst = _ds(b * MB // 2 + 8 * r, 8), _ds(8 * r, 8)
        tiles = [x_v.bitcast(I32)[j, rows, :] for j in range(NT)]
        for s, t in enumerate(_to_residues([sch.start(tiles[0])] + tiles[1:], sch)):
            xr[b % 4][4 * (s % 4) + s // 4, dst, :] = t
            xs, m, inv = _mxu(t).astype(F32), st_v[s, 0], st_v[s, 1]
            uk[0][b % 2][4 * (s % 4) + s // 4, _ds(16 * r, 16), :] = jnp.concatenate(
                [(xs[0:8] - m) * inv, (xs[8:16] - m) * inv], axis=0).astype(BF16)
        yield [uk[0][b % 2].bitcast(I32)[0, _ds(8 * (r + sch.zero), 8), :]]

    def forward_stage(w, b, k, sch):
        dst = ab[w][b % len(ab[w])]
        for p in range(2):
            v = [jnp.dot(sch.lhs((uk[w][b % 2] if w else uk[w][b % 2].bitcast(I32))[
                4 * k + n, 0:MB // 2], n == 0),
                         _mxu(ww[w][p ^ (n & 1), 4 * k + n, 0:64]),
                         preferred_element_type=F32) for n in range(4)]
            d02, d13 = v[0] - v[2], v[1] - v[3]
            x1 = d02 - d13 if p == 0 else d02 + d13
            dst[0, k, p, 0:MB] = v[0] + v[2]
            dst[2, k, 1 - p, 0:MB] = v[1] + v[3]
            dst[1, k, p, 0:MB] = x1
            dst[3, k, p, 0:MB] = d02 + d13 if p == 0 else d02 - d13
            sch.results(x1)
            yield []

    def stats(tiles, sch):
        ones_w = wx_v.bitcast(I32)[...]
        for j in tiles:
            acc = None
            for i in range(0, D // 2, 8):
                v = [t * t for t in _split(x_v.bitcast(I32)[j, i:i + 8, :])]
                acc = v if acc is None else [p + q for p, q in zip(acc, v)]
            sums = jnp.dot(_mxu(jnp.concatenate(
                [ones_w[:, :128] if j % 2 == 0 else sch.tie(ones_w[:, :128], prev),
                 ones_w[:, 128:]], axis=1)),
                           _mxu(x_v.bitcast(I32)[j, 0:D // 2]), preferred_element_type=F32)
            s2 = prev = acc[0] + acc[1]
            for d in (4, 2, 1):
                s2 = s2 + pltpu.roll(s2, d, 0)
            st_v[j, 0], st_v[j, 1] = _ln_scalars(jnp.broadcast_to(sums[0:1], (8, 128)), s2)

    def middle_stage(b, r, sch):
        src = [v[b % len(v)] for v in ab]
        scale = lambda v, f: [(x[0] * f, x[1] * f) for x in v]
        for h in range(2):
            ra = _ds(16 * r + 8 * h, 8)
            ld = lambda q, w, ra=ra: [(src[w][q, k, 0, ra, :], src[w][q, k, 1, ra, :]) for k in range(4)]

            park_v = half_v[2 * (sch.slot % 2) + h]

            def put(q, y):
                x = [park_v[n + sch.zero] for n in range(8)]
                for k in range(4):
                    for p in range(2):
                        cc[b % 2][k, q, p, ra, :] = x[2 * k + p] + y[k][p]
                        cc[b % 2][k, q + 2, p, ra, :] = x[2 * k + p] - y[k][p]

            def park(x):
                for k in range(4):
                    for p in range(2):
                        park_v[2 * k + p] = x[k][p]
                return [park_v[sch.zero]]

            gate = sch.start
            a0, a2, b0, b2 = ld(0, 0), ld(2, 0), ld(0, 1), ld(2, 1)
            a0[0] = (gate(a0[0][0]), a0[0][1])
            e0 = _prod_mod_1(list(map(_cadd, a0, a2)), list(map(_cadd, b0, b2)))
            again = _ds(16 * (r + sch.zero) + 8 * h, 8)
            yield park(e0)
            a0, a2, b0, b2 = (ld(q, w, again) for w in range(2) for q in (0, 2))
            a2[0] = (gate(a2[0][0]), a2[0][1])
            e2 = _prod_mod_m1(list(map(_csub, a0, a2)), scale(map(_csub, b0, b2), 2.0))
            put(0, e2)
            yield [cc[b % 2][0, 0, 0, again, :]]
            four = sch.start(jnp.full((8, 128), 4.0, F32))
            e1 = _prod_mod_i(ld(1, 0), scale(ld(1, 1), four), 1)
            yield park(e1)
            four = sch.start(jnp.full((8, 128), 4.0, F32))
            e3 = _prod_mod_i(ld(3, 0), scale(ld(3, 1), four), -1)
            put(1, e3)
            yield [cc[b % 2][0, 1, 0, again, :]]

    def inverse_stage(b, k, sch):
        src = cc[b % 2]

        def lhs(v, n, first):
            return sch.lhs(jnp.concatenate(
                [_pack(pk_v.at[sch.slot, 2], 4 * n + i // 16, v[i:i + 8], v[i + 8:i + 16])
                 for i in range(0, MB, 16)], axis=0), first)

        for o in range(2):
            p0, p1 = [(src[k, q, 0, 0:MB], src[k, q, 1, 0:MB]) for q in (2 * o, 2 * o + 1)]
            if o == 0:
                e = {0: _cadd(p0, p1), 2: _csub(p0, p1)}
            else:
                e = {1: (p0[0] + p1[1], p0[1] - p1[0]), 3: (p0[0] - p1[1], p0[1] + p1[0])}
            ys = []
            for n in e:
                y = [jnp.dot(lhs(e[n][p], 2 * n + p, n == o and p == 0),
                             _mxu(wt_w[4 * k + (0, 2, 1, 3)[n], p, 0:64]),
                             preferred_element_type=F32)
                     for p in range(2)]
                h = y[0] + y[1] + _mxu(xr[b % 4][4 * k + n, 0:MB // 2]).astype(F32)
                h_v[k + 4 * n, b * MB:b * MB + MB, :] = h.astype(BF16)
                hh = h * h
                sq_v[k + 4 * n] += sum((hh[i:i + 8] for i in range(8, MB, 8)), hh[0:8])
                ys.append(h)
            sch.results(ys[-1])
            yield []

    def sum_stage(b, r, sch):
        for n in range(4):
            s = r + 4 * n if b == nb - 1 else 4 * r + n
            sums = jnp.dot(sch.lhs(wy_v.bitcast(I32)[b], n == 0)[:, :MB],
                           _mxu(h_v.bitcast(I32)[s, b * MB // 2:(b + 1) * MB // 2]),
                           preferred_element_type=F32)
            acc_v[s] += sums[0:8]
        sch.results(sums)
        yield []

    nb = D // MB
    stages = dict(
        s=(seed_stage, 0), t=(table_stage, 1), k=(kernel_stage, 2),
        F=(functools.partial(forward_stage, 1), 3), n=(norm_stage, 2),
        f=(functools.partial(forward_stage, 0), 3), m=(middle_stage, 4),
        i=(inverse_stage, 5), a=(sum_stage, 6))

    def run(step, zero, live=None):
        live = live or {n: (f, step - lag) for n, (f, lag) in stages.items()
                        if 0 <= step - lag < nb and (n, step) != ("n", 2)}
        if step == nb + 4:
            live["z"] = (sum_stage, nb - 1)
        unroll, plan = PLANS["".join(live)]

        def body(it, carry):
            sch = _Schedule(zero >> (step % 32) if unroll == 4 else zero & it, idx_v)
            gens = [{n: f(b, it * unroll + u, sch) for n, (f, b) in live.items()}
                    for u in range(unroll)]
            if step == 3:
                for i in range(9 * unroll):
                    for cp in cp_w(9 * unroll * it + i):
                        cp.start()
            for item in plan.split():
                u, n, *ties = item.split(":")
                if n in live:
                    sch.slot = int(u)
                    sch.run(gens[int(u)][n], *map(int, ties or (-1, -1)))
            for sch.slot, g in enumerate(gens):
                for v in g.values():
                    for _ in v:
                        pass
            return carry + it

        if unroll == 4:
            if step == 101 or step > nb + 3:
                return body(0, 0)
            return jax.lax.fori_loop(zero, 1, lambda _, c: body(0, c), 0)
        return jax.lax.fori_loop(0, 4 // unroll, body, 0)

    _init_index(idx_v)
    acc_v[...] = sq_v[...] = jnp.zeros(acc_v.shape, F32)
    zero = run(0, 0) - 1
    for step in range(1, nb + 5):
        if step == 7:
            cp_d.start()
        if step == 4:
            for cp in cp_par[1]:
                cp.wait()
        if step == 3:
            for half in range(2):
                tiles = range(NT // 2 * half, NT // 2 * (half + 1))
                for j in tiles:
                    cp_x[j].wait()
                if not half:
                    for cp in cp_par[1]:
                        cp.start()
                _transpose_dft(wt_v, w_v, range(4 + 6 * half, 10 + 6 * half))
                stats(tiles, _Schedule(zero, idx_v))
            for q in range(2):
                for s, v in enumerate(_to_residues([st_v[j, q] for j in range(NT)],
                                                   _Schedule(zero, idx_v))):
                    st_v[s, q] = v
            run(101, zero, dict(n=(norm_stage, 0)))
        run(step, zero)

    sums = [acc_v[s] for s in range(16)]
    m2, inv2 = _ln_scalars(
        jnp.concatenate([v[0:1] for v in sums], axis=0),
        jnp.concatenate([jnp.sum(sq_v[j], axis=0, keepdims=True) for j in range(NT)], axis=0))
    wsum = jnp.sum(wr_v[...].astype(F32).reshape(1, D), axis=1, keepdims=True)
    score = _rbf((jnp.concatenate([v[1:2] for v in sums], axis=0) - m2 * wsum) * inv2 + 0.0)
    bits = pltpu.bitcast(score, I32) >> 16
    order = jnp.where(bits < 0, -1 - bits, bits + 32768)
    mu = (_iota((NT, 128), 1) - _iota((NT, 128), 0)) & 127
    pos = 128 * (mu & 15) + 16 * (mu >> 4) + _iota((NT, 128), 0)
    key = pltpu.bitcast((order << 11) + (L - 1 - pos) + (1 << 29), F32)

    h_w, out_w = h_v.bitcast(I32), out_v.bitcast(I32)
    sch, done = _Schedule(zero, idx_v), []
    tie = sch.tie

    def unrouted():
        for q, v in enumerate((1.0 + inv2, m2 * inv2)):
            for j, t in enumerate(_to_time(
                    [jnp.broadcast_to(v[s:s + 1], (8, 128)) for s in range(16)], sch)):
                st_v[j, q] = t
        for i in range(0, D, 16):
            scal = st_v.at[pl.ds(zero * (i + 1), NT)]
            tiles = [h_w[s, i // 2:i // 2 + 8, :] for s in range(16)]
            if len(done) > LAG:
                tiles[0] = tie(tiles[0], done[-LAG])
            for j, v in enumerate(_to_time(tiles, sch)):
                h, mul, sub = _mxu(v).astype(F32), scal[j, 0], scal[j, 1]
                out_v[j, i:i + 16, :] = jnp.concatenate(
                    [h[0:8] * mul - sub, h[8:16] * mul - sub], axis=0).astype(BF16)
                if j % 8 == 7:
                    yield pltpu.bitcast(out_w[j + zero, i // 2:i // 2 + 8, :], F32)

    side = unrouted()

    lane8, sub8 = _iota((CAP, 128), 1), _iota((CAP, 128), 0)
    best = _top8([pltpu.roll(key[i:i + 8], n, 1) if n else key[i:i + 8]
                  for i in (0, 8) for n in range(8)])
    cand = best[0]
    for c in range(1, CAP):
        cand = jnp.where(sub8 == c, best[c], cand)
    best = _top8([pltpu.roll(cand, n, 1) if n else cand for n in range(0, 128, 8)])
    for _ in range(2 * EARLY):
        best[-1] = tie(best[-1], next(side))
    best = [pltpu.bitcast(v, I32)[0, 0] for v in best]
    picks = [L - 1 - (v & (L - 1)) for v in best]

    def schedule(col):
        rnd = [sum([(col[e] == col[c]).astype(I32) for e in range(c)], 0) for c in range(CAP)]
        return (rnd, functools.reduce(jnp.maximum, rnd) + 1,
                lambda n: [lane8 == jnp.where(rnd[c] == n, col[c], -1) for c in range(CAP)])

    _, rounds, lanes = schedule([((t >> 7) + (t & 127)) & 127 for t in picks])

    def out_copy(q, lo, hi):
        j = order[q]
        return pltpu.make_async_copy(
            out_v.at[j, lo:hi], out_hbm.at[lo:hi, _ds(j * 128, 128)], sem_o)

    for n, ref in enumerate((wg_v, wu_v)):
        pltpu.make_async_copy(ref.at[:, 0:D], ref.at[:, 0:D], sem_w.at[n]).wait()

    def gather(n, acc):
        masks = lanes(n)
        tiles = []
        for i in range(0, D // 2, 8):
            v = jnp.zeros((8, 128), I32)
            for c in range(CAP):
                v = jnp.where(masks[c], h_w[picks[c] & 15, i:i + 8, :], v)
            tiles.append(v)
        lhs = jnp.zeros((CAP, 128), F32)
        for c in range(CAP):
            lhs = jnp.where(masks[c] & (sub8 == c), 1.0, lhs)
        aux = [jnp.zeros((CAP, 128), F32)] * 3
        for c in range(CAP):
            hit = pltpu.bitcast(key, I32) == best[c]
            aux = [jnp.where(sub8 == c, jnp.sum(jnp.where(hit, v, 0.0), axis=0, keepdims=True), a)
                   for a, v in zip(aux, (m2, inv2, score))]
        return (acc[0] + jax.lax.dot_general(lhs.astype(BF16), _mxu(jnp.concatenate(tiles, axis=0)),
                                             NT_DIMS, preferred_element_type=F32),
                *[jnp.sum(a, axis=1, keepdims=True) for a in aux])

    h_sel, m_sel, inv_sel, score_sel = jax.lax.fori_loop(
        0, rounds, gather, (jnp.zeros((CAP, D), F32), *[jnp.zeros((CAP, 1), F32)] * 3))
    x_sel = _rbf((h_sel - m_sel) * inv_sel)
    gate = _rbf(jax.nn.sigmoid(score_sel))

    tile, col = [t >> 7 for t in picks], [t & 127 for t in picks]
    rnd, rounds, lanes = schedule(col)
    routed = functools.reduce(jnp.bitwise_or, [1 << j for j in tile])
    spare = CAP - sum((routed >> j) & 1 for j in range(NT))
    n_late = 0
    for j in range(NT):
        hit = (routed >> j) & 1
        fill = (1 - hit) & (spare > 0).astype(I32)
        spare = spare - fill
        order_s[jnp.clip(jnp.where(hit + fill == 1, CAP + n_late, j - n_late), 0, NT - 1)] = j
        n_late = n_late + hit + fill

    order = [order_s[q] for q in range(NT)]

    def early_copies(n):
        lo, hi = (0, 16 * EARLY, MID, D)[n:n + 2]
        return [out_copy(q, lo, hi) for q in range(CAP)]

    def start(copies):
        for cp in copies:
            cp.start()

    start(early_copies(0))
    rate, sent = MID // 8 - 2 * EARLY, [0]

    def project(w_ref):
        parts = []
        for n in range(0, FF // 128, 4):
            for lo in range(0, D, 128):
                hi = min(lo + 128, D)
                xs = x_sel[:, lo:hi]
                if hi - lo == 128 and min(rate, (len(done) - 4) * rate // 70) > sent[0]:
                    sent[0] += 1
                    xs = tie(xs, next(side))
                w = [w_ref.bitcast(I32)[i, lo // 2:hi // 2, :] for i in range(n, n + 4)]
                v = jnp.dot(xs.astype(BF16), _mxu(jnp.concatenate(w, axis=1)),
                            preferred_element_type=F32)
                done.append(v[:, 0:128])
                acc = acc + v if lo else v
            parts.append(acc)
        return _rbf(jnp.concatenate(parts, axis=1))

    g = project(wg_v)
    act = _rbf(g * jax.nn.sigmoid(g)) * project(wu_v)
    for _ in range(rate - sent[0]):
        next(side)
    done.clear()

    cp_d.wait()

    start(early_copies(1))
    rest_side = list(side)

    def placed(r, words):
        idx = jnp.zeros((CAP, 128), I32)
        for c, m in enumerate(lanes(r)):
            idx = jnp.where(m, c, idx)
        return [_gather(w, idx) for w in words]

    def late_copies(lo, hi):
        return [out_copy(CAP + q, lo, hi) for q in range(CAP)]

    def words_of(n):
        return [new_v[n].bitcast(I32)[i:i + 8, :] for i in range(0, new_v[n].shape[0] // 2, 8)]

    tokens = []
    for n, (lo, hi) in enumerate(ROW_CHUNKS):
        a = [act[:, i:i + 128] for i in range(0, FF, 128)]
        for i, token in enumerate(rest_side):
            at = 8 + i * SPAN // len(rest_side) - n * len(a)
            if 0 <= at < len(a):
                a[at] = tie(a[at], token)
        if n == 1:
            start(early_copies(2))
        if n >= 2:
            cut = 12 * 128 // (hi - lo)
            a[cut] = tie(a[cut], tokens[n - 2])
        a = jnp.concatenate(a, axis=1)
        y = _rbf(jax.lax.dot_general(a.astype(BF16), wd_v[lo:hi, :], NT_DIMS,
                                     preferred_element_type=F32))
        new = h_sel[:, lo:hi] + _rbf(x_sel[:, lo:hi] + _rbf(y * gate))
        new_v[n][...] = jnp.concatenate(
            [new.T, jnp.zeros((hi - lo, 128 - CAP), F32)], axis=1).astype(BF16)
        rows = range(lo // 2, hi // 2, 8)
        words = words_of(n)
        both = list(zip(rows, placed(0, words), placed(1, words)))
        for c in range(CAP):
            for i, v0, v1 in both:
                pltpu.store(out_w.at[tile[c], pl.ds(i, 8), :],
                            jnp.where(rnd[c] == 0, v0, v1), mask=lane8 == col[c])
        for cp in late_copies(lo, hi):
            cp.start()
        out_w[tile[0], D // 2:, :] = lane8
        tokens.append(pltpu.bitcast(out_w[tile[0] | zero, D // 2:, :], F32))
    pltpu.make_async_copy(out_v.at[:, 0:D], out_v.at[:, 0:D], sem_o).wait()

    @pl.when(rounds > 2)
    def _():
        def fix(r, carry):
            rows = range(0, D // 2, 8)
            vals = placed(r, sum(map(words_of, range(len(new_v))), []))
            for c, m in enumerate(lanes(r)):
                for i, v in zip(rows, vals):
                    pltpu.store(out_w.at[tile[c], pl.ds(i, 8), :], v, mask=m)
            return carry

        jax.lax.fori_loop(2, rounds, fix, 0)
        for cp in late_copies(0, D):
            cp.start()
        for cp in late_copies(0, D):
            cp.wait()


@jax.jit
def pallas_sequential_preLN__ssm_conv_s4__moe_arch_mod__prompt_kernel(
    A_u: jax.Array,
    A_A_re: jax.Array,
    A_A_im: jax.Array,
    A_B_re: jax.Array,
    A_B_im: jax.Array,
    A_C_re: jax.Array,
    A_C_im: jax.Array,
    A_log_dt: jax.Array,
    A_Dskip: jax.Array,
    B_x: jax.Array,
    B_w_r: jax.Array,
    B_w_gate: jax.Array,
    B_w_up: jax.Array,
    B_w_down: jax.Array,
):
    del B_x
    hbm = pl.BlockSpec(memory_space=pl.ANY)
    out = pl.pallas_call(
        _kernel,
        out_shape=jax.ShapeDtypeStruct((D, L), BF16),
        in_specs=[hbm] * 13,
        out_specs=hbm,
        scratch_shapes=[
            pltpu.VMEM((NT, D + 16, 128), BF16),
            *[pltpu.VMEM((FF // 128, D + 16, 128), BF16)] * 2,
            pltpu.VMEM((D, FF), BF16),
            pltpu.VMEM((6, D, N), BF16),
            *[pltpu.VMEM((D,), BF16)] * 3,
            *[pltpu.VMEM((2, 16, 144, 128), BF16)] * 2,
            pltpu.VMEM((16, 2, 72, 128), I32),
            pltpu.VMEM((2, D, 128), F32),
            pltpu.VMEM((16, D), BF16),
            pltpu.VMEM((D // MB, 16, 128), BF16),
            pltpu.VMEM((2, 256, 128), F32),
            pltpu.VMEM((len(INDEX), 8, 128), I32),
            pltpu.VMEM((4, 3, 32, 16, 128), BF16),
            pltpu.VMEM((NT, D + 16, 128), BF16),
            pltpu.VMEM((NT, 2, 8, 128), F32),
            *[pltpu.VMEM((NT, 8, 128), F32)] * 2,
            pltpu.VMEM((NT, D + 16, 128), BF16),
            *[pltpu.VMEM((4, 4, 10, 8, 128), F32)] * 2,
            *[pltpu.VMEM((4, 4, 2, 112, 128), BF16)] * 2,
            *[pltpu.VMEM((4, 4, 2, 144, 128), BF16)] * 2,
            *[pltpu.VMEM((4, 8, 128), I32)] * 2,
            *[pltpu.VMEM((16, MB + 16, 128), BF16)] * 2,
            *[pltpu.VMEM((16, MB // 2 + 8, 128), I32)] * 2,
            *[pltpu.VMEM((4, 4, 2, MB + 8, 128), F32)] * 2,
            *[pltpu.VMEM((4, 4, 2, MB + 8, 128), F32)] * 2,
            *[pltpu.VMEM((16, MB // 2 + 8, 128), I32)] * 4,
            pltpu.SMEM((NT,), I32),
            pltpu.SemaphoreType.DMA((15,)),
            pltpu.SemaphoreType.DMA((NT,)),
            pltpu.SemaphoreType.DMA((3,)),
            pltpu.SemaphoreType.DMA,
            *[pltpu.VMEM((4, 4, 2, MB + 8, 128), F32)] * 2,
            *[pltpu.VMEM((8, 8, 128), F32)] * 4,
            *[pltpu.VMEM((hi - lo, 128), BF16) for lo, hi in ROW_CHUNKS],
        ],
        compiler_params=pltpu.CompilerParams(vmem_limit_bytes=100 * 1024 * 1024,
                                             disable_bounds_checks=True,
                                             disable_semaphore_checks=True),
    )(A_u.reshape(L, D).T, A_A_re, A_A_im, A_B_re, A_B_im, A_C_re, A_C_im,
      A_log_dt, A_Dskip, B_w_r, B_w_gate, B_w_up, B_w_down.T)
    return out.T.reshape(1, L, D)
```

```python
import functools

import numpy as np
import jax
import jax.numpy as jnp
import jax.experimental.pallas as pl
import jax.experimental.pallas.tpu as pltpu

F32 = jnp.float32
BF16 = jnp.bfloat16
I32 = jnp.int32

L = 2048
D = 576
N = 128
FF = 4608
CAP = 8
NT = L // 128
EPS = 1e-5
MB = 64
PLANS = dict(
    s=(2, ""),
    st=(2, ""),
    n=(4, ""),
    stk=(2, "0:t:-1:4 1:t:-1:3 0:t:-1:4 0:t:-1:7 0:t:-1:15 1:t:-1:10 1:t:6:16 1:t:11:21 0:k "
            "0:k 1:k 0:s:-1:20 0:s:11:23 0:k:-1:23 1:k 1:s:20:-1 1:s 1:k "),
    stkFnf=(4, "1:t:-1:1 0:s:-1:13 0:s:-1:34 1:s:-1:36 1:s:-1:54 2:s:-1:73 3:s:-1:94 0:f "
               "0:n:1:19 0:F 0:t:4:25 0:t:0:19 0:k 0:k 0:k:-1:38 0:t:15:39 0:F 0:f 1:f "
               "1:t:29:43 1:F 1:n:33:47 1:k 1:t:38:55 1:k 1:t:42:57 1:k:-1:61 0:t:44:56 "
               "3:t:47:61 1:F 1:f 2:f 2:n:57:76 2:F 2:t:60:82 2:t:53:76 2:k 2:k 2:s:73:91 "
               "2:k:-1:92 2:t:73:95 2:F 2:f 3:f 3:t:85:100 3:F 3:n:89:104 3:k 3:s:95:111 "
               "3:t:94:-1 3:k 3:t:100:-1 3:k 2:t:100:110 3:F 3:f "),
    stkFnfm=(4, "0:m:-1:2 0:m:-1:5 0:t:-1:7 0:t:-1:14 0:t:-1:12 0:f 0:m:3:13 0:m:-1:18 0:f "
                "0:m:6:21 0:m:6:20 0:k 0:t:8:25 0:n:9:27 1:m:13:30 0:k 0:s:16:33 0:m:15:33 "
                "0:m:13:25 0:k:-1:33 0:s:19:33 1:m:18:33 0:F 1:t:20:35 0:F 1:t:27:42 1:t:24:40 "
                "1:f 1:f 1:m:32:42 1:m:31:46 1:m:34:49 1:m:34:48 1:k 1:t:37:50 1:n:37:55 "
                "2:m:41:58 1:k 1:s:44:61 1:m:43:61 1:m:41:53 1:k:-1:61 1:s:47:61 2:m:43:61 1:F "
                "2:t:48:65 1:F 2:t:55:70 2:t:50:68 2:f 2:f 2:m:60:70 2:m:60:78 2:m:62:77 "
                "2:m:62:76 2:k 2:t:66:78 2:n:65:85 3:m:69:86 2:k 2:s:72:89 2:m:71:89 2:m:69:81 "
                "2:k:-1:92 2:s:75:89 3:m:74:88 2:F 3:t:76:91 2:F 3:t:83:98 3:t:78:96 3:f 3:f "
                "3:m:88:98 3:m:87:102 3:m:90:105 3:m:90:104 3:k 3:t:93:108 3:n:94:110 3:k "
                "3:s:100:-1 3:m:99:-1 3:m:94:106 3:k 3:F 3:s:105:-1 3:F "),
    stkFnfmi=(4, "0:t:-1:2 0:n:-1:8 0:t:-1:3 0:m:-1:4 0:m:-1:7 0:m:-1:19 0:s:-1:40 1:s:-1:76 "
                 "2:s:-1:112 3:s 0:f 0:m:0:13 0:k 0:s:4:33 0:k 0:m:13:23 0:k:-1:33 0:m:14:25 "
                 "0:t:14:32 0:f 0:t:18:33 0:F 1:t:23:40 0:F 1:n:26:47 1:t:24:38 1:m:27:41 0:i "
                 "1:m:29:47 0:i 0:m:32:40 0:m:31:44 1:m:33:54 1:f 1:m:36:51 1:k 1:s:40:71 1:k "
                 "1:m:49:61 1:k:-1:71 1:m:51:63 1:f 1:t:55:76 1:t:51:68 1:F 2:t:59:74 "
                 "2:t:59:75 1:F 2:m:63:76 2:m:63:79 1:i 2:n:64:80 1:i 1:m:68:76 1:m:67:78 2:f "
                 "2:m:72:91 2:m:71:84 2:k 2:s:76:105 2:k 2:m:83:95 2:k:-1:105 2:m:86:97 "
                 "2:t:86:105 2:f 2:t:90:105 2:F 3:t:94:112 2:F 3:t:96:110 3:m:99:113 2:i "
                 "3:n:101:119 3:m:101:119 2:i 2:m:104:112 2:m:103:116 3:f 3:m:108:126 "
                 "3:m:110:123 3:k 3:s:112:143 3:k 3:m:121:133 3:k:-1:142 3:m:123:135 3:f "
                 "3:t:127:-1 3:t:123:140 3:F 3:F 3:i 3:m:139:-1 3:m:139:-1 3:i "),
    stkFnfmia=(4, "0:t:-1:6 0:t:-1:2 0:n:-1:10 0:m:-1:6 0:m:-1:6 0:m:-1:19 0:s:-1:40 1:s:-1:77 "
                  "2:s:-1:114 3:s 0:a 0:f 0:m:1:18 0:k 0:s:5:40 0:k 0:m:15:27 0:m:-1:26 "
                  "0:k:-1:40 0:t:16:30 0:f 0:t:18:34 0:F 0:F 1:t:25:43 1:t:23:41 1:n:28:47 "
                  "1:m:25:43 1:m:27:44 0:i 0:m:32:40 0:i 0:m:34:42 1:a 1:f 1:m:38:56 1:m:36:55 "
                  "1:k 1:s:42:77 1:k 1:m:52:64 1:m:48:66 1:k:-1:77 1:t:53:67 1:f 1:t:55:71 1:F "
                  "1:F 2:t:64:80 2:t:60:78 2:n:65:84 2:m:62:80 2:m:64:81 1:i 1:m:69:77 1:i "
                  "1:m:71:81 2:m:73:93 2:a 2:f 2:m:75:92 2:k 2:s:79:114 2:k 2:m:89:101 "
                  "2:m:85:103 2:k:-1:114 2:t:90:104 2:f 2:t:92:108 2:F 2:F 3:t:99:117 "
                  "3:t:97:115 3:m:99:117 3:m:101:118 2:i 2:m:106:114 3:n:103:121 2:i "
                  "2:m:108:116 3:a 3:f 3:m:112:130 3:m:112:129 3:k 3:s:116:-1 3:k 3:m:126:138 "
                  "3:m:122:140 3:k:-1:147 3:t:127:141 3:f 3:t:129:-1 3:F 3:F 3:i 3:m:143:-1 "
                  "3:i 3:m:145:-1 "),
    tkFnfmia=(4, "0:t:-1:10 0:t:-1:5 0:n:-1:9 0:m:-1:6 0:m:-1:6 0:f 0:a 0:k 0:m:7:18 0:m:1:23 "
                 "0:k 0:m:15:28 0:m:-1:27 0:k:-1:36 0:f 0:t:17:33 0:t:20:38 0:F 0:F 1:n:28:46 "
                 "1:m:27:43 0:i 0:m:31:39 1:t:31:47 1:t:23:42 1:m:30:43 0:i 0:m:34:44 1:f 1:a "
                 "1:k 1:m:44:55 1:m:38:58 1:k 1:m:52:65 1:m:50:64 1:k:-1:73 1:f 1:t:54:70 "
                 "1:t:57:75 1:F 1:F 2:n:65:83 2:m:64:80 1:i 1:m:68:76 2:t:68:84 2:t:61:80 "
                 "2:m:69:80 1:i 1:m:71:79 2:f 2:a 2:k 2:m:81:92 2:m:75:97 2:k 2:m:89:102 "
                 "2:m:87:101 2:t:90:107 2:k:-1:108 2:f 2:t:94:112 2:F 2:F 3:m:101:117 "
                 "3:n:102:120 2:i 2:m:106:114 3:t:105:121 3:t:97:116 3:m:104:118 2:i "
                 "2:m:108:116 3:f 3:a 3:k 3:m:118:129 3:m:109:131 3:k 3:m:126:139 3:m:124:138 "
                 "3:k:-1:147 3:f 3:t:128:144 3:t:131:-1 3:F 3:F 3:i 3:m:143:-1 3:i 3:m:145:-1 "),
    kFnfmia=(4, "1:m:-1:5 1:m:-1:3 0:n:-1:12 0:F 0:m:2:14 0:m:-1:15 0:a 0:F 0:m:7:21 0:k "
                "0:m:9:27 0:m:13:23 0:k 0:m:15:25 0:m:18:31 0:m:20:32 0:k:-1:45 0:i 0:i 0:f "
                "0:f 1:n:36:50 1:F 1:a 1:F 1:m:42:57 1:m:34:56 1:k 1:m:47:64 1:k 1:m:53:66 "
                "1:k:-1:75 1:i 1:i 3:m:63:79 3:m:61:77 1:f 1:m:68:76 1:f 1:m:73:81 2:n:70:86 "
                "2:F 2:m:76:88 2:m:73:89 2:a 2:F 2:m:79:93 2:k 2:m:83:101 2:m:87:97 2:k "
                "2:m:89:101 2:k:-1:119 2:i 2:m:95:105 2:m:90:106 2:i 2:f 2:f 3:n:110:124 3:F "
                "3:a 3:F 3:m:116:130 3:m:111:134 3:k 3:m:121:141 3:m:124:141 3:k 3:k 3:i 3:i "
                "3:f 3:m:142:-1 3:f 3:m:145:-1 "),
    Ffmia=(4, "1:m:-1:9 0:m:-1:5 0:m:-1:10 0:m:-1:12 0:a 0:F 1:m:4:15 0:i 0:m:6:18 0:i "
              "0:m:9:22 0:F 1:m:16:31 0:f 0:m:20:33 0:f 0:m:22:33 1:a 1:m:25:43 1:F 0:m:29:41 "
              "1:i 1:i 1:m:37:50 1:F 1:m:40:54 1:f 1:m:42:57 1:m:45:56 3:m:45:59 2:m:42:58 1:f "
              "2:a 2:F 2:m:53:63 2:m:49:65 3:m:54:68 2:i 2:m:56:67 2:i 2:m:59:75 2:F 3:m:66:83 "
              "2:f 2:m:70:83 2:f 2:m:72:84 3:a 3:m:75:93 3:F 2:m:79:95 3:i 3:i 3:m:85:-1 3:F "
              "3:m:90:-1 3:f 3:m:92:-1 3:m:95:-1 3:f "),
    mia=(4, "1:m:-1:3 0:m:-1:8 0:m:-1:6 0:m:-1:7 0:m:-1:8 0:i 1:m:0:13 0:m:2:10 0:a 0:i "
            "1:m:5:16 2:m:8:25 1:i 1:m:9:22 0:m:10:23 0:m:8:20 1:m:8:20 3:m:11:25 1:a "
            "2:m:13:27 1:i 1:m:14:22 1:m:17:25 0:m:14:22 1:m:17:25 2:m:14:28 2:m:13:27 2:i "
            "3:m:18:32 2:m:20:32 2:a 2:i 3:m:23:-1 3:m:25:-1 3:m:25:-1 3:i 2:m:28:-1 2:m:27:-1 "
            "3:a 3:i 3:m:32:-1 3:m:35:-1 2:m:33:-1 3:m:35:-1 "),
    iaz=(4, "0:i 0:i 1:i 1:i 0:z 2:i 2:i 1:z 3:i 3:i 2:z 0:a 1:a 2:a 3:a 3:z"),
)
ROW_CHUNKS = ((0, 128), (128, 256), (256, 384), (384, 512), (512, D))
LAG = 16
MID, SPAN, EARLY = 384, 50, 8
NT_DIMS = (((1,), (1,)), ((), ()))


def _round_res(step):
    return [int(np.round(r / step)) * step for r in range(16)]


RES1, RES2, RES3 = _round_res(2), _round_res(4), _round_res(8)


def _ds(start, size):
    return pl.ds(start if isinstance(start, int) else pl.multiple_of(start, size), size)


def _iota(shape, dim):
    return jax.lax.broadcasted_iota(I32, shape, dim)


def _rbf(x):
    return x.astype(BF16).astype(F32)


def _cmul(a, b):
    return (a[0] * b[0] - a[1] * b[1], a[0] * b[1] + a[1] * b[0])


def _csq(a):
    t = a[0] * a[1]
    return ((a[0] + a[1]) * (a[0] - a[1]), t + t)


def _cadd(a, b):
    return (a[0] + b[0], a[1] + b[1])


def _csub(a, b):
    return (a[0] - b[0], a[1] - b[1])


def _bfly4(a0, a1, a2, a3, inverse=False):
    s02, d02 = _cadd(a0, a2), _csub(a0, a2)
    s13, d13 = _cadd(a1, a3), _csub(a1, a3)
    p = (d02[0] - d13[1], d02[1] + d13[0])
    m = (d02[0] + d13[1], d02[1] - d13[0])
    if inverse:
        p, m = m, p
    return _cadd(s02, s13), p, _csub(s02, s13), m


def _prod_mod_1(a, b):
    fa, fb = _bfly4(*a), _bfly4(*b)
    return _bfly4(*[_cmul(x, y) for x, y in zip(fa, fb)], inverse=True)


def _prod2(a0, a1, b0, b1, sgn):
    p00, p11 = _cmul(a0, b0), _cmul(a1, b1)
    c1 = _cadd(_cmul(a0, b1), _cmul(a1, b0))
    if sgn > 0:
        return (p00[0] - p11[1], p00[1] + p11[0]), c1
    return (p00[0] + p11[1], p00[1] - p11[0]), c1


def _prod_mod_m1(a, b):
    def split(x):
        p = [(x[k][0] - x[k + 2][1], x[k][1] + x[k + 2][0]) for k in range(2)]
        m = [(x[k][0] + x[k + 2][1], x[k][1] - x[k + 2][0]) for k in range(2)]
        return p, m
    ap, am = split(a)
    bp, bm = split(b)
    cp = _prod2(*ap, *bp, 1)
    cm = _prod2(*am, *bm, -1)
    lo = [_cadd(cp[k], cm[k]) for k in range(2)]
    hi = [(cp[k][1] - cm[k][1], cm[k][0] - cp[k][0]) for k in range(2)]
    return lo + hi


def _prod_mod_i(a, b, sgn):
    sm = [x[0] + x[1] for x in b]
    df = [x[1] - x[0] for x in b]
    asum = [x[0] + x[1] for x in a]
    out = []
    for k in range(4):
        acc = [None, None, None]
        for j in range(4):
            m = (k - j) % 4
            if j <= k:
                t = ((b[m][0], 1), (df[m], 1), (sm[m], 1))
            elif sgn > 0:
                t = ((b[m][1], -1), (sm[m], 1), (df[m], -1))
            else:
                t = ((b[m][1], 1), (sm[m], -1), (df[m], 1))
            for q, (v, (w, s)) in enumerate(zip((asum[j], a[j][0], a[j][1]), t)):
                p = v * w
                if acc[q] is None:
                    acc[q] = p
                else:
                    acc[q] = acc[q] + p if s > 0 else acc[q] - p
        out.append((acc[0] - acc[2], acc[0] + acc[1]))
    return out


def _barrel(v, sch):
    for bit in range(4):
        m = sch.mask("bit%d" % bit)
        v = [jnp.where(m, v[(i + (1 << bit)) % 16], v[i]) for i in range(16)]
    return [v[-s % 16] for s in range(16)]


def _to_residues(tiles, sch):
    return _barrel([t if j == 0 else pltpu.roll(t, j, 1) for j, t in enumerate(tiles)], sch)


def _to_time(res, sch):
    return [t if j == 0 else pltpu.roll(t, 128 - j, 1)
            for j, t in enumerate(_barrel(res, sch))]


def _gather(x, idx, axis=1):
    return jnp.take_along_axis(x, idx, axis=axis, mode="promise_in_bounds")


def _transpose_dft(wt_ref, wu_ref, residues):
    for s in residues:
        for p in range(2):
            wt_ref[4 * (s % 4) + (0, 2, 1, 3)[s // 4], p, 0:64] = pltpu.bitcast(
                _mxu(wu_ref.bitcast(I32)[p, 4 * (s % 4) + s // 4, 0:64]).T, I32)


def _init_dft(wu_ref, wk_ref, tmp_ref, halfway):
    sub, k4 = _iota((8, 128), 0), 4 * _iota((8, 128), 1) + 1

    def cis(t):
        ph = ((k4 * t) & (4 * L - 1)).astype(F32) * (2 * np.pi / (4 * L))
        return jnp.cos(ph), jnp.sin(ph)

    w1, w16 = cis(1), cis(16)
    w32 = _csq(w16)
    fk = [cis(16 * (32 * (sub & 3) + (sub >> 2)))]
    fu = [cis(128 * sub), cis(128 * (sub + 8))]
    for v in range(1, 16):
        fk.append(_cmul(fk[-1], w32))
        if v >= 2:
            fu.append(_cmul(fu[-2], w16))
    for p in range(2):
        for v in range(32):
            tmp_ref[p, 8 * v:8 * v + 8, :] = fu[v % 16][p]
    tw = None
    for s in range(16):
        for v in range(0, 16, 2):
            rows = [slice(128 - s + 8 * i, 136 - s + 8 * i) for i in (v, v + 1)]
            for ref, f in ((wk_ref, fk[v:v + 2]),
                           (wu_ref, [(tmp_ref[0, r, :], tmp_ref[1, r, :]) for r in rows])):
                if s:
                    f = [_cmul(x, tw) for x in f]
                for p in range(2):
                    ref[p, 4 * (s % 4) + s // 4, 8 * v:8 * v + 16, :] = jnp.concatenate(
                        [f[0][p], f[1][p]], axis=0).astype(BF16)
        tw = _cmul(tw, w1) if s else w1
        if s == 7:
            halfway()


def _pack(ref, n, a, b):
    ref[n] = jnp.concatenate([a, b], axis=0).astype(BF16)
    return ref.bitcast(I32)[n]


def _split(w):
    return [pltpu.bitcast(w << 16, F32), pltpu.bitcast(w & -65536, F32)]


FINE = (0, 1, 2, 3, 4, 5, 6, 7, 512, 516, 1024, 1536)


def _k_seeds(z, c, sch):
    pw = {1: z}
    for e in range(1, 10):
        pw[1 << e] = _csq(pw[1 << (e - 1)])
    c8, z16 = _cmul(c, pw[8]), (pw[16][0], 0.0 - pw[16][1])
    pair = lambda a, b: tuple(jnp.where(sch.mask("odd"), q, p) for p, q in zip(a, b))
    seeds = []
    for g in range(2):
        twice = lambda v: tuple(_gather(x, sch.idx("dup%d" % g), 0) for x in v)
        seeds.append([twice(z), twice(pw[32]), twice(pw[512]),
                      pair(twice(c), twice(c8)), pair((1.0, 0.0), twice(z16))])
    return seeds


def _mxu(words):
    return pltpu.bitcast(words, BF16)


def _store_table(ref, tab):
    for i in range(0, len(tab), 2):
        for p in range(2):
            ref[p, 8 * i:8 * i + 16, :] = jnp.concatenate(
                [tab[i][p], tab[i + 1][p]], axis=0).astype(BF16)


def _k_residues(groups, k_last, dskip, tmp_ref, sch):
    idx, nxt = sch.idx("src"), sch.idx("nxt")
    low = lambda x, y: (x & 65535) | (y << 16)
    high = lambda x, y: jax.lax.shift_right_logical(x, 16) | (y & -65536)
    kv, up = {}, {}
    for i, k in enumerate(FINE):
        v = [g[8 * i:8 * i + 8] for g in groups]
        if k == 0:
            v = [x + jnp.where(sch.mask("diag"),
                               _gather(dskip[n // 2], sch.idx("dup%d" % (n % 2)), 0), 0.0)
                 for n, x in enumerate(v)]
        p = [_pack(tmp_ref, 2 * i + h, v[2 * h], v[2 * h + 1]) for h in range(2)]
        both = [_gather(x, idx) for x in p]
        kv[k], kv[k + 8] = low(*both), high(*both)
        if k % 512 == 0:
            up[k] = low(*[_gather(x, nxt) for x in p])
    k_last = _gather(k_last, sch.idx("rows"), 0)
    q0, q1, q2, up0, up01, up2, up3, fine = map(sch.mask, INDEX[-8:])
    s3 = {r: jnp.where(q2, kv[1024 + r], kv[1536 + r]) for r in (0, 8)}
    v0 = jnp.where(q0, kv[0], jnp.where(q1, kv[512], s3[0]))
    v16 = jnp.where(up01, jnp.where(up0, up[0], up[512]),
                    jnp.where(up2, up[1024], jnp.where(up3, up[1536], k_last)))
    s3[16] = v16
    s23, s123, out = {}, {}, [v0]
    for r in range(1, 16):
        k23 = (RES2[r], RES3[r])
        if k23 not in s23:
            s23[k23] = v16 if k23 == (16, 16) else jnp.where(q1, kv[512 + k23[0]], s3[k23[1]])
        k123 = (RES1[r],) + k23
        if k123 not in s123:
            s123[k123] = v16 if k123[0] == 16 else jnp.where(q0, kv[k123[0]], s23[k23])
        if RES1[r] == r:
            out.append(s123[k123])
        else:
            out.append(jnp.where(fine, kv[r], s123[k123]))
    return out


def _ln_scalars(s1, s2):
    mean = s1 * (1.0 / D)
    var = jnp.maximum(s2 * (1.0 / D) - mean * mean, 0.0)
    eps = float(np.asarray(EPS, dtype=BF16))
    sd = _rbf(jnp.sqrt(_rbf(_rbf(var) + eps)))
    return _rbf(mean), 1.0 / sd


def _top8(x):
    def swap(v, pairs):
        for i, j in pairs:
            v[i], v[j] = jnp.maximum(v[i], v[j]), jnp.minimum(v[i], v[j])
        return v

    def merge(a, b):
        v = [jnp.maximum(a[i], b[7 - i]) for i in range(8)]
        return swap(v, [(i, i + d) for d in (4, 2, 1) for i in range(8) if not i & d])

    sort8 = ((0, 2), (1, 3), (4, 6), (5, 7), (0, 4), (1, 5), (2, 6), (3, 7), (0, 1), (2, 3),
             (4, 5), (6, 7), (2, 4), (3, 5), (1, 4), (3, 6), (1, 2), (3, 4), (5, 6))
    v = merge(*[swap(x[i:i + 8], sort8) for i in (0, 8)])
    for d in (4, 2, 1):
        v = merge(v, [pltpu.roll(t, d, 0) for t in v])
    return v


def _init_columns(col_ref, wx_ref, wy_ref, ldt_ref, dsk_ref, wr_ref):
    row, lane = _iota((128, 128), 0), _iota((128, 128), 1)
    split = (row & ~15) + 2 * (row & 7) + ((row >> 3) & 1)
    ldt, dsk, wr = (ref[...].astype(F32).reshape(1, D) for ref in (ldt_ref, dsk_ref, wr_ref))
    for n, vec in enumerate((jnp.exp(ldt), dsk * (1.0 / L))):
        for lo in range(0, D, 128):
            i = min(lo, D - 128)
            diag = jnp.where(split == lane, vec[:, i:i + 128], 0.0)[lo - i:].astype(BF16)
            col_ref[n, lo:i + 128, :] = jnp.dot(diag, jnp.ones((128, 128), BF16),
                                                preferred_element_type=F32)
    sub = _iota((16, D), 0)
    ones_w = jnp.where(sub == 0, 1.0, jnp.where(sub == 1, wr, 0.0))
    wx_ref[...] = ones_w.astype(BF16)
    for lo in range(0, D, MB):
        wy_ref[lo // MB, :, 0:MB] = ones_w[:, lo:lo + MB].astype(BF16)
        wy_ref[lo // MB, :, MB:] = jnp.zeros((16, 128 - MB), BF16)


INDEX = ("true", "bit0", "bit1", "bit2", "bit3", "odd", "dup0", "dup1", "rows", "src", "nxt",
         "diag", "q0", "q1", "q2", "up0", "up01", "up2", "up3", "fine")


def _init_index(idx_ref):
    sub, lane = _iota((8, 128), 0), _iota((8, 128), 1)
    src = lambda b: 8 * ((b >> 1) & 15) + 2 * (sub & 3) + (b & 1)
    is_ = lambda m: jnp.where(m, 1, 0)
    q = lane & 3
    q16 = q + is_(lane >= 124)
    tiles = dict(true=sub + 1, odd=sub & 1, dup0=sub >> 1, dup1=4 + (sub >> 1),
                 rows=2 * (sub & 3) + (sub >> 2), src=src(lane >> 2), nxt=src((lane >> 2) + 1),
                 diag=is_((lane == sub) & ((sub & 1) == 0)), up01=is_(q16 < 2),
                 fine=is_((q == 0) & (lane < 64)),
                 **{"bit%d" % n: (lane >> n) & 1 for n in range(4)},
                 **{"q%d" % n: is_(q == n) for n in range(3)},
                 **{"up%d" % n: is_(q16 == n) for n in (0, 2, 3)})
    for n, name in enumerate(INDEX):
        idx_ref[n] = tiles[name]


class _Schedule:
    def __init__(self, zero, idx_ref):
        self.zero = zero
        self.idx = lambda name: idx_ref[INDEX.index(name) + zero]
        self.mask = lambda name: self.idx(name) != 0
        self.true = self.mask("true")
        self.done, self.pending, self.wait = [], {}, -1

    def tie(self, x, token):
        return jnp.where(self.true, x, token if token.dtype == x.dtype
                         else pltpu.bitcast(token, x.dtype))

    def start(self, x):
        return self.tie(x, self.done[self.wait]) if 0 <= self.wait < len(self.done) else x

    def lhs(self, words, first):
        tiles = [words[i:i + 8] for i in range(0, words.shape[0], 8)]
        for i in range(len(tiles) if first else 0):
            for token in self.pending.pop(len(self.done) + i, ()):
                tiles[i] = self.tie(tiles[i], token)
        return _mxu(jnp.concatenate(tiles, axis=0))

    def results(self, v):
        self.done += [v[i + 8:i + 16] for i in range(0, v.shape[0], 16)]

    def run(self, stage, wait, before):
        self.wait = wait
        self.pending.setdefault(before, []).extend(next(stage))


def _kernel(x_hbm, are_hbm, aim_hbm, bre_hbm, bim_hbm, cre_hbm, cim_hbm,
            ldt_hbm, dsk_hbm, wr_hbm, wg_hbm, wu_hbm, wd_hbm, out_hbm,
            x_v, wg_v, wu_v, wd_v, par_v, ldt_v, dsk_v, wr_v, w_v, wk_v, wt_v, col_v, wx_v, wy_v,
            tmp_v, idx_v, pk_v, h_v, st_v, acc_v, sq_v, out_v, sd0, sd1, ta0, ta1, tb0, tb1, kl0, kl1,
            u0, u1, k0, k1, a0_v, a1_v, c0, c1, r0, r1, r2, r3,
            sem_p, sem_x, sem_w, sem_o, f0_v, f1_v, *rest):
    half_v, new_v = rest[:4], rest[4:]
    cp_vec = [pltpu.make_async_copy(s, d, sem_p.at[n]) for n, (s, d) in enumerate(
        ((ldt_hbm, ldt_v), (dsk_hbm, dsk_v), (wr_hbm, wr_v)))]
    cp_par = [[pltpu.make_async_copy(s.at[lo:hi], par_v.at[n, lo:hi], sem_p.at[3 + 6 * m + n])
               for n, s in enumerate((are_hbm, aim_hbm, bre_hbm, bim_hbm, cre_hbm, cim_hbm))]
              for m, (lo, hi) in enumerate(((0, 4 * MB), (4 * MB, D)))]
    cp_x = [pltpu.make_async_copy(x_hbm.at[:, 128 * j:128 * j + 128], x_v.at[j, 0:D],
                                  sem_x.at[j])
            for j in range(NT)]
    cp_d = pltpu.make_async_copy(wd_hbm, wd_v, sem_w.at[2])

    def cp_w(i):
        return [pltpu.make_async_copy(s.at[:, _ds(128 * i, 128)], d.at[i, 0:D], sem_w.at[n])
                for n, (s, d) in enumerate(((wg_hbm, wg_v), (wu_hbm, wu_v)))]

    for cp in cp_vec + cp_par[0]:
        cp.start()
    for cp in cp_x[:NT // 2]:
        cp.start(priority=1)

    def columns():
        for cp in cp_vec:
            cp.wait()
        for cp in cp_x[NT // 2:]:
            cp.start(priority=1)
        _transpose_dft(wt_v, w_v, range(4))
        _init_columns(col_v, wx_v, wy_v, ldt_v, dsk_v, wr_v)

    _init_dft(w_v, wk_v, tmp_v, columns)
    for cp in cp_par[0]:
        cp.wait()

    sd, ta, tb, kl = (sd0, sd1), (ta0, ta1), (tb0, tb1), (kl0, kl1)
    uk, ab, cc, xr = ((u0, u1), (k0, k1)), ((a0_v, a1_v), (f0_v, f1_v)), (c0, c1), (r0, r1, r2, r3)
    ww, wt_w = (w_v.bitcast(I32), wk_v.bitcast(I32)), wt_v

    def chan(b, r):
        return _ds(b * MB + 16 * r, 16)

    def seed_stage(b, r, sch):
        rows = _ds(b * MB // 2 + 8 * r, 8)
        par = [_split(par_v.bitcast(I32)[n, rows, :]) for n in range(6)]
        for h in range(2):
            a_re, a_im, b_re, b_im, c_re, c_im = [v[h] for v in par]
            dt = sch.start(col_v[0, _ds(b * MB + 16 * r + 8 * h, 8), :])
            mag, ang = jnp.exp(dt * a_re), dt * a_im
            sc = dt * (1.0 / L)
            seeds = _k_seeds((mag * jnp.cos(ang), mag * jnp.sin(ang)),
                             _cmul((c_re, c_im), (sc * b_re, sc * b_im)), sch)
            for g in range(2):
                for n, v in enumerate(seeds[g]):
                    for p in range(2):
                        sd[b % 2][r, 2 * h + g, 2 * n + p] = v[p]
            yield [sd[b % 2][(r + sch.zero), 2 * h, 0]]

    def table_stage(b, r, sch):
        tail = []
        for g in range(4):
            m1, m32, m512, a0, b0 = [
                (sd[b % 2][r, g, 2 * n], sd[b % 2][r, g, 2 * n + 1]) for n in range(5)]
            m32 = (sch.start(m32[0]), m32[1])
            fa = [a0]
            for _ in range(7):
                fa.append(_cmul(fa[-1], m1))
            for src in (0, 4, 8, 10):
                fa.append(_cmul(fa[src], m512))
            tail.append(fa[11][0] * m512[0] - fa[11][1] * m512[1])
            _store_table(ta[b % 2].at[r, g], fa)
            fb = [b0]
            for _ in range(15):
                p = fb[-1]
                fb.append((p[0] * m32[0] + p[1] * m32[1], p[1] * m32[0] - p[0] * m32[1]))
            _store_table(tb[b % 2].at[r, g], fb)
            yield [ta[b % 2].bitcast(I32)[(r + sch.zero), g, 0, 0:8, :],
                   tb[b % 2].bitcast(I32)[(r + sch.zero), g, 0, 0:8, :]]
        last = [jnp.where(sch.mask("odd"), pltpu.roll(tail[h + 1], 1, 0), tail[h])
                for h in (0, 2)]
        last = [pltpu.bitcast(_rbf(jnp.broadcast_to(jnp.sum(v, axis=1, keepdims=True),
                                                    (8, 128))), I32) for v in last]
        kl[b % 2][r] = jax.lax.shift_right_logical(last[0], 16) | last[1]

    def kernel_stage(b, r, sch):
        ta_w, tb_w = ta[b % 2].bitcast(I32), tb[b % 2].bitcast(I32)
        groups = [None] * 4
        for g0 in (0, 2):
            res = [jax.lax.dot_general(sch.lhs(ta_w[r, g, p, 0:48], g == g0 and p == 0),
                                       _mxu(tb_w[r, g, p, 0:64]), NT_DIMS, preferred_element_type=F32)
                   for g in (g0, g0 + 1) for p in range(2)]
            groups[g0], groups[g0 + 1] = res[0] + res[1], res[2] + res[3]
            sch.results(groups[g0 + 1])
            yield []
        dskip = [col_v[1, _ds(b * MB + 16 * r + 8 * h, 8), :] for h in range(2)]
        dst = _ds(8 * r, 8)
        res = _k_residues(groups, kl[b % 2][r], dskip, pk_v.at[sch.slot, 0], sch)
        for s, t in enumerate(res):
            uk[1][b % 2][4 * (s % 4) + s // 4, dst, :] = t
        yield [uk[1][b % 2][0, _ds(8 * (r + sch.zero), 8), :]]

    def norm_stage(b, r, sch):
        rows, dst = _ds(b * MB // 2 + 8 * r, 8), _ds(8 * r, 8)
        tiles = [x_v.bitcast(I32)[j, rows, :] for j in range(NT)]
        for s, t in enumerate(_to_residues([sch.start(tiles[0])] + tiles[1:], sch)):
            xr[b % 4][4 * (s % 4) + s // 4, dst, :] = t
            xs, m, inv = _mxu(t).astype(F32), st_v[s, 0], st_v[s, 1]
            uk[0][b % 2][4 * (s % 4) + s // 4, _ds(16 * r, 16), :] = jnp.concatenate(
                [(xs[0:8] - m) * inv, (xs[8:16] - m) * inv], axis=0).astype(BF16)
        yield [uk[0][b % 2].bitcast(I32)[0, _ds(8 * (r + sch.zero), 8), :]]

    def forward_stage(w, b, k, sch):
        dst = ab[w][b % len(ab[w])]
        for p in range(2):
            v = [jnp.dot(sch.lhs((uk[w][b % 2] if w else uk[w][b % 2].bitcast(I32))[
                4 * k + n, 0:MB // 2], n == 0),
                         _mxu(ww[w][p ^ (n & 1), 4 * k + n, 0:64]),
                         preferred_element_type=F32) for n in range(4)]
            d02, d13 = v[0] - v[2], v[1] - v[3]
            x1 = d02 - d13 if p == 0 else d02 + d13
            dst[0, k, p, 0:MB] = v[0] + v[2]
            dst[2, k, 1 - p, 0:MB] = v[1] + v[3]
            dst[1, k, p, 0:MB] = x1
            dst[3, k, p, 0:MB] = d02 + d13 if p == 0 else d02 - d13
            sch.results(x1)
            yield []

    def stats(tiles, sch):
        ones_w = wx_v.bitcast(I32)[...]
        for j in tiles:
            acc = None
            for i in range(0, D // 2, 8):
                v = [t * t for t in _split(x_v.bitcast(I32)[j, i:i + 8, :])]
                acc = v if acc is None else [p + q for p, q in zip(acc, v)]
            sums = jnp.dot(_mxu(jnp.concatenate(
                [ones_w[:, :128] if j % 2 == 0 else sch.tie(ones_w[:, :128], prev),
                 ones_w[:, 128:]], axis=1)),
                           _mxu(x_v.bitcast(I32)[j, 0:D // 2]), preferred_element_type=F32)
            s2 = prev = acc[0] + acc[1]
            for d in (4, 2, 1):
                s2 = s2 + pltpu.roll(s2, d, 0)
            st_v[j, 0], st_v[j, 1] = _ln_scalars(jnp.broadcast_to(sums[0:1], (8, 128)), s2)

    def middle_stage(b, r, sch):
        src = [v[b % len(v)] for v in ab]
        scale = lambda v, f: [(x[0] * f, x[1] * f) for x in v]
        for h in range(2):
            ra = _ds(16 * r + 8 * h, 8)
            ld = lambda q, w, ra=ra: [(src[w][q, k, 0, ra, :], src[w][q, k, 1, ra, :]) for k in range(4)]

            park_v = half_v[2 * (sch.slot % 2) + h]

            def put(q, y):
                x = [park_v[n + sch.zero] for n in range(8)]
                for k in range(4):
                    for p in range(2):
                        cc[b % 2][k, q, p, ra, :] = x[2 * k + p] + y[k][p]
                        cc[b % 2][k, q + 2, p, ra, :] = x[2 * k + p] - y[k][p]

            def park(x):
                for k in range(4):
                    for p in range(2):
                        park_v[2 * k + p] = x[k][p]
                return [park_v[sch.zero]]

            gate = sch.start
            a0, a2, b0, b2 = ld(0, 0), ld(2, 0), ld(0, 1), ld(2, 1)
            a0[0] = (gate(a0[0][0]), a0[0][1])
            e0 = _prod_mod_1(list(map(_cadd, a0, a2)), list(map(_cadd, b0, b2)))
            again = _ds(16 * (r + sch.zero) + 8 * h, 8)
            yield park(e0)
            a0, a2, b0, b2 = (ld(q, w, again) for w in range(2) for q in (0, 2))
            a2[0] = (gate(a2[0][0]), a2[0][1])
            e2 = _prod_mod_m1(list(map(_csub, a0, a2)), scale(map(_csub, b0, b2), 2.0))
            put(0, e2)
            yield [cc[b % 2][0, 0, 0, again, :]]
            four = sch.start(jnp.full((8, 128), 4.0, F32))
            e1 = _prod_mod_i(ld(1, 0), scale(ld(1, 1), four), 1)
            yield park(e1)
            four = sch.start(jnp.full((8, 128), 4.0, F32))
            e3 = _prod_mod_i(ld(3, 0), scale(ld(3, 1), four), -1)
            put(1, e3)
            yield [cc[b % 2][0, 1, 0, again, :]]

    def inverse_stage(b, k, sch):
        src = cc[b % 2]

        def lhs(v, n, first):
            return sch.lhs(jnp.concatenate(
                [_pack(pk_v.at[sch.slot, 2], 4 * n + i // 16, v[i:i + 8], v[i + 8:i + 16])
                 for i in range(0, MB, 16)], axis=0), first)

        for o in range(2):
            p0, p1 = [(src[k, q, 0, 0:MB], src[k, q, 1, 0:MB]) for q in (2 * o, 2 * o + 1)]
            if o == 0:
                e = {0: _cadd(p0, p1), 2: _csub(p0, p1)}
            else:
                e = {1: (p0[0] + p1[1], p0[1] - p1[0]), 3: (p0[0] - p1[1], p0[1] + p1[0])}
            ys = []
            for n in e:
                y = [jnp.dot(lhs(e[n][p], 2 * n + p, n == o and p == 0),
                             _mxu(wt_w[4 * k + (0, 2, 1, 3)[n], p, 0:64]),
                             preferred_element_type=F32)
                     for p in range(2)]
                h = y[0] + y[1] + _mxu(xr[b % 4][4 * k + n, 0:MB // 2]).astype(F32)
                h_v[k + 4 * n, b * MB:b * MB + MB, :] = h.astype(BF16)
                hh = h * h
                sq_v[k + 4 * n] += sum((hh[i:i + 8] for i in range(8, MB, 8)), hh[0:8])
                ys.append(h)
            sch.results(ys[-1])
            yield []

    def sum_stage(b, r, sch):
        for n in range(4):
            s = r + 4 * n if b == nb - 1 else 4 * r + n
            sums = jnp.dot(sch.lhs(wy_v.bitcast(I32)[b], n == 0)[:, :MB],
                           _mxu(h_v.bitcast(I32)[s, b * MB // 2:(b + 1) * MB // 2]),
                           preferred_element_type=F32)
            acc_v[s] += sums[0:8]
        sch.results(sums)
        yield []

    nb = D // MB
    stages = dict(
        s=(seed_stage, 0), t=(table_stage, 1), k=(kernel_stage, 2),
        F=(functools.partial(forward_stage, 1), 3), n=(norm_stage, 2),
        f=(functools.partial(forward_stage, 0), 3), m=(middle_stage, 4),
        i=(inverse_stage, 5), a=(sum_stage, 6))

    def run(step, zero, live=None):
        live = live or {n: (f, step - lag) for n, (f, lag) in stages.items()
                        if 0 <= step - lag < nb and (n, step) != ("n", 2)}
        if step == nb + 4:
            live["z"] = (sum_stage, nb - 1)
        unroll, plan = PLANS["".join(live)]

        def body(it, carry):
            sch = _Schedule(zero >> (step % 32) if unroll == 4 else zero & it, idx_v)
            gens = [{n: f(b, it * unroll + u, sch) for n, (f, b) in live.items()}
                    for u in range(unroll)]
            if step == 3:
                for i in range(9 * unroll):
                    for cp in cp_w(9 * unroll * it + i):
                        cp.start()
            for item in plan.split():
                u, n, *ties = item.split(":")
                if n in live:
                    sch.slot = int(u)
                    sch.run(gens[int(u)][n], *map(int, ties or (-1, -1)))
            for sch.slot, g in enumerate(gens):
                for v in g.values():
                    for _ in v:
                        pass
            return carry + it

        if unroll == 4:
            if step == 101 or step > nb + 3:
                return body(0, 0)
            return jax.lax.fori_loop(zero, 1, lambda _, c: body(0, c), 0)
        return jax.lax.fori_loop(0, 4 // unroll, body, 0)

    _init_index(idx_v)
    acc_v[...] = sq_v[...] = jnp.zeros(acc_v.shape, F32)
    zero = run(0, 0) - 1
    for step in range(1, nb + 5):
        if step == 4:
            for cp in cp_par[1]:
                cp.wait()
        if step == 3:
            for half in range(2):
                tiles = range(NT // 2 * half, NT // 2 * (half + 1))
                for j in tiles:
                    cp_x[j].wait()
                if half:
                    cp_d.start(priority=1)
                else:
                    for cp in cp_par[1]:
                        cp.start()
                _transpose_dft(wt_v, w_v, range(4 + 6 * half, 10 + 6 * half))
                stats(tiles, _Schedule(zero, idx_v))
            for q in range(2):
                for s, v in enumerate(_to_residues([st_v[j, q] for j in range(NT)],
                                                   _Schedule(zero, idx_v))):
                    st_v[s, q] = v
            run(101, zero, dict(n=(norm_stage, 0)))
        run(step, zero)

    sums = [acc_v[s] for s in range(16)]
    m2, inv2 = _ln_scalars(
        jnp.concatenate([v[0:1] for v in sums], axis=0),
        jnp.concatenate([jnp.sum(sq_v[j], axis=0, keepdims=True) for j in range(NT)], axis=0))
    wsum = jnp.sum(wr_v[...].astype(F32).reshape(1, D), axis=1, keepdims=True)
    score = _rbf((jnp.concatenate([v[1:2] for v in sums], axis=0) - m2 * wsum) * inv2 + 0.0)
    bits = pltpu.bitcast(score, I32) >> 16
    order = jnp.where(bits < 0, -1 - bits, bits + 32768)
    mu = (_iota((NT, 128), 1) - _iota((NT, 128), 0)) & 127
    pos = 128 * (mu & 15) + 16 * (mu >> 4) + _iota((NT, 128), 0)
    key = pltpu.bitcast((order << 11) + (L - 1 - pos) + (1 << 29), F32)

    h_w, out_w = h_v.bitcast(I32), out_v.bitcast(I32)
    sch, done = _Schedule(zero, idx_v), []
    tie = sch.tie

    def unrouted():
        for q, v in enumerate((1.0 + inv2, m2 * inv2)):
            for j, t in enumerate(_to_time(
                    [jnp.broadcast_to(v[s:s + 1], (8, 128)) for s in range(16)], sch)):
                st_v[j, q] = t
        for i in range(0, D, 16):
            scal = st_v.at[pl.ds(zero * (i + 1), NT)]
            tiles = [h_w[s, i // 2:i // 2 + 8, :] for s in range(16)]
            if len(done) > LAG:
                tiles[0] = tie(tiles[0], done[-LAG])
            for j, v in enumerate(_to_time(tiles, sch)):
                h, mul, sub = _mxu(v).astype(F32), scal[j, 0], scal[j, 1]
                out_v[j, i:i + 16, :] = jnp.concatenate(
                    [h[0:8] * mul - sub, h[8:16] * mul - sub], axis=0).astype(BF16)
                if j % 8 == 7:
                    yield pltpu.bitcast(out_w[j + zero, i // 2:i // 2 + 8, :], F32)

    side = unrouted()

    lane8, sub8 = _iota((CAP, 128), 1), _iota((CAP, 128), 0)
    best = _top8([pltpu.roll(key[i:i + 8], n, 1) if n else key[i:i + 8]
                  for i in (0, 8) for n in range(8)])
    cand = best[0]
    for c in range(1, CAP):
        cand = jnp.where(sub8 == c, best[c], cand)
    best = _top8([pltpu.roll(cand, n, 1) if n else cand for n in range(0, 128, 8)])
    for _ in range(2 * EARLY):
        best[-1] = tie(best[-1], next(side))
    best = [pltpu.bitcast(v, I32)[0, 0] for v in best]
    picks = [L - 1 - (v & (L - 1)) for v in best]

    def schedule(col):
        rnd = [sum([(col[e] == col[c]).astype(I32) for e in range(c)], 0) for c in range(CAP)]
        return (rnd, functools.reduce(jnp.maximum, rnd) + 1,
                lambda n: [lane8 == jnp.where(rnd[c] == n, col[c], -1) for c in range(CAP)])

    _, rounds, lanes = schedule([((t >> 7) + (t & 127)) & 127 for t in picks])

    def out_copy(q, lo, hi):
        j = order[q]
        return pltpu.make_async_copy(
            out_v.at[j, lo:hi], out_hbm.at[lo:hi, _ds(j * 128, 128)], sem_o)

    for n, ref in enumerate((wg_v, wu_v)):
        pltpu.make_async_copy(ref.at[:, 0:D], ref.at[:, 0:D], sem_w.at[n]).wait()

    def gather(n, acc):
        masks = lanes(n)
        tiles = []
        for i in range(0, D // 2, 8):
            v = jnp.zeros((8, 128), I32)
            for c in range(CAP):
                v = jnp.where(masks[c], h_w[picks[c] & 15, i:i + 8, :], v)
            tiles.append(v)
        lhs = jnp.zeros((CAP, 128), F32)
        for c in range(CAP):
            lhs = jnp.where(masks[c] & (sub8 == c), 1.0, lhs)
        aux = [jnp.zeros((CAP, 128), F32)] * 3
        for c in range(CAP):
            hit = pltpu.bitcast(key, I32) == best[c]
            aux = [jnp.where(sub8 == c, jnp.sum(jnp.where(hit, v, 0.0), axis=0, keepdims=True), a)
                   for a, v in zip(aux, (m2, inv2, score))]
        return (acc[0] + jax.lax.dot_general(lhs.astype(BF16), _mxu(jnp.concatenate(tiles, axis=0)),
                                             NT_DIMS, preferred_element_type=F32),
                *[jnp.sum(a, axis=1, keepdims=True) for a in aux])

    h_sel, m_sel, inv_sel, score_sel = jax.lax.fori_loop(
        0, rounds, gather, (jnp.zeros((CAP, D), F32), *[jnp.zeros((CAP, 1), F32)] * 3))
    x_sel = _rbf((h_sel - m_sel) * inv_sel)
    gate = _rbf(jax.nn.sigmoid(score_sel))

    tile, col = [t >> 7 for t in picks], [t & 127 for t in picks]
    rnd, rounds, lanes = schedule(col)
    late, again = 0, []
    for j in tile:
        again.append((late >> j) & 1)
        late = late | (1 << j)
    for dup in again[1:]:
        late = late | (late + dup)
    order = []
    for left in (late ^ ((1 << NT) - 1), late):
        for _ in range(CAP):
            order.append((31 - jax.lax.clz(left)) & (NT - 1))
            left = left ^ (1 << order[-1])

    def early_copies(n):
        lo, hi = (0, 16 * EARLY, MID, D)[n:n + 2]
        return [out_copy(q, lo, hi) for q in range(CAP)]

    def start(copies):
        for cp in copies:
            cp.start()

    start(early_copies(0))
    rate, sent = MID // 8 - 2 * EARLY, [0]

    def project(w_ref):
        parts = []
        for n in range(0, FF // 128, 4):
            for lo in range(0, D, 128):
                hi = min(lo + 128, D)
                xs = x_sel[:, lo:hi]
                if hi - lo == 128 and min(rate, (len(done) - 4) * rate // 70) > sent[0]:
                    sent[0] += 1
                    xs = tie(xs, next(side))
                w = [w_ref.bitcast(I32)[i, lo // 2:hi // 2, :] for i in range(n, n + 4)]
                v = jnp.dot(xs.astype(BF16), _mxu(jnp.concatenate(w, axis=1)),
                            preferred_element_type=F32)
                done.append(v[:, 0:128])
                acc = acc + v if lo else v
            parts.append(acc)
        return _rbf(jnp.concatenate(parts, axis=1))

    g = project(wg_v)
    act = _rbf(g * jax.nn.sigmoid(g)) * project(wu_v)
    for _ in range(rate - sent[0]):
        next(side)
    done.clear()

    cp_d.wait()

    start(early_copies(1))
    rest_side = list(side)

    def placed(r, words):
        idx = jnp.zeros((CAP, 128), I32)
        for c, m in enumerate(lanes(r)):
            idx = jnp.where(m, c, idx)
        return [_gather(w, idx) for w in words]

    def late_copies(lo, hi):
        return [out_copy(CAP + q, lo, hi) for q in range(CAP)]

    def words_of(n):
        return [new_v[n].bitcast(I32)[i:i + 8, :] for i in range(0, new_v[n].shape[0] // 2, 8)]

    tokens = []
    for n, (lo, hi) in enumerate(ROW_CHUNKS):
        a = [act[:, i:i + 128] for i in range(0, FF, 128)]
        for i, token in enumerate(rest_side):
            at = 8 + i * SPAN // len(rest_side) - n * len(a)
            if 0 <= at < len(a):
                a[at] = tie(a[at], token)
        if n == 1:
            start(early_copies(2))
        if n >= 2:
            cut = 12 * 128 // (hi - lo)
            a[cut] = tie(a[cut], tokens[n - 2])
        a = jnp.concatenate(a, axis=1)
        y = _rbf(jax.lax.dot_general(a.astype(BF16), wd_v[lo:hi, :], NT_DIMS,
                                     preferred_element_type=F32))
        new = h_sel[:, lo:hi] + _rbf(x_sel[:, lo:hi] + _rbf(y * gate))
        new_v[n][...] = jnp.concatenate(
            [new.T, jnp.zeros((hi - lo, 128 - CAP), F32)], axis=1).astype(BF16)
        rows = range(lo // 2, hi // 2, 8)
        words = words_of(n)
        both = list(zip(rows, placed(0, words), placed(1, words)))
        for c in range(CAP):
            for i, v0, v1 in both:
                pltpu.store(out_w.at[tile[c], pl.ds(i, 8), :],
                            jnp.where(rnd[c] == 0, v0, v1), mask=lane8 == col[c])
        for cp in late_copies(lo, hi):
            cp.start()
        out_w[tile[0], D // 2:, :] = lane8
        tokens.append(pltpu.bitcast(out_w[tile[0] | zero, D // 2:, :], F32))
    pltpu.make_async_copy(out_v.at[:, 0:D], out_v.at[:, 0:D], sem_o).wait()

    @pl.when(rounds > 2)
    def _():
        def fix(r, carry):
            rows = range(0, D // 2, 8)
            vals = placed(r, sum(map(words_of, range(len(new_v))), []))
            for c, m in enumerate(lanes(r)):
                for i, v in zip(rows, vals):
                    pltpu.store(out_w.at[tile[c], pl.ds(i, 8), :], v, mask=m)
            return carry

        jax.lax.fori_loop(2, rounds, fix, 0)
        for cp in late_copies(0, D):
            cp.start()
        for cp in late_copies(0, D):
            cp.wait()


@jax.jit
def pallas_sequential_preLN__ssm_conv_s4__moe_arch_mod__prompt_kernel(
    A_u: jax.Array,
    A_A_re: jax.Array,
    A_A_im: jax.Array,
    A_B_re: jax.Array,
    A_B_im: jax.Array,
    A_C_re: jax.Array,
    A_C_im: jax.Array,
    A_log_dt: jax.Array,
    A_Dskip: jax.Array,
    B_x: jax.Array,
    B_w_r: jax.Array,
    B_w_gate: jax.Array,
    B_w_up: jax.Array,
    B_w_down: jax.Array,
):
    del B_x
    hbm = pl.BlockSpec(memory_space=pl.ANY)
    out = pl.pallas_call(
        _kernel,
        out_shape=jax.ShapeDtypeStruct((D, L), BF16),
        in_specs=[hbm] * 13,
        out_specs=hbm,
        scratch_shapes=[
            pltpu.VMEM((NT, D + 16, 128), BF16),
            *[pltpu.VMEM((FF // 128, D + 16, 128), BF16)] * 2,
            pltpu.VMEM((D, FF), BF16),
            pltpu.VMEM((6, D, N), BF16),
            *[pltpu.VMEM((D,), BF16)] * 3,
            *[pltpu.VMEM((2, 16, 144, 128), BF16)] * 2,
            pltpu.VMEM((16, 2, 72, 128), I32),
            pltpu.VMEM((2, D, 128), F32),
            pltpu.VMEM((16, D), BF16),
            pltpu.VMEM((D // MB, 16, 128), BF16),
            pltpu.VMEM((2, 256, 128), F32),
            pltpu.VMEM((len(INDEX), 8, 128), I32),
            pltpu.VMEM((4, 3, 32, 16, 128), BF16),
            pltpu.VMEM((NT, D + 16, 128), BF16),
            pltpu.VMEM((NT, 2, 8, 128), F32),
            *[pltpu.VMEM((NT, 8, 128), F32)] * 2,
            pltpu.VMEM((NT, D + 16, 128), BF16),
            *[pltpu.VMEM((4, 4, 10, 8, 128), F32)] * 2,
            *[pltpu.VMEM((4, 4, 2, 112, 128), BF16)] * 2,
            *[pltpu.VMEM((4, 4, 2, 144, 128), BF16)] * 2,
            *[pltpu.VMEM((4, 8, 128), I32)] * 2,
            *[pltpu.VMEM((16, MB + 16, 128), BF16)] * 2,
            *[pltpu.VMEM((16, MB // 2 + 8, 128), I32)] * 2,
            *[pltpu.VMEM((4, 4, 2, MB + 8, 128), F32)] * 2,
            *[pltpu.VMEM((4, 4, 2, MB + 8, 128), F32)] * 2,
            *[pltpu.VMEM((16, MB // 2 + 8, 128), I32)] * 4,
            pltpu.SemaphoreType.DMA((15,)),
            pltpu.SemaphoreType.DMA((NT,)),
            pltpu.SemaphoreType.DMA((3,)),
            pltpu.SemaphoreType.DMA,
            *[pltpu.VMEM((4, 4, 2, MB + 8, 128), F32)] * 2,
            *[pltpu.VMEM((8, 8, 128), F32)] * 4,
            *[pltpu.VMEM((hi - lo, 128), BF16) for lo, hi in ROW_CHUNKS],
        ],
        compiler_params=pltpu.CompilerParams(vmem_limit_bytes=100 * 1024 * 1024,
                                             disable_bounds_checks=True,
                                             disable_semaphore_checks=True),
    )(A_u.reshape(L, D).T, A_A_re, A_A_im, A_B_re, A_B_im, A_C_re, A_C_im,
      A_log_dt, A_Dskip, B_w_r, B_w_gate, B_w_up, B_w_down.T)
    return out.T.reshape(1, L, D)
```

```python
import functools

import numpy as np
import jax
import jax.numpy as jnp
import jax.experimental.pallas as pl
import jax.experimental.pallas.tpu as pltpu

F32 = jnp.float32
BF16 = jnp.bfloat16
I32 = jnp.int32

L = 2048
D = 576
N = 128
FF = 4608
CAP = 8
NT = L // 128
EPS = 1e-5
MB = 64
PLANS = dict(
    s=(2, ""),
    st=(2, ""),
    n=(4, ""),
    stk=(2, "0:t:-1:4 1:t:-1:3 0:t:-1:4 0:t:-1:7 0:t:-1:15 1:t:-1:10 1:t:6:16 1:t:11:21 0:k "
            "0:k 1:k 0:s:-1:20 0:s:11:23 0:k:-1:23 1:k 1:s:20:-1 1:s 1:k "),
    stkFnf=(4, "1:t:-1:1 0:s:-1:9 0:s:-1:34 1:s:-1:35 1:s:-1:54 2:s:-1:69 3:s:-1:90 0:f "
               "0:n:1:19 0:F 0:t:4:25 0:t:0:19 0:k 0:t:12:43 0:k 0:k:-1:38 0:F 0:f 1:f "
               "1:t:29:44 1:F 1:n:33:47 1:t:35:58 1:k 1:k 1:t:42:57 1:k:-1:61 0:t:44:56 "
               "3:t:47:61 1:F 1:f 2:f 2:n:57:76 2:F 2:t:61:83 2:t:53:76 2:k 2:k 2:s:73:91 "
               "2:k:-1:92 2:t:70:98 2:F 2:f 3:f 3:t:85:100 3:F 3:n:89:104 3:t:91:-1 3:k "
               "3:s:95:111 3:k 3:t:98:110 3:k 2:t:100:110 3:F 3:f "),
    stkFnfm=(4, "0:m:-1:6 0:m:-1:5 0:t:-1:7 0:t:-1:14 0:t:-1:12 0:f 0:m:3:13 0:m:-1:18 "
                "0:m:3:18 0:f 0:m:6:20 0:k 0:t:8:25 0:n:9:27 0:m:13:33 0:m:13:25 1:m:12:34 0:k "
                "0:s:16:33 0:k:-1:35 0:s:19:33 1:m:18:33 0:F 1:t:20:35 0:F 1:t:27:42 1:t:24:40 "
                "1:f 1:f 1:m:32:42 1:m:31:46 1:m:31:46 1:m:34:48 1:k 1:t:37:50 1:n:37:55 "
                "2:m:39:62 1:k 1:s:44:61 1:m:43:61 1:m:41:53 1:k:-1:63 1:s:47:63 2:m:43:61 1:F "
                "2:t:48:63 1:F 2:t:55:70 2:t:50:68 2:f 2:f 2:m:60:70 2:m:60:78 2:m:59:71 "
                "2:m:62:76 2:k 2:t:66:78 2:n:65:85 2:k 2:s:72:89 2:m:71:89 2:m:69:81 2:k:-1:94 "
                "2:s:75:89 3:m:70:90 3:m:74:89 2:F 3:t:76:91 2:F 3:t:83:98 3:t:78:96 3:f 3:f "
                "3:m:88:98 3:m:87:102 3:m:87:102 3:m:90:104 3:k 3:t:93:108 3:n:94:110 3:k "
                "3:s:100:-1 3:m:99:-1 3:m:94:106 3:k 3:F 3:s:105:-1 3:F "),
    stkFnfmi=(4, "0:t:-1:2 0:n:-1:8 0:t:-1:3 0:m:-1:4 0:m:-1:7 0:m:-1:19 0:s:-1:40 1:s:-1:76 "
                 "2:s:-1:112 3:s 0:f 0:m:0:13 0:k 0:s:4:33 0:k 0:m:13:23 0:k:-1:33 0:m:14:25 "
                 "0:t:14:32 0:f 0:t:18:33 0:F 1:t:23:40 0:F 1:n:26:47 1:t:24:38 1:m:27:41 0:i "
                 "1:m:29:47 0:i 0:m:32:40 0:m:31:44 1:m:33:54 1:f 1:m:36:51 1:k 1:s:40:71 1:k "
                 "1:m:49:61 1:k:-1:71 1:m:51:63 1:f 1:t:55:76 1:t:51:68 1:F 2:t:59:74 "
                 "2:t:59:75 1:F 2:m:63:76 2:m:63:79 1:i 2:n:64:80 1:i 1:m:68:76 1:m:67:78 2:f "
                 "2:m:72:91 2:m:71:84 2:k 2:s:76:105 2:k 2:m:83:95 2:k:-1:105 2:m:86:97 "
                 "2:t:86:105 2:f 2:t:90:105 2:F 3:t:94:112 2:F 3:t:96:110 3:m:99:113 2:i "
                 "3:n:101:119 3:m:101:119 2:i 2:m:104:112 2:m:103:116 3:f 3:m:108:126 "
                 "3:m:110:123 3:k 3:s:112:143 3:k 3:m:121:133 3:k:-1:142 3:m:123:135 3:f "
                 "3:t:127:-1 3:t:123:140 3:F 3:F 3:i 3:m:139:-1 3:m:139:-1 3:i "),
    stkFnfmia=(4, "0:t:-1:6 0:t:-1:2 0:n:-1:10 0:m:-1:6 0:m:-1:6 0:m:-1:19 0:s:-1:40 1:s:-1:77 "
                  "2:s:-1:114 3:s 0:a 0:f 0:m:1:18 0:k 0:s:5:40 0:k 0:m:15:27 0:m:-1:26 "
                  "0:k:-1:40 0:t:16:30 0:f 0:t:18:34 0:F 0:F 1:t:25:43 1:t:23:41 1:n:28:47 "
                  "1:m:25:43 1:m:27:44 0:i 0:m:32:40 0:i 0:m:34:42 1:a 1:f 1:m:38:56 1:m:36:55 "
                  "1:k 1:s:42:77 1:k 1:m:52:64 1:m:48:66 1:k:-1:77 1:t:53:67 1:f 1:t:55:71 1:F "
                  "1:F 2:t:64:80 2:t:60:78 2:n:65:84 2:m:62:80 2:m:64:81 1:i 1:m:69:77 1:i "
                  "1:m:71:81 2:m:73:93 2:a 2:f 2:m:75:92 2:k 2:s:79:114 2:k 2:m:89:101 "
                  "2:m:85:103 2:k:-1:114 2:t:90:104 2:f 2:t:92:108 2:F 2:F 3:t:99:117 "
                  "3:t:97:115 3:m:99:117 3:m:101:118 2:i 2:m:106:114 3:n:103:121 2:i "
                  "2:m:108:116 3:a 3:f 3:m:112:130 3:m:112:129 3:k 3:s:116:-1 3:k 3:m:126:138 "
                  "3:m:122:140 3:k:-1:147 3:t:127:141 3:f 3:t:129:-1 3:F 3:F 3:i 3:m:143:-1 "
                  "3:i 3:m:145:-1 "),
    tkFnfmia=(4, "1:m:-1:5 1:m:-1:3 0:n:-1:12 0:t:-1:3 0:t:-1:15 0:t:-1:21 0:t:-1:28 1:t:-1:40 "
                 "1:t:-1:52 1:t:-1:58 1:t:-1:65 2:t:-1:77 2:t:-1:89 2:t:-1:95 2:t:-1:102 0:F "
                 "0:m:2:14 0:m:-1:15 0:a 0:F 0:m:7:20 0:k 0:m:9:27 0:m:13:23 0:k 0:m:15:25 "
                 "0:m:18:31 0:m:20:32 0:k:-1:45 0:i 0:i 0:f 0:f 1:n:36:50 1:F 1:a 1:F "
                 "1:m:42:56 1:m:34:56 1:k 1:m:47:64 1:k 1:m:53:68 1:k:-1:75 1:i 1:i 3:m:63:79 "
                 "3:m:61:77 1:f 1:m:68:76 1:f 1:m:73:81 2:n:70:86 2:F 2:m:76:88 2:m:73:89 2:a "
                 "2:F 2:m:79:92 2:k 2:m:83:101 2:m:87:97 2:k 2:m:89:101 2:k:-1:119 2:i "
                 "2:m:95:105 2:m:90:106 2:i 3:t:99:111 3:t:-1:126 3:t:-1:132 2:f 2:f "
                 "3:n:110:124 3:F 3:a 3:F 3:m:116:129 3:m:111:134 3:k 3:m:121:141 3:m:124:141 "
                 "3:t:125:139 3:k 3:k 3:i 3:i 3:f 3:m:142:-1 3:f 3:m:145:-1 "),
    kFnfmia=(4, "1:m:-1:5 1:m:-1:3 0:n:-1:12 0:F 0:m:2:14 0:m:-1:15 0:a 0:F 0:m:7:21 0:k "
                "0:m:9:27 0:m:13:23 0:k 0:m:15:25 0:m:18:31 0:m:20:32 0:k:-1:45 0:i 0:i 0:f "
                "0:f 1:n:36:50 1:F 1:a 1:F 1:m:42:57 1:m:34:56 1:k 1:m:47:64 1:k 1:m:53:66 "
                "1:k:-1:75 1:i 1:i 3:m:63:79 3:m:61:77 1:f 1:m:68:76 1:f 1:m:73:81 2:n:70:86 "
                "2:F 2:m:76:88 2:m:73:89 2:a 2:F 2:m:79:93 2:k 2:m:83:101 2:m:87:97 2:k "
                "2:m:89:101 2:k:-1:119 2:i 2:m:95:105 2:m:90:106 2:i 2:f 2:f 3:n:110:124 3:F "
                "3:a 3:F 3:m:116:130 3:m:111:134 3:k 3:m:121:141 3:m:124:141 3:k 3:k 3:i 3:i "
                "3:f 3:m:142:-1 3:f 3:m:145:-1 "),
    Ffmia=(4, "1:m:-1:9 0:m:-1:5 0:m:-1:10 0:m:-1:12 0:a 0:F 1:m:4:15 0:i 0:m:6:18 0:i "
              "0:m:9:22 0:F 1:m:16:31 0:f 0:m:20:33 0:f 0:m:22:33 1:a 1:m:25:43 1:F 0:m:29:41 "
              "1:i 1:i 1:m:37:50 1:F 1:m:40:54 1:f 1:m:42:57 1:m:45:56 3:m:45:59 2:m:42:58 1:f "
              "2:a 2:F 2:m:53:63 2:m:49:65 3:m:54:68 2:i 2:m:56:67 2:i 2:m:59:75 2:F 3:m:66:83 "
              "2:f 2:m:70:83 2:f 2:m:72:84 3:a 3:m:75:93 3:F 2:m:79:95 3:i 3:i 3:m:85:-1 3:F "
              "3:m:90:-1 3:f 3:m:92:-1 3:m:95:-1 3:f "),
    mia=(4, "1:m:-1:3 0:m:-1:8 0:m:-1:6 0:m:-1:7 0:m:-1:8 0:i 1:m:0:13 0:m:2:10 0:a 0:i "
            "1:m:5:16 2:m:8:25 1:i 1:m:9:22 0:m:10:23 0:m:8:20 1:m:8:20 3:m:11:25 1:a "
            "2:m:13:27 1:i 1:m:14:22 1:m:17:25 0:m:14:22 1:m:17:25 2:m:14:28 2:m:13:27 2:i "
            "3:m:18:32 2:m:20:32 2:a 2:i 3:m:23:-1 3:m:25:-1 3:m:25:-1 3:i 2:m:28:-1 2:m:27:-1 "
            "3:a 3:i 3:m:32:-1 3:m:35:-1 2:m:33:-1 3:m:35:-1 "),
    iaz=(4, "0:i 0:i 1:i 1:i 0:z 2:i 2:i 1:z 3:i 3:i 2:z 0:a 1:a 2:a 3:a 3:z"),
)
ROW_CHUNKS = ((0, 128), (128, 256), (256, 384), (384, 512), (512, D))
MID, SPAN, EARLY, LAG, CUT, END = 480, 30, 8, 16, 12, 76
NT_DIMS = (((1,), (1,)), ((), ()))


def _round_res(step):
    return [int(np.round(r / step)) * step for r in range(16)]


RES1, RES2, RES3 = _round_res(2), _round_res(4), _round_res(8)


def _ds(start, size):
    return pl.ds(start if isinstance(start, int) else pl.multiple_of(start, size), size)


def _iota(shape, dim):
    return jax.lax.broadcasted_iota(I32, shape, dim)


def _rbf(x):
    return x.astype(BF16).astype(F32)


def _cmul(a, b):
    return (a[0] * b[0] - a[1] * b[1], a[0] * b[1] + a[1] * b[0])


def _csq(a):
    t = a[0] * a[1]
    return ((a[0] + a[1]) * (a[0] - a[1]), t + t)


def _cadd(a, b):
    return (a[0] + b[0], a[1] + b[1])


def _csub(a, b):
    return (a[0] - b[0], a[1] - b[1])


def _bfly4(a0, a1, a2, a3, inverse=False):
    s02, d02 = _cadd(a0, a2), _csub(a0, a2)
    s13, d13 = _cadd(a1, a3), _csub(a1, a3)
    p = (d02[0] - d13[1], d02[1] + d13[0])
    m = (d02[0] + d13[1], d02[1] - d13[0])
    if inverse:
        p, m = m, p
    return _cadd(s02, s13), p, _csub(s02, s13), m


def _prod_mod_1(a, b):
    fa, fb = _bfly4(*a), _bfly4(*b)
    return _bfly4(*[_cmul(x, y) for x, y in zip(fa, fb)], inverse=True)


def _prod2(a0, a1, b0, b1, sgn):
    p00, p11 = _cmul(a0, b0), _cmul(a1, b1)
    c1 = _cadd(_cmul(a0, b1), _cmul(a1, b0))
    if sgn > 0:
        return (p00[0] - p11[1], p00[1] + p11[0]), c1
    return (p00[0] + p11[1], p00[1] - p11[0]), c1


def _prod_mod_m1(a, b):
    def split(x):
        p = [(x[k][0] - x[k + 2][1], x[k][1] + x[k + 2][0]) for k in range(2)]
        m = [(x[k][0] + x[k + 2][1], x[k][1] - x[k + 2][0]) for k in range(2)]
        return p, m
    ap, am = split(a)
    bp, bm = split(b)
    cp = _prod2(*ap, *bp, 1)
    cm = _prod2(*am, *bm, -1)
    lo = [_cadd(cp[k], cm[k]) for k in range(2)]
    hi = [(cp[k][1] - cm[k][1], cm[k][0] - cp[k][0]) for k in range(2)]
    return lo + hi


def _prod_mod_i(a, b, sgn):
    sm = [x[0] + x[1] for x in b]
    df = [x[1] - x[0] for x in b]
    asum = [x[0] + x[1] for x in a]
    out = []
    for k in range(4):
        acc = [None, None, None]
        for j in range(4):
            m = (k - j) % 4
            if j <= k:
                t = ((b[m][0], 1), (df[m], 1), (sm[m], 1))
            elif sgn > 0:
                t = ((b[m][1], -1), (sm[m], 1), (df[m], -1))
            else:
                t = ((b[m][1], 1), (sm[m], -1), (df[m], 1))
            for q, (v, (w, s)) in enumerate(zip((asum[j], a[j][0], a[j][1]), t)):
                p = v * w
                if acc[q] is None:
                    acc[q] = p
                else:
                    acc[q] = acc[q] + p if s > 0 else acc[q] - p
        out.append((acc[0] - acc[2], acc[0] + acc[1]))
    return out


def _barrel(v, sch):
    for bit in range(4):
        m = sch.mask("bit%d" % bit)
        v = [jnp.where(m, v[(i + (1 << bit)) % 16], v[i]) for i in range(16)]
    return [v[-s % 16] for s in range(16)]


def _to_residues(tiles, sch):
    return _barrel([t if j == 0 else pltpu.roll(t, j, 1) for j, t in enumerate(tiles)], sch)


def _to_time(res, sch):
    return [t if j == 0 else pltpu.roll(t, 128 - j, 1)
            for j, t in enumerate(_barrel(res, sch))]


def _gather(x, idx, axis=1):
    return jnp.take_along_axis(x, idx, axis=axis, mode="promise_in_bounds")


def _transpose_dft(wt_ref, wu_ref, residues):
    for s in residues:
        for p in range(2):
            wt_ref[4 * (s % 4) + (0, 2, 1, 3)[s // 4], p, 0:64] = pltpu.bitcast(
                _mxu(wu_ref.bitcast(I32)[p, 4 * (s % 4) + s // 4, 0:64]).T, I32)


def _init_dft(wu_ref, wk_ref, tmp_ref, halfway):
    sub, k4 = _iota((8, 128), 0), 4 * _iota((8, 128), 1) + 1

    def cis(t):
        ph = ((k4 * t) & (4 * L - 1)).astype(F32) * (2 * np.pi / (4 * L))
        return jnp.cos(ph), jnp.sin(ph)

    w1, w16 = cis(1), cis(16)
    w32 = _csq(w16)
    fk = [cis(16 * (32 * (sub & 3) + (sub >> 2)))]
    fu = [cis(128 * sub), cis(128 * (sub + 8))]
    for v in range(1, 16):
        fk.append(_cmul(fk[-1], w32))
        if v >= 2:
            fu.append(_cmul(fu[-2], w16))
    for p in range(2):
        for v in range(32):
            tmp_ref[p, 8 * v:8 * v + 8, :] = fu[v % 16][p]
    tw = None
    for s in range(16):
        for v in range(0, 16, 2):
            rows = [slice(128 - s + 8 * i, 136 - s + 8 * i) for i in (v, v + 1)]
            for ref, f in ((wk_ref, fk[v:v + 2]),
                           (wu_ref, [(tmp_ref[0, r, :], tmp_ref[1, r, :]) for r in rows])):
                if s:
                    f = [_cmul(x, tw) for x in f]
                for p in range(2):
                    ref[p, 4 * (s % 4) + s // 4, 8 * v:8 * v + 16, :] = jnp.concatenate(
                        [f[0][p], f[1][p]], axis=0).astype(BF16)
        tw = _cmul(tw, w1) if s else w1
        if s == 7:
            halfway()


def _pack(ref, n, a, b):
    ref[n] = jnp.concatenate([a, b], axis=0).astype(BF16)
    return ref.bitcast(I32)[n]


def _split(w):
    return [pltpu.bitcast(w << 16, F32), pltpu.bitcast(w & -65536, F32)]


FINE = (0, 1, 2, 3, 4, 5, 6, 7, 512, 516, 1024, 1536)


def _k_seeds(z, c, sch):
    pw = {1: z}
    for e in range(1, 10):
        pw[1 << e] = _csq(pw[1 << (e - 1)])
    c8, z16 = _cmul(c, pw[8]), (pw[16][0], 0.0 - pw[16][1])
    pair = lambda a, b: tuple(jnp.where(sch.mask("odd"), q, p) for p, q in zip(a, b))
    seeds = []
    for g in range(2):
        twice = lambda v: tuple(_gather(x, sch.idx("dup%d" % g), 0) for x in v)
        seeds.append([twice(z), twice(pw[32]), twice(pw[512]),
                      pair(twice(c), twice(c8)), pair((1.0, 0.0), twice(z16))])
    return seeds


def _mxu(words):
    return pltpu.bitcast(words, BF16)


def _store_table(ref, tab):
    for i in range(0, len(tab), 2):
        for p in range(2):
            ref[p, 8 * i:8 * i + 16, :] = jnp.concatenate(
                [tab[i][p], tab[i + 1][p]], axis=0).astype(BF16)


def _k_residues(groups, k_last, dskip, tmp_ref, sch):
    idx, nxt = sch.idx("src"), sch.idx("nxt")
    low = lambda x, y: (x & 65535) | (y << 16)
    high = lambda x, y: jax.lax.shift_right_logical(x, 16) | (y & -65536)
    kv, up = {}, {}
    for i, k in enumerate(FINE):
        v = [g[8 * i:8 * i + 8] for g in groups]
        if k == 0:
            v = [x + jnp.where(sch.mask("diag"),
                               _gather(dskip[n // 2], sch.idx("dup%d" % (n % 2)), 0), 0.0)
                 for n, x in enumerate(v)]
        p = [_pack(tmp_ref, 2 * i + h, v[2 * h], v[2 * h + 1]) for h in range(2)]
        both = [_gather(x, idx) for x in p]
        kv[k], kv[k + 8] = low(*both), high(*both)
        if k % 512 == 0:
            up[k] = low(*[_gather(x, nxt) for x in p])
    k_last = _gather(k_last, sch.idx("rows"), 0)
    q0, q1, q2, up0, up01, up2, up3, fine = map(sch.mask, INDEX[-8:])
    s3 = {r: jnp.where(q2, kv[1024 + r], kv[1536 + r]) for r in (0, 8)}
    v0 = jnp.where(q0, kv[0], jnp.where(q1, kv[512], s3[0]))
    v16 = jnp.where(up01, jnp.where(up0, up[0], up[512]),
                    jnp.where(up2, up[1024], jnp.where(up3, up[1536], k_last)))
    s3[16] = v16
    s23, s123, out = {}, {}, [v0]
    for r in range(1, 16):
        k23 = (RES2[r], RES3[r])
        if k23 not in s23:
            s23[k23] = v16 if k23 == (16, 16) else jnp.where(q1, kv[512 + k23[0]], s3[k23[1]])
        k123 = (RES1[r],) + k23
        if k123 not in s123:
            s123[k123] = v16 if k123[0] == 16 else jnp.where(q0, kv[k123[0]], s23[k23])
        if RES1[r] == r:
            out.append(s123[k123])
        else:
            out.append(jnp.where(fine, kv[r], s123[k123]))
    return out


def _ln_scalars(s1, s2):
    mean = s1 * (1.0 / D)
    var = jnp.maximum(s2 * (1.0 / D) - mean * mean, 0.0)
    eps = float(np.asarray(EPS, dtype=BF16))
    sd = _rbf(jnp.sqrt(_rbf(_rbf(var) + eps)))
    return _rbf(mean), 1.0 / sd


def _top8(x):
    def swap(v, pairs):
        for i, j in pairs:
            v[i], v[j] = jnp.maximum(v[i], v[j]), jnp.minimum(v[i], v[j])
        return v

    def merge(a, b):
        v = [jnp.maximum(a[i], b[7 - i]) for i in range(8)]
        return swap(v, [(i, i + d) for d in (4, 2, 1) for i in range(8) if not i & d])

    sort8 = ((0, 2), (1, 3), (4, 6), (5, 7), (0, 4), (1, 5), (2, 6), (3, 7), (0, 1), (2, 3),
             (4, 5), (6, 7), (2, 4), (3, 5), (1, 4), (3, 6), (1, 2), (3, 4), (5, 6))
    v = merge(*[swap(x[i:i + 8], sort8) for i in (0, 8)])
    for d in (4, 2, 1):
        v = merge(v, [pltpu.roll(t, d, 0) for t in v])
    return v


def _init_columns(col_ref, wx_ref, wy_ref, ldt_ref, dsk_ref, wr_ref):
    row, lane = _iota((128, 128), 0), _iota((128, 128), 1)
    split = (row & ~15) + 2 * (row & 7) + ((row >> 3) & 1)
    ldt, dsk, wr = (ref[...].astype(F32).reshape(1, D) for ref in (ldt_ref, dsk_ref, wr_ref))
    for n, vec in enumerate((jnp.exp(ldt), dsk * (1.0 / L))):
        for lo in range(0, D, 128):
            i = min(lo, D - 128)
            diag = jnp.where(split == lane, vec[:, i:i + 128], 0.0)[lo - i:].astype(BF16)
            col_ref[n, lo:i + 128, :] = jnp.dot(diag, jnp.ones((128, 128), BF16),
                                                preferred_element_type=F32)
    sub = _iota((16, D), 0)
    ones_w = jnp.where(sub == 0, 1.0, jnp.where(sub == 1, wr, 0.0))
    wx_ref[...] = ones_w.astype(BF16)
    for lo in range(0, D, MB):
        wy_ref[lo // MB, :, 0:MB] = ones_w[:, lo:lo + MB].astype(BF16)
        wy_ref[lo // MB, :, MB:] = jnp.zeros((16, 128 - MB), BF16)


INDEX = ("true", "bit0", "bit1", "bit2", "bit3", "odd", "dup0", "dup1", "rows", "src", "nxt",
         "diag", "q0", "q1", "q2", "up0", "up01", "up2", "up3", "fine")


def _init_index(idx_ref):
    sub, lane = _iota((8, 128), 0), _iota((8, 128), 1)
    src = lambda b: 8 * ((b >> 1) & 15) + 2 * (sub & 3) + (b & 1)
    is_ = lambda m: jnp.where(m, 1, 0)
    q = lane & 3
    q16 = q + is_(lane >= 124)
    tiles = dict(true=sub + 1, odd=sub & 1, dup0=sub >> 1, dup1=4 + (sub >> 1),
                 rows=2 * (sub & 3) + (sub >> 2), src=src(lane >> 2), nxt=src((lane >> 2) + 1),
                 diag=is_((lane == sub) & ((sub & 1) == 0)), up01=is_(q16 < 2),
                 fine=is_((q == 0) & (lane < 64)),
                 **{"bit%d" % n: (lane >> n) & 1 for n in range(4)},
                 **{"q%d" % n: is_(q == n) for n in range(3)},
                 **{"up%d" % n: is_(q16 == n) for n in (0, 2, 3)})
    for n, name in enumerate(INDEX):
        idx_ref[n] = tiles[name]


class _Schedule:
    def __init__(self, zero, idx_ref):
        self.zero = zero
        self.idx = lambda name: idx_ref[INDEX.index(name) + zero]
        self.mask = lambda name: self.idx(name) != 0
        self.true = self.mask("true")
        self.done, self.pending, self.wait = [], {}, -1

    def tie(self, x, token):
        return jnp.where(self.true, x, token if token.dtype == x.dtype
                         else pltpu.bitcast(token, x.dtype))

    def start(self, x):
        return self.tie(x, self.done[self.wait]) if 0 <= self.wait < len(self.done) else x

    def lhs(self, words, first):
        tiles = [words[i:i + 8] for i in range(0, words.shape[0], 8)]
        for i in range(len(tiles) if first else 0):
            for token in self.pending.pop(len(self.done) + i, ()):
                tiles[i] = self.tie(tiles[i], token)
        return _mxu(jnp.concatenate(tiles, axis=0))

    def results(self, v):
        self.done += [v[i + 8:i + 16] for i in range(0, v.shape[0], 16)]

    def run(self, stage, wait, before):
        self.wait = wait
        self.pending.setdefault(before, []).extend(next(stage))


def _kernel(x_hbm, are_hbm, aim_hbm, bre_hbm, bim_hbm, cre_hbm, cim_hbm,
            ldt_hbm, dsk_hbm, wr_hbm, wg_hbm, wu_hbm, wd_hbm, out_hbm,
            x_v, wg_v, wu_v, wd_v, par_v, ldt_v, dsk_v, wr_v, w_v, wk_v, wt_v, col_v, wx_v, wy_v,
            tmp_v, idx_v, pk_v, h_v, st_v, acc_v, sq_v, out_v, sd0, sd1, ta0, ta1, tb0, tb1, kl0, kl1,
            u0, u1, k0, k1, a0_v, a1_v, c0, c1, r0, r1, r2, r3,
            sem_p, sem_x, sem_w, sem_o, f0_v, f1_v, *rest):
    half_v, new_v = rest[:4], rest[4:]
    cp_vec = [pltpu.make_async_copy(s, d, sem_p.at[n]) for n, (s, d) in enumerate(
        ((ldt_hbm, ldt_v), (dsk_hbm, dsk_v), (wr_hbm, wr_v)))]
    cp_par = [[pltpu.make_async_copy(s.at[lo:hi], par_v.at[n, lo:hi], sem_p.at[3 + 6 * m + n])
               for n, s in enumerate((are_hbm, aim_hbm, bre_hbm, bim_hbm, cre_hbm, cim_hbm))]
              for m, (lo, hi) in enumerate(((0, 4 * MB), (4 * MB, D)))]
    cp_x = [pltpu.make_async_copy(x_hbm.at[:, 128 * j:128 * j + 128], x_v.at[j, 0:D],
                                  sem_x.at[j])
            for j in range(NT)]
    cp_d = pltpu.make_async_copy(wd_hbm, wd_v, sem_w.at[2])

    def cp_w(i):
        return [pltpu.make_async_copy(s.at[:, _ds(128 * i, 128)], d.at[i, 0:D], sem_w.at[n])
                for n, (s, d) in enumerate(((wg_hbm, wg_v), (wu_hbm, wu_v)))]

    for cp in cp_vec + cp_par[0]:
        cp.start()
    for cp in cp_x[:NT // 2]:
        cp.start(priority=1)

    def columns():
        for cp in cp_vec:
            cp.wait()
        for cp in cp_x[NT // 2:]:
            cp.start(priority=1)
        _transpose_dft(wt_v, w_v, range(4))
        _init_columns(col_v, wx_v, wy_v, ldt_v, dsk_v, wr_v)

    _init_dft(w_v, wk_v, tmp_v, columns)
    for cp in cp_par[0]:
        cp.wait()

    sd, ta, tb, kl = (sd0, sd1), (ta0, ta1), (tb0, tb1), (kl0, kl1)
    uk, ab, cc, xr = ((u0, u1), (k0, k1)), ((a0_v, a1_v), (f0_v, f1_v)), (c0, c1), (r0, r1, r2, r3)
    ww, wt_w = (w_v.bitcast(I32), wk_v.bitcast(I32)), wt_v

    def chan(b, r):
        return _ds(b * MB + 16 * r, 16)

    def seed_stage(b, r, sch):
        rows = _ds(b * MB // 2 + 8 * r, 8)
        par = [_split(par_v.bitcast(I32)[n, rows, :]) for n in range(6)]
        for h in range(2):
            a_re, a_im, b_re, b_im, c_re, c_im = [v[h] for v in par]
            dt = sch.start(col_v[0, _ds(b * MB + 16 * r + 8 * h, 8), :])
            mag, ang = jnp.exp(dt * a_re), dt * a_im
            sc = dt * (1.0 / L)
            seeds = _k_seeds((mag * jnp.cos(ang), mag * jnp.sin(ang)),
                             _cmul((c_re, c_im), (sc * b_re, sc * b_im)), sch)
            for g in range(2):
                for n, v in enumerate(seeds[g]):
                    for p in range(2):
                        sd[b % 2][r, 2 * h + g, 2 * n + p] = v[p]
            yield [sd[b % 2][(r + sch.zero), 2 * h, 0]]

    def table_stage(b, r, sch):
        tail = []
        for g in range(4):
            m1, m32, m512, a0, b0 = [
                (sd[b % 2][r, g, 2 * n], sd[b % 2][r, g, 2 * n + 1]) for n in range(5)]
            m32 = (sch.start(m32[0]), m32[1])
            fa = [a0]
            for _ in range(7):
                fa.append(_cmul(fa[-1], m1))
            for src in (0, 4, 8, 10):
                fa.append(_cmul(fa[src], m512))
            tail.append(fa[11][0] * m512[0] - fa[11][1] * m512[1])
            _store_table(ta[b % 2].at[r, g], fa)
            fb = [b0]
            for _ in range(15):
                p = fb[-1]
                fb.append((p[0] * m32[0] + p[1] * m32[1], p[1] * m32[0] - p[0] * m32[1]))
            _store_table(tb[b % 2].at[r, g], fb)
            yield [ta[b % 2].bitcast(I32)[(r + sch.zero), g, 0, 0:8, :],
                   tb[b % 2].bitcast(I32)[(r + sch.zero), g, 0, 0:8, :]]
        last = [jnp.where(sch.mask("odd"), pltpu.roll(tail[h + 1], 1, 0), tail[h])
                for h in (0, 2)]
        last = [pltpu.bitcast(_rbf(jnp.broadcast_to(jnp.sum(v, axis=1, keepdims=True),
                                                    (8, 128))), I32) for v in last]
        kl[b % 2][r] = jax.lax.shift_right_logical(last[0], 16) | last[1]

    def kernel_stage(b, r, sch):
        ta_w, tb_w = ta[b % 2].bitcast(I32), tb[b % 2].bitcast(I32)
        groups = [None] * 4
        for g0 in (0, 2):
            res = [jax.lax.dot_general(sch.lhs(ta_w[r, g, p, 0:48], g == g0 and p == 0),
                                       _mxu(tb_w[r, g, p, 0:64]), NT_DIMS, preferred_element_type=F32)
                   for g in (g0, g0 + 1) for p in range(2)]
            groups[g0], groups[g0 + 1] = res[0] + res[1], res[2] + res[3]
            sch.results(groups[g0 + 1])
            yield []
        dskip = [col_v[1, _ds(b * MB + 16 * r + 8 * h, 8), :] for h in range(2)]
        dst = _ds(8 * r, 8)
        res = _k_residues(groups, kl[b % 2][r], dskip, pk_v.at[sch.slot, 0], sch)
        for s, t in enumerate(res):
            uk[1][b % 2][4 * (s % 4) + s // 4, dst, :] = t
        yield [uk[1][b % 2][0, _ds(8 * (r + sch.zero), 8), :]]

    def norm_stage(b, r, sch):
        rows, dst = _ds(b * MB // 2 + 8 * r, 8), _ds(8 * r, 8)
        tiles = [x_v.bitcast(I32)[j, rows, :] for j in range(NT)]
        for s, t in enumerate(_to_residues([sch.start(tiles[0])] + tiles[1:], sch)):
            xr[b % 4][4 * (s % 4) + s // 4, dst, :] = t
            xs, m, inv = _mxu(t).astype(F32), st_v[s, 0], st_v[s, 1]
            uk[0][b % 2][4 * (s % 4) + s // 4, _ds(16 * r, 16), :] = jnp.concatenate(
                [(xs[0:8] - m) * inv, (xs[8:16] - m) * inv], axis=0).astype(BF16)
        yield [uk[0][b % 2].bitcast(I32)[0, _ds(8 * (r + sch.zero), 8), :]]

    def forward_stage(w, b, k, sch):
        dst = ab[w][b % len(ab[w])]
        for p in range(2):
            v = [jnp.dot(sch.lhs((uk[w][b % 2] if w else uk[w][b % 2].bitcast(I32))[
                4 * k + n, 0:MB // 2], n == 0),
                         _mxu(ww[w][p ^ (n & 1), 4 * k + n, 0:64]),
                         preferred_element_type=F32) for n in range(4)]
            d02, d13 = v[0] - v[2], v[1] - v[3]
            x1 = d02 - d13 if p == 0 else d02 + d13
            dst[0, k, p, 0:MB] = v[0] + v[2]
            dst[2, k, 1 - p, 0:MB] = v[1] + v[3]
            dst[1, k, p, 0:MB] = x1
            dst[3, k, p, 0:MB] = d02 + d13 if p == 0 else d02 - d13
            sch.results(x1)
            yield []

    def stats(tiles, sch):
        ones_w = wx_v.bitcast(I32)[...]
        for j in tiles:
            acc = None
            for i in range(0, D // 2, 8):
                v = [t * t for t in _split(x_v.bitcast(I32)[j, i:i + 8, :])]
                acc = v if acc is None else [p + q for p, q in zip(acc, v)]
            sums = jnp.dot(_mxu(jnp.concatenate(
                [ones_w[:, :128] if j % 2 == 0 else sch.tie(ones_w[:, :128], prev),
                 ones_w[:, 128:]], axis=1)),
                           _mxu(x_v.bitcast(I32)[j, 0:D // 2]), preferred_element_type=F32)
            s2 = prev = acc[0] + acc[1]
            for d in (4, 2, 1):
                s2 = s2 + pltpu.roll(s2, d, 0)
            st_v[j, 0], st_v[j, 1] = _ln_scalars(jnp.broadcast_to(sums[0:1], (8, 128)), s2)

    def middle_stage(b, r, sch):
        src = [v[b % len(v)] for v in ab]
        scale = lambda v, f: [(x[0] * f, x[1] * f) for x in v]
        for h in range(2):
            ra = _ds(16 * r + 8 * h, 8)
            ld = lambda q, w, ra=ra: [(src[w][q, k, 0, ra, :], src[w][q, k, 1, ra, :]) for k in range(4)]

            park_v = half_v[2 * (sch.slot % 2) + h]

            def put(q, y):
                x = [park_v[n + sch.zero] for n in range(8)]
                for k in range(4):
                    for p in range(2):
                        cc[b % 2][k, q, p, ra, :] = x[2 * k + p] + y[k][p]
                        cc[b % 2][k, q + 2, p, ra, :] = x[2 * k + p] - y[k][p]

            def park(x):
                for k in range(4):
                    for p in range(2):
                        park_v[2 * k + p] = x[k][p]
                return [park_v[sch.zero]]

            gate = sch.start
            a0, a2, b0, b2 = ld(0, 0), ld(2, 0), ld(0, 1), ld(2, 1)
            a0[0] = (gate(a0[0][0]), a0[0][1])
            e0 = _prod_mod_1(list(map(_cadd, a0, a2)), list(map(_cadd, b0, b2)))
            again = _ds(16 * (r + sch.zero) + 8 * h, 8)
            yield park(e0)
            a0, a2, b0, b2 = (ld(q, w, again) for w in range(2) for q in (0, 2))
            a2[0] = (gate(a2[0][0]), a2[0][1])
            e2 = _prod_mod_m1(list(map(_csub, a0, a2)), scale(map(_csub, b0, b2), 2.0))
            put(0, e2)
            yield [cc[b % 2][0, 0, 0, again, :]]
            four = sch.start(jnp.full((8, 128), 4.0, F32))
            e1 = _prod_mod_i(ld(1, 0), scale(ld(1, 1), four), 1)
            yield park(e1)
            four = sch.start(jnp.full((8, 128), 4.0, F32))
            e3 = _prod_mod_i(ld(3, 0), scale(ld(3, 1), four), -1)
            put(1, e3)
            yield [cc[b % 2][0, 1, 0, again, :]]

    def inverse_stage(b, k, sch):
        src = cc[b % 2]

        def lhs(v, n, first):
            return sch.lhs(jnp.concatenate(
                [_pack(pk_v.at[sch.slot, 2], 4 * n + i // 16, v[i:i + 8], v[i + 8:i + 16])
                 for i in range(0, MB, 16)], axis=0), first)

        for o in range(2):
            p0, p1 = [(src[k, q, 0, 0:MB], src[k, q, 1, 0:MB]) for q in (2 * o, 2 * o + 1)]
            if o == 0:
                e = {0: _cadd(p0, p1), 2: _csub(p0, p1)}
            else:
                e = {1: (p0[0] + p1[1], p0[1] - p1[0]), 3: (p0[0] - p1[1], p0[1] + p1[0])}
            ys = []
            for n in e:
                y = [jnp.dot(lhs(e[n][p], 2 * n + p, n == o and p == 0),
                             _mxu(wt_w[4 * k + (0, 2, 1, 3)[n], p, 0:64]),
                             preferred_element_type=F32)
                     for p in range(2)]
                h = y[0] + y[1] + _mxu(xr[b % 4][4 * k + n, 0:MB // 2]).astype(F32)
                h_v[k + 4 * n, b * MB:b * MB + MB, :] = h.astype(BF16)
                hh = h * h
                sq_v[k + 4 * n] += sum((hh[i:i + 8] for i in range(8, MB, 8)), hh[0:8])
                ys.append(h)
            sch.results(ys[-1])
            yield []

    def sum_stage(b, r, sch):
        for n in range(4):
            s = r + 4 * n if b == nb - 1 else 4 * r + n
            sums = jnp.dot(sch.lhs(wy_v.bitcast(I32)[b], n == 0)[:, :MB],
                           _mxu(h_v.bitcast(I32)[s, b * MB // 2:(b + 1) * MB // 2]),
                           preferred_element_type=F32)
            acc_v[s] += sums[0:8]
        sch.results(sums)
        yield []

    nb = D // MB
    stages = dict(
        s=(seed_stage, 0), t=(table_stage, 1), k=(kernel_stage, 2),
        F=(functools.partial(forward_stage, 1), 3), n=(norm_stage, 2),
        f=(functools.partial(forward_stage, 0), 3), m=(middle_stage, 4),
        i=(inverse_stage, 5), a=(sum_stage, 6))

    def run(step, zero, live=None):
        live = live or {n: (f, step - lag) for n, (f, lag) in stages.items()
                        if 0 <= step - lag < nb and (n, step) != ("n", 2)}
        if step == nb + 4:
            live["z"] = (sum_stage, nb - 1)
        unroll, plan = PLANS["".join(live)]

        def body(it, carry):
            sch = _Schedule(zero >> (step % 32) if unroll == 4 else zero & it, idx_v)
            gens = [{n: f(b, it * unroll + u, sch) for n, (f, b) in live.items()}
                    for u in range(unroll)]
            if step == 3:
                for i in range(9 * unroll):
                    for cp in cp_w(9 * unroll * it + i):
                        cp.start()
            for item in plan.split():
                u, n, *ties = item.split(":")
                if n in live:
                    sch.slot = int(u)
                    sch.run(gens[int(u)][n], *map(int, ties or (-1, -1)))
            for sch.slot, g in enumerate(gens):
                for v in g.values():
                    for _ in v:
                        pass
            return carry + it

        if unroll == 4:
            if step == 101 or step > nb + 3:
                return body(0, 0)
            return jax.lax.fori_loop(zero, 1, lambda _, c: body(0, c), 0)
        return jax.lax.fori_loop(0, 4 // unroll, body, 0)

    _init_index(idx_v)
    acc_v[...] = sq_v[...] = jnp.zeros(acc_v.shape, F32)
    zero = run(0, 0) - 1
    for step in range(1, nb + 5):
        if step == 4:
            for cp in cp_par[1]:
                cp.wait()
        if step == 3:
            for half in range(2):
                tiles = range(NT // 2 * half, NT // 2 * (half + 1))
                for j in tiles:
                    cp_x[j].wait()
                if half:
                    cp_d.start(priority=1)
                else:
                    for cp in cp_par[1]:
                        cp.start()
                _transpose_dft(wt_v, w_v, range(4 + 6 * half, 10 + 6 * half))
                stats(tiles, _Schedule(zero, idx_v))
            for q in range(2):
                for s, v in enumerate(_to_residues([st_v[j, q] for j in range(NT)],
                                                   _Schedule(zero, idx_v))):
                    st_v[s, q] = v
            run(101, zero, dict(n=(norm_stage, 0)))
        run(step, zero)

    sums = [acc_v[s] for s in range(16)]
    m2, inv2 = _ln_scalars(
        jnp.concatenate([v[0:1] for v in sums], axis=0),
        jnp.concatenate([jnp.sum(sq_v[j], axis=0, keepdims=True) for j in range(NT)], axis=0))
    wsum = jnp.sum(wr_v[...].astype(F32).reshape(1, D), axis=1, keepdims=True)
    score = _rbf((jnp.concatenate([v[1:2] for v in sums], axis=0) - m2 * wsum) * inv2 + 0.0)
    bits = pltpu.bitcast(score, I32) >> 16
    order = jnp.where(bits < 0, -1 - bits, bits + 32768)
    mu = (_iota((NT, 128), 1) - _iota((NT, 128), 0)) & 127
    pos = 128 * (mu & 15) + 16 * (mu >> 4) + _iota((NT, 128), 0)
    key = pltpu.bitcast((order << 11) + (L - 1 - pos) + (1 << 29), F32)

    h_w, out_w = h_v.bitcast(I32), out_v.bitcast(I32)
    sch, done = _Schedule(zero, idx_v), []
    tie = sch.tie

    def unrouted():
        for q, v in enumerate((1.0 + inv2, m2 * inv2)):
            for j, t in enumerate(_to_time(
                    [jnp.broadcast_to(v[s:s + 1], (8, 128)) for s in range(16)], sch)):
                st_v[j, q] = t
        for i in range(0, D, 16):
            scal = st_v.at[pl.ds(zero * (i + 1), NT)]
            tiles = [h_w[s, i // 2:i // 2 + 8, :] for s in range(16)]
            if len(done) > LAG:
                tiles[0] = tie(tiles[0], done[-LAG])
            for j, v in enumerate(_to_time(tiles, sch)):
                h, mul, sub = _mxu(v).astype(F32), scal[j, 0], scal[j, 1]
                out_v[j, i:i + 16, :] = jnp.concatenate(
                    [h[0:8] * mul - sub, h[8:16] * mul - sub], axis=0).astype(BF16)
                if j % 8 == 7:
                    yield pltpu.bitcast(out_w[j + zero, i // 2:i // 2 + 8, :], F32)

    side = unrouted()

    lane8, sub8 = _iota((CAP, 128), 1), _iota((CAP, 128), 0)
    best = _top8([pltpu.roll(key[i:i + 8], n, 1) if n else key[i:i + 8]
                  for i in (0, 8) for n in range(8)])
    cand = best[0]
    for c in range(1, CAP):
        cand = jnp.where(sub8 == c, best[c], cand)
    best = _top8([pltpu.roll(cand, n, 1) if n else cand for n in range(0, 128, 8)])
    for _ in range(2 * EARLY):
        best[-1] = tie(best[-1], next(side))
    best = [pltpu.bitcast(v, I32)[0, 0] for v in best]
    picks = [L - 1 - (v & (L - 1)) for v in best]

    def schedule(col):
        rnd = [sum([(col[e] == col[c]).astype(I32) for e in range(c)], 0) for c in range(CAP)]
        return (rnd, functools.reduce(jnp.maximum, rnd) + 1,
                lambda n: [lane8 == jnp.where(rnd[c] == n, col[c], -1) for c in range(CAP)])

    _, rounds, lanes = schedule([((t >> 7) + (t & 127)) & 127 for t in picks])

    def out_copy(q, lo, hi):
        j = order[q]
        return pltpu.make_async_copy(
            out_v.at[j, lo:hi], out_hbm.at[lo:hi, _ds(j * 128, 128)], sem_o)

    for n, ref in enumerate((wg_v, wu_v)):
        pltpu.make_async_copy(ref.at[:, 0:D], ref.at[:, 0:D], sem_w.at[n]).wait()

    def gather(n, acc):
        masks = lanes(n)
        tiles = []
        for i in range(0, D // 2, 8):
            v = jnp.zeros((8, 128), I32)
            for c in range(CAP):
                v = jnp.where(masks[c], h_w[picks[c] & 15, i:i + 8, :], v)
            tiles.append(v)
        lhs = jnp.zeros((CAP, 128), F32)
        for c in range(CAP):
            lhs = jnp.where(masks[c] & (sub8 == c), 1.0, lhs)
        aux = [jnp.zeros((CAP, 128), F32)] * 3
        for c in range(CAP):
            hit = pltpu.bitcast(key, I32) == best[c]
            aux = [jnp.where(sub8 == c, jnp.sum(jnp.where(hit, v, 0.0), axis=0, keepdims=True), a)
                   for a, v in zip(aux, (m2, inv2, score))]
        return (acc[0] + jax.lax.dot_general(lhs.astype(BF16), _mxu(jnp.concatenate(tiles, axis=0)),
                                             NT_DIMS, preferred_element_type=F32),
                *[jnp.sum(a, axis=1, keepdims=True) for a in aux])

    h_sel, m_sel, inv_sel, score_sel = jax.lax.fori_loop(
        0, rounds, gather, (jnp.zeros((CAP, D), F32), *[jnp.zeros((CAP, 1), F32)] * 3))
    x_sel = _rbf((h_sel - m_sel) * inv_sel)
    gate = _rbf(jax.nn.sigmoid(score_sel))

    tile, col = [t >> 7 for t in picks], [t & 127 for t in picks]
    rnd, rounds, lanes = schedule(col)
    late, again = 0, []
    for j in tile:
        again.append((late >> j) & 1)
        late = late | (1 << j)
    for dup in again[1:]:
        late = late | (late + dup)
    order = []
    for left in (late ^ ((1 << NT) - 1), late):
        for _ in range(CAP):
            order.append((31 - jax.lax.clz(left)) & (NT - 1))
            left = left ^ (1 << order[-1])

    def early_copies(n):
        lo, hi = (0, 16 * EARLY, MID, D)[n:n + 2]
        return [out_copy(q, lo, hi) for q in range(CAP)]

    def start(copies):
        for cp in copies:
            cp.start()

    start(early_copies(0))
    rate, sent = MID // 8 - 2 * EARLY, [0]

    def project(w_ref):
        parts = []
        for n in range(0, FF // 128, 4):
            for lo in range(0, D, 128):
                hi = min(lo + 128, D)
                xs = x_sel[:, lo:hi]
                if hi - lo == 128 and min(rate, (len(done) - 4) * rate // END) > sent[0]:
                    sent[0] += 1
                    xs = tie(xs, next(side))
                w = [w_ref.bitcast(I32)[i, lo // 2:hi // 2, :] for i in range(n, n + 4)]
                v = jnp.dot(xs.astype(BF16), _mxu(jnp.concatenate(w, axis=1)),
                            preferred_element_type=F32)
                done.append(v[:, 0:128])
                acc = acc + v if lo else v
            parts.append(acc)
        return _rbf(jnp.concatenate(parts, axis=1))

    g = project(wg_v)
    act = _rbf(g * jax.nn.sigmoid(g)) * project(wu_v)
    for _ in range(rate - sent[0]):
        next(side)
    done.clear()

    cp_d.wait()

    start(early_copies(1))
    rest_side = list(side)

    def placed(r, words):
        idx = jnp.zeros((CAP, 128), I32)
        for c, m in enumerate(lanes(r)):
            idx = jnp.where(m, c, idx)
        return [_gather(w, idx) for w in words]

    def late_copies(lo, hi):
        return [out_copy(CAP + q, lo, hi) for q in range(CAP)]

    def words_of(n):
        return [new_v[n].bitcast(I32)[i:i + 8, :] for i in range(0, new_v[n].shape[0] // 2, 8)]

    tokens = []
    for n, (lo, hi) in enumerate(ROW_CHUNKS):
        a = [act[:, i:i + 128] for i in range(0, FF, 128)]
        for i, token in enumerate(rest_side):
            at = 8 + i * SPAN // len(rest_side) - n * len(a)
            if 0 <= at < len(a):
                a[at] = tie(a[at], token)
        if n == 1:
            start(early_copies(2))
        if n >= 2:
            cut = CUT * 128 // (hi - lo)
            a[cut] = tie(a[cut], tokens[n - 2])
        a = jnp.concatenate(a, axis=1)
        y = _rbf(jax.lax.dot_general(a.astype(BF16), wd_v[lo:hi, :], NT_DIMS,
                                     preferred_element_type=F32))
        new = h_sel[:, lo:hi] + _rbf(x_sel[:, lo:hi] + _rbf(y * gate))
        new_v[n][...] = jnp.concatenate(
            [new.T, jnp.zeros((hi - lo, 128 - CAP), F32)], axis=1).astype(BF16)
        rows = range(lo // 2, hi // 2, 8)
        words = words_of(n)
        both = list(zip(rows, placed(0, words), placed(1, words)))
        for c in range(CAP):
            for i, v0, v1 in both:
                pltpu.store(out_w.at[tile[c], pl.ds(i, 8), :],
                            jnp.where(rnd[c] == 0, v0, v1), mask=lane8 == col[c])
        for cp in late_copies(lo, hi):
            cp.start()
        out_w[tile[0], D // 2:, :] = lane8
        tokens.append(pltpu.bitcast(out_w[tile[0] | zero, D // 2:, :], F32))
    pltpu.make_async_copy(out_v.at[:, 0:D], out_v.at[:, 0:D], sem_o).wait()

    @pl.when(rounds > 2)
    def _():
        def fix(r, carry):
            rows = range(0, D // 2, 8)
            vals = placed(r, sum(map(words_of, range(len(new_v))), []))
            for c, m in enumerate(lanes(r)):
                for i, v in zip(rows, vals):
                    pltpu.store(out_w.at[tile[c], pl.ds(i, 8), :], v, mask=m)
            return carry

        jax.lax.fori_loop(2, rounds, fix, 0)
        for cp in late_copies(0, D):
            cp.start()
        for cp in late_copies(0, D):
            cp.wait()


@jax.jit
def pallas_sequential_preLN__ssm_conv_s4__moe_arch_mod__prompt_kernel(
    A_u: jax.Array,
    A_A_re: jax.Array,
    A_A_im: jax.Array,
    A_B_re: jax.Array,
    A_B_im: jax.Array,
    A_C_re: jax.Array,
    A_C_im: jax.Array,
    A_log_dt: jax.Array,
    A_Dskip: jax.Array,
    B_x: jax.Array,
    B_w_r: jax.Array,
    B_w_gate: jax.Array,
    B_w_up: jax.Array,
    B_w_down: jax.Array,
):
    del B_x
    hbm = pl.BlockSpec(memory_space=pl.ANY)
    out = pl.pallas_call(
        _kernel,
        out_shape=jax.ShapeDtypeStruct((D, L), BF16),
        in_specs=[hbm] * 13,
        out_specs=hbm,
        scratch_shapes=[
            pltpu.VMEM((NT, D + 16, 128), BF16),
            *[pltpu.VMEM((FF // 128, D + 16, 128), BF16)] * 2,
            pltpu.VMEM((D, FF), BF16),
            pltpu.VMEM((6, D, N), BF16),
            *[pltpu.VMEM((D,), BF16)] * 3,
            *[pltpu.VMEM((2, 16, 144, 128), BF16)] * 2,
            pltpu.VMEM((16, 2, 72, 128), I32),
            pltpu.VMEM((2, D, 128), F32),
            pltpu.VMEM((16, D), BF16),
            pltpu.VMEM((D // MB, 16, 128), BF16),
            pltpu.VMEM((2, 256, 128), F32),
            pltpu.VMEM((len(INDEX), 8, 128), I32),
            pltpu.VMEM((4, 3, 32, 16, 128), BF16),
            pltpu.VMEM((NT, D + 16, 128), BF16),
            pltpu.VMEM((NT, 2, 8, 128), F32),
            *[pltpu.VMEM((NT, 8, 128), F32)] * 2,
            pltpu.VMEM((NT, D + 16, 128), BF16),
            *[pltpu.VMEM((4, 4, 10, 8, 128), F32)] * 2,
            *[pltpu.VMEM((4, 4, 2, 112, 128), BF16)] * 2,
            *[pltpu.VMEM((4, 4, 2, 144, 128), BF16)] * 2,
            *[pltpu.VMEM((4, 8, 128), I32)] * 2,
            *[pltpu.VMEM((16, MB + 16, 128), BF16)] * 2,
            *[pltpu.VMEM((16, MB // 2 + 8, 128), I32)] * 2,
            *[pltpu.VMEM((4, 4, 2, MB + 8, 128), F32)] * 2,
            *[pltpu.VMEM((4, 4, 2, MB + 8, 128), F32)] * 2,
            *[pltpu.VMEM((16, MB // 2 + 8, 128), I32)] * 4,
            pltpu.SemaphoreType.DMA((15,)),
            pltpu.SemaphoreType.DMA((NT,)),
            pltpu.SemaphoreType.DMA((3,)),
            pltpu.SemaphoreType.DMA,
            *[pltpu.VMEM((4, 4, 2, MB + 8, 128), F32)] * 2,
            *[pltpu.VMEM((8, 8, 128), F32)] * 4,
            *[pltpu.VMEM((hi - lo, 128), BF16) for lo, hi in ROW_CHUNKS],
        ],
        compiler_params=pltpu.CompilerParams(vmem_limit_bytes=100 * 1024 * 1024,
                                             disable_bounds_checks=True,
                                             disable_semaphore_checks=True),
    )(A_u.reshape(L, D).T, A_A_re, A_A_im, A_B_re, A_B_im, A_C_re, A_C_im,
      A_log_dt, A_Dskip, B_w_r, B_w_gate, B_w_up, B_w_down.T)
    return out.T.reshape(1, L, D)
```

```python
import functools

import numpy as np
import jax
import jax.numpy as jnp
import jax.experimental.pallas as pl
import jax.experimental.pallas.tpu as pltpu

F32 = jnp.float32
BF16 = jnp.bfloat16
I32 = jnp.int32

L = 2048
D = 576
N = 128
FF = 4608
CAP = 8
NT = L // 128
EPS = 1e-5
MB = 64
PLANS = dict(
    s=(2, ""),
    st=(2, ""),
    n=(4, ""),
    stk=(2, "0:t:-1:4 1:t:-1:3 0:t:-1:4 0:t:-1:7 0:t:-1:15 1:t:-1:10 1:t:6:16 1:t:11:21 0:k "
            "0:k 1:k 0:s:-1:20 0:s:11:23 0:k:-1:23 1:k 1:s:20:-1 1:s 1:k "),
    stkFnf=(4, "1:t:-1:1 0:s:-1:9 0:s:-1:34 1:s:-1:35 1:s:-1:54 2:s:-1:69 3:s:-1:90 0:f "
               "0:n:1:19 0:F 0:t:4:25 0:t:0:19 0:k 0:t:12:43 0:k 0:k:-1:38 0:F 0:f 1:f "
               "1:t:29:44 1:F 1:n:33:47 1:t:35:58 1:k 1:k 1:t:42:57 1:k:-1:61 0:t:44:56 "
               "3:t:47:61 1:F 1:f 2:f 2:n:57:76 2:F 2:t:61:83 2:t:53:76 2:k 2:k 2:s:73:91 "
               "2:k:-1:92 2:t:70:98 2:F 2:f 3:f 3:t:85:100 3:F 3:n:89:104 3:t:91:-1 3:k "
               "3:s:95:111 3:k 3:t:98:110 3:k 2:t:100:110 3:F 3:f "),
    stkFnfm=(4, "0:m:-1:6 0:m:-1:5 0:t:-1:7 0:t:-1:14 0:t:-1:12 0:f 0:m:3:13 0:m:-1:18 "
                "0:m:3:18 0:f 0:m:6:20 0:k 0:t:8:25 0:n:9:27 0:m:13:33 0:m:13:25 1:m:12:34 0:k "
                "0:s:16:33 0:k:-1:35 0:s:19:33 1:m:18:33 0:F 1:t:20:35 0:F 1:t:27:42 1:t:24:40 "
                "1:f 1:f 1:m:32:42 1:m:31:46 1:m:31:46 1:m:34:48 1:k 1:t:37:50 1:n:37:55 "
                "2:m:39:62 1:k 1:s:44:61 1:m:43:61 1:m:41:53 1:k:-1:63 1:s:47:63 2:m:43:61 1:F "
                "2:t:48:63 1:F 2:t:55:70 2:t:50:68 2:f 2:f 2:m:60:70 2:m:60:78 2:m:59:71 "
                "2:m:62:76 2:k 2:t:66:78 2:n:65:85 2:k 2:s:72:89 2:m:71:89 2:m:69:81 2:k:-1:94 "
                "2:s:75:89 3:m:70:90 3:m:74:89 2:F 3:t:76:91 2:F 3:t:83:98 3:t:78:96 3:f 3:f "
                "3:m:88:98 3:m:87:102 3:m:87:102 3:m:90:104 3:k 3:t:93:108 3:n:94:110 3:k "
                "3:s:100:-1 3:m:99:-1 3:m:94:106 3:k 3:F 3:s:105:-1 3:F "),
    stkFnfmi=(4, "0:t:-1:2 0:n:-1:8 0:t:-1:3 0:m:-1:6 0:m:-1:7 0:m:-1:19 0:s:-1:40 1:s:-1:76 "
                 "2:s:-1:112 3:s 0:k 0:m:0:16 0:s:4:33 0:f 0:k 0:m:13:23 0:k:-1:33 0:m:14:25 "
                 "0:t:14:35 0:f 0:t:18:33 0:F 1:t:23:40 0:F 1:n:27:47 1:t:24:38 1:m:27:43 0:i "
                 "1:m:29:47 0:i 0:m:32:40 0:m:31:44 1:m:34:54 1:k 1:m:36:54 1:s:40:71 1:f 1:k "
                 "1:m:49:61 1:m:51:63 1:k:-1:71 1:f 1:t:55:79 1:t:51:68 1:F 2:t:59:74 "
                 "2:t:59:75 1:F 2:m:63:78 2:m:63:79 1:i 2:n:65:80 1:i 1:m:68:76 1:m:67:78 2:k "
                 "2:m:72:91 2:m:71:87 2:s:76:105 2:f 2:k 2:m:83:95 2:k:-1:105 2:m:86:97 "
                 "2:t:86:108 2:f 2:t:90:105 2:F 3:t:94:112 2:F 3:t:96:110 3:m:99:115 2:i "
                 "3:n:102:119 3:m:101:119 2:i 2:m:104:112 2:m:103:116 3:k 3:m:108:126 "
                 "3:m:111:126 3:s:112:143 3:f 3:k 3:m:121:133 3:k:-1:142 3:m:123:135 3:f "
                 "3:t:127:-1 3:t:123:140 3:F 3:F 3:i 3:m:139:-1 3:m:139:-1 3:i "),
    stkFnfmia=(4, "0:t:-1:6 0:t:-1:3 0:n:-1:10 0:m:-1:6 0:m:-1:5 0:m:-1:19 0:s:-1:43 1:s:-1:80 "
                  "2:s:-1:117 3:s 0:a 0:f 0:m:1:20 0:k 0:s:5:40 0:k 0:m:14:26 0:m:-1:26 "
                  "0:k:-1:38 0:t:16:30 0:f 0:t:18:32 0:F 0:F 1:t:25:43 1:t:23:42 1:n:28:47 "
                  "1:m:25:43 1:m:27:43 0:i 0:m:32:40 0:i 0:m:34:42 1:a 1:f 1:m:38:56 1:m:36:57 "
                  "1:k 1:s:42:77 1:k 1:m:52:63 1:m:53:67 1:k:-1:75 1:t:53:67 1:f 1:t:55:69 1:F "
                  "1:F 2:t:64:80 2:t:57:76 2:n:65:84 2:m:62:80 2:m:61:80 1:i 1:m:69:77 1:i "
                  "1:m:71:81 2:m:73:93 2:a 2:f 2:m:75:94 2:k 2:s:79:114 2:k 2:m:89:100 "
                  "2:m:87:103 2:k:-1:112 2:t:90:104 2:f 2:t:92:106 2:F 2:F 3:t:99:117 "
                  "3:t:97:116 3:m:99:117 3:m:101:117 2:i 2:m:106:114 3:n:103:121 2:i "
                  "2:m:108:116 3:a 3:f 3:m:113:131 3:m:114:131 3:k 3:s:116:-1 3:k 3:m:126:137 "
                  "3:m:124:140 3:k:-1:145 3:t:127:141 3:f 3:t:129:-1 3:F 3:F 3:i 3:m:143:-1 "
                  "3:i 3:m:145:-1 "),
    tkFnfmia=(4, "1:m:-1:5 1:m:-1:3 0:n:-1:12 0:t:-1:3 0:t:-1:14 0:t:-1:21 0:t:-1:28 1:t:-1:40 "
                 "1:t:-1:51 1:t:-1:58 1:t:-1:65 2:t:-1:77 2:t:-1:88 0:F 0:m:2:14 0:m:-1:15 0:a "
                 "0:F 0:m:7:20 0:k 0:m:9:27 0:m:13:23 0:k 0:m:15:25 0:m:18:31 0:m:20:32 "
                 "0:k:-1:45 0:i 0:i 0:f 0:f 1:n:36:50 1:F 1:a 1:F 1:m:42:56 1:m:34:56 1:k "
                 "1:m:47:64 1:k 1:m:53:68 1:k:-1:75 1:i 1:i 3:m:63:79 3:m:61:77 1:f 1:m:68:76 "
                 "1:f 1:m:73:81 2:n:70:86 2:F 2:m:75:87 2:m:73:95 2:a 2:F 2:m:79:92 2:t:81:95 "
                 "2:t:-1:101 2:k 2:m:83:101 2:m:87:97 2:k 2:m:89:101 2:k:-1:119 2:i 2:m:95:105 "
                 "2:m:87:103 2:i 3:t:99:111 2:f 3:t:106:122 3:t:-1:129 2:f 3:n:110:124 3:F 3:a "
                 "3:F 3:m:116:129 3:m:111:134 3:k 3:m:121:141 3:m:124:141 3:t:125:139 3:k 3:k "
                 "3:i 3:i 3:f 3:m:142:-1 3:f 3:m:145:-1 "),
    kFnfmia=(4, "1:m:-1:5 1:m:-1:3 0:n:-1:12 0:F 0:m:2:14 0:m:-1:15 0:a 0:F 0:m:7:21 0:k "
                "0:m:9:27 0:m:13:23 0:k 0:m:15:25 0:m:18:31 0:m:20:32 0:k:-1:45 0:i 0:i 0:f "
                "0:f 1:n:36:50 1:F 1:a 1:F 1:m:42:57 1:m:34:56 1:k 1:m:47:64 1:k 1:m:53:66 "
                "1:k:-1:75 1:i 1:i 3:m:63:79 3:m:61:77 1:f 1:m:68:76 1:f 1:m:73:81 2:n:70:86 "
                "2:F 2:m:76:88 2:m:73:89 2:a 2:F 2:m:79:93 2:k 2:m:83:101 2:m:87:97 2:k "
                "2:m:89:101 2:k:-1:119 2:i 2:m:95:105 2:m:90:106 2:i 2:f 2:f 3:n:110:124 3:F "
                "3:a 3:F 3:m:116:130 3:m:111:134 3:k 3:m:121:141 3:m:124:141 3:k 3:k 3:i 3:i "
                "3:f 3:m:142:-1 3:f 3:m:145:-1 "),
    Ffmia=(4, "1:m:-1:9 0:m:-1:5 0:m:-1:10 0:m:-1:12 0:a 0:F 1:m:4:15 0:i 0:m:6:18 0:i "
              "0:m:9:22 0:F 1:m:16:31 0:f 0:m:20:33 0:f 0:m:22:33 1:a 1:m:25:43 1:F 0:m:29:41 "
              "1:i 1:i 1:m:37:50 1:F 1:m:40:54 1:f 1:m:42:57 1:m:45:56 3:m:45:59 2:m:42:58 1:f "
              "2:a 2:F 2:m:53:63 2:m:49:65 3:m:54:68 2:i 2:m:56:67 2:i 2:m:59:75 2:F 3:m:66:83 "
              "2:f 2:m:70:83 2:f 2:m:72:84 3:a 3:m:75:93 3:F 2:m:79:95 3:i 3:i 3:m:85:-1 3:F "
              "3:m:90:-1 3:f 3:m:92:-1 3:m:95:-1 3:f "),
    mia=(4, "1:m:-1:3 0:m:-1:8 0:m:-1:6 0:m:-1:7 0:m:-1:8 0:i 1:m:0:13 0:m:2:10 0:a 0:i "
            "1:m:5:16 2:m:8:25 1:i 1:m:9:22 0:m:10:23 0:m:8:20 1:m:8:20 3:m:11:25 1:a "
            "2:m:13:27 1:i 1:m:14:22 1:m:17:25 0:m:14:22 1:m:17:25 2:m:14:28 2:m:13:27 2:i "
            "3:m:18:32 2:m:20:32 2:a 2:i 3:m:23:-1 3:m:25:-1 3:m:25:-1 3:i 2:m:28:-1 2:m:27:-1 "
            "3:a 3:i 3:m:32:-1 3:m:35:-1 2:m:33:-1 3:m:35:-1 "),
    iaz=(4, "0:i 0:i 1:i 1:i 0:z 2:i 2:i 1:z 3:i 3:i 2:z 0:a 1:a 2:a 3:a 3:z"),
)
ROW_CHUNKS = ((0, 128), (128, 256), (256, 384), (384, 512), (512, D))
MID, SPAN, EARLY, LAG, CUT, END = 480, 30, 8, 16, 12, 76
NT_DIMS = (((1,), (1,)), ((), ()))


def _round_res(step):
    return [int(np.round(r / step)) * step for r in range(16)]


RES1, RES2, RES3 = _round_res(2), _round_res(4), _round_res(8)


def _ds(start, size):
    return pl.ds(start if isinstance(start, int) else pl.multiple_of(start, size), size)


def _iota(shape, dim):
    return jax.lax.broadcasted_iota(I32, shape, dim)


def _rbf(x):
    return x.astype(BF16).astype(F32)


def _cmul(a, b):
    return (a[0] * b[0] - a[1] * b[1], a[0] * b[1] + a[1] * b[0])


def _csq(a):
    t = a[0] * a[1]
    return ((a[0] + a[1]) * (a[0] - a[1]), t + t)


def _cadd(a, b):
    return (a[0] + b[0], a[1] + b[1])


def _csub(a, b):
    return (a[0] - b[0], a[1] - b[1])


def _bfly4(a0, a1, a2, a3, inverse=False):
    s02, d02 = _cadd(a0, a2), _csub(a0, a2)
    s13, d13 = _cadd(a1, a3), _csub(a1, a3)
    p = (d02[0] - d13[1], d02[1] + d13[0])
    m = (d02[0] + d13[1], d02[1] - d13[0])
    if inverse:
        p, m = m, p
    return _cadd(s02, s13), p, _csub(s02, s13), m


def _prod_mod_1(a, b):
    fa, fb = _bfly4(*a), _bfly4(*b)
    return _bfly4(*[_cmul(x, y) for x, y in zip(fa, fb)], inverse=True)


def _prod2(a0, a1, b0, b1, sgn):
    p00, p11 = _cmul(a0, b0), _cmul(a1, b1)
    c1 = _cadd(_cmul(a0, b1), _cmul(a1, b0))
    if sgn > 0:
        return (p00[0] - p11[1], p00[1] + p11[0]), c1
    return (p00[0] + p11[1], p00[1] - p11[0]), c1


def _prod_mod_m1(a, b):
    def split(x):
        p = [(x[k][0] - x[k + 2][1], x[k][1] + x[k + 2][0]) for k in range(2)]
        m = [(x[k][0] + x[k + 2][1], x[k][1] - x[k + 2][0]) for k in range(2)]
        return p, m
    ap, am = split(a)
    bp, bm = split(b)
    cp = _prod2(*ap, *bp, 1)
    cm = _prod2(*am, *bm, -1)
    lo = [_cadd(cp[k], cm[k]) for k in range(2)]
    hi = [(cp[k][1] - cm[k][1], cm[k][0] - cp[k][0]) for k in range(2)]
    return lo + hi


def _prod_mod_i(a, b, sgn):
    sm = [x[0] + x[1] for x in b]
    df = [x[1] - x[0] for x in b]
    asum = [x[0] + x[1] for x in a]
    out = []
    for k in range(4):
        acc = [None, None, None]
        for j in range(4):
            m = (k - j) % 4
            if j <= k:
                t = ((b[m][0], 1), (df[m], 1), (sm[m], 1))
            elif sgn > 0:
                t = ((b[m][1], -1), (sm[m], 1), (df[m], -1))
            else:
                t = ((b[m][1], 1), (sm[m], -1), (df[m], 1))
            for q, (v, (w, s)) in enumerate(zip((asum[j], a[j][0], a[j][1]), t)):
                p = v * w
                if acc[q] is None:
                    acc[q] = p
                else:
                    acc[q] = acc[q] + p if s > 0 else acc[q] - p
        out.append((acc[0] - acc[2], acc[0] + acc[1]))
    return out


def _barrel(v, sch):
    for bit in range(4):
        m = sch.mask("bit%d" % bit)
        v = [jnp.where(m, v[(i + (1 << bit)) % 16], v[i]) for i in range(16)]
    return [v[-s % 16] for s in range(16)]


def _to_residues(tiles, sch):
    return _barrel([t if j == 0 else pltpu.roll(t, j, 1) for j, t in enumerate(tiles)], sch)


def _to_time(res, sch):
    return [t if j == 0 else pltpu.roll(t, 128 - j, 1)
            for j, t in enumerate(_barrel(res, sch))]


def _gather(x, idx, axis=1):
    return jnp.take_along_axis(x, idx, axis=axis, mode="promise_in_bounds")


def _transpose_dft(wt_ref, wu_ref, residues):
    for s in residues:
        for p in range(2):
            wt_ref[4 * (s % 4) + (0, 2, 1, 3)[s // 4], p, 0:64] = pltpu.bitcast(
                _mxu(wu_ref.bitcast(I32)[p, 4 * (s % 4) + s // 4, 0:64]).T, I32)


def _init_dft(wu_ref, wk_ref, tmp_ref, halfway):
    sub, k4 = _iota((8, 128), 0), 4 * _iota((8, 128), 1) + 1

    def cis(t):
        ph = ((k4 * t) & (4 * L - 1)).astype(F32) * (2 * np.pi / (4 * L))
        return jnp.cos(ph), jnp.sin(ph)

    w1, w16 = cis(1), cis(16)
    w32 = _csq(w16)
    fk = [cis(16 * (32 * (sub & 3) + (sub >> 2)))]
    fu = [cis(128 * sub), cis(128 * (sub + 8))]
    for v in range(1, 16):
        fk.append(_cmul(fk[-1], w32))
        if v >= 2:
            fu.append(_cmul(fu[-2], w16))
    for p in range(2):
        for v in range(32):
            tmp_ref[p, 8 * v:8 * v + 8, :] = fu[v % 16][p]
    tw = None
    for s in range(16):
        for v in range(0, 16, 2):
            rows = [slice(128 - s + 8 * i, 136 - s + 8 * i) for i in (v, v + 1)]
            for ref, f in ((wk_ref, fk[v:v + 2]),
                           (wu_ref, [(tmp_ref[0, r, :], tmp_ref[1, r, :]) for r in rows])):
                if s:
                    f = [_cmul(x, tw) for x in f]
                for p in range(2):
                    ref[p, 4 * (s % 4) + s // 4, 8 * v:8 * v + 16, :] = jnp.concatenate(
                        [f[0][p], f[1][p]], axis=0).astype(BF16)
        tw = _cmul(tw, w1) if s else w1
        if s == 7:
            halfway()


def _pack(ref, n, a, b):
    ref[n] = jnp.concatenate([a, b], axis=0).astype(BF16)
    return ref.bitcast(I32)[n]


def _split(w):
    return [pltpu.bitcast(w << 16, F32), pltpu.bitcast(w & -65536, F32)]


FINE = (0, 1, 2, 3, 4, 5, 6, 7, 512, 516, 1024, 1536)


def _k_seeds(z, c, sch):
    pw = {1: z}
    for e in range(1, 10):
        pw[1 << e] = _csq(pw[1 << (e - 1)])
    c8, z16 = _cmul(c, pw[8]), (pw[16][0], 0.0 - pw[16][1])
    pair = lambda a, b: tuple(jnp.where(sch.mask("odd"), q, p) for p, q in zip(a, b))
    seeds = []
    for g in range(2):
        twice = lambda v: tuple(_gather(x, sch.idx("dup%d" % g), 0) for x in v)
        seeds.append([twice(z), twice(pw[32]), twice(pw[512]),
                      pair(twice(c), twice(c8)), pair((1.0, 0.0), twice(z16))])
    return seeds


def _mxu(words):
    return pltpu.bitcast(words, BF16)


def _store_table(ref, tab):
    for i in range(0, len(tab), 2):
        for p in range(2):
            ref[p, 8 * i:8 * i + 16, :] = jnp.concatenate(
                [tab[i][p], tab[i + 1][p]], axis=0).astype(BF16)


def _k_residues(groups, k_last, dskip, tmp_ref, sch):
    idx, nxt = sch.idx("src"), sch.idx("nxt")
    low = lambda x, y: (x & 65535) | (y << 16)
    high = lambda x, y: jax.lax.shift_right_logical(x, 16) | (y & -65536)
    kv, up = {}, {}
    for i, k in enumerate(FINE):
        v = [g[8 * i:8 * i + 8] for g in groups]
        if k == 0:
            v = [x + jnp.where(sch.mask("diag"),
                               _gather(dskip[n // 2], sch.idx("dup%d" % (n % 2)), 0), 0.0)
                 for n, x in enumerate(v)]
        p = [_pack(tmp_ref, 2 * i + h, v[2 * h], v[2 * h + 1]) for h in range(2)]
        both = [_gather(x, idx) for x in p]
        kv[k], kv[k + 8] = low(*both), high(*both)
        if k % 512 == 0:
            up[k] = low(*[_gather(x, nxt) for x in p])
    k_last = _gather(k_last, sch.idx("rows"), 0)
    q0, q1, q2, up0, up01, up2, up3, fine = map(sch.mask, INDEX[-8:])
    s3 = {r: jnp.where(q2, kv[1024 + r], kv[1536 + r]) for r in (0, 8)}
    v0 = jnp.where(q0, kv[0], jnp.where(q1, kv[512], s3[0]))
    v16 = jnp.where(up01, jnp.where(up0, up[0], up[512]),
                    jnp.where(up2, up[1024], jnp.where(up3, up[1536], k_last)))
    s3[16] = v16
    s23, s123, out = {}, {}, [v0]
    for r in range(1, 16):
        k23 = (RES2[r], RES3[r])
        if k23 not in s23:
            s23[k23] = v16 if k23 == (16, 16) else jnp.where(q1, kv[512 + k23[0]], s3[k23[1]])
        k123 = (RES1[r],) + k23
        if k123 not in s123:
            s123[k123] = v16 if k123[0] == 16 else jnp.where(q0, kv[k123[0]], s23[k23])
        if RES1[r] == r:
            out.append(s123[k123])
        else:
            out.append(jnp.where(fine, kv[r], s123[k123]))
    return out


def _ln_scalars(s1, s2):
    mean = s1 * (1.0 / D)
    var = jnp.maximum(s2 * (1.0 / D) - mean * mean, 0.0)
    eps = float(np.asarray(EPS, dtype=BF16))
    sd = _rbf(jnp.sqrt(_rbf(_rbf(var) + eps)))
    return _rbf(mean), 1.0 / sd


def _top8(x):
    def swap(v, pairs):
        for i, j in pairs:
            v[i], v[j] = jnp.maximum(v[i], v[j]), jnp.minimum(v[i], v[j])
        return v

    def merge(a, b):
        v = [jnp.maximum(a[i], b[7 - i]) for i in range(8)]
        return swap(v, [(i, i + d) for d in (4, 2, 1) for i in range(8) if not i & d])

    sort8 = ((0, 2), (1, 3), (4, 6), (5, 7), (0, 4), (1, 5), (2, 6), (3, 7), (0, 1), (2, 3),
             (4, 5), (6, 7), (2, 4), (3, 5), (1, 4), (3, 6), (1, 2), (3, 4), (5, 6))
    v = merge(*[swap(x[i:i + 8], sort8) for i in (0, 8)])
    for d in (4, 2, 1):
        v = merge(v, [pltpu.roll(t, d, 0) for t in v])
    return v


def _init_columns(col_ref, wx_ref, wy_ref, ldt_ref, dsk_ref, wr_ref):
    row, lane = _iota((128, 128), 0), _iota((128, 128), 1)
    split = (row & ~15) + 2 * (row & 7) + ((row >> 3) & 1)
    ldt, dsk, wr = (ref[...].astype(F32).reshape(1, D) for ref in (ldt_ref, dsk_ref, wr_ref))
    for n, vec in enumerate((jnp.exp(ldt), dsk * (1.0 / L))):
        for lo in range(0, D, 128):
            i = min(lo, D - 128)
            diag = jnp.where(split == lane, vec[:, i:i + 128], 0.0)[lo - i:].astype(BF16)
            col_ref[n, lo:i + 128, :] = jnp.dot(diag, jnp.ones((128, 128), BF16),
                                                preferred_element_type=F32)
    sub = _iota((16, D), 0)
    ones_w = jnp.where(sub == 0, 1.0, jnp.where(sub == 1, wr, 0.0))
    wx_ref[...] = ones_w.astype(BF16)
    for lo in range(0, D, MB):
        wy_ref[lo // MB, :, 0:MB] = ones_w[:, lo:lo + MB].astype(BF16)
        wy_ref[lo // MB, :, MB:] = jnp.zeros((16, 128 - MB), BF16)


INDEX = ("true", "bit0", "bit1", "bit2", "bit3", "odd", "dup0", "dup1", "rows", "src", "nxt",
         "diag", "q0", "q1", "q2", "up0", "up01", "up2", "up3", "fine")


def _init_index(idx_ref):
    sub, lane = _iota((8, 128), 0), _iota((8, 128), 1)
    src = lambda b: 8 * ((b >> 1) & 15) + 2 * (sub & 3) + (b & 1)
    is_ = lambda m: jnp.where(m, 1, 0)
    q = lane & 3
    q16 = q + is_(lane >= 124)
    tiles = dict(true=sub + 1, odd=sub & 1, dup0=sub >> 1, dup1=4 + (sub >> 1),
                 rows=2 * (sub & 3) + (sub >> 2), src=src(lane >> 2), nxt=src((lane >> 2) + 1),
                 diag=is_((lane == sub) & ((sub & 1) == 0)), up01=is_(q16 < 2),
                 fine=is_((q == 0) & (lane < 64)),
                 **{"bit%d" % n: (lane >> n) & 1 for n in range(4)},
                 **{"q%d" % n: is_(q == n) for n in range(3)},
                 **{"up%d" % n: is_(q16 == n) for n in (0, 2, 3)})
    for n, name in enumerate(INDEX):
        idx_ref[n] = tiles[name]


class _Schedule:
    def __init__(self, zero, idx_ref):
        self.zero = zero
        self.idx = lambda name: idx_ref[INDEX.index(name) + zero]
        self.mask = lambda name: self.idx(name) != 0
        self.true = self.mask("true")
        self.done, self.pending, self.wait = [], {}, -1

    def tie(self, x, token):
        return jnp.where(self.true, x, token if token.dtype == x.dtype
                         else pltpu.bitcast(token, x.dtype))

    def start(self, x):
        return self.tie(x, self.done[self.wait]) if 0 <= self.wait < len(self.done) else x

    def lhs(self, words, first):
        tiles = [words[i:i + 8] for i in range(0, words.shape[0], 8)]
        for i in range(len(tiles) if first else 0):
            for token in self.pending.pop(len(self.done) + i, ()):
                tiles[i] = self.tie(tiles[i], token)
        return _mxu(jnp.concatenate(tiles, axis=0))

    def results(self, v):
        self.done += [v[i + 8:i + 16] for i in range(0, v.shape[0], 16)]

    def run(self, stage, wait, before):
        self.wait = wait
        self.pending.setdefault(before, []).extend(next(stage))


def _kernel(x_hbm, are_hbm, aim_hbm, bre_hbm, bim_hbm, cre_hbm, cim_hbm,
            ldt_hbm, dsk_hbm, wr_hbm, wg_hbm, wu_hbm, wd_hbm, out_hbm,
            x_v, wg_v, wu_v, wd_v, par_v, ldt_v, dsk_v, wr_v, w_v, wk_v, wt_v, col_v, wx_v, wy_v,
            tmp_v, idx_v, pk_v, h_v, st_v, acc_v, sq_v, out_v, sd0, sd1, ta0, ta1, tb0, tb1,
            kl0, kl1,
            u0, u1, k0, k1, a0_v, a1_v, c0, c1, r0, r1, r2, r3,
            sem_p, sem_x, sem_w, sem_o, f0_v, f1_v, *rest):
    half_v, new_v = rest[:4], rest[4:]
    cp_vec = [pltpu.make_async_copy(s, d, sem_p.at[n]) for n, (s, d) in enumerate(
        ((ldt_hbm, ldt_v), (dsk_hbm, dsk_v), (wr_hbm, wr_v)))]
    cp_par = [[pltpu.make_async_copy(s.at[lo:hi], par_v.at[n, lo:hi], sem_p.at[3 + 6 * m + n])
               for n, s in enumerate((are_hbm, aim_hbm, bre_hbm, bim_hbm, cre_hbm, cim_hbm))]
              for m, (lo, hi) in enumerate(((0, 4 * MB), (4 * MB, D)))]
    cp_x = [pltpu.make_async_copy(x_hbm.at[:, 128 * j:128 * j + 128], x_v.at[j, 0:D],
                                  sem_x.at[j])
            for j in range(NT)]
    cp_d = pltpu.make_async_copy(wd_hbm, wd_v, sem_w.at[2])

    def cp_w(i):
        return [pltpu.make_async_copy(s.at[:, _ds(128 * i, 128)], d.at[i, 0:D], sem_w.at[n])
                for n, (s, d) in enumerate(((wg_hbm, wg_v), (wu_hbm, wu_v)))]

    for cp in cp_vec + cp_par[0]:
        cp.start()
    for cp in cp_x[:NT // 2]:
        cp.start(priority=1)

    def columns():
        for cp in cp_vec:
            cp.wait()
        for cp in cp_x[NT // 2:]:
            cp.start(priority=1)
        _transpose_dft(wt_v, w_v, range(4))
        _init_columns(col_v, wx_v, wy_v, ldt_v, dsk_v, wr_v)

    _init_dft(w_v, wk_v, tmp_v, columns)
    for cp in cp_par[0]:
        cp.wait()

    sd, ta, tb, kl = (sd0, sd1), (ta0, ta1), (tb0, tb1), (kl0, kl1)
    uk, ab, cc, xr = ((u0, u1), (k0, k1)), ((a0_v, a1_v), (f0_v, f1_v)), (c0, c1), (r0, r1, r2, r3)
    ww, wt_w = (w_v.bitcast(I32), wk_v.bitcast(I32)), wt_v

    def seed_stage(b, r, sch):
        rows = _ds(b * MB // 2 + 8 * r, 8)
        par = [_split(par_v.bitcast(I32)[n, rows, :]) for n in range(6)]
        for h in range(2):
            a_re, a_im, b_re, b_im, c_re, c_im = [v[h] for v in par]
            dt = sch.start(col_v[0, _ds(b * MB + 16 * r + 8 * h, 8), :])
            mag, ang = jnp.exp(dt * a_re), dt * a_im
            sc = dt * (1.0 / L)
            seeds = _k_seeds((mag * jnp.cos(ang), mag * jnp.sin(ang)),
                             _cmul((c_re, c_im), (sc * b_re, sc * b_im)), sch)
            for g in range(2):
                for n, v in enumerate(seeds[g]):
                    for p in range(2):
                        sd[b % 2][r, 2 * h + g, 2 * n + p] = v[p]
            yield [sd[b % 2][(r + sch.zero), 2 * h, 0]]

    def table_stage(b, r, sch):
        tail = []
        for g in range(4):
            m1, m32, m512, a0, b0 = [
                (sd[b % 2][r, g, 2 * n], sd[b % 2][r, g, 2 * n + 1]) for n in range(5)]
            m32 = (sch.start(m32[0]), m32[1])
            fa = [a0]
            for _ in range(7):
                fa.append(_cmul(fa[-1], m1))
            for src in (0, 4, 8, 10):
                fa.append(_cmul(fa[src], m512))
            tail.append(fa[11][0] * m512[0] - fa[11][1] * m512[1])
            _store_table(ta[b % 2].at[r, g], fa)
            fb = [b0]
            for _ in range(15):
                p = fb[-1]
                fb.append((p[0] * m32[0] + p[1] * m32[1], p[1] * m32[0] - p[0] * m32[1]))
            _store_table(tb[b % 2].at[r, g], fb)
            yield [ta[b % 2].bitcast(I32)[(r + sch.zero), g, 0, 0:8, :],
                   tb[b % 2].bitcast(I32)[(r + sch.zero), g, 0, 0:8, :]]
        last = [jnp.where(sch.mask("odd"), pltpu.roll(tail[h + 1], 1, 0), tail[h])
                for h in (0, 2)]
        last = [pltpu.bitcast(_rbf(jnp.broadcast_to(jnp.sum(v, axis=1, keepdims=True),
                                                    (8, 128))), I32) for v in last]
        kl[b % 2][r] = jax.lax.shift_right_logical(last[0], 16) | last[1]

    def kernel_stage(b, r, sch):
        ta_w, tb_w = ta[b % 2].bitcast(I32), tb[b % 2].bitcast(I32)
        groups = [None] * 4
        for g0 in (0, 2):
            res = [jax.lax.dot_general(sch.lhs(ta_w[r, g, p, 0:48], g == g0 and p == 0),
                                       _mxu(tb_w[r, g, p, 0:64]), NT_DIMS, preferred_element_type=F32)
                   for g in (g0, g0 + 1) for p in range(2)]
            groups[g0], groups[g0 + 1] = res[0] + res[1], res[2] + res[3]
            sch.results(groups[g0 + 1])
            yield []
        dskip = [col_v[1, _ds(b * MB + 16 * r + 8 * h, 8), :] for h in range(2)]
        dst = _ds(8 * r, 8)
        res = _k_residues(groups, kl[b % 2][r], dskip, pk_v.at[sch.slot, 0], sch)
        for s, t in enumerate(res):
            uk[1][b % 2][4 * (s % 4) + s // 4, dst, :] = t
        yield [uk[1][b % 2][0, _ds(8 * (r + sch.zero), 8), :]]

    def norm_stage(b, r, sch):
        rows, dst = _ds(b * MB // 2 + 8 * r, 8), _ds(8 * r, 8)
        tiles = [x_v.bitcast(I32)[j, rows, :] for j in range(NT)]
        for s, t in enumerate(_to_residues([sch.start(tiles[0])] + tiles[1:], sch)):
            xr[b % 4][4 * (s % 4) + s // 4, dst, :] = t
            xs, m, inv = _mxu(t).astype(F32), st_v[s, 0], st_v[s, 1]
            uk[0][b % 2][4 * (s % 4) + s // 4, _ds(16 * r, 16), :] = jnp.concatenate(
                [(xs[0:8] - m) * inv, (xs[8:16] - m) * inv], axis=0).astype(BF16)
        yield [uk[0][b % 2].bitcast(I32)[0, _ds(8 * (r + sch.zero), 8), :]]

    def forward_stage(w, b, k, sch):
        dst = ab[w][b % len(ab[w])]
        for p in range(2):
            v = [jnp.dot(sch.lhs((uk[w][b % 2] if w else uk[w][b % 2].bitcast(I32))[
                4 * k + n, 0:MB // 2], n == 0),
                         _mxu(ww[w][p ^ (n & 1), 4 * k + n, 0:64]),
                         preferred_element_type=F32) for n in range(4)]
            d02, d13 = v[0] - v[2], v[1] - v[3]
            x1 = d02 - d13 if p == 0 else d02 + d13
            dst[0, k, p, 0:MB] = v[0] + v[2]
            dst[2, k, 1 - p, 0:MB] = v[1] + v[3]
            dst[1, k, p, 0:MB] = x1
            dst[3, k, p, 0:MB] = d02 + d13 if p == 0 else d02 - d13
            sch.results(x1)
            yield []

    def stats(tiles, sch):
        ones_w = wx_v.bitcast(I32)[...]
        for j in tiles:
            acc = None
            for i in range(0, D // 2, 8):
                v = [t * t for t in _split(x_v.bitcast(I32)[j, i:i + 8, :])]
                acc = v if acc is None else [p + q for p, q in zip(acc, v)]
            sums = jnp.dot(_mxu(jnp.concatenate(
                [ones_w[:, :128] if j % 2 == 0 else sch.tie(ones_w[:, :128], prev),
                 ones_w[:, 128:]], axis=1)),
                           _mxu(x_v.bitcast(I32)[j, 0:D // 2]), preferred_element_type=F32)
            s2 = prev = acc[0] + acc[1]
            for d in (4, 2, 1):
                s2 = s2 + pltpu.roll(s2, d, 0)
            st_v[j, 0], st_v[j, 1] = _ln_scalars(jnp.broadcast_to(sums[0:1], (8, 128)), s2)

    def middle_stage(b, r, sch):
        src = [v[b % len(v)] for v in ab]
        scale = lambda v, f: [(x[0] * f, x[1] * f) for x in v]
        for h in range(2):
            ra = _ds(16 * r + 8 * h, 8)
            ld = lambda q, w, ra=ra: [(src[w][q, k, 0, ra, :], src[w][q, k, 1, ra, :]) for k in range(4)]

            park_v = half_v[2 * (sch.slot % 2) + h]

            def put(q, y):
                x = [park_v[n + sch.zero] for n in range(8)]
                for k in range(4):
                    for p in range(2):
                        cc[b % 2][k, q, p, ra, :] = x[2 * k + p] + y[k][p]
                        cc[b % 2][k, q + 2, p, ra, :] = x[2 * k + p] - y[k][p]

            def park(x):
                for k in range(4):
                    for p in range(2):
                        park_v[2 * k + p] = x[k][p]
                return [park_v[sch.zero]]

            gate = sch.start
            a0, a2, b0, b2 = ld(0, 0), ld(2, 0), ld(0, 1), ld(2, 1)
            a0[0] = (gate(a0[0][0]), a0[0][1])
            e0 = _prod_mod_1(list(map(_cadd, a0, a2)), list(map(_cadd, b0, b2)))
            again = _ds(16 * (r + sch.zero) + 8 * h, 8)
            yield park(e0)
            a0, a2, b0, b2 = (ld(q, w, again) for w in range(2) for q in (0, 2))
            a2[0] = (gate(a2[0][0]), a2[0][1])
            e2 = _prod_mod_m1(list(map(_csub, a0, a2)), scale(map(_csub, b0, b2), 2.0))
            put(0, e2)
            yield [cc[b % 2][0, 0, 0, again, :]]
            four = sch.start(jnp.full((8, 128), 4.0, F32))
            e1 = _prod_mod_i(ld(1, 0), scale(ld(1, 1), four), 1)
            yield park(e1)
            four = sch.start(jnp.full((8, 128), 4.0, F32))
            e3 = _prod_mod_i(ld(3, 0), scale(ld(3, 1), four), -1)
            put(1, e3)
            yield [cc[b % 2][0, 1, 0, again, :]]

    def inverse_stage(b, k, sch):
        src = cc[b % 2]

        def lhs(v, n, first):
            return sch.lhs(jnp.concatenate(
                [_pack(pk_v.at[sch.slot, 2], 4 * n + i // 16, v[i:i + 8], v[i + 8:i + 16])
                 for i in range(0, MB, 16)], axis=0), first)

        for o in range(2):
            p0, p1 = [(src[k, q, 0, 0:MB], src[k, q, 1, 0:MB]) for q in (2 * o, 2 * o + 1)]
            if o == 0:
                e = {0: _cadd(p0, p1), 2: _csub(p0, p1)}
            else:
                e = {1: (p0[0] + p1[1], p0[1] - p1[0]), 3: (p0[0] - p1[1], p0[1] + p1[0])}
            ys = []
            for n in e:
                y = [jnp.dot(lhs(e[n][p], 2 * n + p, n == o and p == 0),
                             _mxu(wt_w[4 * k + (0, 2, 1, 3)[n], p, 0:64]),
                             preferred_element_type=F32)
                     for p in range(2)]
                h = y[0] + y[1] + _mxu(xr[b % 4][4 * k + n, 0:MB // 2]).astype(F32)
                h_v[k + 4 * n, b * MB:b * MB + MB, :] = h.astype(BF16)
                hh = h * h
                sq_v[k + 4 * n] += sum((hh[i:i + 8] for i in range(8, MB, 8)), hh[0:8])
                ys.append(h)
            sch.results(ys[-1])
            yield []

    def sum_stage(b, r, sch):
        for n in range(4):
            s = r + 4 * n if b == nb - 1 else 4 * r + n
            sums = jnp.dot(sch.lhs(wy_v.bitcast(I32)[b], n == 0)[:, :MB],
                           _mxu(h_v.bitcast(I32)[s, b * MB // 2:(b + 1) * MB // 2]),
                           preferred_element_type=F32)
            acc_v[s] += sums[0:8]
        sch.results(sums)
        yield []

    nb = D // MB
    stages = dict(
        s=(seed_stage, 0), t=(table_stage, 1), k=(kernel_stage, 2),
        F=(functools.partial(forward_stage, 1), 3), n=(norm_stage, 2),
        f=(functools.partial(forward_stage, 0), 3), m=(middle_stage, 4),
        i=(inverse_stage, 5), a=(sum_stage, 6))

    def run(step, zero, live=None):
        live = live or {n: (f, step - lag) for n, (f, lag) in stages.items()
                        if 0 <= step - lag < nb and (n, step) != ("n", 2)}
        if step == nb + 4:
            live["z"] = (sum_stage, nb - 1)
        unroll, plan = PLANS["".join(live)]

        def body(it, carry):
            sch = _Schedule(zero >> (step % 32) if unroll == 4 else zero & it, idx_v)
            gens = [{n: f(b, it * unroll + u, sch) for n, (f, b) in live.items()}
                    for u in range(unroll)]
            if step == 3:
                for i in range(9 * unroll):
                    for cp in cp_w(9 * unroll * it + i):
                        cp.start()
            for item in plan.split():
                u, n, *ties = item.split(":")
                if n in live:
                    sch.slot = int(u)
                    sch.run(gens[int(u)][n], *map(int, ties or (-1, -1)))
            for sch.slot, g in enumerate(gens):
                for v in g.values():
                    for _ in v:
                        pass
            return carry + it

        if unroll == 4:
            if step == 101 or step > nb + 3:
                return body(0, 0)
            return jax.lax.fori_loop(zero, 1, lambda _, c: body(0, c), 0)
        return jax.lax.fori_loop(0, 4 // unroll, body, 0)

    _init_index(idx_v)
    acc_v[...] = sq_v[...] = jnp.zeros(acc_v.shape, F32)
    zero = run(0, 0) - 1
    for step in range(1, nb + 5):
        if step == 4:
            for cp in cp_par[1]:
                cp.wait()
        if step == 3:
            for half in range(2):
                tiles = range(NT // 2 * half, NT // 2 * (half + 1))
                for j in tiles:
                    cp_x[j].wait()
                if half:
                    cp_d.start(priority=1)
                else:
                    for cp in cp_par[1]:
                        cp.start()
                _transpose_dft(wt_v, w_v, range(4 + 6 * half, 10 + 6 * half))
                stats(tiles, _Schedule(zero, idx_v))
            for q in range(2):
                for s, v in enumerate(_to_residues([st_v[j, q] for j in range(NT)],
                                                   _Schedule(zero, idx_v))):
                    st_v[s, q] = v
            run(101, zero, dict(n=(norm_stage, 0)))
        run(step, zero)

    sums = [acc_v[s] for s in range(16)]
    m2, inv2 = _ln_scalars(
        jnp.concatenate([v[0:1] for v in sums], axis=0),
        jnp.concatenate([jnp.sum(sq_v[j], axis=0, keepdims=True) for j in range(NT)], axis=0))
    wsum = jnp.sum(wr_v[...].astype(F32).reshape(1, D), axis=1, keepdims=True)
    score = _rbf((jnp.concatenate([v[1:2] for v in sums], axis=0) - m2 * wsum) * inv2 + 0.0)
    bits = pltpu.bitcast(score, I32) >> 16
    order = jnp.where(bits < 0, -1 - bits, bits + 32768)
    mu = (_iota((NT, 128), 1) - _iota((NT, 128), 0)) & 127
    pos = 128 * (mu & 15) + 16 * (mu >> 4) + _iota((NT, 128), 0)
    key = pltpu.bitcast((order << 11) + (L - 1 - pos) + (1 << 29), F32)

    h_w, out_w = h_v.bitcast(I32), out_v.bitcast(I32)
    sch, done = _Schedule(zero, idx_v), []
    tie = sch.tie

    def unrouted():
        for q, v in enumerate((1.0 + inv2, m2 * inv2)):
            for j, t in enumerate(_to_time(
                    [jnp.broadcast_to(v[s:s + 1], (8, 128)) for s in range(16)], sch)):
                st_v[j, q] = t
        for i in range(0, D, 16):
            scal = st_v.at[pl.ds(zero * (i + 1), NT)]
            tiles = [h_w[s, i // 2:i // 2 + 8, :] for s in range(16)]
            if len(done) > LAG:
                tiles[0] = tie(tiles[0], done[-LAG])
            for j, v in enumerate(_to_time(tiles, sch)):
                h, mul, sub = _mxu(v).astype(F32), scal[j, 0], scal[j, 1]
                out_v[j, i:i + 16, :] = jnp.concatenate(
                    [h[0:8] * mul - sub, h[8:16] * mul - sub], axis=0).astype(BF16)
                if j % 8 == 7:
                    yield pltpu.bitcast(out_w[j + zero, i // 2:i // 2 + 8, :], F32)

    side = unrouted()

    lane8, sub8 = _iota((CAP, 128), 1), _iota((CAP, 128), 0)
    best = _top8([pltpu.roll(key[i:i + 8], n, 1) if n else key[i:i + 8]
                  for i in (0, 8) for n in range(8)])
    cand = best[0]
    for c in range(1, CAP):
        cand = jnp.where(sub8 == c, best[c], cand)
    best = _top8([pltpu.roll(cand, n, 1) if n else cand for n in range(0, 128, 8)])
    for _ in range(2 * EARLY):
        best[-1] = tie(best[-1], next(side))
    best = [pltpu.bitcast(v, I32)[0, 0] for v in best]
    picks = [L - 1 - (v & (L - 1)) for v in best]

    def schedule(col):
        rnd = [sum([(col[e] == col[c]).astype(I32) for e in range(c)], 0) for c in range(CAP)]
        return (rnd, functools.reduce(jnp.maximum, rnd) + 1,
                lambda n: [lane8 == jnp.where(rnd[c] == n, col[c], -1) for c in range(CAP)])

    _, rounds, lanes = schedule([((t >> 7) + (t & 127)) & 127 for t in picks])

    def out_copy(q, lo, hi):
        j = order[q]
        return pltpu.make_async_copy(
            out_v.at[j, lo:hi], out_hbm.at[lo:hi, _ds(j * 128, 128)], sem_o)

    for n, ref in enumerate((wg_v, wu_v)):
        pltpu.make_async_copy(ref.at[:, 0:D], ref.at[:, 0:D], sem_w.at[n]).wait()

    def gather(n, acc):
        masks = lanes(n)
        tiles = []
        for i in range(0, D // 2, 8):
            v = jnp.zeros((8, 128), I32)
            for c in range(CAP):
                v = jnp.where(masks[c], h_w[picks[c] & 15, i:i + 8, :], v)
            tiles.append(v)
        lhs = jnp.zeros((CAP, 128), F32)
        for c in range(CAP):
            lhs = jnp.where(masks[c] & (sub8 == c), 1.0, lhs)
        aux = [jnp.zeros((CAP, 128), F32)] * 3
        for c in range(CAP):
            hit = pltpu.bitcast(key, I32) == best[c]
            aux = [jnp.where(sub8 == c, jnp.sum(jnp.where(hit, v, 0.0), axis=0, keepdims=True), a)
                   for a, v in zip(aux, (m2, inv2, score))]
        return (acc[0] + jax.lax.dot_general(lhs.astype(BF16), _mxu(jnp.concatenate(tiles, axis=0)),
                                             NT_DIMS, preferred_element_type=F32),
                *[jnp.sum(a, axis=1, keepdims=True) for a in aux])

    h_sel, m_sel, inv_sel, score_sel = jax.lax.fori_loop(
        0, rounds, gather, (jnp.zeros((CAP, D), F32), *[jnp.zeros((CAP, 1), F32)] * 3))
    x_sel = _rbf((h_sel - m_sel) * inv_sel)
    gate = _rbf(jax.nn.sigmoid(score_sel))

    tile, col = [t >> 7 for t in picks], [t & 127 for t in picks]
    rnd, rounds, lanes = schedule(col)
    late, again = 0, []
    for j in tile:
        again.append((late >> j) & 1)
        late = late | (1 << j)
    for dup in again[1:]:
        late = late | (late + dup)
    order = []
    for left in (late ^ ((1 << NT) - 1), late):
        for _ in range(CAP):
            order.append((31 - jax.lax.clz(left)) & (NT - 1))
            left = left ^ (1 << order[-1])

    def early_copies(n):
        lo, hi = (0, 16 * EARLY, MID, D)[n:n + 2]
        return [out_copy(q, lo, hi) for q in range(CAP)]

    def start(copies):
        for cp in copies:
            cp.start()

    start(early_copies(0))
    rate, sent = MID // 8 - 2 * EARLY, [0]

    def project(w_ref):
        parts = []
        for n in range(0, FF // 128, 4):
            for lo in range(0, D, 128):
                hi = min(lo + 128, D)
                xs = x_sel[:, lo:hi]
                if hi - lo == 128 and min(rate, (len(done) - 4) * rate // END) > sent[0]:
                    sent[0] += 1
                    xs = tie(xs, next(side))
                w = [w_ref.bitcast(I32)[i, lo // 2:hi // 2, :] for i in range(n, n + 4)]
                v = jnp.dot(xs.astype(BF16), _mxu(jnp.concatenate(w, axis=1)),
                            preferred_element_type=F32)
                done.append(v[:, 0:128])
                acc = acc + v if lo else v
            parts.append(acc)
        return _rbf(jnp.concatenate(parts, axis=1))

    g = project(wg_v)
    act = _rbf(g * jax.nn.sigmoid(g)) * project(wu_v)
    for _ in range(rate - sent[0]):
        next(side)
    done.clear()

    cp_d.wait()

    start(early_copies(1))
    rest_side = list(side)

    def placed(r, words):
        idx = jnp.zeros((CAP, 128), I32)
        for c, m in enumerate(lanes(r)):
            idx = jnp.where(m, c, idx)
        return [_gather(w, idx) for w in words]

    def late_copies(lo, hi):
        return [out_copy(CAP + q, lo, hi) for q in range(CAP)]

    def words_of(n):
        return [new_v[n].bitcast(I32)[i:i + 8, :] for i in range(0, new_v[n].shape[0] // 2, 8)]

    tokens = []
    for n, (lo, hi) in enumerate(ROW_CHUNKS):
        a = [act[:, i:i + 128] for i in range(0, FF, 128)]
        for i, token in enumerate(rest_side):
            at = 8 + i * SPAN // len(rest_side) - n * len(a)
            if 0 <= at < len(a):
                a[at] = tie(a[at], token)
        if n == 1:
            start(early_copies(2))
        if n >= 2:
            cut = CUT * 128 // (hi - lo)
            a[cut] = tie(a[cut], tokens[n - 2])
        a = jnp.concatenate(a, axis=1)
        y = _rbf(jax.lax.dot_general(a.astype(BF16), wd_v[lo:hi, :], NT_DIMS,
                                     preferred_element_type=F32))
        new = h_sel[:, lo:hi] + _rbf(x_sel[:, lo:hi] + _rbf(y * gate))
        new_v[n][...] = jnp.concatenate(
            [new.T, jnp.zeros((hi - lo, 128 - CAP), F32)], axis=1).astype(BF16)
        rows = range(lo // 2, hi // 2, 8)
        words = words_of(n)
        both = list(zip(rows, placed(0, words), placed(1, words)))
        for c in range(CAP):
            for i, v0, v1 in both:
                pltpu.store(out_w.at[tile[c], pl.ds(i, 8), :],
                            jnp.where(rnd[c] == 0, v0, v1), mask=lane8 == col[c])
        for cp in late_copies(lo, hi):
            cp.start()
        out_w[tile[0], D // 2:, :] = lane8
        tokens.append(pltpu.bitcast(out_w[tile[0] | zero, D // 2:, :], F32))
    pltpu.make_async_copy(out_v.at[:, 0:D], out_v.at[:, 0:D], sem_o).wait()

    @pl.when(rounds > 2)
    def _():
        def fix(r, carry):
            rows = range(0, D // 2, 8)
            vals = placed(r, sum(map(words_of, range(len(new_v))), []))
            for c, m in enumerate(lanes(r)):
                for i, v in zip(rows, vals):
                    pltpu.store(out_w.at[tile[c], pl.ds(i, 8), :], v, mask=m)
            return carry

        jax.lax.fori_loop(2, rounds, fix, 0)
        for cp in late_copies(0, D):
            cp.start()
        for cp in late_copies(0, D):
            cp.wait()


@jax.jit
def pallas_sequential_preLN__ssm_conv_s4__moe_arch_mod__prompt_kernel(
    A_u: jax.Array,
    A_A_re: jax.Array,
    A_A_im: jax.Array,
    A_B_re: jax.Array,
    A_B_im: jax.Array,
    A_C_re: jax.Array,
    A_C_im: jax.Array,
    A_log_dt: jax.Array,
    A_Dskip: jax.Array,
    B_x: jax.Array,
    B_w_r: jax.Array,
    B_w_gate: jax.Array,
    B_w_up: jax.Array,
    B_w_down: jax.Array,
):
    del B_x
    hbm = pl.BlockSpec(memory_space=pl.ANY)
    out = pl.pallas_call(
        _kernel,
        out_shape=jax.ShapeDtypeStruct((D, L), BF16),
        in_specs=[hbm] * 13,
        out_specs=hbm,
        scratch_shapes=[
            pltpu.VMEM((NT, D + 16, 128), BF16),
            *[pltpu.VMEM((FF // 128, D + 16, 128), BF16)] * 2,
            pltpu.VMEM((D, FF), BF16),
            pltpu.VMEM((6, D, N), BF16),
            *[pltpu.VMEM((D,), BF16)] * 3,
            *[pltpu.VMEM((2, 16, 144, 128), BF16)] * 2,
            pltpu.VMEM((16, 2, 72, 128), I32),
            pltpu.VMEM((2, D, 128), F32),
            pltpu.VMEM((16, D), BF16),
            pltpu.VMEM((D // MB, 16, 128), BF16),
            pltpu.VMEM((2, 256, 128), F32),
            pltpu.VMEM((len(INDEX), 8, 128), I32),
            pltpu.VMEM((4, 3, 32, 16, 128), BF16),
            pltpu.VMEM((NT, D + 16, 128), BF16),
            pltpu.VMEM((NT, 2, 8, 128), F32),
            *[pltpu.VMEM((NT, 8, 128), F32)] * 2,
            pltpu.VMEM((NT, D + 16, 128), BF16),
            *[pltpu.VMEM((4, 4, 10, 8, 128), F32)] * 2,
            *[pltpu.VMEM((4, 4, 2, 112, 128), BF16)] * 2,
            *[pltpu.VMEM((4, 4, 2, 144, 128), BF16)] * 2,
            *[pltpu.VMEM((4, 8, 128), I32)] * 2,
            *[pltpu.VMEM((16, MB + 16, 128), BF16)] * 2,
            *[pltpu.VMEM((16, MB // 2 + 8, 128), I32)] * 2,
            *[pltpu.VMEM((4, 4, 2, MB + 8, 128), F32)] * 2,
            *[pltpu.VMEM((4, 4, 2, MB + 8, 128), F32)] * 2,
            *[pltpu.VMEM((16, MB // 2 + 8, 128), I32)] * 4,
            pltpu.SemaphoreType.DMA((15,)),
            pltpu.SemaphoreType.DMA((NT,)),
            pltpu.SemaphoreType.DMA((3,)),
            pltpu.SemaphoreType.DMA,
            *[pltpu.VMEM((4, 4, 2, MB + 8, 128), F32)] * 2,
            *[pltpu.VMEM((8, 8, 128), F32)] * 4,
            *[pltpu.VMEM((hi - lo, 128), BF16) for lo, hi in ROW_CHUNKS],
        ],
        compiler_params=pltpu.CompilerParams(vmem_limit_bytes=100 * 1024 * 1024,
                                             disable_bounds_checks=True,
                                             disable_semaphore_checks=True),
    )(A_u.reshape(L, D).T, A_A_re, A_A_im, A_B_re, A_B_im, A_C_re, A_C_im,
      A_log_dt, A_Dskip, B_w_r, B_w_gate, B_w_up, B_w_down.T)
    return out.T.reshape(1, L, D)
```

```python
import functools

import numpy as np
import jax
import jax.numpy as jnp
import jax.experimental.pallas as pl
import jax.experimental.pallas.tpu as pltpu

F32 = jnp.float32
BF16 = jnp.bfloat16
I32 = jnp.int32

L = 2048
D = 576
N = 128
FF = 4608
CAP = 8
NT = L // 128
EPS = 1e-5
MB = 64
PLANS = dict(
    s=(2, ""),
    st=(2, ""),
    n=(4, ""),
    stk=(2, "0:t:-1:4 1:t:-1:3 0:t:-1:4 0:t:-1:7 0:t:-1:15 1:t:-1:10 1:t:6:16 1:t:11:21 0:k "
            "0:k 1:k 0:s:-1:20 0:s:11:23 0:k:-1:23 1:k 1:s:20:-1 1:s 1:k "),
    stkFnf=(4, "1:t:-1:1 0:s:-1:9 0:s:-1:34 1:s:-1:35 1:s:-1:54 2:s:-1:69 3:s:-1:90 0:f "
               "0:n:1:19 0:F 0:t:4:25 0:t:0:19 0:k 0:t:12:43 0:k 0:k:-1:38 0:F 0:f 1:f "
               "1:t:29:44 1:F 1:n:33:47 1:t:35:58 1:k 1:k 1:t:42:57 1:k:-1:61 0:t:44:56 "
               "3:t:47:61 1:F 1:f 2:f 2:n:57:76 2:F 2:t:61:83 2:t:53:76 2:k 2:k 2:s:73:91 "
               "2:k:-1:92 2:t:70:98 2:F 2:f 3:f 3:t:85:100 3:F 3:n:89:104 3:t:91:-1 3:k "
               "3:s:95:111 3:k 3:t:98:110 3:k 2:t:100:110 3:F 3:f "),
    stkFnfm=(4, "0:m:-1:6 0:m:-1:5 0:t:-1:7 0:t:-1:14 0:t:-1:12 0:f 0:m:3:13 0:m:-1:18 "
                "0:m:3:18 0:f 0:m:6:20 0:k 0:t:8:25 0:n:9:27 0:m:13:33 0:m:13:25 1:m:12:34 0:k "
                "0:s:16:33 0:k:-1:35 0:s:19:33 1:m:18:33 0:F 1:t:20:35 0:F 1:t:27:42 1:t:24:40 "
                "1:f 1:f 1:m:32:42 1:m:31:46 1:m:31:46 1:m:34:48 1:k 1:t:37:50 1:n:37:55 "
                "2:m:39:62 1:k 1:s:44:61 1:m:43:61 1:m:41:53 1:k:-1:63 1:s:47:63 2:m:43:61 1:F "
                "2:t:48:63 1:F 2:t:55:70 2:t:50:68 2:f 2:f 2:m:60:70 2:m:60:78 2:m:59:71 "
                "2:m:62:76 2:k 2:t:66:78 2:n:65:85 2:k 2:s:72:89 2:m:71:89 2:m:69:81 2:k:-1:94 "
                "2:s:75:89 3:m:70:90 3:m:74:89 2:F 3:t:76:91 2:F 3:t:83:98 3:t:78:96 3:f 3:f "
                "3:m:88:98 3:m:87:102 3:m:87:102 3:m:90:104 3:k 3:t:93:108 3:n:94:110 3:k "
                "3:s:100:-1 3:m:99:-1 3:m:94:106 3:k 3:F 3:s:105:-1 3:F "),
    stkFnfmi=(4, "0:t:-1:2 0:n:-1:8 0:t:-1:3 0:m:-1:6 0:m:-1:7 0:m:-1:19 0:s:-1:40 1:s:-1:76 "
                 "2:s:-1:112 3:s 0:k 0:m:0:16 0:s:4:33 0:f 0:k 0:m:13:23 0:k:-1:33 0:m:14:25 "
                 "0:t:14:35 0:f 0:t:18:33 0:F 1:t:23:40 1:t:23:38 0:F 1:n:27:47 1:m:27:40 0:i "
                 "1:m:29:47 0:i 0:m:32:40 0:m:31:44 1:m:34:54 1:k 1:m:36:54 1:s:40:71 1:f 1:k "
                 "1:m:49:61 1:m:51:63 1:k:-1:71 1:f 1:t:55:79 1:t:51:68 1:F 2:t:59:74 "
                 "2:t:58:75 1:F 2:m:63:78 2:m:63:79 1:i 2:n:65:80 1:i 1:m:68:76 1:m:67:78 2:k "
                 "2:m:72:91 2:m:71:87 2:s:76:105 2:f 2:k 2:m:83:95 2:k:-1:108 2:m:86:97 "
                 "2:t:86:108 2:f 2:t:90:105 2:F 3:t:94:112 3:t:95:110 2:F 3:m:99:115 2:i "
                 "3:n:102:119 3:m:101:119 2:i 2:m:104:112 2:m:103:116 3:k 3:m:108:126 "
                 "3:m:111:126 3:s:112:143 3:f 3:k 3:m:121:133 3:k:-1:142 3:m:123:135 3:f "
                 "3:t:127:-1 3:t:123:140 3:F 3:F 3:i 3:m:139:-1 3:i 3:m:140:-1 "),
    stkFnfmia=(4, "0:t:-1:6 0:t:-1:3 0:n:-1:10 0:m:-1:6 0:m:-1:5 0:m:-1:19 0:s:-1:43 1:s:-1:80 "
                  "2:s:-1:117 3:s 0:a 0:f 0:m:1:20 0:k 0:s:5:40 0:k 0:m:14:26 0:m:-1:26 "
                  "0:k:-1:38 0:t:16:30 0:f 0:t:18:32 0:F 0:F 1:t:25:43 1:t:23:42 1:n:28:47 "
                  "1:m:25:43 1:m:27:43 0:i 0:m:32:40 0:i 0:m:34:42 1:a 1:f 1:m:38:56 1:m:36:57 "
                  "1:k 1:s:42:77 1:k 1:m:52:63 1:m:53:67 1:k:-1:75 1:t:53:67 1:f 1:t:55:69 1:F "
                  "1:F 2:t:64:80 2:t:57:76 2:n:65:84 2:m:62:80 2:m:61:80 1:i 1:m:69:77 1:i "
                  "1:m:71:81 2:m:73:93 2:a 2:f 2:m:75:94 2:k 2:s:79:114 2:k 2:m:89:100 "
                  "2:m:87:103 2:k:-1:112 2:t:90:104 2:f 2:t:92:106 2:F 2:F 3:t:99:117 "
                  "3:t:97:116 3:m:99:117 3:m:101:117 2:i 2:m:106:114 3:n:103:121 2:i "
                  "2:m:108:116 3:a 3:f 3:m:113:131 3:m:114:131 3:k 3:s:116:-1 3:k 3:m:126:137 "
                  "3:m:124:140 3:k:-1:145 3:t:127:141 3:f 3:t:129:-1 3:F 3:F 3:i 3:m:143:-1 "
                  "3:i 3:m:145:-1 "),
    tkFnfmia=(4, "1:m:-1:5 1:m:-1:3 0:n:-1:12 0:t:-1:3 0:t:-1:14 0:t:-1:21 0:t:-1:28 1:t:-1:40 "
                 "1:t:-1:51 1:t:-1:58 1:t:-1:65 2:t:-1:77 2:t:-1:88 0:F 0:m:2:14 0:m:-1:15 0:a "
                 "0:F 0:m:7:20 0:k 0:m:9:27 0:m:13:23 0:k 0:m:15:25 0:m:18:31 0:m:20:32 "
                 "0:k:-1:45 0:i 0:i 0:f 0:f 1:n:36:50 1:F 1:a 1:F 1:m:42:56 1:m:34:56 1:k "
                 "1:m:47:64 1:k 1:m:53:68 1:k:-1:75 1:i 1:i 3:m:63:79 3:m:61:77 1:f 1:m:68:76 "
                 "1:f 1:m:73:81 2:n:70:86 2:F 2:m:75:87 2:m:73:95 2:a 2:F 2:m:79:92 2:t:81:95 "
                 "2:t:-1:101 2:k 2:m:83:101 2:m:87:97 2:k 2:m:89:101 2:k:-1:119 2:i 2:m:95:105 "
                 "2:m:87:103 2:i 3:t:99:111 2:f 3:t:106:122 3:t:-1:129 2:f 3:n:110:124 3:F 3:a "
                 "3:F 3:m:116:129 3:m:111:134 3:k 3:m:121:141 3:m:124:141 3:t:125:139 3:k 3:k "
                 "3:i 3:i 3:f 3:m:142:-1 3:f 3:m:145:-1 "),
    kFnfmia=(4, "1:m:-1:5 1:m:-1:3 0:n:-1:12 0:F 0:m:2:14 0:m:-1:15 0:a 0:F 0:m:7:21 0:k "
                "0:m:9:27 0:m:13:23 0:k 0:m:15:25 0:m:18:31 0:m:20:32 0:k:-1:45 0:i 0:i 0:f "
                "0:f 1:n:36:50 1:F 1:a 1:F 1:m:42:57 1:m:34:56 1:k 1:m:47:64 1:k 1:m:53:66 "
                "1:k:-1:75 1:i 1:i 3:m:63:79 3:m:61:77 1:f 1:m:68:76 1:f 1:m:73:81 2:n:70:86 "
                "2:F 2:m:76:88 2:m:73:89 2:a 2:F 2:m:79:93 2:k 2:m:83:101 2:m:87:97 2:k "
                "2:m:89:101 2:k:-1:119 2:i 2:m:95:105 2:m:90:106 2:i 2:f 2:f 3:n:110:124 3:F "
                "3:a 3:F 3:m:116:130 3:m:111:134 3:k 3:m:121:141 3:m:124:141 3:k 3:k 3:i 3:i "
                "3:f 3:m:142:-1 3:f 3:m:145:-1 "),
    Ffmia=(4, "1:m:-1:9 0:m:-1:5 0:m:-1:10 0:m:-1:12 0:a 0:F 1:m:4:15 0:i 0:m:6:18 0:i "
              "0:m:9:22 0:F 1:m:16:31 0:f 0:m:20:33 0:f 0:m:22:33 1:a 1:m:25:43 1:F 0:m:29:41 "
              "1:i 1:i 1:m:37:50 1:F 1:m:40:54 1:f 1:m:42:57 1:m:45:56 3:m:45:59 2:m:42:58 1:f "
              "2:a 2:F 2:m:53:63 2:m:49:65 3:m:54:68 2:i 2:m:56:67 2:i 2:m:59:75 2:F 3:m:66:83 "
              "2:f 2:m:70:83 2:f 2:m:72:84 3:a 3:m:75:93 3:F 2:m:79:95 3:i 3:i 3:m:85:-1 3:F "
              "3:m:90:-1 3:f 3:m:92:-1 3:m:95:-1 3:f "),
    mia=(4, "1:m:-1:3 0:m:-1:8 0:m:-1:6 0:m:-1:7 0:m:-1:8 0:i 1:m:0:13 0:m:2:10 0:a 0:i "
            "1:m:5:16 2:m:8:25 1:i 1:m:9:22 0:m:10:23 0:m:8:20 1:m:8:20 3:m:11:25 1:a "
            "2:m:13:27 1:i 1:m:14:22 1:m:17:25 0:m:14:22 1:m:17:25 2:m:14:28 2:m:13:27 2:i "
            "3:m:18:32 2:m:20:32 2:a 2:i 3:m:23:-1 3:m:25:-1 3:m:25:-1 3:i 2:m:28:-1 2:m:27:-1 "
            "3:a 3:i 3:m:32:-1 3:m:35:-1 2:m:33:-1 3:m:35:-1 "),
    iaz=(4, "0:i 0:i 1:i 1:i 0:z 2:i 2:i 1:z 3:i 3:i 2:z 0:a 1:a 2:a 3:a 3:z"),
)
ROW_CHUNKS = ((0, 128), (128, 256), (256, 384), (384, 512), (512, D))
MID, SPAN, EARLY, LAG, CUT, END = 480, 30, 8, 16, 12, 76
NT_DIMS = (((1,), (1,)), ((), ()))


def _round_res(step):
    return [int(np.round(r / step)) * step for r in range(16)]


RES1, RES2, RES3 = _round_res(2), _round_res(4), _round_res(8)


def _ds(start, size):
    return pl.ds(start if isinstance(start, int) else pl.multiple_of(start, size), size)


def _iota(shape, dim):
    return jax.lax.broadcasted_iota(I32, shape, dim)


def _rbf(x):
    return x.astype(BF16).astype(F32)


def _cmul(a, b):
    return (a[0] * b[0] - a[1] * b[1], a[0] * b[1] + a[1] * b[0])


def _csq(a):
    t = a[0] * a[1]
    return ((a[0] + a[1]) * (a[0] - a[1]), t + t)


def _cadd(a, b):
    return (a[0] + b[0], a[1] + b[1])


def _csub(a, b):
    return (a[0] - b[0], a[1] - b[1])


def _bfly4(a0, a1, a2, a3, inverse=False):
    s02, d02 = _cadd(a0, a2), _csub(a0, a2)
    s13, d13 = _cadd(a1, a3), _csub(a1, a3)
    p = (d02[0] - d13[1], d02[1] + d13[0])
    m = (d02[0] + d13[1], d02[1] - d13[0])
    if inverse:
        p, m = m, p
    return _cadd(s02, s13), p, _csub(s02, s13), m


def _prod_mod_1(a, b):
    fa, fb = _bfly4(*a), _bfly4(*b)
    return _bfly4(*[_cmul(x, y) for x, y in zip(fa, fb)], inverse=True)


def _prod2(a0, a1, b0, b1, sgn):
    p00, p11 = _cmul(a0, b0), _cmul(a1, b1)
    c1 = _cadd(_cmul(a0, b1), _cmul(a1, b0))
    if sgn > 0:
        return (p00[0] - p11[1], p00[1] + p11[0]), c1
    return (p00[0] + p11[1], p00[1] - p11[0]), c1


def _prod_mod_m1(a, b):
    def split(x):
        p = [(x[k][0] - x[k + 2][1], x[k][1] + x[k + 2][0]) for k in range(2)]
        m = [(x[k][0] + x[k + 2][1], x[k][1] - x[k + 2][0]) for k in range(2)]
        return p, m
    ap, am = split(a)
    bp, bm = split(b)
    cp = _prod2(*ap, *bp, 1)
    cm = _prod2(*am, *bm, -1)
    lo = [_cadd(cp[k], cm[k]) for k in range(2)]
    hi = [(cp[k][1] - cm[k][1], cm[k][0] - cp[k][0]) for k in range(2)]
    return lo + hi


def _prod_mod_i(a, b, sgn):
    sm = [x[0] + x[1] for x in b]
    df = [x[1] - x[0] for x in b]
    asum = [x[0] + x[1] for x in a]
    out = []
    for k in range(4):
        acc = [None, None, None]
        for j in range(4):
            m = (k - j) % 4
            if j <= k:
                t = ((b[m][0], 1), (df[m], 1), (sm[m], 1))
            elif sgn > 0:
                t = ((b[m][1], -1), (sm[m], 1), (df[m], -1))
            else:
                t = ((b[m][1], 1), (sm[m], -1), (df[m], 1))
            for q, (v, (w, s)) in enumerate(zip((asum[j], a[j][0], a[j][1]), t)):
                p = v * w
                if acc[q] is None:
                    acc[q] = p
                else:
                    acc[q] = acc[q] + p if s > 0 else acc[q] - p
        out.append((acc[0] - acc[2], acc[0] + acc[1]))
    return out


def _barrel(v, sch):
    for bit in range(4):
        m = sch.mask("bit%d" % bit)
        v = [jnp.where(m, v[(i + (1 << bit)) % 16], v[i]) for i in range(16)]
    return [v[-s % 16] for s in range(16)]


def _to_residues(tiles, sch):
    return _barrel([t if j == 0 else pltpu.roll(t, j, 1) for j, t in enumerate(tiles)], sch)


def _to_time(res, sch):
    return [t if j == 0 else pltpu.roll(t, 128 - j, 1)
            for j, t in enumerate(_barrel(res, sch))]


def _gather(x, idx, axis=1):
    return jnp.take_along_axis(x, idx, axis=axis, mode="promise_in_bounds")


def _transpose_dft(wt_ref, wu_ref, residues):
    for s in residues:
        for p in range(2):
            wt_ref[4 * (s % 4) + (0, 2, 1, 3)[s // 4], p, 0:64] = pltpu.bitcast(
                _mxu(wu_ref.bitcast(I32)[p, 4 * (s % 4) + s // 4, 0:64]).T, I32)


def _init_dft(wu_ref, wk_ref, tmp_ref, halfway):
    sub, k4 = _iota((8, 128), 0), 4 * _iota((8, 128), 1) + 1

    def cis(t):
        ph = ((k4 * t) & (4 * L - 1)).astype(F32) * (2 * np.pi / (4 * L))
        return jnp.cos(ph), jnp.sin(ph)

    w1, w16 = cis(1), cis(16)
    w32 = _csq(w16)
    fk = [cis(16 * (32 * (sub & 3) + (sub >> 2)))]
    fu = [cis(128 * sub), cis(128 * (sub + 8))]
    for v in range(1, 16):
        fk.append(_cmul(fk[-1], w32))
        if v >= 2:
            fu.append(_cmul(fu[-2], w16))
    for p in range(2):
        for v in range(32):
            tmp_ref[p, 8 * v:8 * v + 8, :] = fu[v % 16][p]
    tw = None
    for s in range(16):
        for v in range(0, 16, 2):
            rows = [slice(128 - s + 8 * i, 136 - s + 8 * i) for i in (v, v + 1)]
            for ref, f in ((wk_ref, fk[v:v + 2]),
                           (wu_ref, [(tmp_ref[0, r, :], tmp_ref[1, r, :]) for r in rows])):
                if s:
                    f = [_cmul(x, tw) for x in f]
                for p in range(2):
                    ref[p, 4 * (s % 4) + s // 4, 8 * v:8 * v + 16, :] = jnp.concatenate(
                        [f[0][p], f[1][p]], axis=0).astype(BF16)
        tw = _cmul(tw, w1) if s else w1
        if s == 7:
            halfway()


def _pack(ref, n, a, b):
    ref[n] = jnp.concatenate([a, b], axis=0).astype(BF16)
    return ref.bitcast(I32)[n]


def _split(w):
    return [pltpu.bitcast(w << 16, F32), pltpu.bitcast(w & -65536, F32)]


FINE = (0, 1, 2, 3, 4, 5, 6, 7, 512, 516, 1024, 1536)


def _k_seeds(z, c, sch):
    pw = {1: z}
    for e in range(1, 10):
        pw[1 << e] = _csq(pw[1 << (e - 1)])
    c8, z16 = _cmul(c, pw[8]), (pw[16][0], 0.0 - pw[16][1])
    pair = lambda a, b: tuple(jnp.where(sch.mask("odd"), q, p) for p, q in zip(a, b))
    seeds = []
    for g in range(2):
        twice = lambda v: tuple(_gather(x, sch.idx("dup%d" % g), 0) for x in v)
        seeds.append([twice(z), twice(pw[32]), twice(pw[512]),
                      pair(twice(c), twice(c8)), pair((1.0, 0.0), twice(z16))])
    return seeds


def _mxu(words):
    return pltpu.bitcast(words, BF16)


def _store_table(ref, tab):
    for i in range(0, len(tab), 2):
        for p in range(2):
            ref[p, 8 * i:8 * i + 16, :] = jnp.concatenate(
                [tab[i][p], tab[i + 1][p]], axis=0).astype(BF16)


def _k_residues(groups, k_last, dskip, tmp_ref, sch):
    idx, nxt = sch.idx("src"), sch.idx("nxt")
    low = lambda x, y: (x & 65535) | (y << 16)
    high = lambda x, y: jax.lax.shift_right_logical(x, 16) | (y & -65536)
    kv, up = {}, {}
    for i, k in enumerate(FINE):
        v = [g[8 * i:8 * i + 8] for g in groups]
        if k == 0:
            v = [x + jnp.where(sch.mask("diag"),
                               _gather(dskip[n // 2], sch.idx("dup%d" % (n % 2)), 0), 0.0)
                 for n, x in enumerate(v)]
        p = [_pack(tmp_ref, 2 * i + h, v[2 * h], v[2 * h + 1]) for h in range(2)]
        both = [_gather(x, idx) for x in p]
        kv[k], kv[k + 8] = low(*both), high(*both)
        if k % 512 == 0:
            up[k] = low(*[_gather(x, nxt) for x in p])
    k_last = _gather(k_last, sch.idx("rows"), 0)
    q0, q1, q2, up0, up01, up2, up3, fine = map(sch.mask, INDEX[-8:])
    s3 = {r: jnp.where(q2, kv[1024 + r], kv[1536 + r]) for r in (0, 8)}
    v0 = jnp.where(q0, kv[0], jnp.where(q1, kv[512], s3[0]))
    v16 = jnp.where(up01, jnp.where(up0, up[0], up[512]),
                    jnp.where(up2, up[1024], jnp.where(up3, up[1536], k_last)))
    s3[16] = v16
    s23, s123, out = {}, {}, [v0]
    for r in range(1, 16):
        k23 = (RES2[r], RES3[r])
        if k23 not in s23:
            s23[k23] = v16 if k23 == (16, 16) else jnp.where(q1, kv[512 + k23[0]], s3[k23[1]])
        k123 = (RES1[r],) + k23
        if k123 not in s123:
            s123[k123] = v16 if k123[0] == 16 else jnp.where(q0, kv[k123[0]], s23[k23])
        if RES1[r] == r:
            out.append(s123[k123])
        else:
            out.append(jnp.where(fine, kv[r], s123[k123]))
    return out


def _ln_scalars(s1, s2):
    mean = s1 * (1.0 / D)
    var = jnp.maximum(s2 * (1.0 / D) - mean * mean, 0.0)
    eps = float(np.asarray(EPS, dtype=BF16))
    sd = _rbf(jnp.sqrt(_rbf(_rbf(var) + eps)))
    return _rbf(mean), sd


def _top8(x):
    def swap(v, pairs):
        for i, j in pairs:
            v[i], v[j] = jnp.maximum(v[i], v[j]), jnp.minimum(v[i], v[j])
        return v

    def merge(a, b):
        v = [jnp.maximum(a[i], b[7 - i]) for i in range(8)]
        return swap(v, [(i, i + d) for d in (4, 2, 1) for i in range(8) if not i & d])

    sort8 = ((0, 2), (1, 3), (4, 6), (5, 7), (0, 4), (1, 5), (2, 6), (3, 7), (0, 1), (2, 3),
             (4, 5), (6, 7), (2, 4), (3, 5), (1, 4), (3, 6), (1, 2), (3, 4), (5, 6))
    v = merge(*[swap(x[i:i + 8], sort8) for i in (0, 8)])
    for d in (4, 2, 1):
        v = merge(v, [pltpu.roll(t, d, 0) for t in v])
    return v


def _init_columns(col_ref, wx_ref, wy_ref, ldt_ref, dsk_ref, wr_ref):
    row, lane = _iota((128, 128), 0), _iota((128, 128), 1)
    split = (row & ~15) + 2 * (row & 7) + ((row >> 3) & 1)
    ldt, dsk, wr = (ref[...].astype(F32).reshape(1, D) for ref in (ldt_ref, dsk_ref, wr_ref))
    for n, vec in enumerate((jnp.exp(ldt), dsk * (1.0 / L))):
        for lo in range(0, D, 128):
            i = min(lo, D - 128)
            diag = jnp.where(split == lane, vec[:, i:i + 128], 0.0)[lo - i:].astype(BF16)
            col_ref[n, lo:i + 128, :] = jnp.dot(diag, jnp.ones((128, 128), BF16),
                                                preferred_element_type=F32)
    sub = _iota((16, D), 0)
    ones_w = jnp.where(sub == 0, 1.0, jnp.where(sub == 1, wr, 0.0))
    wx_ref[...] = ones_w.astype(BF16)
    for lo in range(0, D, MB):
        wy_ref[lo // MB, :, 0:MB] = ones_w[:, lo:lo + MB].astype(BF16)
        wy_ref[lo // MB, :, MB:] = jnp.zeros((16, 128 - MB), BF16)


INDEX = ("true", "bit0", "bit1", "bit2", "bit3", "odd", "dup0", "dup1", "rows", "src", "nxt",
         "diag", "q0", "q1", "q2", "up0", "up01", "up2", "up3", "fine")


def _init_index(idx_ref):
    sub, lane = _iota((8, 128), 0), _iota((8, 128), 1)
    src = lambda b: 8 * ((b >> 1) & 15) + 2 * (sub & 3) + (b & 1)
    is_ = lambda m: jnp.where(m, 1, 0)
    q = lane & 3
    q16 = q + is_(lane >= 124)
    tiles = dict(true=sub + 1, odd=sub & 1, dup0=sub >> 1, dup1=4 + (sub >> 1),
                 rows=2 * (sub & 3) + (sub >> 2), src=src(lane >> 2), nxt=src((lane >> 2) + 1),
                 diag=is_((lane == sub) & ((sub & 1) == 0)), up01=is_(q16 < 2),
                 fine=is_((q == 0) & (lane < 64)),
                 **{"bit%d" % n: (lane >> n) & 1 for n in range(4)},
                 **{"q%d" % n: is_(q == n) for n in range(3)},
                 **{"up%d" % n: is_(q16 == n) for n in (0, 2, 3)})
    for n, name in enumerate(INDEX):
        idx_ref[n] = tiles[name]


class _Schedule:
    def __init__(self, zero, idx_ref):
        self.zero = zero
        self.idx = lambda name: idx_ref[INDEX.index(name) + zero]
        self.mask = lambda name: self.idx(name) != 0
        self.true = self.mask("true")
        self.done, self.pending, self.wait = [], {}, -1

    def tie(self, x, token):
        return jnp.where(self.true, x, token if token.dtype == x.dtype
                         else pltpu.bitcast(token, x.dtype))

    def start(self, x):
        return self.tie(x, self.done[self.wait]) if 0 <= self.wait < len(self.done) else x

    def lhs(self, words, first):
        tiles = [words[i:i + 8] for i in range(0, words.shape[0], 8)]
        for i in range(len(tiles) if first else 0):
            for token in self.pending.pop(len(self.done) + i, ()):
                tiles[i] = self.tie(tiles[i], token)
        return _mxu(jnp.concatenate(tiles, axis=0))

    def results(self, v):
        self.done += [v[i + 8:i + 16] for i in range(0, v.shape[0], 16)]

    def run(self, stage, wait, before):
        self.wait = wait
        self.pending.setdefault(before, []).extend(next(stage))


def _kernel(x_hbm, are_hbm, aim_hbm, bre_hbm, bim_hbm, cre_hbm, cim_hbm,
            ldt_hbm, dsk_hbm, wr_hbm, wg_hbm, wu_hbm, wd_hbm, out_hbm,
            x_v, wg_v, wu_v, wd_v, par_v, ldt_v, dsk_v, wr_v, w_v, wk_v, wt_v, col_v, wx_v, wy_v,
            tmp_v, idx_v, pk_v, h_v, st_v, acc_v, sq_v, out_v, sd0, sd1, ta0, ta1, tb0, tb1,
            kl0, kl1,
            u0, u1, k0, k1, a0_v, a1_v, c0, c1, r0, r1, r2, r3,
            sem_p, sem_x, sem_w, sem_o, f0_v, f1_v, *rest):
    half_v, new_v = rest[:4], rest[4:]
    cp_vec = [pltpu.make_async_copy(s, d, sem_p.at[n]) for n, (s, d) in enumerate(
        ((ldt_hbm, ldt_v), (dsk_hbm, dsk_v), (wr_hbm, wr_v)))]
    cp_par = [[pltpu.make_async_copy(s.at[lo:hi], par_v.at[n, lo:hi], sem_p.at[3 + 6 * m + n])
               for n, s in enumerate((are_hbm, aim_hbm, bre_hbm, bim_hbm, cre_hbm, cim_hbm))]
              for m, (lo, hi) in enumerate(((0, 4 * MB), (4 * MB, D)))]
    cp_x = [pltpu.make_async_copy(x_hbm.at[:, 128 * j:128 * j + 128], x_v.at[j, 0:D],
                                  sem_x.at[j])
            for j in range(NT)]
    cp_d = pltpu.make_async_copy(wd_hbm, wd_v, sem_w.at[2])

    def cp_w(i):
        return [pltpu.make_async_copy(s.at[:, _ds(128 * i, 128)], d.at[i, 0:D], sem_w.at[n])
                for n, (s, d) in enumerate(((wg_hbm, wg_v), (wu_hbm, wu_v)))]

    for cp in cp_vec + cp_par[0]:
        cp.start()
    for cp in cp_x[:NT // 2]:
        cp.start(priority=1)

    def columns():
        for cp in cp_vec:
            cp.wait()
        for cp in cp_x[NT // 2:]:
            cp.start(priority=1)
        _transpose_dft(wt_v, w_v, range(4))
        _init_columns(col_v, wx_v, wy_v, ldt_v, dsk_v, wr_v)

    _init_dft(w_v, wk_v, tmp_v, columns)
    for cp in cp_par[0]:
        cp.wait()

    sd, ta, tb, kl = (sd0, sd1), (ta0, ta1), (tb0, tb1), (kl0, kl1)
    uk, ab, cc, xr = ((u0, u1), (k0, k1)), ((a0_v, a1_v), (f0_v, f1_v)), (c0, c1), (r0, r1, r2, r3)
    ww, wt_w = (w_v.bitcast(I32), wk_v.bitcast(I32)), wt_v

    def seed_stage(b, r, sch):
        rows = _ds(b * MB // 2 + 8 * r, 8)
        par = [_split(par_v.bitcast(I32)[n, rows, :]) for n in range(6)]
        for h in range(2):
            a_re, a_im, b_re, b_im, c_re, c_im = [v[h] for v in par]
            dt = sch.start(col_v[0, _ds(b * MB + 16 * r + 8 * h, 8), :])
            mag, ang = jnp.exp(dt * a_re), dt * a_im
            sc = dt * (1.0 / L)
            seeds = _k_seeds((mag * jnp.cos(ang), mag * jnp.sin(ang)),
                             _cmul((c_re, c_im), (sc * b_re, sc * b_im)), sch)
            for g in range(2):
                for n, v in enumerate(seeds[g]):
                    for p in range(2):
                        sd[b % 2][r, 2 * h + g, 2 * n + p] = v[p]
            yield [sd[b % 2][(r + sch.zero), 2 * h, 0]]

    def table_stage(b, r, sch):
        tail = []
        for g in range(4):
            m1, m32, m512, a0, b0 = [
                (sd[b % 2][r, g, 2 * n], sd[b % 2][r, g, 2 * n + 1]) for n in range(5)]
            m32 = (sch.start(m32[0]), m32[1])
            fa = [a0]
            for _ in range(7):
                fa.append(_cmul(fa[-1], m1))
            for src in (0, 4, 8, 10):
                fa.append(_cmul(fa[src], m512))
            tail.append(fa[11][0] * m512[0] - fa[11][1] * m512[1])
            _store_table(ta[b % 2].at[r, g], fa)
            fb = [b0]
            for _ in range(15):
                p = fb[-1]
                fb.append((p[0] * m32[0] + p[1] * m32[1], p[1] * m32[0] - p[0] * m32[1]))
            _store_table(tb[b % 2].at[r, g], fb)
            yield [ta[b % 2].bitcast(I32)[(r + sch.zero), g, 0, 0:8, :],
                   tb[b % 2].bitcast(I32)[(r + sch.zero), g, 0, 0:8, :]]
        last = [jnp.where(sch.mask("odd"), pltpu.roll(tail[h + 1], 1, 0), tail[h])
                for h in (0, 2)]
        last = [pltpu.bitcast(_rbf(jnp.broadcast_to(jnp.sum(v, axis=1, keepdims=True),
                                                    (8, 128))), I32) for v in last]
        kl[b % 2][r] = jax.lax.shift_right_logical(last[0], 16) | last[1]

    def kernel_stage(b, r, sch):
        ta_w, tb_w = ta[b % 2].bitcast(I32), tb[b % 2].bitcast(I32)
        groups = [None] * 4
        for g0 in (0, 2):
            res = [jax.lax.dot_general(sch.lhs(ta_w[r, g, p, 0:48], g == g0 and p == 0),
                                       _mxu(tb_w[r, g, p, 0:64]), NT_DIMS, preferred_element_type=F32)
                   for g in (g0, g0 + 1) for p in range(2)]
            groups[g0], groups[g0 + 1] = res[0] + res[1], res[2] + res[3]
            sch.results(groups[g0 + 1])
            yield []
        dskip = [col_v[1, _ds(b * MB + 16 * r + 8 * h, 8), :] for h in range(2)]
        dst = _ds(8 * r, 8)
        res = _k_residues(groups, kl[b % 2][r], dskip, pk_v.at[sch.slot, 0], sch)
        for s, t in enumerate(res):
            uk[1][b % 2][4 * (s % 4) + s // 4, dst, :] = t
        yield [uk[1][b % 2][0, _ds(8 * (r + sch.zero), 8), :]]

    def norm_stage(b, r, sch):
        rows, dst = _ds(b * MB // 2 + 8 * r, 8), _ds(8 * r, 8)
        tiles = [x_v.bitcast(I32)[j, rows, :] for j in range(NT)]
        for s, t in enumerate(_to_residues([sch.start(tiles[0])] + tiles[1:], sch)):
            xr[b % 4][4 * (s % 4) + s // 4, dst, :] = t
            xs, m, inv = _mxu(t).astype(F32), st_v[s, 0], st_v[s, 1]
            uk[0][b % 2][4 * (s % 4) + s // 4, _ds(16 * r, 16), :] = jnp.concatenate(
                [(xs[0:8] - m) * inv, (xs[8:16] - m) * inv], axis=0).astype(BF16)
        yield [uk[0][b % 2].bitcast(I32)[0, _ds(8 * (r + sch.zero), 8), :]]

    def forward_stage(w, b, k, sch):
        dst = ab[w][b % len(ab[w])]
        for p in range(2):
            v = [jnp.dot(sch.lhs((uk[w][b % 2] if w else uk[w][b % 2].bitcast(I32))[
                4 * k + n, 0:MB // 2], n == 0),
                         _mxu(ww[w][p ^ (n & 1), 4 * k + n, 0:64]),
                         preferred_element_type=F32) for n in range(4)]
            d02, d13 = v[0] - v[2], v[1] - v[3]
            x1 = d02 - d13 if p == 0 else d02 + d13
            dst[0, k, p, 0:MB] = v[0] + v[2]
            dst[2, k, 1 - p, 0:MB] = v[1] + v[3]
            dst[1, k, p, 0:MB] = x1
            dst[3, k, p, 0:MB] = d02 + d13 if p == 0 else d02 - d13
            sch.results(x1)
            yield []

    def stats(tiles, sch):
        ones_w = wx_v.bitcast(I32)[...]
        for j in tiles:
            acc = None
            for i in range(0, D // 2, 8):
                v = [t * t for t in _split(x_v.bitcast(I32)[j, i:i + 8, :])]
                acc = v if acc is None else [p + q for p, q in zip(acc, v)]
            sums = jnp.dot(_mxu(jnp.concatenate(
                [ones_w[:, :128] if j % 2 == 0 else sch.tie(ones_w[:, :128], prev),
                 ones_w[:, 128:]], axis=1)),
                           _mxu(x_v.bitcast(I32)[j, 0:D // 2]), preferred_element_type=F32)
            s2 = prev = acc[0] + acc[1]
            for d in (4, 2, 1):
                s2 = s2 + pltpu.roll(s2, d, 0)
            mean, sd = _ln_scalars(jnp.broadcast_to(sums[0:1], (8, 128)), s2)
            st_v[j, 0], st_v[j, 1] = mean, 1.0 / sd

    def middle_stage(b, r, sch):
        src = [v[b % len(v)] for v in ab]
        scale = lambda v, f: [(x[0] * f, x[1] * f) for x in v]
        for h in range(2):
            ra = _ds(16 * r + 8 * h, 8)
            ld = lambda q, w, ra=ra: [(src[w][q, k, 0, ra, :], src[w][q, k, 1, ra, :]) for k in range(4)]

            park_v = half_v[2 * (sch.slot % 2) + h]

            def put(q, y):
                x = [park_v[n + sch.zero] for n in range(8)]
                for k in range(4):
                    for p in range(2):
                        cc[b % 2][k, q, p, ra, :] = x[2 * k + p] + y[k][p]
                        cc[b % 2][k, q + 2, p, ra, :] = x[2 * k + p] - y[k][p]

            def park(x):
                for k in range(4):
                    for p in range(2):
                        park_v[2 * k + p] = x[k][p]
                return [park_v[sch.zero]]

            gate = sch.start
            a0, a2, b0, b2 = ld(0, 0), ld(2, 0), ld(0, 1), ld(2, 1)
            a0[0] = (gate(a0[0][0]), a0[0][1])
            e0 = _prod_mod_1(list(map(_cadd, a0, a2)), list(map(_cadd, b0, b2)))
            again = _ds(16 * (r + sch.zero) + 8 * h, 8)
            yield park(e0)
            a0, a2, b0, b2 = (ld(q, w, again) for w in range(2) for q in (0, 2))
            a2[0] = (gate(a2[0][0]), a2[0][1])
            e2 = _prod_mod_m1(list(map(_csub, a0, a2)), scale(map(_csub, b0, b2), 2.0))
            put(0, e2)
            yield [cc[b % 2][0, 0, 0, again, :]]
            four = sch.start(jnp.full((8, 128), 4.0, F32))
            e1 = _prod_mod_i(ld(1, 0), scale(ld(1, 1), four), 1)
            yield park(e1)
            four = sch.start(jnp.full((8, 128), 4.0, F32))
            e3 = _prod_mod_i(ld(3, 0), scale(ld(3, 1), four), -1)
            put(1, e3)
            yield [cc[b % 2][0, 1, 0, again, :]]

    def inverse_stage(b, k, sch):
        src = cc[b % 2]

        def lhs(v, n, first):
            return sch.lhs(jnp.concatenate(
                [_pack(pk_v.at[sch.slot, 2], 4 * n + i // 16, v[i:i + 8], v[i + 8:i + 16])
                 for i in range(0, MB, 16)], axis=0), first)

        for o in range(2):
            p0, p1 = [(src[k, q, 0, 0:MB], src[k, q, 1, 0:MB]) for q in (2 * o, 2 * o + 1)]
            if o == 0:
                e = {0: _cadd(p0, p1), 2: _csub(p0, p1)}
            else:
                e = {1: (p0[0] + p1[1], p0[1] - p1[0]), 3: (p0[0] - p1[1], p0[1] + p1[0])}
            ys = []
            for n in e:
                y = [jnp.dot(lhs(e[n][p], 2 * n + p, n == o and p == 0),
                             _mxu(wt_w[4 * k + (0, 2, 1, 3)[n], p, 0:64]),
                             preferred_element_type=F32)
                     for p in range(2)]
                h = y[0] + y[1] + _mxu(xr[b % 4][4 * k + n, 0:MB // 2]).astype(F32)
                h_v[k + 4 * n, b * MB:b * MB + MB, :] = h.astype(BF16)
                hh = h * h
                sq_v[k + 4 * n] += sum((hh[i:i + 8] for i in range(8, MB, 8)), hh[0:8])
                ys.append(h)
            sch.results(ys[-1])
            yield []

    def sum_stage(b, r, sch):
        for n in range(4):
            s = r + 4 * n if b == nb - 1 else 4 * r + n
            sums = jnp.dot(sch.lhs(wy_v.bitcast(I32)[b], n == 0)[:, :MB],
                           _mxu(h_v.bitcast(I32)[s, b * MB // 2:(b + 1) * MB // 2]),
                           preferred_element_type=F32)
            acc_v[s] += sums[0:8]
        sch.results(sums)
        yield []

    nb = D // MB
    stages = dict(
        s=(seed_stage, 0), t=(table_stage, 1), k=(kernel_stage, 2),
        F=(functools.partial(forward_stage, 1), 3), n=(norm_stage, 2),
        f=(functools.partial(forward_stage, 0), 3), m=(middle_stage, 4),
        i=(inverse_stage, 5), a=(sum_stage, 6))

    def run(step, zero, live=None):
        live = live or {n: (f, step - lag) for n, (f, lag) in stages.items()
                        if 0 <= step - lag < nb and (n, step) != ("n", 2)}
        if step == nb + 4:
            live["z"] = (sum_stage, nb - 1)
        unroll, plan = PLANS["".join(live)]

        def body(it, carry):
            sch = _Schedule(zero >> (step % 32) if unroll == 4 else zero & it, idx_v)
            gens = [{n: f(b, it * unroll + u, sch) for n, (f, b) in live.items()}
                    for u in range(unroll)]
            if step == 3:
                for i in range(9 * unroll):
                    for cp in cp_w(9 * unroll * it + i):
                        cp.start()
            for item in plan.split():
                u, n, *ties = item.split(":")
                if n in live:
                    sch.slot = int(u)
                    sch.run(gens[int(u)][n], *map(int, ties or (-1, -1)))
            for sch.slot, g in enumerate(gens):
                for v in g.values():
                    for _ in v:
                        pass
            return carry + it

        if unroll == 4:
            if step == 101 or step > nb + 3:
                return body(0, 0)
            return jax.lax.fori_loop(zero, 1, lambda _, c: body(0, c), 0)
        return jax.lax.fori_loop(0, 4 // unroll, body, 0)

    _init_index(idx_v)
    acc_v[...] = sq_v[...] = jnp.zeros(acc_v.shape, F32)
    zero = run(0, 0) - 1
    for step in range(1, nb + 5):
        if step == 4:
            for cp in cp_par[1]:
                cp.wait()
        if step == 3:
            for half in range(2):
                tiles = range(NT // 2 * half, NT // 2 * (half + 1))
                for j in tiles:
                    cp_x[j].wait()
                if half:
                    cp_d.start(priority=1)
                else:
                    for cp in cp_par[1]:
                        cp.start()
                _transpose_dft(wt_v, w_v, range(4 + 6 * half, 10 + 6 * half))
                stats(tiles, _Schedule(zero, idx_v))
            for q in range(2):
                for s, v in enumerate(_to_residues([st_v[j, q] for j in range(NT)],
                                                   _Schedule(zero, idx_v))):
                    st_v[s, q] = v
            run(101, zero, dict(n=(norm_stage, 0)))
        run(step, zero)

    sums = [acc_v[s] for s in range(16)]
    m2, sd2 = _ln_scalars(
        jnp.concatenate([v[0:1] for v in sums], axis=0),
        jnp.concatenate([jnp.sum(sq_v[j], axis=0, keepdims=True) for j in range(NT)], axis=0))
    inv2 = 1.0 / sd2
    wsum = jnp.sum(wr_v[...].astype(F32).reshape(1, D), axis=1, keepdims=True)
    score = _rbf((jnp.concatenate([v[1:2] for v in sums], axis=0) - m2 * wsum) * inv2 + 0.0)
    sub16 = _iota((16, 128), 0)
    for s in range(16):
        h_v[s, D:, :] = jnp.where(sub16 == 0, m2[s:s + 1], jnp.where(
            sub16 == 1, sd2[s:s + 1], score[s:s + 1])).astype(BF16)
    bits = pltpu.bitcast(score, I32) >> 16
    order = jnp.where(bits < 0, -1 - bits, bits + 32768)
    mu = (_iota((NT, 128), 1) - _iota((NT, 128), 0)) & 127
    pos = 128 * (mu & 15) + 16 * (mu >> 4) + _iota((NT, 128), 0)
    key = pltpu.bitcast((order << 11) + (L - 1 - pos) + (1 << 29), F32)

    h_w, out_w = h_v.bitcast(I32), out_v.bitcast(I32)
    sch, done = _Schedule(zero, idx_v), []
    tie = sch.tie

    def unrouted():
        for q, v in enumerate((1.0 + inv2, m2 * inv2)):
            for j, t in enumerate(_to_time(
                    [jnp.broadcast_to(v[s:s + 1], (8, 128)) for s in range(16)], sch)):
                st_v[j, q] = t
        for i in range(0, D, 16):
            scal = st_v.at[pl.ds(zero * (i + 1), NT)]
            tiles = [h_w[s, i // 2:i // 2 + 8, :] for s in range(16)]
            if len(done) > LAG:
                tiles[0] = tie(tiles[0], done[-LAG])
            for j, v in enumerate(_to_time(tiles, sch)):
                h, mul, sub = _mxu(v).astype(F32), scal[j, 0], scal[j, 1]
                out_v[j, i:i + 16, :] = jnp.concatenate(
                    [h[0:8] * mul - sub, h[8:16] * mul - sub], axis=0).astype(BF16)
                if j % 8 == 7:
                    yield pltpu.bitcast(out_w[j + zero, i // 2:i // 2 + 8, :], F32)

    side = unrouted()

    lane8, sub8 = _iota((CAP, 128), 1), _iota((CAP, 128), 0)
    best = _top8([pltpu.roll(key[i:i + 8], n, 1) if n else key[i:i + 8]
                  for i in (0, 8) for n in range(8)])
    cand = best[0]
    for c in range(1, CAP):
        cand = jnp.where(sub8 == c, best[c], cand)
    best = _top8([pltpu.roll(cand, n, 1) if n else cand for n in range(0, 128, 8)])
    for _ in range(2 * EARLY):
        best[-1] = tie(best[-1], next(side))
    best = [pltpu.bitcast(v, I32)[0, 0] for v in best]
    picks = [L - 1 - (v & (L - 1)) for v in best]

    def schedule(col):
        rnd = [sum([(col[e] == col[c]).astype(I32) for e in range(c)], 0) for c in range(CAP)]
        return (rnd, functools.reduce(jnp.maximum, rnd) + 1,
                lambda n: [lane8 == jnp.where(rnd[c] == n, col[c], -1) for c in range(CAP)])

    _, rounds, lanes = schedule([((t >> 7) + (t & 127)) & 127 for t in picks])

    def out_copy(q, lo, hi):
        j = order[q]
        return pltpu.make_async_copy(
            out_v.at[j, lo:hi], out_hbm.at[lo:hi, _ds(j * 128, 128)], sem_o)

    for n, ref in enumerate((wg_v, wu_v)):
        pltpu.make_async_copy(ref.at[:, 0:D], ref.at[:, 0:D], sem_w.at[n]).wait()

    def gather(n, acc):
        masks = lanes(n)
        tiles = []
        for i in range(0, D // 2 + 8, 8):
            v = jnp.zeros((8, 128), I32)
            for c in range(CAP):
                v = jnp.where(masks[c], h_w[picks[c] & 15, i:i + 8, :], v)
            tiles.append(v)
        lhs = jnp.zeros((CAP, 128), F32)
        for c in range(CAP):
            lhs = jnp.where(masks[c] & (sub8 == c), 1.0, lhs)
        return acc + jax.lax.dot_general(lhs.astype(BF16), _mxu(jnp.concatenate(tiles, axis=0)),
                                         NT_DIMS, preferred_element_type=F32)

    h_sel = jax.lax.fori_loop(0, rounds, gather, jnp.zeros((CAP, D + 16), F32))
    m_sel, sd_sel, score_sel = (h_sel[:, D + q:D + q + 1] for q in range(3))
    h_sel = h_sel[:, :D]
    x_sel = _rbf(_rbf(h_sel - m_sel) / sd_sel)
    gate = _rbf(jax.nn.sigmoid(score_sel))

    tile, col = [t >> 7 for t in picks], [t & 127 for t in picks]
    rnd, rounds, lanes = schedule(col)
    late, again = 0, []
    for j in tile:
        again.append((late >> j) & 1)
        late = late | (1 << j)
    for dup in again[1:]:
        late = late | (late + dup)
    order = []
    for left in (late ^ ((1 << NT) - 1), late):
        for _ in range(CAP):
            order.append((31 - jax.lax.clz(left)) & (NT - 1))
            left = left ^ (1 << order[-1])

    def early_copies(n):
        lo, hi = (0, 16 * EARLY, MID, D)[n:n + 2]
        return [out_copy(q, lo, hi) for q in range(CAP)]

    def start(copies):
        for cp in copies:
            cp.start()

    start(early_copies(0))
    rate, sent = MID // 8 - 2 * EARLY, [0]

    def project(w_ref):
        parts = []
        for n in range(0, FF // 128, 4):
            for lo in range(0, D, 128):
                hi = min(lo + 128, D)
                xs = x_sel[:, lo:hi]
                if hi - lo == 128 and min(rate, (len(done) - 4) * rate // END) > sent[0]:
                    sent[0] += 1
                    xs = tie(xs, next(side))
                w = [w_ref.bitcast(I32)[i, lo // 2:hi // 2, :] for i in range(n, n + 4)]
                v = jnp.dot(xs.astype(BF16), _mxu(jnp.concatenate(w, axis=1)),
                            preferred_element_type=F32)
                done.append(v[:, 0:128])
                acc = acc + v if lo else v
            parts.append(acc)
        return _rbf(jnp.concatenate(parts, axis=1))

    g = project(wg_v)
    act = _rbf(g * jax.nn.sigmoid(g)) * project(wu_v)
    for _ in range(rate - sent[0]):
        next(side)
    done.clear()

    cp_d.wait()

    start(early_copies(1))
    rest_side = list(side)

    def placed(r, words):
        idx = jnp.zeros((CAP, 128), I32)
        for c, m in enumerate(lanes(r)):
            idx = jnp.where(m, c, idx)
        return [_gather(w, idx) for w in words]

    def late_copies(lo, hi):
        return [out_copy(CAP + q, lo, hi) for q in range(CAP)]

    def words_of(n):
        return [new_v[n].bitcast(I32)[i:i + 8, :] for i in range(0, new_v[n].shape[0] // 2, 8)]

    tokens = []
    for n, (lo, hi) in enumerate(ROW_CHUNKS):
        a = [act[:, i:i + 128] for i in range(0, FF, 128)]
        for i, token in enumerate(rest_side):
            at = 8 + i * SPAN // len(rest_side) - n * len(a)
            if 0 <= at < len(a):
                a[at] = tie(a[at], token)
        if n == 1:
            start(early_copies(2))
        if n >= 2:
            cut = CUT * 128 // (hi - lo)
            a[cut] = tie(a[cut], tokens[n - 2])
        a = jnp.concatenate(a, axis=1)
        y = _rbf(jax.lax.dot_general(a.astype(BF16), wd_v[lo:hi, :], NT_DIMS,
                                     preferred_element_type=F32))
        new = h_sel[:, lo:hi] + _rbf(x_sel[:, lo:hi] + _rbf(y * gate))
        new_v[n][...] = jnp.concatenate(
            [new.T, jnp.zeros((hi - lo, 128 - CAP), F32)], axis=1).astype(BF16)
        rows = range(lo // 2, hi // 2, 8)
        words = words_of(n)
        both = list(zip(rows, placed(0, words), placed(1, words)))
        for c in range(CAP):
            for i, v0, v1 in both:
                pltpu.store(out_w.at[tile[c], pl.ds(i, 8), :],
                            jnp.where(rnd[c] == 0, v0, v1), mask=lane8 == col[c])
        for cp in late_copies(lo, hi):
            cp.start()
        out_w[tile[0], D // 2:, :] = lane8
        tokens.append(pltpu.bitcast(out_w[tile[0] | zero, D // 2:, :], F32))
    pltpu.make_async_copy(out_v.at[:, 0:D], out_v.at[:, 0:D], sem_o).wait()

    @pl.when(rounds > 2)
    def _():
        def fix(r, carry):
            rows = range(0, D // 2, 8)
            vals = placed(r, sum(map(words_of, range(len(new_v))), []))
            for c, m in enumerate(lanes(r)):
                for i, v in zip(rows, vals):
                    pltpu.store(out_w.at[tile[c], pl.ds(i, 8), :], v, mask=m)
            return carry

        jax.lax.fori_loop(2, rounds, fix, 0)
        for cp in late_copies(0, D):
            cp.start()
        for cp in late_copies(0, D):
            cp.wait()


@jax.jit
def pallas_sequential_preLN__ssm_conv_s4__moe_arch_mod__prompt_kernel(
    A_u: jax.Array,
    A_A_re: jax.Array,
    A_A_im: jax.Array,
    A_B_re: jax.Array,
    A_B_im: jax.Array,
    A_C_re: jax.Array,
    A_C_im: jax.Array,
    A_log_dt: jax.Array,
    A_Dskip: jax.Array,
    B_x: jax.Array,
    B_w_r: jax.Array,
    B_w_gate: jax.Array,
    B_w_up: jax.Array,
    B_w_down: jax.Array,
):
    del B_x
    hbm = pl.BlockSpec(memory_space=pl.ANY)
    out = pl.pallas_call(
        _kernel,
        out_shape=jax.ShapeDtypeStruct((D, L), BF16),
        in_specs=[hbm] * 13,
        out_specs=hbm,
        scratch_shapes=[
            pltpu.VMEM((NT, D + 16, 128), BF16),
            *[pltpu.VMEM((FF // 128, D + 16, 128), BF16)] * 2,
            pltpu.VMEM((D, FF), BF16),
            pltpu.VMEM((6, D, N), BF16),
            *[pltpu.VMEM((D,), BF16)] * 3,
            *[pltpu.VMEM((2, 16, 144, 128), BF16)] * 2,
            pltpu.VMEM((16, 2, 72, 128), I32),
            pltpu.VMEM((2, D, 128), F32),
            pltpu.VMEM((16, D), BF16),
            pltpu.VMEM((D // MB, 16, 128), BF16),
            pltpu.VMEM((2, 256, 128), F32),
            pltpu.VMEM((len(INDEX), 8, 128), I32),
            pltpu.VMEM((4, 3, 32, 16, 128), BF16),
            pltpu.VMEM((NT, D + 16, 128), BF16),
            pltpu.VMEM((NT, 2, 8, 128), F32),
            *[pltpu.VMEM((NT, 8, 128), F32)] * 2,
            pltpu.VMEM((NT, D + 16, 128), BF16),
            *[pltpu.VMEM((4, 4, 10, 8, 128), F32)] * 2,
            *[pltpu.VMEM((4, 4, 2, 112, 128), BF16)] * 2,
            *[pltpu.VMEM((4, 4, 2, 144, 128), BF16)] * 2,
            *[pltpu.VMEM((4, 8, 128), I32)] * 2,
            *[pltpu.VMEM((16, MB + 16, 128), BF16)] * 2,
            *[pltpu.VMEM((16, MB // 2 + 8, 128), I32)] * 2,
            *[pltpu.VMEM((4, 4, 2, MB + 8, 128), F32)] * 2,
            *[pltpu.VMEM((4, 4, 2, MB + 8, 128), F32)] * 2,
            *[pltpu.VMEM((16, MB // 2 + 8, 128), I32)] * 4,
            pltpu.SemaphoreType.DMA((15,)),
            pltpu.SemaphoreType.DMA((NT,)),
            pltpu.SemaphoreType.DMA((3,)),
            pltpu.SemaphoreType.DMA,
            *[pltpu.VMEM((4, 4, 2, MB + 8, 128), F32)] * 2,
            *[pltpu.VMEM((8, 8, 128), F32)] * 4,
            *[pltpu.VMEM((hi - lo, 128), BF16) for lo, hi in ROW_CHUNKS],
        ],
        compiler_params=pltpu.CompilerParams(vmem_limit_bytes=100 * 1024 * 1024,
                                             disable_bounds_checks=True,
                                             disable_semaphore_checks=True),
    )(A_u.reshape(L, D).T, A_A_re, A_A_im, A_B_re, A_B_im, A_C_re, A_C_im,
      A_log_dt, A_Dskip, B_w_r, B_w_gate, B_w_up, B_w_down.T)
    return out.T.reshape(1, L, D)
```

```python
import functools

import numpy as np
import jax
import jax.numpy as jnp
import jax.experimental.pallas as pl
import jax.experimental.pallas.tpu as pltpu

F32 = jnp.float32
BF16 = jnp.bfloat16
I32 = jnp.int32

L = 2048
D = 576
N = 128
FF = 4608
CAP = 8
NT = L // 128
EPS = 1e-5
MB = 64
PLANS = dict(
    s=(2, ""),
    st=(2, ""),
    n=(4, ""),
    stk=(2, "0:t:-1:4 1:t:-1:3 0:t:-1:4 0:t:-1:7 0:t:-1:15 1:t:-1:10 1:t:6:16 1:t:11:21 0:k "
            "0:k 1:k 0:s:-1:20 0:s:11:23 0:k:-1:23 1:k 1:s:20:-1 1:s 1:k "),
    stkFnf=(4, "1:t:-1:1 0:s:-1:9 0:s:-1:34 1:s:-1:35 1:s:-1:54 2:s:-1:69 3:s:-1:90 0:f "
               "0:n:1:19 0:F 0:t:4:25 0:t:0:19 0:k 0:t:12:43 0:k 0:k:-1:38 0:F 0:f 1:f "
               "1:t:29:44 1:F 1:n:33:47 1:t:35:58 1:k 1:k 1:t:42:57 1:k:-1:61 0:t:44:56 "
               "3:t:47:61 1:F 1:f 2:f 2:n:57:76 2:F 2:t:61:83 2:t:53:76 2:k 2:k 2:s:73:91 "
               "2:k:-1:92 2:t:70:98 2:F 2:f 3:f 3:t:85:100 3:F 3:n:89:104 3:t:91:-1 3:k "
               "3:s:95:111 3:k 3:t:98:110 3:k 2:t:100:110 3:F 3:f "),
    stkFnfm=(4, "0:m:-1:6 0:m:-1:5 0:t:-1:7 0:t:-1:14 0:t:-1:12 0:f 0:m:3:13 0:m:-1:18 "
                "0:m:3:18 0:f 0:m:6:20 0:k 0:t:8:25 0:n:9:27 0:m:13:33 0:m:13:25 1:m:12:34 0:k "
                "0:s:16:33 0:k:-1:35 0:s:19:33 1:m:18:33 0:F 1:t:20:35 0:F 1:t:27:42 1:t:24:40 "
                "1:f 1:f 1:m:32:42 1:m:31:46 1:m:31:46 1:m:34:48 1:k 1:t:37:50 1:n:37:55 "
                "2:m:39:62 1:k 1:s:44:61 1:m:43:61 1:m:41:53 1:k:-1:63 1:s:47:63 2:m:43:61 1:F "
                "2:t:48:63 1:F 2:t:55:70 2:t:50:68 2:f 2:f 2:m:60:70 2:m:60:78 2:m:59:71 "
                "2:m:62:76 2:k 2:t:66:78 2:n:65:85 2:k 2:s:72:89 2:m:71:89 2:m:69:81 2:k:-1:94 "
                "2:s:75:89 3:m:70:90 3:m:74:89 2:F 3:t:76:91 2:F 3:t:83:98 3:t:78:96 3:f 3:f "
                "3:m:88:98 3:m:87:102 3:m:87:102 3:m:90:104 3:k 3:t:93:108 3:n:94:110 3:k "
                "3:s:100:-1 3:m:99:-1 3:m:94:106 3:k 3:F 3:s:105:-1 3:F "),
    stkFnfmi=(4, "0:t:-1:2 0:n:-1:8 0:t:-1:3 0:m:-1:6 0:m:-1:7 0:m:-1:19 0:s:-1:40 1:s:-1:76 "
                 "2:s:-1:112 3:s 0:k 0:m:0:16 0:s:4:33 0:f 0:k 0:m:13:23 0:k:-1:33 0:m:14:25 "
                 "0:t:14:35 0:f 0:t:18:33 0:F 1:t:23:40 1:t:23:38 0:F 1:n:27:47 1:m:27:40 0:i "
                 "1:m:29:47 0:i 0:m:32:40 0:m:31:44 1:m:34:54 1:k 1:m:36:54 1:s:40:71 1:f 1:k "
                 "1:m:49:61 1:m:51:63 1:k:-1:71 1:f 1:t:55:79 1:t:51:68 1:F 2:t:59:74 "
                 "2:t:58:75 1:F 2:m:63:78 2:m:63:79 1:i 2:n:65:80 1:i 1:m:68:76 1:m:67:78 2:k "
                 "2:m:72:91 2:m:71:87 2:s:76:105 2:f 2:k 2:m:83:95 2:k:-1:108 2:m:86:97 "
                 "2:t:86:108 2:f 2:t:90:105 2:F 3:t:94:112 3:t:95:110 2:F 3:m:99:115 2:i "
                 "3:n:102:119 3:m:101:119 2:i 2:m:104:112 2:m:103:116 3:k 3:m:108:126 "
                 "3:m:111:126 3:s:112:143 3:f 3:k 3:m:121:133 3:k:-1:142 3:m:123:135 3:f "
                 "3:t:127:-1 3:t:123:140 3:F 3:F 3:i 3:m:139:-1 3:i 3:m:140:-1 "),
    stkFnfmia=(4, "0:t:-1:6 0:t:-1:3 0:n:-1:10 0:m:-1:6 0:m:-1:5 0:m:-1:19 0:s:-1:43 1:s:-1:80 "
                  "2:s:-1:117 3:s 0:a 0:f 0:m:1:20 0:k 0:s:5:40 0:k 0:m:14:26 0:m:-1:26 "
                  "0:k:-1:38 0:t:16:30 0:f 0:t:18:32 0:F 0:F 1:t:25:43 1:t:23:42 1:n:28:47 "
                  "1:m:25:43 1:m:27:43 0:i 0:m:32:40 0:i 0:m:34:42 1:a 1:f 1:m:38:56 1:m:36:57 "
                  "1:k 1:s:42:77 1:k 1:m:52:63 1:m:53:67 1:k:-1:75 1:t:53:67 1:f 1:t:55:69 1:F "
                  "1:F 2:t:64:80 2:t:57:76 2:n:65:84 2:m:62:80 2:m:61:80 1:i 1:m:69:77 1:i "
                  "1:m:71:81 2:m:73:93 2:a 2:f 2:m:75:94 2:k 2:s:79:114 2:k 2:m:89:100 "
                  "2:m:87:103 2:k:-1:112 2:t:90:104 2:f 2:t:92:106 2:F 2:F 3:t:99:117 "
                  "3:t:97:116 3:m:99:117 3:m:101:117 2:i 2:m:106:114 3:n:103:121 2:i "
                  "2:m:108:116 3:a 3:f 3:m:113:131 3:m:114:131 3:k 3:s:116:-1 3:k 3:m:126:137 "
                  "3:m:124:140 3:k:-1:145 3:t:127:141 3:f 3:t:129:-1 3:F 3:F 3:i 3:m:143:-1 "
                  "3:i 3:m:145:-1 "),
    tkFnfmia=(4, "1:m:-1:5 1:m:-1:3 0:n:-1:12 0:t:-1:3 0:t:-1:14 0:t:-1:21 0:t:-1:28 1:t:-1:40 "
                 "1:t:-1:51 1:t:-1:58 1:t:-1:65 2:t:-1:77 2:t:-1:88 0:F 0:m:2:14 0:m:-1:15 0:a "
                 "0:F 0:m:7:20 0:k 0:m:9:27 0:m:13:23 0:k 0:m:15:25 0:m:18:31 0:m:20:32 "
                 "0:k:-1:45 0:i 0:i 0:f 0:f 1:n:36:50 1:F 1:a 1:F 1:m:42:56 1:m:34:56 1:k "
                 "1:m:47:64 1:k 1:m:53:68 1:k:-1:75 1:i 1:i 3:m:63:79 3:m:61:77 1:f 1:m:68:76 "
                 "1:f 1:m:73:81 2:n:70:86 2:F 2:m:75:87 2:m:73:95 2:a 2:F 2:m:79:92 2:t:81:95 "
                 "2:t:-1:101 2:k 2:m:83:101 2:m:87:97 2:k 2:m:89:101 2:k:-1:119 2:i 2:m:95:105 "
                 "2:m:87:103 2:i 3:t:99:111 2:f 3:t:106:122 3:t:-1:129 2:f 3:n:110:124 3:F 3:a "
                 "3:F 3:m:116:129 3:m:111:134 3:k 3:m:121:141 3:m:124:141 3:t:125:139 3:k 3:k "
                 "3:i 3:i 3:f 3:m:142:-1 3:f 3:m:145:-1 "),
    kFnfmia=(4, "1:m:-1:5 1:m:-1:3 0:n:-1:12 0:F 0:m:2:14 0:m:-1:15 0:a 0:F 0:m:7:21 0:k "
                "0:m:9:27 0:m:13:23 0:k 0:m:15:25 0:m:18:31 0:m:20:32 0:k:-1:45 0:i 0:i 0:f "
                "0:f 1:n:36:50 1:F 1:a 1:F 1:m:42:57 1:m:34:56 1:k 1:m:47:64 1:k 1:m:53:66 "
                "1:k:-1:75 1:i 1:i 3:m:63:79 3:m:61:77 1:f 1:m:68:76 1:f 1:m:73:81 2:n:70:86 "
                "2:F 2:m:76:88 2:m:73:89 2:a 2:F 2:m:79:93 2:k 2:m:83:101 2:m:87:97 2:k "
                "2:m:89:101 2:k:-1:119 2:i 2:m:95:105 2:m:90:106 2:i 2:f 2:f 3:n:110:124 3:F "
                "3:a 3:F 3:m:116:130 3:m:111:134 3:k 3:m:121:141 3:m:124:141 3:k 3:k 3:i 3:i "
                "3:f 3:m:142:-1 3:f 3:m:145:-1 "),
    Ffmia=(4, "1:m:-1:9 0:m:-1:5 0:m:-1:10 0:m:-1:12 0:a 0:F 1:m:4:15 0:i 0:m:6:18 0:i "
              "0:m:9:22 0:F 1:m:16:31 0:f 0:m:20:33 0:f 0:m:22:33 1:a 1:m:25:43 1:F 0:m:29:41 "
              "1:i 1:i 1:m:37:50 1:F 1:m:40:54 1:f 1:m:42:57 1:m:45:56 3:m:45:59 2:m:42:58 1:f "
              "2:a 2:F 2:m:53:63 2:m:49:65 3:m:54:68 2:i 2:m:56:67 2:i 2:m:59:75 2:F 3:m:66:83 "
              "2:f 2:m:70:83 2:f 2:m:72:84 3:a 3:m:75:93 3:F 2:m:79:95 3:i 3:i 3:m:85:-1 3:F "
              "3:m:90:-1 3:f 3:m:92:-1 3:m:95:-1 3:f "),
    mia=(4, "1:m:-1:3 0:m:-1:8 0:m:-1:6 0:m:-1:7 0:m:-1:8 0:i 1:m:0:13 0:m:2:10 0:a 0:i "
            "1:m:5:16 2:m:8:25 1:i 1:m:9:22 0:m:10:23 0:m:8:20 1:m:8:20 3:m:11:25 1:a "
            "2:m:13:27 1:i 1:m:14:22 1:m:17:25 0:m:14:22 1:m:17:25 2:m:14:28 2:m:13:27 2:i "
            "3:m:18:32 2:m:20:32 2:a 2:i 3:m:23:-1 3:m:25:-1 3:m:25:-1 3:i 2:m:28:-1 2:m:27:-1 "
            "3:a 3:i 3:m:32:-1 3:m:35:-1 2:m:33:-1 3:m:35:-1 "),
    iaz=(4, "0:i 0:i 1:i 1:i 0:z 2:i 2:i 1:z 3:i 3:i 2:z 0:a 1:a 2:a 3:a 3:z"),
)
ROW_CHUNKS = ((0, 128), (128, 256), (256, 384), (384, 512), (512, D))
STOPS, MID, SPAN, EARLY, LAG, CUT, END = (384,), 480, 30, 8, 16, 12, 76
NT_DIMS = (((1,), (1,)), ((), ()))


def _round_res(step):
    return [int(np.round(r / step)) * step for r in range(16)]


RES1, RES2, RES3 = _round_res(2), _round_res(4), _round_res(8)


def _ds(start, size):
    return pl.ds(start if isinstance(start, int) else pl.multiple_of(start, size), size)


def _iota(shape, dim):
    return jax.lax.broadcasted_iota(I32, shape, dim)


def _rbf(x):
    return x.astype(BF16).astype(F32)


def _cmul(a, b):
    return (a[0] * b[0] - a[1] * b[1], a[0] * b[1] + a[1] * b[0])


def _csq(a):
    t = a[0] * a[1]
    return ((a[0] + a[1]) * (a[0] - a[1]), t + t)


def _cadd(a, b):
    return (a[0] + b[0], a[1] + b[1])


def _csub(a, b):
    return (a[0] - b[0], a[1] - b[1])


def _bfly4(a0, a1, a2, a3, inverse=False):
    s02, d02 = _cadd(a0, a2), _csub(a0, a2)
    s13, d13 = _cadd(a1, a3), _csub(a1, a3)
    p = (d02[0] - d13[1], d02[1] + d13[0])
    m = (d02[0] + d13[1], d02[1] - d13[0])
    if inverse:
        p, m = m, p
    return _cadd(s02, s13), p, _csub(s02, s13), m


def _prod_mod_1(a, b):
    fa, fb = _bfly4(*a), _bfly4(*b)
    return _bfly4(*[_cmul(x, y) for x, y in zip(fa, fb)], inverse=True)


def _prod2(a0, a1, b0, b1, sgn):
    p00, p11 = _cmul(a0, b0), _cmul(a1, b1)
    c1 = _cadd(_cmul(a0, b1), _cmul(a1, b0))
    if sgn > 0:
        return (p00[0] - p11[1], p00[1] + p11[0]), c1
    return (p00[0] + p11[1], p00[1] - p11[0]), c1


def _prod_mod_m1(a, b):
    def split(x):
        p = [(x[k][0] - x[k + 2][1], x[k][1] + x[k + 2][0]) for k in range(2)]
        m = [(x[k][0] + x[k + 2][1], x[k][1] - x[k + 2][0]) for k in range(2)]
        return p, m
    ap, am = split(a)
    bp, bm = split(b)
    cp = _prod2(*ap, *bp, 1)
    cm = _prod2(*am, *bm, -1)
    lo = [_cadd(cp[k], cm[k]) for k in range(2)]
    hi = [(cp[k][1] - cm[k][1], cm[k][0] - cp[k][0]) for k in range(2)]
    return lo + hi


def _prod_mod_i(a, b, sgn):
    sm = [x[0] + x[1] for x in b]
    df = [x[1] - x[0] for x in b]
    asum = [x[0] + x[1] for x in a]
    out = []
    for k in range(4):
        acc = [None, None, None]
        for j in range(4):
            m = (k - j) % 4
            if j <= k:
                t = ((b[m][0], 1), (df[m], 1), (sm[m], 1))
            elif sgn > 0:
                t = ((b[m][1], -1), (sm[m], 1), (df[m], -1))
            else:
                t = ((b[m][1], 1), (sm[m], -1), (df[m], 1))
            for q, (v, (w, s)) in enumerate(zip((asum[j], a[j][0], a[j][1]), t)):
                p = v * w
                if acc[q] is None:
                    acc[q] = p
                else:
                    acc[q] = acc[q] + p if s > 0 else acc[q] - p
        out.append((acc[0] - acc[2], acc[0] + acc[1]))
    return out


def _barrel(v, sch):
    for bit in range(4):
        m = sch.mask("bit%d" % bit)
        v = [jnp.where(m, v[(i + (1 << bit)) % 16], v[i]) for i in range(16)]
    return [v[-s % 16] for s in range(16)]


def _to_residues(tiles, sch):
    return _barrel([t if j == 0 else pltpu.roll(t, j, 1) for j, t in enumerate(tiles)], sch)


def _to_time(res, sch):
    return [t if j == 0 else pltpu.roll(t, 128 - j, 1)
            for j, t in enumerate(_barrel(res, sch))]


def _gather(x, idx, axis=1):
    return jnp.take_along_axis(x, idx, axis=axis, mode="promise_in_bounds")


def _transpose_dft(wt_ref, wu_ref, residues):
    for s in residues:
        for p in range(2):
            wt_ref[4 * (s % 4) + (0, 2, 1, 3)[s // 4], p, 0:64] = pltpu.bitcast(
                _mxu(wu_ref.bitcast(I32)[p, 4 * (s % 4) + s // 4, 0:64]).T, I32)


def _init_dft(wu_ref, wk_ref, tmp_ref, halfway):
    sub, k4 = _iota((8, 128), 0), 4 * _iota((8, 128), 1) + 1

    def cis(t):
        ph = ((k4 * t) & (4 * L - 1)).astype(F32) * (2 * np.pi / (4 * L))
        return jnp.cos(ph), jnp.sin(ph)

    w1, w16 = cis(1), cis(16)
    w32 = _csq(w16)
    fk = [cis(16 * (32 * (sub & 3) + (sub >> 2)))]
    fu = [cis(128 * sub), cis(128 * (sub + 8))]
    for v in range(1, 16):
        fk.append(_cmul(fk[-1], w32))
        if v >= 2:
            fu.append(_cmul(fu[-2], w16))
    for p in range(2):
        for v in range(32):
            tmp_ref[p, 8 * v:8 * v + 8, :] = fu[v % 16][p]
    tw = None
    for s in range(16):
        for v in range(0, 16, 2):
            rows = [slice(128 - s + 8 * i, 136 - s + 8 * i) for i in (v, v + 1)]
            for ref, f in ((wk_ref, fk[v:v + 2]),
                           (wu_ref, [(tmp_ref[0, r, :], tmp_ref[1, r, :]) for r in rows])):
                if s:
                    f = [_cmul(x, tw) for x in f]
                for p in range(2):
                    ref[p, 4 * (s % 4) + s // 4, 8 * v:8 * v + 16, :] = jnp.concatenate(
                        [f[0][p], f[1][p]], axis=0).astype(BF16)
        tw = _cmul(tw, w1) if s else w1
        if s == 7:
            halfway()


def _pack(ref, n, a, b):
    ref[n] = jnp.concatenate([a, b], axis=0).astype(BF16)
    return ref.bitcast(I32)[n]


def _split(w):
    return [pltpu.bitcast(w << 16, F32), pltpu.bitcast(w & -65536, F32)]


FINE = (0, 1, 2, 3, 4, 5, 6, 7, 512, 516, 1024, 1536)


def _k_seeds(z, c, sch):
    pw = {1: z}
    for e in range(1, 10):
        pw[1 << e] = _csq(pw[1 << (e - 1)])
    c8, z16 = _cmul(c, pw[8]), (pw[16][0], 0.0 - pw[16][1])
    pair = lambda a, b: tuple(jnp.where(sch.mask("odd"), q, p) for p, q in zip(a, b))
    seeds = []
    for g in range(2):
        twice = lambda v: tuple(_gather(x, sch.idx("dup%d" % g), 0) for x in v)
        seeds.append([twice(z), twice(pw[32]), twice(pw[512]),
                      pair(twice(c), twice(c8)), pair((1.0, 0.0), twice(z16))])
    return seeds


def _mxu(words):
    return pltpu.bitcast(words, BF16)


def _store_table(ref, tab):
    for i in range(0, len(tab), 2):
        for p in range(2):
            ref[p, 8 * i:8 * i + 16, :] = jnp.concatenate(
                [tab[i][p], tab[i + 1][p]], axis=0).astype(BF16)


def _k_residues(groups, k_last, dskip, tmp_ref, sch):
    idx, nxt = sch.idx("src"), sch.idx("nxt")
    low = lambda x, y: (x & 65535) | (y << 16)
    high = lambda x, y: jax.lax.shift_right_logical(x, 16) | (y & -65536)
    kv, up = {}, {}
    for i, k in enumerate(FINE):
        v = [g[8 * i:8 * i + 8] for g in groups]
        if k == 0:
            v = [x + jnp.where(sch.mask("diag"),
                               _gather(dskip[n // 2], sch.idx("dup%d" % (n % 2)), 0), 0.0)
                 for n, x in enumerate(v)]
        p = [_pack(tmp_ref, 2 * i + h, v[2 * h], v[2 * h + 1]) for h in range(2)]
        both = [_gather(x, idx) for x in p]
        kv[k], kv[k + 8] = low(*both), high(*both)
        if k % 512 == 0:
            up[k] = low(*[_gather(x, nxt) for x in p])
    k_last = _gather(k_last, sch.idx("rows"), 0)
    q0, q1, q2, up0, up01, up2, up3, fine = map(sch.mask, INDEX[-8:])
    s3 = {r: jnp.where(q2, kv[1024 + r], kv[1536 + r]) for r in (0, 8)}
    v0 = jnp.where(q0, kv[0], jnp.where(q1, kv[512], s3[0]))
    v16 = jnp.where(up01, jnp.where(up0, up[0], up[512]),
                    jnp.where(up2, up[1024], jnp.where(up3, up[1536], k_last)))
    s3[16] = v16
    s23, s123, out = {}, {}, [v0]
    for r in range(1, 16):
        k23 = (RES2[r], RES3[r])
        if k23 not in s23:
            s23[k23] = v16 if k23 == (16, 16) else jnp.where(q1, kv[512 + k23[0]], s3[k23[1]])
        k123 = (RES1[r],) + k23
        if k123 not in s123:
            s123[k123] = v16 if k123[0] == 16 else jnp.where(q0, kv[k123[0]], s23[k23])
        if RES1[r] == r:
            out.append(s123[k123])
        else:
            out.append(jnp.where(fine, kv[r], s123[k123]))
    return out


def _ln_scalars(s1, s2):
    mean = s1 * (1.0 / D)
    var = jnp.maximum(s2 * (1.0 / D) - mean * mean, 0.0)
    eps = float(np.asarray(EPS, dtype=BF16))
    sd = _rbf(jnp.sqrt(_rbf(_rbf(var) + eps)))
    return _rbf(mean), sd


def _top8(x):
    def swap(v, pairs):
        for i, j in pairs:
            v[i], v[j] = jnp.maximum(v[i], v[j]), jnp.minimum(v[i], v[j])
        return v

    def merge(a, b):
        v = [jnp.maximum(a[i], b[7 - i]) for i in range(8)]
        return swap(v, [(i, i + d) for d in (4, 2, 1) for i in range(8) if not i & d])

    sort8 = ((0, 2), (1, 3), (4, 6), (5, 7), (0, 4), (1, 5), (2, 6), (3, 7), (0, 1), (2, 3),
             (4, 5), (6, 7), (2, 4), (3, 5), (1, 4), (3, 6), (1, 2), (3, 4), (5, 6))
    v = merge(*[swap(x[i:i + 8], sort8) for i in (0, 8)])
    for d in (4, 2, 1):
        v = merge(v, [pltpu.roll(t, d, 0) for t in v])
    return v


def _init_columns(col_ref, wx_ref, wy_ref, ldt_ref, dsk_ref, wr_ref):
    row, lane = _iota((128, 128), 0), _iota((128, 128), 1)
    split = (row & ~15) + 2 * (row & 7) + ((row >> 3) & 1)
    ldt, dsk, wr = (ref[...].astype(F32).reshape(1, D) for ref in (ldt_ref, dsk_ref, wr_ref))
    for n, vec in enumerate((jnp.exp(ldt), dsk * (1.0 / L))):
        for lo in range(0, D, 128):
            i = min(lo, D - 128)
            diag = jnp.where(split == lane, vec[:, i:i + 128], 0.0)[lo - i:].astype(BF16)
            col_ref[n, lo:i + 128, :] = jnp.dot(diag, jnp.ones((128, 128), BF16),
                                                preferred_element_type=F32)
    sub = _iota((16, D), 0)
    ones_w = jnp.where(sub == 0, 1.0, jnp.where(sub == 1, wr, 0.0))
    wx_ref[...] = ones_w.astype(BF16)
    for lo in range(0, D, MB):
        wy_ref[lo // MB, :, 0:MB] = ones_w[:, lo:lo + MB].astype(BF16)
        wy_ref[lo // MB, :, MB:] = jnp.zeros((16, 128 - MB), BF16)


INDEX = ("true", "bit0", "bit1", "bit2", "bit3", "odd", "dup0", "dup1", "rows", "src", "nxt",
         "diag", "q0", "q1", "q2", "up0", "up01", "up2", "up3", "fine")


def _init_index(idx_ref):
    sub, lane = _iota((8, 128), 0), _iota((8, 128), 1)
    src = lambda b: 8 * ((b >> 1) & 15) + 2 * (sub & 3) + (b & 1)
    is_ = lambda m: jnp.where(m, 1, 0)
    q = lane & 3
    q16 = q + is_(lane >= 124)
    tiles = dict(true=sub + 1, odd=sub & 1, dup0=sub >> 1, dup1=4 + (sub >> 1),
                 rows=2 * (sub & 3) + (sub >> 2), src=src(lane >> 2), nxt=src((lane >> 2) + 1),
                 diag=is_((lane == sub) & ((sub & 1) == 0)), up01=is_(q16 < 2),
                 fine=is_((q == 0) & (lane < 64)),
                 **{"bit%d" % n: (lane >> n) & 1 for n in range(4)},
                 **{"q%d" % n: is_(q == n) for n in range(3)},
                 **{"up%d" % n: is_(q16 == n) for n in (0, 2, 3)})
    for n, name in enumerate(INDEX):
        idx_ref[n] = tiles[name]


class _Schedule:
    def __init__(self, zero, idx_ref):
        self.zero = zero
        self.idx = lambda name: idx_ref[INDEX.index(name) + zero]
        self.mask = lambda name: self.idx(name) != 0
        self.true = self.mask("true")
        self.done, self.pending, self.wait = [], {}, -1

    def tie(self, x, token):
        return jnp.where(self.true, x, token if token.dtype == x.dtype
                         else pltpu.bitcast(token, x.dtype))

    def start(self, x):
        return self.tie(x, self.done[self.wait]) if 0 <= self.wait < len(self.done) else x

    def lhs(self, words, first):
        tiles = [words[i:i + 8] for i in range(0, words.shape[0], 8)]
        for i in range(len(tiles) if first else 0):
            for token in self.pending.pop(len(self.done) + i, ()):
                tiles[i] = self.tie(tiles[i], token)
        return _mxu(jnp.concatenate(tiles, axis=0))

    def results(self, v):
        self.done += [v[i + 8:i + 16] for i in range(0, v.shape[0], 16)]

    def run(self, stage, wait, before):
        self.wait = wait
        self.pending.setdefault(before, []).extend(next(stage))


def _kernel(x_hbm, are_hbm, aim_hbm, bre_hbm, bim_hbm, cre_hbm, cim_hbm,
            ldt_hbm, dsk_hbm, wr_hbm, wg_hbm, wu_hbm, wd_hbm, out_hbm,
            x_v, wg_v, wu_v, wd_v, par_v, ldt_v, dsk_v, wr_v, w_v, wk_v, wt_v, col_v, wx_v, wy_v,
            tmp_v, idx_v, pk_v, h_v, st_v, acc_v, sq_v, out_v, sd0, sd1, ta0, ta1, tb0, tb1,
            kl0, kl1,
            u0, u1, k0, k1, a0_v, a1_v, c0, c1, r0, r1, r2, r3,
            sem_p, sem_x, sem_w, sem_o, f0_v, f1_v, *rest):
    half_v, new_v = rest[:4], rest[4:]
    cp_vec = [pltpu.make_async_copy(s, d, sem_p.at[n]) for n, (s, d) in enumerate(
        ((ldt_hbm, ldt_v), (dsk_hbm, dsk_v), (wr_hbm, wr_v)))]
    cp_par = [[pltpu.make_async_copy(s.at[lo:hi], par_v.at[n, lo:hi], sem_p.at[3 + 6 * m + n])
               for n, s in enumerate((are_hbm, aim_hbm, bre_hbm, bim_hbm, cre_hbm, cim_hbm))]
              for m, (lo, hi) in enumerate(((0, 4 * MB), (4 * MB, D)))]
    cp_x = [pltpu.make_async_copy(x_hbm.at[:, 128 * j:128 * j + 128], x_v.at[j, 0:D],
                                  sem_x.at[j])
            for j in range(NT)]
    cp_d = pltpu.make_async_copy(wd_hbm, wd_v, sem_w.at[2])

    def cp_w(i):
        return [pltpu.make_async_copy(s.at[:, _ds(128 * i, 128)], d.at[i, 0:D], sem_w.at[n])
                for n, (s, d) in enumerate(((wg_hbm, wg_v), (wu_hbm, wu_v)))]

    for cp in cp_vec + cp_par[0]:
        cp.start()
    for cp in cp_x[:NT // 2]:
        cp.start(priority=1)

    def columns():
        for cp in cp_vec:
            cp.wait()
        for cp in cp_x[NT // 2:]:
            cp.start(priority=1)
        _transpose_dft(wt_v, w_v, range(4))
        _init_columns(col_v, wx_v, wy_v, ldt_v, dsk_v, wr_v)

    _init_dft(w_v, wk_v, tmp_v, columns)
    for cp in cp_par[0]:
        cp.wait()

    sd, ta, tb, kl = (sd0, sd1), (ta0, ta1), (tb0, tb1), (kl0, kl1)
    uk, ab, cc, xr = ((u0, u1), (k0, k1)), ((a0_v, a1_v), (f0_v, f1_v)), (c0, c1), (r0, r1, r2, r3)
    ww, wt_w = (w_v.bitcast(I32), wk_v.bitcast(I32)), wt_v

    def seed_stage(b, r, sch):
        rows = _ds(b * MB // 2 + 8 * r, 8)
        par = [_split(par_v.bitcast(I32)[n, rows, :]) for n in range(6)]
        for h in range(2):
            a_re, a_im, b_re, b_im, c_re, c_im = [v[h] for v in par]
            dt = sch.start(col_v[0, _ds(b * MB + 16 * r + 8 * h, 8), :])
            mag, ang = jnp.exp(dt * a_re), dt * a_im
            sc = dt * (1.0 / L)
            seeds = _k_seeds((mag * jnp.cos(ang), mag * jnp.sin(ang)),
                             _cmul((c_re, c_im), (sc * b_re, sc * b_im)), sch)
            for g in range(2):
                for n, v in enumerate(seeds[g]):
                    for p in range(2):
                        sd[b % 2][r, 2 * h + g, 2 * n + p] = v[p]
            yield [sd[b % 2][(r + sch.zero), 2 * h, 0]]

    def table_stage(b, r, sch):
        tail = []
        for g in range(4):
            m1, m32, m512, a0, b0 = [
                (sd[b % 2][r, g, 2 * n], sd[b % 2][r, g, 2 * n + 1]) for n in range(5)]
            m32 = (sch.start(m32[0]), m32[1])
            fa = [a0]
            for _ in range(7):
                fa.append(_cmul(fa[-1], m1))
            for src in (0, 4, 8, 10):
                fa.append(_cmul(fa[src], m512))
            tail.append(fa[11][0] * m512[0] - fa[11][1] * m512[1])
            _store_table(ta[b % 2].at[r, g], fa)
            fb = [b0]
            for _ in range(15):
                p = fb[-1]
                fb.append((p[0] * m32[0] + p[1] * m32[1], p[1] * m32[0] - p[0] * m32[1]))
            _store_table(tb[b % 2].at[r, g], fb)
            yield [ta[b % 2].bitcast(I32)[(r + sch.zero), g, 0, 0:8, :],
                   tb[b % 2].bitcast(I32)[(r + sch.zero), g, 0, 0:8, :]]
        last = [jnp.where(sch.mask("odd"), pltpu.roll(tail[h + 1], 1, 0), tail[h])
                for h in (0, 2)]
        last = [pltpu.bitcast(_rbf(jnp.broadcast_to(jnp.sum(v, axis=1, keepdims=True),
                                                    (8, 128))), I32) for v in last]
        kl[b % 2][r] = jax.lax.shift_right_logical(last[0], 16) | last[1]

    def kernel_stage(b, r, sch):
        ta_w, tb_w = ta[b % 2].bitcast(I32), tb[b % 2].bitcast(I32)
        groups = [None] * 4
        for g0 in (0, 2):
            res = [jax.lax.dot_general(sch.lhs(ta_w[r, g, p, 0:48], g == g0 and p == 0),
                                       _mxu(tb_w[r, g, p, 0:64]), NT_DIMS, preferred_element_type=F32)
                   for g in (g0, g0 + 1) for p in range(2)]
            groups[g0], groups[g0 + 1] = res[0] + res[1], res[2] + res[3]
            sch.results(groups[g0 + 1])
            yield []
        dskip = [col_v[1, _ds(b * MB + 16 * r + 8 * h, 8), :] for h in range(2)]
        dst = _ds(8 * r, 8)
        res = _k_residues(groups, kl[b % 2][r], dskip, pk_v.at[sch.slot, 0], sch)
        for s, t in enumerate(res):
            uk[1][b % 2][4 * (s % 4) + s // 4, dst, :] = t
        yield [uk[1][b % 2][0, _ds(8 * (r + sch.zero), 8), :]]

    def norm_stage(b, r, sch):
        rows, dst = _ds(b * MB // 2 + 8 * r, 8), _ds(8 * r, 8)
        tiles = [x_v.bitcast(I32)[j, rows, :] for j in range(NT)]
        for s, t in enumerate(_to_residues([sch.start(tiles[0])] + tiles[1:], sch)):
            xr[b % 4][4 * (s % 4) + s // 4, dst, :] = t
            xs, m, inv = _mxu(t).astype(F32), st_v[s, 0], st_v[s, 1]
            uk[0][b % 2][4 * (s % 4) + s // 4, _ds(16 * r, 16), :] = jnp.concatenate(
                [(xs[0:8] - m) * inv, (xs[8:16] - m) * inv], axis=0).astype(BF16)
        yield [uk[0][b % 2].bitcast(I32)[0, _ds(8 * (r + sch.zero), 8), :]]

    def forward_stage(w, b, k, sch):
        dst = ab[w][b % len(ab[w])]
        for p in range(2):
            v = [jnp.dot(sch.lhs((uk[w][b % 2] if w else uk[w][b % 2].bitcast(I32))[
                4 * k + n, 0:MB // 2], n == 0),
                         _mxu(ww[w][p ^ (n & 1), 4 * k + n, 0:64]),
                         preferred_element_type=F32) for n in range(4)]
            d02, d13 = v[0] - v[2], v[1] - v[3]
            x1 = d02 - d13 if p == 0 else d02 + d13
            dst[0, k, p, 0:MB] = v[0] + v[2]
            dst[2, k, 1 - p, 0:MB] = v[1] + v[3]
            dst[1, k, p, 0:MB] = x1
            dst[3, k, p, 0:MB] = d02 + d13 if p == 0 else d02 - d13
            sch.results(x1)
            yield []

    def stats(tiles, sch):
        ones_w = wx_v.bitcast(I32)[...]
        for j in tiles:
            acc = None
            for i in range(0, D // 2, 8):
                v = [t * t for t in _split(x_v.bitcast(I32)[j, i:i + 8, :])]
                acc = v if acc is None else [p + q for p, q in zip(acc, v)]
            sums = jnp.dot(_mxu(jnp.concatenate(
                [ones_w[:, :128] if j % 2 == 0 else sch.tie(ones_w[:, :128], prev),
                 ones_w[:, 128:]], axis=1)),
                           _mxu(x_v.bitcast(I32)[j, 0:D // 2]), preferred_element_type=F32)
            s2 = prev = acc[0] + acc[1]
            for d in (4, 2, 1):
                s2 = s2 + pltpu.roll(s2, d, 0)
            mean, sd = _ln_scalars(jnp.broadcast_to(sums[0:1], (8, 128)), s2)
            st_v[j, 0], st_v[j, 1] = mean, 1.0 / sd

    def middle_stage(b, r, sch):
        src = [v[b % len(v)] for v in ab]
        scale = lambda v, f: [(x[0] * f, x[1] * f) for x in v]
        for h in range(2):
            ra = _ds(16 * r + 8 * h, 8)
            ld = lambda q, w, ra=ra: [(src[w][q, k, 0, ra, :], src[w][q, k, 1, ra, :]) for k in range(4)]

            park_v = half_v[2 * (sch.slot % 2) + h]

            def put(q, y):
                x = [park_v[n + sch.zero] for n in range(8)]
                for k in range(4):
                    for p in range(2):
                        cc[b % 2][k, q, p, ra, :] = x[2 * k + p] + y[k][p]
                        cc[b % 2][k, q + 2, p, ra, :] = x[2 * k + p] - y[k][p]

            def park(x):
                for k in range(4):
                    for p in range(2):
                        park_v[2 * k + p] = x[k][p]
                return [park_v[sch.zero]]

            gate = sch.start
            a0, a2, b0, b2 = ld(0, 0), ld(2, 0), ld(0, 1), ld(2, 1)
            a0[0] = (gate(a0[0][0]), a0[0][1])
            e0 = _prod_mod_1(list(map(_cadd, a0, a2)), list(map(_cadd, b0, b2)))
            again = _ds(16 * (r + sch.zero) + 8 * h, 8)
            yield park(e0)
            a0, a2, b0, b2 = (ld(q, w, again) for w in range(2) for q in (0, 2))
            a2[0] = (gate(a2[0][0]), a2[0][1])
            e2 = _prod_mod_m1(list(map(_csub, a0, a2)), scale(map(_csub, b0, b2), 2.0))
            put(0, e2)
            yield [cc[b % 2][0, 0, 0, again, :]]
            four = sch.start(jnp.full((8, 128), 4.0, F32))
            e1 = _prod_mod_i(ld(1, 0), scale(ld(1, 1), four), 1)
            yield park(e1)
            four = sch.start(jnp.full((8, 128), 4.0, F32))
            e3 = _prod_mod_i(ld(3, 0), scale(ld(3, 1), four), -1)
            put(1, e3)
            yield [cc[b % 2][0, 1, 0, again, :]]

    def inverse_stage(b, k, sch):
        src = cc[b % 2]

        def lhs(v, n, first):
            return sch.lhs(jnp.concatenate(
                [_pack(pk_v.at[sch.slot, 2], 4 * n + i // 16, v[i:i + 8], v[i + 8:i + 16])
                 for i in range(0, MB, 16)], axis=0), first)

        for o in range(2):
            p0, p1 = [(src[k, q, 0, 0:MB], src[k, q, 1, 0:MB]) for q in (2 * o, 2 * o + 1)]
            if o == 0:
                e = {0: _cadd(p0, p1), 2: _csub(p0, p1)}
            else:
                e = {1: (p0[0] + p1[1], p0[1] - p1[0]), 3: (p0[0] - p1[1], p0[1] + p1[0])}
            ys = []
            for n in e:
                y = [jnp.dot(lhs(e[n][p], 2 * n + p, n == o and p == 0),
                             _mxu(wt_w[4 * k + (0, 2, 1, 3)[n], p, 0:64]),
                             preferred_element_type=F32)
                     for p in range(2)]
                h = y[0] + y[1] + _mxu(xr[b % 4][4 * k + n, 0:MB // 2]).astype(F32)
                h_v[k + 4 * n, b * MB:b * MB + MB, :] = h.astype(BF16)
                hh = h * h
                sq_v[k + 4 * n] += sum((hh[i:i + 8] for i in range(8, MB, 8)), hh[0:8])
                ys.append(h)
            sch.results(ys[-1])
            yield []

    def sum_stage(b, r, sch):
        for n in range(4):
            s = r + 4 * n if b == nb - 1 else 4 * r + n
            sums = jnp.dot(sch.lhs(wy_v.bitcast(I32)[b], n == 0)[:, :MB],
                           _mxu(h_v.bitcast(I32)[s, b * MB // 2:(b + 1) * MB // 2]),
                           preferred_element_type=F32)
            acc_v[s] += sums[0:8]
        sch.results(sums)
        yield []

    nb = D // MB
    stages = dict(
        s=(seed_stage, 0), t=(table_stage, 1), k=(kernel_stage, 2),
        F=(functools.partial(forward_stage, 1), 3), n=(norm_stage, 2),
        f=(functools.partial(forward_stage, 0), 3), m=(middle_stage, 4),
        i=(inverse_stage, 5), a=(sum_stage, 6))

    def run(step, zero, live=None):
        live = live or {n: (f, step - lag) for n, (f, lag) in stages.items()
                        if 0 <= step - lag < nb and (n, step) != ("n", 2)}
        if step == nb + 4:
            live["z"] = (sum_stage, nb - 1)
        unroll, plan = PLANS["".join(live)]

        def body(it, carry):
            sch = _Schedule(zero >> (step % 32) if unroll == 4 else zero & it, idx_v)
            gens = [{n: f(b, it * unroll + u, sch) for n, (f, b) in live.items()}
                    for u in range(unroll)]
            if step == 3:
                for i in range(9 * unroll):
                    for cp in cp_w(9 * unroll * it + i):
                        cp.start()
            for item in plan.split():
                u, n, *ties = item.split(":")
                if n in live:
                    sch.slot = int(u)
                    sch.run(gens[int(u)][n], *map(int, ties or (-1, -1)))
            for sch.slot, g in enumerate(gens):
                for v in g.values():
                    for _ in v:
                        pass
            return carry + it

        if unroll == 4:
            if step == 101 or step > nb + 3:
                return body(0, 0)
            return jax.lax.fori_loop(zero, 1, lambda _, c: body(0, c), 0)
        return jax.lax.fori_loop(0, 4 // unroll, body, 0)

    _init_index(idx_v)
    acc_v[...] = sq_v[...] = jnp.zeros(acc_v.shape, F32)
    zero = run(0, 0) - 1
    for step in range(1, nb + 5):
        if step == 4:
            for cp in cp_par[1]:
                cp.wait()
        if step == 3:
            for half in range(2):
                tiles = range(NT // 2 * half, NT // 2 * (half + 1))
                for j in tiles:
                    cp_x[j].wait()
                if half:
                    cp_d.start(priority=1)
                else:
                    for cp in cp_par[1]:
                        cp.start()
                _transpose_dft(wt_v, w_v, range(4 + 6 * half, 10 + 6 * half))
                stats(tiles, _Schedule(zero, idx_v))
            for q in range(2):
                for s, v in enumerate(_to_residues([st_v[j, q] for j in range(NT)],
                                                   _Schedule(zero, idx_v))):
                    st_v[s, q] = v
            run(101, zero, dict(n=(norm_stage, 0)))
        run(step, zero)

    sums = [acc_v[s] for s in range(16)]
    m2, sd2 = _ln_scalars(
        jnp.concatenate([v[0:1] for v in sums], axis=0),
        jnp.concatenate([jnp.sum(sq_v[j], axis=0, keepdims=True) for j in range(NT)], axis=0))
    inv2 = 1.0 / sd2
    wsum = jnp.sum(wr_v[...].astype(F32).reshape(1, D), axis=1, keepdims=True)
    score = _rbf((jnp.concatenate([v[1:2] for v in sums], axis=0) - m2 * wsum) * inv2 + 0.0)
    sub16 = _iota((16, 128), 0)
    for s in range(16):
        h_v[s, D:, :] = jnp.where(sub16 == 0, m2[s:s + 1], jnp.where(
            sub16 == 1, sd2[s:s + 1], score[s:s + 1])).astype(BF16)
    bits = pltpu.bitcast(score, I32) >> 16
    order = jnp.where(bits < 0, -1 - bits, bits + 32768)
    mu = (_iota((NT, 128), 1) - _iota((NT, 128), 0)) & 127
    pos = 128 * (mu & 15) + 16 * (mu >> 4) + _iota((NT, 128), 0)
    key = pltpu.bitcast((order << 11) + (L - 1 - pos) + (1 << 29), F32)

    h_w, out_w = h_v.bitcast(I32), out_v.bitcast(I32)
    sch, done = _Schedule(zero, idx_v), []
    tie = sch.tie

    def unrouted():
        for q, v in enumerate((1.0 + inv2, m2 * inv2)):
            for j, t in enumerate(_to_time(
                    [jnp.broadcast_to(v[s:s + 1], (8, 128)) for s in range(16)], sch)):
                st_v[j, q] = t
        for i in range(0, D, 16):
            scal = st_v.at[pl.ds(zero * (i + 1), NT)]
            tiles = [h_w[s, i // 2:i // 2 + 8, :] for s in range(16)]
            if len(done) > LAG:
                tiles[0] = tie(tiles[0], done[-LAG])
            for j, v in enumerate(_to_time(tiles, sch)):
                h, mul, sub = _mxu(v).astype(F32), scal[j, 0], scal[j, 1]
                out_v[j, i:i + 16, :] = jnp.concatenate(
                    [h[0:8] * mul - sub, h[8:16] * mul - sub], axis=0).astype(BF16)
                if j % 8 == 7:
                    yield pltpu.bitcast(out_w[j + zero, i // 2:i // 2 + 8, :], F32)

    side = unrouted()

    lane8, sub8 = _iota((CAP, 128), 1), _iota((CAP, 128), 0)
    best = _top8([pltpu.roll(key[i:i + 8], n, 1) if n else key[i:i + 8]
                  for i in (0, 8) for n in range(8)])
    cand = best[0]
    for c in range(1, CAP):
        cand = jnp.where(sub8 == c, best[c], cand)
    best = _top8([pltpu.roll(cand, n, 1) if n else cand for n in range(0, 128, 8)])
    for _ in range(2 * EARLY):
        best[-1] = tie(best[-1], next(side))
    best = [pltpu.bitcast(v, I32)[0, 0] for v in best]
    picks = [L - 1 - (v & (L - 1)) for v in best]

    def schedule(col):
        rnd = [sum([(col[e] == col[c]).astype(I32) for e in range(c)], 0) for c in range(CAP)]
        return (rnd, functools.reduce(jnp.maximum, rnd) + 1,
                lambda n: [lane8 == jnp.where(rnd[c] == n, col[c], -1) for c in range(CAP)])

    _, rounds, lanes = schedule([((t >> 7) + (t & 127)) & 127 for t in picks])

    def out_copy(q, lo, hi):
        j = order[q]
        return pltpu.make_async_copy(
            out_v.at[j, lo:hi], out_hbm.at[lo:hi, _ds(j * 128, 128)], sem_o)

    for n, ref in enumerate((wg_v, wu_v)):
        pltpu.make_async_copy(ref.at[:, 0:D], ref.at[:, 0:D], sem_w.at[n]).wait()

    def gather(n, acc):
        masks = lanes(n)
        tiles = []
        for i in range(0, D // 2 + 8, 8):
            v = jnp.zeros((8, 128), I32)
            for c in range(CAP):
                v = jnp.where(masks[c], h_w[picks[c] & 15, i:i + 8, :], v)
            tiles.append(v)
        lhs = jnp.zeros((CAP, 128), F32)
        for c in range(CAP):
            lhs = jnp.where(masks[c] & (sub8 == c), 1.0, lhs)
        return acc + jax.lax.dot_general(lhs.astype(BF16), _mxu(jnp.concatenate(tiles, axis=0)),
                                         NT_DIMS, preferred_element_type=F32)

    h_sel = jax.lax.fori_loop(0, rounds, gather, jnp.zeros((CAP, D + 16), F32))
    m_sel, sd_sel, score_sel = (h_sel[:, D + q:D + q + 1] for q in range(3))
    h_sel = h_sel[:, :D]
    x_sel = _rbf(_rbf(h_sel - m_sel) / sd_sel)
    gate = _rbf(jax.nn.sigmoid(score_sel))

    tile, col = [t >> 7 for t in picks], [t & 127 for t in picks]
    rnd, rounds, lanes = schedule(col)
    late, again = 0, []
    for j in tile:
        again.append((late >> j) & 1)
        late = late | (1 << j)
    for dup in again[1:]:
        late = late | (late + dup)
    order = []
    for left in (late ^ ((1 << NT) - 1), late):
        for _ in range(CAP):
            order.append((31 - jax.lax.clz(left)) & (NT - 1))
            left = left ^ (1 << order[-1])

    def early_copies(n):
        lo, hi = (0, 16 * EARLY, *STOPS, MID, D)[n:n + 2]
        return [out_copy(q, lo, hi) for q in range(CAP)]

    def start(copies):
        for cp in copies:
            cp.start()

    start(early_copies(0))
    rate, sent = MID // 8 - 2 * EARLY, [0]

    def project(w_ref):
        parts = []
        for n in range(0, FF // 128, 4):
            for lo in range(0, D, 128):
                hi = min(lo + 128, D)
                xs = x_sel[:, lo:hi]
                if hi - lo == 128 and min(rate, (len(done) - 4) * rate // END) > sent[0]:
                    sent[0] += 1
                    xs = tie(xs, next(side))
                    if 16 * EARLY + 8 * sent[0] in STOPS:
                        start(early_copies(1 + STOPS.index(16 * EARLY + 8 * sent[0])))
                w = [w_ref.bitcast(I32)[i, lo // 2:hi // 2, :] for i in range(n, n + 4)]
                v = jnp.dot(xs.astype(BF16), _mxu(jnp.concatenate(w, axis=1)),
                            preferred_element_type=F32)
                done.append(v[:, 0:128])
                acc = acc + v if lo else v
            parts.append(acc)
        return _rbf(jnp.concatenate(parts, axis=1))

    g = project(wg_v)
    act = _rbf(g * jax.nn.sigmoid(g)) * project(wu_v)
    for _ in range(rate - sent[0]):
        next(side)
    done.clear()

    cp_d.wait()

    start(early_copies(len(STOPS) + 1))
    rest_side = list(side)

    def placed(r, words):
        idx = jnp.zeros((CAP, 128), I32)
        for c, m in enumerate(lanes(r)):
            idx = jnp.where(m, c, idx)
        return [_gather(w, idx) for w in words]

    def late_copies(lo, hi):
        return [out_copy(CAP + q, lo, hi) for q in range(CAP)]

    def words_of(n):
        return [new_v[n].bitcast(I32)[i:i + 8, :] for i in range(0, new_v[n].shape[0] // 2, 8)]

    tokens = []
    for n, (lo, hi) in enumerate(ROW_CHUNKS):
        a = [act[:, i:i + 128] for i in range(0, FF, 128)]
        for i, token in enumerate(rest_side):
            at = 8 + i * SPAN // len(rest_side) - n * len(a)
            if 0 <= at < len(a):
                a[at] = tie(a[at], token)
        if n == 1:
            start(early_copies(len(STOPS) + 2))
        if n >= 2:
            cut = CUT * 128 // (hi - lo)
            a[cut] = tie(a[cut], tokens[n - 2])
        a = jnp.concatenate(a, axis=1)
        y = _rbf(jax.lax.dot_general(a.astype(BF16), wd_v[lo:hi, :], NT_DIMS,
                                     preferred_element_type=F32))
        new = h_sel[:, lo:hi] + _rbf(x_sel[:, lo:hi] + _rbf(y * gate))
        new_v[n][...] = jnp.concatenate(
            [new.T, jnp.zeros((hi - lo, 128 - CAP), F32)], axis=1).astype(BF16)
        rows = range(lo // 2, hi // 2, 8)
        words = words_of(n)
        both = list(zip(rows, placed(0, words), placed(1, words)))
        for c in range(CAP):
            for i, v0, v1 in both:
                pltpu.store(out_w.at[tile[c], pl.ds(i, 8), :],
                            jnp.where(rnd[c] == 0, v0, v1), mask=lane8 == col[c])
        for cp in late_copies(lo, hi):
            cp.start()
        out_w[tile[0], D // 2:, :] = lane8
        tokens.append(pltpu.bitcast(out_w[tile[0] | zero, D // 2:, :], F32))
    pltpu.make_async_copy(out_v.at[:, 0:D], out_v.at[:, 0:D], sem_o).wait()

    @pl.when(rounds > 2)
    def _():
        def fix(r, carry):
            rows = range(0, D // 2, 8)
            vals = placed(r, sum(map(words_of, range(len(new_v))), []))
            for c, m in enumerate(lanes(r)):
                for i, v in zip(rows, vals):
                    pltpu.store(out_w.at[tile[c], pl.ds(i, 8), :], v, mask=m)
            return carry

        jax.lax.fori_loop(2, rounds, fix, 0)
        for cp in late_copies(0, D):
            cp.start()
        for cp in late_copies(0, D):
            cp.wait()


@jax.jit
def pallas_sequential_preLN__ssm_conv_s4__moe_arch_mod__prompt_kernel(
    A_u: jax.Array,
    A_A_re: jax.Array,
    A_A_im: jax.Array,
    A_B_re: jax.Array,
    A_B_im: jax.Array,
    A_C_re: jax.Array,
    A_C_im: jax.Array,
    A_log_dt: jax.Array,
    A_Dskip: jax.Array,
    B_x: jax.Array,
    B_w_r: jax.Array,
    B_w_gate: jax.Array,
    B_w_up: jax.Array,
    B_w_down: jax.Array,
):
    del B_x
    hbm = pl.BlockSpec(memory_space=pl.ANY)
    out = pl.pallas_call(
        _kernel,
        out_shape=jax.ShapeDtypeStruct((D, L), BF16),
        in_specs=[hbm] * 13,
        out_specs=hbm,
        scratch_shapes=[
            pltpu.VMEM((NT, D + 16, 128), BF16),
            *[pltpu.VMEM((FF // 128, D + 16, 128), BF16)] * 2,
            pltpu.VMEM((D, FF), BF16),
            pltpu.VMEM((6, D, N), BF16),
            *[pltpu.VMEM((D,), BF16)] * 3,
            *[pltpu.VMEM((2, 16, 144, 128), BF16)] * 2,
            pltpu.VMEM((16, 2, 72, 128), I32),
            pltpu.VMEM((2, D, 128), F32),
            pltpu.VMEM((16, D), BF16),
            pltpu.VMEM((D // MB, 16, 128), BF16),
            pltpu.VMEM((2, 256, 128), F32),
            pltpu.VMEM((len(INDEX), 8, 128), I32),
            pltpu.VMEM((4, 3, 32, 16, 128), BF16),
            pltpu.VMEM((NT, D + 16, 128), BF16),
            pltpu.VMEM((NT, 2, 8, 128), F32),
            *[pltpu.VMEM((NT, 8, 128), F32)] * 2,
            pltpu.VMEM((NT, D + 16, 128), BF16),
            *[pltpu.VMEM((4, 4, 10, 8, 128), F32)] * 2,
            *[pltpu.VMEM((4, 4, 2, 112, 128), BF16)] * 2,
            *[pltpu.VMEM((4, 4, 2, 144, 128), BF16)] * 2,
            *[pltpu.VMEM((4, 8, 128), I32)] * 2,
            *[pltpu.VMEM((16, MB + 16, 128), BF16)] * 2,
            *[pltpu.VMEM((16, MB // 2 + 8, 128), I32)] * 2,
            *[pltpu.VMEM((4, 4, 2, MB + 8, 128), F32)] * 2,
            *[pltpu.VMEM((4, 4, 2, MB + 8, 128), F32)] * 2,
            *[pltpu.VMEM((16, MB // 2 + 8, 128), I32)] * 4,
            pltpu.SemaphoreType.DMA((15,)),
            pltpu.SemaphoreType.DMA((NT,)),
            pltpu.SemaphoreType.DMA((3,)),
            pltpu.SemaphoreType.DMA,
            *[pltpu.VMEM((4, 4, 2, MB + 8, 128), F32)] * 2,
            *[pltpu.VMEM((8, 8, 128), F32)] * 4,
            *[pltpu.VMEM((hi - lo, 128), BF16) for lo, hi in ROW_CHUNKS],
        ],
        compiler_params=pltpu.CompilerParams(vmem_limit_bytes=100 * 1024 * 1024,
                                             disable_bounds_checks=True,
                                             disable_semaphore_checks=True),
    )(A_u.reshape(L, D).T, A_A_re, A_A_im, A_B_re, A_B_im, A_C_re, A_C_im,
      A_log_dt, A_Dskip, B_w_r, B_w_gate, B_w_up, B_w_down.T)
    return out.T.reshape(1, L, D)
```

```python
import functools

import numpy as np
import jax
import jax.numpy as jnp
import jax.experimental.pallas as pl
import jax.experimental.pallas.tpu as pltpu

F32 = jnp.float32
BF16 = jnp.bfloat16
I32 = jnp.int32

L = 2048
D = 576
N = 128
FF = 4608
CAP = 8
NT = L // 128
EPS = 1e-5
MB = 64
PLANS = dict(
    s=(2, ""),
    st=(2, ""),
    n=(4, ""),
    stk=(2, "0:t:-1:4 1:t:-1:3 0:t:-1:4 0:t:-1:7 0:t:-1:15 1:t:-1:10 1:t:6:16 1:t:11:21 0:k "
            "0:k 1:k 0:s:-1:20 0:s:11:23 0:k:-1:23 1:k 1:s:20:-1 1:s 1:k "),
    stkFnf=(4, "1:t:-1:1 0:s:-1:9 0:s:-1:34 1:s:-1:35 1:s:-1:54 2:s:-1:69 3:s:-1:90 0:f "
               "0:n:1:19 0:F 0:t:4:25 0:t:0:19 0:k 0:t:12:43 0:k 0:k:-1:38 0:F 0:f 1:f "
               "1:t:29:44 1:F 1:n:33:47 1:t:35:58 1:k 1:k 1:t:42:57 1:k:-1:61 0:t:44:56 "
               "3:t:47:61 1:F 1:f 2:f 2:n:57:76 2:F 2:t:61:83 2:t:53:76 2:k 2:k 2:s:73:91 "
               "2:k:-1:92 2:t:70:98 2:F 2:f 3:f 3:t:85:100 3:F 3:n:89:104 3:t:91:-1 3:k "
               "3:s:95:111 3:k 3:t:98:110 3:k 2:t:100:110 3:F 3:f "),
    stkFnfm=(4, "0:m:-1:6 0:m:-1:5 0:t:-1:7 0:t:-1:14 0:t:-1:12 0:f 0:m:3:13 0:m:-1:18 "
                "0:m:3:18 0:f 0:m:6:20 0:k 0:t:8:25 0:n:9:27 0:m:13:33 0:m:13:25 1:m:12:34 0:k "
                "0:s:16:33 0:k:-1:35 0:s:19:33 1:m:18:33 0:F 1:t:20:35 0:F 1:t:27:42 1:t:24:40 "
                "1:f 1:f 1:m:32:42 1:m:31:46 1:m:31:46 1:m:34:48 1:k 1:t:37:50 1:n:37:55 "
                "2:m:39:62 1:k 1:s:44:61 1:m:43:61 1:m:41:53 1:k:-1:63 1:s:47:63 2:m:43:61 1:F "
                "2:t:48:63 1:F 2:t:55:70 2:t:50:68 2:f 2:f 2:m:60:70 2:m:60:78 2:m:59:71 "
                "2:m:62:76 2:k 2:t:66:78 2:n:65:85 2:k 2:s:72:89 2:m:71:89 2:m:69:81 2:k:-1:94 "
                "2:s:75:89 3:m:70:90 3:m:74:89 2:F 3:t:76:91 2:F 3:t:83:98 3:t:78:96 3:f 3:f "
                "3:m:88:98 3:m:87:102 3:m:87:102 3:m:90:104 3:k 3:t:93:108 3:n:94:110 3:k "
                "3:s:100:-1 3:m:99:-1 3:m:94:106 3:k 3:F 3:s:105:-1 3:F "),
    stkFnfmi=(4, "0:t:-1:2 0:n:-1:8 0:t:-1:3 0:m:-1:6 0:m:-1:7 0:m:-1:19 0:s:-1:40 1:s:-1:76 "
                 "2:s:-1:112 3:s 0:k 0:m:0:16 0:s:4:33 0:f 0:k 0:m:13:23 0:k:-1:33 0:m:14:25 "
                 "0:t:14:35 0:f 0:t:18:33 0:F 1:t:23:40 1:t:23:38 0:F 1:n:27:47 1:m:27:40 0:i "
                 "1:m:29:47 0:i 0:m:32:40 0:m:31:44 1:m:34:54 1:k 1:m:36:54 1:s:40:71 1:f 1:k "
                 "1:m:49:61 1:m:51:63 1:k:-1:71 1:f 1:t:55:79 1:t:51:68 1:F 2:t:59:74 "
                 "2:t:58:75 1:F 2:m:63:78 2:m:63:79 1:i 2:n:65:80 1:i 1:m:68:76 1:m:67:78 2:k "
                 "2:m:72:91 2:m:71:87 2:s:76:105 2:f 2:k 2:m:83:95 2:k:-1:108 2:m:86:97 "
                 "2:t:86:108 2:f 2:t:90:105 2:F 3:t:94:112 3:t:95:110 2:F 3:m:99:115 2:i "
                 "3:n:102:119 3:m:101:119 2:i 2:m:104:112 2:m:103:116 3:k 3:m:108:126 "
                 "3:m:111:126 3:s:112:143 3:f 3:k 3:m:121:133 3:k:-1:142 3:m:123:135 3:f "
                 "3:t:127:-1 3:t:123:140 3:F 3:F 3:i 3:m:139:-1 3:i 3:m:140:-1 "),
    stkFnfmia=(4, "0:t:-1:6 0:t:-1:3 0:n:-1:10 0:m:-1:6 0:m:-1:5 0:m:-1:19 0:s:-1:43 1:s:-1:80 "
                  "2:s:-1:117 3:s 0:a 0:f 0:m:1:20 0:k 0:s:5:40 0:k 0:m:14:26 0:m:-1:26 "
                  "0:k:-1:38 0:t:16:30 0:f 0:t:18:32 0:F 0:F 1:t:25:43 1:t:23:42 1:n:28:47 "
                  "1:m:25:43 1:m:27:43 0:i 0:m:32:40 0:i 0:m:34:42 1:a 1:f 1:m:38:56 1:m:36:57 "
                  "1:k 1:s:42:77 1:k 1:m:52:63 1:m:53:67 1:k:-1:75 1:t:53:67 1:f 1:t:55:69 1:F "
                  "1:F 2:t:64:80 2:t:57:76 2:n:65:84 2:m:62:80 2:m:61:80 1:i 1:m:69:77 1:i "
                  "1:m:71:81 2:m:73:93 2:a 2:f 2:m:75:94 2:k 2:s:79:114 2:k 2:m:89:100 "
                  "2:m:87:103 2:k:-1:112 2:t:90:104 2:f 2:t:92:106 2:F 2:F 3:t:99:117 "
                  "3:t:97:116 3:m:99:117 3:m:101:117 2:i 2:m:106:114 3:n:103:121 2:i "
                  "2:m:108:116 3:a 3:f 3:m:113:131 3:m:114:131 3:k 3:s:116:-1 3:k 3:m:126:137 "
                  "3:m:124:140 3:k:-1:145 3:t:127:141 3:f 3:t:129:-1 3:F 3:F 3:i 3:m:143:-1 "
                  "3:i 3:m:145:-1 "),
    tkFnfmia=(4, "1:m:-1:5 1:m:-1:3 0:n:-1:12 0:t:-1:3 0:t:-1:14 0:t:-1:21 0:t:-1:28 1:t:-1:40 "
                 "1:t:-1:51 1:t:-1:58 1:t:-1:65 2:t:-1:77 2:t:-1:88 0:F 0:m:2:14 0:m:-1:15 0:a "
                 "0:F 0:m:7:20 0:k 0:m:9:27 0:m:13:23 0:k 0:m:15:25 0:m:18:31 0:m:20:32 "
                 "0:k:-1:45 0:i 0:i 0:f 0:f 1:n:36:50 1:F 1:a 1:F 1:m:42:56 1:m:34:56 1:k "
                 "1:m:47:64 1:k 1:m:53:68 1:k:-1:75 1:i 1:i 3:m:63:79 3:m:61:77 1:f 1:m:68:76 "
                 "1:f 1:m:73:81 2:n:70:86 2:F 2:m:75:87 2:m:73:95 2:a 2:F 2:m:79:92 2:t:81:95 "
                 "2:t:-1:101 2:k 2:m:83:101 2:m:87:97 2:k 2:m:89:101 2:k:-1:119 2:i 2:m:95:105 "
                 "2:m:87:103 2:i 3:t:99:111 2:f 3:t:106:122 3:t:-1:129 2:f 3:n:110:124 3:F 3:a "
                 "3:F 3:m:116:129 3:m:111:134 3:k 3:m:121:141 3:m:124:141 3:t:125:139 3:k 3:k "
                 "3:i 3:i 3:f 3:m:142:-1 3:f 3:m:145:-1 "),
    kFnfmia=(4, "1:m:-1:5 1:m:-1:3 0:n:-1:12 0:F 0:m:2:14 0:m:-1:15 0:a 0:F 0:m:7:21 0:k "
                "0:m:9:27 0:m:13:23 0:k 0:m:15:25 0:m:18:31 0:m:20:32 0:k:-1:45 0:i 0:i 0:f "
                "0:f 1:n:36:50 1:F 1:a 1:F 1:m:42:57 1:m:34:56 1:k 1:m:47:64 1:k 1:m:53:66 "
                "1:k:-1:75 1:i 1:i 3:m:63:79 3:m:61:77 1:f 1:m:68:76 1:f 1:m:73:81 2:n:70:86 "
                "2:F 2:m:76:88 2:m:73:89 2:a 2:F 2:m:79:93 2:k 2:m:83:101 2:m:87:97 2:k "
                "2:m:89:101 2:k:-1:119 2:i 2:m:95:105 2:m:90:106 2:i 2:f 2:f 3:n:110:124 3:F "
                "3:a 3:F 3:m:116:130 3:m:111:134 3:k 3:m:121:141 3:m:124:141 3:k 3:k 3:i 3:i "
                "3:f 3:m:142:-1 3:f 3:m:145:-1 "),
    Ffmia=(4, "1:m:-1:9 0:m:-1:5 0:m:-1:10 0:m:-1:12 0:a 0:F 1:m:4:15 0:i 0:m:6:18 0:i "
              "0:m:9:22 0:F 1:m:16:31 0:f 0:m:20:33 0:f 0:m:22:33 1:a 1:m:25:43 1:F 0:m:29:41 "
              "1:i 1:i 1:m:37:50 1:F 1:m:40:54 1:f 1:m:42:57 1:m:45:56 3:m:45:59 2:m:42:58 1:f "
              "2:a 2:F 2:m:53:63 2:m:49:65 3:m:54:68 2:i 2:m:56:67 2:i 2:m:59:75 2:F 3:m:66:83 "
              "2:f 2:m:70:83 2:f 2:m:72:84 3:a 3:m:75:93 3:F 2:m:79:95 3:i 3:i 3:m:85:-1 3:F "
              "3:m:90:-1 3:f 3:m:92:-1 3:m:95:-1 3:f "),
    mia=(4, "1:m:-1:3 0:m:-1:8 0:m:-1:6 0:m:-1:7 0:m:-1:8 0:i 1:m:0:13 0:m:2:10 0:a 0:i "
            "1:m:5:16 2:m:8:25 1:i 1:m:9:22 0:m:10:23 0:m:8:20 1:m:8:20 3:m:11:25 1:a "
            "2:m:13:27 1:i 1:m:14:22 1:m:17:25 0:m:14:22 1:m:17:25 2:m:14:28 2:m:13:27 2:i "
            "3:m:18:32 2:m:20:32 2:a 2:i 3:m:23:-1 3:m:25:-1 3:m:25:-1 3:i 2:m:28:-1 2:m:27:-1 "
            "3:a 3:i 3:m:32:-1 3:m:35:-1 2:m:33:-1 3:m:35:-1 "),
    ia=(4, "0:a 1:a 2:a 3:a 0:i 0:i 1:i 1:i 2:i 2:i 3:i 3:i"),
)
ROW_CHUNKS = ((0, 128), (128, 256), (256, 384), (384, 512), (512, D))
STOPS, MID, SPAN, EARLY, LAG, CUT, END = (384,), 480, 30, 8, 16, 12, 76
NT_DIMS = (((1,), (1,)), ((), ()))


def _round_res(step):
    return [int(np.round(r / step)) * step for r in range(16)]


RES1, RES2, RES3 = _round_res(2), _round_res(4), _round_res(8)


def _ds(start, size):
    return pl.ds(start if isinstance(start, int) else pl.multiple_of(start, size), size)


def _iota(shape, dim):
    return jax.lax.broadcasted_iota(I32, shape, dim)


def _rbf(x):
    return x.astype(BF16).astype(F32)


def _cmul(a, b):
    return (a[0] * b[0] - a[1] * b[1], a[0] * b[1] + a[1] * b[0])


def _csq(a):
    t = a[0] * a[1]
    return ((a[0] + a[1]) * (a[0] - a[1]), t + t)


def _cadd(a, b):
    return (a[0] + b[0], a[1] + b[1])


def _csub(a, b):
    return (a[0] - b[0], a[1] - b[1])


def _bfly4(a0, a1, a2, a3, inverse=False):
    s02, d02 = _cadd(a0, a2), _csub(a0, a2)
    s13, d13 = _cadd(a1, a3), _csub(a1, a3)
    p = (d02[0] - d13[1], d02[1] + d13[0])
    m = (d02[0] + d13[1], d02[1] - d13[0])
    if inverse:
        p, m = m, p
    return _cadd(s02, s13), p, _csub(s02, s13), m


def _prod_mod_1(a, b):
    fa, fb = _bfly4(*a), _bfly4(*b)
    return _bfly4(*[_cmul(x, y) for x, y in zip(fa, fb)], inverse=True)


def _prod2(a0, a1, b0, b1, sgn):
    p00, p11 = _cmul(a0, b0), _cmul(a1, b1)
    c1 = _cadd(_cmul(a0, b1), _cmul(a1, b0))
    if sgn > 0:
        return (p00[0] - p11[1], p00[1] + p11[0]), c1
    return (p00[0] + p11[1], p00[1] - p11[0]), c1


def _prod_mod_m1(a, b):
    def split(x):
        p = [(x[k][0] - x[k + 2][1], x[k][1] + x[k + 2][0]) for k in range(2)]
        m = [(x[k][0] + x[k + 2][1], x[k][1] - x[k + 2][0]) for k in range(2)]
        return p, m
    ap, am = split(a)
    bp, bm = split(b)
    cp = _prod2(*ap, *bp, 1)
    cm = _prod2(*am, *bm, -1)
    lo = [_cadd(cp[k], cm[k]) for k in range(2)]
    hi = [(cp[k][1] - cm[k][1], cm[k][0] - cp[k][0]) for k in range(2)]
    return lo + hi


def _prod_mod_i(a, b, sgn):
    sm = [x[0] + x[1] for x in b]
    df = [x[1] - x[0] for x in b]
    asum = [x[0] + x[1] for x in a]
    out = []
    for k in range(4):
        acc = [None, None, None]
        for j in range(4):
            m = (k - j) % 4
            if j <= k:
                t = ((b[m][0], 1), (df[m], 1), (sm[m], 1))
            elif sgn > 0:
                t = ((b[m][1], -1), (sm[m], 1), (df[m], -1))
            else:
                t = ((b[m][1], 1), (sm[m], -1), (df[m], 1))
            for q, (v, (w, s)) in enumerate(zip((asum[j], a[j][0], a[j][1]), t)):
                p = v * w
                if acc[q] is None:
                    acc[q] = p
                else:
                    acc[q] = acc[q] + p if s > 0 else acc[q] - p
        out.append((acc[0] - acc[2], acc[0] + acc[1]))
    return out


def _barrel(v, sch):
    for bit in range(4):
        m = sch.mask("bit%d" % bit)
        v = [jnp.where(m, v[(i + (1 << bit)) % 16], v[i]) for i in range(16)]
    return [v[-s % 16] for s in range(16)]


def _to_residues(tiles, sch):
    return _barrel([t if j == 0 else pltpu.roll(t, j, 1) for j, t in enumerate(tiles)], sch)


def _to_time(res, sch):
    return [t if j == 0 else pltpu.roll(t, 128 - j, 1)
            for j, t in enumerate(_barrel(res, sch))]


def _gather(x, idx, axis=1):
    return jnp.take_along_axis(x, idx, axis=axis, mode="promise_in_bounds")


def _transpose_dft(wt_ref, wu_ref, residues):
    for s in residues:
        for p in range(2):
            wt_ref[4 * (s % 4) + (0, 2, 1, 3)[s // 4], p, 0:64] = pltpu.bitcast(
                _mxu(wu_ref.bitcast(I32)[p, 4 * (s % 4) + s // 4, 0:64]).T, I32)


def _init_dft(wu_ref, wk_ref, tmp_ref, halfway):
    sub, k4 = _iota((8, 128), 0), 4 * _iota((8, 128), 1) + 1

    def cis(t):
        ph = ((k4 * t) & (4 * L - 1)).astype(F32) * (2 * np.pi / (4 * L))
        return jnp.cos(ph), jnp.sin(ph)

    w1, w16 = cis(1), cis(16)
    w32 = _csq(w16)
    fk = [cis(16 * (32 * (sub & 3) + (sub >> 2)))]
    fu = [cis(128 * sub), cis(128 * (sub + 8))]
    for v in range(1, 16):
        fk.append(_cmul(fk[-1], w32))
        if v >= 2:
            fu.append(_cmul(fu[-2], w16))
    for p in range(2):
        for v in range(32):
            tmp_ref[p, 8 * v:8 * v + 8, :] = fu[v % 16][p]
    tw = None
    for s in range(16):
        for v in range(0, 16, 2):
            rows = [slice(128 - s + 8 * i, 136 - s + 8 * i) for i in (v, v + 1)]
            for ref, f in ((wk_ref, fk[v:v + 2]),
                           (wu_ref, [(tmp_ref[0, r, :], tmp_ref[1, r, :]) for r in rows])):
                if s:
                    f = [_cmul(x, tw) for x in f]
                for p in range(2):
                    ref[p, 4 * (s % 4) + s // 4, 8 * v:8 * v + 16, :] = jnp.concatenate(
                        [f[0][p], f[1][p]], axis=0).astype(BF16)
        tw = _cmul(tw, w1) if s else w1
        if s == 7:
            halfway()


def _pack(ref, n, a, b):
    ref[n] = jnp.concatenate([a, b], axis=0).astype(BF16)
    return ref.bitcast(I32)[n]


def _split(w):
    return [pltpu.bitcast(w << 16, F32), pltpu.bitcast(w & -65536, F32)]


FINE = (0, 1, 2, 3, 4, 5, 6, 7, 512, 516, 1024, 1536)


def _k_seeds(z, c, sch):
    pw = {1: z}
    for e in range(1, 10):
        pw[1 << e] = _csq(pw[1 << (e - 1)])
    c8, z16 = _cmul(c, pw[8]), (pw[16][0], 0.0 - pw[16][1])
    pair = lambda a, b: tuple(jnp.where(sch.mask("odd"), q, p) for p, q in zip(a, b))
    seeds = []
    for g in range(2):
        twice = lambda v: tuple(_gather(x, sch.idx("dup%d" % g), 0) for x in v)
        seeds.append([twice(z), twice(pw[32]), twice(pw[512]),
                      pair(twice(c), twice(c8)), pair((1.0, 0.0), twice(z16))])
    return seeds


def _mxu(words):
    return pltpu.bitcast(words, BF16)


def _store_table(ref, tab):
    for i in range(0, len(tab), 2):
        for p in range(2):
            ref[p, 8 * i:8 * i + 16, :] = jnp.concatenate(
                [tab[i][p], tab[i + 1][p]], axis=0).astype(BF16)


def _k_residues(groups, k_last, dskip, tmp_ref, sch):
    idx, nxt = sch.idx("src"), sch.idx("nxt")
    low = lambda x, y: (x & 65535) | (y << 16)
    high = lambda x, y: jax.lax.shift_right_logical(x, 16) | (y & -65536)
    kv, up = {}, {}
    for i, k in enumerate(FINE):
        v = [g[8 * i:8 * i + 8] for g in groups]
        if k == 0:
            v = [x + jnp.where(sch.mask("diag"),
                               _gather(dskip[n // 2], sch.idx("dup%d" % (n % 2)), 0), 0.0)
                 for n, x in enumerate(v)]
        p = [_pack(tmp_ref, 2 * i + h, v[2 * h], v[2 * h + 1]) for h in range(2)]
        both = [_gather(x, idx) for x in p]
        kv[k], kv[k + 8] = low(*both), high(*both)
        if k % 512 == 0:
            up[k] = low(*[_gather(x, nxt) for x in p])
    k_last = _gather(k_last, sch.idx("rows"), 0)
    q0, q1, q2, up0, up01, up2, up3, fine = map(sch.mask, INDEX[-8:])
    s3 = {r: jnp.where(q2, kv[1024 + r], kv[1536 + r]) for r in (0, 8)}
    v0 = jnp.where(q0, kv[0], jnp.where(q1, kv[512], s3[0]))
    v16 = jnp.where(up01, jnp.where(up0, up[0], up[512]),
                    jnp.where(up2, up[1024], jnp.where(up3, up[1536], k_last)))
    s3[16] = v16
    s23, s123, out = {}, {}, [v0]
    for r in range(1, 16):
        k23 = (RES2[r], RES3[r])
        if k23 not in s23:
            s23[k23] = v16 if k23 == (16, 16) else jnp.where(q1, kv[512 + k23[0]], s3[k23[1]])
        k123 = (RES1[r],) + k23
        if k123 not in s123:
            s123[k123] = v16 if k123[0] == 16 else jnp.where(q0, kv[k123[0]], s23[k23])
        if RES1[r] == r:
            out.append(s123[k123])
        else:
            out.append(jnp.where(fine, kv[r], s123[k123]))
    return out


def _ln_scalars(s1, s2):
    mean = s1 * (1.0 / D)
    var = jnp.maximum(s2 * (1.0 / D) - mean * mean, 0.0)
    eps = float(np.asarray(EPS, dtype=BF16))
    sd = _rbf(jnp.sqrt(_rbf(_rbf(var) + eps)))
    return _rbf(mean), sd


def _top8(x):
    def swap(v, pairs):
        for i, j in pairs:
            v[i], v[j] = jnp.maximum(v[i], v[j]), jnp.minimum(v[i], v[j])
        return v

    def merge(a, b):
        v = [jnp.maximum(a[i], b[7 - i]) for i in range(8)]
        return swap(v, [(i, i + d) for d in (4, 2, 1) for i in range(8) if not i & d])

    sort8 = ((0, 2), (1, 3), (4, 6), (5, 7), (0, 4), (1, 5), (2, 6), (3, 7), (0, 1), (2, 3),
             (4, 5), (6, 7), (2, 4), (3, 5), (1, 4), (3, 6), (1, 2), (3, 4), (5, 6))
    v = merge(*[swap(x[i:i + 8], sort8) for i in (0, 8)])
    for d in (4, 2, 1):
        v = merge(v, [pltpu.roll(t, d, 0) for t in v])
    return v


def _init_columns(col_ref, wx_ref, wy_ref, ldt_ref, dsk_ref, wr_ref):
    row, lane = _iota((128, 128), 0), _iota((128, 128), 1)
    split = (row & ~15) + 2 * (row & 7) + ((row >> 3) & 1)
    ldt, dsk, wr = (ref[...].astype(F32).reshape(1, D) for ref in (ldt_ref, dsk_ref, wr_ref))
    for n, vec in enumerate((jnp.exp(ldt), dsk * (1.0 / L))):
        for lo in range(0, D, 128):
            i = min(lo, D - 128)
            diag = jnp.where(split == lane, vec[:, i:i + 128], 0.0)[lo - i:].astype(BF16)
            col_ref[n, lo:i + 128, :] = jnp.dot(diag, jnp.ones((128, 128), BF16),
                                                preferred_element_type=F32)
    diag = jnp.where(row == lane, wr[:, D - 128:], 0.0)[128 - MB:].astype(BF16)
    col_ref[2, 0:MB, :] = jnp.dot(diag, jnp.ones((128, 128), BF16), preferred_element_type=F32)
    sub = _iota((16, D), 0)
    ones_w = jnp.where(sub == 0, 1.0, jnp.where(sub == 1, wr, 0.0))
    wx_ref[...] = ones_w.astype(BF16)
    for lo in range(0, D, MB):
        wy_ref[lo // MB, :, 0:MB] = ones_w[:, lo:lo + MB].astype(BF16)
        wy_ref[lo // MB, :, MB:] = jnp.zeros((16, 128 - MB), BF16)


INDEX = ("true", "bit0", "bit1", "bit2", "bit3", "odd", "dup0", "dup1", "rows", "src", "nxt",
         "diag", "q0", "q1", "q2", "up0", "up01", "up2", "up3", "fine")


def _init_index(idx_ref):
    sub, lane = _iota((8, 128), 0), _iota((8, 128), 1)
    src = lambda b: 8 * ((b >> 1) & 15) + 2 * (sub & 3) + (b & 1)
    is_ = lambda m: jnp.where(m, 1, 0)
    q = lane & 3
    q16 = q + is_(lane >= 124)
    tiles = dict(true=sub + 1, odd=sub & 1, dup0=sub >> 1, dup1=4 + (sub >> 1),
                 rows=2 * (sub & 3) + (sub >> 2), src=src(lane >> 2), nxt=src((lane >> 2) + 1),
                 diag=is_((lane == sub) & ((sub & 1) == 0)), up01=is_(q16 < 2),
                 fine=is_((q == 0) & (lane < 64)),
                 **{"bit%d" % n: (lane >> n) & 1 for n in range(4)},
                 **{"q%d" % n: is_(q == n) for n in range(3)},
                 **{"up%d" % n: is_(q16 == n) for n in (0, 2, 3)})
    for n, name in enumerate(INDEX):
        idx_ref[n] = tiles[name]


class _Schedule:
    def __init__(self, zero, idx_ref):
        self.zero = zero
        self.idx = lambda name: idx_ref[INDEX.index(name) + zero]
        self.mask = lambda name: self.idx(name) != 0
        self.true = self.mask("true")
        self.done, self.pending, self.wait = [], {}, -1

    def tie(self, x, token):
        return jnp.where(self.true, x, token if token.dtype == x.dtype
                         else pltpu.bitcast(token, x.dtype))

    def start(self, x):
        return self.tie(x, self.done[self.wait]) if 0 <= self.wait < len(self.done) else x

    def lhs(self, words, first):
        tiles = [words[i:i + 8] for i in range(0, words.shape[0], 8)]
        for i in range(len(tiles) if first else 0):
            for token in self.pending.pop(len(self.done) + i, ()):
                tiles[i] = self.tie(tiles[i], token)
        return _mxu(jnp.concatenate(tiles, axis=0))

    def results(self, v):
        self.done += [v[i + 8:i + 16] for i in range(0, v.shape[0], 16)]

    def run(self, stage, wait, before):
        self.wait = wait
        self.pending.setdefault(before, []).extend(next(stage))


def _kernel(x_hbm, are_hbm, aim_hbm, bre_hbm, bim_hbm, cre_hbm, cim_hbm,
            ldt_hbm, dsk_hbm, wr_hbm, wg_hbm, wu_hbm, wd_hbm, out_hbm,
            x_v, wg_v, wu_v, wd_v, par_v, ldt_v, dsk_v, wr_v, w_v, wk_v, wt_v, col_v, wx_v, wy_v,
            tmp_v, idx_v, pk_v, h_v, st_v, acc_v, sq_v, out_v, sd0, sd1, ta0, ta1, tb0, tb1,
            kl0, kl1,
            u0, u1, k0, k1, a0_v, a1_v, c0, c1, r0, r1, r2, r3,
            sem_p, sem_x, sem_w, sem_o, f0_v, f1_v, *rest):
    half_v, new_v = rest[:4], rest[4:]
    cp_vec = [pltpu.make_async_copy(s, d, sem_p.at[n]) for n, (s, d) in enumerate(
        ((ldt_hbm, ldt_v), (dsk_hbm, dsk_v), (wr_hbm, wr_v)))]
    cp_par = [[pltpu.make_async_copy(s.at[lo:hi], par_v.at[n, lo:hi], sem_p.at[3 + 6 * m + n])
               for n, s in enumerate((are_hbm, aim_hbm, bre_hbm, bim_hbm, cre_hbm, cim_hbm))]
              for m, (lo, hi) in enumerate(((0, 4 * MB), (4 * MB, D)))]
    cp_x = [pltpu.make_async_copy(x_hbm.at[:, 128 * j:128 * j + 128], x_v.at[j, 0:D],
                                  sem_x.at[j])
            for j in range(NT)]
    cp_d = pltpu.make_async_copy(wd_hbm, wd_v, sem_w.at[2])

    def cp_w(i):
        return [pltpu.make_async_copy(s.at[:, _ds(128 * i, 128)], d.at[i, 0:D], sem_w.at[n])
                for n, (s, d) in enumerate(((wg_hbm, wg_v), (wu_hbm, wu_v)))]

    for cp in cp_vec + cp_par[0]:
        cp.start()
    for cp in cp_x[:NT // 2]:
        cp.start(priority=1)

    def columns():
        for cp in cp_vec:
            cp.wait()
        for cp in cp_x[NT // 2:]:
            cp.start(priority=1)
        _transpose_dft(wt_v, w_v, range(4))
        _init_columns(col_v, wx_v, wy_v, ldt_v, dsk_v, wr_v)

    _init_dft(w_v, wk_v, tmp_v, columns)
    for cp in cp_par[0]:
        cp.wait()

    sd, ta, tb, kl = (sd0, sd1), (ta0, ta1), (tb0, tb1), (kl0, kl1)
    uk, ab, cc, xr = ((u0, u1), (k0, k1)), ((a0_v, a1_v), (f0_v, f1_v)), (c0, c1), (r0, r1, r2, r3)
    ww, wt_w = (w_v.bitcast(I32), wk_v.bitcast(I32)), wt_v

    def seed_stage(b, r, sch):
        rows = _ds(b * MB // 2 + 8 * r, 8)
        par = [_split(par_v.bitcast(I32)[n, rows, :]) for n in range(6)]
        for h in range(2):
            a_re, a_im, b_re, b_im, c_re, c_im = [v[h] for v in par]
            dt = sch.start(col_v[0, _ds(b * MB + 16 * r + 8 * h, 8), :])
            mag, ang = jnp.exp(dt * a_re), dt * a_im
            sc = dt * (1.0 / L)
            seeds = _k_seeds((mag * jnp.cos(ang), mag * jnp.sin(ang)),
                             _cmul((c_re, c_im), (sc * b_re, sc * b_im)), sch)
            for g in range(2):
                for n, v in enumerate(seeds[g]):
                    for p in range(2):
                        sd[b % 2][r, 2 * h + g, 2 * n + p] = v[p]
            yield [sd[b % 2][(r + sch.zero), 2 * h, 0]]

    def table_stage(b, r, sch):
        tail = []
        for g in range(4):
            m1, m32, m512, a0, b0 = [
                (sd[b % 2][r, g, 2 * n], sd[b % 2][r, g, 2 * n + 1]) for n in range(5)]
            m32 = (sch.start(m32[0]), m32[1])
            fa = [a0]
            for _ in range(7):
                fa.append(_cmul(fa[-1], m1))
            for src in (0, 4, 8, 10):
                fa.append(_cmul(fa[src], m512))
            tail.append(fa[11][0] * m512[0] - fa[11][1] * m512[1])
            _store_table(ta[b % 2].at[r, g], fa)
            fb = [b0]
            for _ in range(15):
                p = fb[-1]
                fb.append((p[0] * m32[0] + p[1] * m32[1], p[1] * m32[0] - p[0] * m32[1]))
            _store_table(tb[b % 2].at[r, g], fb)
            yield [ta[b % 2].bitcast(I32)[(r + sch.zero), g, 0, 0:8, :],
                   tb[b % 2].bitcast(I32)[(r + sch.zero), g, 0, 0:8, :]]
        last = [jnp.where(sch.mask("odd"), pltpu.roll(tail[h + 1], 1, 0), tail[h])
                for h in (0, 2)]
        last = [pltpu.bitcast(_rbf(jnp.broadcast_to(jnp.sum(v, axis=1, keepdims=True),
                                                    (8, 128))), I32) for v in last]
        kl[b % 2][r] = jax.lax.shift_right_logical(last[0], 16) | last[1]

    def kernel_stage(b, r, sch):
        ta_w, tb_w = ta[b % 2].bitcast(I32), tb[b % 2].bitcast(I32)
        groups = [None] * 4
        for g0 in (0, 2):
            res = [jax.lax.dot_general(sch.lhs(ta_w[r, g, p, 0:48], g == g0 and p == 0),
                                       _mxu(tb_w[r, g, p, 0:64]), NT_DIMS, preferred_element_type=F32)
                   for g in (g0, g0 + 1) for p in range(2)]
            groups[g0], groups[g0 + 1] = res[0] + res[1], res[2] + res[3]
            sch.results(groups[g0 + 1])
            yield []
        dskip = [col_v[1, _ds(b * MB + 16 * r + 8 * h, 8), :] for h in range(2)]
        dst = _ds(8 * r, 8)
        res = _k_residues(groups, kl[b % 2][r], dskip, pk_v.at[sch.slot, 0], sch)
        for s, t in enumerate(res):
            uk[1][b % 2][4 * (s % 4) + s // 4, dst, :] = t
        yield [uk[1][b % 2][0, _ds(8 * (r + sch.zero), 8), :]]

    def norm_stage(b, r, sch):
        rows, dst = _ds(b * MB // 2 + 8 * r, 8), _ds(8 * r, 8)
        tiles = [x_v.bitcast(I32)[j, rows, :] for j in range(NT)]
        for s, t in enumerate(_to_residues([sch.start(tiles[0])] + tiles[1:], sch)):
            xr[b % 4][4 * (s % 4) + s // 4, dst, :] = t
            xs, m, inv = _mxu(t).astype(F32), st_v[s, 0], st_v[s, 1]
            uk[0][b % 2][4 * (s % 4) + s // 4, _ds(16 * r, 16), :] = jnp.concatenate(
                [(xs[0:8] - m) * inv, (xs[8:16] - m) * inv], axis=0).astype(BF16)
        yield [uk[0][b % 2].bitcast(I32)[0, _ds(8 * (r + sch.zero), 8), :]]

    def forward_stage(w, b, k, sch):
        dst = ab[w][b % len(ab[w])]
        for p in range(2):
            v = [jnp.dot(sch.lhs((uk[w][b % 2] if w else uk[w][b % 2].bitcast(I32))[
                4 * k + n, 0:MB // 2], n == 0),
                         _mxu(ww[w][p ^ (n & 1), 4 * k + n, 0:64]),
                         preferred_element_type=F32) for n in range(4)]
            d02, d13 = v[0] - v[2], v[1] - v[3]
            x1 = d02 - d13 if p == 0 else d02 + d13
            dst[0, k, p, 0:MB] = v[0] + v[2]
            dst[2, k, 1 - p, 0:MB] = v[1] + v[3]
            dst[1, k, p, 0:MB] = x1
            dst[3, k, p, 0:MB] = d02 + d13 if p == 0 else d02 - d13
            sch.results(x1)
            yield []

    def stats(tiles, sch):
        ones_w = wx_v.bitcast(I32)[...]
        for j in tiles:
            acc = None
            for i in range(0, D // 2, 8):
                v = [t * t for t in _split(x_v.bitcast(I32)[j, i:i + 8, :])]
                acc = v if acc is None else [p + q for p, q in zip(acc, v)]
            sums = jnp.dot(_mxu(jnp.concatenate(
                [ones_w[:, :128] if j % 2 == 0 else sch.tie(ones_w[:, :128], prev),
                 ones_w[:, 128:]], axis=1)),
                           _mxu(x_v.bitcast(I32)[j, 0:D // 2]), preferred_element_type=F32)
            s2 = prev = acc[0] + acc[1]
            for d in (4, 2, 1):
                s2 = s2 + pltpu.roll(s2, d, 0)
            mean, sd = _ln_scalars(jnp.broadcast_to(sums[0:1], (8, 128)), s2)
            st_v[j, 0], st_v[j, 1] = mean, 1.0 / sd

    def middle_stage(b, r, sch):
        src = [v[b % len(v)] for v in ab]
        scale = lambda v, f: [(x[0] * f, x[1] * f) for x in v]
        for h in range(2):
            ra = _ds(16 * r + 8 * h, 8)
            ld = lambda q, w, ra=ra: [(src[w][q, k, 0, ra, :], src[w][q, k, 1, ra, :]) for k in range(4)]

            park_v = half_v[2 * (sch.slot % 2) + h]

            def put(q, y):
                x = [park_v[n + sch.zero] for n in range(8)]
                for k in range(4):
                    for p in range(2):
                        cc[b % 2][k, q, p, ra, :] = x[2 * k + p] + y[k][p]
                        cc[b % 2][k, q + 2, p, ra, :] = x[2 * k + p] - y[k][p]

            def park(x):
                for k in range(4):
                    for p in range(2):
                        park_v[2 * k + p] = x[k][p]
                return [park_v[sch.zero]]

            gate = sch.start
            a0, a2, b0, b2 = ld(0, 0), ld(2, 0), ld(0, 1), ld(2, 1)
            a0[0] = (gate(a0[0][0]), a0[0][1])
            e0 = _prod_mod_1(list(map(_cadd, a0, a2)), list(map(_cadd, b0, b2)))
            again = _ds(16 * (r + sch.zero) + 8 * h, 8)
            yield park(e0)
            a0, a2, b0, b2 = (ld(q, w, again) for w in range(2) for q in (0, 2))
            a2[0] = (gate(a2[0][0]), a2[0][1])
            e2 = _prod_mod_m1(list(map(_csub, a0, a2)), scale(map(_csub, b0, b2), 2.0))
            put(0, e2)
            yield [cc[b % 2][0, 0, 0, again, :]]
            four = sch.start(jnp.full((8, 128), 4.0, F32))
            e1 = _prod_mod_i(ld(1, 0), scale(ld(1, 1), four), 1)
            yield park(e1)
            four = sch.start(jnp.full((8, 128), 4.0, F32))
            e3 = _prod_mod_i(ld(3, 0), scale(ld(3, 1), four), -1)
            put(1, e3)
            yield [cc[b % 2][0, 1, 0, again, :]]

    def inverse_stage(b, k, sch):
        src = cc[b % 2]

        def lhs(v, n, first):
            return sch.lhs(jnp.concatenate(
                [_pack(pk_v.at[sch.slot, 2], 4 * n + i // 16, v[i:i + 8], v[i + 8:i + 16])
                 for i in range(0, MB, 16)], axis=0), first)

        for o in range(2):
            p0, p1 = [(src[k, q, 0, 0:MB], src[k, q, 1, 0:MB]) for q in (2 * o, 2 * o + 1)]
            if o == 0:
                e = {0: _cadd(p0, p1), 2: _csub(p0, p1)}
            else:
                e = {1: (p0[0] + p1[1], p0[1] - p1[0]), 3: (p0[0] - p1[1], p0[1] + p1[0])}
            ys = []
            for n in e:
                y = [jnp.dot(lhs(e[n][p], 2 * n + p, n == o and p == 0),
                             _mxu(wt_w[4 * k + (0, 2, 1, 3)[n], p, 0:64]),
                             preferred_element_type=F32)
                     for p in range(2)]
                h = y[0] + y[1] + _mxu(xr[b % 4][4 * k + n, 0:MB // 2]).astype(F32)
                h_v[k + 4 * n, b * MB:b * MB + MB, :] = h.astype(BF16)
                hh = h * h
                sq_v[k + 4 * n] += sum((hh[i:i + 8] for i in range(8, MB, 8)), hh[0:8])
                ys.append(h)
                if b == nb - 1:
                    sums = []
                    for v in (h, h * col_v[2, 0:MB, :]):
                        v = sum((v[i:i + 8] for i in range(8, MB, 8)), v[0:8])
                        for d in (4, 2, 1):
                            v = v + pltpu.roll(v, d, 0)
                        sums.append(v)
                    acc_v[k + 4 * n] += jnp.where(sch.mask("odd"), sums[1], sums[0])
            sch.results(ys[-1])
            yield []

    def sum_stage(b, r, sch):
        for n in range(4):
            s = 4 * r + n
            sums = jnp.dot(sch.lhs(wy_v.bitcast(I32)[b], n == 0)[:, :MB],
                           _mxu(h_v.bitcast(I32)[s, b * MB // 2:(b + 1) * MB // 2]),
                           preferred_element_type=F32)
            acc_v[s] += sums[0:8]
        sch.results(sums)
        yield []

    nb = D // MB
    stages = dict(
        s=(seed_stage, 0), t=(table_stage, 1), k=(kernel_stage, 2),
        F=(functools.partial(forward_stage, 1), 3), n=(norm_stage, 2),
        f=(functools.partial(forward_stage, 0), 3), m=(middle_stage, 4),
        i=(inverse_stage, 5), a=(sum_stage, 6))

    def run(step, zero, live=None):
        live = live or {n: (f, step - lag) for n, (f, lag) in stages.items()
                        if 0 <= step - lag < nb and (n, step) != ("n", 2)}
        unroll, plan = PLANS["".join(live)]

        def body(it, carry):
            sch = _Schedule(zero >> (step % 32) if unroll == 4 else zero & it, idx_v)
            gens = [{n: f(b, it * unroll + u, sch) for n, (f, b) in live.items()}
                    for u in range(unroll)]
            if step == 3:
                for i in range(9 * unroll):
                    for cp in cp_w(9 * unroll * it + i):
                        cp.start()
            for item in plan.split():
                u, n, *ties = item.split(":")
                if n in live:
                    sch.slot = int(u)
                    sch.run(gens[int(u)][n], *map(int, ties or (-1, -1)))
            for sch.slot, g in enumerate(gens):
                for v in g.values():
                    for _ in v:
                        pass
            return carry + it

        if unroll == 4:
            if step == 101 or step > nb + 3:
                return body(0, 0)
            return jax.lax.fori_loop(zero, 1, lambda _, c: body(0, c), 0)
        return jax.lax.fori_loop(0, 4 // unroll, body, 0)

    _init_index(idx_v)
    acc_v[...] = sq_v[...] = jnp.zeros(acc_v.shape, F32)
    zero = run(0, 0) - 1
    for step in range(1, nb + 5):
        if step == 4:
            for cp in cp_par[1]:
                cp.wait()
        if step == 3:
            for half in range(2):
                tiles = range(NT // 2 * half, NT // 2 * (half + 1))
                for j in tiles:
                    cp_x[j].wait()
                if half:
                    cp_d.start(priority=1)
                else:
                    for cp in cp_par[1]:
                        cp.start()
                _transpose_dft(wt_v, w_v, range(4 + 6 * half, 10 + 6 * half))
                stats(tiles, _Schedule(zero, idx_v))
            for q in range(2):
                for s, v in enumerate(_to_residues([st_v[j, q] for j in range(NT)],
                                                   _Schedule(zero, idx_v))):
                    st_v[s, q] = v
            run(101, zero, dict(n=(norm_stage, 0)))
        run(step, zero)

    sums = [acc_v[s] for s in range(16)]
    m2, sd2 = _ln_scalars(
        jnp.concatenate([v[0:1] for v in sums], axis=0),
        jnp.concatenate([jnp.sum(sq_v[j], axis=0, keepdims=True) for j in range(NT)], axis=0))
    inv2 = 1.0 / sd2
    wsum = jnp.sum(wr_v[...].astype(F32).reshape(1, D), axis=1, keepdims=True)
    score = _rbf((jnp.concatenate([v[1:2] for v in sums], axis=0) - m2 * wsum) * inv2 + 0.0)
    sub16 = _iota((16, 128), 0)
    for s in range(16):
        h_v[s, D:, :] = jnp.where(sub16 == 0, m2[s:s + 1], jnp.where(
            sub16 == 1, sd2[s:s + 1], score[s:s + 1])).astype(BF16)
    bits = pltpu.bitcast(score, I32) >> 16
    order = jnp.where(bits < 0, -1 - bits, bits + 32768)
    mu = (_iota((NT, 128), 1) - _iota((NT, 128), 0)) & 127
    pos = 128 * (mu & 15) + 16 * (mu >> 4) + _iota((NT, 128), 0)
    key = pltpu.bitcast((order << 11) + (L - 1 - pos) + (1 << 29), F32)

    h_w, out_w = h_v.bitcast(I32), out_v.bitcast(I32)
    sch, done = _Schedule(zero, idx_v), []
    tie = sch.tie

    def unrouted():
        for q, v in enumerate((1.0 + inv2, m2 * inv2)):
            for j, t in enumerate(_to_time(
                    [jnp.broadcast_to(v[s:s + 1], (8, 128)) for s in range(16)], sch)):
                st_v[j, q] = t
        for i in range(0, D, 16):
            scal = st_v.at[pl.ds(zero * (i + 1), NT)]
            tiles = [h_w[s, i // 2:i // 2 + 8, :] for s in range(16)]
            if len(done) > LAG:
                tiles[0] = tie(tiles[0], done[-LAG])
            for j, v in enumerate(_to_time(tiles, sch)):
                h, mul, sub = _mxu(v).astype(F32), scal[j, 0], scal[j, 1]
                out_v[j, i:i + 16, :] = jnp.concatenate(
                    [h[0:8] * mul - sub, h[8:16] * mul - sub], axis=0).astype(BF16)
                if j % 8 == 7:
                    yield pltpu.bitcast(out_w[j + zero, i // 2:i // 2 + 8, :], F32)

    side = unrouted()

    lane8, sub8 = _iota((CAP, 128), 1), _iota((CAP, 128), 0)
    best = _top8([pltpu.roll(key[i:i + 8], n, 1) if n else key[i:i + 8]
                  for i in (0, 8) for n in range(8)])
    cand = best[0]
    for c in range(1, CAP):
        cand = jnp.where(sub8 == c, best[c], cand)
    best = _top8([pltpu.roll(cand, n, 1) if n else cand for n in range(0, 128, 8)])
    for _ in range(2 * EARLY):
        best[-1] = tie(best[-1], next(side))
    best = [pltpu.bitcast(v, I32)[0, 0] for v in best]
    picks = [L - 1 - (v & (L - 1)) for v in best]

    def schedule(col):
        rnd = [sum([(col[e] == col[c]).astype(I32) for e in range(c)], 0) for c in range(CAP)]
        return (rnd, functools.reduce(jnp.maximum, rnd) + 1,
                lambda n: [lane8 == jnp.where(rnd[c] == n, col[c], -1) for c in range(CAP)])

    _, rounds, lanes = schedule([((t >> 7) + (t & 127)) & 127 for t in picks])

    def out_copy(q, lo, hi):
        j = order[q]
        return pltpu.make_async_copy(
            out_v.at[j, lo:hi], out_hbm.at[lo:hi, _ds(j * 128, 128)], sem_o)

    for n, ref in enumerate((wg_v, wu_v)):
        pltpu.make_async_copy(ref.at[:, 0:D], ref.at[:, 0:D], sem_w.at[n]).wait()

    def gather(n, acc):
        masks = lanes(n)
        tiles = []
        for i in range(0, D // 2 + 8, 8):
            v = jnp.zeros((8, 128), I32)
            for c in range(CAP):
                v = jnp.where(masks[c], h_w[picks[c] & 15, i:i + 8, :], v)
            tiles.append(v)
        lhs = jnp.zeros((CAP, 128), F32)
        for c in range(CAP):
            lhs = jnp.where(masks[c] & (sub8 == c), 1.0, lhs)
        return acc + jax.lax.dot_general(lhs.astype(BF16), _mxu(jnp.concatenate(tiles, axis=0)),
                                         NT_DIMS, preferred_element_type=F32)

    h_sel = jax.lax.fori_loop(0, rounds, gather, jnp.zeros((CAP, D + 16), F32))
    m_sel, sd_sel, score_sel = (h_sel[:, D + q:D + q + 1] for q in range(3))
    h_sel = h_sel[:, :D]
    x_sel = _rbf(_rbf(h_sel - m_sel) / sd_sel)
    gate = _rbf(jax.nn.sigmoid(score_sel))

    tile, col = [t >> 7 for t in picks], [t & 127 for t in picks]
    rnd, rounds, lanes = schedule(col)
    late, again = 0, []
    for j in tile:
        again.append((late >> j) & 1)
        late = late | (1 << j)
    for dup in again[1:]:
        late = late | (late + dup)
    order = []
    for left in (late ^ ((1 << NT) - 1), late):
        for _ in range(CAP):
            order.append((31 - jax.lax.clz(left)) & (NT - 1))
            left = left ^ (1 << order[-1])

    def early_copies(n):
        lo, hi = (0, 16 * EARLY, *STOPS, MID, D)[n:n + 2]
        return [out_copy(q, lo, hi) for q in range(CAP)]

    def start(copies):
        for cp in copies:
            cp.start()

    start(early_copies(0))
    rate, sent = MID // 8 - 2 * EARLY, [0]

    def project(w_ref):
        parts = []
        for n in range(0, FF // 128, 4):
            for lo in range(0, D, 128):
                hi = min(lo + 128, D)
                xs = x_sel[:, lo:hi]
                if hi - lo == 128 and min(rate, (len(done) - 4) * rate // END) > sent[0]:
                    sent[0] += 1
                    xs = tie(xs, next(side))
                    if 16 * EARLY + 8 * sent[0] in STOPS:
                        start(early_copies(1 + STOPS.index(16 * EARLY + 8 * sent[0])))
                w = [w_ref.bitcast(I32)[i, lo // 2:hi // 2, :] for i in range(n, n + 4)]
                v = jnp.dot(xs.astype(BF16), _mxu(jnp.concatenate(w, axis=1)),
                            preferred_element_type=F32)
                done.append(v[:, 0:128])
                acc = acc + v if lo else v
            parts.append(acc)
        return _rbf(jnp.concatenate(parts, axis=1))

    g = project(wg_v)
    act = _rbf(g * jax.nn.sigmoid(g)) * project(wu_v)
    for _ in range(rate - sent[0]):
        next(side)
    done.clear()

    cp_d.wait()

    start(early_copies(len(STOPS) + 1))
    rest_side = list(side)

    def placed(r, words):
        idx = jnp.zeros((CAP, 128), I32)
        for c, m in enumerate(lanes(r)):
            idx = jnp.where(m, c, idx)
        return [_gather(w, idx) for w in words]

    def late_copies(lo, hi):
        return [out_copy(CAP + q, lo, hi) for q in range(CAP)]

    def words_of(n):
        return [new_v[n].bitcast(I32)[i:i + 8, :] for i in range(0, new_v[n].shape[0] // 2, 8)]

    tokens = []
    for n, (lo, hi) in enumerate(ROW_CHUNKS):
        a = [act[:, i:i + 128] for i in range(0, FF, 128)]
        for i, token in enumerate(rest_side):
            at = 8 + i * SPAN // len(rest_side) - n * len(a)
            if 0 <= at < len(a):
                a[at] = tie(a[at], token)
        if n == 1:
            start(early_copies(len(STOPS) + 2))
        if n >= 2:
            cut = CUT * 128 // (hi - lo)
            a[cut] = tie(a[cut], tokens[n - 2])
        a = jnp.concatenate(a, axis=1)
        y = _rbf(jax.lax.dot_general(a.astype(BF16), wd_v[lo:hi, :], NT_DIMS,
                                     preferred_element_type=F32))
        new = h_sel[:, lo:hi] + _rbf(x_sel[:, lo:hi] + _rbf(y * gate))
        new_v[n][...] = jnp.concatenate(
            [new.T, jnp.zeros((hi - lo, 128 - CAP), F32)], axis=1).astype(BF16)
        rows = range(lo // 2, hi // 2, 8)
        words = words_of(n)
        both = list(zip(rows, placed(0, words), placed(1, words)))
        for c in range(CAP):
            for i, v0, v1 in both:
                pltpu.store(out_w.at[tile[c], pl.ds(i, 8), :],
                            jnp.where(rnd[c] == 0, v0, v1), mask=lane8 == col[c])
        for cp in late_copies(lo, hi):
            cp.start()
        out_w[tile[0], D // 2:, :] = lane8
        tokens.append(pltpu.bitcast(out_w[tile[0] | zero, D // 2:, :], F32))
    pltpu.make_async_copy(out_v.at[:, 0:D], out_v.at[:, 0:D], sem_o).wait()

    @pl.when(rounds > 2)
    def _():
        def fix(r, carry):
            rows = range(0, D // 2, 8)
            vals = placed(r, sum(map(words_of, range(len(new_v))), []))
            for c, m in enumerate(lanes(r)):
                for i, v in zip(rows, vals):
                    pltpu.store(out_w.at[tile[c], pl.ds(i, 8), :], v, mask=m)
            return carry

        jax.lax.fori_loop(2, rounds, fix, 0)
        for cp in late_copies(0, D):
            cp.start()
        for cp in late_copies(0, D):
            cp.wait()


@jax.jit
def pallas_sequential_preLN__ssm_conv_s4__moe_arch_mod__prompt_kernel(
    A_u: jax.Array,
    A_A_re: jax.Array,
    A_A_im: jax.Array,
    A_B_re: jax.Array,
    A_B_im: jax.Array,
    A_C_re: jax.Array,
    A_C_im: jax.Array,
    A_log_dt: jax.Array,
    A_Dskip: jax.Array,
    B_x: jax.Array,
    B_w_r: jax.Array,
    B_w_gate: jax.Array,
    B_w_up: jax.Array,
    B_w_down: jax.Array,
):
    del B_x
    hbm = pl.BlockSpec(memory_space=pl.ANY)
    out = pl.pallas_call(
        _kernel,
        out_shape=jax.ShapeDtypeStruct((D, L), BF16),
        in_specs=[hbm] * 13,
        out_specs=hbm,
        scratch_shapes=[
            pltpu.VMEM((NT, D + 16, 128), BF16),
            *[pltpu.VMEM((FF // 128, D + 16, 128), BF16)] * 2,
            pltpu.VMEM((D, FF), BF16),
            pltpu.VMEM((6, D, N), BF16),
            *[pltpu.VMEM((D,), BF16)] * 3,
            *[pltpu.VMEM((2, 16, 144, 128), BF16)] * 2,
            pltpu.VMEM((16, 2, 72, 128), I32),
            pltpu.VMEM((3, D, 128), F32),
            pltpu.VMEM((16, D), BF16),
            pltpu.VMEM((D // MB, 16, 128), BF16),
            pltpu.VMEM((2, 256, 128), F32),
            pltpu.VMEM((len(INDEX), 8, 128), I32),
            pltpu.VMEM((4, 3, 32, 16, 128), BF16),
            pltpu.VMEM((NT, D + 16, 128), BF16),
            pltpu.VMEM((NT, 2, 8, 128), F32),
            *[pltpu.VMEM((NT, 8, 128), F32)] * 2,
            pltpu.VMEM((NT, D + 16, 128), BF16),
            *[pltpu.VMEM((4, 4, 10, 8, 128), F32)] * 2,
            *[pltpu.VMEM((4, 4, 2, 112, 128), BF16)] * 2,
            *[pltpu.VMEM((4, 4, 2, 144, 128), BF16)] * 2,
            *[pltpu.VMEM((4, 8, 128), I32)] * 2,
            *[pltpu.VMEM((16, MB + 16, 128), BF16)] * 2,
            *[pltpu.VMEM((16, MB // 2 + 8, 128), I32)] * 2,
            *[pltpu.VMEM((4, 4, 2, MB + 8, 128), F32)] * 2,
            *[pltpu.VMEM((4, 4, 2, MB + 8, 128), F32)] * 2,
            *[pltpu.VMEM((16, MB // 2 + 8, 128), I32)] * 4,
            pltpu.SemaphoreType.DMA((15,)),
            pltpu.SemaphoreType.DMA((NT,)),
            pltpu.SemaphoreType.DMA((3,)),
            pltpu.SemaphoreType.DMA,
            *[pltpu.VMEM((4, 4, 2, MB + 8, 128), F32)] * 2,
            *[pltpu.VMEM((8, 8, 128), F32)] * 4,
            *[pltpu.VMEM((hi - lo, 128), BF16) for lo, hi in ROW_CHUNKS],
        ],
        compiler_params=pltpu.CompilerParams(vmem_limit_bytes=100 * 1024 * 1024,
                                             disable_bounds_checks=True,
                                             disable_semaphore_checks=True),
    )(A_u.reshape(L, D).T, A_A_re, A_A_im, A_B_re, A_B_im, A_C_re, A_C_im,
      A_log_dt, A_Dskip, B_w_r, B_w_gate, B_w_up, B_w_down.T)
    return out.T.reshape(1, L, D)
```
